```python
import jax
import jax.numpy as jnp

def _softmax(x, axis=-1):
    return jax.nn.softmax(x, axis=axis)
def _gelu(x):
    return jax.nn.gelu(x, approximate=True)
def _silu(x):
    return jax.nn.silu(x)
def _sigmoid(x):
    return jax.nn.sigmoid(x)
def _layernorm(x, axis=-1, eps=1e-5):
    m = jnp.mean(x, axis=axis, keepdims=True)
    v = jnp.var(x, axis=axis, keepdims=True)
    return (x - m) / jnp.sqrt(v + eps)
def _scatter_add(tgt, idx, src, axis=0):
    return tgt.at[idx].add(src)
def _segment_sum(src, seg, n):
    return jax.ops.segment_sum(src, seg, n)
class _Rng:
    def __init__(self, key):
        self._k = key
    def _next(self):
        self._k, sub = jax.random.split(self._k)
        return sub
    def normal(self, shape):
        return jax.random.normal(self._next(), shape, dtype=jnp.bfloat16)
    def randint(self, lo, hi, shape):
        return jax.random.randint(self._next(), shape, lo, hi, dtype=jnp.int32)
    def uniform(self, shape, lo=0.0, hi=1.0):
        return jax.random.uniform(self._next(), shape, jnp.bfloat16, lo, hi)
    def permutation(self, n):
        return jax.random.permutation(self._next(), n)


kernel_name = 'parallel_sum__sliding_local_dilated__mixer_token_mlp__prompt'

def setup_inputs():
    _rng = _Rng(jax.random.key(int.from_bytes(__import__("os").urandom(4), "little")))
    _w = (lambda a: (lambda t: t.astype(jnp.bfloat16) if jnp.issubdtype(t.dtype, jnp.floating) else t)(jnp.asarray(a)))
    def _A_setup():
        B, S, D = 1, 2048, 448
        return {
            "x": _w((lambda *s: _rng.normal(s) * 0.05)(B, S, D)),
            "wqkv": _w((lambda *s: _rng.normal(s) * 0.05)(D, 3 * D)),
            "wo": _w((lambda *s: _rng.normal(s) * 0.05)(D, D)),
        }
    _A_in = _A_setup()

    def _B_setup():
        B, S, D, F = 1, 2048, 448, 1792
        return {
            "x": _w((lambda *s: _rng.normal(s) * 0.05)(B, S, D)),
            "w1": _w((lambda *s: _rng.normal(s) * 0.05)(S, F) * (S ** -0.5)),
            "b1": _w((lambda *s: _rng.normal(s) * 0.05)(F) * 0.02),
            "w2": _w((lambda *s: _rng.normal(s) * 0.05)(F, S) * (F ** -0.5)),
            "b2": _w((lambda *s: _rng.normal(s) * 0.05)(S) * 0.02),
        }
    _B_in = _B_setup()

    return {
        "A_x": _A_in["x"],
        "A_wqkv": _A_in["wqkv"],
        "A_wo": _A_in["wo"],
        "B_x": _B_in["x"],
        "B_w1": _B_in["w1"],
        "B_b1": _B_in["b1"],
        "B_w2": _B_in["w2"],
        "B_b2": _B_in["b2"],
    }

def reference(A_x, A_wqkv, A_wo, B_x, B_w1, B_b1, B_w2, B_b2):
    def _A_ref(x, wqkv, wo):
        B, S, D = x.shape
        H = 16; Dh = D // H
        W, dil = 8, 2
        qkv = (lambda x, *d: x.transpose(*d))((x @ wqkv).reshape(B, S, 3, H, Dh), 2, 0, 3, 1, 4)
        q, k, v = qkv[0], qkv[1], qkv[2]
        scale = Dh ** -0.5
        pos = jnp.arange(S)
        off = jnp.arange(W) * dil
        idx = pos[:, None] - off[None, :]
        mask = idx >= 0
        idx_c = jnp.where(mask, idx, 0).reshape(-1)
        kg = k[:, :, idx_c, :].reshape(B, H, S, W, Dh)
        vg = v[:, :, idx_c, :].reshape(B, H, S, W, Dh)
        logits = jnp.einsum("bhsd,bhswd->bhsw", q, kg) * scale
        logits = jnp.where(mask[None, None, :, :], logits, -1e9)
        attn = _softmax(logits, axis=-1)
        o = jnp.einsum("bhsw,bhswd->bhsd", attn, vg)
        return (lambda x, *d: x.transpose(*d))(o, 0, 2, 1, 3).reshape(B, S, D) @ wo

    def _B_ref(x, w1, b1, w2, b2):
        B, S, D = x.shape
        h = _layernorm(x, axis=-1)
        u = jnp.einsum("bsd,sf->bdf", h, w1) + b1
        u = _gelu(u)
        y = jnp.einsum("bdf,fs->bds", u, w2) + b2
        return (lambda x, *d: x.transpose(*d))(y, 0, 2, 1)

    x = A_x
    xn = _layernorm(x, axis=-1)
    return x + _A_ref(xn, A_wqkv, A_wo) + _B_ref(xn, B_w1, B_b1, B_w2, B_b2)
```

```python
import functools
import jax
import jax.numpy as jnp
from jax import lax
import jax.experimental.pallas as pl
import jax.experimental.pallas.tpu as pltpu

S, D, F = 2048, 448, 1792
H, DH, W, DIL = 16, 28, 8, 2
LB = 128
NB = S // LB
T = 256
NC = S // T
BPC = T // LB
NFB = F // LB
EPS = 1e-5
SCALE = DH ** -0.5
f32 = jnp.float32
bf16 = jnp.bfloat16
u32 = jnp.uint32


def _gelu(x):
    c = 0.7978845608028654
    return 0.5 * x * (1.0 + jnp.tanh(c * (x + 0.044715 * (x * x * x))))


def _pk(x):
    return pltpu.bitcast(x.astype(bf16), u32)


def _up(x):
    return pltpu.bitcast(x, bf16)


def _kernel(x_hbm, wqkv_hbm, wo_hbm, w1_hbm, b1_hbm, w2_hbm, b2_hbm, out_hbm,
            x_v, wqkv_v, wo_v, w1_v, w2_v, b1_v, b2_v, out_v,
            wt_s, wp_s, wo_s, wo2_s, wot_s, xnT_s, hT_s, u_s, g_s, qkv_s, oT_s,
            sx, sw1, sw2, smisc, sout):
    def cp_x(i):
        return pltpu.make_async_copy(x_hbm.at[0, :, pl.ds(i * T, T)], x_v.at[:, pl.ds(i * T, T)], sx.at[i])

    def cp_w1(i):
        return pltpu.make_async_copy(w1_hbm.at[pl.ds(i * T, T), :], w1_v.at[pl.ds(i * T, T), :], sw1.at[i])

    cp_w2 = pltpu.make_async_copy(w2_hbm, w2_v, sw2.at[0])

    def cp_out(i):
        return pltpu.make_async_copy(out_v.at[:, pl.ds(i * T, T)], out_hbm.at[0, :, pl.ds(i * T, T)], sout.at[i])

    cp_wqkv = pltpu.make_async_copy(wqkv_hbm, wqkv_v, smisc.at[0])
    cp_wo = pltpu.make_async_copy(wo_hbm, wo_v, smisc.at[1])
    cp_b1 = pltpu.make_async_copy(b1_hbm, b1_v, smisc.at[2])
    cp_b2 = pltpu.make_async_copy(b2_hbm, b2_v, smisc.at[3])

    cp_x(0).start(); cp_w1(0).start()
    cp_x(1).start(); cp_w1(1).start()
    cp_x(2).start(); cp_w1(2).start()
    cp_x(3).start()
    cp_wqkv.start()
    cp_w1(3).start()

    qkv_s[0, D:3 * D, :] = jnp.zeros((2 * D, LB), f32)

    def prep_wqkv():
        wT = wqkv_v[...].astype(f32).T
        for c in range(4):
            cw = min(LB, D - c * LB)
            wt_s[c, :, 0:cw] = wT[:, c * LB:c * LB + cw]
        for p in range(3):
            for d in range(DH):
                r = (p * D + d * H) // 2
                for c in range(4):
                    cw = min(LB, D - c * LB)
                    t = wt_s[c, pl.ds(p * D + d, H, stride=DH), :]
                    wp_s[r:r + H // 2, c * LB:c * LB + cw] = _pk(t)[:, 0:cw]

    def prep_wo():
        wo = wo_v[...].astype(f32)
        for c in range(4):
            cw = min(LB, D - c * LB)
            wo_s[c, :, 0:cw] = wo[:, c * LB:c * LB + cw]
        for d in range(DH):
            for c in range(4):
                cw = min(LB, D - c * LB)
                t = wo_s[c, pl.ds(d, H, stride=DH), :]
                wo2_s[d * H:(d + 1) * H, c * LB:c * LB + cw] = t[:, 0:cw]
        wot_s[...] = _pk(wo2_s[...].T)

    def ln_chunk(i):
        cols = slice(i * T, (i + 1) * T)
        xt = x_v[:, cols].astype(f32)
        mu = jnp.sum(xt, axis=0, keepdims=True) * (1.0 / D)
        xc = xt - mu
        var = jnp.sum(xc * xc, axis=0, keepdims=True) * (1.0 / D)
        xn = xc * lax.rsqrt(var + EPS)
        mu2 = jnp.sum(xn, axis=0, keepdims=True) * (1.0 / D)
        hc = xn - mu2
        var2 = jnp.sum(hc * hc, axis=0, keepdims=True) * (1.0 / D)
        h = hc * lax.rsqrt(var2 + EPS)
        xnT_s[:, cols] = _pk(xn)
        hT_s[:, cols] = _pk(h)

    def u_chunk(i0, i1, last=False):
        rows = slice(i0 * T, i1 * T)
        h = _up(hT_s[:, rows])
        if not last:
            r = jnp.dot(h, w1_v[rows, :], preferred_element_type=f32)
            if i0 == 0:
                u_s[...] = r
            else:
                u_s[...] += r
        else:
            for n in range(NFB):
                cs = slice(n * LB, (n + 1) * LB)
                r = jnp.dot(h, w1_v[rows, cs], preferred_element_type=f32)
                r = r + u_s[:, cs] + b1_v[n:n + 1, :].astype(f32)
                g_s[:, cs] = _pk(_gelu(r))

    def stage_a(i):
        r = jnp.dot(_up(wp_s[...]), _up(xnT_s[:, i * T:(i + 1) * T]), preferred_element_type=f32)
        for b in range(BPC):
            qkv_s[i * BPC + b + 1] = r[:, b * LB:(b + 1) * LB]

    lane = lax.broadcasted_iota(jnp.int32, (H, LB), 1)

    def shifted(cur, prev, w):
        if w == 0:
            return cur
        z = jnp.where(lane < LB - DIL * w, cur, prev)
        return pltpu.roll(z, DIL * w, 1)

    def stage_b(j):
        accs = [None] * W
        for d in range(DH):
            r = d * H
            q = qkv_s[j + 1, r:r + H, :]
            k = qkv_s[j + 1, D + r:D + r + H, :]
            kp = qkv_s[j, D + r:D + r + H, :]
            for w in range(W):
                t = q * shifted(k, kp, w)
                accs[w] = t if d == 0 else accs[w] + t
        lg = [a * SCALE for a in accs]
        if j == 0:
            lg = [lg[0]] + [jnp.where(lane >= DIL * w, lg[w], -1e9) for w in range(1, W)]
        m = lg[0]
        for w in range(1, W):
            m = jnp.maximum(m, lg[w])
        e = [jnp.exp(l - m) for l in lg]
        den = e[0]
        for w in range(1, W):
            den = den + e[w]
        inv = 1.0 / den
        p = [x * inv for x in e]
        for d in range(DH):
            r = d * H
            v = qkv_s[j + 1, 2 * D + r:2 * D + r + H, :]
            vp = qkv_s[j, 2 * D + r:2 * D + r + H, :]
            o = p[0] * v
            for w in range(1, W):
                o = o + p[w] * shifted(v, vp, w)
            oT_s[r // 2:(r + H) // 2, j * LB:(j + 1) * LB] = _pk(o)

    def stage_bb(i):
        for b in range(BPC):
            stage_b(i * BPC + b)

    def stage_c(i):
        cols = slice(i * T, (i + 1) * T)
        y = jnp.dot(_up(g_s[...]), w2_v[:, cols], preferred_element_type=f32)
        y = y + jnp.dot(_up(wot_s[...]), _up(oT_s[:, cols]), preferred_element_type=f32)
        b2 = jnp.concatenate([b2_v[i * BPC + b:i * BPC + b + 1, :] for b in range(BPC)], axis=1).astype(f32)
        o = y + b2 + x_v[:, cols].astype(f32)
        out_v[:, cols] = o.astype(bf16)
        cp_out(i).start()

    cp_x(0).wait()
    ln_chunk(0)
    cp_w1(0).wait(); cp_x(1).wait()
    for i in range(4, NC):
        cp_x(i).start()
    cp_wo.start(); cp_b1.start(); cp_b2.start()
    for i in range(4, NC):
        cp_w1(i).start()
    cp_w2.start()
    u_chunk(0, 1); ln_chunk(1)
    cp_w1(1).wait(); cp_x(2).wait()
    u_chunk(1, 2); ln_chunk(2)
    cp_w1(2).wait(); cp_x(3).wait()
    u_chunk(2, 3); ln_chunk(3)
    cp_w1(3).wait(); cp_wqkv.wait()
    u_chunk(3, 4); prep_wqkv()
    stage_a(0)
    for i in range(4, NC):
        cp_x(i).wait()
    cp_wo.wait(); cp_b1.wait(); cp_b2.wait()
    cp_w1(4).wait(); cp_w1(5).wait()
    stage_a(1)
    ln_chunk(4); ln_chunk(5)
    u_chunk(4, 6)
    stage_bb(0)
    ln_chunk(6); ln_chunk(7)
    prep_wo()
    cp_w1(6).wait(); cp_w1(7).wait()
    stage_a(2)
    u_chunk(6, 8, last=True)
    stage_bb(1)
    stage_a(3)
    stage_a(4)
    stage_bb(2)
    cp_w2.wait()
    stage_c(0)
    stage_a(5)
    stage_bb(3)
    stage_c(1)
    stage_a(6)
    stage_bb(4)
    stage_c(2)
    stage_a(7)
    stage_bb(5)
    stage_c(3)
    stage_c(4)
    stage_bb(6)
    stage_c(5)
    stage_c(6)
    stage_bb(7)
    stage_c(7)
    for i in range(NC):
        cp_out(i).wait()


@jax.jit
def pallas_parallel_sum__sliding_local_dilated__mixer_token_mlp__prompt_kernel(A_x, A_wqkv, A_wo, B_x, B_w1, B_b1, B_w2, B_b2):
    del B_x
    hbm = pl.BlockSpec(memory_space=pltpu.HBM)
    outT = pl.pallas_call(
        _kernel,
        out_shape=jax.ShapeDtypeStruct((1, D, S), bf16),
        in_specs=[hbm] * 7,
        out_specs=hbm,
        scratch_shapes=[
            pltpu.VMEM((D, S), bf16),
            pltpu.VMEM((D, 3 * D), bf16),
            pltpu.VMEM((D, D), bf16),
            pltpu.VMEM((S, F), bf16),
            pltpu.VMEM((F, S), bf16),
            pltpu.VMEM((NFB, LB), bf16),
            pltpu.VMEM((NB, LB), bf16),
            pltpu.VMEM((D, S), bf16),
            pltpu.VMEM((4, 3 * D, LB), f32),
            pltpu.VMEM((3 * D // 2, D), u32),
            pltpu.VMEM((4, D, LB), f32),
            pltpu.VMEM((D, D), f32),
            pltpu.VMEM((D // 2, D), u32),
            pltpu.VMEM((D // 2, S), u32),
            pltpu.VMEM((D // 2, S), u32),
            pltpu.VMEM((D, F), f32),
            pltpu.VMEM((D // 2, F), u32),
            pltpu.VMEM((NB + 1, 3 * D, LB), f32),
            pltpu.VMEM((D // 2, S), u32),
            pltpu.SemaphoreType.DMA((NC,)),
            pltpu.SemaphoreType.DMA((NC,)),
            pltpu.SemaphoreType.DMA((1,)),
            pltpu.SemaphoreType.DMA((4,)),
            pltpu.SemaphoreType.DMA((NC,)),
        ],
        compiler_params=pltpu.CompilerParams(vmem_limit_bytes=100 * 1024 * 1024),
    )(jnp.swapaxes(A_x, 1, 2), A_wqkv, A_wo, B_w1, B_b1.reshape(NFB, LB), B_w2, B_b2.reshape(NB, LB))
    return jnp.swapaxes(outT, 1, 2)
```

```python
import jax
import jax.numpy as jnp
from jax import lax
import jax.experimental.pallas as pl
import jax.experimental.pallas.tpu as pltpu

S, D, F = 2048, 448, 1792
H, DH, W, DIL = 16, 28, 8, 2
LB = 128
NB = S // LB
NFB = F // LB
HH = H // 2
WH = W // 2
SH = DIL * WH
EPS = 1e-5
SCALE = DH ** -0.5
f32 = jnp.float32
bf16 = jnp.bfloat16
u32 = jnp.uint32
i32 = jnp.int32

SCOPES = False
P = dict(LND=640, BD=400, G=4, L=4, LS=170, PP=150, MARG=300)


def _gelu(x):
    c = 0.7978845608028654
    return 0.5 * x * (1.0 + jnp.tanh(c * (x + 0.044715 * (x * x * x))))


def _pk(x):
    return pltpu.bitcast(x.astype(bf16), u32)


def _up(x):
    return pltpu.bitcast(x, bf16)


def _rowsum8(a):
    return jnp.broadcast_to(jnp.sum(a, axis=0, keepdims=True), (8, a.shape[1]))


def _tie(val, dep):
    if dep is None:
        return val
    z = lax.shift_right_logical(pltpu.bitcast(dep, u32), jnp.uint32(31))
    z = lax.shift_right_logical(z, jnp.uint32(1))
    return pltpu.bitcast(pltpu.bitcast(val, u32) | z, val.dtype)


def _kernel(x_hbm, wqkv_hbm, wo_hbm, w1_hbm, b1_hbm, w2_hbm, b2_hbm, out_hbm,
            x_v, wqkv_v, wo_v, w1_v, w2_v, b1_v, b2_v, out_v,
            wt_s, wp_s, wo_s, wo2_s, wot_s, xnT_s, hT_s, u_s, g_s, qkv_s, oT_s, op_s, b2f_s,
            sems):
    sem_ctr = [1]

    def mk(src, dst):
        c = pltpu.make_async_copy(src, dst, sems.at[sem_ctr[0]])
        sem_ctr[0] += 1
        return c

    def cp_x(b0, b1):
        sl = pl.ds(b0 * LB, (b1 - b0) * LB)
        return mk(x_hbm.at[0, :, sl], x_v.at[:, sl])

    def cp_w1(b0, b1):
        sl = pl.ds(b0 * LB, (b1 - b0) * LB)
        return mk(w1_hbm.at[sl, :], w1_v.at[sl, :])

    tl = []
    clock = [0]
    hist = []

    def wait(name, *cps):
        if SCOPES:
            with jax.named_scope("wait_" + name):
                for c in cps:
                    c.wait()
        else:
            for c in cps:
                c.wait()
        tl.clear()
        hist.clear()
        clock[0] = 0

    def mm(lhs, rhs):
        r = jnp.dot(lhs, rhs, preferred_element_type=f32)
        m, k = lhs.shape
        dur = m * (-(-k // LB)) * (-(-rhs.shape[1] // LB)) // 4
        tl.append((clock[0] + dur - min(dur, m), clock[0] + dur, r))
        clock[0] += dur
        return r

    def at(t):
        if t is None or t < 0:
            return None
        assert t < clock[0], (t, clock[0])
        best = None
        for (a, b, r) in tl:
            if a <= t:
                fr = min((t - a) / (b - a), 0.999)
                best = r[int(fr * (r.shape[0] // 8)) * 8:int(fr * (r.shape[0] // 8)) * 8 + 8, 0:LB]
        return best

    def prep_wqkv():
        wT = wqkv_v[...].astype(f32).T
        for c in range(4):
            cw = min(LB, D - c * LB)
            wt_s[c, :, 0:cw] = wT[:, c * LB:c * LB + cw]
        for p in range(3):
            for d in range(DH):
                r = (p * D + d * H) // 2
                for c in range(4):
                    cw = min(LB, D - c * LB)
                    t = wt_s[c, pl.ds(p * D + d, H, stride=DH), :]
                    wp_s[r:r + H // 2, c * LB:c * LB + cw] = _pk(t[:, 0:cw])

    def prep_wo():
        wo = wo_v[...].astype(f32)
        for c in range(4):
            cw = min(LB, D - c * LB)
            wo_s[c, :, 0:cw] = wo[:, c * LB:c * LB + cw]
        for hh in range(2):
            for d in range(DH):
                r = hh * (D // 2) + d * HH
                for c in range(4):
                    cw = min(LB, D - c * LB)
                    t = wo_s[c, pl.ds(hh * (D // 2) + d, HH, stride=DH), :]
                    wo2_s[r:r + HH, c * LB:c * LB + cw] = t[:, 0:cw]
        wot_s[...] = _pk(wo2_s[...].T)

    RG = 16
    NG = D // RG

    def ln(b, t0=None, dur=None):
        cols = slice(b * LB, (b + 1) * LB)

        def dep(fr):
            return None if t0 is None else at(t0 + fr * dur)

        def xg(g):
            return x_v[g * RG:(g + 1) * RG, cols].astype(f32)

        def x2(v):
            return jnp.concatenate([v, v], axis=0)

        s = xg(0) + x2(_tie(jnp.zeros((8, LB), f32), dep(0.0))) if dep(0.0) is not None else xg(0)
        for g in range(1, NG):
            s = s + xg(g)
        mu = _rowsum8(s) * (1.0 / D)
        s = None
        for g in range(NG):
            if g % 14 == 0:
                mu = _tie(mu, dep(0.14 + 0.11 * (g // 14)))
            c = xg(g) - x2(mu)
            s = c * c if s is None else s + c * c
        r1 = lax.rsqrt(_rowsum8(s) * (1.0 / D) + EPS)
        s1 = s2 = None
        for g in range(NG):
            if g % 7 == 0:
                mu = _tie(mu, dep(0.40 + 0.09 * (g // 7)))
            xn = (xg(g) - x2(mu)) * x2(r1)
            xnT_s[g * RG // 2:(g + 1) * RG // 2, cols] = _pk(xn)
            s1 = xn if s1 is None else s1 + xn
            s2 = xn * xn if s2 is None else s2 + xn * xn
        mu2 = _rowsum8(s1) * (1.0 / D)
        var2 = _rowsum8(s2) * (1.0 / D) - mu2 * mu2
        r2 = lax.rsqrt(var2 + EPS)
        a = r1 * r2
        bb = mu2 * r2
        for g in range(NG):
            if g % 14 == 0:
                mu = _tie(mu, dep(0.80 + 0.11 * (g // 14)))
            h = (xg(g) - x2(mu)) * x2(a) - x2(bb)
            hT_s[g * RG // 2:(g + 1) * RG // 2, cols] = _pk(h)

    def stage_u(b0, b1, n0=0, n1=NFB, last=False):
        rows = slice(b0 * LB, b1 * LB)
        step = 1 if last else max(1, 4 // (b1 - b0))
        for n in range(n0, n1, step):
            cs = slice(n * LB, min(n + step, n1) * LB)
            if last:
                r = u_s[:, cs] + b1_v[n:n + 1, :].astype(f32)
                for k0 in range(b0, b1, 4):
                    kr = slice(k0 * LB, (k0 + 4) * LB)
                    r = r + mm(_up(hT_s[:, kr]), w1_v[kr, cs])
                g_s[:, cs] = _pk(_gelu(r))
            else:
                r = mm(_up(hT_s[:, rows]), w1_v[rows, cs])
                if b0 == 0:
                    u_s[:, cs] = r
                else:
                    u_s[:, cs] += r

    def stage_a(b, p0=0, p1=3):
        r = mm(_up(wp_s[p0 * D // 2:p1 * D // 2, :]), _up(xnT_s[:, b * LB:(b + 1) * LB]))
        qkv_s[b + 1, p0 * D:p1 * D, :] = r

    lane0 = lax.broadcasted_iota(i32, (HH, LB), 1)
    lane2 = 2 * lane0
    zeros8 = jnp.zeros((HH, LB), f32)

    def mk_shift(*deps):
        deps = [d for d in deps if d is not None]
        lane = lane2
        if deps:
            bits = pltpu.bitcast(deps[0], u32)
            for d in deps[1:]:
                bits = bits | pltpu.bitcast(d, u32)
            lane = lane2 | pltpu.bitcast(lax.shift_right_logical(bits, jnp.uint32(31)), i32)

        def fwd(cur, prev, sh):
            if sh == 0:
                return cur
            return pltpu.roll(jnp.where(lane < 2 * (LB - sh), cur, prev), sh, 1)

        def bwd(cur, nxt):
            return pltpu.roll(jnp.where(lane >= 2 * SH, cur, nxt), LB - SH, 1)
        return fwd, bwd

    def grp_shift(t):
        deps = [at(t)]
        if P["L"] and len(hist) >= P["L"]:
            deps += hist[-P["L"]]
        return mk_shift(*deps)

    raw, probs, pps = {}, {}, {}

    def attn_qk(j, hh, t, bd):
        jn = min(j + 1, NB - 1)
        acc = [None] * WH
        accp = [None] * WH
        for d in range(DH):
            if d % P["G"] == 0:
                if d > 0:
                    hist.append(acc + accp)
                fwd, bwd = grp_shift(t + d * bd // DH)
            r = d * H + hh * HH
            q = qkv_s[j + 1, r:r + HH, :]
            qp = bwd(q, qkv_s[jn + 1, r:r + HH, :])
            k = qkv_s[j + 1, D + r:D + r + HH, :]
            kp = qkv_s[j, D + r:D + r + HH, :]
            for a in range(WH):
                ks = fwd(k, kp, DIL * a)
                t0, t1 = q * ks, qp * ks
                acc[a] = t0 if d == 0 else acc[a] + t0
                accp[a] = t1 if d == 0 else accp[a] + t1
        hist.append(acc + accp)
        raw[j, hh] = (acc, accp)

    def attn_sm(j, hh, t):
        fwd, _ = mk_shift(at(t))
        acc, accp = raw[j, hh]
        prev = raw.pop((j - 1, hh))[1] if j > 0 else [zeros8] * WH
        lg = acc + [fwd(accp[a], prev[a], SH) for a in range(WH)]
        lg = [a * SCALE for a in lg]
        if j == 0:
            lg = [lg[0]] + [jnp.where(lane0 >= DIL * w, lg[w], -1e9) for w in range(1, W)]
        m = lg[0]
        for w in range(1, W):
            m = jnp.maximum(m, lg[w])
        e = [jnp.exp(l - m) for l in lg]
        den = e[0]
        for w in range(1, W):
            den = den + e[w]
        inv = 1.0 / den
        probs[j, hh] = [x * inv for x in e]

    def attn_pp(j, hh, t):
        _, bwd = mk_shift(at(t))
        p = probs[j, hh]
        pn = probs[min(j + 1, NB - 1), hh]
        pps[j, hh] = [bwd(p[WH + a], pn[WH + a]) for a in range(WH)]

    def attn_pv(j, hh, t, bd):
        p = probs.pop((j, hh))
        pp = pps.pop((j, hh))
        for d2 in range(DH // 2):
            os_ = []
            for d in (2 * d2, 2 * d2 + 1):
                if d % P["G"] == 0:
                    if d > 0:
                        hist.append([])
                    fwd, _ = grp_shift(t + d * bd // DH)
                r = d * H + hh * HH
                v = qkv_s[j + 1, 2 * D + r:2 * D + r + HH, :]
                vp = qkv_s[j, 2 * D + r:2 * D + r + HH, :]
                o = op = None
                for a in range(WH):
                    vs = fwd(v, vp, DIL * a)
                    o = p[a] * vs if a == 0 else o + p[a] * vs
                    op = pp[a] * vs if a == 0 else op + pp[a] * vs
                opp = zeros8 if j == 0 else op_s[r:r + HH, :]
                if j < NB - 1:
                    op_s[r:r + HH, :] = op
                os_.append(o + fwd(op, opp, SH))
            ro = (hh * (D // 2) + 2 * d2 * HH) // 2
            oT_s[ro:ro + HH, j * LB:(j + 1) * LB] = _pk(jnp.concatenate(os_, axis=0))
        hist.append([])

    mains = []
    for j in range(NB + 2):
        if j < NB:
            mains.append(("qk", j, 0))
        if 0 <= j - 2 < NB:
            mains.append(("pv", j - 2, 1))
        if j < NB:
            mains.append(("qk", j, 1))
        elif j == NB:
            mains.append(None)
        if 0 <= j - 1 < NB:
            if j == 1:
                mains.append(None)
            mains.append(("pv", j - 1, 0))
    slot_ctr = [0]

    def slot(t, bd):
        n = slot_ctr[0]
        slot_ctr[0] += 1
        it = mains[n]
        if it is not None:
            (attn_qk if it[0] == "qk" else attn_pv)(it[1], it[2], t, bd)
        if n > 0 and mains[n - 1] is not None and mains[n - 1][0] == "qk":
            attn_sm(mains[n - 1][1], mains[n - 1][2], t + P["LS"])
        if n + 1 < len(mains) and mains[n + 1] is not None and mains[n + 1][0] == "pv":
            attn_pp(mains[n + 1][1], mains[n + 1][2], t + bd - P["PP"])

    C_PIECES = [(0, 2, 1), (2, 2, 1), (4, 2, 1), (6, 1, 1), (7, 1, 2)]

    def out_copy(it, boff, nb, r0, r1):
        off = it * (8 * LB) + boff * LB
        if not isinstance(it, int):
            off = pl.multiple_of(off, LB)
        sl = pl.ds(off, nb * LB)
        rs = pl.ds(r0, r1 - r0)
        return pltpu.make_async_copy(out_v.at[rs, sl], out_hbm.at[0, rs, sl], sems.at[0])

    def c_body(it, carry):
        for (boff, nb, ns) in C_PIECES:
            cols = pl.ds(pl.multiple_of(it * (8 * LB) + boff * LB, LB), nb * LB)
            y = jnp.dot(_up(g_s[...]), w2_v[:, cols], preferred_element_type=f32)
            y = y + jnp.dot(_up(wot_s[...]), _up(oT_s[:, cols]), preferred_element_type=f32)
            o = y + b2f_s[:, cols] + x_v[:, cols].astype(f32)
            rp = D // ns
            for q in range(ns):
                out_v[q * rp:(q + 1) * rp, cols] = o[q * rp:(q + 1) * rp, :].astype(bf16)
                out_copy(it, boff, nb, q * rp, (q + 1) * rp).start()
        return carry

    x0 = cp_x(0, 2); w1_0 = cp_w1(0, 2)
    x1 = cp_x(2, 4); w1_1 = cp_w1(2, 4)
    wqkv = mk(wqkv_hbm, wqkv_v)
    x2 = cp_x(4, 16); w1_2 = cp_w1(4, 8)
    wo = mk(wo_hbm, wo_v); b1c = mk(b1_hbm, b1_v); b2c = mk(b2_hbm, b2_v)
    w1_3 = cp_w1(8, 16)
    w2 = mk(w2_hbm, w2_v)
    for c in (x0, w1_0, x1, w1_1, wqkv, x2, w1_2, wo, b1c, b2c, w1_3, w2):
        c.start()

    qkv_s[0, D:3 * D, :] = jnp.zeros((2 * D, LB), f32)
    for buf in (xnT_s, hT_s, g_s, oT_s):
        buf[0:8, 0:64] = jnp.zeros((8, 64), u32)

    LND, BD, MARG = P["LND"], P["BD"], P["MARG"]
    wait("x0", x0)
    ln(0); ln(1)
    wait("w1_0", w1_0)
    stage_u(0, 2, 0, 10)
    wait("r2", x1, w1_1)
    stage_u(0, 2, 10, NFB)
    ln(2, -150, 480); ln(3, 250, 480)
    stage_u(2, 4, 0, 8)
    wait("wqkv", wqkv)
    stage_u(2, 4, 8, NFB)
    prep_wqkv()
    t = clock[0]
    stage_a(0); stage_a(1); stage_a(2); stage_a(3, 0, 1)
    for tt in (1850, 2300, 3150, 3550):
        slot(t + tt, BD)
    wait("mid", x2, w1_2)
    stage_a(3, 1, 3)
    ln(4, -100, 700)
    t = clock[0] - 200
    nb = 5
    for b in range(4, 16):
        stage_a(b)
        while nb < 16 and t + LND <= clock[0] - 150:
            ln(nb, t, LND)
            t += LND
            nb += 1
    stage_u(4, 8)
    while t + BD + MARG <= clock[0]:
        slot(t, BD)
        t += BD
    wait("fin", wo, b1c, b2c, w1_3, w2)
    stage_u(8, 16, last=True)
    prep_wo()
    for b in range(NB):
        b2f_s[:, b * LB:(b + 1) * LB] = b2_v[b:b + 1, :].astype(f32)
    t = 400
    left = len(mains) - slot_ctr[0]
    bd2 = (clock[0] - t - MARG) // left
    for _ in range(left):
        slot(t, bd2)
        t += bd2

    lax.fori_loop(0, 2, c_body, 0)
    outs = [out_copy(it, boff, nb_, q * (D // ns), (q + 1) * (D // ns))
            for it in range(2) for (boff, nb_, ns) in C_PIECES for q in range(ns)]
    wait("out", *outs)


@jax.jit
def pallas_parallel_sum__sliding_local_dilated__mixer_token_mlp__prompt_kernel(A_x, A_wqkv, A_wo, B_x, B_w1, B_b1, B_w2, B_b2):
    del B_x
    hbm = pl.BlockSpec(memory_space=pltpu.HBM)
    outT = pl.pallas_call(
        _kernel,
        out_shape=jax.ShapeDtypeStruct((1, D, S), bf16),
        in_specs=[hbm] * 7,
        out_specs=hbm,
        scratch_shapes=[
            pltpu.VMEM((D, S), bf16),
            pltpu.VMEM((D, 3 * D), bf16),
            pltpu.VMEM((D, D), bf16),
            pltpu.VMEM((S, F), bf16),
            pltpu.VMEM((F, S), bf16),
            pltpu.VMEM((NFB, LB), bf16),
            pltpu.VMEM((NB, LB), bf16),
            pltpu.VMEM((D, S), bf16),
            pltpu.VMEM((4, 3 * D, LB), f32),
            pltpu.VMEM((3 * D // 2, D), u32),
            pltpu.VMEM((4, D, LB), f32),
            pltpu.VMEM((D, D), f32),
            pltpu.VMEM((D // 2, D), u32),
            pltpu.VMEM((D // 2, S), u32),
            pltpu.VMEM((D // 2, S), u32),
            pltpu.VMEM((D, F), f32),
            pltpu.VMEM((D // 2, F), u32),
            pltpu.VMEM((NB + 1, 3 * D, LB), f32),
            pltpu.VMEM((D // 2, S), u32),
            pltpu.VMEM((D, LB), f32),
            pltpu.VMEM((1, S), f32),
            pltpu.SemaphoreType.DMA((16,)),
        ],
        compiler_params=pltpu.CompilerParams(vmem_limit_bytes=100 * 1024 * 1024,
                                             disable_bounds_checks=True,
                                             disable_semaphore_checks=True),
    )(jnp.swapaxes(A_x, 1, 2), A_wqkv, A_wo, B_w1, B_b1.reshape(NFB, LB), B_w2, B_b2.reshape(NB, LB))
    return jnp.swapaxes(outT, 1, 2)
```

```python
import jax
import jax.numpy as jnp
from jax import lax
import jax.experimental.pallas as pl
import jax.experimental.pallas.tpu as pltpu

S, D, F = 2048, 448, 1792
H, DH, W, DIL = 16, 28, 8, 2
LB = 128
NB = S // LB
NFB = F // LB
HH = H // 2
WH = W // 2
SH = DIL * WH
EPS = 1e-5
SCALE = DH ** -0.5
f32 = jnp.float32
bf16 = jnp.bfloat16
u32 = jnp.uint32
i32 = jnp.int32

SCOPES = False
P = dict(LND=640, BD=400, G=4, L=4, LS=170, PP=150, MARG=300, N3=10)


def _gelu(x):
    c = 0.7978845608028654
    return 0.5 * x * (1.0 + jnp.tanh(c * (x + 0.044715 * (x * x * x))))


def _pk(x):
    return pltpu.bitcast(x.astype(bf16), u32)


def _up(x):
    return pltpu.bitcast(x, bf16)


def _rowsum8(a):
    return jnp.broadcast_to(jnp.sum(a, axis=0, keepdims=True), (8, a.shape[1]))


def _tie(val, dep):
    if dep is None:
        return val
    z = lax.shift_right_logical(pltpu.bitcast(dep, u32), jnp.uint32(31))
    z = lax.shift_right_logical(z, jnp.uint32(1))
    return pltpu.bitcast(pltpu.bitcast(val, u32) | z, val.dtype)


def _kernel(x_hbm, wqkv_hbm, wo_hbm, w1_hbm, b1_hbm, w2_hbm, b2_hbm, out_hbm,
            x_v, wqkv_v, wo_v, w1_v, w2_v, b1_v, b2_v, out_v,
            wt_s, wp_s, wo_s, wo2_s, wot_s, xnT_s, hT_s, u_s, g_s, qkv_s, oT_s, op_s, b2f_s,
            sems):
    sem_ctr = [1]

    def mk(src, dst):
        c = pltpu.make_async_copy(src, dst, sems.at[sem_ctr[0]])
        sem_ctr[0] += 1
        return c

    def cp_x(b0, b1):
        sl = pl.ds(b0 * LB, (b1 - b0) * LB)
        return mk(x_hbm.at[0, :, sl], x_v.at[:, sl])

    def cp_w1(b0, b1):
        sl = pl.ds(b0 * LB, (b1 - b0) * LB)
        return mk(w1_hbm.at[sl, :], w1_v.at[sl, :])

    tl = []
    clock = [0]
    hist = []

    def wait(name, *cps):
        if SCOPES:
            with jax.named_scope("wait_" + name):
                for c in cps:
                    c.wait()
        else:
            for c in cps:
                c.wait()
        tl.clear()
        hist.clear()
        clock[0] = 0

    def mm(lhs, rhs):
        r = jnp.dot(lhs, rhs, preferred_element_type=f32)
        m, k = lhs.shape
        dur = m * (-(-k // LB)) * (-(-rhs.shape[1] // LB)) // 4
        tl.append((clock[0] + dur - min(dur, m), clock[0] + dur, r))
        clock[0] += dur
        return r

    def at(t):
        if t is None or t < 0:
            return None
        assert t < clock[0], (t, clock[0])
        best = None
        for (a, b, r) in tl:
            if a <= t:
                fr = min((t - a) / (b - a), 0.999)
                best = r[int(fr * (r.shape[0] // 8)) * 8:int(fr * (r.shape[0] // 8)) * 8 + 8, 0:LB]
        return best

    def prep_wqkv():
        nct = -(-3 * D // LB)
        done = 0
        for p in range(3):
            need = -(-(p + 1) * D // LB)
            for ct in range(done, need):
                w = min(LB, 3 * D - ct * LB)
                wT = wqkv_v[:, ct * LB:ct * LB + w].astype(f32).T
                for c in range(4):
                    cw = min(LB, D - c * LB)
                    wt_s[c, ct * LB:ct * LB + w, 0:cw] = wT[:, c * LB:c * LB + cw]
            done = need
            for d in range(DH):
                r = (p * D + d * H) // 2
                for c in range(4):
                    cw = min(LB, D - c * LB)
                    t = wt_s[c, pl.ds(p * D + d, H, stride=DH), :]
                    wp_s[r:r + H // 2, c * LB:c * LB + cw] = _pk(t[:, 0:cw])

    def prep_wo():
        wo = wo_v[...].astype(f32)
        for c in range(4):
            cw = min(LB, D - c * LB)
            wo_s[c, :, 0:cw] = wo[:, c * LB:c * LB + cw]
        for hh in range(2):
            for d in range(DH):
                r = hh * (D // 2) + d * HH
                for c in range(4):
                    cw = min(LB, D - c * LB)
                    t = wo_s[c, pl.ds(hh * (D // 2) + d, HH, stride=DH), :]
                    wo2_s[r:r + HH, c * LB:c * LB + cw] = t[:, 0:cw]
        wot_s[...] = _pk(wo2_s[...].T)

    RG = 16
    NG = D // RG

    def ln(b, t0=None, dur=None):
        cols = slice(b * LB, (b + 1) * LB)

        def dep(fr):
            return None if t0 is None else at(t0 + fr * dur)

        def xg(g):
            return x_v[g * RG:(g + 1) * RG, cols].astype(f32)

        def x2(v):
            return jnp.concatenate([v, v], axis=0)

        s = xg(0) + x2(_tie(jnp.zeros((8, LB), f32), dep(0.0))) if dep(0.0) is not None else xg(0)
        for g in range(1, NG):
            s = s + xg(g)
        mu = _rowsum8(s) * (1.0 / D)
        s = None
        for g in range(NG):
            if g % 14 == 0:
                mu = _tie(mu, dep(0.14 + 0.11 * (g // 14)))
            c = xg(g) - x2(mu)
            s = c * c if s is None else s + c * c
        r1 = lax.rsqrt(_rowsum8(s) * (1.0 / D) + EPS)
        s1 = s2 = None
        for g in range(NG):
            if g % 7 == 0:
                mu = _tie(mu, dep(0.40 + 0.09 * (g // 7)))
            xn = (xg(g) - x2(mu)) * x2(r1)
            xnT_s[g * RG // 2:(g + 1) * RG // 2, cols] = _pk(xn)
            s1 = xn if s1 is None else s1 + xn
            s2 = xn * xn if s2 is None else s2 + xn * xn
        mu2 = _rowsum8(s1) * (1.0 / D)
        var2 = _rowsum8(s2) * (1.0 / D) - mu2 * mu2
        r2 = lax.rsqrt(var2 + EPS)
        a = r1 * r2
        bb = mu2 * r2
        for g in range(NG):
            if g % 14 == 0:
                mu = _tie(mu, dep(0.80 + 0.11 * (g // 14)))
            h = (xg(g) - x2(mu)) * x2(a) - x2(bb)
            hT_s[g * RG // 2:(g + 1) * RG // 2, cols] = _pk(h)

    def stage_u(b0, b1, n0=0, n1=NFB, last=False):
        rows = slice(b0 * LB, b1 * LB)
        step = 1 if last else max(1, 4 // (b1 - b0))
        for n in range(n0, n1, step):
            cs = slice(n * LB, min(n + step, n1) * LB)
            if last:
                r = u_s[:, cs] + b1_v[n:n + 1, :].astype(f32)
                for k0 in range(b0, b1, 4):
                    kr = slice(k0 * LB, (k0 + 4) * LB)
                    r = r + mm(_up(hT_s[:, kr]), w1_v[kr, cs])
                g_s[:, cs] = _pk(_gelu(r))
            else:
                r = mm(_up(hT_s[:, rows]), w1_v[rows, cs])
                if b0 == 0:
                    u_s[:, cs] = r
                else:
                    u_s[:, cs] += r

    def stage_a(b, p0=0, p1=3):
        r = mm(_up(wp_s[p0 * D // 2:p1 * D // 2, :]), _up(xnT_s[:, b * LB:(b + 1) * LB]))
        qkv_s[b + 1, p0 * D:p1 * D, :] = r

    lane0 = lax.broadcasted_iota(i32, (HH, LB), 1)
    lane2 = 2 * lane0
    zeros8 = jnp.zeros((HH, LB), f32)

    def mk_shift(*deps):
        deps = [d for d in deps if d is not None]
        lane = lane2
        if deps:
            bits = pltpu.bitcast(deps[0], u32)
            for d in deps[1:]:
                bits = bits | pltpu.bitcast(d, u32)
            lane = lane2 | pltpu.bitcast(lax.shift_right_logical(bits, jnp.uint32(31)), i32)

        def fwd(cur, prev, sh):
            if sh == 0:
                return cur
            return pltpu.roll(jnp.where(lane < 2 * (LB - sh), cur, prev), sh, 1)

        def bwd(cur, nxt):
            return pltpu.roll(jnp.where(lane >= 2 * SH, cur, nxt), LB - SH, 1)
        return fwd, bwd

    def grp_shift(t):
        deps = [at(t)]
        if P["L"] and len(hist) >= P["L"]:
            deps += hist[-P["L"]]
        return mk_shift(*deps)

    raw, probs, pps = {}, {}, {}

    def attn_qk(j, hh, t, bd):
        jn = min(j + 1, NB - 1)
        acc = [None] * WH
        accp = [None] * WH
        for d in range(DH):
            if d % P["G"] == 0:
                if d > 0:
                    hist.append(acc + accp)
                fwd, bwd = grp_shift(t + d * bd // DH)
            r = d * H + hh * HH
            q = qkv_s[j + 1, r:r + HH, :]
            qp = bwd(q, qkv_s[jn + 1, r:r + HH, :])
            k = qkv_s[j + 1, D + r:D + r + HH, :]
            kp = qkv_s[j, D + r:D + r + HH, :]
            for a in range(WH):
                ks = fwd(k, kp, DIL * a)
                t0, t1 = q * ks, qp * ks
                acc[a] = t0 if d == 0 else acc[a] + t0
                accp[a] = t1 if d == 0 else accp[a] + t1
        hist.append(acc + accp)
        raw[j, hh] = (acc, accp)

    def attn_sm(j, hh, t):
        fwd, _ = mk_shift(at(t))
        acc, accp = raw[j, hh]
        prev = raw.pop((j - 1, hh))[1] if j > 0 else [zeros8] * WH
        lg = acc + [fwd(accp[a], prev[a], SH) for a in range(WH)]
        lg = [a * SCALE for a in lg]
        if j == 0:
            lg = [lg[0]] + [jnp.where(lane0 >= DIL * w, lg[w], -1e9) for w in range(1, W)]
        m = lg[0]
        for w in range(1, W):
            m = jnp.maximum(m, lg[w])
        e = [jnp.exp(l - m) for l in lg]
        den = e[0]
        for w in range(1, W):
            den = den + e[w]
        inv = 1.0 / den
        probs[j, hh] = [x * inv for x in e]

    def attn_pp(j, hh, t):
        _, bwd = mk_shift(at(t))
        p = probs[j, hh]
        pn = probs[min(j + 1, NB - 1), hh]
        pps[j, hh] = [bwd(p[WH + a], pn[WH + a]) for a in range(WH)]

    def attn_pv(j, hh, t, bd):
        p = probs.pop((j, hh))
        pp = pps.pop((j, hh))
        for d2 in range(DH // 2):
            os_ = []
            for d in (2 * d2, 2 * d2 + 1):
                if d % P["G"] == 0:
                    if d > 0:
                        hist.append([])
                    fwd, _ = grp_shift(t + d * bd // DH)
                r = d * H + hh * HH
                v = qkv_s[j + 1, 2 * D + r:2 * D + r + HH, :]
                vp = qkv_s[j, 2 * D + r:2 * D + r + HH, :]
                o = op = None
                for a in range(WH):
                    vs = fwd(v, vp, DIL * a)
                    o = p[a] * vs if a == 0 else o + p[a] * vs
                    op = pp[a] * vs if a == 0 else op + pp[a] * vs
                opp = zeros8 if j == 0 else op_s[r:r + HH, :]
                if j < NB - 1:
                    op_s[r:r + HH, :] = op
                os_.append(o + fwd(op, opp, SH))
            ro = (hh * (D // 2) + 2 * d2 * HH) // 2
            oT_s[ro:ro + HH, j * LB:(j + 1) * LB] = _pk(jnp.concatenate(os_, axis=0))
        hist.append([])

    mains = []
    for j in range(NB + 2):
        if j < NB:
            mains.append(("qk", j, 0))
        if 0 <= j - 2 < NB:
            mains.append(("pv", j - 2, 1))
        if j < NB:
            mains.append(("qk", j, 1))
        elif j == NB:
            mains.append(None)
        if 0 <= j - 1 < NB:
            if j == 1:
                mains.append(None)
            mains.append(("pv", j - 1, 0))
    slot_ctr = [0]

    def slot(t, bd):
        n = slot_ctr[0]
        slot_ctr[0] += 1
        it = mains[n]
        if it is not None:
            (attn_qk if it[0] == "qk" else attn_pv)(it[1], it[2], t, bd)
        if n > 0 and mains[n - 1] is not None and mains[n - 1][0] == "qk":
            attn_sm(mains[n - 1][1], mains[n - 1][2], t + P["LS"])
        if n + 1 < len(mains) and mains[n + 1] is not None and mains[n + 1][0] == "pv":
            attn_pp(mains[n + 1][1], mains[n + 1][2], t + bd - P["PP"])

    C_PIECES = [(0, 2, 1), (2, 2, 1), (4, 2, 1), (6, 1, 1), (7, 1, 2)]

    def out_copy(it, boff, nb, r0, r1):
        off = it * (8 * LB) + boff * LB
        if not isinstance(it, int):
            off = pl.multiple_of(off, LB)
        sl = pl.ds(off, nb * LB)
        rs = pl.ds(r0, r1 - r0)
        return pltpu.make_async_copy(out_v.at[rs, sl], out_hbm.at[0, rs, sl], sems.at[0])

    def c_body(it, carry):
        for (boff, nb, ns) in C_PIECES:
            cols = pl.ds(pl.multiple_of(it * (8 * LB) + boff * LB, LB), nb * LB)
            y = jnp.dot(_up(g_s[...]), w2_v[:, cols], preferred_element_type=f32)
            y = y + jnp.dot(_up(wot_s[...]), _up(oT_s[:, cols]), preferred_element_type=f32)
            o = y + b2f_s[:, cols] + x_v[:, cols].astype(f32)
            rp = D // ns
            for q in range(ns):
                out_v[q * rp:(q + 1) * rp, cols] = o[q * rp:(q + 1) * rp, :].astype(bf16)
                out_copy(it, boff, nb, q * rp, (q + 1) * rp).start()
        return carry

    x0 = cp_x(0, 2); w1_0 = cp_w1(0, 1); w1_1 = cp_w1(1, 2)
    x1 = cp_x(2, 4); w1_2 = cp_w1(2, 4)
    wqkv = mk(wqkv_hbm, wqkv_v)
    x2 = cp_x(4, 16); w1_3 = cp_w1(4, 16)
    wo = mk(wo_hbm, wo_v); b1c = mk(b1_hbm, b1_v); b2c = mk(b2_hbm, b2_v)
    w2 = mk(w2_hbm, w2_v)
    for c in (x0, w1_0, w1_1, x1, w1_2, wqkv, x2, w1_3, wo, b1c, b2c, w2):
        c.start()

    qkv_s[0, D:3 * D, :] = jnp.zeros((2 * D, LB), f32)
    for buf in (xnT_s, hT_s, g_s, oT_s):
        buf[0:8, 0:64] = jnp.zeros((8, 64), u32)

    LND, BD, MARG = P["LND"], P["BD"], P["MARG"]
    wait("x0", x0)
    ln(0); ln(1)
    wait("r1", w1_0)
    stage_u(0, 1, 0, 12)
    wait("r2", w1_1, x1)
    stage_u(0, 2, 12, NFB)
    stage_u(1, 2, 0, 12)
    ln(2, 0, 750); ln(3, 800, 750)
    wait("r3", w1_2)
    stage_u(2, 4, 0, P["N3"])
    wait("wqkv", wqkv)
    stage_u(2, 4, P["N3"], NFB)
    prep_wqkv()
    stage_a(0); stage_a(1)
    wait("mid", x2)
    t = 0
    nb = 4
    for b in range(2, 16):
        stage_a(b)
        while nb < 16 and t + LND <= clock[0] - 150:
            ln(nb, t, LND)
            t += LND
            nb += 1
    while t + BD + MARG <= clock[0]:
        slot(t, BD)
        t += BD
    wait("fin", w1_3, wo, b1c, b2c)
    stage_u(4, 16, last=True)
    prep_wo()
    for b in range(NB):
        b2f_s[:, b * LB:(b + 1) * LB] = b2_v[b:b + 1, :].astype(f32)
    t = 400
    left = len(mains) - slot_ctr[0]
    bd2 = (clock[0] - t - MARG) // left
    for _ in range(left):
        slot(t, bd2)
        t += bd2
    wait("w2", w2)

    lax.fori_loop(0, 2, c_body, 0)
    outs = [out_copy(it, boff, nb_, q * (D // ns), (q + 1) * (D // ns))
            for it in range(2) for (boff, nb_, ns) in C_PIECES for q in range(ns)]
    wait("out", *outs)


@jax.jit
def pallas_parallel_sum__sliding_local_dilated__mixer_token_mlp__prompt_kernel(A_x, A_wqkv, A_wo, B_x, B_w1, B_b1, B_w2, B_b2):
    del B_x
    hbm = pl.BlockSpec(memory_space=pltpu.HBM)
    outT = pl.pallas_call(
        _kernel,
        out_shape=jax.ShapeDtypeStruct((1, D, S), bf16),
        in_specs=[hbm] * 7,
        out_specs=hbm,
        scratch_shapes=[
            pltpu.VMEM((D, S), bf16),
            pltpu.VMEM((D, 3 * D), bf16),
            pltpu.VMEM((D, D), bf16),
            pltpu.VMEM((S, F), bf16),
            pltpu.VMEM((F, S), bf16),
            pltpu.VMEM((NFB, LB), bf16),
            pltpu.VMEM((NB, LB), bf16),
            pltpu.VMEM((D, S), bf16),
            pltpu.VMEM((4, 3 * D, LB), f32),
            pltpu.VMEM((3 * D // 2, D), u32),
            pltpu.VMEM((4, D, LB), f32),
            pltpu.VMEM((D, D), f32),
            pltpu.VMEM((D // 2, D), u32),
            pltpu.VMEM((D // 2, S), u32),
            pltpu.VMEM((D // 2, S), u32),
            pltpu.VMEM((D, F), f32),
            pltpu.VMEM((D // 2, F), u32),
            pltpu.VMEM((NB + 1, 3 * D, LB), f32),
            pltpu.VMEM((D // 2, S), u32),
            pltpu.VMEM((D, LB), f32),
            pltpu.VMEM((1, S), f32),
            pltpu.SemaphoreType.DMA((16,)),
        ],
        compiler_params=pltpu.CompilerParams(vmem_limit_bytes=100 * 1024 * 1024,
                                             disable_bounds_checks=True,
                                             disable_semaphore_checks=True),
    )(jnp.swapaxes(A_x, 1, 2), A_wqkv, A_wo, B_w1, B_b1.reshape(NFB, LB), B_w2, B_b2.reshape(NB, LB))
    return jnp.swapaxes(outT, 1, 2)
```

```python
import jax
import jax.numpy as jnp
from jax import lax
import jax.experimental.pallas as pl
import jax.experimental.pallas.tpu as pltpu

S, D, F = 2048, 448, 1792
H, DH, W, DIL = 16, 28, 8, 2
LB = 128
NB = S // LB
NFB = F // LB
HH = H // 2
WH = W // 2
SH = DIL * WH
HD = D // 2
HA = 3 * D // 2
K1 = 2 * LB
UB0 = 4
NUP = (NB - UB0) // 2
KC = F // 2 + K1
EPS = 1e-5
SCALE = DH ** -0.5
f32 = jnp.float32
bf16 = jnp.bfloat16
u32 = jnp.uint32
i32 = jnp.int32

SCOPES = False
P = dict(LND=640, BD=420, G=4, L=4, LS=170, PP=150, MARG=300, N3=8, PVD=680, PV0=50, HSD=250, CORD=(4, 2, 1, 3, 0, 5, 6), TS0=100, TSD=420, TG=1, KSPLIT=True, PVB=520, PVL=500, OS0=3050, OSD=300, UORD=(4, 2, 1, 3, 0, 5, 6), US0=100, USD=350, R6S=1800, PMIN=2, CH=0, DLB=True, PVPOS=16, PVD2=420, NQ0=3, NQ1=4, UE0=200, UED=2200, PW0=900)


def _gelu(x):
    c = 0.7978845608028654
    hx = 0.5 * x
    return hx + hx * jnp.tanh(x * (c + (c * 0.044715) * (x * x)))


def _pk(x):
    return pltpu.bitcast(x.astype(bf16), u32)


def _up(x):
    return pltpu.bitcast(x, bf16)


def _upf(x):
    return pltpu.bitcast(x, bf16).astype(f32)


def _cat(xs, axis):
    return xs[0] if len(xs) == 1 else jnp.concatenate(xs, axis=axis)


def _rowsum8(a):
    return jnp.broadcast_to(jnp.sum(a, axis=0, keepdims=True), (8, a.shape[1]))


def _tie(val, dep):
    if dep is None:
        return val
    z = lax.shift_right_logical(pltpu.bitcast(dep, u32), jnp.uint32(31))
    z = lax.shift_right_logical(z, jnp.uint32(1))
    return pltpu.bitcast(pltpu.bitcast(val, u32) | z, val.dtype)


def _lhs_ops(a11, a12, a21, a22):
    n2 = a12.shape[1]

    def ext(s, full):
        return s if n2 == full.shape[1] else jnp.concatenate([s, full[:, n2:]], axis=1)
    return [ext(a11[:, :n2] + a22, a11), ext(a21[:, :n2] + a22, a21), a11, a22,
            a11[:, :n2] + a12, a21 - a11, a12 - a22]


def _rhs_sums(b11, b12, b21, b22):
    n2 = b21.shape[0]

    def ext(s, full):
        return s if n2 == full.shape[0] else jnp.concatenate([s, full[n2:]], axis=0)
    return {0: ext(b11[:n2] + b22, b11), 2: ext(b12[:n2] - b22, b12), 3: b21 - b11[:n2],
            5: b11 + b12, 6: b21 + b22}


def _combine(m):
    c12 = m[2] + m[4]
    c21 = m[1] + m[3]
    x = (m[2] - m[1]) + m[0]
    return ((x + m[6]) + (c21 - c12), c12, c21, x + m[5])


def _kernel(x_hbm, wqkv_hbm, wo_hbm, w1_hbm, b1_hbm, w2_hbm, b2_hbm, out_hbm,
            x_v, wqkv_v, wo_v, w1_v, w2_v, b1_v, b2_v, out_v,
            wt_s, lw_s, wo_s, wo2_s, xnT_s, hT_s, lh_s, u_s, lc_s, qk_s, v_s, pr_s, ol_s, op_s, b2f_s, rs_s,
            sems):
    sem_ctr = [1]

    class Group:
        def __init__(self, pairs):
            self.cps = [pltpu.make_async_copy(a, b, sems.at[sem_ctr[0]]) for (a, b) in pairs]
            sem_ctr[0] += 1

        def start(self):
            for c in self.cps:
                c.start()

        def wait(self):
            for c in self.cps:
                c.wait()

    def mk(src, dst):
        return Group([(src, dst)])

    def cp_x(p0, p1):
        return Group([(x_hbm.at[0, :, pl.ds(p * 2 * LB, 2 * LB)], x_v.at[p]) for p in range(p0, p1)])

    def cp_w2(p0, p1):
        return Group([(w2_hbm.at[:, pl.ds(p * 2 * LB, 2 * LB)], w2_v.at[p]) for p in range(p0, p1)])

    def cp_w1(b0, b1):
        sl = pl.ds(b0 * LB, (b1 - b0) * LB)
        return mk(w1_hbm.at[sl, :], w1_v.at[sl, :])

    tl = []
    mxu = [0, 0, 0, 0]
    nxt = [0]
    hist = []

    tasks = []
    dls = []

    def task(t_emit, fn, *args):
        tasks.append((t_emit, fn, args))

    def flush(t=None):
        while tasks and (t is None or tasks[0][0] < t):
            _, fn, args = tasks.pop(0)
            fn(*args)

    def reset():
        assert not tasks
        dls.clear()
        tl.clear()
        hist.clear()
        mxu[:] = [0, 0, 0, 0]
        nxt[0] = 0

    def now():
        return sum(mxu) // 4

    def wait(name, *cps):
        flush()
        if SCOPES:
            with jax.named_scope("wait_" + name):
                for c in cps:
                    c.wait()
        else:
            for c in cps:
                c.wait()
        reset()

    def mm1(lhs, rhs, pace=True):
        flush(now())
        start = mxu[nxt[0]]
        due = [v for (t, v) in dls if t <= start] if (pace and lhs.shape[1] >= LB) else []
        if due:
            dls[:] = [(t, v) for (t, v) in dls if t > start]
        if P["CH"] and lhs.shape[1] >= LB:
            prev = at(start - P["CH"])
            if prev is not None:
                due = due + [pltpu.bitcast(prev, u32)]
        if due:
            z = due[0]
            for v in due[1:]:
                z = z | v
            tile = _up(_tie(pltpu.bitcast(lhs[0:16, 0:LB], u32), z))
            row = tile if lhs.shape[1] == LB else jnp.concatenate([tile, lhs[0:16, LB:]], axis=1)
            lhs = jnp.concatenate([row, lhs[16:]], axis=0)
        r = jnp.dot(lhs, rhs.astype(bf16), preferred_element_type=f32)
        m, k = lhs.shape
        kt = -(-k // LB)
        first_done = None
        for n in range(-(-rhs.shape[1] // LB)):
            end = 0
            for _ in range(kt):
                mxu[nxt[0]] += m
                end = max(end, mxu[nxt[0]])
                nxt[0] = (nxt[0] + 1) % 4
            if first_done is None:
                first_done = end
        if pace:
            tl.append((first_done - m, first_done, r))
        return r

    def mm(lhs, rhs):
        k = lhs.shape[1]
        if rhs.shape[1] > LB or not P["KSPLIT"]:
            return mm1(lhs, rhs)
        r, k0 = None, 0
        while k0 < k:
            k1 = min(k, k0 + (4 - nxt[0]) * LB)
            part = mm1(lhs[:, k0:k1], rhs[k0:k1], pace=(k1 - k0 > P['PMIN'] * LB - LB or k <= 2 * LB))
            r = part if r is None else r + part
            k0 = k1
        return r

    def at(t):
        if t is None or t < 0:
            return None
        t = min(t, now() - 1)
        best = None
        for (a, b, r) in tl:
            if a <= t and (best is None or min(b, t) > best[0]):
                row = int(min((t - a) / (b - a), 0.999) * (r.shape[0] // 8)) * 8
                best = (min(b, t), r, row)
        return None if best is None else best[1][best[2]:best[2] + 8, 0:LB]

    def strassen(lhs, sums, raw11, raw22, order, split_last=False, pre=None, head=0):
        m = [None] * 7

        def rhs(p, k0, k1):
            flush(now())
            if p == 1:
                return raw11(k0, k1)
            if p == 4:
                return raw22(k0, k1)
            return pre(p, k0, k1) if pre is not None else sums[p][k0:k1]

        if head:
            for p in order:
                m[p] = mm(lhs(p, 0, head * LB), rhs(p, 0, head * LB))
        for p in order:
            r = rhs(p, head * LB, None)
            l = lhs(p, head * LB, head * LB + r.shape[0])
            if split_last and p == order[-1]:
                kk = (-(-r.shape[0] // LB) - 2) * LB
                hm = l.shape[0] // 2
                hd = mm(l[:, :kk], r[:kk]) if kk else None
                tail = jnp.concatenate([mm(l[:hm, kk:], r[kk:]), mm(l[hm:, kk:], r[kk:])], axis=0)
                v = tail if hd is None else hd + tail
            else:
                v = mm(l, r)
            m[p] = v if m[p] is None else m[p] + v
        return m

    def tiles(fn, n):
        def get(k0, k1):
            return _cat([fn(i) for i in range(k0 // LB, n if k1 is None else k1 // LB)], 0)
        return get

    SIDX = {0: 0, 2: 1, 3: 2, 5: 3, 6: 4}
    RSK = KC // 2

    rs_ready = set()

    def put_sums(sm, ro):
        for p, v in sm.items():
            rs_s[ro:ro + v.shape[0] // 2, SIDX[p] * LB:(SIDX[p] + 1) * LB] = _pk(v)

    def tsum(ld, r0, slot_, i, t0, dur):
        for g in range(LB // 16):
            dep = at(t0 + g * dur // 8)
            t1 = ld(slice(r0 + g * 16, r0 + g * 16 + 16)).astype(f32)
            t2 = ld(slice(r0 + LB + g * 16, r0 + LB + g * 16 + 16)).astype(f32)
            d2 = None if dep is None else jnp.concatenate([dep, dep], axis=0)
            sm = _rhs_sums(_tie(t1[:, :LB], d2), t1[:, LB:], t2[:, :LB], _tie(t2[:, LB:], d2))
            put_sums(sm, slot_ * RSK + i * (LB // 2) + g * 8)
        rs_ready.add((slot_, i))

    def osum(oslot, slot_, t0, dur):
        ng = K1 // 16
        for g in range(ng):
            dep = at(t0 + g * dur // ng)
            r1 = oslot * HD + g * 8
            b11, b12 = _upf(_tie(ol_s[r1:r1 + 8, 0:LB], dep)), _upf(ol_s[r1:r1 + 8, LB:])
            if K1 + g * 16 < D:
                r2 = r1 + K1 // 2
                sm = _rhs_sums(b11, b12, _upf(ol_s[r2:r2 + 8, 0:LB]), _upf(_tie(ol_s[r2:r2 + 8, LB:], dep)))
                put_sums(sm, slot_ * RSK + F // 4 + g * 8)
            else:
                ro = slot_ * RSK + F // 4 + g * 8
                rs_s[ro:ro + 8, SIDX[0] * LB:(SIDX[0] + 1) * LB] = ol_s[r1:r1 + 8, 0:LB]
                rs_s[ro:ro + 8, SIDX[2] * LB:(SIDX[2] + 1) * LB] = ol_s[r1:r1 + 8, LB:]
                put_sums({5: b11 + b12}, ro)
        rs_ready.update({(slot_, NFB // 2), (slot_, NFB // 2 + 1)})

    def pre_of(slot_, k, short=0):
        def pre(p, k0, k1):
            if k1 is None:
                k1 = k - short if p in (3, 6) else k
            assert all((slot_, i) in rs_ready for i in range(k0 // LB, -(-k1 // LB))), (slot_, k0, k1, rs_ready)
            return _up(rs_s[slot_ * RSK + k0 // 2:slot_ * RSK + k1 // 2, SIDX[p] * LB:(SIDX[p] + 1) * LB])
        return pre

    def add_tasks(todo):
        tasks.extend(todo)
        tasks.sort(key=lambda x: x[0])

    def wrow(g):
        p, d = divmod(g, DH)
        t = [wt_s[c, pl.ds(p * D + d, H, stride=DH), :] for c in range(4)]
        return jnp.concatenate(t[0:2], axis=1), jnp.concatenate([t[2], t[3][:, 0:D - 3 * LB]], axis=1)

    def prep_wqkv():
        for ct in range(-(-3 * D // LB)):
            w = min(LB, 3 * D - ct * LB)
            wT = wqkv_v[:, ct * LB:ct * LB + w].astype(f32).T
            for c in range(4):
                cw = min(LB, D - c * LB)
                wt_s[c, ct * LB:ct * LB + w, 0:cw] = wT[:, c * LB:c * LB + cw]
        ng = HA // H
        for g in range(ng):
            a11, a12 = wrow(g)
            a21, a22 = wrow(g + ng)
            for p, v in enumerate(_lhs_ops(a11, a12, a21, a22)):
                lw_s[p * (HA // 2) + g * 8:p * (HA // 2) + g * 8 + 8, 0:v.shape[1]] = _pk(v)

    def prep_wo(t0):
        wo = wo_v[...].astype(f32) + _tie(jnp.zeros((8, LB), f32), at(t0))[0:1, 0:1]
        for c in range(4):
            cw = min(LB, D - c * LB)
            wo_s[c, :, 0:cw] = wo[:, c * LB:c * LB + cw]
        for hh in range(2):
            for d in range(DH):
                r = hh * HD + d * HH
                for c in range(4):
                    cw = min(LB, D - c * LB)
                    t = wo_s[c, pl.ds(hh * HD + d, HH, stride=DH), :]
                    wo2_s[r:r + HH, c * LB:c * LB + cw] = t[:, 0:cw]
        wot = wo2_s[...].T
        ops = _lhs_ops(wot[0:HD, 0:K1], wot[0:HD, K1:D], wot[HD:D, 0:K1], wot[HD:D, K1:D])
        for p, v in enumerate(ops):
            lc_s[p * (HD // 2):(p + 1) * (HD // 2), F // 2:F // 2 + v.shape[1]] = _pk(v)

    RG = 16
    NG = D // RG

    def ln(b, t0=None, dur=None):
        cols = slice(b * LB, (b + 1) * LB)

        def dep(fr):
            return None if t0 is None else at(t0 + fr * dur)

        def xg(g):
            return x_v[b // 2, g * RG:(g + 1) * RG, (b % 2) * LB:(b % 2 + 1) * LB].astype(f32)

        def x2(v):
            return jnp.concatenate([v, v], axis=0)

        s = xg(0) + x2(_tie(jnp.zeros((8, LB), f32), dep(0.0))) if dep(0.0) is not None else xg(0)
        for g in range(1, NG):
            s = s + xg(g)
        mu = _rowsum8(s) * (1.0 / D)
        s = None
        for g in range(NG):
            if g % 14 == 0:
                mu = _tie(mu, dep(0.14 + 0.11 * (g // 14)))
            c = xg(g) - x2(mu)
            s = c * c if s is None else s + c * c
        r1 = lax.rsqrt(_rowsum8(s) * (1.0 / D) + EPS)
        s1 = s2 = None
        for g in range(NG):
            if g % 7 == 0:
                mu = _tie(mu, dep(0.40 + 0.09 * (g // 7)))
            xn = (xg(g) - x2(mu)) * x2(r1)
            xnT_s[g * RG // 2:(g + 1) * RG // 2, cols] = _pk(xn)
            s1 = xn if s1 is None else s1 + xn
            s2 = xn * xn if s2 is None else s2 + xn * xn
        mu2 = _rowsum8(s1) * (1.0 / D)
        var2 = _rowsum8(s2) * (1.0 / D) - mu2 * mu2
        r2 = lax.rsqrt(var2 + EPS)
        a = r1 * r2
        bb = mu2 * r2
        for g in range(NG):
            if g % 14 == 0:
                mu = _tie(mu, dep(0.80 + 0.11 * (g // 14)))
            h = (xg(g) - x2(mu)) * x2(a) - x2(bb)
            hT_s[g * RG // 2:(g + 1) * RG // 2, cols] = _pk(h)

    def hsum(b, t0, dur):
        k = (b - UB0) // 2
        c0, c1 = slice(b * LB, (b + 1) * LB), slice((b + 1) * LB, (b + 2) * LB)
        ng = HD // RG
        for g in range(ng):
            dep = at(t0 + (g // 2) * 2 * dur // ng)
            top, bot = slice(g * 8, g * 8 + 8), slice(HD // 2 + g * 8, HD // 2 + g * 8 + 8)
            ops = _lhs_ops(_upf(_tie(hT_s[top, c0], dep)), _upf(hT_s[top, c1]),
                           _upf(hT_s[bot, c0]), _upf(_tie(hT_s[bot, c1], dep)))
            for p in (0, 1, 4, 5, 6):
                lh_s[p * (HD // 2) + g * 8:p * (HD // 2) + g * 8 + 8, k * LB:(k + 1) * LB] = _pk(ops[p])

    def stage_u(b0, b1, n0=0, n1=NFB):
        rows = slice(b0 * LB, b1 * LB)
        step = max(1, 4 // (b1 - b0))
        for n in range(n0, n1, step):
            cs = slice(n * LB, min(n + step, n1) * LB)
            r = mm(_up(hT_s[:, rows]), w1_v[rows, cs])
            if b0 == 0:
                u_s[:, cs] = r
            else:
                u_s[:, cs] += r

    def blk(b):
        return slice(b * LB, (b + 1) * LB)

    lc_ready = set()

    def u_epilogue(i, m, g0, g1, t0, dur):
        c0, c1 = blk(2 * i), blk(2 * i + 1)
        for g in range(g0, g1):
            dep = at(t0 + (g - g0) * dur // (g1 - g0))
            bia = [_tie(jnp.broadcast_to(b1_v[2 * i + e:2 * i + e + 1, :].astype(f32), (8, LB)), dep) for e in range(2)]
            bia = [jnp.concatenate([b, b], axis=0) for b in bia]
            top, bot = slice(g * 16, g * 16 + 16), slice(HD + g * 16, HD + g * 16 + 16)
            q = _combine([x[top] for x in m])
            gl = [_gelu(q[0] + (u_s[top, c0] + bia[0])), _gelu(q[1] + (u_s[top, c1] + bia[1])),
                  _gelu(q[2] + (u_s[bot, c0] + bia[0])), _gelu(q[3] + (u_s[bot, c1] + bia[1]))]
            for p, v in enumerate(_lhs_ops(*gl)):
                lc_s[p * (HD // 2) + g * 8:p * (HD // 2) + g * 8 + 8, blk(i)] = _pk(v)
        if g1 == HD // 16:
            lc_ready.add(i)

    def stage_u_last(i, order, edur):
        raw11 = tiles(lambda k: w1_v[blk(UB0 + 2 * k), blk(2 * i)], NUP)
        raw22 = tiles(lambda k: w1_v[blk(UB0 + 2 * k + 1), blk(2 * i + 1)], NUP)

        def lhs(p, k0, k1):
            ks = range(k0 // LB, k1 // LB)
            if p == 2:
                return _up(_cat([hT_s[0:HD // 2, blk(UB0 + 2 * k)] for k in ks], 1))
            if p == 3:
                return _up(_cat([hT_s[HD // 2:HD, blk(UB0 + 2 * k + 1)] for k in ks], 1))
            return _up(lh_s[p * (HD // 2):(p + 1) * (HD // 2), k0:k1])
        m = strassen(lhs, None, raw11, raw22, order, pre=pre_of(i % 3, NUP * LB))
        for k in range(NUP):
            rs_ready.discard((i % 3, k))
        t = now() - P["UE0"]
        ng = HD // 16
        add_tasks([(t + (g + 2) * edur // ng, u_epilogue, (i, m, g, g + 2, t + g * edur // ng, 2 * edur // ng))
                   for g in range(0, ng, 2)])

    def stage_a(b, odd=False, split_last=False):
        flush(now())
        c0, c1 = slice(b * LB, (b + 1) * LB), slice((b + 1) * LB, (b + 2) * LB)
        k1, k2 = slice(0, K1 // 2), slice(K1 // 2, D // 2)
        sums = _rhs_sums(_upf(xnT_s[k1, c0]), _upf(xnT_s[k1, c1]), _upf(xnT_s[k2, c0]), _upf(xnT_s[k2, c1]))

        def lhs(p, k0, k1_):
            return _up(lw_s[p * (HA // 2):(p + 1) * (HA // 2), k0:k1_])
        order = (6, 4, 2, 1, 3, 0, 5) if odd else (4, 2, 1, 3, 0, 5, 6)
        q = _combine(strassen(lhs, sums, lambda a, b_: _up(xnT_s[k1, c0]), lambda a, b_: _up(xnT_s[k2, c1]),
                              order, split_last))
        for e in range(2):
            qk_s[b + e + 1, 0:HA, :] = q[e]
            qk_s[b + e + 1, HA:2 * D, :] = q[2 + e][0:2 * D - HA]
            v_s[b + e + 1] = q[2 + e][2 * D - HA:]

    lane0 = lax.broadcasted_iota(i32, (HH, LB), 1)
    lane2 = 2 * lane0
    zeros8 = jnp.zeros((HH, LB), f32)

    def mk_shift(*deps):
        deps = [d for d in deps if d is not None]
        lane = lane2
        if deps:
            bits = pltpu.bitcast(deps[0], u32)
            for d in deps[1:]:
                bits = bits | pltpu.bitcast(d, u32)
            lane = lane2 | pltpu.bitcast(lax.shift_right_logical(bits, jnp.uint32(31)), i32)

        def fwd(cur, prev, sh):
            if sh == 0:
                return cur
            return pltpu.roll(jnp.where(lane < 2 * (LB - sh), cur, prev), sh, 1)

        def bwd(cur, nxt_):
            return pltpu.roll(jnp.where(lane >= 2 * SH, cur, nxt_), LB - SH, 1)
        return fwd, bwd

    def grp_shift(t):
        deps = [at(t)]
        if P["L"] and len(hist) >= P["L"]:
            deps += hist[-P["L"]]
        return mk_shift(*deps)

    raw, probs = {}, {}

    def attn_qk(j, hh, t, bd):
        jn = min(j + 1, NB - 1)
        acc = [None] * WH
        accp = [None] * WH
        for d in range(DH):
            if d % P["G"] == 0:
                if d > 0:
                    hist.append(acc + accp)
                fwd, bwd = grp_shift(t + d * bd // DH)
            r = d * H + hh * HH
            q = qk_s[j + 1, r:r + HH, :]
            qp = bwd(q, qk_s[jn + 1, r:r + HH, :])
            k = qk_s[j + 1, D + r:D + r + HH, :]
            kp = qk_s[j, D + r:D + r + HH, :]
            for a in range(WH):
                ks = fwd(k, kp, DIL * a)
                t0, t1 = q * ks, qp * ks
                acc[a] = t0 if d == 0 else acc[a] + t0
                accp[a] = t1 if d == 0 else accp[a] + t1
        hist.append(acc + accp)
        raw[j, hh] = (acc, accp)

    def attn_sm(j, hh, t):
        fwd, _ = mk_shift(at(t))
        acc, accp = raw[j, hh]
        prev = raw.pop((j - 1, hh))[1] if j > 0 else [zeros8] * WH
        lg = acc + [fwd(accp[a], prev[a], SH) for a in range(WH)]
        lg = [a * SCALE for a in lg]
        if j == 0:
            lg = [lg[0]] + [jnp.where(lane0 >= DIL * w, lg[w], -1e9) for w in range(1, W)]
        m = lg[0]
        for w in range(1, W):
            m = jnp.maximum(m, lg[w])
        e = [jnp.exp(l - m) for l in lg]
        den = e[0]
        for w in range(1, W):
            den = den + e[w]
        inv = 1.0 / den
        p = [x * inv for x in e]
        for a in range(WH):
            pr_s[j, (hh * W + a) * HH:(hh * W + a + 1) * HH, :] = p[a]
        probs[j, hh] = p[WH:]

    def attn_pp(j, hh, t):
        _, bwd = mk_shift(at(t))
        p = probs.pop((j, hh))
        pn = probs[j + 1, hh] if j + 1 < NB else p
        for a in range(WH):
            pr_s[j, (hh * W + WH + a) * HH:(hh * W + WH + a + 1) * HH, :] = bwd(p[a], pn[a])

    def attn_pv(j, hh, slot_, e, t, bd, t_dl=None):
        pa = [pr_s[j, (hh * W + a) * HH:(hh * W + a + 1) * HH, :] for a in range(W)]
        p, pp = pa[:WH], pa[WH:]
        acc_or = None
        for d2 in range(DH // 2):
            os_ = []
            for d in (2 * d2, 2 * d2 + 1):
                if d % P["G"] == 0:
                    if d > 0:
                        hist.append([])
                    fwd, _ = grp_shift(t + d * bd // DH)
                r = d * H + hh * HH
                v = v_s[j + 1, r:r + HH, :]
                vp = v_s[j, r:r + HH, :]
                o = op = None
                for a in range(WH):
                    vs = fwd(v, vp, DIL * a)
                    o = p[a] * vs if a == 0 else o + p[a] * vs
                    op = pp[a] * vs if a == 0 else op + pp[a] * vs
                opp = zeros8 if (isinstance(j, int) and j == 0) else op_s[r:r + HH, :]
                op_s[r:r + HH, :] = op
                os_.append(o + fwd(op, opp, SH))
            ro = slot_ * HD + (hh * HD + 2 * d2 * HH) // 2
            ol_s[ro:ro + HH, e * LB:(e + 1) * LB] = _pk(jnp.concatenate(os_, axis=0))
            if t_dl is not None:
                ob = pltpu.bitcast(os_[1], u32)
                if P["DLB"]:
                    ob = ob | pltpu.bitcast(os_[0], u32)
                acc_or = ob if acc_or is None else acc_or | ob
        hist.append([])
        if t_dl is not None:
            dls.append((t_dl, acc_or))

    mains = [("qk", j, hh) for j in range(NB) for hh in range(2)]
    npv = P["PVPOS"]
    mains = mains[:npv] + [("pv", j, hh) for j in range(2) for hh in range(2)] + mains[npv:] + [None, None]
    slot_ctr = [0]

    def slot(t, bd):
        n = slot_ctr[0]
        slot_ctr[0] += 1
        it = mains[n]
        if it is None:
            pass
        elif it[0] == "qk":
            attn_qk(it[1], it[2], t, bd)
        else:
            attn_pv(it[1], it[2], 1, it[1], t, bd, t + bd + P["PVL"])
        if n >= 1 and mains[n - 1] is not None and mains[n - 1][0] == "qk":
            attn_sm(mains[n - 1][1], mains[n - 1][2], t + P["LS"])
        if n >= 2 and mains[n - 2] is not None and mains[n - 2][0] == "qk":
            _, j, hh = mains[n - 2]
            if j > 0:
                attn_pp(j - 1, hh, t + P["PP"])
            if j == NB - 1:
                attn_pp(j, hh, t + P["PP"])

    NPRE = 2
    NPC = 3
    CD = 7 * (KC // LB) * HD // 4

    def lanes(pidx, e0, e1):
        off = pidx * (2 * LB) + e0 * LB
        if not isinstance(pidx, int):
            off = pl.multiple_of(off, LB)
        return pl.ds(off, (e1 - e0) * LB)

    def out_copy(pidx, e0, e1, r0, r1):
        sl = lanes(pidx, e0, e1)
        rs = pl.ds(r0, r1 - r0)
        return pltpu.make_async_copy(out_v.at[pidx, rs, pl.ds(e0 * LB, (e1 - e0) * LB)], out_hbm.at[0, rs, sl], sems.at[0])

    def out_parts(fine):
        return [(1, 2, 0, HD), (0, 2, HD, D), (0, 1, 0, HD)] if fine else [(0, 2, 0, D)]

    def piece(pidx, sl, pn, fine=False, head=0, nqk=0):
        sn = (sl + 1) % 3
        t0 = now()
        k1, k2 = slice(sl * HD, sl * HD + K1 // 2), slice(sl * HD + K1 // 2, (sl + 1) * HD)
        nw = NFB // 2
        raw11 = tiles(lambda i: w2_v[pidx, blk(2 * i), 0:LB] if i < nw else _up(ol_s[k1, 0:LB]), nw + 1)
        raw22 = tiles(lambda i: w2_v[pidx, blk(2 * i + 1), LB:] if i < nw else _up(ol_s[k2, LB:]), nw + 1)

        def lhs(p, k0, k1_):
            assert all(i in lc_ready for i in range(k0 // LB, min(nw, k1_ // LB))), (k0, k1_, lc_ready)
            return _up(lc_s[p * (HD // 2):(p + 1) * (HD // 2), k0:k1_])
        todo = []
        for i in range(nw):
            tt = t0 + P['TS0'] + i * P['TSD']
            todo.append((tt + P['TSD'], tsum, (lambda rs: w2_v[pn, rs, :], 2 * i * LB, sn, i, tt, P['TSD'])))
        t = t0 + P["PV0"]
        pvd, pvb = (P["PVD"], P["PVB"]) if nqk == 0 else (P["PVD2"], P["PVD2"])
        for e in range(2):
            for hh in range(2):
                todo.append((t + pvb, attn_pv, (pn * 2 + e, hh, sn, e, t, pvb, t + pvb + P["PVL"])))
                t += pvd
        for _ in range(nqk):
            todo.append((t + pvd, slot, (t, pvd)))
            t += pvd
        todo.append((t0 + P["OS0"] + P["OSD"], osum, (sn, sn, t0 + P["OS0"], P["OSD"])))
        add_tasks(todo)
        q = _combine(strassen(lhs, None, raw11, raw22, P['CORD'], pre=pre_of(sl, KC, 2 * K1 - D), head=head))
        flush()
        for (e0, e1, r0, r1) in out_parts(fine):
            cols = slice(e0 * LB, e1 * LB)
            for h0 in range(r0, r1, HD):
                y = _cat([q[2 * (h0 // HD) + e] for e in range(e0, e1)], 1)
                o = y + b2f_s[pidx, 0:1, cols] + x_v[pidx, h0:h0 + HD, cols].astype(f32)
                out_v[pidx, h0:h0 + HD, cols] = o.astype(bf16)
            out_copy(pidx, e0, e1, r0, r1).start()

    def c_body(it, carry):
        reset()
        rs_ready.update({(0, i) for i in range(KC // LB)})
        lc_ready.update(range(NFB // 2))
        for c in range(NPC):
            pidx = NPRE + it * NPC + c
            piece(pidx, c, lax.rem(pidx + 1, NB // 2), fine=c == NPC - 1)
        return carry

    x0 = cp_x(0, 1); w1_0 = cp_w1(0, 1); w1_1 = cp_w1(1, 2)
    x1 = cp_x(1, 2); w1_2 = cp_w1(2, 4)
    wqkv = mk(wqkv_hbm, wqkv_v)
    x2 = cp_x(2, NB // 2); w1_3 = cp_w1(4, 16)
    wo = mk(wo_hbm, wo_v); b1c = mk(b1_hbm, b1_v); b2c = mk(b2_hbm, b2_v)
    w2a = cp_w2(0, NPRE + 1); w2 = cp_w2(NPRE + 1, NB // 2)
    for c in (x0, w1_0, w1_1, x1, w1_2, wqkv, x2, w1_3, wo, b1c, b2c, w2a, w2):
        c.start()

    qk_s[0, D:2 * D, :] = jnp.zeros((D, LB), f32)
    v_s[0] = jnp.zeros((D, LB), f32)
    for buf in (xnT_s, hT_s, lh_s, ol_s, rs_s):
        buf[0:8, 0:64] = jnp.zeros((8, 64), u32)

    LND, BD, MARG = P["LND"], P["BD"], P["MARG"]
    wait("x0", x0)
    ln(0); ln(1)
    wait("r1", w1_0)
    stage_u(0, 1, 0, 12)
    wait("r2", w1_1, x1)
    stage_u(0, 2, 12, NFB)
    stage_u(1, 2, 0, 12)
    ln(2, 0, 750); ln(3, 800, 750)
    wait("r3", w1_2)
    stage_u(2, 4, 0, P["N3"])
    wait("wqkv", wqkv)
    stage_u(2, 4, P["N3"], NFB)
    prep_wqkv()
    stage_a(0, split_last=True)
    wait("mid", x2)
    AD = 7 * HA // 2
    UD = 7 * NUP * HD // 4
    r5 = (NB // 2 - 1) * AD
    t = 0
    todo = []
    for b in range(UB0, NB, 2):
        for fn, bb, dur in ((ln, b, LND), (ln, b + 1, LND), (hsum, b, P["HSD"])):
            todo.append((t + dur, fn, (bb, t, dur)))
            t += dur
    n5 = 0
    while t + BD + MARG <= r5:
        todo.append((t + BD, slot, (t, BD)))
        t += BD
        n5 += 1
    add_tasks(todo)
    for n, b in enumerate(range(2, NB, 2)):
        stage_a(b, odd=n % 2 == 1, split_last=b == NB - 2)
    wait("fin", w1_3, wo, b1c, b2c, w2a)
    r6 = (NFB // 2) * UD
    todo = []
    for i in range(NFB // 2 + 1):
        if i == 0:
            t0, dt = -200, 130
        elif i == 1:
            t0, dt = 700, 260
        else:
            t0, dt = (i - 1) * UD + P["US0"], P["USD"]
        if i < NFB // 2:
            for k in range(NUP):
                tt = t0 + k * dt
                todo.append((tt + dt, tsum, (lambda rs, i=i: w1_v[rs, 2 * i * LB:(2 * i + 2) * LB], (UB0 + 2 * k) * LB, i % 3, k, tt, dt)))
        else:
            for k in range(NFB // 2):
                tt = t0 + k * 300
                todo.append((tt + 300, tsum, (lambda rs: w2_v[0, rs, :], 2 * k * LB, 1, k, tt, 300)))
    left = len(mains) - n5 - P["NQ0"] - P["NQ1"]
    t = P["R6S"]
    bd2 = (r6 - t) // left
    for _ in range(left):
        todo.append((t + min(bd2, 600), slot, (t, min(bd2, 600))))
        t += bd2
    todo.append((r6 - 100, osum, (1, 1, r6 - 500, 400)))
    todo.append((P["PW0"] + 1, prep_wo, (P["PW0"],)))
    add_tasks(todo)
    for b in range(NB):
        b2f_s[b // 2, 0:1, (b % 2) * LB:(b % 2 + 1) * LB] = b2_v[b:b + 1, :].astype(f32)
    for i in range(NFB // 2):
        stage_u_last(i, (1, 4, 2, 3, 0, 5, 6) if i == 0 else P["UORD"], P["UED"] if i < NFB // 2 - 1 else 1200)
    piece(0, 1, 1, head=4, nqk=P["NQ0"])
    piece(1, 2, 2, nqk=P["NQ1"])
    assert slot_ctr[0] == len(mains)
    wait("w2", w2)

    lax.fori_loop(0, 2, c_body, 0)
    outs = [out_copy(pidx, *part) for pidx in range(NB // 2)
            for part in out_parts(pidx >= NPRE and (pidx - NPRE) % NPC == NPC - 1)]
    wait("out", *outs)


@jax.jit
def pallas_parallel_sum__sliding_local_dilated__mixer_token_mlp__prompt_kernel(A_x, A_wqkv, A_wo, B_x, B_w1, B_b1, B_w2, B_b2):
    del B_x
    hbm = pl.BlockSpec(memory_space=pltpu.HBM)
    outT = pl.pallas_call(
        _kernel,
        out_shape=jax.ShapeDtypeStruct((1, D, S), bf16),
        in_specs=[hbm] * 7,
        out_specs=hbm,
        scratch_shapes=[
            pltpu.VMEM((NB // 2, D, 2 * LB), bf16),
            pltpu.VMEM((D, 3 * D), bf16),
            pltpu.VMEM((D, D), bf16),
            pltpu.VMEM((S, F), bf16),
            pltpu.VMEM((NB // 2, F, 2 * LB), bf16),
            pltpu.VMEM((NFB, LB), bf16),
            pltpu.VMEM((NB, LB), bf16),
            pltpu.VMEM((NB // 2, D, 2 * LB), bf16),
            pltpu.VMEM((4, 3 * D, LB), f32),
            pltpu.VMEM((7 * HA // 2, K1), u32),
            pltpu.VMEM((4, D, LB), f32),
            pltpu.VMEM((D, D), f32),
            pltpu.VMEM((HD, S), u32),
            pltpu.VMEM((HD, S), u32),
            pltpu.VMEM((7 * HD // 2, NUP * LB), u32),
            pltpu.VMEM((D, F), f32),
            pltpu.VMEM((7 * HD // 2, KC), u32),
            pltpu.VMEM((NB + 1, 2 * D, LB), f32),
            pltpu.VMEM((NB + 1, D, LB), f32),
            pltpu.VMEM((NB, 2 * W * HH, LB), f32),
            pltpu.VMEM((3 * HD, 2 * LB), u32),
            pltpu.VMEM((D, LB), f32),
            pltpu.VMEM((NB // 2, 32, 2 * LB), f32),
            pltpu.VMEM((3 * KC // 2, 5 * LB), u32),
            pltpu.SemaphoreType.DMA((16,)),
        ],
        compiler_params=pltpu.CompilerParams(vmem_limit_bytes=100 * 1024 * 1024,
                                             disable_bounds_checks=True,
                                             disable_semaphore_checks=True),
    )(jnp.swapaxes(A_x, 1, 2), A_wqkv, A_wo, B_w1, B_b1.reshape(NFB, LB), B_w2, B_b2.reshape(NB, LB))
    return jnp.swapaxes(outT, 1, 2)
```

```python
import jax
import jax.numpy as jnp
from jax import lax
import jax.experimental.pallas as pl
import jax.experimental.pallas.tpu as pltpu

S, D, F = 2048, 448, 1792
H, DH, W, DIL = 16, 28, 8, 2
LB = 128
NB = S // LB
NP = NB // 2
NFB = F // LB
NFP = NFB // 2
HH = H // 2
WH = W // 2
SH = DIL * WH
HD = D // 2
QD = D // 4
HA = 3 * HD
UB0 = 4
NUP = (NB - UB0) // 2
KC = F // 2 + HD
RSK = (NFP + 2) * LB // 2
EPS = 1e-5
SCALE = DH ** -0.5
f32 = jnp.float32
bf16 = jnp.bfloat16
u32 = jnp.uint32
i32 = jnp.int32

SCOPES = False
P = dict(LND=640, BD=440, G=4, L=4, LS=170, PP=150, MARG=300, N3=10, PVD=680, PV0=50, HSD=560, HG=80,
         CORD=(4, 2, 1, 3, 0, 5, 6), TS0=100, TSD=420, PVB=520, PVL=500, OS0=3050, OSD=300,
         UORD=(4, 2, 1, 3, 0, 5, 6), US0=100, USD=350, R6S=1800, PVPOS=16, PVD2=420, NQ0=3, NQ1=3,
         UE0=0, UED=2200, UEL=1300, PW0=900, LNQ1=4, LNQ3=4, LNA=0.3, LNB=0.42, LNBD=0.33)


def _gelu(x):
    c = 0.7978845608028654
    hx = 0.5 * x
    return hx + hx * jnp.tanh(x * (c + (c * 0.044715) * (x * x)))


def _pk(x):
    return pltpu.bitcast(x.astype(bf16), u32)


def _up(x):
    return pltpu.bitcast(x, bf16)


def _upf(x):
    return pltpu.bitcast(x, bf16).astype(f32)


def _cat(xs, axis):
    return xs[0] if len(xs) == 1 else jnp.concatenate(xs, axis=axis)


def _x2(v):
    return jnp.concatenate([v, v], axis=0)


def _blk(b):
    return slice(b * LB, (b + 1) * LB)


def _rowsum8(a):
    return jnp.broadcast_to(jnp.sum(a, axis=0, keepdims=True), (8, a.shape[1]))


def _zero(*deps):
    deps = [d for d in deps if d is not None]
    if not deps:
        return None
    bits = pltpu.bitcast(deps[0], u32)
    for d in deps[1:]:
        bits = bits | pltpu.bitcast(d, u32)
    return lax.shift_right_logical(lax.shift_right_logical(bits, jnp.uint32(31)), jnp.uint32(1))


def _orz(v, z):
    return v if z is None else pltpu.bitcast(pltpu.bitcast(v, u32) | z, v.dtype)


def _pkz(v, z):
    return _pk(v if z is None else jnp.concatenate([_orz(v[0:8], z), v[8:16]], axis=0))


def _lhs_ops(a11, a12, a21, a22):
    return [a11 + a22, a21 + a22, a11, a22, a11 + a12, a21 - a11, a12 - a22]


SIDX = {0: 0, 2: 1, 3: 2, 5: 3, 6: 4}


def _rhs_sums(b11, b12, b21, b22):
    return {0: b11 + b22, 2: b12 - b22, 3: b21 - b11, 5: b11 + b12, 6: b21 + b22}


def _combine(m):
    c12 = m[2] + m[4]
    c21 = m[1] + m[3]
    x = (m[2] - m[1]) + m[0]
    return ((x + m[6]) + (c21 - c12), c12, c21, x + m[5])


def _kernel(x_hbm, wqkv_hbm, wo_hbm, w1_hbm, b1_hbm, w2_hbm, b2_hbm, out_hbm,
            x_v, wqkv_v, wo_v, w1_v, w2_v, b1_v, b2_v, out_v,
            wt_s, lw_s, wo_s, wo2_s, xnT_s, ra_s, hT_s, lh_s, u_s, lc_s, qk_s, v_s, pr_s, ol_s, op_s,
            b2f_s, rs_s, sems):
    sem_ctr = [1]

    class Group:
        def __init__(self, pairs):
            self.cps = [pltpu.make_async_copy(a, b, sems.at[sem_ctr[0]]) for (a, b) in pairs]
            sem_ctr[0] += 1

        def start(self):
            for c in self.cps:
                c.start()

        def wait(self):
            for c in self.cps:
                c.wait()

    def cp_x(p0, p1):
        return [(x_hbm.at[0, :, pl.ds(p * 2 * LB, 2 * LB)], x_v.at[p]) for p in range(p0, p1)]

    def cp_w2(p0, p1):
        return [(w2_hbm.at[:, pl.ds(p * 2 * LB, 2 * LB)], w2_v.at[p]) for p in range(p0, p1)]

    def cp_w1(b0, b1):
        sl = pl.ds(b0 * LB, (b1 - b0) * LB)
        return [(w1_hbm.at[sl, :], w1_v.at[sl, :])]

    tl = []
    mxu = [0, 0, 0, 0]
    nxt = [0]
    hist = []
    tasks = []
    dls = []
    ready = set()

    def add_tasks(todo):
        tasks.extend(todo)
        tasks.sort(key=lambda x: x[0])

    def flush(t=None):
        while tasks and (t is None or tasks[0][0] < t):
            _, fn, args = tasks.pop(0)
            fn(*args)

    def reset():
        assert not tasks
        dls.clear()
        tl.clear()
        hist.clear()
        mxu[:] = [0, 0, 0, 0]
        nxt[0] = 0

    def now():
        return sum(mxu) // 4

    def wait(name, *cps):
        flush()
        if SCOPES:
            with jax.named_scope("wait_" + name):
                for c in cps:
                    c.wait()
        else:
            for c in cps:
                c.wait()
        reset()

    def mm1(lhs, rhs, pace=True):
        flush(now())
        start = mxu[nxt[0]]
        due = [v for (t, v) in dls if t <= start] if pace else []
        if due:
            dls[:] = [(t, v) for (t, v) in dls if t > start]
            tile = _up(pltpu.bitcast(lhs[0:16, 0:LB], u32) | _zero(*due))
            row = tile if lhs.shape[1] == LB else jnp.concatenate([tile, lhs[0:16, LB:]], axis=1)
            lhs = jnp.concatenate([row, lhs[16:]], axis=0)
        r = jnp.dot(lhs, rhs, preferred_element_type=f32)
        m, k = lhs.shape
        first_done = None
        for _ in range(-(-rhs.shape[1] // LB)):
            end = 0
            for _ in range(-(-k // LB)):
                mxu[nxt[0]] += m
                end = max(end, mxu[nxt[0]])
                nxt[0] = (nxt[0] + 1) % 4
            if first_done is None:
                first_done = end
        if pace:
            tl.append((first_done - m, first_done, r))
        return r

    def mm(lhs, rhs):
        k = lhs.shape[1]
        if rhs.shape[1] > LB:
            return mm1(lhs, rhs)
        r, k0 = None, 0
        while k0 < k:
            k1 = min(k, k0 + (4 - nxt[0]) * LB)
            part = mm1(lhs[:, k0:k1], rhs[k0:k1], pace=k1 - k0 > LB)
            r = part if r is None else r + part
            k0 = k1
        return r

    def at(t):
        if t is None or t < 0:
            return None
        t = min(t, now() - 1)
        best = None
        for (a, b, r) in tl:
            if a <= t and (best is None or min(b, t) > best[0]):
                row = int(min((t - a) / (b - a), 0.999) * (r.shape[0] // 8)) * 8
                best = (min(b, t), r, row)
        return None if best is None else best[1][best[2]:best[2] + 8, 0:LB]

    def strassen(lhs, rhs, k, order, split_last=False, head=0):
        m = [None] * 7

        def ops(p, k0, k1):
            flush(now())
            return lhs(p, k0, k1), rhs(p, k0, k1)

        if head:
            for p in order:
                m[p] = mm(*ops(p, 0, head * LB))
        for p in order:
            l, r = ops(p, head * LB, k)
            if split_last and p == order[-1]:
                kk = (-(-r.shape[0] // LB) - 2) * LB
                hm = l.shape[0] // 2
                hd = mm(l[:, :kk], r[:kk]) if kk else None
                tail = jnp.concatenate([mm(l[:hm, kk:], r[kk:]), mm(l[hm:, kk:], r[kk:])], axis=0)
                v = tail if hd is None else hd + tail
            else:
                v = mm(l, r)
            m[p] = v if m[p] is None else m[p] + v
        return m

    def put_sums(dst, sm, ro, z):
        for p, v in sm.items():
            dst[ro:ro + 8, _blk(SIDX[p])] = _pkz(v, z)

    def tsum(ld, r0, slot_, i, t0, dur):
        for g in range(LB // 16):
            z = _zero(at(t0 + g * dur // 8))
            t1 = ld(slice(r0 + g * 16, r0 + g * 16 + 16)).astype(f32)
            t2 = ld(slice(r0 + LB + g * 16, r0 + LB + g * 16 + 16)).astype(f32)
            sm = _rhs_sums(t1[:, :LB], t1[:, LB:], t2[:, :LB], t2[:, LB:])
            put_sums(rs_s, sm, slot_ * RSK + i * (LB // 2) + g * 8, z)
        ready.add(("rs", slot_, i))

    def osum(slot_, t0, dur):
        ng = HD // 16
        for g in range(ng):
            z = _zero(at(t0 + g * dur // ng))
            r1, r2 = slot_ * HD + g * 8, slot_ * HD + QD + g * 8
            sm = _rhs_sums(_upf(ol_s[r1:r1 + 8, 0:LB]), _upf(ol_s[r1:r1 + 8, LB:]),
                           _upf(ol_s[r2:r2 + 8, 0:LB]), _upf(ol_s[r2:r2 + 8, LB:]))
            put_sums(rs_s, sm, slot_ * RSK + F // 4 + g * 8, z)
        ready.update({("rs", slot_, NFP), ("rs", slot_, NFP + 1)})

    def stored_rhs(slot_, p, k0, k1):
        assert all(("rs", slot_, i) in ready for i in range(k0 // LB, -(-k1 // LB))), (slot_, k0, k1)
        return _up(rs_s[slot_ * RSK + k0 // 2:slot_ * RSK + k1 // 2, _blk(SIDX[p])])

    def wrows(hh, g):
        p, d = divmod(2 * g, DH)
        out = []
        for kh in range(2):
            t = [jnp.concatenate([wt_s[2 * kh + c, pl.ds(p * D + hh * HD + d + e, HH, stride=DH), :]
                                  for e in range(2)], axis=0) for c in range(2)]
            out.append(jnp.concatenate([t[0], t[1][:, 0:HD - LB]], axis=1))
        return out

    def prep_wqkv():
        done = set()
        ng = HA // 16

        def need(hh, p):
            lo = p * D + hh * HD
            for ct in range(lo // LB, -(-(lo + HD) // LB)):
                if ct in done:
                    continue
                done.add(ct)
                w = min(LB, 3 * D - ct * LB)
                for kh in range(2):
                    wT = wqkv_v[kh * HD:(kh + 1) * HD, ct * LB:ct * LB + w].astype(f32).T
                    wt_s[2 * kh, ct * LB:ct * LB + w, :] = wT[:, 0:LB]
                    wt_s[2 * kh + 1, ct * LB:ct * LB + w, 0:HD - LB] = wT[:, LB:HD]

        def put(p, g, v):
            lw_s[p * (HA // 2) + g * 8:p * (HA // 2) + g * 8 + 8, :] = _pk(v)

        for g in range(ng):
            need(0, 2 * g // DH)
            a11, a12 = wrows(0, g)
            put(2, g, a11)
            put(4, g, a11 + a12)
        for g in range(ng):
            need(1, 2 * g // DH)
            ops = _lhs_ops(*wrows(0, g), *wrows(1, g))
            for p in (1, 3, 0, 5, 6):
                put(p, g, ops[p])

    def prep_wo(t0):
        wo = wo_v[...].astype(f32) + _orz(jnp.zeros((8, LB), f32), _zero(at(t0)))[0:1, 0:1]
        for c in range(4):
            cw = min(LB, D - c * LB)
            wo_s[c, :, 0:cw] = wo[:, c * LB:c * LB + cw]
        for hh in range(2):
            for d in range(DH):
                r = hh * HD + d * HH
                for c in range(4):
                    cw = min(LB, D - c * LB)
                    t = wo_s[c, pl.ds(hh * HD + d, HH, stride=DH), :]
                    wo2_s[r:r + HH, c * LB:c * LB + cw] = t[:, 0:cw]
        w1t, w2t = wo2_s[0:HD, :].T, wo2_s[HD:D, :].T
        for p, v in enumerate(_lhs_ops(w1t[0:HD], w2t[0:HD], w1t[HD:D], w2t[HD:D])):
            lc_s[p * QD:(p + 1) * QD, F // 2:KC] = _pk(v)
        ready.add(("lc", NFP))

    RG = 16
    NG = D // RG
    stat2 = {}

    def ln(b, t0=None, dur=None):
        def dep(fr):
            return None if t0 is None else at(t0 + fr * dur)

        def xg(g):
            return x_v[b // 2, g * RG:(g + 1) * RG, _blk(b % 2)].astype(f32)

        def halves(*vs):
            return [] if vs[0] is None else [v[i * 8:i * 8 + 8] for v in vs for i in range(2)]

        x0 = jnp.broadcast_to(xg(0)[0:1], (8, LB))
        s = q = None
        for g in range(NG):
            if g % P["LNQ1"] == 0 and t0 is not None:
                x0 = _orz(x0, _zero(dep(P["LNA"] * g / NG), *halves(s, q)))
            c = xg(g) - _x2(x0)
            s = c if s is None else s + c
            q = c * c if q is None else q + c * c
        dm = _rowsum8(s) * (1.0 / D)
        mu = x0 + dm
        r1 = lax.rsqrt(jnp.maximum(_rowsum8(q) * (1.0 / D) - dm * dm, 0.0) + EPS)
        s1 = s2 = z = None
        for g in range(NG):
            if g % P["LNQ3"] == 0 and t0 is not None:
                z = _zero(dep(P["LNB"] + P["LNBD"] * g / NG), *halves(s1, s2))
            xn = (xg(g) - _x2(mu)) * _x2(r1)
            xnT_s[g * 8:g * 8 + 8, _blk(b)] = _pkz(xn, z)
            s1 = xn if s1 is None else s1 + xn
            s2 = xn * xn if s2 is None else s2 + xn * xn
        mu2 = _rowsum8(s1) * (1.0 / D)
        var2 = jnp.maximum(_rowsum8(s2) * (1.0 / D) - mu2 * mu2, 0.0)
        stat2[b] = (mu2, lax.rsqrt(var2 + EPS))

    def hpair(b, t0=None, dur=None):
        ng = HD // RG
        st = [stat2.pop(b), stat2.pop(b + 1)]
        for g in range(ng):
            t = None if t0 is None else t0 + g * dur // ng
            zi = _zero(at(None if t is None else t - P["HG"]))
            z = _zero(at(t))
            xq, hq = [], []
            for r in (g * 8, QD + g * 8):
                for e in range(2):
                    xn = _upf(_orz(xnT_s[r:r + 8, _blk(b + e)], zi))
                    xq.append(xn)
                    hq.append((xn - _x2(st[e][0])) * _x2(st[e][1]))
            put_sums(ra_s, _rhs_sums(*xq), (b // 2) * QD + g * 8, z)
            if b < UB0:
                for n, v in enumerate(hq):
                    r = (n // 2) * QD + g * 8
                    hT_s[r:r + 8, _blk(b + n % 2)] = _pkz(v, z)
            else:
                for p, v in enumerate(_lhs_ops(*hq)):
                    lh_s[p * QD + g * 8:p * QD + g * 8 + 8, _blk((b - UB0) // 2)] = _pkz(v, z)
        ready.add(("xn", b))

    def stage_u(b0, b1, n0=0, n1=NFB):
        rows = slice(b0 * LB, b1 * LB)
        step = max(1, 4 // (b1 - b0))
        for n in range(n0, n1, step):
            cs = slice(n * LB, min(n + step, n1) * LB)
            r = mm(_up(hT_s[:, rows]), w1_v[rows, cs])
            if b0 == 0:
                u_s[:, cs] = r
            else:
                u_s[:, cs] += r

    def u_epilogue(i, m, g0, g1, t0, dur):
        c0, c1 = _blk(2 * i), _blk(2 * i + 1)
        for g in range(g0, g1):
            z = _zero(at(t0 + (g - g0) * dur // (g1 - g0)))
            bia = [b1_v[2 * i + e:2 * i + e + 1, :].astype(f32) for e in range(2)]
            top, bot = slice(g * 16, g * 16 + 16), slice(HD + g * 16, HD + g * 16 + 16)
            q = _combine([x[top] for x in m])
            gl = [_gelu(q[0] + (u_s[top, c0] + bia[0])), _gelu(q[1] + (u_s[top, c1] + bia[1])),
                  _gelu(q[2] + (u_s[bot, c0] + bia[0])), _gelu(q[3] + (u_s[bot, c1] + bia[1]))]
            for p, v in enumerate(_lhs_ops(*gl)):
                lc_s[p * QD + g * 8:p * QD + g * 8 + 8, _blk(i)] = _pkz(v, z)
        if g1 == HD // 16:
            ready.add(("lc", i))

    def stage_u_last(i, order, edur):
        def lhs(p, k0, k1):
            return _up(lh_s[p * QD:(p + 1) * QD, k0:k1])

        def rhs(p, k0, k1):
            if p in SIDX:
                return stored_rhs(i % 3, p, k0, k1)
            e = 0 if p == 1 else 1
            return _cat([w1_v[_blk(UB0 + 2 * k + e), _blk(2 * i + e)] for k in range(k0 // LB, k1 // LB)], 0)
        m = strassen(lhs, rhs, NUP * LB, order)
        for k in range(NUP):
            ready.discard(("rs", i % 3, k))
        t = now() - P["UE0"]
        ng = HD // 16
        add_tasks([(t + (g + 2) * edur // ng, u_epilogue, (i, m, g, g + 2, t + g * edur // ng, 2 * edur // ng))
                   for g in range(0, ng, 2)])

    def stage_a(b, odd=False, split_last=False):
        def lhs(p, k0, k1):
            return _up(lw_s[p * (HA // 2):(p + 1) * (HA // 2), :])

        def rhs(p, k0, k1):
            assert ("xn", b) in ready
            if p in SIDX:
                return _up(ra_s[(b // 2) * QD:(b // 2 + 1) * QD, _blk(SIDX[p])])
            return _up(xnT_s[0:QD, _blk(b)] if p == 1 else xnT_s[QD:HD, _blk(b + 1)])
        order = (6, 4, 2, 1, 3, 0, 5) if odd else (4, 2, 1, 3, 0, 5, 6)
        q = _combine(strassen(lhs, rhs, HD, order, split_last))
        for hh in range(2):
            for e in range(2):
                qk_s[b + e + 1, hh * D:(hh + 1) * D, :] = q[2 * hh + e][0:D]
                v_s[b + e + 1, hh * HD:(hh + 1) * HD, :] = q[2 * hh + e][D:HA]
        ready.update({("qkv", b), ("qkv", b + 1)})

    lane0 = lax.broadcasted_iota(i32, (HH, LB), 1)
    lane2 = 2 * lane0
    zeros8 = jnp.zeros((HH, LB), f32)

    def mk_shift(*deps):
        deps = [d for d in deps if d is not None]
        lane = lane2
        if deps:
            bits = pltpu.bitcast(deps[0], u32)
            for d in deps[1:]:
                bits = bits | pltpu.bitcast(d, u32)
            lane = lane2 | pltpu.bitcast(lax.shift_right_logical(bits, jnp.uint32(31)), i32)

        def fwd(cur, prev, sh):
            if sh == 0:
                return cur
            return pltpu.roll(jnp.where(lane < 2 * (LB - sh), cur, prev), sh, 1)

        def bwd(cur, nxt_):
            return pltpu.roll(jnp.where(lane >= 2 * SH, cur, nxt_), LB - SH, 1)
        return fwd, bwd

    def grp_shift(t):
        deps = [at(t)]
        if P["L"] and len(hist) >= P["L"]:
            deps += hist[-P["L"]]
        return mk_shift(*deps)

    raw, probs = {}, {}

    def attn_qk(j, hh, t, bd):
        jn = min(j + 1, NB - 1)
        assert ("qkv", jn) in ready
        acc = [None] * WH
        accp = [None] * WH
        for d in range(DH):
            if d % P["G"] == 0:
                if d > 0:
                    hist.append(acc + accp)
                fwd, bwd = grp_shift(t + d * bd // DH)
            r = hh * D + d * HH
            q = qk_s[j + 1, r:r + HH, :]
            qp = bwd(q, qk_s[jn + 1, r:r + HH, :])
            k = qk_s[j + 1, HD + r:HD + r + HH, :]
            kp = qk_s[j, HD + r:HD + r + HH, :] if j > 0 else zeros8
            for a in range(WH):
                ks = fwd(k, kp, DIL * a)
                t0, t1 = q * ks, qp * ks
                acc[a] = t0 if d == 0 else acc[a] + t0
                accp[a] = t1 if d == 0 else accp[a] + t1
        hist.append(acc + accp)
        raw[j, hh] = (acc, accp)

    def attn_sm(j, hh, t):
        fwd, _ = mk_shift(at(t))
        acc, accp = raw[j, hh]
        prev = raw.pop((j - 1, hh))[1] if j > 0 else [zeros8] * WH
        lg = acc + [fwd(accp[a], prev[a], SH) for a in range(WH)]
        lg = [a * SCALE for a in lg]
        if j == 0:
            lg = [lg[0]] + [jnp.where(lane0 >= DIL * w, lg[w], -1e9) for w in range(1, W)]
        m = lg[0]
        for w in range(1, W):
            m = jnp.maximum(m, lg[w])
        e = [jnp.exp(l - m) for l in lg]
        den = e[0]
        for w in range(1, W):
            den = den + e[w]
        inv = 1.0 / den
        p = [x * inv for x in e]
        for a in range(WH):
            pr_s[j, (hh * W + a) * HH:(hh * W + a + 1) * HH, :] = p[a]
        probs[j, hh] = p[WH:]

    def attn_pp(j, hh, t):
        _, bwd = mk_shift(at(t))
        p = probs.pop((j, hh))
        pn = probs[j + 1, hh] if j + 1 < NB else p
        for a in range(WH):
            pr_s[j, (hh * W + WH + a) * HH:(hh * W + WH + a + 1) * HH, :] = bwd(p[a], pn[a])
        ready.add(("pr", j, hh))

    def attn_pv(j, hh, slot_, e, t, bd, t_dl):
        assert not isinstance(j, int) or ("pr", j, hh) in ready
        pa = [pr_s[j, (hh * W + a) * HH:(hh * W + a + 1) * HH, :] for a in range(W)]
        p, pp = pa[:WH], pa[WH:]
        outs = []
        for d2 in range(DH // 2):
            os_ = []
            for d in (2 * d2, 2 * d2 + 1):
                if d % P["G"] == 0:
                    if d > 0:
                        hist.append([])
                    fwd, _ = grp_shift(t + d * bd // DH)
                r = hh * HD + d * HH
                v = v_s[j + 1, r:r + HH, :]
                vp = v_s[j, r:r + HH, :]
                o = op = None
                for a in range(WH):
                    vs = fwd(v, vp, DIL * a)
                    o = p[a] * vs if a == 0 else o + p[a] * vs
                    op = pp[a] * vs if a == 0 else op + pp[a] * vs
                opp = zeros8 if (isinstance(j, int) and j == 0) else op_s[r:r + HH, :]
                op_s[r:r + HH, :] = op
                os_.append(o + fwd(op, opp, SH))
            ro = slot_ * HD + hh * QD + d2 * HH
            ol_s[ro:ro + HH, _blk(e)] = _pk(jnp.concatenate(os_, axis=0))
            outs += os_
        hist.append([])
        bits = pltpu.bitcast(outs[0], u32)
        for o in outs[1:]:
            bits = bits | pltpu.bitcast(o, u32)
        dls.append((t_dl, bits))

    mains = [("qk", j, hh) for j in range(NB) for hh in range(2)]
    mains = (mains[:P["PVPOS"]] + [("pv", j, hh) for j in range(2) for hh in range(2)]
             + mains[P["PVPOS"]:] + [None, None])
    slot_ctr = [0]

    def slot(t, bd):
        n = slot_ctr[0]
        slot_ctr[0] += 1
        it = mains[n]
        if it is None:
            pass
        elif it[0] == "qk":
            attn_qk(it[1], it[2], t, bd)
        else:
            attn_pv(it[1], it[2], 1, it[1], t, bd, t + bd + P["PVL"])
        if n >= 1 and mains[n - 1] is not None and mains[n - 1][0] == "qk":
            attn_sm(mains[n - 1][1], mains[n - 1][2], t + P["LS"])
        if n >= 2 and mains[n - 2] is not None and mains[n - 2][0] == "qk":
            _, j, hh = mains[n - 2]
            if j > 0:
                attn_pp(j - 1, hh, t + P["PP"])
            if j == NB - 1:
                attn_pp(j, hh, t + P["PP"])

    NPRE = 2
    NPC = 3

    def out_copy(pidx, e0, e1, r0, r1):
        off = pidx * (2 * LB) + e0 * LB
        if not isinstance(pidx, int):
            off = pl.multiple_of(off, LB)
        rs = pl.ds(r0, r1 - r0)
        return pltpu.make_async_copy(out_v.at[pidx, rs, pl.ds(e0 * LB, (e1 - e0) * LB)],
                                     out_hbm.at[0, rs, pl.ds(off, (e1 - e0) * LB)], sems.at[0])

    def out_parts(fine):
        return [(1, 2, 0, HD), (0, 2, HD, D), (0, 1, 0, HD)] if fine else [(0, 2, 0, D)]

    def piece(pidx, sl, pn, fine=False, head=0, nqk=0):
        sn = (sl + 1) % 3
        t0 = now()

        def lhs(p, k0, k1):
            assert all(("lc", i) in ready for i in range(k0 // LB, min(NFP + 1, -(-k1 // LB)))), (k0, k1)
            return _up(lc_s[p * QD:(p + 1) * QD, k0:k1])

        def rhs(p, k0, k1):
            if p in SIDX:
                return stored_rhs(sl, p, k0, k1)
            e = 0 if p == 1 else 1
            parts = [w2_v[pidx, _blk(2 * i + e), _blk(e)] for i in range(k0 // LB, min(NFP, k1 // LB))]
            if k1 == KC:
                parts.append(_up(ol_s[sl * HD + e * QD:sl * HD + (e + 1) * QD, _blk(e)]))
            return _cat(parts, 0)
        todo = []
        for i in range(NFP):
            tt = t0 + P["TS0"] + i * P["TSD"]
            todo.append((tt + P["TSD"], tsum, (lambda rs: w2_v[pn, rs, :], 2 * i * LB, sn, i, tt, P["TSD"])))
        t = t0 + P["PV0"]
        pvd, pvb = (P["PVD"], P["PVB"]) if nqk == 0 else (P["PVD2"], P["PVD2"])
        for _ in range(nqk):
            todo.append((t + pvd, slot, (t, pvd)))
            t += pvd if mains[slot_plan[0]] is not None else 0
            slot_plan[0] += 1
        for e in range(2):
            for hh in range(2):
                todo.append((t + pvb, attn_pv, (pn * 2 + e, hh, sn, e, t, pvb, t + pvb + P["PVL"])))
                t += pvd
        todo.append((t0 + P["OS0"] + P["OSD"], osum, (sn, t0 + P["OS0"], P["OSD"])))
        add_tasks(todo)
        q = _combine(strassen(lhs, rhs, KC, P["CORD"], head=head))
        flush()
        for (e0, e1, r0, r1) in out_parts(fine):
            cols = slice(e0 * LB, e1 * LB)
            for h0 in range(r0, r1, HD):
                y = _cat([q[2 * (h0 // HD) + e] for e in range(e0, e1)], 1)
                o = y + b2f_s[pidx, 0:1, cols] + x_v[pidx, h0:h0 + HD, cols].astype(f32)
                out_v[pidx, h0:h0 + HD, cols] = o.astype(bf16)
            out_copy(pidx, e0, e1, r0, r1).start()

    def c_body(it, carry):
        reset()
        ready.update({("rs", 0, i) for i in range(NFP + 2)} | {("lc", i) for i in range(NFP + 1)})
        for c in range(NPC):
            pidx = NPRE + it * NPC + c
            piece(pidx, c, lax.rem(pidx + 1, NP), fine=c == NPC - 1)
        return carry

    x0 = Group(cp_x(0, 1))
    g1 = Group(cp_w1(0, 1))
    g2 = Group(cp_w1(1, 2) + cp_x(1, 2))
    g3 = Group(cp_w1(2, UB0))
    g4 = Group([(wqkv_hbm, wqkv_v)])
    g5 = Group(cp_x(2, NP))
    g6 = Group(cp_w1(UB0, NB) + [(wo_hbm, wo_v), (b1_hbm, b1_v), (b2_hbm, b2_v)] + cp_w2(0, NPRE + 1))
    g7 = Group(cp_w2(NPRE + 1, NP))
    for c in (x0, g1, g2, g3, g4, g5, g6, g7):
        c.start()

    v_s[0] = jnp.zeros((D, LB), f32)
    for buf in (xnT_s, ra_s, hT_s, lh_s, ol_s, rs_s):
        buf[0:8, 0:64] = jnp.zeros((8, 64), u32)

    LND, BD, MARG = P["LND"], P["BD"], P["MARG"]

    def ln_tasks(b, t):
        todo = []
        for fn, bb, dur, adv in ((ln, b, LND, 0.8), (ln, b + 1, LND, 0.86), (hpair, b, P["HSD"], 1.0)):
            todo.append((t + int(dur * adv), fn, (bb, t, dur)))
            t += int(dur * adv)
        return todo, t

    wait("x0", x0)
    ln(0); ln(1); hpair(0)
    wait("r1", g1)
    stage_u(0, 1, 0, 12)
    wait("r2", g2)
    add_tasks(ln_tasks(2, 0)[0])
    stage_u(0, 2, 12, NFB)
    stage_u(1, 2, 0, 12)
    wait("r3", g3)
    stage_u(2, 4, 0, P["N3"])
    wait("wqkv", g4)
    stage_u(2, 4, P["N3"], NFB)
    prep_wqkv()
    stage_a(0, split_last=True)
    wait("mid", g5)
    AD = 7 * HA // 2
    UD = 7 * NUP * HD // 4
    r5 = (NP - 1) * AD
    t = 0
    for b in range(UB0, NB, 2):
        todo, t = ln_tasks(b, t)
        add_tasks(todo)
    n5 = 0
    while t + BD + MARG <= r5:
        add_tasks([(t + BD, slot, (t, BD))])
        t += BD
        n5 += 1
    for n, b in enumerate(range(2, NB, 2)):
        stage_a(b, odd=n % 2 == 1, split_last=b == NB - 2)
    wait("fin", g6)
    r6 = NFP * UD
    todo = []
    for i in range(NFP + 1):
        if i == 0:
            t0, dt = -200, 130
        elif i == 1:
            t0, dt = 700, 260
        else:
            t0, dt = (i - 1) * UD + P["US0"], P["USD"]
        if i < NFP:
            for k in range(NUP):
                tt = t0 + k * dt
                todo.append((tt + dt, tsum, (lambda rs, i=i: w1_v[rs, 2 * i * LB:(2 * i + 2) * LB],
                                             (UB0 + 2 * k) * LB, i % 3, k, tt, dt)))
        else:
            for k in range(NFP):
                tt = t0 + k * 300
                todo.append((tt + 300, tsum, (lambda rs: w2_v[0, rs, :], 2 * k * LB, 1, k, tt, 300)))
    left = len(mains) - n5 - P["NQ0"] - P["NQ1"]
    slot_plan = [n5 + left]
    t = P["R6S"]
    bd2 = (r6 - t) // left
    for _ in range(left):
        todo.append((t + min(bd2, 600), slot, (t, min(bd2, 600))))
        t += bd2
    todo.append((r6 - 100, osum, (1, r6 - 500, 400)))
    todo.append((P["PW0"] + 1, prep_wo, (P["PW0"],)))
    add_tasks(todo)
    for b in range(NB):
        b2f_s[b // 2, 0:1, _blk(b % 2)] = b2_v[b:b + 1, :].astype(f32)
    for i in range(NFP):
        stage_u_last(i, (1, 4, 2, 3, 0, 5, 6) if i == 0 else P["UORD"], P["UED"] if i < NFP - 1 else P["UEL"])
    piece(0, 1, 1, head=4, nqk=P["NQ0"])
    piece(1, 2, 2, nqk=P["NQ1"])
    assert slot_ctr[0] == len(mains)
    wait("w2", g7)

    lax.fori_loop(0, 2, c_body, 0)
    outs = [out_copy(pidx, *part) for pidx in range(NP)
            for part in out_parts(pidx >= NPRE and (pidx - NPRE) % NPC == NPC - 1)]
    wait("out", *outs)


@jax.jit
def pallas_parallel_sum__sliding_local_dilated__mixer_token_mlp__prompt_kernel(A_x, A_wqkv, A_wo, B_x, B_w1, B_b1, B_w2, B_b2):
    del B_x
    hbm = pl.BlockSpec(memory_space=pltpu.HBM)
    outT = pl.pallas_call(
        _kernel,
        out_shape=jax.ShapeDtypeStruct((1, D, S), bf16),
        in_specs=[hbm] * 7,
        out_specs=hbm,
        scratch_shapes=[
            pltpu.VMEM((NP, D, 2 * LB), bf16),
            pltpu.VMEM((D, 3 * D), bf16),
            pltpu.VMEM((D, D), bf16),
            pltpu.VMEM((S, F), bf16),
            pltpu.VMEM((NP, F, 2 * LB), bf16),
            pltpu.VMEM((NFB, LB), bf16),
            pltpu.VMEM((NB, LB), bf16),
            pltpu.VMEM((NP, D, 2 * LB), bf16),
            pltpu.VMEM((4, 3 * D, LB), f32),
            pltpu.VMEM((7 * HA // 2, HD), u32),
            pltpu.VMEM((4, D, LB), f32),
            pltpu.VMEM((D, D), f32),
            pltpu.VMEM((HD, S), u32),
            pltpu.VMEM((NP * QD, 5 * LB), u32),
            pltpu.VMEM((HD, UB0 * LB), u32),
            pltpu.VMEM((7 * QD, NUP * LB), u32),
            pltpu.VMEM((D, F), f32),
            pltpu.VMEM((7 * QD, KC), u32),
            pltpu.VMEM((NB + 1, 2 * D, LB), f32),
            pltpu.VMEM((NB + 1, D, LB), f32),
            pltpu.VMEM((NB, 2 * W * HH, LB), f32),
            pltpu.VMEM((3 * HD, 2 * LB), u32),
            pltpu.VMEM((D, LB), f32),
            pltpu.VMEM((NP, 32, 2 * LB), f32),
            pltpu.VMEM((3 * RSK, 5 * LB), u32),
            pltpu.SemaphoreType.DMA((9,)),
        ],
        compiler_params=pltpu.CompilerParams(vmem_limit_bytes=100 * 1024 * 1024,
                                             disable_bounds_checks=True,
                                             disable_semaphore_checks=True),
    )(jnp.swapaxes(A_x, 1, 2), A_wqkv, A_wo, B_w1, B_b1.reshape(NFB, LB), B_w2, B_b2.reshape(NB, LB))
    return jnp.swapaxes(outT, 1, 2)
```

```python
import jax
import jax.numpy as jnp
from jax import lax
import jax.experimental.pallas as pl
import jax.experimental.pallas.tpu as pltpu

S, D, F = 2048, 448, 1792
H, DH, W, DIL = 16, 28, 8, 2
LB = 128
NB = S // LB
NP = NB // 2
NFB = F // LB
NFP = NFB // 2
HH = H // 2
WH = W // 2
SH = DIL * WH
HD = D // 2
QD = D // 4
HA = 3 * HD
UB0 = 4
NUP = (NB - UB0) // 2
KC = F // 2 + HD
RSK = (NFP + 2) * LB // 2
EPS = 1e-5
SCALE = DH ** -0.5
f32 = jnp.float32
bf16 = jnp.bfloat16
u32 = jnp.uint32
i32 = jnp.int32

SCOPES = False
P = dict(LND=640, BD=440, G=4, L=4, LS=170, PP=150, MARG=300, N3=10, PVD=680, PV0=50, HSD=560, HG=80,
         CORD=(4, 2, 1, 3, 0, 5, 6), TS0=100, TSD=420, PVB=520, PVL=500, OS0=3050, OSD=300,
         UORD=(4, 2, 1, 3, 0, 5, 6), US0=100, USD=350, R6S=1800, PVPOS=16, PVD2=400, NQ0=1, NQ1=5, HL=250,
         UE0=-200, UED=2100, UEL=1300, PW0=-1000, PWD=400, UG=50, UM=24, PWL=2100, SK0=900, LNQ1=4, LNQ3=4, LNA=0.3, LNB=0.42, LNBD=0.33)


def _gelu(x, z=None):
    c = 0.7978845608028654
    hx = 0.5 * x
    return hx + hx * jnp.tanh(_orz(x * (c + (c * 0.044715) * (x * x)), z))


def _pk(x):
    return pltpu.bitcast(x.astype(bf16), u32)


def _up(x):
    return pltpu.bitcast(x, bf16)


def _upf(x):
    return pltpu.bitcast(x, bf16).astype(f32)


def _cat(xs, axis):
    return xs[0] if len(xs) == 1 else jnp.concatenate(xs, axis=axis)


def _x2(v):
    return jnp.concatenate([v, v], axis=0)


def _blk(b):
    return slice(b * LB, (b + 1) * LB)


def _rowsum8(a):
    return jnp.broadcast_to(jnp.sum(a, axis=0, keepdims=True), (8, a.shape[1]))


def _zero(*deps):
    deps = [d for d in deps if d is not None]
    if not deps:
        return None
    bits = pltpu.bitcast(deps[0], u32)
    for d in deps[1:]:
        bits = bits | pltpu.bitcast(d, u32)
    return lax.shift_right_logical(lax.shift_right_logical(bits, jnp.uint32(31)), jnp.uint32(1))


def _orz(v, z):
    return v if z is None else pltpu.bitcast(pltpu.bitcast(v, u32) | z, v.dtype)


def _pkz(v, z):
    return _pk(v if z is None else jnp.concatenate([_orz(v[0:8], z), v[8:16]], axis=0))


def _lhs_ops(a11, a12, a21, a22):
    return [a11 + a22, a21 + a22, a11, a22, a11 + a12, a21 - a11, a12 - a22]


SIDX = {0: 0, 2: 1, 3: 2, 5: 3, 6: 4}


def _rhs_sums(b11, b12, b21, b22):
    return {0: b11 + b22, 2: b12 - b22, 3: b21 - b11, 5: b11 + b12, 6: b21 + b22}


def _combine(m):
    c12 = m[2] + m[4]
    c21 = m[1] + m[3]
    x = (m[2] - m[1]) + m[0]
    return ((x + m[6]) + (c21 - c12), c12, c21, x + m[5])


def _kernel(x_hbm, wqkv_hbm, wo_hbm, w1_hbm, b1_hbm, w2_hbm, b2_hbm, out_hbm,
            x_v, wqkv_v, wo_v, w1_v, w2_v, b1_v, b2_v, out_v,
            wt_s, lw_s, wo_s, xnT_s, ra_s, hT_s, lh_s, u_s, lc_s, qk_s, v_s, pr_s, ol_s, op_s,
            b2f_s, rs_s, sems):
    sem_ctr = [1]

    class Group:
        def __init__(self, pairs):
            self.cps = [pltpu.make_async_copy(a, b, sems.at[sem_ctr[0]]) for (a, b) in pairs]
            sem_ctr[0] += 1

        def start(self):
            for c in self.cps:
                c.start()

        def wait(self):
            for c in self.cps:
                c.wait()

    def cp_x(p0, p1):
        return [(x_hbm.at[0, :, pl.ds(p * 2 * LB, 2 * LB)], x_v.at[p]) for p in range(p0, p1)]

    def cp_w2(p0, p1):
        return [(w2_hbm.at[:, pl.ds(p * 2 * LB, 2 * LB)], w2_v.at[p]) for p in range(p0, p1)]

    def cp_w1(b0, b1):
        sl = pl.ds(b0 * LB, (b1 - b0) * LB)
        return [(w1_hbm.at[sl, :], w1_v.at[sl, :])]

    tl = []
    mxu = [0, 0, 0, 0]
    nxt = [0]
    hist = []
    tasks = []
    dls = []
    ready = set()

    def add_tasks(todo):
        tasks.extend(todo)
        tasks.sort(key=lambda x: x[0])

    def flush(t=None):
        while tasks and (t is None or tasks[0][0] < t):
            _, fn, args = tasks.pop(0)
            fn(*args)

    def reset():
        assert not tasks
        dls.clear()
        tl.clear()
        hist.clear()
        mxu[:] = [0, 0, 0, 0]
        nxt[0] = 0

    def now():
        return sum(mxu) // 4

    def wait(name, *cps):
        flush()
        if SCOPES:
            with jax.named_scope("wait_" + name):
                for c in cps:
                    c.wait()
        else:
            for c in cps:
                c.wait()
        reset()

    def mm1(lhs, rhs, pace=True):
        flush(now())
        start = mxu[nxt[0]]
        due = [v for (t, v) in dls if t <= start] if pace else []
        if due:
            dls[:] = [(t, v) for (t, v) in dls if t > start]
            tile = _up(pltpu.bitcast(lhs[0:16, 0:LB], u32) | _zero(*due))
            row = tile if lhs.shape[1] == LB else jnp.concatenate([tile, lhs[0:16, LB:]], axis=1)
            lhs = jnp.concatenate([row, lhs[16:]], axis=0)
        r = jnp.dot(lhs, rhs, preferred_element_type=f32)
        m, k = lhs.shape
        first_done = None
        for _ in range(-(-rhs.shape[1] // LB)):
            end = 0
            for _ in range(-(-k // LB)):
                mxu[nxt[0]] += m
                end = max(end, mxu[nxt[0]])
                nxt[0] = (nxt[0] + 1) % 4
            if first_done is None:
                first_done = end
        if pace:
            tl.append((first_done - m, first_done, r))
        return r

    def mm(lhs, rhs):
        k = lhs.shape[1]
        if rhs.shape[1] > LB:
            return mm1(lhs, rhs)
        r, k0 = None, 0
        while k0 < k:
            k1 = min(k, k0 + (4 - nxt[0]) * LB)
            part = mm1(lhs[:, k0:k1], rhs[k0:k1], pace=k1 - k0 > LB)
            r = part if r is None else r + part
            k0 = k1
        return r

    def at(t):
        if t is None or t < 0:
            return None
        t = min(t, now() - 1)
        best = None
        for (a, b, r) in tl:
            if a <= t and (best is None or min(b, t) > best[0]):
                row = int(min((t - a) / (b - a), 0.999) * (r.shape[0] // 8)) * 8
                best = (min(b, t), r, row)
        return None if best is None else best[1][best[2]:best[2] + 8, 0:LB]

    def strassen(lhs, rhs, k, order, split_last=False, head=0):
        m = [None] * 7

        def ops(p, k0, k1):
            flush(now())
            return lhs(p, k0, k1), rhs(p, k0, k1)

        if head:
            for p in order:
                m[p] = mm(*ops(p, 0, head * LB))
        for p in order:
            l, r = ops(p, head * LB, k)
            if split_last and p == order[-1]:
                kk = (-(-r.shape[0] // LB) - 2) * LB
                hm = l.shape[0] // 2
                hd = mm(l[:, :kk], r[:kk]) if kk else None
                tail = jnp.concatenate([mm(l[:hm, kk:], r[kk:]), mm(l[hm:, kk:], r[kk:])], axis=0)
                v = tail if hd is None else hd + tail
            else:
                v = mm(l, r)
            m[p] = v if m[p] is None else m[p] + v
        return m

    def put_sums(dst, sm, ro, z):
        for p, v in sm.items():
            dst[ro:ro + 8, _blk(SIDX[p])] = _pkz(v, z)

    def tsum(ld, r0, slot_, i, t0, dur):
        for g in range(LB // 16):
            z = _zero(at(t0 + g * dur // 8))
            t1 = ld(slice(r0 + g * 16, r0 + g * 16 + 16)).astype(f32)
            t2 = ld(slice(r0 + LB + g * 16, r0 + LB + g * 16 + 16)).astype(f32)
            sm = _rhs_sums(t1[:, :LB], t1[:, LB:], t2[:, :LB], t2[:, LB:])
            put_sums(rs_s, sm, slot_ * RSK + i * (LB // 2) + g * 8, z)
        ready.add(("rs", slot_, i))

    def osum(slot_, t0, dur):
        ng = HD // 16
        for g in range(ng):
            z = _zero(at(t0 + g * dur // ng))
            r1, r2 = slot_ * HD + g * 8, slot_ * HD + QD + g * 8
            sm = _rhs_sums(_upf(ol_s[r1:r1 + 8, 0:LB]), _upf(ol_s[r1:r1 + 8, LB:]),
                           _upf(ol_s[r2:r2 + 8, 0:LB]), _upf(ol_s[r2:r2 + 8, LB:]))
            put_sums(rs_s, sm, slot_ * RSK + F // 4 + g * 8, z)
        ready.update({("rs", slot_, NFP), ("rs", slot_, NFP + 1)})

    def stored_rhs(slot_, p, k0, k1):
        assert all(("rs", slot_, i) in ready for i in range(k0 // LB, -(-k1 // LB))), (slot_, k0, k1)
        return _up(rs_s[slot_ * RSK + k0 // 2:slot_ * RSK + k1 // 2, _blk(SIDX[p])])

    def wrows(hh, g):
        p, d = divmod(2 * g, DH)
        out = []
        for kh in range(2):
            t = [jnp.concatenate([wt_s[2 * kh + c, pl.ds(p * D + hh * HD + d + e, HH, stride=DH), :]
                                  for e in range(2)], axis=0) for c in range(2)]
            out.append(jnp.concatenate([t[0], t[1][:, 0:HD - LB]], axis=1))
        return out

    def prep_wqkv():
        done = set()
        ng = HA // 16

        def need(hh, p):
            lo = p * D + hh * HD
            for ct in range(lo // LB, -(-(lo + HD) // LB)):
                if ct in done:
                    continue
                done.add(ct)
                w = min(LB, 3 * D - ct * LB)
                for kh in range(2):
                    wT = wqkv_v[kh * HD:(kh + 1) * HD, ct * LB:ct * LB + w].astype(f32).T
                    wt_s[2 * kh, ct * LB:ct * LB + w, :] = wT[:, 0:LB]
                    wt_s[2 * kh + 1, ct * LB:ct * LB + w, 0:HD - LB] = wT[:, LB:HD]

        def put(p, g, v):
            lw_s[p * (HA // 2) + g * 8:p * (HA // 2) + g * 8 + 8, :] = _pk(v)

        for g in range(ng):
            need(0, 2 * g // DH)
            a11, a12 = wrows(0, g)
            put(2, g, a11)
            put(4, g, a11 + a12)
        for g in range(ng):
            need(1, 2 * g // DH)
            ops = _lhs_ops(*wrows(0, g), *wrows(1, g))
            for p in (1, 3, 0, 5, 6):
                put(p, g, ops[p])

    def prep_wo(t0, dur):
        for g in range(D // 16):
            w = wo_v[g * 16:g * 16 + 16, :].astype(f32)
            z = _zero(at(t0 + g * dur // (D // 16)))
            for c in range(4):
                cw = min(LB, D - c * LB)
                t = w[:, c * LB:c * LB + cw]
                if z is not None:
                    t = _orz(t, _x2(z)[:, 0:cw])
                wo_s[c, g * 16:g * 16 + 16, 0:cw] = t
        wt = []
        for hh in range(2):
            cols = []
            for c in range(4):
                cw = min(LB, D - c * LB)
                rows = [wo_s[c, pl.ds(hh * HD + d, HH, stride=DH), :][:, 0:cw] for d in range(DH)]
                cols.append(jnp.concatenate(rows, axis=0).astype(bf16).T.astype(f32))
            wt.append(jnp.concatenate(cols, axis=0))
        for p, v in enumerate(_lhs_ops(wt[0][0:HD], wt[1][0:HD], wt[0][HD:D], wt[1][HD:D])):
            lc_s[p * QD:(p + 1) * QD, F // 2:KC] = _pk(v)
        ready.add(("lc", NFP))
        got = lc_s[:, F // 2:F // 2 + LB]
        bits = got[0:8]
        for r in range(8, 7 * QD, 8):
            bits = bits | got[r:r + 8]
        dls.append((P["PWL"], bits))

    RG = 16
    NG = D // RG
    stat2 = {}

    def ln(b, t0=None, dur=None):
        def dep(fr):
            return None if t0 is None else at(t0 + fr * dur)

        def xg(g):
            return x_v[b // 2, g * RG:(g + 1) * RG, _blk(b % 2)].astype(f32)

        def halves(*vs):
            return [] if vs[0] is None else [v[i * 8:i * 8 + 8] for v in vs for i in range(2)]

        x0 = jnp.broadcast_to(xg(0)[0:1], (8, LB))
        s = q = None
        for g in range(NG):
            if g % P["LNQ1"] == 0 and t0 is not None:
                x0 = _orz(x0, _zero(dep(P["LNA"] * g / NG), *halves(s, q)))
            c = xg(g) - _x2(x0)
            s = c if s is None else s + c
            q = c * c if q is None else q + c * c
        dm = _rowsum8(s) * (1.0 / D)
        mu = x0 + dm
        r1 = lax.rsqrt(jnp.maximum(_rowsum8(q) * (1.0 / D) - dm * dm, 0.0) + EPS)
        s1 = s2 = z = None
        for g in range(NG):
            if g % P["LNQ3"] == 0 and t0 is not None:
                z = _zero(dep(P["LNB"] + P["LNBD"] * g / NG), *halves(s1, s2))
            xn = (xg(g) - _x2(mu)) * _x2(r1)
            xnT_s[g * 8:g * 8 + 8, _blk(b)] = _pkz(xn, z)
            s1 = xn if s1 is None else s1 + xn
            s2 = xn * xn if s2 is None else s2 + xn * xn
        mu2 = _rowsum8(s1) * (1.0 / D)
        var2 = jnp.maximum(_rowsum8(s2) * (1.0 / D) - mu2 * mu2, 0.0)
        stat2[b] = (mu2, lax.rsqrt(var2 + EPS))

    def hpair(b, t0=None, dur=None):
        ng = HD // RG
        st = [stat2.pop(b), stat2.pop(b + 1)]
        for g in range(ng):
            t = None if t0 is None else t0 + g * dur // ng
            zi = _zero(at(None if t is None else t - P["HG"]))
            z = _zero(at(t))
            xq, hq = [], []
            for r in (g * 8, QD + g * 8):
                for e in range(2):
                    xn = _upf(_orz(xnT_s[r:r + 8, _blk(b + e)], zi))
                    xq.append(xn)
                    hq.append((xn - _x2(st[e][0])) * _x2(st[e][1]))
            put_sums(ra_s, _rhs_sums(*xq), (b // 2) * QD + g * 8, z)
            if b < UB0:
                for n, v in enumerate(hq):
                    r = (n // 2) * QD + g * 8
                    hT_s[r:r + 8, _blk(b + n % 2)] = _pkz(v, z)
            else:
                for p, v in enumerate(_lhs_ops(*hq)):
                    lh_s[p * QD + g * 8:p * QD + g * 8 + 8, _blk((b - UB0) // 2)] = _pkz(v, z)
        ready.add(("xn", b))
        if t0 is not None and b >= UB0 and P["HL"]:
            got = ra_s[(b // 2) * QD:(b // 2 + 1) * QD, :]
            tiles_ = [got[r:r + 8, _blk(c)] for r in range(0, QD, 8) for c in range(5)]
            bits = tiles_[0]
            for v in tiles_[1:]:
                bits = bits | v
            dls.append((t0 + dur + P["HL"], bits))

    def stage_u(b0, b1, n0=0, n1=NFB):
        rows = slice(b0 * LB, b1 * LB)
        step = max(1, 4 // (b1 - b0))
        for n in range(n0, n1, step):
            cs = slice(n * LB, min(n + step, n1) * LB)
            r = mm(_up(hT_s[:, rows]), w1_v[rows, cs])
            if b0 == 0:
                u_s[:, cs] = r
            else:
                u_s[:, cs] += r

    def u_epilogue(i, m, g0, g1, t0, dur):
        c0, c1 = _blk(2 * i), _blk(2 * i + 1)
        for g in range(g0, g1):
            t = t0 + (g - g0) * dur // (g1 - g0)
            z = _zero(at(t))
            if P["UM"] == 0:
                zi = [_zero(at(t - P["UG"]))] * 4
            else:
                zi = [_zero(at(t - P["UG"] - (3 - n) * P["UM"])) for n in range(4)]
            zi = [None if v is None else _x2(v) for v in zi]
            bia = [b1_v[2 * i + e:2 * i + e + 1, :].astype(f32) for e in range(2)]
            top, bot = slice(g * 16, g * 16 + 16), slice(HD + g * 16, HD + g * 16 + 16)
            q = _combine([x[top] for x in m])
            gl = [_gelu(q[0] + (u_s[top, c0] + bia[0]), zi[3]), _gelu(q[1] + (u_s[top, c1] + bia[1]), zi[0]),
                  _gelu(q[2] + (u_s[bot, c0] + bia[0]), zi[1]), _gelu(q[3] + (u_s[bot, c1] + bia[1]), zi[2])]
            for p, v in enumerate(_lhs_ops(*gl)):
                lc_s[p * QD + g * 8:p * QD + g * 8 + 8, _blk(i)] = _pkz(v, z)
        if g1 == HD // 16:
            ready.add(("lc", i))

    def stage_u_last(i, order, edur):
        def lhs(p, k0, k1):
            return _up(lh_s[p * QD:(p + 1) * QD, k0:k1])

        def rhs(p, k0, k1):
            if p in SIDX:
                return stored_rhs(i % 3, p, k0, k1)
            e = 0 if p == 1 else 1
            return _cat([w1_v[_blk(UB0 + 2 * k + e), _blk(2 * i + e)] for k in range(k0 // LB, k1 // LB)], 0)
        m = strassen(lhs, rhs, NUP * LB, order)
        for k in range(NUP):
            ready.discard(("rs", i % 3, k))
        t = now() - P["UE0"]
        ng = HD // 16
        add_tasks([(t + (g + 2) * edur // ng, u_epilogue, (i, m, g, g + 2, t + g * edur // ng, 2 * edur // ng))
                   for g in range(0, ng, 2)])

    def stage_a(b, odd=False, split_last=False):
        def lhs(p, k0, k1):
            return _up(lw_s[p * (HA // 2):(p + 1) * (HA // 2), :])

        def rhs(p, k0, k1):
            assert ("xn", b) in ready
            if p in SIDX:
                return _up(ra_s[(b // 2) * QD:(b // 2 + 1) * QD, _blk(SIDX[p])])
            return _up(xnT_s[0:QD, _blk(b)] if p == 1 else xnT_s[QD:HD, _blk(b + 1)])
        order = (6, 4, 2, 1, 3, 0, 5) if odd else (4, 2, 1, 3, 0, 5, 6)
        q = _combine(strassen(lhs, rhs, HD, order, split_last))
        for hh in range(2):
            for e in range(2):
                qk_s[b + e + 1, hh * D:(hh + 1) * D, :] = q[2 * hh + e][0:D]
                v_s[b + e + 1, hh * HD:(hh + 1) * HD, :] = q[2 * hh + e][D:HA]
        ready.update({("qkv", b), ("qkv", b + 1)})

    lane0 = lax.broadcasted_iota(i32, (HH, LB), 1)
    lane2 = 2 * lane0
    zeros8 = jnp.zeros((HH, LB), f32)

    def mk_shift(*deps):
        deps = [d for d in deps if d is not None]
        lane = lane2
        if deps:
            bits = pltpu.bitcast(deps[0], u32)
            for d in deps[1:]:
                bits = bits | pltpu.bitcast(d, u32)
            lane = lane2 | pltpu.bitcast(lax.shift_right_logical(bits, jnp.uint32(31)), i32)

        def fwd(cur, prev, sh):
            if sh == 0:
                return cur
            return pltpu.roll(jnp.where(lane < 2 * (LB - sh), cur, prev), sh, 1)

        def bwd(cur, nxt_):
            return pltpu.roll(jnp.where(lane >= 2 * SH, cur, nxt_), LB - SH, 1)
        return fwd, bwd

    def grp_shift(t):
        deps = [at(t)]
        if P["L"] and len(hist) >= P["L"]:
            deps += hist[-P["L"]]
        return mk_shift(*deps)

    raw, probs = {}, {}

    def attn_qk(j, hh, t, bd):
        jn = min(j + 1, NB - 1)
        assert ("qkv", jn) in ready
        acc = [None] * WH
        accp = [None] * WH
        for d in range(DH):
            if d % P["G"] == 0:
                if d > 0:
                    hist.append(acc + accp)
                fwd, bwd = grp_shift(t + d * bd // DH)
            r = hh * D + d * HH
            q = qk_s[j + 1, r:r + HH, :]
            qp = bwd(q, qk_s[jn + 1, r:r + HH, :])
            k = qk_s[j + 1, HD + r:HD + r + HH, :]
            kp = qk_s[j, HD + r:HD + r + HH, :] if j > 0 else zeros8
            for a in range(WH):
                ks = fwd(k, kp, DIL * a)
                t0, t1 = q * ks, qp * ks
                acc[a] = t0 if d == 0 else acc[a] + t0
                accp[a] = t1 if d == 0 else accp[a] + t1
        hist.append(acc + accp)
        raw[j, hh] = (acc, accp)

    def attn_sm(j, hh, t):
        fwd, _ = mk_shift(at(t))
        acc, accp = raw[j, hh]
        prev = raw.pop((j - 1, hh))[1] if j > 0 else [zeros8] * WH
        lg = acc + [fwd(accp[a], prev[a], SH) for a in range(WH)]
        lg = [a * SCALE for a in lg]
        if j == 0:
            lg = [lg[0]] + [jnp.where(lane0 >= DIL * w, lg[w], -1e9) for w in range(1, W)]
        m = lg[0]
        for w in range(1, W):
            m = jnp.maximum(m, lg[w])
        e = [jnp.exp(l - m) for l in lg]
        den = e[0]
        for w in range(1, W):
            den = den + e[w]
        inv = 1.0 / den
        p = [x * inv for x in e]
        for a in range(WH):
            pr_s[j, (hh * W + a) * HH:(hh * W + a + 1) * HH, :] = p[a]
        probs[j, hh] = p[WH:]

    def attn_pp(j, hh, t):
        _, bwd = mk_shift(at(t))
        p = probs.pop((j, hh))
        pn = probs[j + 1, hh] if j + 1 < NB else p
        for a in range(WH):
            pr_s[j, (hh * W + WH + a) * HH:(hh * W + WH + a + 1) * HH, :] = bwd(p[a], pn[a])
        ready.add(("pr", j, hh))

    def attn_pv(j, hh, slot_, e, t, bd, t_dl):
        assert not isinstance(j, int) or ("pr", j, hh) in ready
        pa = [pr_s[j, (hh * W + a) * HH:(hh * W + a + 1) * HH, :] for a in range(W)]
        p, pp = pa[:WH], pa[WH:]
        outs = []
        for d2 in range(DH // 2):
            os_ = []
            for d in (2 * d2, 2 * d2 + 1):
                if d % P["G"] == 0:
                    if d > 0:
                        hist.append([])
                    fwd, _ = grp_shift(t + d * bd // DH)
                r = hh * HD + d * HH
                v = v_s[j + 1, r:r + HH, :]
                vp = v_s[j, r:r + HH, :]
                o = op = None
                for a in range(WH):
                    vs = fwd(v, vp, DIL * a)
                    o = p[a] * vs if a == 0 else o + p[a] * vs
                    op = pp[a] * vs if a == 0 else op + pp[a] * vs
                opp = zeros8 if (isinstance(j, int) and j == 0) else op_s[r:r + HH, :]
                op_s[r:r + HH, :] = op
                os_.append(o + fwd(op, opp, SH))
            ro = slot_ * HD + hh * QD + d2 * HH
            ol_s[ro:ro + HH, _blk(e)] = _pk(jnp.concatenate(os_, axis=0))
            outs += os_
        hist.append([])
        bits = pltpu.bitcast(outs[0], u32)
        for o in outs[1:]:
            bits = bits | pltpu.bitcast(o, u32)
        dls.append((t_dl, bits))

    mains = [("qk", j, hh) for j in range(NB) for hh in range(2)]
    mains = (mains[:P["PVPOS"]] + [("pv", j, hh) for j in range(2) for hh in range(2)]
             + mains[P["PVPOS"]:] + [None, None])
    slot_ctr = [0]

    def slot(t, bd):
        n = slot_ctr[0]
        slot_ctr[0] += 1
        it = mains[n]
        if it is None:
            pass
        elif it[0] == "qk":
            attn_qk(it[1], it[2], t, bd)
        else:
            attn_pv(it[1], it[2], 1, it[1], t, bd, t + bd + P["PVL"])
        if n >= 1 and mains[n - 1] is not None and mains[n - 1][0] == "qk":
            attn_sm(mains[n - 1][1], mains[n - 1][2], t + P["LS"])
        if n >= 2 and mains[n - 2] is not None and mains[n - 2][0] == "qk":
            _, j, hh = mains[n - 2]
            if j > 0:
                attn_pp(j - 1, hh, t + P["PP"])
            if j == NB - 1:
                attn_pp(j, hh, t + P["PP"])

    NPRE = 2
    NPC = 3

    def out_copy(pidx, e0, e1, r0, r1):
        off = pidx * (2 * LB) + e0 * LB
        if not isinstance(pidx, int):
            off = pl.multiple_of(off, LB)
        rs = pl.ds(r0, r1 - r0)
        return pltpu.make_async_copy(out_v.at[pidx, rs, pl.ds(e0 * LB, (e1 - e0) * LB)],
                                     out_hbm.at[0, rs, pl.ds(off, (e1 - e0) * LB)], sems.at[0])

    def out_parts(fine):
        return [(1, 2, 0, HD), (0, 2, HD, D), (0, 1, 0, HD)] if fine else [(0, 2, 0, D)]

    def piece(pidx, sl, pn, fine=False, head=0, nqk=0, tskip=0):
        sn = (sl + 1) % 3
        t0 = now()

        def lhs(p, k0, k1):
            assert all(("lc", i) in ready for i in range(k0 // LB, min(NFP + 1, -(-k1 // LB)))), (k0, k1)
            return _up(lc_s[p * QD:(p + 1) * QD, k0:k1])

        def rhs(p, k0, k1):
            if p in SIDX:
                return stored_rhs(sl, p, k0, k1)
            e = 0 if p == 1 else 1
            parts = [w2_v[pidx, _blk(2 * i + e), _blk(e)] for i in range(k0 // LB, min(NFP, k1 // LB))]
            if k1 == KC:
                parts.append(_up(ol_s[sl * HD + e * QD:sl * HD + (e + 1) * QD, _blk(e)]))
            return _cat(parts, 0)
        todo = []
        for i in range(NFP):
            tt = t0 + P["TS0"] + i * P["TSD"]
            todo.append((tt + P["TSD"], tsum, (lambda rs: w2_v[pn, rs, :], 2 * i * LB, sn, i, tt, P["TSD"])))
        t = t0 + P["PV0"]
        pvd, pvb = (P["PVD"], P["PVB"]) if nqk == 0 and tskip == 0 else (P["PVD2"], P["PVD2"])
        t += tskip
        for _ in range(nqk):
            todo.append((t + pvd, slot, (t, pvd)))
            t += pvd if mains[slot_plan[0]] is not None else 0
            slot_plan[0] += 1
        for e in range(2):
            for hh in range(2):
                todo.append((t + pvb, attn_pv, (pn * 2 + e, hh, sn, e, t, pvb, t + pvb + P["PVL"])))
                t += pvd
        todo.append((t0 + P["OS0"] + P["OSD"], osum, (sn, t0 + P["OS0"], P["OSD"])))
        add_tasks(todo)
        q = _combine(strassen(lhs, rhs, KC, P["CORD"], head=head))
        flush()
        for (e0, e1, r0, r1) in out_parts(fine):
            cols = slice(e0 * LB, e1 * LB)
            for h0 in range(r0, r1, HD):
                y = _cat([q[2 * (h0 // HD) + e] for e in range(e0, e1)], 1)
                o = y + b2f_s[pidx, 0:1, cols] + x_v[pidx, h0:h0 + HD, cols].astype(f32)
                out_v[pidx, h0:h0 + HD, cols] = o.astype(bf16)
            out_copy(pidx, e0, e1, r0, r1).start()

    def c_body(it, carry):
        reset()
        ready.update({("rs", 0, i) for i in range(NFP + 2)} | {("lc", i) for i in range(NFP + 1)})
        for c in range(NPC):
            pidx = NPRE + it * NPC + c
            piece(pidx, c, lax.rem(pidx + 1, NP), fine=c == NPC - 1)
        return carry

    x0 = Group(cp_x(0, 1))
    g1 = Group(cp_w1(0, 1))
    g2 = Group(cp_w1(1, 2) + cp_x(1, 2))
    g3 = Group(cp_w1(2, UB0))
    g4 = Group([(wqkv_hbm, wqkv_v)])
    g5 = Group(cp_x(2, NP))
    g6 = Group(cp_w1(UB0, NB) + [(wo_hbm, wo_v), (b1_hbm, b1_v), (b2_hbm, b2_v)] + cp_w2(0, NPRE + 1))
    g7 = Group(cp_w2(NPRE + 1, NP))
    for c in (x0, g1, g2, g3, g4, g5, g6, g7):
        c.start()

    v_s[0] = jnp.zeros((D, LB), f32)
    for buf in (xnT_s, ra_s, hT_s, lh_s, ol_s, rs_s):
        buf[0:8, 0:64] = jnp.zeros((8, 64), u32)

    LND, BD, MARG = P["LND"], P["BD"], P["MARG"]

    def ln_tasks(b, t):
        todo = []
        for fn, bb, dur, adv in ((ln, b, LND, 0.8), (ln, b + 1, LND, 0.86), (hpair, b, P["HSD"], 1.0)):
            todo.append((t + int(dur * adv), fn, (bb, t, dur)))
            t += int(dur * adv)
        return todo, t

    wait("x0", x0)
    ln(0); ln(1); hpair(0)
    wait("r1", g1)
    stage_u(0, 1, 0, 12)
    wait("r2", g2)
    add_tasks(ln_tasks(2, 0)[0])
    stage_u(0, 2, 12, NFB)
    stage_u(1, 2, 0, 12)
    wait("r3", g3)
    stage_u(2, 4, 0, P["N3"])
    wait("wqkv", g4)
    stage_u(2, 4, P["N3"], NFB)
    prep_wqkv()
    stage_a(0, split_last=True)
    wait("mid", g5)
    AD = 7 * HA // 2
    UD = 7 * NUP * HD // 4
    r5 = (NP - 1) * AD
    t = 0
    for b in range(UB0, NB, 2):
        todo, t = ln_tasks(b, t)
        add_tasks(todo)
    n5 = 0
    while t + BD + MARG <= r5:
        add_tasks([(t + BD, slot, (t, BD))])
        t += BD
        n5 += 1
    for n, b in enumerate(range(2, NB, 2)):
        stage_a(b, odd=n % 2 == 1, split_last=b == NB - 2)
    wait("fin", g6)
    r6 = NFP * UD
    todo = []
    for i in range(NFP + 1):
        if i == 0:
            t0, dt = -200, 130
        elif i == 1:
            t0, dt = 700, 260
        else:
            t0, dt = (i - 1) * UD + P["US0"], P["USD"]
        if i < NFP:
            for k in range(NUP):
                tt = t0 + k * dt
                todo.append((tt + dt, tsum, (lambda rs, i=i: w1_v[rs, 2 * i * LB:(2 * i + 2) * LB],
                                             (UB0 + 2 * k) * LB, i % 3, k, tt, dt)))
        else:
            for k in range(NFP):
                tt = t0 + k * 300
                todo.append((tt + 300, tsum, (lambda rs: w2_v[0, rs, :], 2 * k * LB, 1, k, tt, 300)))
    left = len(mains) - n5 - P["NQ0"] - P["NQ1"]
    slot_plan = [n5 + left]
    t = P["R6S"]
    bd2 = (r6 - t) // left
    for _ in range(left):
        todo.append((t + min(bd2, 600), slot, (t, min(bd2, 600))))
        t += bd2
    todo.append((r6 - 100, osum, (1, r6 - 500, 400)))
    todo.append((P["PW0"] + P["PWD"], prep_wo, (P["PW0"], P["PWD"])))
    add_tasks(todo)
    for b in range(NB):
        b2f_s[b // 2, 0:1, _blk(b % 2)] = b2_v[b:b + 1, :].astype(f32)
    for i in range(NFP):
        stage_u_last(i, (1, 4, 2, 3, 0, 5, 6) if i == 0 else P["UORD"], P["UED"] if i < NFP - 1 else P["UEL"])
    piece(0, 1, 1, head=4, nqk=P["NQ0"], tskip=P["SK0"])
    piece(1, 2, 2, nqk=P["NQ1"])
    assert slot_ctr[0] == len(mains)
    wait("w2", g7)

    lax.fori_loop(0, 2, c_body, 0)
    outs = [out_copy(pidx, *part) for pidx in range(NP)
            for part in out_parts(pidx >= NPRE and (pidx - NPRE) % NPC == NPC - 1)]
    wait("out", *outs)


@jax.jit
def pallas_parallel_sum__sliding_local_dilated__mixer_token_mlp__prompt_kernel(A_x, A_wqkv, A_wo, B_x, B_w1, B_b1, B_w2, B_b2):
    del B_x
    hbm = pl.BlockSpec(memory_space=pltpu.HBM)
    outT = pl.pallas_call(
        _kernel,
        out_shape=jax.ShapeDtypeStruct((1, D, S), bf16),
        in_specs=[hbm] * 7,
        out_specs=hbm,
        scratch_shapes=[
            pltpu.VMEM((NP, D, 2 * LB), bf16),
            pltpu.VMEM((D, 3 * D), bf16),
            pltpu.VMEM((D, D), bf16),
            pltpu.VMEM((S, F), bf16),
            pltpu.VMEM((NP, F, 2 * LB), bf16),
            pltpu.VMEM((NFB, LB), bf16),
            pltpu.VMEM((NB, LB), bf16),
            pltpu.VMEM((NP, D, 2 * LB), bf16),
            pltpu.VMEM((4, 3 * D, LB), f32),
            pltpu.VMEM((7 * HA // 2, HD), u32),
            pltpu.VMEM((4, D, LB), f32),
            pltpu.VMEM((HD, S), u32),
            pltpu.VMEM((NP * QD, 5 * LB), u32),
            pltpu.VMEM((HD, UB0 * LB), u32),
            pltpu.VMEM((7 * QD, NUP * LB), u32),
            pltpu.VMEM((D, F), f32),
            pltpu.VMEM((7 * QD, KC), u32),
            pltpu.VMEM((NB + 1, 2 * D, LB), f32),
            pltpu.VMEM((NB + 1, D, LB), f32),
            pltpu.VMEM((NB, 2 * W * HH, LB), f32),
            pltpu.VMEM((3 * HD, 2 * LB), u32),
            pltpu.VMEM((D, LB), f32),
            pltpu.VMEM((NP, 32, 2 * LB), f32),
            pltpu.VMEM((3 * RSK, 5 * LB), u32),
            pltpu.SemaphoreType.DMA((9,)),
        ],
        compiler_params=pltpu.CompilerParams(vmem_limit_bytes=100 * 1024 * 1024,
                                             disable_bounds_checks=True,
                                             disable_semaphore_checks=True),
    )(jnp.swapaxes(A_x, 1, 2), A_wqkv, A_wo, B_w1, B_b1.reshape(NFB, LB), B_w2, B_b2.reshape(NB, LB))
    return jnp.swapaxes(outT, 1, 2)
```

```python
import jax
import jax.numpy as jnp
from jax import lax
import jax.experimental.pallas as pl
import jax.experimental.pallas.tpu as pltpu

S, D, F = 2048, 448, 1792
H, DH, W, DIL = 16, 28, 8, 2
LB = 128
NB = S // LB
NP = NB // 2
NFB = F // LB
NFP = NFB // 2
HH = H // 2
WH = W // 2
SH = DIL * WH
HD = D // 2
QD = D // 4
HA = 3 * HD
UB0 = 4
NUP = (NB - UB0) // 2
KC = F // 2 + HD
RSK = (NFP + 2) * LB // 2
EPS = 1e-5
SCALE = DH ** -0.5
f32 = jnp.float32
bf16 = jnp.bfloat16
u32 = jnp.uint32
i32 = jnp.int32

SCOPES = False
P = dict(LND=640, BD=440, G=4, L=4, LS=170, PP=150, MARG=300, N3=40, E3=6, W3T=700, W3D=600, W2T=200, W2D=450, W2X=300, E1=3, L2T=250, L2D=480, H2D=420, PVD=680, PV0=50, HSD=560, HG=80,
         CORD=(4, 2, 1, 3, 0, 5, 6), TS0=100, TSD=420, PVB=520, PVL=500, OS0=3050, OSD=300,
         UORD=(4, 2, 1, 3, 0, 5, 6), US0=100, USD=350, R6S=1800, PVPOS=16, PVD2=400, NQ0=1, NQ1=5, HL=250,
         UE0=-200, UED=2100, UEL=1300, PW0=-1000, PWD=400, UG=50, UM=24, PWL=2100, SK0=900, LNQ1=4, LNQ3=4, LNA=0.3, LNB=0.42, LNBD=0.33)


def _gelu(x, z=None):
    c = 0.7978845608028654
    hx = 0.5 * x
    return hx + hx * jnp.tanh(_orz(x * (c + (c * 0.044715) * (x * x)), z))


def _pk(x):
    return pltpu.bitcast(x.astype(bf16), u32)


def _up(x):
    return pltpu.bitcast(x, bf16)


def _upf(x):
    return pltpu.bitcast(x, bf16).astype(f32)


def _cat(xs, axis):
    return xs[0] if len(xs) == 1 else jnp.concatenate(xs, axis=axis)


def _x2(v):
    return jnp.concatenate([v, v], axis=0)


def _blk(b):
    return slice(b * LB, (b + 1) * LB)


def _rowsum8(a):
    return jnp.broadcast_to(jnp.sum(a, axis=0, keepdims=True), (8, a.shape[1]))


def _zero(*deps):
    deps = [d for d in deps if d is not None]
    if not deps:
        return None
    bits = pltpu.bitcast(deps[0], u32)
    for d in deps[1:]:
        bits = bits | pltpu.bitcast(d, u32)
    return lax.shift_right_logical(lax.shift_right_logical(bits, jnp.uint32(31)), jnp.uint32(1))


def _orz(v, z):
    return v if z is None else pltpu.bitcast(pltpu.bitcast(v, u32) | z, v.dtype)


def _pkz(v, z):
    return _pk(v if z is None else jnp.concatenate([_orz(v[0:8], z), v[8:16]], axis=0))


def _lhs_ops(a11, a12, a21, a22):
    return [a11 + a22, a21 + a22, a11, a22, a11 + a12, a21 - a11, a12 - a22]


SIDX = {0: 0, 2: 1, 3: 2, 5: 3, 6: 4}


def _rhs_sums(b11, b12, b21, b22):
    return {0: b11 + b22, 2: b12 - b22, 3: b21 - b11, 5: b11 + b12, 6: b21 + b22}


def _combine(m):
    c12 = m[2] + m[4]
    c21 = m[1] + m[3]
    x = (m[2] - m[1]) + m[0]
    return ((x + m[6]) + (c21 - c12), c12, c21, x + m[5])


def _kernel(x_hbm, wqkv_hbm, wo_hbm, w1_hbm, b1_hbm, w2_hbm, b2_hbm, out_hbm,
            x_v, wqkv_v, wo_v, w1_v, w2_v, b1_v, b2_v, out_v,
            wt_s, lw_s, wo_s, xnT_s, ra_s, lh_s, um_s, lc_s, qk_s, v_s, pr_s, ol_s, op_s,
            b2f_s, rs_s, sems):
    sem_ctr = [1]

    class Group:
        def __init__(self, pairs):
            self.cps = [pltpu.make_async_copy(a, b, sems.at[sem_ctr[0]]) for (a, b) in pairs]
            sem_ctr[0] += 1

        def start(self):
            for c in self.cps:
                c.start()

        def wait(self):
            for c in self.cps:
                c.wait()

    def cp_x(p0, p1):
        return [(x_hbm.at[0, :, pl.ds(p * 2 * LB, 2 * LB)], x_v.at[p]) for p in range(p0, p1)]

    def cp_w2(p0, p1):
        return [(w2_hbm.at[:, pl.ds(p * 2 * LB, 2 * LB)], w2_v.at[p]) for p in range(p0, p1)]

    def cp_w1(b0, b1, i0=0, i1=NFP):
        sl = pl.ds(b0 * LB, (b1 - b0) * LB)
        cl = pl.ds(i0 * 2 * LB, (i1 - i0) * 2 * LB)
        return [(w1_hbm.at[sl, cl], w1_v.at[sl, cl])]

    tl = []
    mxu = [0, 0, 0, 0]
    nxt = [0]
    hist = []
    tasks = []
    dls = []
    ready = set()

    def add_tasks(todo):
        tasks.extend(todo)
        tasks.sort(key=lambda x: x[0])

    def flush(t=None):
        while tasks and (t is None or tasks[0][0] < t):
            _, fn, args = tasks.pop(0)
            fn(*args)

    def reset():
        assert not tasks
        dls.clear()
        tl.clear()
        hist.clear()
        mxu[:] = [0, 0, 0, 0]
        nxt[0] = 0

    def now():
        return sum(mxu) // 4

    def wait(name, *cps):
        flush()
        if SCOPES:
            with jax.named_scope("wait_" + name):
                for c in cps:
                    c.wait()
        else:
            for c in cps:
                c.wait()
        reset()

    def mm1(lhs, rhs, pace=True):
        flush(now())
        start = mxu[nxt[0]]
        due = [v for (t, v) in dls if t <= start] if pace else []
        if due:
            dls[:] = [(t, v) for (t, v) in dls if t > start]
            tile = _up(pltpu.bitcast(lhs[0:16, 0:LB], u32) | _zero(*due))
            row = tile if lhs.shape[1] == LB else jnp.concatenate([tile, lhs[0:16, LB:]], axis=1)
            lhs = jnp.concatenate([row, lhs[16:]], axis=0)
        r = jnp.dot(lhs, rhs, preferred_element_type=f32)
        m, k = lhs.shape
        first_done = None
        for _ in range(-(-rhs.shape[1] // LB)):
            end = 0
            for _ in range(-(-k // LB)):
                mxu[nxt[0]] += m
                end = max(end, mxu[nxt[0]])
                nxt[0] = (nxt[0] + 1) % 4
            if first_done is None:
                first_done = end
        if pace:
            tl.append((first_done - m, first_done, r))
        return r

    def mm(lhs, rhs, init=None):
        k = lhs.shape[1]
        r, k0 = init, 0
        while k0 < k:
            k1 = min(k, k0 + (4 - nxt[0]) * LB)
            part = mm1(lhs[:, k0:k1], rhs[k0:k1], pace=k1 - k0 > LB)
            r = part if r is None else r + part
            k0 = k1
        return r

    def at(t):
        if t is None or t < 0:
            return None
        t = min(t, now() - 1)
        best = None
        for (a, b, r) in tl:
            if a <= t and (best is None or min(b, t) > best[0]):
                row = int(min((t - a) / (b - a), 0.999) * (r.shape[0] // 8)) * 8
                best = (min(b, t), r, row)
        return None if best is None else best[1][best[2]:best[2] + 8, 0:LB]

    def strassen(lhs, rhs, k, order, split_last=False, head=0, init=None):
        m = [None] * 7

        def ops(p, k0, k1):
            flush(now())
            return lhs(p, k0, k1), rhs(p, k0, k1)

        if head:
            for p in order:
                m[p] = mm(*ops(p, 0, head * LB))
        for p in order:
            l, r = ops(p, head * LB, k)
            if split_last and p == order[-1]:
                kk = (-(-r.shape[0] // LB) - 2) * LB
                hm = l.shape[0] // 2
                hd = mm(l[:, :kk], r[:kk]) if kk else None
                tail = jnp.concatenate([mm(l[:hm, kk:], r[kk:]), mm(l[hm:, kk:], r[kk:])], axis=0)
                v = tail if hd is None else hd + tail
            else:
                v = mm(l, r, None if init is None else init[p])
            m[p] = v if m[p] is None else m[p] + v
        return m

    def put_sums(dst, sm, ro, z):
        for p, v in sm.items():
            dst[ro:ro + 8, _blk(SIDX[p])] = _pkz(v, z)

    def tsum(ld, r0, slot_, i, t0, dur):
        for g in range(LB // 16):
            z = _zero(at(t0 + g * dur // 8))
            t1 = ld(slice(r0 + g * 16, r0 + g * 16 + 16)).astype(f32)
            t2 = ld(slice(r0 + LB + g * 16, r0 + LB + g * 16 + 16)).astype(f32)
            sm = _rhs_sums(t1[:, :LB], t1[:, LB:], t2[:, :LB], t2[:, LB:])
            put_sums(rs_s, sm, slot_ * RSK + i * (LB // 2) + g * 8, z)
        ready.add(("rs", slot_, i))

    def osum(slot_, t0, dur):
        ng = HD // 16
        for g in range(ng):
            z = _zero(at(t0 + g * dur // ng))
            r1, r2 = slot_ * HD + g * 8, slot_ * HD + QD + g * 8
            sm = _rhs_sums(_upf(ol_s[r1:r1 + 8, 0:LB]), _upf(ol_s[r1:r1 + 8, LB:]),
                           _upf(ol_s[r2:r2 + 8, 0:LB]), _upf(ol_s[r2:r2 + 8, LB:]))
            put_sums(rs_s, sm, slot_ * RSK + F // 4 + g * 8, z)
        ready.update({("rs", slot_, NFP), ("rs", slot_, NFP + 1)})

    def stored_rhs(slot_, p, k0, k1):
        assert all(("rs", slot_, i) in ready for i in range(k0 // LB, -(-k1 // LB))), (slot_, k0, k1)
        return _up(rs_s[slot_ * RSK + k0 // 2:slot_ * RSK + k1 // 2, _blk(SIDX[p])])

    def wrows(hh, g, z=None):
        p, d = divmod(2 * g, DH)
        t = [jnp.concatenate([wt_s[c, pl.ds(p * D + hh * HD + d + e, HH, stride=DH), :]
                              for e in range(2)], axis=0) for c in range(2)]
        if z is not None:
            t = [_orz(v, _x2(z)) for v in t]
        w = jnp.concatenate([t[0], t[1][:, 0:HD - LB]], axis=1)
        return [pltpu.bitcast(w << 16, f32), pltpu.bitcast(w & -65536, f32)]

    def prep_wqkv():
        done = set()
        ng = HA // 16

        def need(hh, p, z=None):
            lo = p * D + hh * HD
            for ct in range(lo // LB, -(-(lo + HD) // LB)):
                if ct in done:
                    continue
                done.add(ct)
                w = min(LB, 3 * D - ct * LB)
                k1, k2 = [pltpu.bitcast(wqkv_v[kh * HD:(kh + 1) * HD, ct * LB:ct * LB + w].astype(f32), i32)
                          for kh in range(2)]
                wd = lax.shift_right_logical(k1, 16) | k2
                if z is not None:
                    wd = jnp.concatenate([_orz(wd[r:r + 8], z[:, 0:w]) if r % LB == 0 else wd[r:r + 8]
                                          for r in range(0, HD, 8)], axis=0)
                wT = wd.T
                wt_s[0, ct * LB:ct * LB + w, :] = wT[:, 0:LB]
                wt_s[1, ct * LB:ct * LB + w, 0:HD - LB] = wT[:, LB:HD]

        def put(p, g, v):
            lw_s[p * (HA // 2) + g * 8:p * (HA // 2) + g * 8 + 8, :] = _pk(v)

        def half(hh, g0, g1, t0=None, dur=None):
            pr, ps = ((2, 4), (3, 1))[hh]
            for g in range(g0, g1):
                t = None if t0 is None else t0 + (g - g0) * dur // (g1 - g0)
                need(hh, 2 * g // DH, _zero(at(None if t is None else t - P["W2X"])))
                a1, a2 = wrows(hh, g, _zero(at(t)))
                put(pr, g, a2 if hh else a1)
                put(ps, g, a1 + a2)
            if g1 == ng:
                ready.update({("lw", pr), ("lw", ps)})
        half(0, 0, ng)
        t, dt = now() + P["W2T"], P["W2D"] // 3
        add_tasks([(t + (n + 1) * dt, half, (1, 14 * n, 14 * n + 14, t + n * dt, dt)) for n in range(3)])

        def rest(g0, g1, t0, dur):
            for g in range(g0, g1):
                z = _zero(at(t0 + (g - g0) * dur // (g1 - g0)))
                ops = _lhs_ops(*wrows(0, g, z), *wrows(1, g, z))
                for p in (0, 5, 6):
                    put(p, g, ops[p])
            if g1 == ng:
                ready.update({("lw", 0), ("lw", 5), ("lw", 6)})
        t, dt = now() + P["W3T"], P["W3D"] // 7
        add_tasks([(t + (n + 1) * dt, rest, (6 * n, 6 * n + 6, t + n * dt, dt)) for n in range(7)])

    def prep_wo(t0, dur):
        for g in range(D // 16):
            w = wo_v[g * 16:g * 16 + 16, :].astype(f32)
            z = _zero(at(t0 + g * dur // (D // 16)))
            for c in range(4):
                cw = min(LB, D - c * LB)
                t = w[:, c * LB:c * LB + cw]
                if z is not None:
                    t = _orz(t, _x2(z)[:, 0:cw])
                wo_s[c, g * 16:g * 16 + 16, 0:cw] = t
        wt = []
        for hh in range(2):
            cols = []
            for c in range(4):
                cw = min(LB, D - c * LB)
                rows = [wo_s[c, pl.ds(hh * HD + d, HH, stride=DH), :][:, 0:cw] for d in range(DH)]
                cols.append(jnp.concatenate(rows, axis=0).astype(bf16).T.astype(f32))
            wt.append(jnp.concatenate(cols, axis=0))
        for p, v in enumerate(_lhs_ops(wt[0][0:HD], wt[1][0:HD], wt[0][HD:D], wt[1][HD:D])):
            lc_s[p * QD:(p + 1) * QD, F // 2:KC] = _pk(v)
        ready.add(("lc", NFP))
        got = lc_s[:, F // 2:F // 2 + LB]
        bits = got[0:8]
        for r in range(8, 7 * QD, 8):
            bits = bits | got[r:r + 8]
        dls.append((P["PWL"], bits))

    RG = 16
    NG = D // RG
    stat2 = {}

    def ln(b, t0=None, dur=None):
        def dep(fr):
            return None if t0 is None else at(t0 + fr * dur)

        def xg(g):
            return x_v[b // 2, g * RG:(g + 1) * RG, _blk(b % 2)].astype(f32)

        def halves(*vs):
            return [] if vs[0] is None else [v[i * 8:i * 8 + 8] for v in vs for i in range(2)]

        x0 = jnp.broadcast_to(xg(0)[0:1], (8, LB))
        s = q = None
        for g in range(NG):
            if g % P["LNQ1"] == 0 and t0 is not None:
                x0 = _orz(x0, _zero(dep(P["LNA"] * g / NG), *halves(s, q)))
            c = xg(g) - _x2(x0)
            s = c if s is None else s + c
            q = c * c if q is None else q + c * c
        dm = _rowsum8(s) * (1.0 / D)
        mu = x0 + dm
        r1 = lax.rsqrt(jnp.maximum(_rowsum8(q) * (1.0 / D) - dm * dm, 0.0) + EPS)
        s1 = s2 = z = None
        for g in range(NG):
            if g % P["LNQ3"] == 0 and t0 is not None:
                z = _zero(dep(P["LNB"] + P["LNBD"] * g / NG), *halves(s1, s2))
            xn = (xg(g) - _x2(mu)) * _x2(r1)
            xnT_s[g * 8:g * 8 + 8, _blk(b)] = _pkz(xn, z)
            s1 = xn if s1 is None else s1 + xn
            s2 = xn * xn if s2 is None else s2 + xn * xn
        mu2 = _rowsum8(s1) * (1.0 / D)
        var2 = jnp.maximum(_rowsum8(s2) * (1.0 / D) - mu2 * mu2, 0.0)
        stat2[b] = (mu2, lax.rsqrt(var2 + EPS))

    def hpair(b, t0=None, dur=None):
        ng = HD // RG
        st = [stat2.pop(b), stat2.pop(b + 1)]
        for g in range(ng):
            t = None if t0 is None else t0 + g * dur // ng
            zi = _zero(at(None if t is None else t - P["HG"]))
            z = _zero(at(t))
            xq, hq = [], []
            for r in (g * 8, QD + g * 8):
                for e in range(2):
                    xn = _upf(_orz(xnT_s[r:r + 8, _blk(b + e)], zi))
                    xq.append(xn)
                    hq.append((xn - _x2(st[e][0])) * _x2(st[e][1]))
            put_sums(ra_s, _rhs_sums(*xq), (b // 2) * QD + g * 8, z)
            for p, v in enumerate(_lhs_ops(*hq)):
                lh_s[p * QD + g * 8:p * QD + g * 8 + 8, _blk(b // 2)] = _pkz(v, z)
        ready.add(("xn", b))
        if t0 is not None and b >= UB0 and P["HL"]:
            got = ra_s[(b // 2) * QD:(b // 2 + 1) * QD, :]
            tiles_ = [got[r:r + 8, _blk(c)] for r in range(0, QD, 8) for c in range(5)]
            bits = tiles_[0]
            for v in tiles_[1:]:
                bits = bits | v
            dls.append((t0 + dur + P["HL"], bits))

    def w1_ld(i):
        return lambda rs: w1_v[rs, 2 * i * LB:(2 * i + 2) * LB]

    def ujob(kp, i, p, split=False):
        flush(now())
        assert ("xn", 2 * kp) in ready
        l = _up(lh_s[p * QD:(p + 1) * QD, _blk(kp)])
        if p in SIDX:
            r = stored_rhs(3 + kp, p, i * LB, (i + 1) * LB)
        else:
            e = 0 if p == 1 else 1
            r = w1_v[_blk(2 * kp + e), _blk(2 * i + e)]
        v = jnp.concatenate([mm1(l[:QD], r), mm1(l[QD:], r)], axis=0) if split else mm1(l, r)
        rows = slice(p * HD, (p + 1) * HD)
        um_s[rows, _blk(i)] = v if kp == 0 else um_s[rows, _blk(i)] + v

    def u_early(kp, i0, i1, carry, n, t0, dt, nsplit=0):
        for k, i in enumerate(range(i0, i1)):
            add_tasks([(t0 + (k + 1) * dt, tsum, (w1_ld(i), 2 * kp * LB, 3 + kp, i, t0 + k * dt, dt))])
        jobs = (carry + [(kp, i, p) for i in range(i0, i1) for p in (1, 4)]
                + [(kp, i, p) for i in range(i0, i1) for p in SIDX])
        for c, job in enumerate(jobs[:n]):
            ujob(*job, split=c >= n - nsplit)
        return jobs[n:]

    def u_epilogue(i, m, g0, g1, t0, dur):
        for g in range(g0, g1):
            t = t0 + (g - g0) * dur // (g1 - g0)
            z = _zero(at(t))
            if P["UM"] == 0:
                zi = [_zero(at(t - P["UG"]))] * 4
            else:
                zi = [_zero(at(t - P["UG"] - (3 - n) * P["UM"])) for n in range(4)]
            zi = [None if v is None else _x2(v) for v in zi]
            bia = [b1_v[2 * i + e:2 * i + e + 1, :].astype(f32) for e in range(2)]
            top = slice(g * 16, g * 16 + 16)
            q = _combine([x[top] for x in m])
            gl = [_gelu(q[0] + bia[0], zi[3]), _gelu(q[1] + bia[1], zi[0]),
                  _gelu(q[2] + bia[0], zi[1]), _gelu(q[3] + bia[1], zi[2])]
            for p, v in enumerate(_lhs_ops(*gl)):
                lc_s[p * QD + g * 8:p * QD + g * 8 + 8, _blk(i)] = _pkz(v, z)
        if g1 == HD // 16:
            ready.add(("lc", i))

    def stage_u_last(i, order, edur):
        def lhs(p, k0, k1):
            return _up(lh_s[p * QD:(p + 1) * QD, UB0 // 2 * LB + k0:UB0 // 2 * LB + k1])

        def rhs(p, k0, k1):
            if p in SIDX:
                return stored_rhs(i % 3, p, k0, k1)
            e = 0 if p == 1 else 1
            return _cat([w1_v[_blk(UB0 + 2 * k + e), _blk(2 * i + e)] for k in range(k0 // LB, k1 // LB)], 0)
        m = strassen(lhs, rhs, NUP * LB, order, init=[um_s[p * HD:(p + 1) * HD, _blk(i)] for p in range(7)])
        for k in range(NUP):
            ready.discard(("rs", i % 3, k))
        t = now() - P["UE0"]
        ng = HD // 16
        add_tasks([(t + (g + 2) * edur // ng, u_epilogue, (i, m, g, g + 2, t + g * edur // ng, 2 * edur // ng))
                   for g in range(0, ng, 2)])

    def stage_a(b, odd=False, split_last=False):
        def lhs(p, k0, k1):
            assert ("lw", p) in ready
            return _up(lw_s[p * (HA // 2):(p + 1) * (HA // 2), :])

        def rhs(p, k0, k1):
            assert ("xn", b) in ready
            if p in SIDX:
                return _up(ra_s[(b // 2) * QD:(b // 2 + 1) * QD, _blk(SIDX[p])])
            return _up(xnT_s[0:QD, _blk(b)] if p == 1 else xnT_s[QD:HD, _blk(b + 1)])
        order = (6, 4, 2, 1, 3, 0, 5) if odd else (4, 2, 1, 3, 0, 5, 6)
        q = _combine(strassen(lhs, rhs, HD, order, split_last))
        for hh in range(2):
            for e in range(2):
                qk_s[b + e + 1, hh * D:(hh + 1) * D, :] = q[2 * hh + e][0:D]
                v_s[b + e + 1, hh * HD:(hh + 1) * HD, :] = q[2 * hh + e][D:HA]
        ready.update({("qkv", b), ("qkv", b + 1)})

    lane0 = lax.broadcasted_iota(i32, (HH, LB), 1)
    lane2 = 2 * lane0
    zeros8 = jnp.zeros((HH, LB), f32)

    def mk_shift(*deps):
        deps = [d for d in deps if d is not None]
        lane = lane2
        if deps:
            bits = pltpu.bitcast(deps[0], u32)
            for d in deps[1:]:
                bits = bits | pltpu.bitcast(d, u32)
            lane = lane2 | pltpu.bitcast(lax.shift_right_logical(bits, jnp.uint32(31)), i32)

        def fwd(cur, prev, sh):
            if sh == 0:
                return cur
            return pltpu.roll(jnp.where(lane < 2 * (LB - sh), cur, prev), sh, 1)

        def bwd(cur, nxt_):
            return pltpu.roll(jnp.where(lane >= 2 * SH, cur, nxt_), LB - SH, 1)
        return fwd, bwd

    def grp_shift(t):
        deps = [at(t)]
        if P["L"] and len(hist) >= P["L"]:
            deps += hist[-P["L"]]
        return mk_shift(*deps)

    raw, probs = {}, {}

    def attn_qk(j, hh, t, bd):
        jn = min(j + 1, NB - 1)
        assert ("qkv", jn) in ready
        acc = [None] * WH
        accp = [None] * WH
        for d in range(DH):
            if d % P["G"] == 0:
                if d > 0:
                    hist.append(acc + accp)
                fwd, bwd = grp_shift(t + d * bd // DH)
            r = hh * D + d * HH
            q = qk_s[j + 1, r:r + HH, :]
            qp = bwd(q, qk_s[jn + 1, r:r + HH, :])
            k = qk_s[j + 1, HD + r:HD + r + HH, :]
            kp = qk_s[j, HD + r:HD + r + HH, :] if j > 0 else zeros8
            for a in range(WH):
                ks = fwd(k, kp, DIL * a)
                t0, t1 = q * ks, qp * ks
                acc[a] = t0 if d == 0 else acc[a] + t0
                accp[a] = t1 if d == 0 else accp[a] + t1
        hist.append(acc + accp)
        raw[j, hh] = (acc, accp)

    def attn_sm(j, hh, t):
        fwd, _ = mk_shift(at(t))
        acc, accp = raw[j, hh]
        prev = raw.pop((j - 1, hh))[1] if j > 0 else [zeros8] * WH
        lg = acc + [fwd(accp[a], prev[a], SH) for a in range(WH)]
        lg = [a * SCALE for a in lg]
        if j == 0:
            lg = [lg[0]] + [jnp.where(lane0 >= DIL * w, lg[w], -1e9) for w in range(1, W)]
        m = lg[0]
        for w in range(1, W):
            m = jnp.maximum(m, lg[w])
        e = [jnp.exp(l - m) for l in lg]
        den = e[0]
        for w in range(1, W):
            den = den + e[w]
        inv = 1.0 / den
        p = [x * inv for x in e]
        for a in range(WH):
            pr_s[j, (hh * W + a) * HH:(hh * W + a + 1) * HH, :] = p[a]
        probs[j, hh] = p[WH:]

    def attn_pp(j, hh, t):
        _, bwd = mk_shift(at(t))
        p = probs.pop((j, hh))
        pn = probs[j + 1, hh] if j + 1 < NB else p
        for a in range(WH):
            pr_s[j, (hh * W + WH + a) * HH:(hh * W + WH + a + 1) * HH, :] = bwd(p[a], pn[a])
        ready.add(("pr", j, hh))

    def attn_pv(j, hh, slot_, e, t, bd, t_dl):
        assert not isinstance(j, int) or ("pr", j, hh) in ready
        pa = [pr_s[j, (hh * W + a) * HH:(hh * W + a + 1) * HH, :] for a in range(W)]
        p, pp = pa[:WH], pa[WH:]
        outs = []
        for d2 in range(DH // 2):
            os_ = []
            for d in (2 * d2, 2 * d2 + 1):
                if d % P["G"] == 0:
                    if d > 0:
                        hist.append([])
                    fwd, _ = grp_shift(t + d * bd // DH)
                r = hh * HD + d * HH
                v = v_s[j + 1, r:r + HH, :]
                vp = v_s[j, r:r + HH, :]
                o = op = None
                for a in range(WH):
                    vs = fwd(v, vp, DIL * a)
                    o = p[a] * vs if a == 0 else o + p[a] * vs
                    op = pp[a] * vs if a == 0 else op + pp[a] * vs
                opp = zeros8 if (isinstance(j, int) and j == 0) else op_s[r:r + HH, :]
                op_s[r:r + HH, :] = op
                os_.append(o + fwd(op, opp, SH))
            ro = slot_ * HD + hh * QD + d2 * HH
            ol_s[ro:ro + HH, _blk(e)] = _pk(jnp.concatenate(os_, axis=0))
            outs += os_
        hist.append([])
        bits = pltpu.bitcast(outs[0], u32)
        for o in outs[1:]:
            bits = bits | pltpu.bitcast(o, u32)
        dls.append((t_dl, bits))

    mains = [("qk", j, hh) for j in range(NB) for hh in range(2)]
    mains = (mains[:P["PVPOS"]] + [("pv", j, hh) for j in range(2) for hh in range(2)]
             + mains[P["PVPOS"]:] + [None, None])
    slot_ctr = [0]

    def slot(t, bd):
        n = slot_ctr[0]
        slot_ctr[0] += 1
        it = mains[n]
        if it is None:
            pass
        elif it[0] == "qk":
            attn_qk(it[1], it[2], t, bd)
        else:
            attn_pv(it[1], it[2], 1, it[1], t, bd, t + bd + P["PVL"])
        if n >= 1 and mains[n - 1] is not None and mains[n - 1][0] == "qk":
            attn_sm(mains[n - 1][1], mains[n - 1][2], t + P["LS"])
        if n >= 2 and mains[n - 2] is not None and mains[n - 2][0] == "qk":
            _, j, hh = mains[n - 2]
            if j > 0:
                attn_pp(j - 1, hh, t + P["PP"])
            if j == NB - 1:
                attn_pp(j, hh, t + P["PP"])

    NPRE = 2
    NPC = 3

    def out_copy(pidx, e0, e1, r0, r1):
        off = pidx * (2 * LB) + e0 * LB
        if not isinstance(pidx, int):
            off = pl.multiple_of(off, LB)
        rs = pl.ds(r0, r1 - r0)
        return pltpu.make_async_copy(out_v.at[pidx, rs, pl.ds(e0 * LB, (e1 - e0) * LB)],
                                     out_hbm.at[0, rs, pl.ds(off, (e1 - e0) * LB)], sems.at[0])

    def out_parts(fine):
        return [(1, 2, 0, HD), (0, 2, HD, D), (0, 1, 0, HD)] if fine else [(0, 2, 0, D)]

    def piece(pidx, sl, pn, fine=False, head=0, nqk=0, tskip=0):
        sn = (sl + 1) % 3
        t0 = now()

        def lhs(p, k0, k1):
            assert all(("lc", i) in ready for i in range(k0 // LB, min(NFP + 1, -(-k1 // LB)))), (k0, k1)
            return _up(lc_s[p * QD:(p + 1) * QD, k0:k1])

        def rhs(p, k0, k1):
            if p in SIDX:
                return stored_rhs(sl, p, k0, k1)
            e = 0 if p == 1 else 1
            parts = [w2_v[pidx, _blk(2 * i + e), _blk(e)] for i in range(k0 // LB, min(NFP, k1 // LB))]
            if k1 == KC:
                parts.append(_up(ol_s[sl * HD + e * QD:sl * HD + (e + 1) * QD, _blk(e)]))
            return _cat(parts, 0)
        todo = []
        for i in range(NFP):
            tt = t0 + P["TS0"] + i * P["TSD"]
            todo.append((tt + P["TSD"], tsum, (lambda rs: w2_v[pn, rs, :], 2 * i * LB, sn, i, tt, P["TSD"])))
        t = t0 + P["PV0"]
        pvd, pvb = (P["PVD"], P["PVB"]) if nqk == 0 and tskip == 0 else (P["PVD2"], P["PVD2"])
        t += tskip
        for _ in range(nqk):
            todo.append((t + pvd, slot, (t, pvd)))
            t += pvd if mains[slot_plan[0]] is not None else 0
            slot_plan[0] += 1
        for e in range(2):
            for hh in range(2):
                todo.append((t + pvb, attn_pv, (pn * 2 + e, hh, sn, e, t, pvb, t + pvb + P["PVL"])))
                t += pvd
        todo.append((t0 + P["OS0"] + P["OSD"], osum, (sn, t0 + P["OS0"], P["OSD"])))
        add_tasks(todo)
        q = _combine(strassen(lhs, rhs, KC, P["CORD"], head=head))
        flush()
        for (e0, e1, r0, r1) in out_parts(fine):
            cols = slice(e0 * LB, e1 * LB)
            for h0 in range(r0, r1, HD):
                y = _cat([q[2 * (h0 // HD) + e] for e in range(e0, e1)], 1)
                o = y + b2f_s[pidx, 0:1, cols] + x_v[pidx, h0:h0 + HD, cols].astype(f32)
                out_v[pidx, h0:h0 + HD, cols] = o.astype(bf16)
            out_copy(pidx, e0, e1, r0, r1).start()

    def c_body(it, carry):
        reset()
        ready.update({("rs", 0, i) for i in range(NFP + 2)} | {("lc", i) for i in range(NFP + 1)})
        for c in range(NPC):
            pidx = NPRE + it * NPC + c
            piece(pidx, c, lax.rem(pidx + 1, NP), fine=c == NPC - 1)
        return carry

    x0 = Group(cp_x(0, 1))
    E1 = P["E1"]
    g1 = Group(cp_w1(0, 2, 0, E1))
    g2 = Group(cp_w1(0, 2, E1, NFP) + cp_x(1, 2))
    E3 = P["E3"]
    g3 = Group(cp_w1(2, UB0, 0, E3))
    g4 = Group((cp_w1(2, UB0, E3, NFP) if E3 < NFP else []) + [(wqkv_hbm, wqkv_v)])
    g5 = Group(cp_x(2, NP))
    g6 = Group(cp_w1(UB0, NB) + [(wo_hbm, wo_v), (b1_hbm, b1_v), (b2_hbm, b2_v)] + cp_w2(0, NPRE + 1))
    g7 = Group(cp_w2(NPRE + 1, NP))
    for c in (x0, g1, g2, g3, g4, g5, g6, g7):
        c.start()

    v_s[0] = jnp.zeros((D, LB), f32)
    for buf in (xnT_s, ra_s, lh_s, ol_s, rs_s):
        buf[0:8, 0:64] = jnp.zeros((8, 64), u32)

    LND, BD, MARG = P["LND"], P["BD"], P["MARG"]

    def ln_tasks(b, t, lnd=LND, hsd=P["HSD"]):
        todo = []
        for fn, bb, dur, adv in ((ln, b, lnd, 0.8), (ln, b + 1, lnd, 0.86), (hpair, b, hsd, 1.0)):
            todo.append((t + int(dur * adv), fn, (bb, t, dur)))
            t += int(dur * adv)
        return todo, t

    wait("x0", x0)
    ln(0); ln(1); hpair(0)
    wait("r1", g1)
    left_ = u_early(0, 0, E1, [], 7 * E1 // 4 * 4, -200, 100)
    wait("r2", g2)
    add_tasks(ln_tasks(2, P["L2T"], P["L2D"], P["H2D"])[0])
    n2 = (len(left_) + 7 * (NFP - E1)) // 4 * 4
    left_ = u_early(0, E1, NFP, left_, n2, -200, 120)
    wait("r3", g3)
    left_ = u_early(1, 0, E3, left_, P["N3"], -200, 140)
    wait("wqkv", g4)
    n4 = len(left_) + 7 * (NFP - E3)
    u_early(1, E3, NFP, left_, n4, -200, 100, nsplit=n4 % 4)
    prep_wqkv()
    stage_a(0, split_last=True)
    wait("mid", g5)
    AD = 7 * HA // 2
    UD = 7 * NUP * HD // 4
    r5 = (NP - 1) * AD
    t = 0
    for b in range(UB0, NB, 2):
        todo, t = ln_tasks(b, t)
        add_tasks(todo)
    n5 = 0
    while t + BD + MARG <= r5:
        add_tasks([(t + BD, slot, (t, BD))])
        t += BD
        n5 += 1
    for n, b in enumerate(range(2, NB, 2)):
        stage_a(b, odd=n % 2 == 1, split_last=b == NB - 2)
    wait("fin", g6)
    r6 = NFP * UD
    todo = []
    for i in range(NFP + 1):
        if i == 0:
            t0, dt = -200, 130
        elif i == 1:
            t0, dt = 700, 260
        else:
            t0, dt = (i - 1) * UD + P["US0"], P["USD"]
        if i < NFP:
            for k in range(NUP):
                tt = t0 + k * dt
                todo.append((tt + dt, tsum, (w1_ld(i), (UB0 + 2 * k) * LB, i % 3, k, tt, dt)))
        else:
            for k in range(NFP):
                tt = t0 + k * 300
                todo.append((tt + 300, tsum, (lambda rs: w2_v[0, rs, :], 2 * k * LB, 1, k, tt, 300)))
    left = len(mains) - n5 - P["NQ0"] - P["NQ1"]
    slot_plan = [n5 + left]
    t = P["R6S"]
    bd2 = (r6 - t) // left
    for _ in range(left):
        todo.append((t + min(bd2, 600), slot, (t, min(bd2, 600))))
        t += bd2
    todo.append((r6 - 100, osum, (1, r6 - 500, 400)))
    todo.append((P["PW0"] + P["PWD"], prep_wo, (P["PW0"], P["PWD"])))
    add_tasks(todo)
    for b in range(NB):
        b2f_s[b // 2, 0:1, _blk(b % 2)] = b2_v[b:b + 1, :].astype(f32)
    for i in range(NFP):
        stage_u_last(i, (1, 4, 2, 3, 0, 5, 6) if i == 0 else P["UORD"], P["UED"] if i < NFP - 1 else P["UEL"])
    piece(0, 1, 1, head=4, nqk=P["NQ0"], tskip=P["SK0"])
    piece(1, 2, 2, nqk=P["NQ1"])
    assert slot_ctr[0] == len(mains)
    wait("w2", g7)

    lax.fori_loop(0, 2, c_body, 0)
    outs = [out_copy(pidx, *part) for pidx in range(NP)
            for part in out_parts(pidx >= NPRE and (pidx - NPRE) % NPC == NPC - 1)]
    wait("out", *outs)


@jax.jit
def pallas_parallel_sum__sliding_local_dilated__mixer_token_mlp__prompt_kernel(A_x, A_wqkv, A_wo, B_x, B_w1, B_b1, B_w2, B_b2):
    del B_x
    hbm = pl.BlockSpec(memory_space=pltpu.HBM)
    outT = pl.pallas_call(
        _kernel,
        out_shape=jax.ShapeDtypeStruct((1, D, S), bf16),
        in_specs=[hbm] * 7,
        out_specs=hbm,
        scratch_shapes=[
            pltpu.VMEM((NP, D, 2 * LB), bf16),
            pltpu.VMEM((D, 3 * D), bf16),
            pltpu.VMEM((D, D), bf16),
            pltpu.VMEM((S, F), bf16),
            pltpu.VMEM((NP, F, 2 * LB), bf16),
            pltpu.VMEM((NFB, LB), bf16),
            pltpu.VMEM((NB, LB), bf16),
            pltpu.VMEM((NP, D, 2 * LB), bf16),
            pltpu.VMEM((2, 3 * D, LB), i32),
            pltpu.VMEM((7 * HA // 2, HD), u32),
            pltpu.VMEM((4, D, LB), f32),
            pltpu.VMEM((HD, S), u32),
            pltpu.VMEM((NP * QD, 5 * LB), u32),
            pltpu.VMEM((7 * QD, NP * LB), u32),
            pltpu.VMEM((7 * HD, NFP * LB), f32),
            pltpu.VMEM((7 * QD, KC), u32),
            pltpu.VMEM((NB + 1, 2 * D, LB), f32),
            pltpu.VMEM((NB + 1, D, LB), f32),
            pltpu.VMEM((NB, 2 * W * HH, LB), f32),
            pltpu.VMEM((3 * HD, 2 * LB), u32),
            pltpu.VMEM((D, LB), f32),
            pltpu.VMEM((NP, 32, 2 * LB), f32),
            pltpu.VMEM((5 * RSK, 5 * LB), u32),
            pltpu.SemaphoreType.DMA((9,)),
        ],
        compiler_params=pltpu.CompilerParams(vmem_limit_bytes=100 * 1024 * 1024,
                                             disable_bounds_checks=True,
                                             disable_semaphore_checks=True),
    )(jnp.swapaxes(A_x, 1, 2), A_wqkv, A_wo, B_w1, B_b1.reshape(NFB, LB), B_w2, B_b2.reshape(NB, LB))
    return jnp.swapaxes(outT, 1, 2)
```

```python
import jax
import jax.numpy as jnp
from jax import lax
import jax.experimental.pallas as pl
import jax.experimental.pallas.tpu as pltpu

S, D, F = 2048, 448, 1792
H, DH, W, DIL = 16, 28, 8, 2
LB = 128
NB = S // LB
NP = NB // 2
NFB = F // LB
NFP = NFB // 2
HH = H // 2
WH = W // 2
SH = DIL * WH
HD = D // 2
QD = D // 4
HA = 3 * HD
UB0 = 4
NUP = (NB - UB0) // 2
KC = F // 2 + 2 * LB
RSK = (NFP + 2) * LB // 2
NQ = NFP // 2
KL = NQ * LB + QD
ED = D // 8
RRK = 2 * LB
EPS = 1e-5
SCALE = DH ** -0.5
f32 = jnp.float32
bf16 = jnp.bfloat16
u32 = jnp.uint32
i32 = jnp.int32

SCOPES = False
P = dict(LORD=(4, 2, 1, 3, 0, 5, 6), BOUT=(2, 1, 3, 0), RR0=0, RR1=800, RRM=100, OC1=60,
         BPV=tuple((0.05 + 0.78 * i, 600) for i in range(8)),
         BVB=560, BVD=700, RT=False,
         LND=560, BD=440, G=4, L=4, LS=170, PP=150, MARG=300, N3=40, E3=6, W3T=700, W3D=600, W2T=200, W2D=450, W2X=300, E1=3, L2T=250, L2D=480, H2D=420, PVD=680, PV0=50, HSD=480, HG=80,
         CORD=(4, 2, 1, 3, 0, 5, 6), TS0=100, TSD=420, PVB=520, PVL=500, OS0=3050, OSD=300,
         UORD=(4, 2, 1, 3, 0, 5, 6), US0=100, USD=350, R6S=1900, PVPOS=18, PVD2=400, NQ0=3, NQ1=7, QM1=750, LL0=1200, UR=False, HL=300,
         UE0=-200, UED=2100, UEL=1300, PW0=500, PWD=300, PW1=1300, PWE=400, UG=50, UM=24, PWL=2100, SK0=1500, LNQ1=4, LNQ3=4, LNA=0.3, LNB=0.42, LNBD=0.33)


def _gelu(x, z=None):
    c = 0.7978845608028654
    hx = 0.5 * x
    return hx + hx * jnp.tanh(_orz(x * (c + (c * 0.044715) * (x * x)), z))


def _pk(x):
    return pltpu.bitcast(x.astype(bf16), u32)


def _up(x):
    return pltpu.bitcast(x, bf16)


def _upf(x):
    return pltpu.bitcast(x, bf16).astype(f32)


def _cat(xs, axis):
    return xs[0] if len(xs) == 1 else jnp.concatenate(xs, axis=axis)


def _x2(v):
    return jnp.concatenate([v, v], axis=0)


def _blk(b):
    return slice(b * LB, (b + 1) * LB)


def _rowsum8(a):
    return jnp.broadcast_to(jnp.sum(a, axis=0, keepdims=True), (8, a.shape[1]))


_TRUE = []


def _zero(*deps):
    deps = [d for d in deps if d is not None]
    if not deps:
        return None
    bits = pltpu.bitcast(deps[0], u32)
    for d in deps[1:]:
        bits = bits | pltpu.bitcast(d, u32)
    return bits


def _orz(v, z):
    if z is None:
        return v
    m = _TRUE[0] if v.shape[0] == 8 else _x2(_TRUE[0])
    return jnp.where(m[:, 0:v.shape[1]] > 0, v, pltpu.bitcast(z, v.dtype))


def _pkz(v, z):
    return _pk(v if z is None else jnp.concatenate([_orz(v[0:8], z), v[8:16]], axis=0))


def _lhs_ops(a11, a12, a21, a22):
    return [a11 + a22, a21 + a22, a11, a22, a11 + a12, a21 - a11, a12 - a22]


SIDX = {0: 0, 2: 1, 3: 2, 5: 3, 6: 4}


def _rhs_sums(b11, b12, b21, b22):
    return {0: b11 + b22, 2: b12 - b22, 3: b21 - b11, 5: b11 + b12, 6: b21 + b22}


def _combine(m):
    c12 = m[2] + m[4]
    c21 = m[1] + m[3]
    x = (m[2] - m[1]) + m[0]
    return ((x + m[6]) + (c21 - c12), c12, c21, x + m[5])


def _kernel(x_hbm, wqkv_hbm, wo_hbm, w1_hbm, b1_hbm, w2_hbm, b2_hbm, out_hbm,
            x_v, wqkv_v, wo_v, w1_v, w2_v, b1_v, b2_v, out_v,
            wt_s, lw_s, wo_s, wq_s, xnT_s, ra_s, lh_s, um_s, lc_s, qk_s, v_s, pr_s, ol_s, op_s,
            b2f_s, rs_s, ll_s, rr_s, olc_s, oln_s, one_s, sems):
    sem_ctr = [1]

    class Group:
        def __init__(self, pairs):
            self.cps = [pltpu.make_async_copy(a, b, sems.at[sem_ctr[0]]) for (a, b) in pairs]
            sem_ctr[0] += 1

        def start(self):
            for c in self.cps:
                c.start()

        def wait(self):
            for c in self.cps:
                c.wait()

    def cp_x(p0, p1):
        return [(x_hbm.at[0, :, pl.ds(p * 2 * LB, 2 * LB)], x_v.at[p]) for p in range(p0, p1)]

    def cp_w2(p0, p1):
        return [(w2_hbm.at[:, pl.ds(p * 2 * LB, 2 * LB)], w2_v.at[p]) for p in range(p0, p1)]

    def cp_w1(b0, b1, i0=0, i1=NFP):
        sl = pl.ds(b0 * LB, (b1 - b0) * LB)
        cl = pl.ds(i0 * 2 * LB, (i1 - i0) * 2 * LB)
        return [(w1_hbm.at[sl, cl], w1_v.at[sl, cl])]

    tl = []
    mxu = [0, 0, 0, 0]
    nxt = [0]
    hist = []
    tasks = []
    dls = []
    ready = set()

    def add_tasks(todo):
        tasks.extend(todo)
        tasks.sort(key=lambda x: x[0])

    def flush(t=None):
        while tasks and (t is None or tasks[0][0] < t):
            _, fn, args = tasks.pop(0)
            fn(*args)

    def reset():
        assert not tasks
        dls.clear()
        tl.clear()
        hist.clear()
        mxu[:] = [0, 0, 0, 0]
        nxt[0] = 0

    def now():
        return sum(mxu) // 4

    def wait(name, *cps):
        flush()
        if SCOPES:
            with jax.named_scope("wait_" + name):
                for c in cps:
                    c.wait()
        else:
            for c in cps:
                c.wait()
        reset()

    def mm1(lhs, rhs, pace=True):
        flush(now())
        start = mxu[nxt[0]]
        due = [v for (t, v) in dls if t <= start] if pace else []
        if due:
            dls[:] = [(t, v) for (t, v) in dls if t > start]
            tile = _up(_orz(pltpu.bitcast(lhs[0:16, 0:LB], u32), _zero(*due)))
            row = tile if lhs.shape[1] == LB else jnp.concatenate([tile, lhs[0:16, LB:]], axis=1)
            lhs = jnp.concatenate([row, lhs[16:]], axis=0)
        r = jnp.dot(lhs, rhs, preferred_element_type=f32)
        m, k = lhs.shape
        first_done = None
        for _ in range(-(-rhs.shape[1] // LB)):
            end = 0
            for _ in range(-(-k // LB)):
                mxu[nxt[0]] += m
                end = max(end, mxu[nxt[0]])
                nxt[0] = (nxt[0] + 1) % 4
            if first_done is None:
                first_done = end
        if pace:
            tl.append((first_done - m, first_done, r))
        return r

    def mm(lhs, rhs, init=None):
        k = lhs.shape[1]
        r, k0 = init, 0
        while k0 < k:
            k1 = min(k, k0 + (4 - nxt[0]) * LB)
            part = mm1(lhs[:, k0:k1], rhs[k0:k1], pace=k1 - k0 > LB)
            r = part if r is None else r + part
            k0 = k1
        return r

    def at(t):
        if t is None or t < 0:
            return None
        t = min(t, now() - 1)
        best = None
        for (a, b, r) in tl:
            if a <= t and (best is None or min(b, t) > best[0]):
                row = int(min((t - a) / (b - a), 0.999) * (r.shape[0] // 8)) * 8
                best = (min(b, t), r, row)
        return None if best is None else best[1][best[2]:best[2] + 8, 0:LB]

    def strassen(lhs, rhs, k, order, split_last=False, head=0, init=None):
        m = [None] * 7

        def ops(p, k0, k1):
            flush(now())
            return lhs(p, k0, k1), rhs(p, k0, k1)

        if head:
            for p in order:
                m[p] = mm(*ops(p, 0, head * LB))
        for p in order:
            l, r = ops(p, head * LB, k)
            if split_last and p == order[-1]:
                kk = (-(-r.shape[0] // LB) - 2) * LB
                hm = l.shape[0] // 2
                hd = mm(l[:, :kk], r[:kk]) if kk else None
                tail = jnp.concatenate([mm(l[:hm, kk:], r[kk:]), mm(l[hm:, kk:], r[kk:])], axis=0)
                v = tail if hd is None else hd + tail
            else:
                v = mm(l, r, None if init is None else init[p])
            m[p] = v if m[p] is None else m[p] + v
        return m

    def put_sums(dst, sm, ro, z):
        for p, v in sm.items():
            dst[ro:ro + 8, _blk(SIDX[p])] = _pkz(v, z)

    def tsum(ld, r0, slot_, i, t0, dur):
        for g in range(LB // 16):
            z = _zero(at(t0 + g * dur // 8))
            t1 = ld(slice(r0 + g * 16, r0 + g * 16 + 16)).astype(f32)
            t2 = ld(slice(r0 + LB + g * 16, r0 + LB + g * 16 + 16)).astype(f32)
            sm = _rhs_sums(t1[:, :LB], t1[:, LB:], t2[:, :LB], t2[:, LB:])
            put_sums(rs_s, sm, slot_ * RSK + i * (LB // 2) + g * 8, z)
        ready.add(("rs", slot_, i))

    def osum(slot_, t0, dur):
        ng = HD // 16
        for g in range(ng):
            z = _zero(at(t0 + g * dur // ng))
            r1, r2 = slot_ * HD + g * 8, slot_ * HD + QD + g * 8
            sm = _rhs_sums(_upf(ol_s[r1:r1 + 8, 0:LB]), _upf(ol_s[r1:r1 + 8, LB:]),
                           _upf(ol_s[r2:r2 + 8, 0:LB]), _upf(ol_s[r2:r2 + 8, LB:]))
            put_sums(rs_s, sm, slot_ * RSK + F // 4 + g * 8 + (g // 7) * 8, z)
        ready.update({("rs", slot_, NFP), ("rs", slot_, NFP + 1)})

    def stored_rhs(slot_, p, k0, k1):
        assert all(("rs", slot_, i) in ready for i in range(k0 // LB, -(-k1 // LB))), (slot_, k0, k1)
        return _up(rs_s[slot_ * RSK + k0 // 2:slot_ * RSK + k1 // 2, _blk(SIDX[p])])

    def wrows(hh, g, z=None):
        p, d = divmod(2 * g, DH)
        t = [jnp.concatenate([wt_s[c, pl.ds(p * D + hh * HD + d + e, HH, stride=DH), :]
                              for e in range(2)], axis=0) for c in range(2)]
        if z is not None:
            t = [_orz(v, _x2(z)) for v in t]
        w = jnp.concatenate([t[0], t[1][:, 0:HD - LB]], axis=1)
        return [pltpu.bitcast(w << 16, f32), pltpu.bitcast(w & -65536, f32)]

    def prep_wqkv():
        done = set()
        ng = HA // 16

        def need(hh, p, z=None):
            lo = p * D + hh * HD
            for ct in range(lo // LB, -(-(lo + HD) // LB)):
                if ct in done:
                    continue
                done.add(ct)
                w = min(LB, 3 * D - ct * LB)
                k1, k2 = [pltpu.bitcast(wqkv_v[kh * HD:(kh + 1) * HD, ct * LB:ct * LB + w].astype(f32), i32)
                          for kh in range(2)]
                wd = lax.shift_right_logical(k1, 16) | k2
                if z is not None:
                    wd = jnp.concatenate([_orz(wd[r:r + 8], z[:, 0:w]) if r % LB == 0 else wd[r:r + 8]
                                          for r in range(0, HD, 8)], axis=0)
                wT = wd.T
                wt_s[0, ct * LB:ct * LB + w, :] = wT[:, 0:LB]
                wt_s[1, ct * LB:ct * LB + w, 0:HD - LB] = wT[:, LB:HD]

        def put(p, g, v):
            lw_s[p * (HA // 2) + g * 8:p * (HA // 2) + g * 8 + 8, :] = _pk(v)

        def half(hh, g0, g1, t0=None, dur=None):
            pr, ps = ((2, 4), (3, 1))[hh]
            for g in range(g0, g1):
                t = None if t0 is None else t0 + (g - g0) * dur // (g1 - g0)
                need(hh, 2 * g // DH, _zero(at(None if t is None else t - P["W2X"])))
                a1, a2 = wrows(hh, g, _zero(at(t)))
                put(pr, g, a2 if hh else a1)
                put(ps, g, a1 + a2)
            if g1 == ng:
                ready.update({("lw", pr), ("lw", ps)})
        half(0, 0, ng)
        t, dt = now() + P["W2T"], P["W2D"] // 3
        add_tasks([(t + (n + 1) * dt, half, (1, 14 * n, 14 * n + 14, t + n * dt, dt)) for n in range(3)])

        def rest(g0, g1, t0, dur):
            for g in range(g0, g1):
                z = _zero(at(t0 + (g - g0) * dur // (g1 - g0)))
                ops = _lhs_ops(*wrows(0, g, z), *wrows(1, g, z))
                for p in (0, 5, 6):
                    put(p, g, ops[p])
            if g1 == ng:
                ready.update({("lw", 0), ("lw", 5), ("lw", 6)})
        t, dt = now() + P["W3T"], P["W3D"] // 7
        add_tasks([(t + (n + 1) * dt, rest, (6 * n, 6 * n + 6, t + n * dt, dt)) for n in range(7)])

    def prep_wo_a(t0, dur):
        for g in range(HD // 16):
            k1, k2 = [pltpu.bitcast(wo_v[hh * HD + g * 16:hh * HD + g * 16 + 16, :].astype(f32), i32)
                      for hh in range(2)]
            w = lax.shift_right_logical(k1, 16) | k2
            z = _zero(at(t0 + g * dur // (HD // 16)))
            for c in range(4):
                cw = min(LB, D - c * LB)
                wo_s[c, g * 16:g * 16 + 16, 0:cw] = _orz(w[:, c * LB:c * LB + cw], None if z is None else _x2(z)[:, 0:cw])

    def prep_wo_b(h, t0, dur):
        for c in range(4):
            cw = min(LB, D - c * LB)
            rows = [wo_s[c, pl.ds(d, HH, stride=DH), :][:, 0:cw] for d in range(h * DH // 2, (h + 1) * DH // 2)]
            rows.append(jnp.zeros((LB - QD, cw), i32))
            wq_s[c * LB:c * LB + cw, _blk(h)] = jnp.concatenate(rows, axis=0).T
        bits = None
        for g in range(HD // 16):
            z = _zero(at(t0 + g * dur // (HD // 16)))
            a = []
            for r in (g * 16, HD + g * 16):
                w = _orz(wq_s[r:r + 16, _blk(h)], None if z is None else _x2(z))
                a += [pltpu.bitcast(w << 16, f32), pltpu.bitcast(w & -65536, f32)]
            for p, v in enumerate(_lhs_ops(*a)):
                lc_s[p * QD + g * 8:p * QD + g * 8 + 8, _blk(NFP + h)] = _pk(v)
                bits = pltpu.bitcast(v[0:8], u32) if bits is None else bits | pltpu.bitcast(v[0:8], u32)
        ready.add(("lc", NFP + h))
        dls.append((t0 + dur + 250, bits))

    def llsum(qd, p0, p1, t0, dur):
        i0 = 2 * qd if qd < NQ else NFP
        assert ("lc", i0) in ready and ("lc", i0 + 1) in ready
        n, tot = 0, (p1 - p0) * (QD // 16)
        for p in range(p0, p1):
            for g in range(QD // 16):
                z = _zero(at(t0 + n * dur // tot))
                n += 1
                a = [_orz(lc_s[p * QD + h * ED + g * 8:p * QD + h * ED + g * 8 + 8, _blk(i0 + e)],
                          z if h == e else None) for h in range(2) for e in range(2)]
                ops = _lhs_ops(*[_upf(v) for v in a])
                for q in range(7):
                    r = (p * 7 + q) * ED + g * 8
                    ll_s[r:r + 8, _blk(qd)] = a[0] if q == 2 else a[3] if q == 3 else _pk(ops[q])

    RG = 16
    NG = D // RG
    stat2 = {}

    def ln(b, t0=None, dur=None):
        def dep(fr):
            return None if t0 is None else at(t0 + fr * dur)

        def xg(g):
            return x_v[b // 2, g * RG:(g + 1) * RG, _blk(b % 2)].astype(f32)

        def halves(*vs):
            return [] if vs[0] is None else [v[i * 8:i * 8 + 8] for v in vs for i in range(2)]

        x0 = jnp.broadcast_to(xg(0)[0:1], (8, LB))
        s = q = None
        for g in range(NG):
            if g % P["LNQ1"] == 0 and t0 is not None:
                x0 = _orz(x0, _zero(dep(P["LNA"] * g / NG), *halves(s, q)))
            c = xg(g) - _x2(x0)
            s = c if s is None else s + c
            q = c * c if q is None else q + c * c
        dm = _rowsum8(s) * (1.0 / D)
        mu = x0 + dm
        r1 = lax.rsqrt(jnp.maximum(_rowsum8(q) * (1.0 / D) - dm * dm, 0.0) + EPS)
        s1 = s2 = z = None
        for g in range(NG):
            if g % P["LNQ3"] == 0 and t0 is not None:
                z = _zero(dep(P["LNB"] + P["LNBD"] * g / NG), *halves(s1, s2))
            xn = (xg(g) - _x2(mu)) * _x2(r1)
            xnT_s[g * 8:g * 8 + 8, _blk(b)] = _pkz(xn, z)
            s1 = xn if s1 is None else s1 + xn
            s2 = xn * xn if s2 is None else s2 + xn * xn
        mu2 = _rowsum8(s1) * (1.0 / D)
        var2 = jnp.maximum(_rowsum8(s2) * (1.0 / D) - mu2 * mu2, 0.0)
        stat2[b] = (mu2, lax.rsqrt(var2 + EPS))

    def hpair(b, t0=None, dur=None):
        ng = HD // RG
        st = [stat2.pop(b), stat2.pop(b + 1)]
        for g in range(ng):
            t = None if t0 is None else t0 + g * dur // ng
            zi = _zero(at(None if t is None else t - P["HG"]))
            z = _zero(at(t))
            xq, hq = [], []
            for r in (g * 8, QD + g * 8):
                for e in range(2):
                    xn = _upf(_orz(xnT_s[r:r + 8, _blk(b + e)], zi))
                    xq.append(xn)
                    hq.append((xn - _x2(st[e][0])) * _x2(st[e][1]))
            put_sums(ra_s, _rhs_sums(*xq), (b // 2) * QD + g * 8, z)
            for p, v in enumerate(_lhs_ops(*hq)):
                lh_s[p * QD + g * 8:p * QD + g * 8 + 8, _blk(b // 2)] = _pkz(v, z)
        ready.add(("xn", b))
        if t0 is not None and b >= UB0 and P["HL"]:
            got = ra_s[(b // 2) * QD:(b // 2 + 1) * QD, :]
            tiles_ = [got[r:r + 8, _blk(c)] for r in range(0, QD, 8) for c in range(5)]
            bits = tiles_[0]
            for v in tiles_[1:]:
                bits = bits | v
            dls.append((t0 + dur + P["HL"], bits))

    def w1_ld(i):
        return lambda rs: w1_v[rs, 2 * i * LB:(2 * i + 2) * LB]

    def ujob(kp, i, p, split=False):
        flush(now())
        assert ("xn", 2 * kp) in ready
        l = _up(lh_s[p * QD:(p + 1) * QD, _blk(kp)])
        if p in SIDX:
            r = stored_rhs(3 + kp, p, i * LB, (i + 1) * LB)
        else:
            e = 0 if p == 1 else 1
            r = w1_v[_blk(2 * kp + e), _blk(2 * i + e)]
        v = jnp.concatenate([mm1(l[:QD], r), mm1(l[QD:], r)], axis=0) if split else mm1(l, r)
        rows = slice(p * HD, (p + 1) * HD)
        um_s[rows, _blk(i)] = v if kp == 0 else um_s[rows, _blk(i)] + v

    def u_early(kp, i0, i1, carry, n, t0, dt, nsplit=0):
        for k, i in enumerate(range(i0, i1)):
            add_tasks([(t0 + (k + 1) * dt, tsum, (w1_ld(i), 2 * kp * LB, 3 + kp, i, t0 + k * dt, dt))])
        jobs = (carry + [(kp, i, p) for i in range(i0, i1) for p in (1, 4)]
                + [(kp, i, p) for i in range(i0, i1) for p in SIDX])
        for c, job in enumerate(jobs[:n]):
            ujob(*job, split=c >= n - nsplit)
        return jobs[n:]

    def u_epilogue(i, m, g0, g1, t0, dur):
        for g in range(g0, g1):
            t = t0 + (g - g0) * dur // (g1 - g0)
            z = _zero(at(t))
            if P["UM"] == 0:
                zi = [_zero(at(t - P["UG"]))] * 4
            else:
                zi = [_zero(at(t - P["UG"] - (3 - n) * P["UM"])) for n in range(4)]
            zi = [None if v is None else _x2(v) for v in zi]
            bia = [b1_v[2 * i + e:2 * i + e + 1, :].astype(f32) for e in range(2)]
            top = slice(g * 16, g * 16 + 16)
            q = _combine([x[top] for x in m])
            gl = [_gelu(q[0] + bia[0], zi[3]), _gelu(q[1] + bia[1], zi[0]),
                  _gelu(q[2] + bia[0], zi[1]), _gelu(q[3] + bia[1], zi[2])]
            for p, v in enumerate(_lhs_ops(*gl)):
                lc_s[p * QD + g * 8:p * QD + g * 8 + 8, _blk(i)] = _pkz(v, z if P["UR"] else None)
        if g1 == HD // 16:
            ready.add(("lc", i))

    def stage_u_last(i, order, edur):
        def lhs(p, k0, k1):
            return _up(lh_s[p * QD:(p + 1) * QD, UB0 // 2 * LB + k0:UB0 // 2 * LB + k1])

        def rhs(p, k0, k1):
            if p in SIDX:
                return stored_rhs(i % 3, p, k0, k1)
            e = 0 if p == 1 else 1
            return _cat([w1_v[_blk(UB0 + 2 * k + e), _blk(2 * i + e)] for k in range(k0 // LB, k1 // LB)], 0)
        m = strassen(lhs, rhs, NUP * LB, order, init=[um_s[p * HD:(p + 1) * HD, _blk(i)] for p in range(7)])
        for k in range(NUP):
            ready.discard(("rs", i % 3, k))
        t = now() - P["UE0"]
        ng = HD // 16
        add_tasks([(t + (g + 2) * edur // ng, u_epilogue, (i, m, g, g + 2, t + g * edur // ng, 2 * edur // ng))
                   for g in range(0, ng, 2)])

    def stage_a(b, odd=False, split_last=False):
        def lhs(p, k0, k1):
            assert ("lw", p) in ready
            return _up(lw_s[p * (HA // 2):(p + 1) * (HA // 2), :])

        def rhs(p, k0, k1):
            assert ("xn", b) in ready
            if p in SIDX:
                return _up(ra_s[(b // 2) * QD:(b // 2 + 1) * QD, _blk(SIDX[p])])
            return _up(xnT_s[0:QD, _blk(b)] if p == 1 else xnT_s[QD:HD, _blk(b + 1)])
        order = (6, 4, 2, 1, 3, 0, 5) if odd else (4, 2, 1, 3, 0, 5, 6)
        q = _combine(strassen(lhs, rhs, HD, order, split_last))
        for hh in range(2):
            for e in range(2):
                qk_s[b + e + 1, hh * D:(hh + 1) * D, :] = q[2 * hh + e][0:D]
                v_s[b + e + 1, hh * HD:(hh + 1) * HD, :] = q[2 * hh + e][D:HA]
        ready.update({("qkv", b), ("qkv", b + 1)})

    lane0 = lax.broadcasted_iota(i32, (HH, LB), 1)
    zeros8 = jnp.zeros((HH, LB), f32)

    def mk_shift(*deps):
        lane = _orz(lane0, _zero(*deps))

        def fwd(cur, prev, sh):
            if sh == 0:
                return cur
            return pltpu.roll(jnp.where(lane < LB - sh, cur, prev), sh, 1)

        def bwd(cur, nxt_):
            return pltpu.roll(jnp.where(lane >= SH, cur, nxt_), LB - SH, 1)
        return fwd, bwd

    def grp_shift(t):
        deps = [at(t)]
        if P["L"] and len(hist) >= P["L"]:
            deps += hist[-P["L"]]
        return mk_shift(*deps)

    raw, probs = {}, {}

    def attn_qk(j, hh, t, bd):
        jn = min(j + 1, NB - 1)
        assert ("qkv", jn) in ready
        acc = [None] * WH
        accp = [None] * WH
        for d in range(DH):
            if d % P["G"] == 0:
                if d > 0:
                    hist.append(acc + accp)
                fwd, bwd = grp_shift(t + d * bd // DH)
            r = hh * D + d * HH
            q = qk_s[j + 1, r:r + HH, :]
            qp = bwd(q, qk_s[jn + 1, r:r + HH, :])
            k = qk_s[j + 1, HD + r:HD + r + HH, :]
            kp = qk_s[j, HD + r:HD + r + HH, :] if j > 0 else zeros8
            for a in range(WH):
                ks = fwd(k, kp, DIL * a)
                t0, t1 = q * ks, qp * ks
                acc[a] = t0 if d == 0 else acc[a] + t0
                accp[a] = t1 if d == 0 else accp[a] + t1
        hist.append(acc + accp)
        raw[j, hh] = (acc, accp)

    def attn_sm(j, hh, t):
        fwd, _ = mk_shift(at(t))
        acc, accp = raw[j, hh]
        prev = raw.pop((j - 1, hh))[1] if j > 0 else [zeros8] * WH
        lg = acc + [fwd(accp[a], prev[a], SH) for a in range(WH)]
        lg = [a * SCALE for a in lg]
        if j == 0:
            lg = [lg[0]] + [jnp.where(lane0 >= DIL * w, lg[w], -1e9) for w in range(1, W)]
        m = lg[0]
        for w in range(1, W):
            m = jnp.maximum(m, lg[w])
        e = [jnp.exp(l - m) for l in lg]
        den = e[0]
        for w in range(1, W):
            den = den + e[w]
        inv = 1.0 / den
        p = [x * inv for x in e]
        for a in range(WH):
            pr_s[j, (hh * W + a) * HH:(hh * W + a + 1) * HH, :] = p[a]
        probs[j, hh] = p[WH:]

    def attn_pp(j, hh, t):
        _, bwd = mk_shift(at(t))
        p = probs.pop((j, hh))
        pn = probs[j + 1, hh] if j + 1 < NB else p
        for a in range(WH):
            pr_s[j, (hh * W + WH + a) * HH:(hh * W + WH + a + 1) * HH, :] = bwd(p[a], pn[a])
        ready.add(("pr", j, hh))

    def attn_pv(j, hh, slot_, e, t, bd, t_dl, dst=None):
        dst = ol_s if dst is None else dst
        assert not isinstance(j, int) or ("pr", j, hh) in ready
        pa = [pr_s[j, (hh * W + a) * HH:(hh * W + a + 1) * HH, :] for a in range(W)]
        p, pp = pa[:WH], pa[WH:]
        outs = []
        for d2 in range(DH // 2):
            os_ = []
            for d in (2 * d2, 2 * d2 + 1):
                if d % P["G"] == 0:
                    if d > 0:
                        hist.append([])
                    fwd, _ = grp_shift(t + d * bd // DH)
                r = hh * HD + d * HH
                v = v_s[j + 1, r:r + HH, :]
                vp = v_s[j, r:r + HH, :]
                o = op = None
                for a in range(WH):
                    vs = fwd(v, vp, DIL * a)
                    o = p[a] * vs if a == 0 else o + p[a] * vs
                    op = pp[a] * vs if a == 0 else op + pp[a] * vs
                opp = zeros8 if (isinstance(j, int) and j == 0) else op_s[r:r + HH, :]
                op_s[r:r + HH, :] = op
                os_.append(o + fwd(op, opp, SH))
            ro = slot_ * HD + hh * QD + d2 * HH
            dst[ro:ro + HH, _blk(e)] = _pk(jnp.concatenate(os_, axis=0))
            outs += os_
        hist.append([])
        bits = pltpu.bitcast(outs[0], u32)
        for o in outs[1:]:
            bits = bits | pltpu.bitcast(o, u32)
        dls.append((t_dl, bits))

    mains = [("qk", j, hh) for j in range(NB) for hh in range(2)]
    mains = (mains[:P["PVPOS"]] + [("pv", j, hh) for j in range(8) for hh in range(2)]
             + mains[P["PVPOS"]:] + [None, None])
    slot_ctr = [0]

    def slot(t, bd):
        n = slot_ctr[0]
        slot_ctr[0] += 1
        it = mains[n]
        if it is None:
            pass
        elif it[0] == "qk":
            attn_qk(it[1], it[2], t, bd)
        else:
            j = it[1]
            if j < 4:
                attn_pv(j, it[2], 1 + j // 2, j % 2, t, bd, t + bd + P["PVL"])
                if j % 2 == 1 and it[2] == 1:
                    add_tasks([(t + bd + 800, osum, (1 + j // 2, t + bd + 400, 400))])
            else:
                attn_pv(j, it[2], 0, j - 4, t, bd, t + bd + P["PVL"], olc_s)
        if n >= 1 and mains[n - 1] is not None and mains[n - 1][0] == "qk":
            attn_sm(mains[n - 1][1], mains[n - 1][2], t + P["LS"])
        if n >= 2 and mains[n - 2] is not None and mains[n - 2][0] == "qk":
            _, j, hh = mains[n - 2]
            if j > 0:
                attn_pp(j - 1, hh, t + P["PP"])
            if j == NB - 1:
                attn_pp(j, hh, t + P["PP"])

    NPRE = 2
    CD = 7 * (NFP + 2) * HD // 4

    def out_copy(pidx, e0, e1, r0, r1):
        off = pidx * (2 * LB) + e0 * LB
        if not isinstance(pidx, int):
            off = pl.multiple_of(off, LB)
        rs = pl.ds(r0, r1 - r0)
        return pltpu.make_async_copy(out_v.at[pidx, rs, pl.ds(e0 * LB, (e1 - e0) * LB)],
                                     out_hbm.at[0, rs, pl.ds(off, (e1 - e0) * LB)], sems.at[0])

    def piece(pidx, sl, head=0):
        def lhs(p, k0, k1):
            assert all(("lc", i) in ready for i in range(k0 // LB, k1 // LB)), (k0, k1)
            return _up(lc_s[p * QD:(p + 1) * QD, k0:k1])

        def rhs(p, k0, k1):
            if p in SIDX:
                return stored_rhs(sl, p, k0, k1)
            e = 0 if p == 1 else 1
            parts = [w2_v[pidx, _blk(2 * i + e), _blk(e)] for i in range(k0 // LB, min(NFP, k1 // LB))]
            if k1 == KC:
                for h in range(2):
                    r = sl * HD + e * QD + h * ED
                    parts.append(_up(jnp.concatenate([ol_s[r:r + ED, _blk(e)], jnp.zeros((8, LB), u32)], axis=0)))
            return _cat(parts, 0)
        q = _combine(strassen(lhs, rhs, KC, P["CORD"], head=head))
        for a in range(2):
            rows = slice(a * HD, (a + 1) * HD)
            o = jnp.concatenate(q[2 * a:2 * a + 2], axis=1) + b2f_s[pidx, 0:1, :] + x_v[pidx, rows, :].astype(f32)
            out_v[pidx, rows, :] = o.astype(bf16)
        out_copy(pidx, 0, 2, 0, D).start()

    TOP = {0: ((0, 0), 1, (1, 1)), 1: ((0, 0),), 2: ((0, 1), -1, (1, 1)), 3: ((1, 0), -1, (0, 0)),
           4: ((1, 1),), 5: ((0, 0), 1, (0, 1)), 6: ((1, 0), 1, (1, 1))}

    def top_op(p, blk):
        t = TOP[p]
        if len(t) == 1:
            return blk(*t[0])
        return blk(*t[0]) + blk(*t[2]) if t[1] > 0 else blk(*t[0]) - blk(*t[2])

    def rr_prep(ps, pa, osrc, n0, n1, t0, dur):
        for n in range(n0, n1):
            z = _zero(at(t0 + (n - n0) * dur // (n1 - n0)))
            qd, g = divmod(n, 8)
            cache = {}

            def wblk(i):
                def blk(x, y):
                    if (i, x, y) not in cache:
                        r = (2 * i + x) * LB + g * 16
                        cache[i, x, y] = w2_v[pa + y, r:r + 16, :].astype(f32)
                    return cache[i, x, y]
                return blk

            def oblk(h):
                def blk(x, y):
                    if (h, x, y) not in cache:
                        r = x * QD + h * ED + g * 8
                        cache[h, x, y] = _upf(osrc[r:r + 8, y * 2 * LB:(y + 1) * 2 * LB])
                    return cache[h, x, y]
                return blk
            for p in ps:
                raw_p = p not in SIDX
                ro = p * RRK + g * 8
                if qd == NQ:
                    if not raw_p:
                        r = top_op(p, wblk(2 * NQ))
                        for e in range(2):
                            rr_s[ro:ro + 8, _blk(7 + e)] = _pkz(r[:, _blk(e)], z)
                    continue
                if qd < NQ:
                    r1, r2 = top_op(p, wblk(2 * qd)), top_op(p, wblk(2 * qd + 1))
                    ro += qd * (LB // 2)
                else:
                    r1, r2 = top_op(p, oblk(0)), top_op(p, oblk(1))
                    ro += NQ * (LB // 2)
                z2 = None if z is None else _x2(z)
                if P["RT"]:
                    c11, c22, zo = r1[:, :LB], r2[:, LB:], z
                else:
                    c11, c22, zo = _orz(r1[:, :LB], z2), _orz(r2[:, LB:], z2), None
                sm = _rhs_sums(c11, r1[:, LB:], r2[:, :LB], c22)
                if not raw_p:
                    sm.update({1: c11, 4: c22})
                for q, v in sm.items():
                    rr_s[ro:ro + 8, _blk(q)] = _pkz(v, zo)
        if n1 == NRG:
            ready.update({("rr", p) for p in ps})

    NRG = 8 * (NQ + 1) + 7
    PD = 8 * QD
    BORD = (1, 3, 4, 2, 0, 5, 6)

    def ol_copy(y, t0, dur):
        for r in range(0, HD, 8):
            z = _zero(at(t0 + r * dur // HD)) if r % 32 == 0 else z
            for e in (2 * y, 2 * y + 1):
                olc_s[r:r + 8, _blk(e)] = _orz(oln_s[r:r + 8, _blk(e)], z)

    def rr_tasks(ps, pa, osrc, t0, t1):
        wgt = [8, 8, 8, 2, 7]
        cuts = list(range(0, NRG, 8)) + [NRG]
        todo, acc = [], 0
        for a, b, w in zip(cuts[:-1], cuts[1:], wgt):
            ta, tb = t0 + acc * (t1 - t0) // 33, t0 + (acc + w) * (t1 - t0) // 33
            todo.append((tb, rr_prep, (ps, pa, osrc, a, b, ta, tb - ta)))
            acc += w
        return todo

    def big_piece(pa, pan):
        order = BORD
        t0 = now()
        todo = []
        for n in range(7):
            ta, tb = t0 + n * PD + P["RR0"], t0 + n * PD + P["RR1"]
            if n < 6:
                todo += rr_tasks((order[n + 1],), pa, olc_s, ta, tb)
            else:
                todo += rr_tasks((order[0],), pan, oln_s, ta, tb - P["RRM"])
        todo.append((t0 + 6 * PD + 400, ol_copy, (0, t0 + 6 * PD, 400)))
        todo.append((t0 + 7 * PD - P["OC1"], ol_copy, (1, t0 + 7 * PD - P["OC1"] - 200, 200)))
        for n, (f, bd) in enumerate(P["BPV"]):
            e, hh = divmod(n, 2)
            t = t0 + int(f * PD)
            todo.append((t + bd, attn_pv, (pan * 2 + e, hh, 0, e, t, bd, t + bd + P["PVL"], oln_s)))
        add_tasks(todo)
        m = [None] * 7
        for p in order:
            flush(now())
            assert ("rr", p) in ready
            ready.discard(("rr", p))
            x, y = TOP[p][0]

            def lhs(q, k0, k1):
                return _up(ll_s[(p * 7 + q) * ED:(p * 7 + q + 1) * ED, 0:KL])

            def rhs(q, k0, k1):
                if p in SIDX or q in SIDX:
                    return _up(rr_s[p * RRK:p * RRK + KL // 2, _blk(q)])
                h = 0 if q == 1 else 1
                return _cat([w2_v[pa + y, _blk(2 * (2 * qd + h) + x), _blk(h)] for qd in range(NQ)]
                            + [_up(olc_s[x * QD + h * ED:x * QD + (h + 1) * ED, _blk(2 * y + h)])], 0)
            rl = (_up(rr_s[p * RRK:p * RRK + LB // 2, 7 * LB:9 * LB]) if p in SIDX
                  else w2_v[pa + y, _blk(4 * NQ + x), :])
            ll = _up(lc_s[p * QD:(p + 1) * QD, _blk(2 * NQ)])
            ex = [mm1(ll[:QD], rl), mm1(ll[QD:], rl)]
            c = _combine(strassen(lhs, rhs, KL, P["LORD"]))
            m[p] = jnp.concatenate([jnp.concatenate(c[0:2], axis=1) + ex[0],
                                    jnp.concatenate(c[2:4], axis=1) + ex[1]], axis=0)
        flush()
        q = _combine(m)
        for n in P["BOUT"]:
            a, y = divmod(n, 2)
            rows = slice(a * HD, (a + 1) * HD)
            o = q[n] + b2f_s[pa + y, 0:1, :] + x_v[pa + y, rows, :].astype(f32)
            out_v[pa + y, rows, :] = o.astype(bf16)
            out_copy(pa + y, 0, 2, a * HD, (a + 1) * HD).start()

    def c_body(it, carry):
        reset()
        _TRUE[:] = [one_s[...]]
        ready.add(("rr", BORD[0]))
        pa = NPRE + 2 * it
        big_piece(pa, lax.rem(pa + 2, NP))
        return carry

    x0 = Group(cp_x(0, 1))
    E1 = P["E1"]
    g1 = Group(cp_w1(0, 2, 0, E1))
    g2 = Group(cp_w1(0, 2, E1, NFP) + cp_x(1, 2))
    E3 = P["E3"]
    g3 = Group(cp_w1(2, UB0, 0, E3))
    g4 = Group((cp_w1(2, UB0, E3, NFP) if E3 < NFP else []) + [(wqkv_hbm, wqkv_v)])
    g5 = Group(cp_x(2, NP))
    g6 = Group(cp_w1(UB0, NB) + [(wo_hbm, wo_v), (b1_hbm, b1_v), (b2_hbm, b2_v)] + cp_w2(0, NPRE + 1))
    g7 = Group(cp_w2(NPRE + 1, NP))
    for c in (x0, g1, g2, g3, g4, g5, g6, g7):
        c.start()

    v_s[0] = jnp.zeros((D, LB), f32)
    for sl in (1, 2):
        for h in range(2):
            r = sl * RSK + F // 4 + h * (LB // 2) + ED
            rs_s[r:r + 8, :] = jnp.zeros((8, 5 * LB), u32)
    for buf in (xnT_s, ra_s, lh_s, ol_s, rs_s, rr_s, olc_s, oln_s, ll_s, lc_s):
        buf[0:8, 0:64] = jnp.zeros((8, 64), u32)

    LND, BD, MARG = P["LND"], P["BD"], P["MARG"]

    def ln_tasks(b, t, lnd=LND, hsd=P["HSD"]):
        todo = []
        for fn, bb, dur, adv in ((ln, b, lnd, 0.8), (ln, b + 1, lnd, 0.86), (hpair, b, hsd, 1.0)):
            todo.append((t + int(dur * adv), fn, (bb, t, dur)))
            t += int(dur * adv)
        return todo, t

    wait("x0", x0)
    one_s[...] = lax.shift_right_logical(pltpu.bitcast(x_v[0, 0:16, 0:LB], i32), 1) | 1
    _TRUE[:] = [one_s[...]]
    ln(0); ln(1); hpair(0)
    wait("r1", g1)
    left_ = u_early(0, 0, E1, [], 7 * E1 // 4 * 4, -200, 100)
    wait("r2", g2)
    add_tasks(ln_tasks(2, P["L2T"], P["L2D"], P["H2D"])[0])
    n2 = (len(left_) + 7 * (NFP - E1)) // 4 * 4
    left_ = u_early(0, E1, NFP, left_, n2, -200, 120)
    wait("r3", g3)
    left_ = u_early(1, 0, E3, left_, P["N3"], -200, 140)
    wait("wqkv", g4)
    n4 = len(left_) + 7 * (NFP - E3)
    u_early(1, E3, NFP, left_, n4, -200, 100, nsplit=n4 % 4)
    prep_wqkv()
    stage_a(0, split_last=True)
    wait("mid", g5)
    AD = 7 * HA // 2
    UD = 7 * NUP * HD // 4
    r5 = (NP - 1) * AD
    t = 0
    for b in range(UB0, NB, 2):
        todo, t = ln_tasks(b, t)
        add_tasks(todo)
    n5 = 0
    while t + BD + MARG <= r5:
        add_tasks([(t + BD, slot, (t, BD))])
        t += BD
        n5 += 1
    for n, b in enumerate(range(2, NB, 2)):
        stage_a(b, odd=n % 2 == 1, split_last=b == NB - 2)
    wait("fin", g6)
    r6 = NFP * UD
    todo = []
    for i in range(NFP + 1):
        if i == 0:
            t0, dt = -200, 130
        elif i == 1:
            t0, dt = 700, 260
        else:
            t0, dt = (i - 1) * UD + P["US0"], P["USD"]
        if i < NFP:
            for k in range(NUP):
                tt = t0 + k * dt
                todo.append((tt + dt, tsum, (w1_ld(i), (UB0 + 2 * k) * LB, i % 3, k, tt, dt)))
        else:
            for k in range(NFP):
                tt = t0 + k * 300
                todo.append((tt + 300, tsum, (lambda rs: w2_v[0, rs, :], 2 * k * LB, 1, k, tt, 300)))
    for k in range(NFP):
        tt = r6 + P["TS0"] + k * P["TSD"]
        todo.append((tt + P["TSD"], tsum, (lambda rs: w2_v[1, rs, :], 2 * k * LB, 2, k, tt, P["TSD"])))
    left = len(mains) - n5 - P["NQ0"] - P["NQ1"]
    t = P["R6S"]
    bd2 = (r6 - t) // left
    for _ in range(left):
        todo.append((t + min(bd2, 600), slot, (t, min(bd2, 600))))
        t += bd2
    for t, t1, n in ((r6 + P["SK0"], r6 + CD, P["NQ0"]), (r6 + CD, r6 + 2 * CD - P["QM1"], P["NQ1"] - 2)):
        bd = (t1 - t) // max(n, 1)
        for i in range(n):
            todo.append((t + i * bd + min(bd, 600), slot, (t + i * bd, min(bd, 600))))
    for i in range(2):
        t = r6 + 2 * CD - P["QM1"] + i * 300
        todo.append((t + 300, slot, (t, 300)))
    t, dt = r6 + P["LL0"], (2 * CD - P["LL0"] - 200) // (7 * (NQ + 1))
    for qd in range(NQ + 1):
        for p in range(7):
            todo.append((t + dt, llsum, (qd, p, p + 1, t, dt)))
            t += dt
    todo += rr_tasks((BORD[0],), NPRE, olc_s, r6 + CD + 300, r6 + 2 * CD - 300)
    todo.append((P["PW0"] + P["PWD"], prep_wo_a, (P["PW0"], P["PWD"])))
    for h in range(2):
        t = P["PW1"] + h * P["PWE"]
        todo.append((t + P["PWE"], prep_wo_b, (h, t, P["PWE"])))
    add_tasks(todo)
    for b in range(NB):
        b2f_s[b // 2, 0:1, _blk(b % 2)] = b2_v[b:b + 1, :].astype(f32)
    for i in range(NFP):
        stage_u_last(i, (1, 4, 2, 3, 0, 5, 6) if i == 0 else P["UORD"], P["UED"] if i < NFP - 1 else P["UEL"])
    piece(0, 1, head=4)
    piece(1, 2)
    flush()
    assert slot_ctr[0] == len(mains)
    wait("w2", g7)

    lax.fori_loop(0, (NP - NPRE) // 2, c_body, 0)
    outs = [out_copy(pidx, 0, 2, 0, D) for pidx in range(NPRE)]
    outs += [out_copy(pidx, 0, 2, a * HD, (a + 1) * HD) for pidx in range(NPRE, NP) for a in range(2)]
    wait("out", *outs)


@jax.jit
def pallas_parallel_sum__sliding_local_dilated__mixer_token_mlp__prompt_kernel(A_x, A_wqkv, A_wo, B_x, B_w1, B_b1, B_w2, B_b2):
    del B_x
    hbm = pl.BlockSpec(memory_space=pltpu.HBM)
    outT = pl.pallas_call(
        _kernel,
        out_shape=jax.ShapeDtypeStruct((1, D, S), bf16),
        in_specs=[hbm] * 7,
        out_specs=hbm,
        scratch_shapes=[
            pltpu.VMEM((NP, D, 2 * LB), bf16),
            pltpu.VMEM((D, 3 * D), bf16),
            pltpu.VMEM((D, D), bf16),
            pltpu.VMEM((S, F), bf16),
            pltpu.VMEM((NP, F, 2 * LB), bf16),
            pltpu.VMEM((NFB, LB), bf16),
            pltpu.VMEM((NB, LB), bf16),
            pltpu.VMEM((NP, D, 2 * LB), bf16),
            pltpu.VMEM((2, 3 * D, LB), i32),
            pltpu.VMEM((7 * HA // 2, HD), u32),
            pltpu.VMEM((4, HD, LB), i32),
            pltpu.VMEM((D, 2 * LB), i32),
            pltpu.VMEM((HD, S), u32),
            pltpu.VMEM((NP * QD, 5 * LB), u32),
            pltpu.VMEM((7 * QD, NP * LB), u32),
            pltpu.VMEM((7 * HD, NFP * LB), f32),
            pltpu.VMEM((7 * QD, KC), u32),
            pltpu.VMEM((NB + 1, 2 * D, LB), f32),
            pltpu.VMEM((NB + 1, D, LB), f32),
            pltpu.VMEM((NB, 2 * W * HH, LB), f32),
            pltpu.VMEM((3 * HD, 2 * LB), u32),
            pltpu.VMEM((D, LB), f32),
            pltpu.VMEM((NP, 32, 2 * LB), f32),
            pltpu.VMEM((5 * RSK, 5 * LB), u32),
            pltpu.VMEM((49 * ED, 4 * LB), u32),
            pltpu.VMEM((7 * RRK, 9 * LB), u32),
            pltpu.VMEM((HD, 4 * LB), u32),
            pltpu.VMEM((HD, 4 * LB), u32),
            pltpu.VMEM((8, LB), i32),
            pltpu.SemaphoreType.DMA((9,)),
        ],
        compiler_params=pltpu.CompilerParams(vmem_limit_bytes=100 * 1024 * 1024,
                                             disable_bounds_checks=True,
                                             disable_semaphore_checks=True),
    )(jnp.swapaxes(A_x, 1, 2), A_wqkv, A_wo, B_w1, B_b1.reshape(NFB, LB), B_w2, B_b2.reshape(NB, LB))
    return jnp.swapaxes(outT, 1, 2)
```

```python
import jax
import jax.numpy as jnp
from jax import lax
import jax.experimental.pallas as pl
import jax.experimental.pallas.tpu as pltpu

S, D, F = 2048, 448, 1792
H, DH, W, DIL = 16, 28, 8, 2
LB = 128
NB = S // LB
NP = NB // 2
NFB = F // LB
NFP = NFB // 2
HH = H // 2
WH = W // 2
SH = DIL * WH
HD = D // 2
QD = D // 4
HA = 3 * HD
UB0 = 4
NUP = (NB - UB0) // 2
KC = F // 2 + 2 * LB
RSK = NFP * LB // 2
NQ = NFP // 2
KL = NQ * LB + QD
ED = D // 8
RRK = 2 * LB
EPS = 1e-5
SCALE = DH ** -0.5
f32 = jnp.float32
bf16 = jnp.bfloat16
u32 = jnp.uint32
i32 = jnp.int32

SCOPES = False
P = dict(LORD=(4, 2, 1, 3, 0, 5, 6), EP0=50, EPD=700, RR0=0, RR1=800, RRM=100, OC1=60,
         BPV=tuple((0.05 + 0.8 * i, 620) for i in range(8)),
         BVB=560, BVD=700, RT=False,
         LND=400, BD=370, G=4, L=4, LS=170, PP=150, MARG=300, N3=40, E3=6, W3T=700, W3D=600, W2T=200, W2D=450, W2X=300, E1=3, L2T=250, L2D=480, H2D=420, PVD=680, PV0=50, HSD=360, HG=0,
         CORD=(4, 2, 1, 3, 0, 5, 6), TS0=100, TSD=420, PVB=520, PVL=500, OS0=3050, OSD=300,
         UORD=(4, 2, 1, 3, 0, 5, 6), US0=100, USD=350, R6S=1900, PVPOS=12, R6E=3000, LL2=500, RP0=2500, RP1=11000, PVD2=400, NQ0=3, NQ1=7, QM1=750, LL0=1200, UR=False, HR=False, LNI=True, TI=False, HL=300,
         UE0=-200, UED=2100, UEL=1400, PW0=500, PWD=300, PW1=1300, PWE=400, UG=50, UM=24, PWL=2100, SK0=1500, LNQ1=4, LNQ3=4, LNA=0.3, LNB=0.42, LNBD=0.33)


def _gelu(x, z=None):
    c = 0.7978845608028654
    hx = 0.5 * x
    return hx + hx * jnp.tanh(_orz(x * (c + (c * 0.044715) * (x * x)), z))


def _pk(x):
    return pltpu.bitcast(x.astype(bf16), u32)


def _up(x):
    return pltpu.bitcast(x, bf16)


def _upf(x):
    return pltpu.bitcast(x, bf16).astype(f32)


def _cat(xs, axis):
    return xs[0] if len(xs) == 1 else jnp.concatenate(xs, axis=axis)


def _x2(v):
    return jnp.concatenate([v, v], axis=0)


def _blk(b):
    return slice(b * LB, (b + 1) * LB)


def _rowsum8(a):
    return jnp.broadcast_to(jnp.sum(a, axis=0, keepdims=True), (8, a.shape[1]))


_TRUE = []


def _zero(*deps):
    deps = [d for d in deps if d is not None]
    if not deps:
        return None
    bits = pltpu.bitcast(deps[0], u32)
    for d in deps[1:]:
        bits = bits | pltpu.bitcast(d, u32)
    return bits


def _orz(v, z):
    if z is None:
        return v
    m = _TRUE[0] if v.shape[0] == 8 else _x2(_TRUE[0])
    return jnp.where(m[:, 0:v.shape[1]] > 0, v, pltpu.bitcast(z, v.dtype))


def _pkz(v, z):
    return _pk(v if z is None else jnp.concatenate([_orz(v[0:8], z), v[8:16]], axis=0))


def _lhs_ops(a11, a12, a21, a22):
    return [a11 + a22, a21 + a22, a11, a22, a11 + a12, a21 - a11, a12 - a22]


SIDX = {0: 0, 2: 1, 3: 2, 5: 3, 6: 4}


def _rhs_sums(b11, b12, b21, b22):
    return {0: b11 + b22, 2: b12 - b22, 3: b21 - b11, 5: b11 + b12, 6: b21 + b22}


def _combine(m):
    c12 = m[2] + m[4]
    c21 = m[1] + m[3]
    x = (m[2] - m[1]) + m[0]
    return ((x + m[6]) + (c21 - c12), c12, c21, x + m[5])


def _kernel(x_hbm, wqkv_hbm, wo_hbm, w1_hbm, b1_hbm, w2_hbm, b2_hbm, out_hbm,
            x_v, wqkv_v, wo_v, w1_v, w2_v, b1_v, b2_v, out_v,
            wt_s, lw_s, wo_s, wq_s, xnT_s, ra_s, lh_s, um_s, lc_s, qk_s, v_s, pr_s, op_s,
            b2f_s, rs_s, ll_s, rr_s, ola_s, olb_s, one_s, sems):
    sem_ctr = [1]

    class Group:
        def __init__(self, pairs):
            self.cps = [pltpu.make_async_copy(a, b, sems.at[sem_ctr[0]]) for (a, b) in pairs]
            sem_ctr[0] += 1

        def start(self):
            for c in self.cps:
                c.start()

        def wait(self):
            for c in self.cps:
                c.wait()

    def cp_x(p0, p1):
        return [(x_hbm.at[0, :, pl.ds(p * 2 * LB, 2 * LB)], x_v.at[p]) for p in range(p0, p1)]

    def cp_w2(p0, p1):
        return [(w2_hbm.at[:, pl.ds(p * 2 * LB, 2 * LB)], w2_v.at[p]) for p in range(p0, p1)]

    def cp_w1(b0, b1, i0=0, i1=NFP):
        sl = pl.ds(b0 * LB, (b1 - b0) * LB)
        cl = pl.ds(i0 * 2 * LB, (i1 - i0) * 2 * LB)
        return [(w1_hbm.at[sl, cl], w1_v.at[sl, cl])]

    tl = []
    mxu = [0, 0, 0, 0]
    nxt = [0]
    hist = []
    tasks = []
    dls = []
    ready = set()

    def add_tasks(todo):
        tasks.extend(todo)
        tasks.sort(key=lambda x: x[0])

    def flush(t=None):
        while tasks and (t is None or tasks[0][0] < t):
            _, fn, args = tasks.pop(0)
            fn(*args)

    def reset():
        assert not tasks
        dls.clear()
        tl.clear()
        hist.clear()
        mxu[:] = [0, 0, 0, 0]
        nxt[0] = 0

    def now():
        return sum(mxu) // 4

    def wait(name, *cps):
        flush()
        if SCOPES:
            with jax.named_scope("wait_" + name):
                for c in cps:
                    c.wait()
        else:
            for c in cps:
                c.wait()
        reset()

    def mm1(lhs, rhs, pace=True):
        flush(now())
        start = mxu[nxt[0]]
        due = [v for (t, v) in dls if t <= start] if pace else []
        if due:
            dls[:] = [(t, v) for (t, v) in dls if t > start]
            tile = _up(_orz(pltpu.bitcast(lhs[0:16, 0:LB], u32), _zero(*due)))
            row = tile if lhs.shape[1] == LB else jnp.concatenate([tile, lhs[0:16, LB:]], axis=1)
            lhs = jnp.concatenate([row, lhs[16:]], axis=0)
        r = jnp.dot(lhs, rhs, preferred_element_type=f32)
        m, k = lhs.shape
        first_done = None
        for _ in range(-(-rhs.shape[1] // LB)):
            end = 0
            for _ in range(-(-k // LB)):
                mxu[nxt[0]] += m
                end = max(end, mxu[nxt[0]])
                nxt[0] = (nxt[0] + 1) % 4
            if first_done is None:
                first_done = end
        if pace:
            tl.append((first_done - m, first_done, r))
        return r

    def mm(lhs, rhs, init=None):
        k = lhs.shape[1]
        r, k0 = init, 0
        while k0 < k:
            k1 = min(k, k0 + (4 - nxt[0]) * LB)
            part = mm1(lhs[:, k0:k1], rhs[k0:k1], pace=k1 - k0 > LB)
            r = part if r is None else r + part
            k0 = k1
        return r

    def at(t):
        if t is None or t < 0:
            return None
        t = min(t, now() - 1)
        best = None
        for (a, b, r) in tl:
            if a <= t and (best is None or min(b, t) > best[0]):
                row = int(min((t - a) / (b - a), 0.999) * (r.shape[0] // 8)) * 8
                best = (min(b, t), r, row)
        return None if best is None else best[1][best[2]:best[2] + 8, 0:LB]

    def strassen(lhs, rhs, k, order, split_last=False, head=0, init=None):
        m = [None] * 7

        def ops(p, k0, k1):
            flush(now())
            return lhs(p, k0, k1), rhs(p, k0, k1)

        if head:
            for p in order:
                m[p] = mm(*ops(p, 0, head * LB))
        for p in order:
            l, r = ops(p, head * LB, k)
            if split_last and p == order[-1]:
                kk = (-(-r.shape[0] // LB) - 2) * LB
                hm = l.shape[0] // 2
                hd = mm(l[:, :kk], r[:kk], None if init is None else init[p]) if kk else None
                tail = jnp.concatenate([mm(l[:hm, kk:], r[kk:]), mm(l[hm:, kk:], r[kk:])], axis=0)
                v = tail if hd is None else hd + tail
            else:
                v = mm(l, r, None if init is None else init[p])
            m[p] = v if m[p] is None else m[p] + v
        return m

    def put_sums(dst, sm, ro, z):
        for p, v in sm.items():
            dst[ro:ro + 8, _blk(SIDX[p])] = _pkz(v, z)

    def tsum(ld, r0, slot_, i, t0, dur):
        for g in range(LB // 16):
            z = _zero(at(t0 + g * dur // 8))
            t1 = ld(slice(r0 + g * 16, r0 + g * 16 + 16)).astype(f32)
            t2 = ld(slice(r0 + LB + g * 16, r0 + LB + g * 16 + 16)).astype(f32)
            if P["TI"] and z is not None:
                sm = _rhs_sums(_orz(t1[:, :LB], _x2(z)), t1[:, LB:], t2[:, :LB], _orz(t2[:, LB:], _x2(z)))
                z = None
            else:
                sm = _rhs_sums(t1[:, :LB], t1[:, LB:], t2[:, :LB], t2[:, LB:])
            put_sums(rs_s, sm, slot_ * RSK + i * (LB // 2) + g * 8, z)
        ready.add(("rs", slot_, i))

    def stored_rhs(slot_, p, k0, k1):
        assert all(("rs", slot_, i) in ready for i in range(k0 // LB, -(-k1 // LB))), (slot_, k0, k1)
        return _up(rs_s[slot_ * RSK + k0 // 2:slot_ * RSK + k1 // 2, _blk(SIDX[p])])

    def wrows(hh, g, z=None):
        p, d = divmod(2 * g, DH)
        t = [jnp.concatenate([wt_s[c, pl.ds(p * D + hh * HD + d + e, HH, stride=DH), :]
                              for e in range(2)], axis=0) for c in range(2)]
        if z is not None:
            t = [_orz(v, _x2(z)) for v in t]
        w = jnp.concatenate([t[0], t[1][:, 0:HD - LB]], axis=1)
        return [pltpu.bitcast(w << 16, f32), pltpu.bitcast(w & -65536, f32)]

    def prep_wqkv():
        done = set()
        ng = HA // 16

        def need(hh, p, z=None):
            lo = p * D + hh * HD
            for ct in range(lo // LB, -(-(lo + HD) // LB)):
                if ct in done:
                    continue
                done.add(ct)
                w = min(LB, 3 * D - ct * LB)
                k1, k2 = [pltpu.bitcast(wqkv_v[kh * HD:(kh + 1) * HD, ct * LB:ct * LB + w].astype(f32), i32)
                          for kh in range(2)]
                wd = lax.shift_right_logical(k1, 16) | k2
                if z is not None:
                    wd = jnp.concatenate([_orz(wd[r:r + 8], z[:, 0:w]) if r % LB == 0 else wd[r:r + 8]
                                          for r in range(0, HD, 8)], axis=0)
                wT = wd.T
                wt_s[0, ct * LB:ct * LB + w, :] = wT[:, 0:LB]
                wt_s[1, ct * LB:ct * LB + w, 0:HD - LB] = wT[:, LB:HD]

        def put(p, g, v):
            lw_s[p * (HA // 2) + g * 8:p * (HA // 2) + g * 8 + 8, :] = _pk(v)

        def half(hh, g0, g1, t0=None, dur=None):
            pr, ps = ((2, 4), (3, 1))[hh]
            for g in range(g0, g1):
                t = None if t0 is None else t0 + (g - g0) * dur // (g1 - g0)
                need(hh, 2 * g // DH, _zero(at(None if t is None else t - P["W2X"])))
                a1, a2 = wrows(hh, g, _zero(at(t)))
                put(pr, g, a2 if hh else a1)
                put(ps, g, a1 + a2)
            if g1 == ng:
                ready.update({("lw", pr), ("lw", ps)})
        half(0, 0, ng)
        t, dt = now() + P["W2T"], P["W2D"] // 3
        add_tasks([(t + (n + 1) * dt, half, (1, 14 * n, 14 * n + 14, t + n * dt, dt)) for n in range(3)])

        def rest(g0, g1, t0, dur):
            for g in range(g0, g1):
                z = _zero(at(t0 + (g - g0) * dur // (g1 - g0)))
                ops = _lhs_ops(*wrows(0, g, z), *wrows(1, g, z))
                for p in (0, 5, 6):
                    put(p, g, ops[p])
            if g1 == ng:
                ready.update({("lw", 0), ("lw", 5), ("lw", 6)})
        t, dt = now() + P["W3T"], P["W3D"] // 7
        add_tasks([(t + (n + 1) * dt, rest, (6 * n, 6 * n + 6, t + n * dt, dt)) for n in range(7)])

    def prep_wo_a(t0, dur):
        for g in range(HD // 16):
            k1, k2 = [pltpu.bitcast(wo_v[hh * HD + g * 16:hh * HD + g * 16 + 16, :].astype(f32), i32)
                      for hh in range(2)]
            w = lax.shift_right_logical(k1, 16) | k2
            z = _zero(at(t0 + g * dur // (HD // 16)))
            for c in range(4):
                cw = min(LB, D - c * LB)
                wo_s[c, g * 16:g * 16 + 16, 0:cw] = _orz(w[:, c * LB:c * LB + cw], None if z is None else _x2(z)[:, 0:cw])

    def prep_wo_b(h, t0, dur):
        for c in range(4):
            cw = min(LB, D - c * LB)
            rows = [wo_s[c, pl.ds(d, HH, stride=DH), :][:, 0:cw] for d in range(h * DH // 2, (h + 1) * DH // 2)]
            rows.append(jnp.zeros((LB - QD, cw), i32))
            wq_s[c * LB:c * LB + cw, _blk(h)] = jnp.concatenate(rows, axis=0).T
        bits = None
        for g in range(HD // 16):
            z = _zero(at(t0 + g * dur // (HD // 16)))
            a = []
            for r in (g * 16, HD + g * 16):
                w = _orz(wq_s[r:r + 16, _blk(h)], None if z is None else _x2(z))
                a += [pltpu.bitcast(w << 16, f32), pltpu.bitcast(w & -65536, f32)]
            for p, v in enumerate(_lhs_ops(*a)):
                lc_s[p * QD + g * 8:p * QD + g * 8 + 8, _blk(NFP + h)] = _pk(v)
                bits = pltpu.bitcast(v[0:8], u32) if bits is None else bits | pltpu.bitcast(v[0:8], u32)
        ready.update({("lc", NFP + h, g) for g in range(HD // 16)})
        dls.append((t0 + dur + 250, bits))

    def llsum(qd, g, t0, dur):
        i0 = 2 * qd if qd < NQ else NFP
        assert all(("lc", i0 + e, g + 7 * h) in ready for e in range(2) for h in range(2))
        for p in range(7):
            z = _zero(at(t0 + p * dur // 7))
            a = [_orz(lc_s[p * QD + h * ED + g * 8:p * QD + h * ED + g * 8 + 8, _blk(i0 + e)],
                      z if h == e else None) for h in range(2) for e in range(2)]
            ops = _lhs_ops(*[_upf(v) for v in a])
            for q in (0, 1, 4, 5, 6):
                r = (p * 7 + q) * ED + g * 8
                ll_s[r:r + 8, _blk(qd)] = _pk(ops[q])
        ready.add(("ll", qd, g))

    RG = 16
    NG = D // RG
    stat2 = {}

    def ln(b, t0=None, dur=None):
        def dep(fr):
            return None if t0 is None else at(t0 + fr * dur)

        def xg(g):
            return x_v[b // 2, g * RG:(g + 1) * RG, _blk(b % 2)].astype(f32)

        def halves(*vs):
            return [] if vs[0] is None else [v[i * 8:i * 8 + 8] for v in vs for i in range(2)]

        x0 = jnp.broadcast_to(xg(0)[0:1], (8, LB))
        s = q = None
        for g in range(NG):
            if g % P["LNQ1"] == 0 and t0 is not None:
                x0 = _orz(x0, _zero(dep(P["LNA"] * g / NG), *halves(s, q)))
            c = xg(g) - _x2(x0)
            s = c if s is None else s + c
            q = c * c if q is None else q + c * c
        dm = _rowsum8(s) * (1.0 / D)
        mu = x0 + dm
        r1 = lax.rsqrt(jnp.maximum(_rowsum8(q) * (1.0 / D) - dm * dm, 0.0) + EPS)
        s1 = s2 = z = None
        for g in range(NG):
            if g % P["LNQ3"] == 0 and t0 is not None:
                z = _zero(dep(P["LNB"] + P["LNBD"] * g / NG), *halves(s1, s2))
                if P["LNI"]:
                    mu, z = _orz(mu, z), None
            xn = (xg(g) - _x2(mu)) * _x2(r1)
            xnT_s[g * 8:g * 8 + 8, _blk(b)] = _pkz(xn, z)
            s1 = xn if s1 is None else s1 + xn
            s2 = xn * xn if s2 is None else s2 + xn * xn
        mu2 = _rowsum8(s1) * (1.0 / D)
        var2 = jnp.maximum(_rowsum8(s2) * (1.0 / D) - mu2 * mu2, 0.0)
        stat2[b] = (mu2, lax.rsqrt(var2 + EPS))

    def hpair(b, t0=None, dur=None):
        ng = HD // RG
        st = [stat2.pop(b), stat2.pop(b + 1)]
        for g in range(ng):
            t = None if t0 is None else t0 + g * dur // ng
            zi = _zero(at(None if t is None else t - P["HG"]))
            z = _zero(at(t)) if P["HR"] else None
            xq, hq = [], []
            for r in (g * 8, QD + g * 8):
                for e in range(2):
                    xn = _upf(_orz(xnT_s[r:r + 8, _blk(b + e)], zi))
                    xq.append(xn)
                    hq.append((xn - _x2(st[e][0])) * _x2(st[e][1]))
            put_sums(ra_s, _rhs_sums(*xq), (b // 2) * QD + g * 8, z)
            for p, v in enumerate(_lhs_ops(*hq)):
                lh_s[p * QD + g * 8:p * QD + g * 8 + 8, _blk(b // 2)] = _pkz(v, z)
        ready.add(("xn", b))
        if t0 is not None and b >= UB0 and P["HL"]:
            got = ra_s[(b // 2) * QD:(b // 2 + 1) * QD, :]
            tiles_ = [got[r:r + 8, _blk(c)] for r in range(0, QD, 8) for c in range(5)]
            bits = tiles_[0]
            for v in tiles_[1:]:
                bits = bits | v
            dls.append((t0 + dur + P["HL"], bits))

    def w1_ld(i):
        return lambda rs: w1_v[rs, 2 * i * LB:(2 * i + 2) * LB]

    def ujob(kp, i, p, split=False):
        flush(now())
        assert ("xn", 2 * kp) in ready
        l = _up(lh_s[p * QD:(p + 1) * QD, _blk(kp)])
        if p in SIDX:
            r = stored_rhs(3 + kp, p, i * LB, (i + 1) * LB)
        else:
            e = 0 if p == 1 else 1
            r = w1_v[_blk(2 * kp + e), _blk(2 * i + e)]
        v = jnp.concatenate([mm1(l[:QD], r), mm1(l[QD:], r)], axis=0) if split else mm1(l, r)
        rows = slice(p * HD, (p + 1) * HD)
        um_s[rows, _blk(i)] = v if kp == 0 else um_s[rows, _blk(i)] + v

    def u_early(kp, i0, i1, carry, n, t0, dt, nsplit=0):
        for k, i in enumerate(range(i0, i1)):
            add_tasks([(t0 + (k + 1) * dt, tsum, (w1_ld(i), 2 * kp * LB, 3 + kp, i, t0 + k * dt, dt))])
        jobs = (carry + [(kp, i, p) for i in range(i0, i1) for p in (1, 4)]
                + [(kp, i, p) for i in range(i0, i1) for p in SIDX])
        for c, job in enumerate(jobs[:n]):
            ujob(*job, split=c >= n - nsplit)
        return jobs[n:]

    def u_epilogue(i, m, gs, t0, dur):
        for n, g in enumerate(gs):
            t = -10 ** 6 if t0 is None else t0 + n * dur // len(gs)
            zi = [_zero(at(t - P["UG"] - (3 - n) * P["UM"])) for n in range(4)]
            zi = [None if v is None else _x2(v) for v in zi]
            bia = [b1_v[2 * i + e:2 * i + e + 1, :].astype(f32) for e in range(2)]
            top = slice(g * 16, g * 16 + 16)
            q = _combine([x[top] for x in m])
            gl = [_gelu(q[0] + bia[0], zi[3]), _gelu(q[1] + bia[1], zi[0]),
                  _gelu(q[2] + bia[0], zi[1]), _gelu(q[3] + bia[1], zi[2])]
            for p, v in enumerate(_lhs_ops(*gl)):
                lc_s[p * QD + g * 8:p * QD + g * 8 + 8, _blk(i)] = _pk(v)
            ready.add(("lc", i, g))

    def stage_u_last(i, order, edur, split_last=False):
        def lhs(p, k0, k1):
            return _up(lh_s[p * QD:(p + 1) * QD, UB0 // 2 * LB + k0:UB0 // 2 * LB + k1])

        def rhs(p, k0, k1):
            if p in SIDX:
                return stored_rhs(i % 3, p, k0, k1)
            e = 0 if p == 1 else 1
            return _cat([w1_v[_blk(UB0 + 2 * k + e), _blk(2 * i + e)] for k in range(k0 // LB, k1 // LB)], 0)
        m = strassen(lhs, rhs, NUP * LB, order, split_last, init=[um_s[p * HD:(p + 1) * HD, _blk(i)] for p in range(7)])
        for k in range(NUP):
            ready.discard(("rs", i % 3, k))
        if edur is None:
            u_epilogue(i, m, list(range(HD // 16)), None, None)
            return
        t = now() - P["UE0"]
        add_tasks([(t + (g + 1) * edur // 7, u_epilogue, (i, m, [g, g + 7], t + g * edur // 7, edur // 7))
                   for g in range(7)])

    def stage_a(b, odd=False, split_last=False):
        def lhs(p, k0, k1):
            assert ("lw", p) in ready
            return _up(lw_s[p * (HA // 2):(p + 1) * (HA // 2), :])

        def rhs(p, k0, k1):
            assert ("xn", b) in ready
            if p in SIDX:
                return _up(ra_s[(b // 2) * QD:(b // 2 + 1) * QD, _blk(SIDX[p])])
            return _up(xnT_s[0:QD, _blk(b)] if p == 1 else xnT_s[QD:HD, _blk(b + 1)])
        order = (6, 4, 2, 1, 3, 0, 5) if odd else (4, 2, 1, 3, 0, 5, 6)
        q = _combine(strassen(lhs, rhs, HD, order, split_last))
        for hh in range(2):
            for e in range(2):
                qk_s[b + e + 1, hh * D:(hh + 1) * D, :] = q[2 * hh + e][0:D]
                v_s[b + e + 1, hh * HD:(hh + 1) * HD, :] = q[2 * hh + e][D:HA]
        ready.update({("qkv", b), ("qkv", b + 1)})

    lane0 = lax.broadcasted_iota(i32, (HH, LB), 1)
    zeros8 = jnp.zeros((HH, LB), f32)

    def mk_shift(*deps):
        lane = _orz(lane0, _zero(*deps))

        def fwd(cur, prev, sh):
            if sh == 0:
                return cur
            return pltpu.roll(jnp.where(lane < LB - sh, cur, prev), sh, 1)

        def bwd(cur, nxt_):
            return pltpu.roll(jnp.where(lane >= SH, cur, nxt_), LB - SH, 1)
        return fwd, bwd

    def grp_shift(t):
        deps = [at(t)]
        if P["L"] and len(hist) >= P["L"]:
            deps += hist[-P["L"]]
        return mk_shift(*deps)

    raw, probs = {}, {}

    def attn_qk(j, hh, t, bd):
        jn = min(j + 1, NB - 1)
        assert ("qkv", jn) in ready
        acc = [None] * WH
        accp = [None] * WH
        for d in range(DH):
            if d % P["G"] == 0:
                if d > 0:
                    hist.append(acc + accp)
                fwd, bwd = grp_shift(t + d * bd // DH)
            r = hh * D + d * HH
            q = qk_s[j + 1, r:r + HH, :]
            qp = bwd(q, qk_s[jn + 1, r:r + HH, :])
            k = qk_s[j + 1, HD + r:HD + r + HH, :]
            kp = qk_s[j, HD + r:HD + r + HH, :] if j > 0 else zeros8
            for a in range(WH):
                ks = fwd(k, kp, DIL * a)
                t0, t1 = q * ks, qp * ks
                acc[a] = t0 if d == 0 else acc[a] + t0
                accp[a] = t1 if d == 0 else accp[a] + t1
        hist.append(acc + accp)
        raw[j, hh] = (acc, accp)

    def attn_sm(j, hh, t):
        fwd, _ = mk_shift(at(t))
        acc, accp = raw[j, hh]
        prev = raw.pop((j - 1, hh))[1] if j > 0 else [zeros8] * WH
        lg = acc + [fwd(accp[a], prev[a], SH) for a in range(WH)]
        lg = [a * SCALE for a in lg]
        if j == 0:
            lg = [lg[0]] + [jnp.where(lane0 >= DIL * w, lg[w], -1e9) for w in range(1, W)]
        m = lg[0]
        for w in range(1, W):
            m = jnp.maximum(m, lg[w])
        e = [jnp.exp(l - m) for l in lg]
        den = e[0]
        for w in range(1, W):
            den = den + e[w]
        inv = 1.0 / den
        p = [x * inv for x in e]
        for a in range(WH):
            pr_s[j, (hh * W + a) * HH:(hh * W + a + 1) * HH, :] = p[a]
        probs[j, hh] = p[WH:]

    def attn_pp(j, hh, t):
        _, bwd = mk_shift(at(t))
        p = probs.pop((j, hh))
        pn = probs[j + 1, hh] if j + 1 < NB else p
        for a in range(WH):
            pr_s[j, (hh * W + WH + a) * HH:(hh * W + WH + a + 1) * HH, :] = bwd(p[a], pn[a])
        ready.add(("pr", j, hh))

    def attn_pv(j, hh, dst, e, t, bd, t_dl):
        assert not isinstance(j, int) or ("pr", j, hh) in ready
        pa = [pr_s[j, (hh * W + a) * HH:(hh * W + a + 1) * HH, :] for a in range(W)]
        p, pp = pa[:WH], pa[WH:]
        outs = []
        for d2 in range(DH // 2):
            os_ = []
            for d in (2 * d2, 2 * d2 + 1):
                if d % P["G"] == 0:
                    if d > 0:
                        hist.append([])
                    fwd, _ = grp_shift(t + d * bd // DH)
                r = hh * HD + d * HH
                v = v_s[j + 1, r:r + HH, :]
                vp = v_s[j, r:r + HH, :]
                o = op = None
                for a in range(WH):
                    vs = fwd(v, vp, DIL * a)
                    o = p[a] * vs if a == 0 else o + p[a] * vs
                    op = pp[a] * vs if a == 0 else op + pp[a] * vs
                opp = zeros8 if (isinstance(j, int) and j == 0) else op_s[r:r + HH, :]
                op_s[r:r + HH, :] = op
                os_.append(o + fwd(op, opp, SH))
            ro = hh * QD + d2 * HH
            dst[ro:ro + HH, _blk(e)] = _pk(jnp.concatenate(os_, axis=0))
            outs += os_
        hist.append([])
        bits = pltpu.bitcast(outs[0], u32)
        for o in outs[1:]:
            bits = bits | pltpu.bitcast(o, u32)
        dls.append((t_dl, bits))

    mains = [("qk", j, hh) for j in range(NB) for hh in range(2)]
    mains = (mains[:P["PVPOS"]] + [("pv", j, hh) for j in range(4) for hh in range(2)]
             + mains[P["PVPOS"]:] + [None, None])
    slot_ctr = [0]

    def slot(t, bd):
        n = slot_ctr[0]
        slot_ctr[0] += 1
        it = mains[n]
        if it is None:
            pass
        elif it[0] == "qk":
            attn_qk(it[1], it[2], t, bd)
        else:
            attn_pv(it[1], it[2], ola_s, it[1], t, bd, t + bd + P["PVL"])
        if n >= 1 and mains[n - 1] is not None and mains[n - 1][0] == "qk":
            attn_sm(mains[n - 1][1], mains[n - 1][2], t + P["LS"])
        if n >= 2 and mains[n - 2] is not None and mains[n - 2][0] == "qk":
            _, j, hh = mains[n - 2]
            if j > 0:
                attn_pp(j - 1, hh, t + P["PP"])
            if j == NB - 1:
                attn_pp(j, hh, t + P["PP"])


    def out_copy(pidx, e0, e1, r0, r1):
        off = pidx * (2 * LB) + e0 * LB
        if not isinstance(pidx, int):
            off = pl.multiple_of(off, LB)
        rs = pl.ds(r0, r1 - r0)
        return pltpu.make_async_copy(out_v.at[pidx, rs, pl.ds(e0 * LB, (e1 - e0) * LB)],
                                     out_hbm.at[0, rs, pl.ds(off, (e1 - e0) * LB)], sems.at[0])

    TOP = {0: ((0, 0), 1, (1, 1)), 1: ((0, 0),), 2: ((0, 1), -1, (1, 1)), 3: ((1, 0), -1, (0, 0)),
           4: ((1, 1),), 5: ((0, 0), 1, (0, 1)), 6: ((1, 0), 1, (1, 1))}

    def top_op(p, blk):
        t = TOP[p]
        if len(t) == 1:
            return blk(*t[0])
        return blk(*t[0]) + blk(*t[2]) if t[1] > 0 else blk(*t[0]) - blk(*t[2])

    def rr_prep(ps, pa, osrc, n0, n1, t0, dur):
        for n in range(n0, n1):
            z = _zero(at(t0 + (n - n0) * dur // (n1 - n0)))
            qd, g = divmod(n, 8)
            cache = {}

            def wblk(i):
                def blk(x, y):
                    if (i, x, y) not in cache:
                        r = (2 * i + x) * LB + g * 16
                        cache[i, x, y] = w2_v[pa + y, r:r + 16, :].astype(f32)
                    return cache[i, x, y]
                return blk

            def oblk(h):
                def blk(x, y):
                    if (h, x, y) not in cache:
                        r = x * QD + h * ED + g * 8
                        cache[h, x, y] = _upf(osrc[r:r + 8, y * 2 * LB:(y + 1) * 2 * LB])
                    return cache[h, x, y]
                return blk
            for p in ps:
                raw_p = p not in SIDX
                ro = p * RRK + g * 8
                if qd == NQ:
                    if not raw_p:
                        r = top_op(p, wblk(2 * NQ))
                        for e in range(2):
                            rr_s[ro:ro + 8, _blk(7 + e)] = _pkz(r[:, _blk(e)], z)
                    continue
                if qd < NQ:
                    r1, r2 = top_op(p, wblk(2 * qd)), top_op(p, wblk(2 * qd + 1))
                    ro += qd * (LB // 2)
                else:
                    r1, r2 = top_op(p, oblk(0)), top_op(p, oblk(1))
                    ro += NQ * (LB // 2)
                z2 = None if z is None else _x2(z)
                if P["RT"]:
                    c11, c22, zo = r1[:, :LB], r2[:, LB:], z
                else:
                    c11, c22, zo = _orz(r1[:, :LB], z2), _orz(r2[:, LB:], z2), None
                sm = _rhs_sums(c11, r1[:, LB:], r2[:, :LB], c22)
                if not raw_p:
                    sm.update({1: c11, 4: c22})
                for q, v in sm.items():
                    rr_s[ro:ro + 8, _blk(q)] = _pkz(v, zo)
        if n1 == NRG:
            ready.update({("rr", p) for p in ps})

    NRG = 8 * (NQ + 1) + 7
    PD = 8 * QD
    BORD = (1, 3, 4, 2, 0, 5, 6)

    def rr_tasks(ps, pa, osrc, t0, t1):
        wgt = [8, 8, 8, 2, 7]
        cuts = list(range(0, NRG, 8)) + [NRG]
        todo, acc = [], 0
        for a, b, w in zip(cuts[:-1], cuts[1:], wgt):
            ta, tb = t0 + acc * (t1 - t0) // 33, t0 + (acc + w) * (t1 - t0) // 33
            todo.append((tb, rr_prep, (ps, pa, osrc, a, b, ta, tb - ta)))
            acc += w
        return todo

    def big_piece(pa, pan, olc_s, oln_s, last):
        order = BORD
        t0 = now()
        todo = []
        for n in range(7):
            ta, tb = t0 + n * PD + P["RR0"], t0 + n * PD + P["RR1"]
            if n < 6:
                todo += rr_tasks((order[n + 1],), pa, olc_s, ta, tb)
            else:
                todo += rr_tasks((order[0],), pan, oln_s, ta, tb - (P["RRM"] if last else 0))
        for n, (f, bd) in enumerate(P["BPV"]):
            e, hh = divmod(n, 2)
            t = t0 + int(f * PD)
            todo.append((t + bd, attn_pv, (pan * 2 + e, hh, oln_s, e, t, bd, t + bd + P["PVL"])))
        add_tasks(todo)
        m = [None] * 7
        for p in order:
            flush(now())
            assert ("rr", p) in ready
            ready.discard(("rr", p))
            x, y = TOP[p][0]

            def lhs(q, k0, k1):
                if q in (2, 3):
                    rows = slice(p * QD + (q - 2) * ED, p * QD + (q - 1) * ED)
                    return _up(jnp.concatenate([lc_s[rows, _blk(2 * qd + q - 2)] for qd in range(NQ)]
                                               + [lc_s[rows, (NFP + q - 2) * LB:(NFP + q - 2) * LB + QD]], axis=1))
                return _up(ll_s[(p * 7 + q) * ED:(p * 7 + q + 1) * ED, 0:KL])

            def rhs(q, k0, k1):
                if p in SIDX or q in SIDX:
                    return _up(rr_s[p * RRK:p * RRK + KL // 2, _blk(q)])
                h = 0 if q == 1 else 1
                return _cat([w2_v[pa + y, _blk(2 * (2 * qd + h) + x), _blk(h)] for qd in range(NQ)]
                            + [_up(olc_s[x * QD + h * ED:x * QD + (h + 1) * ED, _blk(2 * y + h)])], 0)
            rl = (_up(rr_s[p * RRK:p * RRK + LB // 2, 7 * LB:9 * LB]) if p in SIDX
                  else w2_v[pa + y, _blk(4 * NQ + x), :])
            ll = _up(lc_s[p * QD:(p + 1) * QD, _blk(2 * NQ)])
            ex = [mm1(ll[:QD], rl), mm1(ll[QD:], rl)]
            c = _combine(strassen(lhs, rhs, KL, P["LORD"]))
            m[p] = jnp.concatenate([jnp.concatenate(c[0:2], axis=1) + ex[0],
                                    jnp.concatenate(c[2:4], axis=1) + ex[1]], axis=0)
            n = {3: 2, 2: 1, 5: 3}.get(p)
            if n is not None:
                t = now() + P["EP0"]
                add_tasks([(t + P["EPD"], b_out, (pa, n, list(m), (0, HD, 0, 2), t, P["EPD"]))])
        if last:
            flush()
            for part in LAST_PARTS:
                b_out(pa, 0, m, part)
        else:
            t = now() + P["EP0"]
            add_tasks([(t + P["EPD"], b_out, (pa, 0, m, (0, HD, 0, 2), t, P["EPD"]))])

    LAST_PARTS = [(0, QD, 1, 2), (QD, HD, 0, 2), (0, QD, 0, 1)]

    def b_out(pa, n, m, part, t0=None, dur=None):
        a, y = divmod(n, 2)
        r0, r1, e0, e1 = part
        cols = slice(e0 * LB, e1 * LB)
        for r in range(r0, r1, 16):
            mm_ = [None if v is None else v[r:r + 16, cols] for v in m]
            c12, c21 = (lambda: mm_[2] + mm_[4]), (lambda: mm_[1] + mm_[3])
            xx = lambda: (mm_[2] - mm_[1]) + mm_[0]
            c = (c12() if n == 1 else c21() if n == 2 else xx() + mm_[5] if n == 3
                 else (xx() + mm_[6]) + (c21() - c12()))
            rows = slice(a * HD + r, a * HD + r + 16)
            o = c + b2f_s[pa + y, 0:1, cols] + x_v[pa + y, rows, cols].astype(f32)
            z = None if t0 is None else _zero(at(t0 + (r - r0) * dur // (r1 - r0)))
            if z is not None:
                o = jnp.concatenate([_orz(o[:, 0:LB], _x2(z)), o[:, LB:]], axis=1)
            out_v[pa + y, rows, cols] = o.astype(bf16)
        out_copy(pa + y, e0, e1, a * HD + r0, a * HD + r1).start()

    def c_body(it, carry):
        reset()
        _TRUE[:] = [one_s[...]]
        ready.add(("rr", BORD[0]))
        pa = 4 * it
        big_piece(pa, pa + 2, ola_s, olb_s, False)
        big_piece(pa + 2, lax.rem(pa + 4, NP), olb_s, ola_s, True)
        return carry

    x0 = Group(cp_x(0, 1))
    E1 = P["E1"]
    g1 = Group(cp_w1(0, 2, 0, E1))
    g2 = Group(cp_w1(0, 2, E1, NFP) + cp_x(1, 2))
    E3 = P["E3"]
    g3 = Group(cp_w1(2, UB0, 0, E3))
    g4 = Group((cp_w1(2, UB0, E3, NFP) if E3 < NFP else []) + [(wqkv_hbm, wqkv_v)])
    g5 = Group(cp_x(2, NP))
    g6 = Group(cp_w1(UB0, NB) + [(wo_hbm, wo_v), (b1_hbm, b1_v), (b2_hbm, b2_v)] + cp_w2(0, 1))
    g7 = Group(cp_w2(1, NP))
    for c in (x0, g1, g2, g3, g4, g5, g6, g7):
        c.start()

    v_s[0] = jnp.zeros((D, LB), f32)
    for buf in (xnT_s, ra_s, lh_s, rs_s, rr_s, ola_s, olb_s, ll_s, lc_s):
        buf[0:8, 0:64] = jnp.zeros((8, 64), u32)

    LND, BD, MARG = P["LND"], P["BD"], P["MARG"]

    def ln_tasks(b, t, lnd=LND, hsd=P["HSD"]):
        todo = []
        for fn, bb, dur, adv in ((ln, b, lnd, 0.8), (ln, b + 1, lnd, 0.86), (hpair, b, hsd, 1.0)):
            todo.append((t + int(dur * adv), fn, (bb, t, dur)))
            t += int(dur * adv)
        return todo, t

    wait("x0", x0)
    one_s[...] = lax.shift_right_logical(pltpu.bitcast(x_v[0, 0:16, 0:LB], i32), 1) | 1
    _TRUE[:] = [one_s[...]]
    ln(0); ln(1); hpair(0)
    wait("r1", g1)
    left_ = u_early(0, 0, E1, [], 7 * E1 // 4 * 4, -200, 100)
    wait("r2", g2)
    add_tasks(ln_tasks(2, P["L2T"], P["L2D"], P["H2D"])[0])
    n2 = (len(left_) + 7 * (NFP - E1)) // 4 * 4
    left_ = u_early(0, E1, NFP, left_, n2, -200, 120)
    wait("r3", g3)
    left_ = u_early(1, 0, E3, left_, P["N3"], -200, 140)
    wait("wqkv", g4)
    n4 = len(left_) + 7 * (NFP - E3)
    u_early(1, E3, NFP, left_, n4, -200, 100, nsplit=n4 % 4)
    prep_wqkv()
    stage_a(0, split_last=True)
    wait("mid", g5)
    AD = 7 * HA // 2
    UD = 7 * NUP * HD // 4
    r5 = (NP - 1) * AD
    t = 0
    for b in range(UB0, NB, 2):
        todo, t = ln_tasks(b, t)
        add_tasks(todo)
    n5 = 0
    while t + BD + MARG <= r5:
        add_tasks([(t + BD, slot, (t, BD))])
        t += BD
        n5 += 1
    for n, b in enumerate(range(2, NB, 2)):
        stage_a(b, odd=n % 2 == 1, split_last=b == NB - 2)
    wait("fin", g6)
    r6 = NFP * UD
    todo = []
    for i in range(NFP):
        if i == 0:
            t0, dt = -200, 130
        elif i == 1:
            t0, dt = 700, 260
        else:
            t0, dt = (i - 1) * UD + P["US0"], P["USD"]
        for k in range(NUP):
            tt = t0 + k * dt
            todo.append((tt + dt, tsum, (w1_ld(i), (UB0 + 2 * k) * LB, i % 3, k, tt, dt)))
    left = len(mains) - n5 - 2
    t = P["R6S"]
    bd2 = (r6 - P["R6E"] - t) // left
    for _ in range(left):
        todo.append((t + min(bd2, 600), slot, (t, min(bd2, 600))))
        t += bd2
    for i in range(2):
        todo.append((t + (i + 1) * 300, slot, (t + i * 300, 300)))
    for qd, t0, dur in ((NQ, UD + 300, 2 * UD - 300), (0, 3 * UD + 300, 2 * UD - 300), (1, 5 * UD + 300, UD - 100),
                        (2, 6 * UD + P["LL2"], P["UEL"])):
        for g in range(7):
            todo.append((t0 + (g + 1) * dur // 7, llsum, (qd, g, t0 + g * dur // 7, dur // 7)))
    todo += rr_tasks((BORD[0],), 0, ola_s, P["RP0"], P["RP1"])
    todo.append((P["PW0"] + P["PWD"], prep_wo_a, (P["PW0"], P["PWD"])))
    for h in range(2):
        t = P["PW1"] + h * P["PWE"]
        todo.append((t + P["PWE"], prep_wo_b, (h, t, P["PWE"])))
    add_tasks(todo)
    for b in range(NB):
        b2f_s[b // 2, 0:1, _blk(b % 2)] = b2_v[b:b + 1, :].astype(f32)
    for i in range(NFP):
        stage_u_last(i, (1, 4, 2, 3, 0, 5, 6) if i == 0 else P["UORD"],
                     None if i == NFP - 1 else P["UEL"] if i == NFP - 2 else P["UED"], split_last=i == NFP - 1)
    flush()
    assert slot_ctr[0] == len(mains) and all(("ll", qd, g) in ready for qd in range(NQ + 1) for g in range(7))
    wait("w2", g7)

    lax.fori_loop(0, NP // 4, c_body, 0)
    outs = []
    for pa in range(0, NP, 2):
        outs += [out_copy(pa + n % 2, 0, 2, n // 2 * HD, (n // 2 + 1) * HD) for n in (1, 2, 3)]
        outs += [out_copy(pa, e0, e1, r0, r1) for (r0, r1, e0, e1) in (LAST_PARTS if pa % 4 else [(0, HD, 0, 2)])]
    wait("out", *outs)


@jax.jit
def pallas_parallel_sum__sliding_local_dilated__mixer_token_mlp__prompt_kernel(A_x, A_wqkv, A_wo, B_x, B_w1, B_b1, B_w2, B_b2):
    del B_x
    hbm = pl.BlockSpec(memory_space=pltpu.HBM)
    outT = pl.pallas_call(
        _kernel,
        out_shape=jax.ShapeDtypeStruct((1, D, S), bf16),
        in_specs=[hbm] * 7,
        out_specs=hbm,
        scratch_shapes=[
            pltpu.VMEM((NP, D, 2 * LB), bf16),
            pltpu.VMEM((D, 3 * D), bf16),
            pltpu.VMEM((D, D), bf16),
            pltpu.VMEM((S, F), bf16),
            pltpu.VMEM((NP, F, 2 * LB), bf16),
            pltpu.VMEM((NFB, LB), bf16),
            pltpu.VMEM((NB, LB), bf16),
            pltpu.VMEM((NP, D, 2 * LB), bf16),
            pltpu.VMEM((2, 3 * D, LB), i32),
            pltpu.VMEM((7 * HA // 2, HD), u32),
            pltpu.VMEM((4, HD, LB), i32),
            pltpu.VMEM((D, 2 * LB), i32),
            pltpu.VMEM((HD, S), u32),
            pltpu.VMEM((NP * QD, 5 * LB), u32),
            pltpu.VMEM((7 * QD, NP * LB), u32),
            pltpu.VMEM((7 * HD, NFP * LB), f32),
            pltpu.VMEM((7 * QD, KC), u32),
            pltpu.VMEM((NB + 1, 2 * D, LB), f32),
            pltpu.VMEM((NB + 1, D, LB), f32),
            pltpu.VMEM((NB, 2 * W * HH, LB), f32),
            pltpu.VMEM((D, LB), f32),
            pltpu.VMEM((NP, 32, 2 * LB), f32),
            pltpu.VMEM((5 * RSK, 5 * LB), u32),
            pltpu.VMEM((49 * ED, 4 * LB), u32),
            pltpu.VMEM((7 * RRK, 9 * LB), u32),
            pltpu.VMEM((HD, 4 * LB), u32),
            pltpu.VMEM((HD, 4 * LB), u32),
            pltpu.VMEM((8, LB), i32),
            pltpu.SemaphoreType.DMA((9,)),
        ],
        compiler_params=pltpu.CompilerParams(vmem_limit_bytes=100 * 1024 * 1024,
                                             disable_bounds_checks=True,
                                             disable_semaphore_checks=True),
    )(jnp.swapaxes(A_x, 1, 2), A_wqkv, A_wo, B_w1, B_b1.reshape(NFB, LB), B_w2, B_b2.reshape(NB, LB))
    return jnp.swapaxes(outT, 1, 2)
```

```python
import jax
import jax.numpy as jnp
from jax import lax
import jax.experimental.pallas as pl
import jax.experimental.pallas.tpu as pltpu

S, D, F = 2048, 448, 1792
H, DH, W, DIL = 16, 28, 8, 2
LB = 128
NB = S // LB
NP = NB // 2
NFB = F // LB
NFP = NFB // 2
HH = H // 2
WH = W // 2
SH = DIL * WH
HD = D // 2
QD = D // 4
HA = 3 * HD
UB0 = 4
NUP = (NB - UB0) // 2
KC = F // 2 + 2 * LB
RSK = NFP * LB // 2
NQ = NFP // 2
KL = NQ * LB + QD
ED = D // 8
RRK = 2 * LB
EPS = 1e-5
SCALE = DH ** -0.5
f32 = jnp.float32
bf16 = jnp.bfloat16
u32 = jnp.uint32
i32 = jnp.int32

SCOPES = False
P = dict(LORD=(2, 4, 1, 3, 0, 5, 6), BORD=(1, 3, 2, 4, 0, 5, 6), DEF=True, OT=False, EP0=0, EPL=250, EPD=840, RR0=0, RR1=800, RRM=100, OC1=60,
         BPV=tuple((0.05 + 0.8 * i, 620) for i in range(8)),
         BVB=560, BVD=700, RT=1, STG=(),
         LND=400, BD=370, G=4, LAG=200, CAP=2000, LS=170, PP=150, MARG=300, N3=40, E3=6, W3T=700, W3D=600, W2T=200, W2D=450, W2X=300, E1=3, L2T=250, L2D=480, H2D=420, PVD=680, PV0=50, HSD=360, HG=0,
         CORD=(4, 2, 1, 3, 0, 5, 6), TS0=100, TSD=420, PVB=520, PVL=500, OS0=3050, OSD=300,
         UORD=(4, 2, 1, 3, 0, 5, 6), US0=100, USD=350, R6S=1900, PVPOS=12, R6E=2400, LL2=500, RP0=14200, RP1=16000, PVD2=400, NQ0=3, NQ1=7, QM1=750, LL0=1200, UR=False, HR=False, LNI=True, TI=False, HL=300,
         UE0=-200, UED=2100, UEL=1400, PW0=500, PWD=300, PW1=1300, PWE=400, UG=50, UM=24, PWL=2100, SK0=1500, LNQ1=4, LNQ3=4, LNA=0.3, LNB=0.42, LNBD=0.33)


def _gelu(x, z=None):
    c = 0.7978845608028654
    hx = 0.5 * x
    return hx + hx * jnp.tanh(_orz(x * (c + (c * 0.044715) * (x * x)), z))


def _pk(x):
    return pltpu.bitcast(x.astype(bf16), u32)


def _up(x):
    return pltpu.bitcast(x, bf16)


def _upf(x):
    return pltpu.bitcast(x, bf16).astype(f32)


def _cat(xs, axis):
    return xs[0] if len(xs) == 1 else jnp.concatenate(xs, axis=axis)


def _x2(v):
    return jnp.concatenate([v, v], axis=0)


def _blk(b):
    return slice(b * LB, (b + 1) * LB)


def _rowsum8(a):
    return jnp.broadcast_to(jnp.sum(a, axis=0, keepdims=True), (8, a.shape[1]))


_TRUE = []


def _zero(*deps):
    deps = [d for d in deps if d is not None]
    if not deps:
        return None
    bits = pltpu.bitcast(deps[0], u32)
    for d in deps[1:]:
        bits = bits | pltpu.bitcast(d, u32)
    return bits


def _orz(v, z):
    if z is None:
        return v
    m = _TRUE[0] if v.shape[0] == 8 else _x2(_TRUE[0])
    return jnp.where(m[:, 0:v.shape[1]] > 0, v, pltpu.bitcast(z, v.dtype))


def _pkz(v, z):
    return _pk(v if z is None else jnp.concatenate([_orz(v[0:8], z), v[8:16]], axis=0))


def _lhs_ops(a11, a12, a21, a22):
    return [a11 + a22, a21 + a22, a11, a22, a11 + a12, a21 - a11, a12 - a22]


SIDX = {0: 0, 2: 1, 3: 2, 5: 3, 6: 4}


def _rhs_sums(b11, b12, b21, b22):
    return {0: b11 + b22, 2: b12 - b22, 3: b21 - b11, 5: b11 + b12, 6: b21 + b22}


def _combine(m):
    c12 = m[2] + m[4]
    c21 = m[1] + m[3]
    x = (m[2] - m[1]) + m[0]
    return ((x + m[6]) + (c21 - c12), c12, c21, x + m[5])


def _kernel(x_hbm, wqkv_hbm, wo_hbm, w1_hbm, b1_hbm, w2_hbm, b2_hbm, out_hbm,
            x_v, wqkv_v, wo_v, w1_v, w2_v, b1_v, b2_v, out_v,
            wt_s, lw_s, wo_s, wq_s, xnT_s, ra_s, lh_s, um_s, lc_s, qk_s, v_s, pr_s, op_s,
            b2f_s, rs_s, ll_s, rr_s, ola_s, olb_s, wf_s, one_s, sems):
    sem_ctr = [1]

    class Group:
        def __init__(self, pairs):
            self.cps = [pltpu.make_async_copy(a, b, sems.at[sem_ctr[0]]) for (a, b) in pairs]
            sem_ctr[0] += 1

        def start(self):
            for c in self.cps:
                c.start()

        def wait(self):
            for c in self.cps:
                c.wait()

    def cp_x(p0, p1):
        return [(x_hbm.at[0, :, pl.ds(p * 2 * LB, 2 * LB)], x_v.at[p]) for p in range(p0, p1)]

    def cp_w2(p0, p1):
        return [(w2_hbm.at[:, pl.ds(p * 2 * LB, 2 * LB)], w2_v.at[p]) for p in range(p0, p1)]

    def cp_w1(b0, b1, i0=0, i1=NFP):
        sl = pl.ds(b0 * LB, (b1 - b0) * LB)
        cl = pl.ds(i0 * 2 * LB, (i1 - i0) * 2 * LB)
        return [(w1_hbm.at[sl, cl], w1_v.at[sl, cl])]

    tl = []
    mxu = [0, 0, 0, 0]
    nxt = [0]
    hist = []
    tasks = []
    dls = []
    ready = set()

    def add_tasks(todo):
        tasks.extend(todo)
        tasks.sort(key=lambda x: x[0])

    def flush(t=None):
        while tasks and (t is None or tasks[0][0] < t):
            _, fn, args = tasks.pop(0)
            fn(*args)

    def reset():
        assert not tasks
        dls.clear()
        tl.clear()
        hist.clear()
        mxu[:] = [0, 0, 0, 0]
        nxt[0] = 0

    def now():
        return sum(mxu) // 4

    def wait(name, *cps):
        flush()
        if SCOPES:
            with jax.named_scope("wait_" + name):
                for c in cps:
                    c.wait()
        else:
            for c in cps:
                c.wait()
        reset()

    def mm1(lhs, rhs, pace=True):
        flush(now())
        start = mxu[nxt[0]]
        due = [v for (t, v) in dls if t <= start] if pace else []
        if due:
            dls[:] = [(t, v) for (t, v) in dls if t > start]
            tile = _up(_orz(pltpu.bitcast(lhs[0:16, 0:LB], u32), _zero(*due)))
            row = tile if lhs.shape[1] == LB else jnp.concatenate([tile, lhs[0:16, LB:]], axis=1)
            lhs = jnp.concatenate([row, lhs[16:]], axis=0)
        r = jnp.dot(lhs, rhs, preferred_element_type=f32)
        m, k = lhs.shape
        first_done = None
        for _ in range(-(-rhs.shape[1] // LB)):
            end = 0
            for _ in range(-(-k // LB)):
                mxu[nxt[0]] += m
                end = max(end, mxu[nxt[0]])
                nxt[0] = (nxt[0] + 1) % 4
            if first_done is None:
                first_done = end
        if pace:
            tl.append((first_done - m, first_done, r))
        return r

    def mm(lhs, rhs, init=None):
        k = lhs.shape[1]
        r, k0 = init, 0
        while k0 < k:
            k1 = min(k, k0 + (4 - nxt[0]) * LB)
            part = mm1(lhs[:, k0:k1], rhs[k0:k1], pace=k1 - k0 > LB)
            r = part if r is None else r + part
            k0 = k1
        return r

    def at(t):
        if t is None or t < 0:
            return None
        t = min(t, now() - 1)
        best = None
        for (a, b, r) in tl:
            if a <= t and (best is None or min(b, t) > best[0]):
                row = int(min((t - a) / (b - a), 0.999) * (r.shape[0] // 8)) * 8
                best = (min(b, t), r, row)
        return None if best is None else best[1][best[2]:best[2] + 8, 0:LB]

    def strassen(lhs, rhs, k, order, split_last=False, head=0, init=None):
        m = [None] * 7

        def ops(p, k0, k1):
            flush(now())
            return lhs(p, k0, k1), rhs(p, k0, k1)

        if head:
            for p in order:
                m[p] = mm(*ops(p, 0, head * LB))
        for p in order:
            l, r = ops(p, head * LB, k)
            if split_last and p == order[-1]:
                kk = (-(-r.shape[0] // LB) - 2) * LB
                hm = l.shape[0] // 2
                hd = mm(l[:, :kk], r[:kk], None if init is None else init[p]) if kk else None
                tail = jnp.concatenate([mm(l[:hm, kk:], r[kk:]), mm(l[hm:, kk:], r[kk:])], axis=0)
                v = tail if hd is None else hd + tail
            else:
                v = mm(l, r, None if init is None else init[p])
            m[p] = v if m[p] is None else m[p] + v
        return m

    def put_sums(dst, sm, ro, z):
        for p, v in sm.items():
            dst[ro:ro + 8, _blk(SIDX[p])] = _pkz(v, z)

    def tsum(ld, r0, slot_, i, t0, dur):
        for g in range(LB // 16):
            z = _zero(at(t0 + g * dur // 8))
            t1 = ld(slice(r0 + g * 16, r0 + g * 16 + 16)).astype(f32)
            t2 = ld(slice(r0 + LB + g * 16, r0 + LB + g * 16 + 16)).astype(f32)
            if P["TI"] and z is not None:
                sm = _rhs_sums(_orz(t1[:, :LB], _x2(z)), t1[:, LB:], t2[:, :LB], _orz(t2[:, LB:], _x2(z)))
                z = None
            else:
                sm = _rhs_sums(t1[:, :LB], t1[:, LB:], t2[:, :LB], t2[:, LB:])
            put_sums(rs_s, sm, slot_ * RSK + i * (LB // 2) + g * 8, z)
        ready.add(("rs", slot_, i))

    def stored_rhs(slot_, p, k0, k1):
        assert all(("rs", slot_, i) in ready for i in range(k0 // LB, -(-k1 // LB))), (slot_, k0, k1)
        return _up(rs_s[slot_ * RSK + k0 // 2:slot_ * RSK + k1 // 2, _blk(SIDX[p])])

    def wrows(hh, g, z=None):
        p, d = divmod(2 * g, DH)
        t = [jnp.concatenate([wt_s[c, pl.ds(p * D + hh * HD + d + e, HH, stride=DH), :]
                              for e in range(2)], axis=0) for c in range(2)]
        if z is not None:
            t = [_orz(v, _x2(z)) for v in t]
        w = jnp.concatenate([t[0], t[1][:, 0:HD - LB]], axis=1)
        return [pltpu.bitcast(w << 16, f32), pltpu.bitcast(w & -65536, f32)]

    def prep_wqkv():
        done = set()
        ng = HA // 16

        def need(hh, p, z=None):
            lo = p * D + hh * HD
            for ct in range(lo // LB, -(-(lo + HD) // LB)):
                if ct in done:
                    continue
                done.add(ct)
                w = min(LB, 3 * D - ct * LB)
                k1, k2 = [pltpu.bitcast(wqkv_v[kh * HD:(kh + 1) * HD, ct * LB:ct * LB + w].astype(f32), i32)
                          for kh in range(2)]
                wd = lax.shift_right_logical(k1, 16) | k2
                if z is not None:
                    wd = jnp.concatenate([_orz(wd[r:r + 8], z[:, 0:w]) if r % LB == 0 else wd[r:r + 8]
                                          for r in range(0, HD, 8)], axis=0)
                wT = wd.T
                wt_s[0, ct * LB:ct * LB + w, :] = wT[:, 0:LB]
                wt_s[1, ct * LB:ct * LB + w, 0:HD - LB] = wT[:, LB:HD]

        def put(p, g, v):
            lw_s[p * (HA // 2) + g * 8:p * (HA // 2) + g * 8 + 8, :] = _pk(v)

        def half(hh, g0, g1, t0=None, dur=None):
            pr, ps = ((2, 4), (3, 1))[hh]
            for g in range(g0, g1):
                t = None if t0 is None else t0 + (g - g0) * dur // (g1 - g0)
                need(hh, 2 * g // DH, _zero(at(None if t is None else t - P["W2X"])))
                a1, a2 = wrows(hh, g, _zero(at(t)))
                put(pr, g, a2 if hh else a1)
                put(ps, g, a1 + a2)
            if g1 == ng:
                ready.update({("lw", pr), ("lw", ps)})
        half(0, 0, ng)
        t, dt = now() + P["W2T"], P["W2D"] // 3
        add_tasks([(t + (n + 1) * dt, half, (1, 14 * n, 14 * n + 14, t + n * dt, dt)) for n in range(3)])

        def rest(g0, g1, t0, dur):
            for g in range(g0, g1):
                z = _zero(at(t0 + (g - g0) * dur // (g1 - g0)))
                ops = _lhs_ops(*wrows(0, g, z), *wrows(1, g, z))
                for p in (0, 5, 6):
                    put(p, g, ops[p])
            if g1 == ng:
                ready.update({("lw", 0), ("lw", 5), ("lw", 6)})
        t, dt = now() + P["W3T"], P["W3D"] // 7
        add_tasks([(t + (n + 1) * dt, rest, (6 * n, 6 * n + 6, t + n * dt, dt)) for n in range(7)])

    def prep_wo_a(t0, dur):
        for g in range(HD // 16):
            k1, k2 = [pltpu.bitcast(wo_v[hh * HD + g * 16:hh * HD + g * 16 + 16, :].astype(f32), i32)
                      for hh in range(2)]
            w = lax.shift_right_logical(k1, 16) | k2
            z = _zero(at(t0 + g * dur // (HD // 16)))
            for c in range(4):
                cw = min(LB, D - c * LB)
                wo_s[c, g * 16:g * 16 + 16, 0:cw] = _orz(w[:, c * LB:c * LB + cw], None if z is None else _x2(z)[:, 0:cw])

    def prep_wo_b(h, t0, dur):
        for c in range(4):
            cw = min(LB, D - c * LB)
            rows = [wo_s[c, pl.ds(d, HH, stride=DH), :][:, 0:cw] for d in range(h * DH // 2, (h + 1) * DH // 2)]
            rows.append(jnp.zeros((LB - QD, cw), i32))
            wq_s[c * LB:c * LB + cw, _blk(h)] = jnp.concatenate(rows, axis=0).T
        bits = None
        for g in range(HD // 16):
            z = _zero(at(t0 + g * dur // (HD // 16)))
            a = []
            for r in (g * 16, HD + g * 16):
                w = _orz(wq_s[r:r + 16, _blk(h)], None if z is None else _x2(z))
                a += [pltpu.bitcast(w << 16, f32), pltpu.bitcast(w & -65536, f32)]
            for p, v in enumerate(_lhs_ops(*a)):
                lc_s[p * QD + g * 8:p * QD + g * 8 + 8, _blk(NFP + h)] = _pk(v)
                bits = pltpu.bitcast(v[0:8], u32) if bits is None else bits | pltpu.bitcast(v[0:8], u32)
        ready.update({("lc", NFP + h, g) for g in range(HD // 16)})
        dls.append((t0 + dur + 250, bits))

    def llsum(qd, g, t0, dur):
        i0 = 2 * qd if qd < NQ else NFP
        assert all(("lc", i0 + e, g + 7 * h) in ready for e in range(2) for h in range(2))
        for p in range(7):
            z = _zero(at(t0 + p * dur // 7))
            a = [_orz(lc_s[p * QD + h * ED + g * 8:p * QD + h * ED + g * 8 + 8, _blk(i0 + e)],
                      z if h == e else None) for h in range(2) for e in range(2)]
            ops = _lhs_ops(*[_upf(v) for v in a])
            for q in (0, 1, 4, 5, 6):
                r = (p * 7 + q) * ED + g * 8
                ll_s[r:r + 8, _blk(qd)] = _pk(ops[q])
        ready.add(("ll", qd, g))

    RG = 16
    NG = D // RG
    stat2 = {}

    def ln(b, t0=None, dur=None):
        def dep(fr):
            return None if t0 is None else at(t0 + fr * dur)

        def xg(g):
            return x_v[b // 2, g * RG:(g + 1) * RG, _blk(b % 2)].astype(f32)

        def halves(*vs):
            return [] if vs[0] is None else [v[i * 8:i * 8 + 8] for v in vs for i in range(2)]

        x0 = jnp.broadcast_to(xg(0)[0:1], (8, LB))
        s = q = None
        for g in range(NG):
            if g % P["LNQ1"] == 0 and t0 is not None:
                x0 = _orz(x0, _zero(dep(P["LNA"] * g / NG), *halves(s, q)))
            c = xg(g) - _x2(x0)
            s = c if s is None else s + c
            q = c * c if q is None else q + c * c
        dm = _rowsum8(s) * (1.0 / D)
        mu = x0 + dm
        r1 = lax.rsqrt(jnp.maximum(_rowsum8(q) * (1.0 / D) - dm * dm, 0.0) + EPS)
        s1 = s2 = z = None
        for g in range(NG):
            if g % P["LNQ3"] == 0 and t0 is not None:
                z = _zero(dep(P["LNB"] + P["LNBD"] * g / NG), *halves(s1, s2))
                if P["LNI"]:
                    mu, z = _orz(mu, z), None
            xn = (xg(g) - _x2(mu)) * _x2(r1)
            xnT_s[g * 8:g * 8 + 8, _blk(b)] = _pkz(xn, z)
            s1 = xn if s1 is None else s1 + xn
            s2 = xn * xn if s2 is None else s2 + xn * xn
        mu2 = _rowsum8(s1) * (1.0 / D)
        var2 = jnp.maximum(_rowsum8(s2) * (1.0 / D) - mu2 * mu2, 0.0)
        stat2[b] = (mu2, lax.rsqrt(var2 + EPS))

    def hpair(b, t0=None, dur=None):
        ng = HD // RG
        st = [stat2.pop(b), stat2.pop(b + 1)]
        for g in range(ng):
            t = None if t0 is None else t0 + g * dur // ng
            zi = _zero(at(None if t is None else t - P["HG"]))
            z = _zero(at(t)) if P["HR"] else None
            xq, hq = [], []
            for r in (g * 8, QD + g * 8):
                for e in range(2):
                    xn = _upf(_orz(xnT_s[r:r + 8, _blk(b + e)], zi))
                    xq.append(xn)
                    hq.append((xn - _x2(st[e][0])) * _x2(st[e][1]))
            put_sums(ra_s, _rhs_sums(*xq), (b // 2) * QD + g * 8, z)
            for p, v in enumerate(_lhs_ops(*hq)):
                lh_s[p * QD + g * 8:p * QD + g * 8 + 8, _blk(b // 2)] = _pkz(v, z)
        ready.add(("xn", b))
        if t0 is not None and b >= UB0 and P["HL"]:
            got = ra_s[(b // 2) * QD:(b // 2 + 1) * QD, :]
            tiles_ = [got[r:r + 8, _blk(c)] for r in range(0, QD, 8) for c in range(5)]
            bits = tiles_[0]
            for v in tiles_[1:]:
                bits = bits | v
            dls.append((t0 + dur + P["HL"], bits))

    def w1_ld(i):
        return lambda rs: w1_v[rs, 2 * i * LB:(2 * i + 2) * LB]

    def ujob(kp, i, p, split=False):
        flush(now())
        assert ("xn", 2 * kp) in ready
        l = _up(lh_s[p * QD:(p + 1) * QD, _blk(kp)])
        if p in SIDX:
            r = stored_rhs(3 + kp, p, i * LB, (i + 1) * LB)
        else:
            e = 0 if p == 1 else 1
            r = w1_v[_blk(2 * kp + e), _blk(2 * i + e)]
        v = jnp.concatenate([mm1(l[:QD], r), mm1(l[QD:], r)], axis=0) if split else mm1(l, r)
        rows = slice(p * HD, (p + 1) * HD)
        um_s[rows, _blk(i)] = v if kp == 0 else um_s[rows, _blk(i)] + v

    def u_early(kp, i0, i1, carry, n, t0, dt, nsplit=0):
        for k, i in enumerate(range(i0, i1)):
            add_tasks([(t0 + (k + 1) * dt, tsum, (w1_ld(i), 2 * kp * LB, 3 + kp, i, t0 + k * dt, dt))])
        jobs = (carry + [(kp, i, p) for i in range(i0, i1) for p in (1, 4)]
                + [(kp, i, p) for i in range(i0, i1) for p in SIDX])
        for c, job in enumerate(jobs[:n]):
            ujob(*job, split=c >= n - nsplit)
        return jobs[n:]

    def u_epilogue(i, m, gs, t0, dur):
        for n, g in enumerate(gs):
            t = -10 ** 6 if t0 is None else t0 + n * dur // len(gs)
            zi = [_zero(at(t - P["UG"] - (3 - n) * P["UM"])) for n in range(4)]
            zi = [None if v is None else _x2(v) for v in zi]
            bia = [b1_v[2 * i + e:2 * i + e + 1, :].astype(f32) for e in range(2)]
            top = slice(g * 16, g * 16 + 16)
            q = _combine([x[top] for x in m])
            gl = [_gelu(q[0] + bia[0], zi[3]), _gelu(q[1] + bia[1], zi[0]),
                  _gelu(q[2] + bia[0], zi[1]), _gelu(q[3] + bia[1], zi[2])]
            for p, v in enumerate(_lhs_ops(*gl)):
                lc_s[p * QD + g * 8:p * QD + g * 8 + 8, _blk(i)] = _pk(v)
            ready.add(("lc", i, g))

    def stage_u_last(i, order, edur, split_last=False):
        def lhs(p, k0, k1):
            return _up(lh_s[p * QD:(p + 1) * QD, UB0 // 2 * LB + k0:UB0 // 2 * LB + k1])

        def rhs(p, k0, k1):
            if p in SIDX:
                return stored_rhs(i % 3, p, k0, k1)
            e = 0 if p == 1 else 1
            return _cat([w1_v[_blk(UB0 + 2 * k + e), _blk(2 * i + e)] for k in range(k0 // LB, k1 // LB)], 0)
        m = strassen(lhs, rhs, NUP * LB, order, split_last, init=[um_s[p * HD:(p + 1) * HD, _blk(i)] for p in range(7)])
        for k in range(NUP):
            ready.discard(("rs", i % 3, k))
        if edur is None:
            u_epilogue(i, m, list(range(HD // 16)), None, None)
            return
        t = now() - P["UE0"]
        add_tasks([(t + (g + 1) * edur // 7, u_epilogue, (i, m, [g, g + 7], t + g * edur // 7, edur // 7))
                   for g in range(7)])

    def stage_a(b, odd=False, split_last=False):
        def lhs(p, k0, k1):
            assert ("lw", p) in ready
            return _up(lw_s[p * (HA // 2):(p + 1) * (HA // 2), :])

        def rhs(p, k0, k1):
            assert ("xn", b) in ready
            if p in SIDX:
                return _up(ra_s[(b // 2) * QD:(b // 2 + 1) * QD, _blk(SIDX[p])])
            return _up(xnT_s[0:QD, _blk(b)] if p == 1 else xnT_s[QD:HD, _blk(b + 1)])
        order = (6, 4, 2, 1, 3, 0, 5) if odd else (4, 2, 1, 3, 0, 5, 6)
        q = _combine(strassen(lhs, rhs, HD, order, split_last))
        for hh in range(2):
            for e in range(2):
                qk_s[b + e + 1, hh * D:(hh + 1) * D, :] = q[2 * hh + e][0:D]
                v_s[b + e + 1, hh * HD:(hh + 1) * HD, :] = q[2 * hh + e][D:HA]
        ready.update({("qkv", b), ("qkv", b + 1)})

    lane0 = lax.broadcasted_iota(i32, (HH, LB), 1)
    zeros8 = jnp.zeros((HH, LB), f32)

    def mk_shift(*deps):
        lane = _orz(lane0, _zero(*deps))

        def fwd(cur, prev, sh):
            if sh == 0:
                return cur
            return pltpu.roll(jnp.where(lane < LB - sh, cur, prev), sh, 1)

        def bwd(cur, nxt_):
            return pltpu.roll(jnp.where(lane >= SH, cur, nxt_), LB - SH, 1)
        return fwd, bwd

    def grp_shift(t, bd):
        lag = max(2, -(-P["LAG"] * DH // (P["G"] * bd)))
        deps = [at(t)]
        if len(hist) >= lag:
            deps += hist[-lag]
        return mk_shift(*deps)

    raw, probs = {}, {}

    def attn_qk(j, hh, t, bd):
        jn = min(j + 1, NB - 1)
        assert ("qkv", jn) in ready
        acc = [None] * WH
        accp = [None] * WH
        for d in range(DH):
            if d % P["G"] == 0:
                if d > 0:
                    hist.append(acc + accp)
                fwd, bwd = grp_shift(t + d * bd // DH, bd)
            r = hh * D + d * HH
            q = qk_s[j + 1, r:r + HH, :]
            qp = bwd(q, qk_s[jn + 1, r:r + HH, :])
            k = qk_s[j + 1, HD + r:HD + r + HH, :]
            kp = qk_s[j, HD + r:HD + r + HH, :] if j > 0 else zeros8
            for a in range(WH):
                ks = fwd(k, kp, DIL * a)
                t0, t1 = q * ks, qp * ks
                acc[a] = t0 if d == 0 else acc[a] + t0
                accp[a] = t1 if d == 0 else accp[a] + t1
        hist.append(acc + accp)
        raw[j, hh] = (acc, accp)

    def attn_sm(j, hh, t):
        fwd, _ = mk_shift(at(t))
        acc, accp = raw[j, hh]
        prev = raw.pop((j - 1, hh))[1] if j > 0 else [zeros8] * WH
        lg = acc + [fwd(accp[a], prev[a], SH) for a in range(WH)]
        lg = [a * SCALE for a in lg]
        if j == 0:
            lg = [lg[0]] + [jnp.where(lane0 >= DIL * w, lg[w], -1e9) for w in range(1, W)]
        m = lg[0]
        for w in range(1, W):
            m = jnp.maximum(m, lg[w])
        e = [jnp.exp(l - m) for l in lg]
        den = e[0]
        for w in range(1, W):
            den = den + e[w]
        inv = 1.0 / den
        p = [x * inv for x in e]
        for a in range(WH):
            pr_s[j, (hh * W + a) * HH:(hh * W + a + 1) * HH, :] = p[a]
        probs[j, hh] = p[WH:]

    def attn_pp(j, hh, t):
        _, bwd = mk_shift(at(t))
        p = probs.pop((j, hh))
        pn = probs[j + 1, hh] if j + 1 < NB else p
        for a in range(WH):
            pr_s[j, (hh * W + WH + a) * HH:(hh * W + WH + a + 1) * HH, :] = bwd(p[a], pn[a])
        ready.add(("pr", j, hh))

    def attn_pv(j, hh, dst, e, t, bd, t_dl):
        assert not isinstance(j, int) or ("pr", j, hh) in ready
        pa = [pr_s[j, (hh * W + a) * HH:(hh * W + a + 1) * HH, :] for a in range(W)]
        p, pp = pa[:WH], pa[WH:]
        outs = []
        for d in range(DH):
            if d % P["G"] == 0:
                if d > 0:
                    hist.append([])
                fwd, _ = grp_shift(t + d * bd // DH, bd)
            r = hh * HD + d * HH
            v = v_s[j + 1, r:r + HH, :]
            vp = v_s[j, r:r + HH, :]
            o = op = None
            for a in range(WH):
                vs = fwd(v, vp, DIL * a)
                o = p[a] * vs if a == 0 else o + p[a] * vs
                op = pp[a] * vs if a == 0 else op + pp[a] * vs
            opp = zeros8 if (isinstance(j, int) and j == 0) else op_s[r:r + HH, :]
            op_s[r:r + HH, :] = op
            outs.append(o + fwd(op, _orz(opp, _zero(o)) if P["OT"] else opp, SH))
            dst[r:r + HH, _blk(e)] = outs[-1]
        hist.append([])
        bits = pltpu.bitcast(outs[0], u32)
        for o in outs[1:]:
            bits = bits | pltpu.bitcast(o, u32)
        dls.append((t_dl, bits))

    mains = [("qk", j, hh) for j in range(NB) for hh in range(2)]
    mains = (mains[:P["PVPOS"]] + [("pv", j, hh) for j in range(4) for hh in range(2)]
             + mains[P["PVPOS"]:] + [None, None])
    slot_ctr = [0]

    def slot(t, bd):
        n = slot_ctr[0]
        slot_ctr[0] += 1
        it = mains[n]
        if it is None:
            pass
        elif it[0] == "qk":
            attn_qk(it[1], it[2], t, bd)
        else:
            attn_pv(it[1], it[2], ola_s, it[1], t, bd, t + bd + P["PVL"])
        if n >= 1 and mains[n - 1] is not None and mains[n - 1][0] == "qk":
            attn_sm(mains[n - 1][1], mains[n - 1][2], t + P["LS"])
        if n >= 2 and mains[n - 2] is not None and mains[n - 2][0] == "qk":
            _, j, hh = mains[n - 2]
            if j > 0:
                attn_pp(j - 1, hh, t + P["PP"])
            if j == NB - 1:
                attn_pp(j, hh, t + P["PP"])


    def out_copy(pidx, e0, e1, r0, r1):
        off = pidx * (2 * LB) + e0 * LB
        if not isinstance(pidx, int):
            off = pl.multiple_of(off, LB)
        rs = pl.ds(r0, r1 - r0)
        return pltpu.make_async_copy(out_v.at[pidx, rs, pl.ds(e0 * LB, (e1 - e0) * LB)],
                                     out_hbm.at[0, rs, pl.ds(off, (e1 - e0) * LB)], sems.at[0])

    TOP = {0: ((0, 0), 1, (1, 1)), 1: ((0, 0),), 2: ((0, 1), -1, (1, 1)), 3: ((1, 0), -1, (0, 0)),
           4: ((1, 1),), 5: ((0, 0), 1, (0, 1)), 6: ((1, 0), 1, (1, 1))}

    def top_op(p, blk):
        t = TOP[p]
        if len(t) == 1:
            return blk(*t[0])
        return blk(*t[0]) + blk(*t[2]) if t[1] > 0 else blk(*t[0]) - blk(*t[2])

    def rr_prep(ps, pa, osrc, n0, n1, t0, dur):
        for n in range(n0, n1):
            z = _zero(at(t0 + (n - n0) * dur // (n1 - n0)))
            qd, g = divmod(n, 8)
            cache = {}

            def wblk(i):
                def blk(x, y):
                    if (i, x, y) not in cache:
                        rf = (x * NFP + i) * LB + g * 16
                        if x == y and x in P["STG"] and ps[0] in SIDX:
                            cache[i, x, y] = wf_s[rf:rf + 16, :]
                        else:
                            r = (2 * i + x) * LB + g * 16
                            cache[i, x, y] = w2_v[pa + y, r:r + 16, :].astype(f32)
                            if x == y and x in P["STG"]:
                                wf_s[rf:rf + 16, :] = cache[i, x, y]
                    return cache[i, x, y]
                return blk

            def oblk(h):
                def blk(x, y):
                    if (h, x, y) not in cache:
                        r = x * HD + h * QD + g * 16
                        cache[h, x, y] = osrc[r:r + 16, y * 2 * LB:(y + 1) * 2 * LB]
                    return cache[h, x, y]
                return blk
            for p in ps:
                raw_p = p not in SIDX
                ro = p * RRK + g * 8
                if qd == NQ:
                    if raw_p and TOP[p][0][0] in P["STG"]:
                        top_op(p, wblk(2 * NQ))
                    if not raw_p:
                        r = top_op(p, wblk(2 * NQ))
                        for e in range(2):
                            rr_s[ro:ro + 8, _blk(7 + e)] = _pkz(r[:, _blk(e)], z)
                    continue
                if qd < NQ:
                    r1, r2 = top_op(p, wblk(2 * qd)), top_op(p, wblk(2 * qd + 1))
                    ro += qd * (LB // 2)
                else:
                    r1, r2 = top_op(p, oblk(0)), top_op(p, oblk(1))
                    ro += NQ * (LB // 2)
                if P["RT"] == 1:
                    c11, c22 = [v if z is None else jnp.concatenate([_orz(v[0:8], z), v[8:16]], axis=0)
                                for v in (r1[:, :LB], r2[:, LB:])]
                else:
                    c11, c22 = [v if z is None else _orz(v, _x2(z)) for v in (r1[:, :LB], r2[:, LB:])]
                zo = None
                sm = _rhs_sums(c11, r1[:, LB:], r2[:, :LB], c22)
                if not raw_p or qd > NQ:
                    sm.update({1: c11, 4: c22})
                for q, v in sm.items():
                    rr_s[ro:ro + 8, _blk(q)] = _pkz(v, zo)
        if n1 == NRG:
            ready.update({("rr", p) for p in ps})

    NRG = 8 * (NQ + 1) + 7
    PD = 8 * QD
    BORD = P["BORD"]

    def rr_tasks(ps, pa, osrc, t0, t1):
        wgt = [8, 8, 8, 2, 7]
        cuts = list(range(0, NRG, 8)) + [NRG]
        todo, acc = [], 0
        for a, b, w in zip(cuts[:-1], cuts[1:], wgt):
            ta, tb = t0 + acc * (t1 - t0) // 33, t0 + (acc + w) * (t1 - t0) // 33
            todo.append((tb, rr_prep, (ps, pa, osrc, a, b, ta, tb - ta)))
            acc += w
        return todo

    def big_piece(pa, pan, olc_s, oln_s, last):
        order = BORD
        t0 = now()
        todo = []
        for n in range(7):
            ta, tb = t0 + n * PD + P["RR0"], t0 + n * PD + P["RR1"]
            if n < 6:
                todo += rr_tasks((order[n + 1],), pa, olc_s, ta, tb)
            else:
                todo += rr_tasks((order[0],), pan, oln_s, ta, tb - (P["RRM"] if last else 0))
        for n, (f, bd) in enumerate(P["BPV"]):
            e, hh = divmod(n, 2)
            t = t0 + int(f * PD)
            todo.append((t + bd, attn_pv, (pan * 2 + e, hh, oln_s, e, t, bd, t + bd + P["PVL"])))
        add_tasks(todo)
        m = [None] * 7
        for p in order:
            flush(now())
            assert ("rr", p) in ready
            ready.discard(("rr", p))
            x, y = TOP[p][0]

            def lhs(q, k0, k1):
                if q in (2, 3):
                    rows = slice(p * QD + (q - 2) * ED, p * QD + (q - 1) * ED)
                    return _up(jnp.concatenate([lc_s[rows, _blk(2 * qd + q - 2)] for qd in range(NQ)]
                                               + [lc_s[rows, (NFP + q - 2) * LB:(NFP + q - 2) * LB + QD]], axis=1))
                return _up(ll_s[(p * 7 + q) * ED:(p * 7 + q + 1) * ED, 0:KL])

            def rhs(q, k0, k1):
                if p in SIDX or q in SIDX:
                    return _up(rr_s[p * RRK:p * RRK + KL // 2, _blk(q)])
                h = 0 if q == 1 else 1
                return _cat([w2_v[pa + y, _blk(2 * (2 * qd + h) + x), _blk(h)] for qd in range(NQ)]
                            + [_up(rr_s[p * RRK + NQ * LB // 2:p * RRK + KL // 2, _blk(q)])], 0)
            rl = (_up(rr_s[p * RRK:p * RRK + LB // 2, 7 * LB:9 * LB]) if p in SIDX
                  else w2_v[pa + y, _blk(4 * NQ + x), :])
            ll = _up(lc_s[p * QD:(p + 1) * QD, _blk(2 * NQ)])
            ex = [mm1(ll[:QD], rl), mm1(ll[QD:], rl)]
            e12, e21 = ex[0][:, LB:], ex[1][:, :LB]
            e11 = (ex[0][:, :LB] + e12) - e21
            lf = strassen(lhs, rhs, KL, P["LORD"])
            c12 = (lf[2] + e12) + lf[4]
            c21 = (lf[1] + e21) + lf[3]
            xx = (lf[2] - lf[1]) + lf[0]
            c22 = (xx + ex[1][:, LB:]) + lf[5]
            c11 = ((xx + e11) + (c21 - c12)) + lf[6]
            m[p] = jnp.concatenate([jnp.concatenate([c11, c12], axis=1),
                                    jnp.concatenate([c21, c22], axis=1)], axis=0)
            n = {3: 2, order[3]: 1, 5: 3}.get(p)
            if n is not None:
                t, epd = now() + P["EP0"], P["EPL"] if (last and n == 3) else P["EPD"]
                if P["DEF"]:
                    add_tasks([(t + epd, b_out, (pa, n, list(m), (0, HD, 0, 2), t, epd))])
                else:
                    b_out(pa, n, m, (0, HD, 0, 2))
        if last:
            flush()
            for part in LAST_PARTS:
                b_out(pa, 0, m, part)
        else:
            t = now() + P["EP0"]
            add_tasks([(t + P["EPD"], b_out, (pa, 0, m, (0, HD, 0, 2), t, P["EPD"]))])

    LAST_PARTS = [(0, QD, 1, 2), (QD, HD, 0, 2), (0, QD, 0, 1)]

    def b_out(pa, n, m, part, t0=None, dur=None):
        a, y = divmod(n, 2)
        r0, r1, e0, e1 = part
        cols = slice(e0 * LB, e1 * LB)
        for r in range(r0, r1, 16):
            mm_ = [None if v is None else v[r:r + 16, cols] for v in m]
            c12, c21 = (lambda: mm_[2] + mm_[4]), (lambda: mm_[1] + mm_[3])
            xx = lambda: (mm_[2] - mm_[1]) + mm_[0]
            c = (c12() if n == 1 else c21() if n == 2 else xx() + mm_[5] if n == 3
                 else (xx() + mm_[6]) + (c21() - c12()))
            rows = slice(a * HD + r, a * HD + r + 16)
            o = c + b2f_s[pa + y, 0:1, cols] + x_v[pa + y, rows, cols].astype(f32)
            z = None if t0 is None else _zero(at(t0 + (r - r0) * dur // (r1 - r0)))
            if z is not None:
                o = jnp.concatenate([_orz(o[:, 0:LB], _x2(z)), o[:, LB:]], axis=1)
            out_v[pa + y, rows, cols] = o.astype(bf16)
        out_copy(pa + y, e0, e1, a * HD + r0, a * HD + r1).start()

    def c_body(it, carry):
        reset()
        _TRUE[:] = [one_s[...]]
        ready.add(("rr", BORD[0]))
        pa = 4 * it
        big_piece(pa, pa + 2, ola_s, olb_s, False)
        big_piece(pa + 2, lax.rem(pa + 4, NP), olb_s, ola_s, True)
        return carry

    x0 = Group(cp_x(0, 1))
    E1 = P["E1"]
    g1 = Group(cp_w1(0, 2, 0, E1))
    g2 = Group(cp_w1(0, 2, E1, NFP) + cp_x(1, 2))
    E3 = P["E3"]
    g3 = Group(cp_w1(2, UB0, 0, E3))
    g4 = Group((cp_w1(2, UB0, E3, NFP) if E3 < NFP else []) + [(wqkv_hbm, wqkv_v)])
    g5 = Group(cp_x(2, NP))
    g6 = Group(cp_w1(UB0, NB) + [(wo_hbm, wo_v), (b1_hbm, b1_v), (b2_hbm, b2_v)] + cp_w2(0, 1))
    g7 = Group(cp_w2(1, NP))
    for c in (x0, g1, g2, g3, g4, g5, g6, g7):
        c.start()

    v_s[0] = jnp.zeros((D, LB), f32)
    for buf in (xnT_s, ra_s, lh_s, rs_s, rr_s, ola_s, olb_s, ll_s, lc_s, wf_s):
        buf[0:8, 0:64] = jnp.zeros((8, 64), buf.dtype)

    LND, BD, MARG = P["LND"], P["BD"], P["MARG"]

    def ln_tasks(b, t, lnd=LND, hsd=P["HSD"]):
        todo = []
        for fn, bb, dur, adv in ((ln, b, lnd, 0.8), (ln, b + 1, lnd, 0.86), (hpair, b, hsd, 1.0)):
            todo.append((t + int(dur * adv), fn, (bb, t, dur)))
            t += int(dur * adv)
        return todo, t

    wait("x0", x0)
    one_s[...] = lax.shift_right_logical(pltpu.bitcast(x_v[0, 0:16, 0:LB], i32), 1) | 1
    _TRUE[:] = [one_s[...]]
    ln(0); ln(1); hpair(0)
    wait("r1", g1)
    left_ = u_early(0, 0, E1, [], 7 * E1 // 4 * 4, -200, 100)
    wait("r2", g2)
    add_tasks(ln_tasks(2, P["L2T"], P["L2D"], P["H2D"])[0])
    n2 = (len(left_) + 7 * (NFP - E1)) // 4 * 4
    left_ = u_early(0, E1, NFP, left_, n2, -200, 120)
    wait("r3", g3)
    left_ = u_early(1, 0, E3, left_, P["N3"], -200, 140)
    wait("wqkv", g4)
    n4 = len(left_) + 7 * (NFP - E3)
    u_early(1, E3, NFP, left_, n4, -200, 100, nsplit=n4 % 4)
    prep_wqkv()
    stage_a(0, split_last=True)
    wait("mid", g5)
    AD = 7 * HA // 2
    UD = 7 * NUP * HD // 4
    r5 = (NP - 1) * AD
    t = 0
    for b in range(UB0, NB, 2):
        todo, t = ln_tasks(b, t)
        add_tasks(todo)
    n5 = 0
    while t + BD + MARG <= r5:
        add_tasks([(t + BD, slot, (t, BD))])
        t += BD
        n5 += 1
    for n, b in enumerate(range(2, NB, 2)):
        stage_a(b, odd=n % 2 == 1, split_last=b == NB - 2)
    wait("fin", g6)
    r6 = NFP * UD
    todo = []
    for i in range(NFP):
        if i == 0:
            t0, dt = -200, 130
        elif i == 1:
            t0, dt = 700, 260
        else:
            t0, dt = (i - 1) * UD + P["US0"], P["USD"]
        for k in range(NUP):
            tt = t0 + k * dt
            todo.append((tt + dt, tsum, (w1_ld(i), (UB0 + 2 * k) * LB, i % 3, k, tt, dt)))
    left = len(mains) - n5 - 2
    t = P["R6S"]
    bd2 = (r6 - P["R6E"] - t) // left
    for _ in range(left):
        todo.append((t + min(bd2, P["CAP"]), slot, (t, min(bd2, P["CAP"]))))
        t += bd2
    for i in range(2):
        todo.append((t + (i + 1) * 300, slot, (t + i * 300, 300)))
    for qd, t0, dur in ((NQ, UD + 300, 2 * UD - 300), (0, 3 * UD + 300, 2 * UD - 300), (1, 5 * UD + 300, UD - 100),
                        (2, 6 * UD + P["LL2"], P["UEL"])):
        for g in range(7):
            todo.append((t0 + (g + 1) * dur // 7, llsum, (qd, g, t0 + g * dur // 7, dur // 7)))
    todo += rr_tasks((BORD[0],), 0, ola_s, P["RP0"], P["RP1"])
    todo.append((P["PW0"] + P["PWD"], prep_wo_a, (P["PW0"], P["PWD"])))
    for h in range(2):
        t = P["PW1"] + h * P["PWE"]
        todo.append((t + P["PWE"], prep_wo_b, (h, t, P["PWE"])))
    add_tasks(todo)
    for b in range(NB):
        b2f_s[b // 2, 0:1, _blk(b % 2)] = b2_v[b:b + 1, :].astype(f32)
    for i in range(NFP):
        stage_u_last(i, (1, 4, 2, 3, 0, 5, 6) if i == 0 else P["UORD"],
                     None if i == NFP - 1 else P["UEL"] if i == NFP - 2 else P["UED"], split_last=i == NFP - 1)
    flush()
    assert slot_ctr[0] == len(mains) and all(("ll", qd, g) in ready for qd in range(NQ + 1) for g in range(7))
    wait("w2", g7)

    lax.fori_loop(0, NP // 4, c_body, 0)
    outs = []
    for pa in range(0, NP, 2):
        outs += [out_copy(pa + n % 2, 0, 2, n // 2 * HD, (n // 2 + 1) * HD) for n in (1, 2, 3)]
        outs += [out_copy(pa, e0, e1, r0, r1) for (r0, r1, e0, e1) in (LAST_PARTS if pa % 4 else [(0, HD, 0, 2)])]
    wait("out", *outs)


@jax.jit
def pallas_parallel_sum__sliding_local_dilated__mixer_token_mlp__prompt_kernel(A_x, A_wqkv, A_wo, B_x, B_w1, B_b1, B_w2, B_b2):
    del B_x
    hbm = pl.BlockSpec(memory_space=pltpu.HBM)
    outT = pl.pallas_call(
        _kernel,
        out_shape=jax.ShapeDtypeStruct((1, D, S), bf16),
        in_specs=[hbm] * 7,
        out_specs=hbm,
        scratch_shapes=[
            pltpu.VMEM((NP, D, 2 * LB), bf16),
            pltpu.VMEM((D, 3 * D), bf16),
            pltpu.VMEM((D, D), bf16),
            pltpu.VMEM((S, F), bf16),
            pltpu.VMEM((NP, F, 2 * LB), bf16),
            pltpu.VMEM((NFB, LB), bf16),
            pltpu.VMEM((NB, LB), bf16),
            pltpu.VMEM((NP, D, 2 * LB), bf16),
            pltpu.VMEM((2, 3 * D, LB), i32),
            pltpu.VMEM((7 * HA // 2, HD), u32),
            pltpu.VMEM((4, HD, LB), i32),
            pltpu.VMEM((D, 2 * LB), i32),
            pltpu.VMEM((HD, S), u32),
            pltpu.VMEM((NP * QD, 5 * LB), u32),
            pltpu.VMEM((7 * QD, NP * LB), u32),
            pltpu.VMEM((7 * HD, NFP * LB), f32),
            pltpu.VMEM((7 * QD, KC), u32),
            pltpu.VMEM((NB + 1, 2 * D, LB), f32),
            pltpu.VMEM((NB + 1, D, LB), f32),
            pltpu.VMEM((NB, 2 * W * HH, LB), f32),
            pltpu.VMEM((D, LB), f32),
            pltpu.VMEM((NP, 32, 2 * LB), f32),
            pltpu.VMEM((5 * RSK, 5 * LB), u32),
            pltpu.VMEM((49 * ED, 4 * LB), u32),
            pltpu.VMEM((7 * RRK, 9 * LB), u32),
            pltpu.VMEM((D, 4 * LB), f32),
            pltpu.VMEM((D, 4 * LB), f32),
            pltpu.VMEM((F, 2 * LB), f32),
            pltpu.VMEM((8, LB), i32),
            pltpu.SemaphoreType.DMA((9,)),
        ],
        compiler_params=pltpu.CompilerParams(vmem_limit_bytes=100 * 1024 * 1024,
                                             disable_bounds_checks=True,
                                             disable_semaphore_checks=True),
    )(jnp.swapaxes(A_x, 1, 2), A_wqkv, A_wo, B_w1, B_b1.reshape(NFB, LB), B_w2, B_b2.reshape(NB, LB))
    return jnp.swapaxes(outT, 1, 2)
```

```python
import jax
import jax.numpy as jnp
from jax import lax
import jax.experimental.pallas as pl
import jax.experimental.pallas.tpu as pltpu

S, D, F = 2048, 448, 1792
H, DH, W, DIL = 16, 28, 8, 2
LB = 128
NB = S // LB
NP = NB // 2
NFB = F // LB
NFP = NFB // 2
HH = H // 2
WH = W // 2
SH = DIL * WH
HD = D // 2
QD = D // 4
HA = 3 * HD
UB0 = 4
NUP = (NB - UB0) // 2
KC = F // 2 + 2 * LB
RSK = NFP * LB // 2
NQ = NFP // 2
KL = NQ * LB + QD
ED = D // 8
RRK = 2 * LB
EPS = 1e-5
SCALE = DH ** -0.5
f32 = jnp.float32
bf16 = jnp.bfloat16
u32 = jnp.uint32
i32 = jnp.int32

SCOPES = False
P = dict(LORD=(2, 4, 1, 3, 0, 5, 6), BORD=(1, 3, 2, 4, 0, 5, 6), DEF=True, OT=False, EP0=0, EPL=250, EPD=840, RR0=0, RR1=800, RRM=100, OC1=60,
         BPV=tuple((0.05 + 0.8 * i, 620) for i in range(8)),
         BVB=560, BVD=700, RT=1, STG=(),
         LND=400, BD=370, G=4, LAG=200, CAP=2000, LS=170, PP=150, MARG=300, N3=40, E3=6, W3T=700, W3D=600, W2T=200, W2D=450, W2X=300, E1=3, L2T=250, L2D=480, H2D=420, PVD=680, PV0=50, HSD=360, HG=0,
         CORD=(4, 2, 1, 3, 0, 5, 6), TS0=100, TSD=420, PVB=520, PVL=500, OS0=3050, OSD=300,
         UORD=(4, 2, 1, 3, 0, 5, 6), US0=100, USD=350, R6S=1900, PVPOS=12, R6E=2400, LL2=500, RP0=14200, RP1=16000, PVD2=400, NQ0=3, NQ1=7, QM1=750, LL0=1200, UR=False, HR=False, LNI=True, TI=True, HA4=True, HL=300,
         UE0=-200, UED=2100, UEL=1400, PW0=500, PWD=300, PW1=1300, PWE=400, UG=50, UM=24, PWL=2100, SK0=1500, LNQ1=4, LNQ3=4, LNA=0.3, LNB=0.42, LNBD=0.33)


def _gelu_half(hx, z=None):
    c = 0.7978845608028654
    return hx + hx * jnp.tanh(_orz(hx * (2.0 * c + (8.0 * c * 0.044715) * (hx * hx)), z))


def _pk(x):
    return pltpu.bitcast(x.astype(bf16), u32)


def _up(x):
    return pltpu.bitcast(x, bf16)


def _upf(x):
    return pltpu.bitcast(x, bf16).astype(f32)


def _cat(xs, axis):
    return xs[0] if len(xs) == 1 else jnp.concatenate(xs, axis=axis)


def _x2(v):
    return jnp.concatenate([v, v], axis=0)


def _blk(b):
    return slice(b * LB, (b + 1) * LB)


def _rowsum8(a):
    return jnp.broadcast_to(jnp.sum(a, axis=0, keepdims=True), (8, a.shape[1]))


_TRUE = []


def _zero(*deps):
    deps = [d for d in deps if d is not None]
    if not deps:
        return None
    bits = pltpu.bitcast(deps[0], u32)
    for d in deps[1:]:
        bits = bits | pltpu.bitcast(d, u32)
    return bits


def _orz(v, z):
    if z is None:
        return v
    m = _TRUE[0] if v.shape[0] == 8 else _x2(_TRUE[0])
    return jnp.where(m[:, 0:v.shape[1]] > 0, v, pltpu.bitcast(z, v.dtype))


def _pkz(v, z):
    return _pk(v if z is None else jnp.concatenate([_orz(v[0:8], z), v[8:16]], axis=0))


def _lhs_ops(a11, a12, a21, a22):
    return [a11 + a22, a21 + a22, a11, a22, a11 + a12, a21 - a11, a12 - a22]


SIDX = {0: 0, 2: 1, 3: 2, 5: 3, 6: 4}


def _rhs_sums(b11, b12, b21, b22):
    return {0: b11 + b22, 2: b12 - b22, 3: b21 - b11, 5: b11 + b12, 6: b21 + b22}


def _combine(m):
    c12 = m[2] + m[4]
    c21 = m[1] + m[3]
    x = (m[2] - m[1]) + m[0]
    return ((x + m[6]) + (c21 - c12), c12, c21, x + m[5])


def _kernel(x_hbm, wqkv_hbm, wo_hbm, w1_hbm, b1_hbm, w2_hbm, b2_hbm, out_hbm,
            x_v, wqkv_v, wo_v, w1_v, w2_v, b1_v, b2_v, out_v,
            wt_s, lw_s, wo_s, wq_s, xnT_s, ra_s, lh_s, um_s, lc_s, qk_s, v_s, pr_s, op_s,
            b2f_s, rs_s, ll_s, rr_s, ola_s, olb_s, wf_s, one_s, sems):
    sem_ctr = [1]

    class Group:
        def __init__(self, pairs):
            self.cps = [pltpu.make_async_copy(a, b, sems.at[sem_ctr[0]]) for (a, b) in pairs]
            sem_ctr[0] += 1

        def start(self):
            for c in self.cps:
                c.start()

        def wait(self):
            for c in self.cps:
                c.wait()

    def cp_x(p0, p1):
        return [(x_hbm.at[0, :, pl.ds(p * 2 * LB, 2 * LB)], x_v.at[p]) for p in range(p0, p1)]

    def cp_w2(p0, p1):
        return [(w2_hbm.at[:, pl.ds(p * 2 * LB, 2 * LB)], w2_v.at[p]) for p in range(p0, p1)]

    def cp_w1(b0, b1, i0=0, i1=NFP):
        sl = pl.ds(b0 * LB, (b1 - b0) * LB)
        cl = pl.ds(i0 * 2 * LB, (i1 - i0) * 2 * LB)
        return [(w1_hbm.at[sl, cl], w1_v.at[sl, cl])]

    tl = []
    mxu = [0, 0, 0, 0]
    nxt = [0]
    hist = []
    tasks = []
    dls = []
    ready = set()

    def add_tasks(todo):
        tasks.extend(todo)
        tasks.sort(key=lambda x: x[0])

    def flush(t=None):
        while tasks and (t is None or tasks[0][0] < t):
            _, fn, args = tasks.pop(0)
            fn(*args)

    def reset():
        assert not tasks
        dls.clear()
        tl.clear()
        hist.clear()
        mxu[:] = [0, 0, 0, 0]
        nxt[0] = 0

    def now():
        return sum(mxu) // 4

    def wait(name, *cps):
        flush()
        if SCOPES:
            with jax.named_scope("wait_" + name):
                for c in cps:
                    c.wait()
        else:
            for c in cps:
                c.wait()
        reset()

    def mm1(lhs, rhs, pace=True):
        flush(now())
        start = mxu[nxt[0]]
        due = [v for (t, v) in dls if t <= start] if pace else []
        if due:
            dls[:] = [(t, v) for (t, v) in dls if t > start]
            tile = _up(_orz(pltpu.bitcast(lhs[0:16, 0:LB], u32), _zero(*due)))
            row = tile if lhs.shape[1] == LB else jnp.concatenate([tile, lhs[0:16, LB:]], axis=1)
            lhs = jnp.concatenate([row, lhs[16:]], axis=0)
        r = jnp.dot(lhs, rhs, preferred_element_type=f32)
        m, k = lhs.shape
        first_done = None
        for _ in range(-(-rhs.shape[1] // LB)):
            end = 0
            for _ in range(-(-k // LB)):
                mxu[nxt[0]] += m
                end = max(end, mxu[nxt[0]])
                nxt[0] = (nxt[0] + 1) % 4
            if first_done is None:
                first_done = end
        if pace:
            tl.append((first_done - m, first_done, r))
        return r

    def mm(lhs, rhs, init=None):
        k = lhs.shape[1]
        r, k0 = init, 0
        while k0 < k:
            k1 = min(k, k0 + (4 - nxt[0]) * LB)
            part = mm1(lhs[:, k0:k1], rhs[k0:k1], pace=k1 - k0 > LB)
            r = part if r is None else r + part
            k0 = k1
        return r

    def at(t):
        if t is None or t < 0:
            return None
        t = min(t, now() - 1)
        best = None
        for (a, b, r) in tl:
            if a <= t and (best is None or min(b, t) > best[0]):
                row = int(min((t - a) / (b - a), 0.999) * (r.shape[0] // 8)) * 8
                best = (min(b, t), r, row)
        return None if best is None else best[1][best[2]:best[2] + 8, 0:LB]

    def strassen(lhs, rhs, k, order, split_last=False, head=0, init=None):
        m = [None] * 7

        def ops(p, k0, k1):
            flush(now())
            return lhs(p, k0, k1), rhs(p, k0, k1)

        if head:
            for p in order:
                m[p] = mm(*ops(p, 0, head * LB))
        for p in order:
            l, r = ops(p, head * LB, k)
            if split_last and p == order[-1]:
                kk = (-(-r.shape[0] // LB) - 2) * LB
                hm = l.shape[0] // 2
                hd = mm(l[:, :kk], r[:kk], None if init is None else init[p]) if kk else None
                tail = jnp.concatenate([mm(l[:hm, kk:], r[kk:]), mm(l[hm:, kk:], r[kk:])], axis=0)
                v = tail if hd is None else hd + tail
            else:
                v = mm(l, r, None if init is None else init[p])
            m[p] = v if m[p] is None else m[p] + v
        return m

    def put_sums(dst, sm, ro, z):
        for p, v in sm.items():
            dst[ro:ro + 8, _blk(SIDX[p])] = _pkz(v, z)

    def tsum(ld, r0, slot_, i, t0, dur):
        for g in range(LB // 16):
            z = _zero(at(t0 + g * dur // 8))
            t1 = ld(slice(r0 + g * 16, r0 + g * 16 + 16)).astype(f32)
            t2 = ld(slice(r0 + LB + g * 16, r0 + LB + g * 16 + 16)).astype(f32)
            if P["TI"] and z is not None:
                b11, b22 = [jnp.concatenate([_orz(v[0:8], z), v[8:16]], axis=0) for v in (t1[:, :LB], t2[:, LB:])]
                sm = _rhs_sums(b11, t1[:, LB:], t2[:, :LB], b22)
                z = None
            else:
                sm = _rhs_sums(t1[:, :LB], t1[:, LB:], t2[:, :LB], t2[:, LB:])
            put_sums(rs_s, sm, slot_ * RSK + i * (LB // 2) + g * 8, z)
        ready.add(("rs", slot_, i))

    def stored_rhs(slot_, p, k0, k1):
        assert all(("rs", slot_, i) in ready for i in range(k0 // LB, -(-k1 // LB))), (slot_, k0, k1)
        return _up(rs_s[slot_ * RSK + k0 // 2:slot_ * RSK + k1 // 2, _blk(SIDX[p])])

    def wrows(hh, g, z=None):
        p, d = divmod(2 * g, DH)
        t = [jnp.concatenate([wt_s[c, pl.ds(p * D + hh * HD + d + e, HH, stride=DH), :]
                              for e in range(2)], axis=0) for c in range(2)]
        if z is not None:
            t = [_orz(v, _x2(z)) for v in t]
        w = jnp.concatenate([t[0], t[1][:, 0:HD - LB]], axis=1)
        return [pltpu.bitcast(w << 16, f32), pltpu.bitcast(w & -65536, f32)]

    def prep_wqkv():
        done = set()
        ng = HA // 16

        def need(hh, p, z=None):
            lo = p * D + hh * HD
            for ct in range(lo // LB, -(-(lo + HD) // LB)):
                if ct in done:
                    continue
                done.add(ct)
                w = min(LB, 3 * D - ct * LB)
                k1, k2 = [pltpu.bitcast(wqkv_v[kh * HD:(kh + 1) * HD, ct * LB:ct * LB + w].astype(f32), i32)
                          for kh in range(2)]
                wd = lax.shift_right_logical(k1, 16) | k2
                if z is not None:
                    wd = jnp.concatenate([_orz(wd[r:r + 8], z[:, 0:w]) if r % LB == 0 else wd[r:r + 8]
                                          for r in range(0, HD, 8)], axis=0)
                wT = wd.T
                wt_s[0, ct * LB:ct * LB + w, :] = wT[:, 0:LB]
                wt_s[1, ct * LB:ct * LB + w, 0:HD - LB] = wT[:, LB:HD]

        def put(p, g, v):
            lw_s[p * (HA // 2) + g * 8:p * (HA // 2) + g * 8 + 8, :] = _pk(v)

        def half(hh, g0, g1, t0=None, dur=None):
            pr, ps = ((2, 4), (3, 1))[hh]
            for g in range(g0, g1):
                t = None if t0 is None else t0 + (g - g0) * dur // (g1 - g0)
                need(hh, 2 * g // DH, _zero(at(None if t is None else t - P["W2X"])))
                a1, a2 = wrows(hh, g, _zero(at(t)))
                put(pr, g, a2 if hh else a1)
                put(ps, g, a1 + a2)
            if g1 == ng:
                ready.update({("lw", pr), ("lw", ps)})
        half(0, 0, ng)
        t, dt = now() + P["W2T"], P["W2D"] // 3
        add_tasks([(t + (n + 1) * dt, half, (1, 14 * n, 14 * n + 14, t + n * dt, dt)) for n in range(3)])

        def rest(g0, g1, t0, dur):
            for g in range(g0, g1):
                z = _zero(at(t0 + (g - g0) * dur // (g1 - g0)))
                ops = _lhs_ops(*wrows(0, g, z), *wrows(1, g, z))
                for p in (0, 5, 6):
                    put(p, g, ops[p])
            if g1 == ng:
                ready.update({("lw", 0), ("lw", 5), ("lw", 6)})
        t, dt = now() + P["W3T"], P["W3D"] // 7
        add_tasks([(t + (n + 1) * dt, rest, (6 * n, 6 * n + 6, t + n * dt, dt)) for n in range(7)])

    def prep_wo_a(t0, dur):
        for g in range(HD // 16):
            k1, k2 = [pltpu.bitcast(wo_v[hh * HD + g * 16:hh * HD + g * 16 + 16, :].astype(f32), i32)
                      for hh in range(2)]
            w = lax.shift_right_logical(k1, 16) | k2
            z = _zero(at(t0 + g * dur // (HD // 16)))
            for c in range(4):
                cw = min(LB, D - c * LB)
                wo_s[c, g * 16:g * 16 + 16, 0:cw] = _orz(w[:, c * LB:c * LB + cw], None if z is None else _x2(z)[:, 0:cw])

    def prep_wo_b(h, t0, dur):
        for c in range(4):
            cw = min(LB, D - c * LB)
            rows = [wo_s[c, pl.ds(d, HH, stride=DH), :][:, 0:cw] for d in range(h * DH // 2, (h + 1) * DH // 2)]
            rows.append(jnp.zeros((LB - QD, cw), i32))
            wq_s[c * LB:c * LB + cw, _blk(h)] = jnp.concatenate(rows, axis=0).T
        bits = None
        for g in range(HD // 16):
            z = _zero(at(t0 + g * dur // (HD // 16)))
            a = []
            for r in (g * 16, HD + g * 16):
                w = _orz(wq_s[r:r + 16, _blk(h)], None if z is None else _x2(z))
                a += [pltpu.bitcast(w << 16, f32), pltpu.bitcast(w & -65536, f32)]
            for p, v in enumerate(_lhs_ops(*a)):
                lc_s[p * QD + g * 8:p * QD + g * 8 + 8, _blk(NFP + h)] = _pk(v)
                bits = pltpu.bitcast(v[0:8], u32) if bits is None else bits | pltpu.bitcast(v[0:8], u32)
        ready.update({("lc", NFP + h, g) for g in range(HD // 16)})
        dls.append((t0 + dur + 250, bits))

    def llsum(qd, g, t0, dur):
        i0 = 2 * qd if qd < NQ else NFP
        assert all(("lc", i0 + e, g + 7 * h) in ready for e in range(2) for h in range(2))
        for p in range(7):
            z = _zero(at(t0 + p * dur // 7))
            a = [_orz(lc_s[p * QD + h * ED + g * 8:p * QD + h * ED + g * 8 + 8, _blk(i0 + e)],
                      z if h == e else None) for h in range(2) for e in range(2)]
            ops = _lhs_ops(*[_upf(v) for v in a])
            for q in (0, 1, 4, 5, 6):
                r = (p * 7 + q) * ED + g * 8
                ll_s[r:r + 8, _blk(qd)] = _pk(ops[q])
        ready.add(("ll", qd, g))

    RG = 16
    NG = D // RG
    stat2 = {}

    def ln(b, t0=None, dur=None):
        def dep(fr):
            return None if t0 is None else at(t0 + fr * dur)

        def xg(g):
            return x_v[b // 2, g * RG:(g + 1) * RG, _blk(b % 2)].astype(f32)

        def halves(*vs):
            return [] if vs[0] is None else [v[i * 8:i * 8 + 8] for v in vs for i in range(2)]

        x0 = jnp.broadcast_to(xg(0)[0:1], (8, LB))
        s = q = None
        for g in range(NG):
            if g % P["LNQ1"] == 0 and t0 is not None:
                x0 = _orz(x0, _zero(dep(P["LNA"] * g / NG), *halves(s, q)))
            c = xg(g) - _x2(x0)
            s = c if s is None else s + c
            q = c * c if q is None else q + c * c
        dm = _rowsum8(s) * (1.0 / D)
        mu = x0 + dm
        r1 = lax.rsqrt(jnp.maximum(_rowsum8(q) * (1.0 / D) - dm * dm, 0.0) + EPS)
        s1 = s2 = z = None
        for g in range(NG):
            if g % P["LNQ3"] == 0 and t0 is not None:
                z = _zero(dep(P["LNB"] + P["LNBD"] * g / NG), *halves(s1, s2))
                if P["LNI"]:
                    mu, z = _orz(mu, z), None
            xn = (xg(g) - _x2(mu)) * _x2(r1)
            xnT_s[g * 8:g * 8 + 8, _blk(b)] = _pkz(xn, z)
            s1 = xn if s1 is None else s1 + xn
            s2 = xn * xn if s2 is None else s2 + xn * xn
        mu2 = _rowsum8(s1) * (1.0 / D)
        var2 = jnp.maximum(_rowsum8(s2) * (1.0 / D) - mu2 * mu2, 0.0)
        stat2[b] = (mu2, 0.5 * lax.rsqrt(var2 + EPS))

    def hpair(b, t0=None, dur=None):
        ng = HD // RG
        st = [stat2.pop(b), stat2.pop(b + 1)]
        for g in range(ng):
            t = None if t0 is None else t0 + g * dur // ng
            zi = _zero(at(None if t is None else t - P["HG"]))
            z = _zero(at(t)) if P["HR"] else None
            xq, hq = [], []
            for r in (g * 8, QD + g * 8):
                for e in range(2):
                    xn = _upf(_orz(xnT_s[r:r + 8, _blk(b + e)], zi if (P["HA4"] or (r >= QD) == (e == 1)) else None))
                    xq.append(xn)
                    hq.append((xn - _x2(st[e][0])) * _x2(st[e][1]))
            put_sums(ra_s, _rhs_sums(*xq), (b // 2) * QD + g * 8, z)
            for p, v in enumerate(_lhs_ops(*hq)):
                lh_s[p * QD + g * 8:p * QD + g * 8 + 8, _blk(b // 2)] = _pkz(v, z)
        ready.add(("xn", b))
        if t0 is not None and b >= UB0 and P["HL"]:
            got = ra_s[(b // 2) * QD:(b // 2 + 1) * QD, :]
            tiles_ = [got[r:r + 8, _blk(c)] for r in range(0, QD, 8) for c in range(5)]
            bits = tiles_[0]
            for v in tiles_[1:]:
                bits = bits | v
            dls.append((t0 + dur + P["HL"], bits))

    def w1_ld(i):
        return lambda rs: w1_v[rs, 2 * i * LB:(2 * i + 2) * LB]

    def ujob(kp, i, p, split=False):
        flush(now())
        assert ("xn", 2 * kp) in ready
        l = _up(lh_s[p * QD:(p + 1) * QD, _blk(kp)])
        if p in SIDX:
            r = stored_rhs(3 + kp, p, i * LB, (i + 1) * LB)
        else:
            e = 0 if p == 1 else 1
            r = w1_v[_blk(2 * kp + e), _blk(2 * i + e)]
        v = jnp.concatenate([mm1(l[:QD], r), mm1(l[QD:], r)], axis=0) if split else mm1(l, r)
        if kp == 1 and p in (2, 3):
            v = v + 0.5 * b1_v[2 * i + 3 - p:2 * i + 4 - p, :].astype(f32)
        rows = slice(p * HD, (p + 1) * HD)
        um_s[rows, _blk(i)] = v if kp == 0 else um_s[rows, _blk(i)] + v

    def u_early(kp, i0, i1, carry, n, t0, dt, nsplit=0):
        for k, i in enumerate(range(i0, i1)):
            add_tasks([(t0 + (k + 1) * dt, tsum, (w1_ld(i), 2 * kp * LB, 3 + kp, i, t0 + k * dt, dt))])
        jobs = (carry + [(kp, i, p) for i in range(i0, i1) for p in (1, 4)]
                + [(kp, i, p) for i in range(i0, i1) for p in SIDX])
        for c, job in enumerate(jobs[:n]):
            ujob(*job, split=c >= n - nsplit)
        return jobs[n:]

    def u_epilogue(i, m, gs, t0, dur):
        for n, g in enumerate(gs):
            t = -10 ** 6 if t0 is None else t0 + n * dur // len(gs)
            zi = [_zero(at(t - P["UG"] - (3 - n) * P["UM"])) for n in range(4)]
            zi = [None if v is None else _x2(v) for v in zi]
            q = _combine([x[g * 16:g * 16 + 16] for x in m])
            gl = [_gelu_half(q[0], zi[3]), _gelu_half(q[1], zi[0]), _gelu_half(q[2], zi[1]), _gelu_half(q[3], zi[2])]
            for p, v in enumerate(_lhs_ops(*gl)):
                lc_s[p * QD + g * 8:p * QD + g * 8 + 8, _blk(i)] = _pk(v)
            ready.add(("lc", i, g))

    def stage_u_last(i, order, edur, split_last=False):
        def lhs(p, k0, k1):
            return _up(lh_s[p * QD:(p + 1) * QD, UB0 // 2 * LB + k0:UB0 // 2 * LB + k1])

        def rhs(p, k0, k1):
            if p in SIDX:
                return stored_rhs(i % 3, p, k0, k1)
            e = 0 if p == 1 else 1
            return _cat([w1_v[_blk(UB0 + 2 * k + e), _blk(2 * i + e)] for k in range(k0 // LB, k1 // LB)], 0)
        m = strassen(lhs, rhs, NUP * LB, order, split_last, init=[um_s[p * HD:(p + 1) * HD, _blk(i)] for p in range(7)])
        for k in range(NUP):
            ready.discard(("rs", i % 3, k))
        if edur is None:
            u_epilogue(i, m, list(range(HD // 16)), None, None)
            return
        t = now() - P["UE0"]
        add_tasks([(t + (g + 1) * edur // 7, u_epilogue, (i, m, [g, g + 7], t + g * edur // 7, edur // 7))
                   for g in range(7)])

    def stage_a(b, odd=False, split_last=False):
        def lhs(p, k0, k1):
            assert ("lw", p) in ready
            return _up(lw_s[p * (HA // 2):(p + 1) * (HA // 2), :])

        def rhs(p, k0, k1):
            assert ("xn", b) in ready
            if p in SIDX:
                return _up(ra_s[(b // 2) * QD:(b // 2 + 1) * QD, _blk(SIDX[p])])
            return _up(xnT_s[0:QD, _blk(b)] if p == 1 else xnT_s[QD:HD, _blk(b + 1)])
        order = (6, 4, 2, 1, 3, 0, 5) if odd else (4, 2, 1, 3, 0, 5, 6)
        q = _combine(strassen(lhs, rhs, HD, order, split_last))
        for hh in range(2):
            for e in range(2):
                qk_s[b + e + 1, hh * D:(hh + 1) * D, :] = q[2 * hh + e][0:D]
                v_s[b + e + 1, hh * HD:(hh + 1) * HD, :] = q[2 * hh + e][D:HA]
        ready.update({("qkv", b), ("qkv", b + 1)})

    lane0 = lax.broadcasted_iota(i32, (HH, LB), 1)
    zeros8 = jnp.zeros((HH, LB), f32)

    def mk_shift(*deps):
        lane = _orz(lane0, _zero(*deps))

        def fwd(cur, prev, sh):
            if sh == 0:
                return cur
            return pltpu.roll(jnp.where(lane < LB - sh, cur, prev), sh, 1)

        def bwd(cur, nxt_):
            return pltpu.roll(jnp.where(lane >= SH, cur, nxt_), LB - SH, 1)
        return fwd, bwd

    def grp_shift(t, bd):
        lag = max(2, -(-P["LAG"] * DH // (P["G"] * bd)))
        deps = [at(t)]
        if len(hist) >= lag:
            deps += hist[-lag]
        return mk_shift(*deps)

    raw, probs = {}, {}

    def attn_qk(j, hh, t, bd):
        jn = min(j + 1, NB - 1)
        assert ("qkv", jn) in ready
        acc = [None] * WH
        accp = [None] * WH
        for d in range(DH):
            if d % P["G"] == 0:
                if d > 0:
                    hist.append(acc + accp)
                fwd, bwd = grp_shift(t + d * bd // DH, bd)
            r = hh * D + d * HH
            q = qk_s[j + 1, r:r + HH, :]
            qp = bwd(q, qk_s[jn + 1, r:r + HH, :])
            k = qk_s[j + 1, HD + r:HD + r + HH, :]
            kp = qk_s[j, HD + r:HD + r + HH, :] if j > 0 else zeros8
            for a in range(WH):
                ks = fwd(k, kp, DIL * a)
                t0, t1 = q * ks, qp * ks
                acc[a] = t0 if d == 0 else acc[a] + t0
                accp[a] = t1 if d == 0 else accp[a] + t1
        hist.append(acc + accp)
        raw[j, hh] = (acc, accp)

    def attn_sm(j, hh, t):
        fwd, _ = mk_shift(at(t))
        acc, accp = raw[j, hh]
        prev = raw.pop((j - 1, hh))[1] if j > 0 else [zeros8] * WH
        lg = acc + [fwd(accp[a], prev[a], SH) for a in range(WH)]
        lg = [a * SCALE for a in lg]
        if j == 0:
            lg = [lg[0]] + [jnp.where(lane0 >= DIL * w, lg[w], -1e9) for w in range(1, W)]
        m = lg[0]
        for w in range(1, W):
            m = jnp.maximum(m, lg[w])
        e = [jnp.exp(l - m) for l in lg]
        den = e[0]
        for w in range(1, W):
            den = den + e[w]
        inv = 1.0 / den
        p = [x * inv for x in e]
        for a in range(WH):
            pr_s[j, (hh * W + a) * HH:(hh * W + a + 1) * HH, :] = p[a]
        probs[j, hh] = p[WH:]

    def attn_pp(j, hh, t):
        _, bwd = mk_shift(at(t))
        p = probs.pop((j, hh))
        pn = probs[j + 1, hh] if j + 1 < NB else p
        for a in range(WH):
            pr_s[j, (hh * W + WH + a) * HH:(hh * W + WH + a + 1) * HH, :] = bwd(p[a], pn[a])
        ready.add(("pr", j, hh))

    def attn_pv(j, hh, dst, e, t, bd, t_dl):
        assert not isinstance(j, int) or ("pr", j, hh) in ready
        pa = [pr_s[j, (hh * W + a) * HH:(hh * W + a + 1) * HH, :] for a in range(W)]
        p, pp = pa[:WH], pa[WH:]
        outs = []
        for d in range(DH):
            if d % P["G"] == 0:
                if d > 0:
                    hist.append([])
                fwd, _ = grp_shift(t + d * bd // DH, bd)
            r = hh * HD + d * HH
            v = v_s[j + 1, r:r + HH, :]
            vp = v_s[j, r:r + HH, :]
            o = op = None
            for a in range(WH):
                vs = fwd(v, vp, DIL * a)
                o = p[a] * vs if a == 0 else o + p[a] * vs
                op = pp[a] * vs if a == 0 else op + pp[a] * vs
            opp = zeros8 if (isinstance(j, int) and j == 0) else op_s[r:r + HH, :]
            op_s[r:r + HH, :] = op
            outs.append(o + fwd(op, _orz(opp, _zero(o)) if P["OT"] else opp, SH))
            dst[r:r + HH, _blk(e)] = outs[-1]
        hist.append([])
        bits = pltpu.bitcast(outs[0], u32)
        for o in outs[1:]:
            bits = bits | pltpu.bitcast(o, u32)
        dls.append((t_dl, bits))

    mains = [("qk", j, hh) for j in range(NB) for hh in range(2)]
    mains = (mains[:P["PVPOS"]] + [("pv", j, hh) for j in range(4) for hh in range(2)]
             + mains[P["PVPOS"]:] + [None, None])
    slot_ctr = [0]

    def slot(t, bd):
        n = slot_ctr[0]
        slot_ctr[0] += 1
        it = mains[n]
        if it is None:
            pass
        elif it[0] == "qk":
            attn_qk(it[1], it[2], t, bd)
        else:
            attn_pv(it[1], it[2], ola_s, it[1], t, bd, t + bd + P["PVL"])
        if n >= 1 and mains[n - 1] is not None and mains[n - 1][0] == "qk":
            attn_sm(mains[n - 1][1], mains[n - 1][2], t + P["LS"])
        if n >= 2 and mains[n - 2] is not None and mains[n - 2][0] == "qk":
            _, j, hh = mains[n - 2]
            if j > 0:
                attn_pp(j - 1, hh, t + P["PP"])
            if j == NB - 1:
                attn_pp(j, hh, t + P["PP"])


    def out_copy(pidx, e0, e1, r0, r1):
        off = pidx * (2 * LB) + e0 * LB
        if not isinstance(pidx, int):
            off = pl.multiple_of(off, LB)
        rs = pl.ds(r0, r1 - r0)
        return pltpu.make_async_copy(out_v.at[pidx, rs, pl.ds(e0 * LB, (e1 - e0) * LB)],
                                     out_hbm.at[0, rs, pl.ds(off, (e1 - e0) * LB)], sems.at[0])

    TOP = {0: ((0, 0), 1, (1, 1)), 1: ((0, 0),), 2: ((0, 1), -1, (1, 1)), 3: ((1, 0), -1, (0, 0)),
           4: ((1, 1),), 5: ((0, 0), 1, (0, 1)), 6: ((1, 0), 1, (1, 1))}

    def top_op(p, blk):
        t = TOP[p]
        if len(t) == 1:
            return blk(*t[0])
        return blk(*t[0]) + blk(*t[2]) if t[1] > 0 else blk(*t[0]) - blk(*t[2])

    def rr_prep(ps, pa, osrc, n0, n1, t0, dur):
        for n in range(n0, n1):
            z = _zero(at(t0 + (n - n0) * dur // (n1 - n0)))
            qd, g = divmod(n, 8)
            cache = {}

            def wblk(i):
                def blk(x, y):
                    if (i, x, y) not in cache:
                        rf = (x * NFP + i) * LB + g * 16
                        if x == y and x in P["STG"] and ps[0] in SIDX:
                            cache[i, x, y] = wf_s[rf:rf + 16, :]
                        else:
                            r = (2 * i + x) * LB + g * 16
                            cache[i, x, y] = w2_v[pa + y, r:r + 16, :].astype(f32)
                            if x == y and x in P["STG"]:
                                wf_s[rf:rf + 16, :] = cache[i, x, y]
                    return cache[i, x, y]
                return blk

            def oblk(h):
                def blk(x, y):
                    if (h, x, y) not in cache:
                        r = x * HD + h * QD + g * 16
                        cache[h, x, y] = osrc[r:r + 16, y * 2 * LB:(y + 1) * 2 * LB]
                    return cache[h, x, y]
                return blk
            for p in ps:
                raw_p = p not in SIDX
                ro = p * RRK + g * 8
                if qd == NQ:
                    if raw_p and TOP[p][0][0] in P["STG"]:
                        top_op(p, wblk(2 * NQ))
                    if not raw_p:
                        r = top_op(p, wblk(2 * NQ))
                        for e in range(2):
                            rr_s[ro:ro + 8, _blk(7 + e)] = _pkz(r[:, _blk(e)], z)
                    continue
                if qd < NQ:
                    r1, r2 = top_op(p, wblk(2 * qd)), top_op(p, wblk(2 * qd + 1))
                    ro += qd * (LB // 2)
                else:
                    r1, r2 = top_op(p, oblk(0)), top_op(p, oblk(1))
                    ro += NQ * (LB // 2)
                if P["RT"] == 1:
                    c11, c22 = [v if z is None else jnp.concatenate([_orz(v[0:8], z), v[8:16]], axis=0)
                                for v in (r1[:, :LB], r2[:, LB:])]
                else:
                    c11, c22 = [v if z is None else _orz(v, _x2(z)) for v in (r1[:, :LB], r2[:, LB:])]
                zo = None
                sm = _rhs_sums(c11, r1[:, LB:], r2[:, :LB], c22)
                if not raw_p or qd > NQ:
                    sm.update({1: c11, 4: c22})
                for q, v in sm.items():
                    rr_s[ro:ro + 8, _blk(q)] = _pkz(v, zo)
        if n1 == NRG:
            ready.update({("rr", p) for p in ps})

    NRG = 8 * (NQ + 1) + 7
    PD = 8 * QD
    BORD = P["BORD"]

    def rr_tasks(ps, pa, osrc, t0, t1):
        wgt = [8, 8, 8, 2, 7]
        cuts = list(range(0, NRG, 8)) + [NRG]
        todo, acc = [], 0
        for a, b, w in zip(cuts[:-1], cuts[1:], wgt):
            ta, tb = t0 + acc * (t1 - t0) // 33, t0 + (acc + w) * (t1 - t0) // 33
            todo.append((tb, rr_prep, (ps, pa, osrc, a, b, ta, tb - ta)))
            acc += w
        return todo

    def big_piece(pa, pan, olc_s, oln_s, last):
        order = BORD
        t0 = now()
        todo = []
        for n in range(7):
            ta, tb = t0 + n * PD + P["RR0"], t0 + n * PD + P["RR1"]
            if n < 6:
                todo += rr_tasks((order[n + 1],), pa, olc_s, ta, tb)
            else:
                todo += rr_tasks((order[0],), pan, oln_s, ta, tb - (P["RRM"] if last else 0))
        for n, (f, bd) in enumerate(P["BPV"]):
            e, hh = divmod(n, 2)
            t = t0 + int(f * PD)
            todo.append((t + bd, attn_pv, (pan * 2 + e, hh, oln_s, e, t, bd, t + bd + P["PVL"])))
        add_tasks(todo)
        m = [None] * 7
        for p in order:
            flush(now())
            assert ("rr", p) in ready
            ready.discard(("rr", p))
            x, y = TOP[p][0]

            def lhs(q, k0, k1):
                if q in (2, 3):
                    rows = slice(p * QD + (q - 2) * ED, p * QD + (q - 1) * ED)
                    return _up(jnp.concatenate([lc_s[rows, _blk(2 * qd + q - 2)] for qd in range(NQ)]
                                               + [lc_s[rows, (NFP + q - 2) * LB:(NFP + q - 2) * LB + QD]], axis=1))
                return _up(ll_s[(p * 7 + q) * ED:(p * 7 + q + 1) * ED, 0:KL])

            def rhs(q, k0, k1):
                if p in SIDX or q in SIDX:
                    return _up(rr_s[p * RRK:p * RRK + KL // 2, _blk(q)])
                h = 0 if q == 1 else 1
                return _cat([w2_v[pa + y, _blk(2 * (2 * qd + h) + x), _blk(h)] for qd in range(NQ)]
                            + [_up(rr_s[p * RRK + NQ * LB // 2:p * RRK + KL // 2, _blk(q)])], 0)
            rl = (_up(rr_s[p * RRK:p * RRK + LB // 2, 7 * LB:9 * LB]) if p in SIDX
                  else w2_v[pa + y, _blk(4 * NQ + x), :])
            ll = _up(lc_s[p * QD:(p + 1) * QD, _blk(2 * NQ)])
            ex = [mm1(ll[:QD], rl), mm1(ll[QD:], rl)]
            e12, e21 = ex[0][:, LB:], ex[1][:, :LB]
            e11 = (ex[0][:, :LB] + e12) - e21
            lf = strassen(lhs, rhs, KL, P["LORD"])
            if p in (2, 3):
                for q in (2, 3):
                    lf[q] = lf[q] + b2f_s[pa + 3 - p, 0:1, _blk(3 - q)]
            c12 = (lf[2] + e12) + lf[4]
            c21 = (lf[1] + e21) + lf[3]
            xx = (lf[2] - lf[1]) + lf[0]
            c22 = (xx + ex[1][:, LB:]) + lf[5]
            c11 = ((xx + e11) + (c21 - c12)) + lf[6]
            m[p] = jnp.concatenate([jnp.concatenate([c11, c12], axis=1),
                                    jnp.concatenate([c21, c22], axis=1)], axis=0)
            n = {3: 2, order[3]: 1, 5: 3}.get(p)
            if n is not None:
                t, epd = now() + P["EP0"], P["EPL"] if (last and n == 3) else P["EPD"]
                if P["DEF"]:
                    add_tasks([(t + epd, b_out, (pa, n, list(m), (0, HD, 0, 2), t, epd))])
                else:
                    b_out(pa, n, m, (0, HD, 0, 2))
        if last:
            flush()
            for part in LAST_PARTS:
                b_out(pa, 0, m, part)
        else:
            t = now() + P["EP0"]
            add_tasks([(t + P["EPD"], b_out, (pa, 0, m, (0, HD, 0, 2), t, P["EPD"]))])

    LAST_PARTS = [(0, QD, 1, 2), (QD, HD, 0, 2), (0, QD, 0, 1)]

    def b_out(pa, n, m, part, t0=None, dur=None):
        a, y = divmod(n, 2)
        r0, r1, e0, e1 = part
        cols = slice(e0 * LB, e1 * LB)
        for r in range(r0, r1, 16):
            mm_ = [None if v is None else v[r:r + 16, cols] for v in m]
            c12, c21 = (lambda: mm_[2] + mm_[4]), (lambda: mm_[1] + mm_[3])
            xx = lambda: (mm_[2] - mm_[1]) + mm_[0]
            c = (c12() if n == 1 else c21() if n == 2 else xx() + mm_[5] if n == 3
                 else (xx() + mm_[6]) + (c21() - c12()))
            rows = slice(a * HD + r, a * HD + r + 16)
            o = c + x_v[pa + y, rows, cols].astype(f32)
            z = None if t0 is None else _zero(at(t0 + (r - r0) * dur // (r1 - r0)))
            if z is not None:
                o = jnp.concatenate([_orz(o[:, 0:LB], _x2(z)), o[:, LB:]], axis=1)
            out_v[pa + y, rows, cols] = o.astype(bf16)
        out_copy(pa + y, e0, e1, a * HD + r0, a * HD + r1).start()

    def c_body(it, carry):
        reset()
        _TRUE[:] = [one_s[...]]
        ready.add(("rr", BORD[0]))
        pa = 4 * it
        big_piece(pa, pa + 2, ola_s, olb_s, False)
        big_piece(pa + 2, lax.rem(pa + 4, NP), olb_s, ola_s, True)
        return carry

    x0 = Group(cp_x(0, 1))
    E1 = P["E1"]
    g1 = Group(cp_w1(0, 2, 0, E1))
    g2 = Group(cp_w1(0, 2, E1, NFP) + cp_x(1, 2))
    E3 = P["E3"]
    g3 = Group([(b1_hbm, b1_v)] + cp_w1(2, UB0, 0, E3))
    g4 = Group((cp_w1(2, UB0, E3, NFP) if E3 < NFP else []) + [(wqkv_hbm, wqkv_v)])
    g5 = Group(cp_x(2, NP))
    g6 = Group(cp_w1(UB0, NB) + [(wo_hbm, wo_v), (b2_hbm, b2_v)] + cp_w2(0, 1))
    g7 = Group(cp_w2(1, NP))
    for c in (x0, g1, g2, g3, g4, g5, g6, g7):
        c.start()

    v_s[0] = jnp.zeros((D, LB), f32)
    for buf in (xnT_s, ra_s, lh_s, rs_s, rr_s, ola_s, olb_s, ll_s, lc_s, wf_s):
        buf[0:8, 0:64] = jnp.zeros((8, 64), buf.dtype)

    LND, BD, MARG = P["LND"], P["BD"], P["MARG"]

    def ln_tasks(b, t, lnd=LND, hsd=P["HSD"]):
        todo = []
        for fn, bb, dur, adv in ((ln, b, lnd, 0.8), (ln, b + 1, lnd, 0.86), (hpair, b, hsd, 1.0)):
            todo.append((t + int(dur * adv), fn, (bb, t, dur)))
            t += int(dur * adv)
        return todo, t

    wait("x0", x0)
    one_s[...] = lax.shift_right_logical(pltpu.bitcast(x_v[0, 0:16, 0:LB], i32), 1) | 1
    _TRUE[:] = [one_s[...]]
    ln(0); ln(1); hpair(0)
    wait("r1", g1)
    left_ = u_early(0, 0, E1, [], 7 * E1 // 4 * 4, -200, 100)
    wait("r2", g2)
    add_tasks(ln_tasks(2, P["L2T"], P["L2D"], P["H2D"])[0])
    n2 = (len(left_) + 7 * (NFP - E1)) // 4 * 4
    left_ = u_early(0, E1, NFP, left_, n2, -200, 120)
    wait("r3", g3)
    left_ = u_early(1, 0, E3, left_, P["N3"], -200, 140)
    wait("wqkv", g4)
    n4 = len(left_) + 7 * (NFP - E3)
    u_early(1, E3, NFP, left_, n4, -200, 100, nsplit=n4 % 4)
    prep_wqkv()
    stage_a(0, split_last=True)
    wait("mid", g5)
    AD = 7 * HA // 2
    UD = 7 * NUP * HD // 4
    r5 = (NP - 1) * AD
    t = 0
    for b in range(UB0, NB, 2):
        todo, t = ln_tasks(b, t)
        add_tasks(todo)
    n5 = 0
    while t + BD + MARG <= r5:
        add_tasks([(t + BD, slot, (t, BD))])
        t += BD
        n5 += 1
    for n, b in enumerate(range(2, NB, 2)):
        stage_a(b, odd=n % 2 == 1, split_last=b == NB - 2)
    wait("fin", g6)
    r6 = NFP * UD
    todo = []
    for i in range(NFP):
        if i == 0:
            t0, dt = -200, 130
        elif i == 1:
            t0, dt = 700, 260
        else:
            t0, dt = (i - 1) * UD + P["US0"], P["USD"]
        for k in range(NUP):
            tt = t0 + k * dt
            todo.append((tt + dt, tsum, (w1_ld(i), (UB0 + 2 * k) * LB, i % 3, k, tt, dt)))
    left = len(mains) - n5 - 2
    t = P["R6S"]
    bd2 = (r6 - P["R6E"] - t) // left
    for _ in range(left):
        todo.append((t + min(bd2, P["CAP"]), slot, (t, min(bd2, P["CAP"]))))
        t += bd2
    for i in range(2):
        todo.append((t + (i + 1) * 300, slot, (t + i * 300, 300)))
    for qd, t0, dur in ((NQ, UD + 300, 2 * UD - 300), (0, 3 * UD + 300, 2 * UD - 300), (1, 5 * UD + 300, UD - 100),
                        (2, 6 * UD + P["LL2"], P["UEL"])):
        for g in range(7):
            todo.append((t0 + (g + 1) * dur // 7, llsum, (qd, g, t0 + g * dur // 7, dur // 7)))
    todo += rr_tasks((BORD[0],), 0, ola_s, P["RP0"], P["RP1"])
    todo.append((P["PW0"] + P["PWD"], prep_wo_a, (P["PW0"], P["PWD"])))
    for h in range(2):
        t = P["PW1"] + h * P["PWE"]
        todo.append((t + P["PWE"], prep_wo_b, (h, t, P["PWE"])))
    add_tasks(todo)
    for b in range(NB):
        b2f_s[b // 2, 0:1, _blk(b % 2)] = b2_v[b:b + 1, :].astype(f32)
    for i in range(NFP):
        stage_u_last(i, (1, 4, 2, 3, 0, 5, 6) if i == 0 else P["UORD"],
                     None if i == NFP - 1 else P["UEL"] if i == NFP - 2 else P["UED"], split_last=i == NFP - 1)
    flush()
    assert slot_ctr[0] == len(mains) and all(("ll", qd, g) in ready for qd in range(NQ + 1) for g in range(7))
    wait("w2", g7)

    lax.fori_loop(0, NP // 4, c_body, 0)
    outs = []
    for pa in range(0, NP, 2):
        outs += [out_copy(pa + n % 2, 0, 2, n // 2 * HD, (n // 2 + 1) * HD) for n in (1, 2, 3)]
        outs += [out_copy(pa, e0, e1, r0, r1) for (r0, r1, e0, e1) in (LAST_PARTS if pa % 4 else [(0, HD, 0, 2)])]
    wait("out", *outs)


@jax.jit
def pallas_parallel_sum__sliding_local_dilated__mixer_token_mlp__prompt_kernel(A_x, A_wqkv, A_wo, B_x, B_w1, B_b1, B_w2, B_b2):
    del B_x
    hbm = pl.BlockSpec(memory_space=pltpu.HBM)
    outT = pl.pallas_call(
        _kernel,
        out_shape=jax.ShapeDtypeStruct((1, D, S), bf16),
        in_specs=[hbm] * 7,
        out_specs=hbm,
        scratch_shapes=[
            pltpu.VMEM((NP, D, 2 * LB), bf16),
            pltpu.VMEM((D, 3 * D), bf16),
            pltpu.VMEM((D, D), bf16),
            pltpu.VMEM((S, F), bf16),
            pltpu.VMEM((NP, F, 2 * LB), bf16),
            pltpu.VMEM((NFB, LB), bf16),
            pltpu.VMEM((NB, LB), bf16),
            pltpu.VMEM((NP, D, 2 * LB), bf16),
            pltpu.VMEM((2, 3 * D, LB), i32),
            pltpu.VMEM((7 * HA // 2, HD), u32),
            pltpu.VMEM((4, HD, LB), i32),
            pltpu.VMEM((D, 2 * LB), i32),
            pltpu.VMEM((HD, S), u32),
            pltpu.VMEM((NP * QD, 5 * LB), u32),
            pltpu.VMEM((7 * QD, NP * LB), u32),
            pltpu.VMEM((7 * HD, NFP * LB), f32),
            pltpu.VMEM((7 * QD, KC), u32),
            pltpu.VMEM((NB + 1, 2 * D, LB), f32),
            pltpu.VMEM((NB + 1, D, LB), f32),
            pltpu.VMEM((NB, 2 * W * HH, LB), f32),
            pltpu.VMEM((D, LB), f32),
            pltpu.VMEM((NP, 32, 2 * LB), f32),
            pltpu.VMEM((5 * RSK, 5 * LB), u32),
            pltpu.VMEM((49 * ED, 4 * LB), u32),
            pltpu.VMEM((7 * RRK, 9 * LB), u32),
            pltpu.VMEM((D, 4 * LB), f32),
            pltpu.VMEM((D, 4 * LB), f32),
            pltpu.VMEM((F, 2 * LB), f32),
            pltpu.VMEM((8, LB), i32),
            pltpu.SemaphoreType.DMA((9,)),
        ],
        compiler_params=pltpu.CompilerParams(vmem_limit_bytes=100 * 1024 * 1024,
                                             disable_bounds_checks=True,
                                             disable_semaphore_checks=True),
    )(jnp.swapaxes(A_x, 1, 2), A_wqkv, A_wo, B_w1, B_b1.reshape(NFB, LB), B_w2, B_b2.reshape(NB, LB))
    return jnp.swapaxes(outT, 1, 2)
```

```python
import jax
import jax.numpy as jnp
from jax import lax
import jax.experimental.pallas as pl
import jax.experimental.pallas.tpu as pltpu

S, D, F = 2048, 448, 1792
H, DH, W, DIL = 16, 28, 8, 2
LB = 128
NB = S // LB
NP = NB // 2
NFB = F // LB
NFP = NFB // 2
HH = H // 2
WH = W // 2
SH = DIL * WH
HD = D // 2
QD = D // 4
ED = D // 8
HA = 3 * HD
UB0 = 4
NUP = (NB - UB0) // 2
RSK = NFP * LB // 2
NQ = NFP // 2
KL = NQ * LB + QD
RRK = 2 * LB
EPS = 1e-5
SCALE = DH ** -0.5
f32 = jnp.float32
bf16 = jnp.bfloat16
u32 = jnp.uint32
i32 = jnp.int32

SCOPES = False
P = dict(
    E1=3, E3=6, N3=40, L2T=250, L2D=480, H2D=420, W2T=200, W2D=450, W2X=300, W3T=700, W3D=600,
    LND=400, HSD=360, HL=300, LNA=0.3, LNB=0.42, LNBD=0.33, LNV=0.8, LNW=0.86,
    BD=370, MARG=300, LAG=200, LS=170, PP=150, PVL=500, PVPOS=12,
    US0=100, USD=350, UE0=200, UED=2100, UEL=1400, UG=50, UM=24, R6S=1900, R6E=2400,
    LL0=300, LL2=500, RP0=14200, RP1=16000, PW0=500, PWD=300, PW1=1300, PWE=400,
    RR0=0, RR1=800, RRM=100, RW=(8, 8, 8, 2, 7), BV0=45, BVS=717, BVD=620, EP0=0, EPD=840, EPL=250,
)
G = 4


def _pk(x):
    return pltpu.bitcast(x.astype(bf16), u32)


def _up(x):
    return pltpu.bitcast(x, bf16)


def _upf(x):
    return pltpu.bitcast(x, bf16).astype(f32)


def _word(lo, hi):
    lo, hi = [pltpu.bitcast(v.astype(f32), i32) for v in (lo, hi)]
    return lax.shift_right_logical(lo, 16) | hi


def _unword(w):
    return [pltpu.bitcast(w << 16, f32), pltpu.bitcast(w & -65536, f32)]


def _cat(xs, axis):
    return xs[0] if len(xs) == 1 else jnp.concatenate(xs, axis=axis)


def _x2(v):
    return jnp.concatenate([v, v], axis=0)


def _blk(b):
    return slice(b * LB, (b + 1) * LB)


def _rowsum8(a):
    return jnp.broadcast_to(jnp.sum(a, axis=0, keepdims=True), (8, a.shape[1]))


def _token(*deps):
    deps = [d for d in deps if d is not None]
    if not deps:
        return None
    bits = pltpu.bitcast(deps[0], u32)
    for d in deps[1:]:
        bits = bits | pltpu.bitcast(d, u32)
    return bits


def _lhs_ops(a11, a12, a21, a22):
    return [a11 + a22, a21 + a22, a11, a22, a11 + a12, a21 - a11, a12 - a22]


SIDX = {0: 0, 2: 1, 3: 2, 5: 3, 6: 4}
TOP = {0: ((0, 0), 1, (1, 1)), 1: ((0, 0),), 2: ((0, 1), -1, (1, 1)), 3: ((1, 0), -1, (0, 0)),
       4: ((1, 1),), 5: ((0, 0), 1, (0, 1)), 6: ((1, 0), 1, (1, 1))}


def _rhs_sums(b11, b12, b21, b22):
    return {0: b11 + b22, 2: b12 - b22, 3: b21 - b11, 5: b11 + b12, 6: b21 + b22}


def _rhs_op(p, blk):
    t = TOP[p]
    if len(t) == 1:
        return blk(*t[0])
    return blk(*t[0]) + blk(*t[2]) if t[1] > 0 else blk(*t[0]) - blk(*t[2])


def _combine(m, n=None):
    c12 = lambda: m[2] + m[4]
    c21 = lambda: m[1] + m[3]
    x = lambda: (m[2] - m[1]) + m[0]
    c = [lambda: (x() + m[6]) + (c21() - c12()), c12, c21, lambda: x() + m[5]]
    return [f() for f in c] if n is None else c[n]()


def _kernel(x_hbm, wqkv_hbm, wo_hbm, w1_hbm, b1_hbm, w2_hbm, b2_hbm, out_hbm,
            x_v, wqkv_v, wo_v, w1_v, w2_v, b1_v, b2_v, out_v,
            wt_s, lw_s, wo_s, wq_s, xnT_s, ra_s, lh_s, um_s, lc_s, qk_s, v_s, pr_s, op_s,
            b2f_s, rs_s, ll_s, rr_s, ola_s, olb_s, one_s, sems):
    sem_ctr = [1]

    class Group:
        def __init__(self, pairs):
            self.cps = [pltpu.make_async_copy(a, b, sems.at[sem_ctr[0]]) for (a, b) in pairs]
            sem_ctr[0] += 1

        def start(self):
            for c in self.cps:
                c.start()

        def wait(self):
            for c in self.cps:
                c.wait()

    def cp_x(p0, p1):
        return [(x_hbm.at[0, :, pl.ds(p * 2 * LB, 2 * LB)], x_v.at[p]) for p in range(p0, p1)]

    def cp_w2(p0, p1):
        return [(w2_hbm.at[:, pl.ds(p * 2 * LB, 2 * LB)], w2_v.at[p]) for p in range(p0, p1)]

    def cp_w1(b0, b1, i0=0, i1=NFP):
        sl = pl.ds(b0 * LB, (b1 - b0) * LB)
        cl = pl.ds(i0 * 2 * LB, (i1 - i0) * 2 * LB)
        return [(w1_hbm.at[sl, cl], w1_v.at[sl, cl])]

    tl = []
    mxu = [0, 0, 0, 0]
    nxt = [0]
    hist = []
    tasks = []
    dls = []
    ready = set()
    pos = []

    def tie(v, z):
        if z is None:
            return v
        rep = v.shape[0] // 8
        m, z = [_cat([a] * rep, 0)[:, 0:v.shape[1]] for a in (pos[0], z)]
        return jnp.where(m > 0, v, pltpu.bitcast(z, v.dtype))

    def tie8(v, z):
        return v if z is None else jnp.concatenate([tie(v[0:8], z), v[8:16]], axis=0)

    def add_tasks(todo):
        tasks.extend(todo)
        tasks.sort(key=lambda x: x[0])

    def flush(t=None):
        while tasks and (t is None or tasks[0][0] < t):
            _, fn, args = tasks.pop(0)
            fn(*args)

    def reset():
        assert not tasks
        dls.clear()
        tl.clear()
        hist.clear()
        mxu[:] = [0, 0, 0, 0]
        nxt[0] = 0

    def now():
        return sum(mxu) // 4

    def wait(name, *cps):
        flush()
        if SCOPES:
            with jax.named_scope("wait_" + name):
                for c in cps:
                    c.wait()
        else:
            for c in cps:
                c.wait()
        reset()

    def mm1(lhs, rhs, pace=True):
        flush(now())
        start = mxu[nxt[0]]
        due = [v for (t, v) in dls if t <= start] if pace else []
        if due:
            dls[:] = [(t, v) for (t, v) in dls if t > start]
            tile = _up(tie(pltpu.bitcast(lhs[0:16, 0:LB], u32), _token(*due)))
            row = tile if lhs.shape[1] == LB else jnp.concatenate([tile, lhs[0:16, LB:]], axis=1)
            lhs = jnp.concatenate([row, lhs[16:]], axis=0)
        r = jnp.dot(lhs, rhs, preferred_element_type=f32)
        m, k = lhs.shape
        first_done = None
        for _ in range(-(-rhs.shape[1] // LB)):
            end = 0
            for _ in range(-(-k // LB)):
                mxu[nxt[0]] += m
                end = max(end, mxu[nxt[0]])
                nxt[0] = (nxt[0] + 1) % 4
            if first_done is None:
                first_done = end
        if pace:
            tl.append((first_done - m, first_done, r))
        return r

    def mm(lhs, rhs, init=None):
        k = lhs.shape[1]
        r, k0 = init, 0
        while k0 < k:
            k1 = min(k, k0 + (4 - nxt[0]) * LB)
            part = mm1(lhs[:, k0:k1], rhs[k0:k1], pace=k1 - k0 > LB)
            r = part if r is None else r + part
            k0 = k1
        return r

    def at(t, *more):
        best = None
        if t is not None and t >= 0:
            t = min(t, now() - 1)
            for (a, b, r) in tl:
                if a <= t and (best is None or min(b, t) > best[0]):
                    row = int(min((t - a) / (b - a), 0.999) * (r.shape[0] // 8)) * 8
                    best = (min(b, t), r, row)
        return _token(None if best is None else best[1][best[2]:best[2] + 8, 0:LB], *more)

    def strassen(lhs, rhs, order, split_last=False, init=None):
        m = [None] * 7
        for p in order:
            flush(now())
            l, r = lhs(p), rhs(p)
            c0 = None if init is None else init[p]
            if split_last and p == order[-1]:
                kk = (-(-r.shape[0] // LB) - 2) * LB
                hm = l.shape[0] // 2
                hd = mm(l[:, :kk], r[:kk], c0) if kk else c0
                tail = jnp.concatenate([mm(l[:hm, kk:], r[kk:]), mm(l[hm:, kk:], r[kk:])], axis=0)
                m[p] = tail if hd is None else hd + tail
            else:
                m[p] = mm(l, r, c0)
        return m

    def wrows(hh, g, z=None):
        p, d = divmod(2 * g, DH)
        t = [jnp.concatenate([wt_s[c, pl.ds(p * D + hh * HD + d + e, HH, stride=DH), :]
                              for e in range(2)], axis=0) for c in range(2)]
        return _unword(jnp.concatenate([tie(t[0], z), tie(t[1][:, 0:HD - LB], z)], axis=1))

    def prep_wqkv():
        done = set()
        ng = HA // 16

        def need(hh, p, z):
            lo = p * D + hh * HD
            for ct in range(lo // LB, -(-(lo + HD) // LB)):
                if ct in done:
                    continue
                done.add(ct)
                cols = slice(ct * LB, min((ct + 1) * LB, 3 * D))
                wd = _word(wqkv_v[0:HD, cols], wqkv_v[HD:D, cols])
                wd = jnp.concatenate([tie(wd[r:r + 8], z if r % LB == 0 else None) for r in range(0, HD, 8)], axis=0)
                wT = wd.T
                wt_s[0, cols, :] = wT[:, 0:LB]
                wt_s[1, cols, 0:HD - LB] = wT[:, LB:HD]

        def put(p, g, v):
            lw_s[p * (HA // 2) + g * 8:p * (HA // 2) + g * 8 + 8, :] = _pk(v)

        def half(hh, g0, g1, t0=None, dur=None):
            pr, ps = ((2, 4), (3, 1))[hh]
            for g in range(g0, g1):
                t = None if t0 is None else t0 + (g - g0) * dur // (g1 - g0)
                need(hh, 2 * g // DH, at(None if t is None else t - P["W2X"]))
                a1, a2 = wrows(hh, g, at(t))
                put(pr, g, a2 if hh else a1)
                put(ps, g, a1 + a2)
            if g1 == ng:
                ready.update({("lw", pr), ("lw", ps)})

        def rest(g0, g1, t0, dur):
            assert ("lw", 1) in ready
            for g in range(g0, g1):
                z = at(t0 + (g - g0) * dur // (g1 - g0))
                ops = _lhs_ops(*wrows(0, g, z), *wrows(1, g, z))
                for p in (0, 5, 6):
                    put(p, g, ops[p])
            if g1 == ng:
                ready.update({("lw", 0), ("lw", 5), ("lw", 6)})
        half(0, 0, ng)
        t, dt = now() + P["W2T"], P["W2D"] // 3
        add_tasks([(t + (n + 1) * dt, half, (1, 14 * n, 14 * n + 14, t + n * dt, dt)) for n in range(3)])
        t, dt = now() + P["W3T"], P["W3D"] // 7
        add_tasks([(t + (n + 1) * dt, rest, (6 * n, 6 * n + 6, t + n * dt, dt)) for n in range(7)])

    def prep_wo_a(t0, dur):
        for g in range(HD // 16):
            w = _word(wo_v[g * 16:g * 16 + 16, :], wo_v[HD + g * 16:HD + g * 16 + 16, :])
            z = at(t0 + g * dur // (HD // 16))
            for c in range(4):
                cw = min(LB, D - c * LB)
                wo_s[c, g * 16:g * 16 + 16, 0:cw] = tie(w[:, c * LB:c * LB + cw], z)
        ready.add("wo")

    def prep_wo_b(h, t0, dur):
        assert "wo" in ready
        for c in range(4):
            cw = min(LB, D - c * LB)
            rows = [wo_s[c, pl.ds(d, HH, stride=DH), :][:, 0:cw] for d in range(h * DH // 2, (h + 1) * DH // 2)]
            rows.append(jnp.zeros((LB - QD, cw), i32))
            wq_s[c * LB:c * LB + cw, _blk(h)] = jnp.concatenate(rows, axis=0).T
        outs = []
        for g in range(HD // 16):
            z = at(t0 + g * dur // (HD // 16))
            a = [v for r in (g * 16, HD + g * 16) for v in _unword(tie(wq_s[r:r + 16, _blk(h)], z))]
            for p, v in enumerate(_lhs_ops(*a)):
                lc_s[p * QD + g * 8:p * QD + g * 8 + 8, _blk(NFP + h)] = _pk(v)
                outs.append(v[0:8])
        ready.update({("lc", NFP + h, g) for g in range(HD // 16)})
        dls.append((t0 + dur + 250, _token(*outs)))

    RG = 16
    NG = D // RG
    stat2 = {}

    def ln(b, t0=None, dur=None):
        def xg(g):
            return x_v[b // 2, g * RG:(g + 1) * RG, _blk(b % 2)].astype(f32)

        def step(v, g, fr, s, q):
            if t0 is None or g % 4:
                return v
            acc = [] if s is None else [s[0:8], s[8:16], q[0:8], q[8:16]]
            return tie(v, at(t0 + fr * dur, *acc))

        x0 = jnp.broadcast_to(xg(0)[0:1], (8, LB))
        s = q = None
        for g in range(NG):
            x0 = step(x0, g, P["LNA"] * g / NG, s, q)
            c = xg(g) - _x2(x0)
            s = c if s is None else s + c
            q = c * c if q is None else q + c * c
        dm = _rowsum8(s) * (1.0 / D)
        mu = x0 + dm
        r1 = lax.rsqrt(jnp.maximum(_rowsum8(q) * (1.0 / D) - dm * dm, 0.0) + EPS)
        s = q = None
        for g in range(NG):
            mu = step(mu, g, P["LNB"] + P["LNBD"] * g / NG, s, q)
            xn = (xg(g) - _x2(mu)) * _x2(r1)
            xnT_s[g * 8:g * 8 + 8, _blk(b)] = _pk(xn)
            s = xn if s is None else s + xn
            q = xn * xn if q is None else q + xn * xn
        mu2 = _rowsum8(s) * (1.0 / D)
        var2 = jnp.maximum(_rowsum8(q) * (1.0 / D) - mu2 * mu2, 0.0)
        stat2[b] = (mu2, 0.5 * lax.rsqrt(var2 + EPS))

    def hpair(b, t0=None, dur=None):
        ng = HD // RG
        st = [stat2.pop(b), stat2.pop(b + 1)]
        for g in range(ng):
            z = at(None if t0 is None else t0 + g * dur // ng)
            xq = [_upf(tie(xnT_s[r:r + 8, _blk(b + e)], z)) for r in (g * 8, QD + g * 8) for e in range(2)]
            hq = [(v - _x2(st[n % 2][0])) * _x2(st[n % 2][1]) for n, v in enumerate(xq)]
            ro = (b // 2) * QD + g * 8
            for p, v in _rhs_sums(*xq).items():
                ra_s[ro:ro + 8, _blk(SIDX[p])] = _pk(v)
            for p, v in enumerate(_lhs_ops(*hq)):
                lh_s[p * QD + g * 8:p * QD + g * 8 + 8, _blk(b // 2)] = _pk(v)
        ready.add(("xn", b))
        if b >= UB0:
            got = ra_s[(b // 2) * QD:(b // 2 + 1) * QD, :]
            dls.append((t0 + dur + P["HL"], _token(*[got[r:r + 8, _blk(c)] for r in range(0, QD, 8) for c in range(5)])))

    def ln_tasks(b, t, lnd, hsd):
        for fn, bb, dur, adv in ((ln, b, lnd, P["LNV"]), (ln, b + 1, lnd, P["LNW"]), (hpair, b, hsd, 1.0)):
            add_tasks([(t + int(dur * adv), fn, (bb, t, dur))])
            t += int(dur * adv)
        return t

    def tsum(kp, i, slot_, n, t0, dur):
        for g in range(LB // 16):
            z = at(t0 + g * dur // 8)
            t1, t2 = [w1_v[(2 * kp + e) * LB + g * 16:(2 * kp + e) * LB + g * 16 + 16,
                           2 * i * LB:(2 * i + 2) * LB].astype(f32) for e in range(2)]
            ro = slot_ * RSK + n * (LB // 2) + g * 8
            for p, v in _rhs_sums(tie8(t1[:, :LB], z), t1[:, LB:], t2[:, :LB], tie8(t2[:, LB:], z)).items():
                rs_s[ro:ro + 8, _blk(SIDX[p])] = _pk(v)
        ready.add(("rs", kp, i))

    def u_rhs(p, i, kps, slot_, n0):
        if p in SIDX:
            assert all(("rs", kp, i) in ready for kp in kps)
            ro = slot_ * RSK + n0 * (LB // 2)
            return _up(rs_s[ro:ro + len(kps) * (LB // 2), _blk(SIDX[p])])
        e = 0 if p == 1 else 1
        return _cat([w1_v[_blk(2 * kp + e), _blk(2 * i + e)] for kp in kps], 0)

    def ujob(kp, i, p, split):
        flush(now())
        assert ("xn", 2 * kp) in ready
        l, r = _up(lh_s[p * QD:(p + 1) * QD, _blk(kp)]), u_rhs(p, i, [kp], 3 + kp, i)
        v = jnp.concatenate([mm1(l[:QD], r), mm1(l[QD:], r)], axis=0) if split else mm1(l, r)
        if kp == 1 and p in (2, 3):
            v = v + 0.5 * b1_v[2 * i + 3 - p:2 * i + 4 - p, :].astype(f32)
        rows = slice(p * HD, (p + 1) * HD)
        um_s[rows, _blk(i)] = v if kp == 0 else um_s[rows, _blk(i)] + v

    def u_early(kp, i0, i1, carry, n, dt, nsplit=0):
        for k, i in enumerate(range(i0, i1)):
            add_tasks([((k + 1) * dt - 200, tsum, (kp, i, 3 + kp, i, k * dt - 200, dt))])
        jobs = (carry + [(kp, i, p) for i in range(i0, i1) for p in (1, 4)]
                + [(kp, i, p) for i in range(i0, i1) for p in SIDX])
        for c, job in enumerate(jobs[:n]):
            ujob(*job, c >= n - nsplit)
        return jobs[n:]

    def gelu_half(hx, z):
        c = 0.7978845608028654
        return hx + hx * jnp.tanh(tie(hx * (2.0 * c + (8.0 * c * 0.044715) * (hx * hx)), z))

    def u_epilogue(i, m, gs, t0, dur):
        for n, g in enumerate(gs):
            t = None if t0 is None else t0 + n * dur // len(gs) - P["UG"]
            q = _combine([x[g * 16:g * 16 + 16] for x in m])
            gl = [gelu_half(v, at(None if t is None else t - k * P["UM"])) for v, k in zip(q, (0, 3, 2, 1))]
            for p, v in enumerate(_lhs_ops(*gl)):
                lc_s[p * QD + g * 8:p * QD + g * 8 + 8, _blk(i)] = _pk(v)
            ready.add(("lc", i, g))

    def u_last(i, order, edur):
        kps = list(range(UB0 // 2, NP))
        m = strassen(lambda p: _up(lh_s[p * QD:(p + 1) * QD, UB0 // 2 * LB:]),
                     lambda p: u_rhs(p, i, kps, i % 3, 0), order, split_last=edur is None,
                     init=[um_s[p * HD:(p + 1) * HD, _blk(i)] for p in range(7)])
        if edur is None:
            u_epilogue(i, m, list(range(HD // 16)), None, None)
        else:
            t = now() + P["UE0"]
            add_tasks([(t + (g + 1) * edur // 7, u_epilogue, (i, m, [g, g + 7], t + g * edur // 7, edur // 7))
                       for g in range(7)])

    def llsum(qd, g, t0, dur):
        i0 = 2 * qd if qd < NQ else NFP
        assert all(("lc", i0 + e, g + 7 * h) in ready for e in range(2) for h in range(2))
        for p in range(7):
            z = at(t0 + p * dur // 7)
            a = [tie(lc_s[p * QD + h * ED + g * 8:p * QD + h * ED + g * 8 + 8, _blk(i0 + e)], z if h == e else None)
                 for h in range(2) for e in range(2)]
            ops = _lhs_ops(*[_upf(v) for v in a])
            for q in (0, 1, 4, 5, 6):
                r = (p * 7 + q) * ED + g * 8
                ll_s[r:r + 8, _blk(qd)] = _pk(ops[q])
        ready.add(("ll", qd, g))

    def stage_a(b, odd=False, split_last=False):
        def lhs(p):
            assert ("lw", p) in ready
            return _up(lw_s[p * (HA // 2):(p + 1) * (HA // 2), :])

        def rhs(p):
            assert ("xn", b) in ready
            if p in SIDX:
                return _up(ra_s[(b // 2) * QD:(b // 2 + 1) * QD, _blk(SIDX[p])])
            return _up(xnT_s[0:QD, _blk(b)] if p == 1 else xnT_s[QD:HD, _blk(b + 1)])
        order = (6, 4, 2, 1, 3, 0, 5) if odd else (4, 2, 1, 3, 0, 5, 6)
        q = _combine(strassen(lhs, rhs, order, split_last))
        for hh in range(2):
            for e in range(2):
                qk_s[b + e, hh * D:(hh + 1) * D, :] = q[2 * hh + e][0:D]
                v_s[b + e + 1, hh * HD:(hh + 1) * HD, :] = q[2 * hh + e][D:HA]
        ready.update({("qkv", b), ("qkv", b + 1)})

    lane0 = lax.broadcasted_iota(i32, (HH, LB), 1)
    zeros8 = jnp.zeros((HH, LB), f32)

    def mk_shift(z):
        lane = tie(lane0, z)

        def fwd(cur, prev, sh):
            if sh == 0:
                return cur
            return pltpu.roll(jnp.where(lane < LB - sh, cur, prev), sh, 1)

        def bwd(cur, nxt_):
            return pltpu.roll(jnp.where(lane >= SH, cur, nxt_), LB - SH, 1)
        return fwd, bwd

    def grp_shift(t, bd):
        lag = max(2, -(-P["LAG"] * DH // (G * bd)))
        return mk_shift(at(t, *(hist[-lag] if len(hist) >= lag else [])))

    raw, probs = {}, {}

    def attn_qk(j, hh, t, bd):
        jn = min(j + 1, NB - 1)
        assert ("qkv", jn) in ready
        acc = [None] * WH
        accp = [None] * WH
        for d in range(DH):
            if d % G == 0:
                if d > 0:
                    hist.append(acc + accp)
                fwd, bwd = grp_shift(t + d * bd // DH, bd)
            r = hh * D + d * HH
            q = qk_s[j, r:r + HH, :]
            qp = bwd(q, qk_s[jn, r:r + HH, :])
            k = qk_s[j, HD + r:HD + r + HH, :]
            kp = qk_s[j - 1, HD + r:HD + r + HH, :] if j > 0 else zeros8
            for a in range(WH):
                ks = fwd(k, kp, DIL * a)
                t0, t1 = q * ks, qp * ks
                acc[a] = t0 if d == 0 else acc[a] + t0
                accp[a] = t1 if d == 0 else accp[a] + t1
        hist.append(acc + accp)
        raw[j, hh] = (acc, accp)

    def attn_sm(j, hh, t):
        fwd, _ = mk_shift(at(t))
        acc, accp = raw[j, hh]
        prev = raw.pop((j - 1, hh))[1] if j > 0 else [zeros8] * WH
        lg = acc + [fwd(accp[a], prev[a], SH) for a in range(WH)]
        lg = [a * SCALE for a in lg]
        if j == 0:
            lg = [lg[0]] + [jnp.where(lane0 >= DIL * w, lg[w], -1e9) for w in range(1, W)]
        m = lg[0]
        for w in range(1, W):
            m = jnp.maximum(m, lg[w])
        e = [jnp.exp(l - m) for l in lg]
        den = e[0]
        for w in range(1, W):
            den = den + e[w]
        inv = 1.0 / den
        p = [x * inv for x in e]
        for a in range(WH):
            pr_s[j, (hh * W + a) * HH:(hh * W + a + 1) * HH, :] = p[a]
        probs[j, hh] = p[WH:]

    def attn_pp(j, hh, t):
        _, bwd = mk_shift(at(t))
        p = probs.pop((j, hh))
        pn = probs[j + 1, hh] if j + 1 < NB else p
        for a in range(WH):
            pr_s[j, (hh * W + WH + a) * HH:(hh * W + WH + a + 1) * HH, :] = bwd(p[a], pn[a])
        ready.add(("pr", j, hh))

    def attn_pv(j, hh, dst, e, t, bd):
        assert not isinstance(j, int) or ("pr", j, hh) in ready
        assert e == 0 or ("o", dst, hh, e - 1) in ready
        pa = [pr_s[j, (hh * W + a) * HH:(hh * W + a + 1) * HH, :] for a in range(W)]
        p, pp = pa[:WH], pa[WH:]
        outs = []
        for d in range(DH):
            if d % G == 0:
                if d > 0:
                    hist.append([])
                fwd, _ = grp_shift(t + d * bd // DH, bd)
            r = hh * HD + d * HH
            v = v_s[j + 1, r:r + HH, :]
            vp = v_s[j, r:r + HH, :]
            o = op = None
            for a in range(WH):
                vs = fwd(v, vp, DIL * a)
                o = p[a] * vs if a == 0 else o + p[a] * vs
                op = pp[a] * vs if a == 0 else op + pp[a] * vs
            opp = zeros8 if (isinstance(j, int) and j == 0) else op_s[r:r + HH, :]
            op_s[r:r + HH, :] = op
            outs.append(o + fwd(op, opp, SH))
            ol[dst][r:r + HH, _blk(e)] = outs[-1]
        hist.append([])
        ready.add(("o", dst, hh, e))
        dls.append((t + bd + P["PVL"], _token(*outs)))

    ol = [ola_s, olb_s]
    mains = [("qk", j, hh) for j in range(NB) for hh in range(2)]
    mains = (mains[:P["PVPOS"]] + [("pv", j, hh) for j in range(4) for hh in range(2)]
             + mains[P["PVPOS"]:] + [None, None])
    slot_ctr = [0]

    def slot(t, bd):
        n = slot_ctr[0]
        slot_ctr[0] += 1
        it = mains[n]
        if it is None:
            pass
        elif it[0] == "qk":
            attn_qk(it[1], it[2], t, bd)
        else:
            attn_pv(it[1], it[2], 0, it[1], t, bd)
        if n >= 1 and mains[n - 1] is not None and mains[n - 1][0] == "qk":
            attn_sm(mains[n - 1][1], mains[n - 1][2], t + P["LS"])
        if n >= 2 and mains[n - 2] is not None and mains[n - 2][0] == "qk":
            _, j, hh = mains[n - 2]
            if j > 0:
                attn_pp(j - 1, hh, t + P["PP"])
            if j == NB - 1:
                attn_pp(j, hh, t + P["PP"])

    NRG = 8 * (NQ + 1) + 7
    PD = 8 * QD
    BORD = (1, 3, 2, 4, 0, 5, 6)
    LORD = (2, 4, 1, 3, 0, 5, 6)
    LAST_PARTS = [(0, QD, 1, 2), (QD, HD, 0, 2), (0, QD, 0, 1)]

    def rr_prep(p, pa, src, n0, n1, t0, dur):
        assert ("rr", p) not in ready
        for n in range(n0, n1):
            z = at(t0 + (n - n0) * dur // (n1 - n0))
            qd, g = divmod(n, 8)

            def wrow(i):
                return _rhs_op(p, lambda x, y: w2_v[pa + y, (2 * i + x) * LB + g * 16:(2 * i + x) * LB + g * 16 + 16, :]
                               .astype(f32))

            def orow(h):
                def blk(x, y):
                    assert ("o", src, x, 2 * y + 1) in ready
                    r = x * HD + h * QD + g * 16
                    return ol[src][r:r + 16, y * 2 * LB:(y + 1) * 2 * LB]
                return _rhs_op(p, blk)
            ro = p * RRK + g * 8
            if qd == NQ:
                if p in SIDX:
                    r = wrow(2 * NQ)
                    for e in range(2):
                        rr_s[ro:ro + 8, _blk(7 + e)] = _pk(tie8(r[:, _blk(e)], z))
                continue
            r1, r2 = (wrow(2 * qd), wrow(2 * qd + 1)) if qd < NQ else (orow(0), orow(1))
            ro += min(qd, NQ) * (LB // 2)
            c11, c22 = tie8(r1[:, :LB], z), tie8(r2[:, LB:], z)
            sm = _rhs_sums(c11, r1[:, LB:], r2[:, :LB], c22)
            if p in SIDX or qd > NQ:
                sm.update({1: c11, 4: c22})
            for q, v in sm.items():
                rr_s[ro:ro + 8, _blk(q)] = _pk(v)
        if n1 == NRG:
            ready.add(("rr", p))

    def rr_tasks(p, pa, src, t0, t1):
        cuts = list(range(0, NRG, 8)) + [NRG]
        acc, tot = 0, sum(P["RW"])
        for a, b, w in zip(cuts[:-1], cuts[1:], P["RW"]):
            ta, tb = t0 + acc * (t1 - t0) // tot, t0 + (acc + w) * (t1 - t0) // tot
            add_tasks([(tb, rr_prep, (p, pa, src, a, b, ta, tb - ta))])
            acc += w

    def out_copy(pidx, e0, e1, r0, r1):
        off = pidx * (2 * LB) + e0 * LB
        if not isinstance(pidx, int):
            off = pl.multiple_of(off, LB)
        rs = pl.ds(r0, r1 - r0)
        return pltpu.make_async_copy(out_v.at[pidx, rs, pl.ds(e0 * LB, (e1 - e0) * LB)],
                                     out_hbm.at[0, rs, pl.ds(off, (e1 - e0) * LB)], sems.at[0])

    def b_out(pa, n, m, part, t0=None, dur=None):
        a, y = divmod(n, 2)
        r0, r1, e0, e1 = part
        cols = slice(e0 * LB, e1 * LB)
        for r in range(r0, r1, 16):
            c = _combine([None if v is None else v[r:r + 16, cols] for v in m], n)
            rows = slice(a * HD + r, a * HD + r + 16)
            o = c + x_v[pa + y, rows, cols].astype(f32)
            if t0 is not None:
                o = jnp.concatenate([tie(o[:, 0:LB], at(t0 + (r - r0) * dur // (r1 - r0))), o[:, LB:]], axis=1)
            out_v[pa + y, rows, cols] = o.astype(bf16)
        out_copy(pa + y, e0, e1, a * HD + r0, a * HD + r1).start()

    def big_piece(pa, pan, cur, last):
        t0 = now()
        for n in range(7):
            ta, tb = t0 + n * PD + P["RR0"], t0 + n * PD + P["RR1"]
            if n < 6:
                rr_tasks(BORD[n + 1], pa, cur, ta, tb)
            else:
                rr_tasks(BORD[0], pan, 1 - cur, ta, tb - (P["RRM"] if last else 0))
        ready.difference_update({("o", 1 - cur, hh, e) for hh in range(2) for e in range(4)})
        for n in range(8):
            e, hh = divmod(n, 2)
            t = t0 + P["BV0"] + n * P["BVS"]
            add_tasks([(t + P["BVD"], attn_pv, (pan * 2 + e, hh, 1 - cur, e, t, P["BVD"]))])
        m = [None] * 7
        for p in BORD:
            flush(now())
            assert ("rr", p) in ready
            x, y = TOP[p][0]

            def lhs(q):
                if q in (2, 3):
                    rows = slice(p * QD + (q - 2) * ED, p * QD + (q - 1) * ED)
                    return _up(jnp.concatenate([lc_s[rows, _blk(2 * qd + q - 2)] for qd in range(NQ)]
                                               + [lc_s[rows, (NFP + q - 2) * LB:(NFP + q - 2) * LB + QD]], axis=1))
                return _up(ll_s[(p * 7 + q) * ED:(p * 7 + q + 1) * ED, 0:KL])

            def rhs(q):
                if p in SIDX or q in SIDX:
                    return _up(rr_s[p * RRK:p * RRK + KL // 2, _blk(q)])
                h = 0 if q == 1 else 1
                return _cat([w2_v[pa + y, _blk(2 * (2 * qd + h) + x), _blk(h)] for qd in range(NQ)]
                            + [_up(rr_s[p * RRK + NQ * LB // 2:p * RRK + KL // 2, _blk(q)])], 0)
            rl = (_up(rr_s[p * RRK:p * RRK + LB // 2, 7 * LB:9 * LB]) if p in SIDX
                  else w2_v[pa + y, _blk(4 * NQ + x), :])
            ll = _up(lc_s[p * QD:(p + 1) * QD, _blk(2 * NQ)])
            ex = [mm1(ll[:QD], rl), mm1(ll[QD:], rl)]
            e12, e21 = ex[0][:, LB:], ex[1][:, :LB]
            e11 = (ex[0][:, :LB] + e12) - e21
            lf = strassen(lhs, rhs, LORD)
            ready.discard(("rr", p))
            if p in (2, 3):
                for q in (2, 3):
                    lf[q] = lf[q] + b2f_s[pa + 3 - p, 0:1, _blk(3 - q)]
            c12 = (lf[2] + e12) + lf[4]
            c21 = (lf[1] + e21) + lf[3]
            xx = (lf[2] - lf[1]) + lf[0]
            c22 = (xx + ex[1][:, LB:]) + lf[5]
            c11 = ((xx + e11) + (c21 - c12)) + lf[6]
            m[p] = jnp.concatenate([jnp.concatenate([c11, c12], axis=1),
                                    jnp.concatenate([c21, c22], axis=1)], axis=0)
            n = {3: 2, 4: 1, 5: 3, 6: 0}.get(p)
            if n is not None and not (last and n == 0):
                t, epd = now() + P["EP0"], P["EPL"] if (last and n == 3) else P["EPD"]
                add_tasks([(t + epd, b_out, (pa, n, list(m), (0, HD, 0, 2), t, epd))])
        if last:
            flush()
            for part in LAST_PARTS:
                b_out(pa, 0, m, part)

    def c_body(it, carry):
        reset()
        pos[:] = [one_s[...]]
        ready.update({("rr", BORD[0])} | {("o", 0, hh, e) for hh in range(2) for e in range(4)})
        big_piece(4 * it, 4 * it + 2, 0, False)
        big_piece(4 * it + 2, lax.rem(4 * it + 4, NP), 1, True)
        assert ("rr", BORD[0]) in ready and all(("o", 0, hh, 3) in ready for hh in range(2))
        return carry

    E1, E3 = P["E1"], P["E3"]
    x0 = Group(cp_x(0, 1))
    g1 = Group(cp_w1(0, 2, 0, E1))
    g2 = Group(cp_w1(0, 2, E1, NFP) + cp_x(1, 2))
    g3 = Group([(b1_hbm, b1_v)] + cp_w1(2, UB0, 0, E3))
    g4 = Group((cp_w1(2, UB0, E3, NFP) if E3 < NFP else []) + [(wqkv_hbm, wqkv_v)])
    g5 = Group(cp_x(2, NP))
    g6 = Group(cp_w1(UB0, NB) + [(wo_hbm, wo_v), (b2_hbm, b2_v)] + cp_w2(0, 1))
    g7 = Group(cp_w2(1, NP))
    for c in (x0, g1, g2, g3, g4, g5, g6, g7):
        c.start()

    v_s[0] = jnp.zeros((D, LB), f32)
    for buf in (xnT_s, ra_s, lh_s, rs_s, rr_s, ola_s, olb_s, ll_s, lc_s):
        buf[0:8, 0:64] = jnp.zeros((8, 64), buf.dtype)

    wait("x0", x0)
    one_s[...] = lax.shift_right_logical(pltpu.bitcast(x_v[0, 0:16, 0:LB], i32), 1) | 1
    pos[:] = [one_s[...]]
    ln(0)
    ln(1)
    hpair(0)
    wait("r1", g1)
    jobs = u_early(0, 0, E1, [], 7 * E1 // 4 * 4, 100)
    wait("r2", g2)
    ln_tasks(2, P["L2T"], P["L2D"], P["H2D"])
    jobs = u_early(0, E1, NFP, jobs, (len(jobs) + 7 * (NFP - E1)) // 4 * 4, 120)
    wait("r3", g3)
    jobs = u_early(1, 0, E3, jobs, P["N3"], 140)
    wait("wqkv", g4)
    n4 = len(jobs) + 7 * (NFP - E3)
    u_early(1, E3, NFP, jobs, n4, 100, nsplit=n4 % 4)
    prep_wqkv()
    stage_a(0, split_last=True)

    wait("mid", g5)
    AD = 7 * HA // 2
    t = 0
    for b in range(UB0, NB, 2):
        t = ln_tasks(b, t, P["LND"], P["HSD"])
    n5 = ((NP - 1) * AD - P["MARG"] - t) // P["BD"]
    add_tasks([(t + (n + 1) * P["BD"], slot, (t + n * P["BD"], P["BD"])) for n in range(n5)])
    for n, b in enumerate(range(2, NB, 2)):
        stage_a(b, odd=n % 2 == 1, split_last=b == NB - 2)

    wait("fin", g6)
    UD = 7 * NUP * HD // 4
    for i in range(NFP):
        t0, dt = (-200, 130) if i == 0 else (700, 260) if i == 1 else ((i - 1) * UD + P["US0"], P["USD"])
        add_tasks([(t0 + (k + 1) * dt, tsum, (UB0 // 2 + k, i, i % 3, k, t0 + k * dt, dt)) for k in range(NUP)])
    left = len(mains) - n5 - 2
    bd = (NFP * UD - P["R6E"] - P["R6S"]) // left
    add_tasks([(P["R6S"] + (n + 1) * bd, slot, (P["R6S"] + n * bd, bd)) for n in range(left)])
    t = P["R6S"] + left * bd
    add_tasks([(t + (n + 1) * 300, slot, (t + n * 300, 300)) for n in range(2)])
    for qd, t0, t1 in ((NQ, UD + P["LL0"], 3 * UD), (0, 3 * UD + P["LL0"], 5 * UD), (1, 5 * UD + P["LL0"], 6 * UD + 200),
                       (2, 6 * UD + P["LL2"], 6 * UD + P["LL2"] + P["UEL"])):
        dt = (t1 - t0) // 7
        add_tasks([(t0 + (g + 1) * dt, llsum, (qd, g, t0 + g * dt, dt)) for g in range(7)])
    rr_tasks(BORD[0], 0, 0, P["RP0"], P["RP1"])
    add_tasks([(P["PW0"] + P["PWD"], prep_wo_a, (P["PW0"], P["PWD"]))])
    add_tasks([(P["PW1"] + (h + 1) * P["PWE"], prep_wo_b, (h, P["PW1"] + h * P["PWE"], P["PWE"])) for h in range(2)])
    for b in range(NB):
        b2f_s[b // 2, 0:1, _blk(b % 2)] = b2_v[b:b + 1, :].astype(f32)
    for i in range(NFP):
        u_last(i, (1, 4, 2, 3, 0, 5, 6) if i == 0 else (4, 2, 1, 3, 0, 5, 6),
               None if i == NFP - 1 else P["UEL"] if i == NFP - 2 else P["UED"])
    flush()
    assert slot_ctr[0] == len(mains) and all(("ll", qd, g) in ready for qd in range(NQ + 1) for g in range(7))
    assert all(("pr", j, hh) in ready for j in range(NB) for hh in range(2)) and ("rr", BORD[0]) in ready

    wait("w2", g7)
    lax.fori_loop(0, NP // 4, c_body, 0)
    outs = []
    for pa in range(0, NP, 2):
        outs += [out_copy(pa + n % 2, 0, 2, n // 2 * HD, (n // 2 + 1) * HD) for n in (1, 2, 3)]
        outs += [out_copy(pa, e0, e1, r0, r1) for (r0, r1, e0, e1) in (LAST_PARTS if pa % 4 else [(0, HD, 0, 2)])]
    wait("out", *outs)


@jax.jit
def pallas_parallel_sum__sliding_local_dilated__mixer_token_mlp__prompt_kernel(A_x, A_wqkv, A_wo, B_x, B_w1, B_b1, B_w2, B_b2):
    del B_x
    hbm = pl.BlockSpec(memory_space=pltpu.HBM)
    outT = pl.pallas_call(
        _kernel,
        out_shape=jax.ShapeDtypeStruct((1, D, S), bf16),
        in_specs=[hbm] * 7,
        out_specs=hbm,
        scratch_shapes=[
            pltpu.VMEM((NP, D, 2 * LB), bf16),
            pltpu.VMEM((D, 3 * D), bf16),
            pltpu.VMEM((D, D), bf16),
            pltpu.VMEM((S, F), bf16),
            pltpu.VMEM((NP, F, 2 * LB), bf16),
            pltpu.VMEM((NFB, LB), bf16),
            pltpu.VMEM((NB, LB), bf16),
            pltpu.VMEM((NP, D, 2 * LB), bf16),
            pltpu.VMEM((2, 3 * D + 64, LB), i32),
            pltpu.VMEM((7 * HA // 2, HD), u32),
            pltpu.VMEM((4, HD + 32, LB), i32),
            pltpu.VMEM((D, 2 * LB), i32),
            pltpu.VMEM((HD, S), u32),
            pltpu.VMEM((NP * QD, 5 * LB), u32),
            pltpu.VMEM((7 * QD, NP * LB), u32),
            pltpu.VMEM((7 * HD, NFP * LB), f32),
            pltpu.VMEM((7 * QD, (NFP + 2) * LB), u32),
            pltpu.VMEM((NB, 2 * D, LB), f32),
            pltpu.VMEM((NB + 1, D, LB), f32),
            pltpu.VMEM((NB, 2 * W * HH, LB), f32),
            pltpu.VMEM((D, LB), f32),
            pltpu.VMEM((NP, 32, 2 * LB), f32),
            pltpu.VMEM((5 * RSK, 5 * LB), u32),
            pltpu.VMEM((49 * ED, 4 * LB), u32),
            pltpu.VMEM((7 * RRK, 9 * LB), u32),
            pltpu.VMEM((D, 4 * LB), f32),
            pltpu.VMEM((D, 4 * LB), f32),
            pltpu.VMEM((8, LB), i32),
            pltpu.SemaphoreType.DMA((9,)),
        ],
        compiler_params=pltpu.CompilerParams(vmem_limit_bytes=100 * 1024 * 1024,
                                             disable_bounds_checks=True,
                                             disable_semaphore_checks=True),
    )(jnp.swapaxes(A_x, 1, 2), A_wqkv, A_wo, B_w1, B_b1.reshape(NFB, LB), B_w2, B_b2.reshape(NB, LB))
    return jnp.swapaxes(outT, 1, 2)
```

```python
import jax
import jax.numpy as jnp
from jax import lax
import jax.experimental.pallas as pl
import jax.experimental.pallas.tpu as pltpu

S, D, F = 2048, 448, 1792
H, DH, W, DIL = 16, 28, 8, 2
LB = 128
NB = S // LB
NP = NB // 2
NFB = F // LB
NFP = NFB // 2
HH = H // 2
WH = W // 2
SH = DIL * WH
HD = D // 2
QD = D // 4
ED = D // 8
HA = 3 * HD
UB0 = 2
NUP = (NB - UB0) // 2
RSK = NFP * LB // 2
NQ = NFP // 2
KL = NQ * LB + QD
RRK = 2 * LB
EPS = 1e-5
SCALE = DH ** -0.5
f32 = jnp.float32
bf16 = jnp.bfloat16
u32 = jnp.uint32
i32 = jnp.int32

SCOPES = False
P = dict(
    E1=3, N2=16, NA3=2, T1=-200, T2=-200, S3=0, L2T=230, L2D=380, H2T=900, H2D=420, L4T=1000, L5T=0, W2X=300,
    WQ=(-450, 200, -200, 300), WKV=(50, 380, 450, 420),
    LND=400, HSD=360, HL=300, LNA=0.3, LNB=0.42, LNBD=0.33, LNV=0.8, LNW=0.86,
    BD=370, MARG=300, LAG=200, LS=170, PP=150, PVL=500, PVPOS=12,
    US0=100, USD=360, UE0=200, UED=2500, UEL=1700, UG=50, UM=24, R6S=1900, R6E=2700,
    LL0=300, LL2=500, RP0=16600, RP1=18700, PW0=500, PWD=300, PW1=1300, PWE=400,
    RR0=-48, RR1=800, RRM=-20, RW=(8, 8, 8, 2, 7), BV0=117, BVS=717, BVD=620, EP0=0, EPD=864, EPL=290, SGR=8, SGT=8, SH4=1,
)
G = 4


def _as(x, dtype):
    return x if x.dtype == dtype else pltpu.bitcast(x, dtype)


def _pk(x):
    return pltpu.bitcast(x.astype(bf16), u32)


def _up(x):
    return pltpu.bitcast(x, bf16)


def _upf(x):
    return pltpu.bitcast(x, bf16).astype(f32)


def _word(lo, hi):
    lo, hi = [pltpu.bitcast(v.astype(f32), i32) for v in (lo, hi)]
    return lax.shift_right_logical(lo, 16) | hi


def _unword(w):
    return [pltpu.bitcast(w << 16, f32), pltpu.bitcast(w & -65536, f32)]


def _cat(xs, axis):
    return xs[0] if len(xs) == 1 else jnp.concatenate(xs, axis=axis)


def _x2(v):
    return jnp.concatenate([v, v], axis=0)


def _blk(b):
    return slice(b * LB, (b + 1) * LB)


def _rowsum8(a):
    return jnp.broadcast_to(jnp.sum(a, axis=0, keepdims=True), (8, a.shape[1]))


def _token(*deps):
    deps = [d for d in deps if d is not None]
    if not deps:
        return None
    if len(deps) == 1:
        return deps[0]
    bits = _as(deps[0], u32)
    for d in deps[1:]:
        bits = bits | _as(d, u32)
    return bits


def _lhs_ops(a11, a12, a21, a22):
    return [a11 + a22, a21 + a22, a11, a22, a11 + a12, a21 - a11, a12 - a22]


SIDX = {0: 0, 2: 1, 3: 2, 5: 3, 6: 4}
TOP = {0: ((0, 0), 1, (1, 1)), 1: ((0, 0),), 2: ((0, 1), -1, (1, 1)), 3: ((1, 0), -1, (0, 0)),
       4: ((1, 1),), 5: ((0, 0), 1, (0, 1)), 6: ((1, 0), 1, (1, 1))}


def _rhs_sums(b11, b12, b21, b22):
    return {0: b11 + b22, 2: b12 - b22, 3: b21 - b11, 5: b11 + b12, 6: b21 + b22}


def _rhs_op(p, blk):
    t = TOP[p]
    if len(t) == 1:
        return blk(*t[0])
    return blk(*t[0]) + blk(*t[2]) if t[1] > 0 else blk(*t[0]) - blk(*t[2])


def _combine(m, n=None):
    c12 = lambda: m[2] + m[4]
    c21 = lambda: m[1] + m[3]
    x = lambda: (m[2] - m[1]) + m[0]
    c = [lambda: (x() + m[6]) + (c21() - c12()), c12, c21, lambda: x() + m[5]]
    return [f() for f in c] if n is None else c[n]()


def _kernel(x_hbm, wqkv_hbm, wo_hbm, w1_hbm, b1_hbm, w2_hbm, b2_hbm, out_hbm,
            x_v, wqkv_v, wo_v, w1_v, w2_v, b1_v, b2_v, out_v,
            wt_s, lw_s, wo_s, wq_s, xnT_s, ra_s, lh_s, um_s, lc_s, qk_s, v_s, pr_s, op_s,
            b2f_s, rs_s, ll_s, rr_s, ola_s, olb_s, one_s, sems):
    sem_ctr = [1]

    class Group:
        def __init__(self, pairs):
            self.cps = [pltpu.make_async_copy(a, b, sems.at[sem_ctr[0]]) for (a, b) in pairs]
            sem_ctr[0] += 1

        def start(self):
            for c in self.cps:
                c.start()

        def wait(self):
            for c in self.cps:
                c.wait()

    def cp_x(p0, p1):
        return [(x_hbm.at[0, :, pl.ds(p * 2 * LB, 2 * LB)], x_v.at[p]) for p in range(p0, p1)]

    def cp_w2(p0, p1):
        return [(w2_hbm.at[:, pl.ds(p * 2 * LB, 2 * LB)], w2_v.at[p]) for p in range(p0, p1)]

    def cp_w1(b0, b1, i0=0, i1=NFP):
        sl = pl.ds(b0 * LB, (b1 - b0) * LB)
        cl = pl.ds(i0 * 2 * LB, (i1 - i0) * 2 * LB)
        return [(w1_hbm.at[sl, cl], w1_v.at[sl, cl])]

    tl = []
    mxu = [0, 0, 0, 0]
    nxt = [0]
    hist = []
    tasks = []
    dls = []
    ready = set()
    pos = []
    true = {}

    def tie(v, z):
        if z is None:
            return v
        def fit(a):
            a = _cat([a] * (v.shape[0] // 8), 0)
            return a if v.shape[1] == LB else a[:, 0:v.shape[1]]
        if v.shape not in true:
            true[v.shape] = fit(pos[0]) > 0
        return lax.select(true[v.shape], v, fit(_as(z, v.dtype)))

    def tie8(v, z):
        return v if z is None else jnp.concatenate([tie(v[0:8], z), v[8:16]], axis=0)

    def add_tasks(todo):
        tasks.extend(todo)
        tasks.sort(key=lambda x: x[0])

    def flush(t=None):
        while tasks and (t is None or tasks[0][0] < t):
            _, fn, args = tasks.pop(0)
            fn(*args)

    def reset():
        assert not tasks
        dls.clear()
        tl.clear()
        hist.clear()
        mxu[:] = [0, 0, 0, 0]
        nxt[0] = 0

    def now():
        return sum(mxu) // 4

    def wait(name, *cps):
        flush()
        if SCOPES:
            with jax.named_scope("wait_" + name):
                for c in cps:
                    c.wait()
        else:
            for c in cps:
                c.wait()
        reset()

    def mm1(lhs, rhs, pace=True):
        flush(now())
        start = mxu[nxt[0]]
        due = [v for (t, v) in dls if t <= start] if pace else []
        if due:
            dls[:] = [(t, v) for (t, v) in dls if t > start]
            tile = _up(tie(pltpu.bitcast(lhs[0:16, 0:LB], u32), _token(*due)))
            row = tile if lhs.shape[1] == LB else jnp.concatenate([tile, lhs[0:16, LB:]], axis=1)
            lhs = jnp.concatenate([row, lhs[16:]], axis=0)
        r = jnp.dot(lhs, rhs, preferred_element_type=f32)
        m, k = lhs.shape
        first_done = None
        for _ in range(-(-rhs.shape[1] // LB)):
            end = 0
            for _ in range(-(-k // LB)):
                mxu[nxt[0]] += m
                end = max(end, mxu[nxt[0]])
                nxt[0] = (nxt[0] + 1) % 4
            if first_done is None:
                first_done = end
        if pace:
            tl.append((first_done - m, first_done, r))
        return r

    def mm(lhs, rhs, init=None):
        k = lhs.shape[1]
        r, k0 = init, 0
        while k0 < k:
            k1 = min(k, k0 + (4 - nxt[0]) * LB)
            part = mm1(lhs[:, k0:k1], rhs[k0:k1], pace=k1 - k0 > LB)
            r = part if r is None else r + part
            k0 = k1
        return r

    def at(t, *more):
        best = None
        if t is not None and t >= 0:
            t = min(t, now() - 1)
            for (a, b, r) in tl:
                if a <= t and (best is None or min(b, t) > best[0]):
                    row = int(min((t - a) / (b - a), 0.999) * (r.shape[0] // 8)) * 8
                    best = (min(b, t), r, row)
        return _token(None if best is None else best[1][best[2]:best[2] + 8, 0:LB], *more)

    def strassen(lhs, rhs, order, split_last=False, init=None, m=None):
        m = [None] * 7 if m is None else m
        for p in order:
            flush(now())
            l, r = lhs(p), rhs(p)
            c0 = None if init is None else init[p]
            if split_last and p == order[-1]:
                kk = (-(-r.shape[0] // LB) - 2) * LB
                hm = l.shape[0] // 2
                hd = mm(l[:, :kk], r[:kk], c0) if kk else c0
                tail = jnp.concatenate([mm(l[:hm, kk:], r[kk:]), mm(l[hm:, kk:], r[kk:])], axis=0)
                m[p] = tail if hd is None else hd + tail
            else:
                m[p] = mm(l, r, c0)
        return m

    def wrows(hh, g, z=None):
        p, d = divmod(2 * g, DH)
        t = [jnp.concatenate([wt_s[c, pl.ds(p * D + hh * HD + d + e, HH, stride=DH), :]
                              for e in range(2)], axis=0) for c in range(2)]
        return _unword(jnp.concatenate([tie(t[0], z), tie(t[1][:, 0:HD - LB], z)], axis=1))

    wt_done = set()

    def prep_wqkv(part, ga, gb, paced):
        def need(hh, p, z):
            lo = p * D + hh * HD
            for ct in range(lo // LB, -(-(lo + HD) // LB)):
                if ct in wt_done:
                    continue
                wt_done.add(ct)
                cols = slice(ct * LB, min((ct + 1) * LB, 3 * D))
                wd = _word(wqkv_v[0:HD, cols], wqkv_v[HD:D, cols])
                wd = jnp.concatenate([tie(wd[r:r + 8], z if r % LB == 0 else None) for r in range(0, HD, 8)], axis=0)
                wT = wd.T
                wt_s[0, cols, :] = wT[:, 0:LB]
                wt_s[1, cols, 0:HD - LB] = wT[:, LB:HD]

        def put(p, g, v):
            lw_s[p * (HA // 2) + g * 8:p * (HA // 2) + g * 8 + 8, :] = _pk(v)

        def half(hh, g0, g1, t0=None, dur=None):
            pr, ps = ((2, 4), (3, 1))[hh]
            for g in range(g0, g1):
                t = None if t0 is None else t0 + (g - g0) * dur // (g1 - g0)
                need(hh, 2 * g // DH, at(None if t is None else t - P["W2X"]))
                a1, a2 = wrows(hh, g, at(t))
                put(pr, g, a2 if hh else a1)
                put(ps, g, a1 + a2)
            if g1 == gb:
                ready.update({("lw", part, pr), ("lw", part, ps)})

        def rest(g0, g1, t0, dur):
            assert ("lw", part, 1) in ready
            for g in range(g0, g1):
                z = at(t0 + (g - g0) * dur // (g1 - g0))
                ops = _lhs_ops(*wrows(0, g, z), *wrows(1, g, z))
                for p in (0, 5, 6):
                    put(p, g, ops[p])
            if g1 == gb:
                ready.update({("lw", part, 0), ("lw", part, 5), ("lw", part, 6)})
        t2, d2, t3, d3 = paced
        half(0, ga, gb)
        n = (gb - ga) // 14
        add_tasks([(now() + t2 + (k + 1) * d2 // n, half,
                    (1, ga + 14 * k, ga + 14 * k + 14, now() + t2 + k * d2 // n, d2 // n)) for k in range(n)])
        n = (gb - ga) // 7
        add_tasks([(now() + t3 + (k + 1) * d3 // n, rest,
                    (ga + 7 * k, ga + 7 * k + 7, now() + t3 + k * d3 // n, d3 // n)) for k in range(n)])

    def prep_wo_a(t0, dur):
        for g in range(HD // 16):
            w = _word(wo_v[g * 16:g * 16 + 16, :], wo_v[HD + g * 16:HD + g * 16 + 16, :])
            z = at(t0 + g * dur // (HD // 16))
            for c in range(4):
                cw = min(LB, D - c * LB)
                wo_s[c, g * 16:g * 16 + 16, 0:cw] = tie(w[:, c * LB:c * LB + cw], z)
        ready.add("wo")

    def prep_wo_b(h, t0, dur):
        assert "wo" in ready
        for c in range(4):
            cw = min(LB, D - c * LB)
            rows = [wo_s[c, pl.ds(d, HH, stride=DH), :][:, 0:cw] for d in range(h * DH // 2, (h + 1) * DH // 2)]
            rows.append(jnp.zeros((LB - QD, cw), i32))
            wq_s[c * LB:c * LB + cw, _blk(h)] = jnp.concatenate(rows, axis=0).T
        outs = []
        for g in range(HD // 16):
            z = at(t0 + g * dur // (HD // 16))
            a = [v for r in (g * 16, HD + g * 16) for v in _unword(tie(wq_s[r:r + 16, _blk(h)], z))]
            for p, v in enumerate(_lhs_ops(*a)):
                lc_s[p * QD + g * 8:p * QD + g * 8 + 8, _blk(NFP + h)] = _pk(v)
                outs.append(v[0:8])
        ready.update({("lc", NFP + h, g) for g in range(HD // 16)})
        dls.append((t0 + dur + 250, _token(*outs)))

    RG = 16
    NG = D // RG
    stat2 = {}

    def ln(b, t0=None, dur=None):
        def xg(g):
            return x_v[b // 2, g * RG:(g + 1) * RG, _blk(b % 2)].astype(f32)

        def step(v, g, fr, s, q):
            if t0 is None or g % 4:
                return v
            acc = [] if s is None else [s[0:8], s[8:16], q[0:8], q[8:16]]
            return tie(v, at(t0 + fr * dur, *acc))

        x0 = jnp.broadcast_to(xg(0)[0:1], (8, LB))
        s = q = None
        for g in range(NG):
            x0 = step(x0, g, P["LNA"] * g / NG, s, q)
            c = xg(g) - _x2(x0)
            s = c if s is None else s + c
            q = c * c if q is None else q + c * c
        dm = _rowsum8(s) * (1.0 / D)
        mu = x0 + dm
        r1 = lax.rsqrt(jnp.maximum(_rowsum8(q) * (1.0 / D) - dm * dm, 0.0) + EPS)
        s = q = None
        for g in range(NG):
            mu = step(mu, g, P["LNB"] + P["LNBD"] * g / NG, s, q)
            xn = (xg(g) - _x2(mu)) * _x2(r1)
            xnT_s[g * 8:g * 8 + 8, _blk(b)] = _pk(xn)
            s = xn if s is None else s + xn
            q = xn * xn if q is None else q + xn * xn
        mu2 = _rowsum8(s) * (1.0 / D)
        var2 = jnp.maximum(_rowsum8(q) * (1.0 / D) - mu2 * mu2, 0.0)
        stat2[b] = (mu2, 0.5 * lax.rsqrt(var2 + EPS))

    def hpair(b, t0=None, dur=None):
        ng = HD // RG
        st = [stat2.pop(b), stat2.pop(b + 1)]
        for g in range(ng):
            zz = [at(None if t0 is None else t0 + (4 * g + k * P["SH4"]) * dur // (4 * ng)) for k in (0, 1, 2, 3)]
            xq = [_upf(tie(xnT_s[r:r + 8, _blk(b + e)], zz[2 * (r >= QD) + e]))
                  for r in (g * 8, QD + g * 8) for e in range(2)]
            hq = [(v - _x2(st[n % 2][0])) * _x2(st[n % 2][1]) for n, v in enumerate(xq)]
            ro = (b // 2) * QD + g * 8
            for p, v in _rhs_sums(*xq).items():
                ra_s[ro:ro + 8, _blk(SIDX[p])] = _pk(v)
            for p, v in enumerate(_lhs_ops(*hq)):
                lh_s[p * QD + g * 8:p * QD + g * 8 + 8, _blk(b // 2)] = _pk(v)
        ready.add(("xn", b))
        if b >= 6:
            got = ra_s[(b // 2) * QD:(b // 2 + 1) * QD, :]
            dls.append((t0 + dur + P["HL"], _token(*[got[r:r + 8, _blk(c)] for r in range(0, QD, 8) for c in range(5)])))

    def ln_tasks(b, t, lnd, hsd):
        for fn, bb, dur, adv in ((ln, b, lnd, P["LNV"]), (ln, b + 1, lnd, P["LNW"]), (hpair, b, hsd, 1.0)):
            add_tasks([(t + int(dur * adv), fn, (bb, t, dur))])
            t += int(dur * adv)
        return t

    def tsum(kp, i, slot_, n, t0, dur):
        for g in range(LB // 16):
            z, z2 = at(t0 + g * dur // 8), at(t0 + g * dur // 8 + P["SGT"])
            t1, t2 = [w1_v[(2 * kp + e) * LB + g * 16:(2 * kp + e) * LB + g * 16 + 16,
                           2 * i * LB:(2 * i + 2) * LB].astype(f32) for e in range(2)]
            ro = slot_ * RSK + n * (LB // 2) + g * 8
            for p, v in _rhs_sums(tie8(t1[:, :LB], z), t1[:, LB:], t2[:, :LB], tie8(t2[:, LB:], z2)).items():
                rs_s[ro:ro + 8, _blk(SIDX[p])] = _pk(v)
        ready.add(("rs", kp, i))

    def u_rhs(p, i, kps, slot_, n0):
        if p in SIDX:
            assert all(("rs", kp, i) in ready for kp in kps)
            ro = slot_ * RSK + n0 * (LB // 2)
            return _up(rs_s[ro:ro + len(kps) * (LB // 2), _blk(SIDX[p])])
        e = 0 if p == 1 else 1
        return _cat([w1_v[_blk(2 * kp + e), _blk(2 * i + e)] for kp in kps], 0)

    LATE = (NFP - 1, 6)

    def ujob(kp, i, p, split):
        flush(now())
        assert ("xn", 2 * kp) in ready
        l, r = _up(lh_s[p * QD:(p + 1) * QD, _blk(kp)]), u_rhs(p, i, [kp], 3 + kp, i)
        v = jnp.concatenate([mm1(l[:QD], r), mm1(l[QD:], r)], axis=0) if split else mm1(l, r)
        if p in (2, 3):
            v = v + 0.5 * b1_v[2 * i + 3 - p:2 * i + 4 - p, :].astype(f32)
        rows = slice(p * HD, (p + 1) * HD)
        um_s[rows, _blk(i)] = v

    def u_early(kp, i0, i1, carry, n, t0, dt, nsplit=0):
        for k, i in enumerate(range(i0, i1)):
            add_tasks([(t0 + (k + 1) * dt, tsum, (kp, i, 3 + kp, i, t0 + k * dt, dt))])
        jobs = (carry + [(kp, i, p) for i in range(i0, i1) for p in (1, 4)]
                + [(kp, i, p) for i in range(i0, i1) for p in SIDX if (i, p) != LATE])
        for c, job in enumerate(jobs[:n]):
            ujob(*job, c >= n - nsplit)
        return jobs[n:]

    def gelu_half(hx, z):
        c = 0.7978845608028654
        return hx + hx * jnp.tanh(tie(hx * (2.0 * c + (8.0 * c * 0.044715) * (hx * hx)), z))

    def u_epilogue(i, m, gs, t0, dur):
        for n, g in enumerate(gs):
            t = None if t0 is None else t0 + n * dur // len(gs) - P["UG"]
            q = _combine([x[g * 16:g * 16 + 16] for x in m])
            gl = [gelu_half(v, at(None if t is None else t - k * P["UM"])) for v, k in zip(q, (0, 3, 2, 1))]
            for p, v in enumerate(_lhs_ops(*gl)):
                lc_s[p * QD + g * 8:p * QD + g * 8 + 8, _blk(i)] = _pk(v)
            ready.add(("lc", i, g))

    def u_last(i, order, edur):
        kps = list(range(UB0 // 2, NP))
        m = strassen(lambda p: _up(lh_s[p * QD:(p + 1) * QD, (0 if (i, p) == LATE else UB0 // 2 * LB):]),
                     lambda p: _cat([u_rhs(p, i, [0], 3, i)] * ((i, p) == LATE) + [u_rhs(p, i, kps, i % 3, 0)], 0),
                     order, init=[None if (i, p) == LATE else um_s[p * HD:(p + 1) * HD, _blk(i)] for p in range(7)])
        if edur is None:
            u_epilogue(i, m, list(range(HD // 16)), None, None)
        else:
            t = now() + P["UE0"]
            add_tasks([(t + (g + 1) * edur // 7, u_epilogue, (i, m, [g, g + 7], t + g * edur // 7, edur // 7))
                       for g in range(7)])

    def llsum(qd, g, t0, dur):
        i0 = 2 * qd if qd < NQ else NFP
        assert all(("lc", i0 + e, g + 7 * h) in ready for e in range(2) for h in range(2))
        for p in range(7):
            zz = [at(t0 + p * dur // 7), at(t0 + p * dur // 7 + P["SGT"])]
            a = [tie(lc_s[p * QD + h * ED + g * 8:p * QD + h * ED + g * 8 + 8, _blk(i0 + e)], zz[h] if h == e else None)
                 for h in range(2) for e in range(2)]
            ops = _lhs_ops(*[_upf(v) for v in a])
            for q in (0, 1, 4, 5, 6):
                r = (p * 7 + q) * ED + g * 8
                ll_s[r:r + 8, _blk(qd)] = _pk(ops[q])
        ready.add(("ll", qd, g))

    AORD = (4, 2, 1, 3, 0, 5, 6)

    def stage_a(b, parts="qkv", order=AORD, split_last=False, m=None):
        r0, r1 = {"q": (0, HD), "kv": (HD, HA), "qkv": (0, HA)}[parts]

        def lhs(p):
            assert all(("lw", pt, p) in ready for pt in ("q", "kv") if pt in parts)
            return _up(lw_s[(p * HA + r0) // 2:(p * HA + r1) // 2, :])

        def rhs(p):
            assert ("xn", b) in ready
            if p in SIDX:
                return _up(ra_s[(b // 2) * QD:(b // 2 + 1) * QD, _blk(SIDX[p])])
            return _up(xnT_s[0:QD, _blk(b)] if p == 1 else xnT_s[QD:HD, _blk(b + 1)])
        m = strassen(lhs, rhs, order, split_last, m=m)
        for n, ps in enumerate((range(7), (2, 4), (1, 3), (0, 1, 2, 5))):
            if all(m[p] is not None for p in ps) and any(p in order for p in ps):
                hh, e = divmod(n, 2)
                c = _combine(m, n)
                qk_s[b + e, hh * D + r0:hh * D + min(r1, D), :] = c[0:min(r1, D) - r0]
                if r1 > D:
                    v_s[b + e + 1, hh * HD:(hh + 1) * HD, :] = c[D - r0:]
        if all(v is not None for v in m):
            ready.update({(pt, b + e) for pt in ("q", "kv") if pt in parts for e in range(2)})
        return m

    lane0 = lax.broadcasted_iota(i32, (HH, LB), 1)
    zeros8 = jnp.zeros((HH, LB), f32)

    def mk_shift(z):
        lane = tie(lane0, z)
        masks = {}

        def pick(n, a, b):
            if n not in masks:
                masks[n] = lane < n
            return lax.select(masks[n], a, b)

        def fwd(cur, prev, sh):
            return cur if sh == 0 else pltpu.roll(pick(LB - sh, cur, prev), sh, 1)

        def bwd(cur, nxt_):
            return pltpu.roll(pick(SH, nxt_, cur), LB - SH, 1)
        return fwd, bwd

    def grp_shift(t, bd):
        lag = max(2, -(-P["LAG"] * DH // (G * bd)))
        return mk_shift(at(t, *(hist[-lag] if len(hist) >= lag else [])))

    raw, probs = {}, {}

    def attn_qk(j, hh, t, bd):
        jn = min(j + 1, NB - 1)
        assert ("q", jn) in ready and ("kv", j) in ready
        acc = [None] * WH
        accp = [None] * WH
        for d in range(DH):
            if d % G == 0:
                if d > 0:
                    hist.append(acc + accp)
                fwd, bwd = grp_shift(t + d * bd // DH, bd)
            r = hh * D + d * HH
            q = qk_s[j, r:r + HH, :]
            qp = bwd(q, qk_s[jn, r:r + HH, :])
            k = qk_s[j, HD + r:HD + r + HH, :]
            kp = qk_s[j - 1, HD + r:HD + r + HH, :] if j > 0 else zeros8
            for a in range(WH):
                ks = fwd(k, kp, DIL * a)
                t0, t1 = q * ks, qp * ks
                acc[a] = t0 if d == 0 else acc[a] + t0
                accp[a] = t1 if d == 0 else accp[a] + t1
        hist.append(acc + accp)
        raw[j, hh] = (acc, accp)

    def attn_sm(j, hh, t):
        fwd, _ = mk_shift(at(t))
        acc, accp = raw[j, hh]
        prev = raw.pop((j - 1, hh))[1] if j > 0 else [zeros8] * WH
        lg = acc + [fwd(accp[a], prev[a], SH) for a in range(WH)]
        lg = [a * SCALE for a in lg]
        if j == 0:
            lg = [lg[0]] + [jnp.where(lane0 >= DIL * w, lg[w], -1e9) for w in range(1, W)]
        m = lg[0]
        for w in range(1, W):
            m = jnp.maximum(m, lg[w])
        e = [jnp.exp(l - m) for l in lg]
        den = e[0]
        for w in range(1, W):
            den = den + e[w]
        inv = 1.0 / den
        p = [x * inv for x in e]
        for a in range(WH):
            pr_s[j, (hh * W + a) * HH:(hh * W + a + 1) * HH, :] = p[a]
        probs[j, hh] = p[WH:]

    def attn_pp(j, hh, t):
        _, bwd = mk_shift(at(t))
        p = probs.pop((j, hh))
        pn = probs[j + 1, hh] if j + 1 < NB else p
        for a in range(WH):
            pr_s[j, (hh * W + WH + a) * HH:(hh * W + WH + a + 1) * HH, :] = bwd(p[a], pn[a])
        ready.add(("pr", j, hh))

    def attn_pv(j, hh, dst, e, t, bd):
        assert not isinstance(j, int) or ("pr", j, hh) in ready
        assert e == 0 or ("o", dst, hh, e - 1) in ready
        pa = [pr_s[j, (hh * W + a) * HH:(hh * W + a + 1) * HH, :] for a in range(W)]
        p, pp = pa[:WH], pa[WH:]
        outs = []
        for d in range(DH):
            if d % G == 0:
                if d > 0:
                    hist.append([])
                fwd, _ = grp_shift(t + d * bd // DH, bd)
            r = hh * HD + d * HH
            v = v_s[j + 1, r:r + HH, :]
            vp = v_s[j, r:r + HH, :]
            o = op = None
            for a in range(WH):
                vs = fwd(v, vp, DIL * a)
                o = p[a] * vs if a == 0 else o + p[a] * vs
                op = pp[a] * vs if a == 0 else op + pp[a] * vs
            opp = zeros8 if (isinstance(j, int) and j == 0) else op_s[r:r + HH, :]
            op_s[r:r + HH, :] = op
            outs.append(o + fwd(op, opp, SH))
            ol[dst][r:r + HH, _blk(e)] = outs[-1]
        hist.append([])
        ready.add(("o", dst, hh, e))
        dls.append((t + bd + P["PVL"], _token(*outs)))

    ol = [ola_s, olb_s]
    mains = [("qk", j, hh) for j in range(NB) for hh in range(2)]
    mains = (mains[:P["PVPOS"]] + [("pv", j, hh) for j in range(4) for hh in range(2)]
             + mains[P["PVPOS"]:] + [None, None])
    slot_ctr = [0]

    def slot(t, bd):
        n = slot_ctr[0]
        slot_ctr[0] += 1
        it = mains[n]
        if it is None:
            pass
        elif it[0] == "qk":
            attn_qk(it[1], it[2], t, bd)
        else:
            attn_pv(it[1], it[2], 0, it[1], t, bd)
        if n >= 1 and mains[n - 1] is not None and mains[n - 1][0] == "qk":
            attn_sm(mains[n - 1][1], mains[n - 1][2], t + P["LS"])
        if n >= 2 and mains[n - 2] is not None and mains[n - 2][0] == "qk":
            _, j, hh = mains[n - 2]
            if j > 0:
                attn_pp(j - 1, hh, t + P["PP"])
            if j == NB - 1:
                attn_pp(j, hh, t + P["PP"])

    NRG = 8 * (NQ + 1) + 7
    PD = 8 * QD
    BORD = (1, 3, 2, 4, 0, 5, 6)
    LORD = (2, 4, 1, 3, 0, 5, 6)
    LAST_PARTS = [(0, QD, 1, 2), (QD, HD, 0, 2), (0, QD, 0, 1)]

    def rr_prep(p, pa, src, n0, n1, t0, dur):
        assert ("rr", p) not in ready
        for n in range(n0, n1):
            z = at(t0 + (n - n0) * dur // (n1 - n0))
            z2 = at(t0 + (n - n0) * dur // (n1 - n0) + P["SGR"])
            qd, g = divmod(n, 8)

            def wrow(i):
                return _rhs_op(p, lambda x, y: w2_v[pa + y, (2 * i + x) * LB + g * 16:(2 * i + x) * LB + g * 16 + 16, :]
                               .astype(f32))

            def orow(h):
                def blk(x, y):
                    assert ("o", src, x, 2 * y + 1) in ready
                    r = x * HD + h * QD + g * 16
                    return ol[src][r:r + 16, y * 2 * LB:(y + 1) * 2 * LB]
                return _rhs_op(p, blk)
            ro = p * RRK + g * 8
            if qd == NQ:
                if p in SIDX:
                    r = wrow(2 * NQ)
                    for e in range(2):
                        rr_s[ro:ro + 8, _blk(7 + e)] = _pk(tie8(r[:, _blk(e)], z))
                continue
            r1, r2 = (wrow(2 * qd), wrow(2 * qd + 1)) if qd < NQ else (orow(0), orow(1))
            ro += min(qd, NQ) * (LB // 2)
            c11, c22 = tie8(r1[:, :LB], z), tie8(r2[:, LB:], z2)
            sm = _rhs_sums(c11, r1[:, LB:], r2[:, :LB], c22)
            if p in SIDX or qd > NQ:
                sm.update({1: c11, 4: c22})
            for q, v in sm.items():
                rr_s[ro:ro + 8, _blk(q)] = _pk(v)
        if n1 == NRG:
            ready.add(("rr", p))

    def rr_tasks(p, pa, src, t0, t1):
        cuts = list(range(0, NRG, 8)) + [NRG]
        acc, tot = 0, sum(P["RW"])
        for a, b, w in zip(cuts[:-1], cuts[1:], P["RW"]):
            ta, tb = t0 + acc * (t1 - t0) // tot, t0 + (acc + w) * (t1 - t0) // tot
            add_tasks([(tb, rr_prep, (p, pa, src, a, b, ta, tb - ta))])
            acc += w

    def out_copy(pidx, e0, e1, r0, r1):
        off = pidx * (2 * LB) + e0 * LB
        if not isinstance(pidx, int):
            off = pl.multiple_of(off, LB)
        rs = pl.ds(r0, r1 - r0)
        return pltpu.make_async_copy(out_v.at[pidx, rs, pl.ds(e0 * LB, (e1 - e0) * LB)],
                                     out_hbm.at[0, rs, pl.ds(off, (e1 - e0) * LB)], sems.at[0])

    def b_out(pa, n, m, part, t0=None, dur=None):
        a, y = divmod(n, 2)
        r0, r1, e0, e1 = part
        cols = slice(e0 * LB, e1 * LB)
        for r in range(r0, r1, 16):
            c = _combine([None if v is None else v[r:r + 16, cols] for v in m], n)
            rows = slice(a * HD + r, a * HD + r + 16)
            o = c + x_v[pa + y, rows, cols].astype(f32)
            if t0 is not None:
                o = jnp.concatenate([tie(o[:, 0:LB], at(t0 + (r - r0) * dur // (r1 - r0))), o[:, LB:]], axis=1)
            out_v[pa + y, rows, cols] = o.astype(bf16)
        out_copy(pa + y, e0, e1, a * HD + r0, a * HD + r1).start()

    def big_piece(pa, pan, cur, last):
        t0 = now()
        for n in range(7):
            ta, tb = t0 + n * PD + P["RR0"], t0 + n * PD + P["RR1"]
            if n < 6:
                rr_tasks(BORD[n + 1], pa, cur, ta, tb)
            else:
                rr_tasks(BORD[0], pan, 1 - cur, ta, tb - (P["RRM"] if last else 0))
        ready.difference_update({("o", 1 - cur, hh, e) for hh in range(2) for e in range(4)})
        for n in range(8):
            e, hh = divmod(n, 2)
            t = t0 + P["BV0"] + n * P["BVS"]
            add_tasks([(t + P["BVD"], attn_pv, (pan * 2 + e, hh, 1 - cur, e, t, P["BVD"]))])
        m = [None] * 7
        for p in BORD:
            flush(now())
            assert ("rr", p) in ready
            x, y = TOP[p][0]

            def lhs(q):
                if q in (2, 3):
                    rows = slice(p * QD + (q - 2) * ED, p * QD + (q - 1) * ED)
                    return _up(jnp.concatenate([lc_s[rows, _blk(2 * qd + q - 2)] for qd in range(NQ)]
                                               + [lc_s[rows, (NFP + q - 2) * LB:(NFP + q - 2) * LB + QD]], axis=1))
                return _up(ll_s[(p * 7 + q) * ED:(p * 7 + q + 1) * ED, 0:KL])

            def rhs(q):
                if p in SIDX or q in SIDX:
                    return _up(rr_s[p * RRK:p * RRK + KL // 2, _blk(q)])
                h = 0 if q == 1 else 1
                return _cat([w2_v[pa + y, _blk(2 * (2 * qd + h) + x), _blk(h)] for qd in range(NQ)]
                            + [_up(rr_s[p * RRK + NQ * LB // 2:p * RRK + KL // 2, _blk(q)])], 0)
            rl = (_up(rr_s[p * RRK:p * RRK + LB // 2, 7 * LB:9 * LB]) if p in SIDX
                  else w2_v[pa + y, _blk(4 * NQ + x), :])
            ll = _up(lc_s[p * QD:(p + 1) * QD, _blk(2 * NQ)])
            ex = [mm1(ll[:QD], rl), mm1(ll[QD:], rl)]
            e12, e21 = ex[0][:, LB:], ex[1][:, :LB]
            e11 = (ex[0][:, :LB] + e12) - e21
            lf = strassen(lhs, rhs, LORD)
            ready.discard(("rr", p))
            if p in (2, 3):
                for q in (2, 3):
                    lf[q] = lf[q] + b2f_s[pa + 3 - p, 0:1, _blk(3 - q)]
            c12 = (lf[2] + e12) + lf[4]
            c21 = (lf[1] + e21) + lf[3]
            xx = (lf[2] - lf[1]) + lf[0]
            c22 = (xx + ex[1][:, LB:]) + lf[5]
            c11 = ((xx + e11) + (c21 - c12)) + lf[6]
            m[p] = jnp.concatenate([jnp.concatenate([c11, c12], axis=1),
                                    jnp.concatenate([c21, c22], axis=1)], axis=0)
            n = {3: 2, 4: 1, 5: 3, 6: 0}.get(p)
            if n is not None and not (last and n == 0):
                t, epd = now() + P["EP0"], P["EPL"] if (last and n == 3) else P["EPD"]
                add_tasks([(t + epd, b_out, (pa, n, list(m), (0, HD, 0, 2), t, epd))])
        if last:
            flush()
            for part in LAST_PARTS:
                b_out(pa, 0, m, part)

    def c_body(it, carry):
        reset()
        pos[:] = [one_s[...]]
        true.clear()
        ready.update({("rr", BORD[0])} | {("o", 0, hh, e) for hh in range(2) for e in range(4)})
        big_piece(4 * it, 4 * it + 2, 0, False)
        big_piece(4 * it + 2, lax.rem(4 * it + 4, NP), 1, True)
        assert ("rr", BORD[0]) in ready and all(("o", 0, hh, 3) in ready for hh in range(2))
        return carry

    E1 = P["E1"]
    x0 = Group(cp_x(0, 1))
    g1 = Group([(b1_hbm, b1_v)] + cp_w1(0, 2, 0, E1))
    g2 = Group(cp_w1(0, 2, E1, NFP) + cp_x(1, 2))
    wq, wkv = [[(wqkv_hbm.at[:, cl], wqkv_v.at[:, cl])] for cl in (pl.ds(0, 4 * LB), pl.ds(4 * LB, 3 * D - 4 * LB))]
    g3 = Group(wq)
    g4 = Group(wkv + cp_x(2, 3))
    g5 = Group(cp_x(3, NP))
    g6 = Group(cp_w1(UB0, NB) + [(wo_hbm, wo_v), (b2_hbm, b2_v)] + cp_w2(0, 1))
    g7 = Group(cp_w2(1, NP))
    for c in (x0, g1, g2, g3, g4, g5, g6, g7):
        c.start()

    v_s[0] = jnp.zeros((D, LB), f32)
    for buf in (xnT_s, ra_s, lh_s, rs_s, rr_s, ola_s, olb_s, ll_s, lc_s):
        buf[0:8, 0:64] = jnp.zeros((8, 64), buf.dtype)

    wait("x0", x0)
    one_s[...] = lax.shift_right_logical(pltpu.bitcast(x_v[0, 0:16, 0:LB], i32), 1) | 1
    pos[:] = [one_s[...]]
    ln(0)
    ln(1)
    hpair(0)
    wait("r1", g1)
    jobs = u_early(0, 0, E1, [], 7 * E1 // 4 * 4, P["T1"], 100)
    wait("r2", g2)
    t, dt = P["L2T"], P["L2D"]
    add_tasks([(t + int((k + 1) * dt * P["LNV"]), ln, (2 + k, t + int(k * dt * P["LNV"]), dt)) for k in range(2)])
    jobs = u_early(0, E1, NFP, jobs, P["N2"], P["T2"], 100)
    wait("wq", g3)
    add_tasks([(P["H2T"] + P["H2D"], hpair, (2, P["H2T"], P["H2D"]))])
    u_early(0, 0, 0, jobs, len(jobs), 0, 1, nsplit=P["S3"])
    prep_wqkv("q", 0, HD // 16, P["WQ"])
    stage_a(0, "q", split_last=True)
    m = stage_a(2, "q", AORD[:P["NA3"]])
    wait("wkv", g4)
    stage_a(2, "q", AORD[P["NA3"]:], split_last=True, m=m)
    prep_wqkv("kv", HD // 16, HA // 16, P["WKV"])
    t = ln_tasks(4, now() + P["L4T"], P["LND"], P["HSD"])
    n4 = min(4, (now() + 14 * HD - P["MARG"] - t) // P["BD"])
    add_tasks([(t + (n + 1) * P["BD"], slot, (t + n * P["BD"], P["BD"])) for n in range(n4)])
    stage_a(0, "kv")
    stage_a(2, "kv", order=(6,) + AORD[:6])

    wait("mid", g5)
    AD = 7 * HA // 2
    t = P["L5T"]
    for b in range(6, NB, 2):
        t = ln_tasks(b, t, P["LND"], P["HSD"])
    n5 = ((NP - 2) * AD - P["MARG"] - t) // P["BD"]
    add_tasks([(t + (n + 1) * P["BD"], slot, (t + n * P["BD"], P["BD"])) for n in range(n5)])
    n5 += n4
    for n, b in enumerate(range(4, NB, 2)):
        stage_a(b, order=(6,) + AORD[:6] if n % 2 else AORD)

    wait("fin", g6)
    UD = 7 * NUP * HD // 4
    for i in range(NFP):
        t0, dt = (-200, 130) if i == 0 else (800, 270) if i == 1 else ((i - 1) * UD + P["US0"], P["USD"])
        add_tasks([(t0 + (k + 1) * dt, tsum, (UB0 // 2 + k, i, i % 3, k, t0 + k * dt, dt)) for k in range(NUP)])
    left = len(mains) - n5 - 2
    bd = (NFP * UD - P["R6E"] - P["R6S"]) // left
    add_tasks([(P["R6S"] + (n + 1) * bd, slot, (P["R6S"] + n * bd, bd)) for n in range(left)])
    t = P["R6S"] + left * bd
    add_tasks([(t + (n + 1) * 300, slot, (t + n * 300, 300)) for n in range(2)])
    for qd, t0, t1 in ((NQ, UD + P["LL0"], 3 * UD), (0, 3 * UD + P["LL0"], 5 * UD), (1, 5 * UD + P["LL0"], 6 * UD + 200),
                       (2, 6 * UD + P["LL2"], 6 * UD + P["LL2"] + P["UEL"])):
        dt = (t1 - t0) // 7
        add_tasks([(t0 + (g + 1) * dt, llsum, (qd, g, t0 + g * dt, dt)) for g in range(7)])
    rr_tasks(BORD[0], 0, 0, P["RP0"], P["RP1"])
    add_tasks([(P["PW0"] + P["PWD"], prep_wo_a, (P["PW0"], P["PWD"]))])
    add_tasks([(P["PW1"] + (h + 1) * P["PWE"], prep_wo_b, (h, P["PW1"] + h * P["PWE"], P["PWE"])) for h in range(2)])
    for b in range(NB):
        b2f_s[b // 2, 0:1, _blk(b % 2)] = b2_v[b:b + 1, :].astype(f32)
    for i in range(NFP):
        u_last(i, (1, 4, 2, 3, 0, 5, 6) if i == 0 else (4, 2, 1, 3, 0, 5, 6),
               None if i == NFP - 1 else P["UEL"] if i == NFP - 2 else P["UED"])
    flush()
    assert slot_ctr[0] == len(mains) and all(("ll", qd, g) in ready for qd in range(NQ + 1) for g in range(7))
    assert all(("pr", j, hh) in ready for j in range(NB) for hh in range(2)) and ("rr", BORD[0]) in ready

    wait("w2", g7)
    lax.fori_loop(0, NP // 4, c_body, 0)
    outs = []
    for pa in range(0, NP, 2):
        outs += [out_copy(pa + n % 2, 0, 2, n // 2 * HD, (n // 2 + 1) * HD) for n in (1, 2, 3)]
        outs += [out_copy(pa, e0, e1, r0, r1) for (r0, r1, e0, e1) in (LAST_PARTS if pa % 4 else [(0, HD, 0, 2)])]
    wait("out", *outs)


@jax.jit
def pallas_parallel_sum__sliding_local_dilated__mixer_token_mlp__prompt_kernel(A_x, A_wqkv, A_wo, B_x, B_w1, B_b1, B_w2, B_b2):
    del B_x
    hbm = pl.BlockSpec(memory_space=pltpu.HBM)
    outT = pl.pallas_call(
        _kernel,
        out_shape=jax.ShapeDtypeStruct((1, D, S), bf16),
        in_specs=[hbm] * 7,
        out_specs=hbm,
        scratch_shapes=[
            pltpu.VMEM((NP, D, 2 * LB), bf16),
            pltpu.VMEM((D, 3 * D), bf16),
            pltpu.VMEM((D, D), bf16),
            pltpu.VMEM((S, F), bf16),
            pltpu.VMEM((NP, F, 2 * LB), bf16),
            pltpu.VMEM((NFB, LB), bf16),
            pltpu.VMEM((NB, LB), bf16),
            pltpu.VMEM((NP, D, 2 * LB), bf16),
            pltpu.VMEM((2, 3 * D + 64, LB), i32),
            pltpu.VMEM((7 * HA // 2, HD), u32),
            pltpu.VMEM((4, HD + 32, LB), i32),
            pltpu.VMEM((D, 2 * LB), i32),
            pltpu.VMEM((HD, S), u32),
            pltpu.VMEM((NP * QD, 5 * LB), u32),
            pltpu.VMEM((7 * QD, NP * LB), u32),
            pltpu.VMEM((7 * HD, NFP * LB), f32),
            pltpu.VMEM((7 * QD, (NFP + 2) * LB), u32),
            pltpu.VMEM((NB, 2 * D, LB), f32),
            pltpu.VMEM((NB + 1, D, LB), f32),
            pltpu.VMEM((NB, 2 * W * HH, LB), f32),
            pltpu.VMEM((D, LB), f32),
            pltpu.VMEM((NP, 32, 2 * LB), f32),
            pltpu.VMEM((4 * RSK, 5 * LB), u32),
            pltpu.VMEM((49 * ED, 4 * LB), u32),
            pltpu.VMEM((7 * RRK, 9 * LB), u32),
            pltpu.VMEM((D, 4 * LB), f32),
            pltpu.VMEM((D, 4 * LB), f32),
            pltpu.VMEM((8, LB), i32),
            pltpu.SemaphoreType.DMA((9,)),
        ],
        compiler_params=pltpu.CompilerParams(vmem_limit_bytes=100 * 1024 * 1024,
                                             disable_bounds_checks=True,
                                             disable_semaphore_checks=True),
    )(jnp.swapaxes(A_x, 1, 2), A_wqkv, A_wo, B_w1, B_b1.reshape(NFB, LB), B_w2, B_b2.reshape(NB, LB))
    return jnp.swapaxes(outT, 1, 2)
```

```python
import jax
import jax.numpy as jnp
from jax import lax
import jax.experimental.pallas as pl
import jax.experimental.pallas.tpu as pltpu

S, D, F = 2048, 448, 1792
H, DH, W, DIL = 16, 28, 8, 2
LB = 128
NB = S // LB
NP = NB // 2
NFB = F // LB
NFP = NFB // 2
HH = H // 2
WH = W // 2
SH = DIL * WH
HD = D // 2
QD = D // 4
ED = D // 8
HA = 3 * HD
UB0 = 2
NUP = (NB - UB0) // 2
RSK = NFP * LB // 2
NQ = NFP // 2
KL = NQ * LB + QD
RRK = 2 * LB
EPS = 1e-5
SCALE = DH ** -0.5
f32 = jnp.float32
bf16 = jnp.bfloat16
u32 = jnp.uint32
i32 = jnp.int32

SCOPES = False
P = dict(
    E1=3, N2=16, NA3=2, T1=-200, T2=-200, S3=0, L2T=230, L2D=380, H2T=900, H2D=360, L4T=1000, L5T=60, W2X=500,
    QA=-410, QB=200, QC=-200, QE=330, KA=50, KB=320, KC=450, KE=390,
    LND=400, HSD=360, HL=300, LNA=0.32, LNB=0.42, LNBD=0.33, LNV=0.8, LNW=0.86,
    BD=370, MARG=300, LAG=200, LS=150, PP=130, PVL=500, PVPOS=12,
    US0=100, USD=360, UE0=240, UED=2320, UEL=1700, UG=70, UM=0, R6S=1750, R6E=3150,
    LL0=300, LL2=550, RP0=16600, RP1=18700, PW0=560, PWD=300, PW1=1380, PWE=400,
    RR0=-48, RR1=800, RRM=-20, RW=(8, 8, 8, 2, 7), BV0=117, BVS=717, BVD=620, EP0=0, EPD=864, EPL=290, SGR=8, SGT=8, SH4=1,
)
G = 4


def _as(x, dtype):
    return x if x.dtype == dtype else pltpu.bitcast(x, dtype)


def _pk(x):
    return pltpu.bitcast(x.astype(bf16), u32)


def _up(x):
    return pltpu.bitcast(x, bf16)


def _upf(x):
    return pltpu.bitcast(x, bf16).astype(f32)


def _word(lo, hi):
    lo, hi = [pltpu.bitcast(v.astype(f32), i32) for v in (lo, hi)]
    return lax.shift_right_logical(lo, 16) | hi


def _unword(w):
    return [pltpu.bitcast(w << 16, f32), pltpu.bitcast(w & -65536, f32)]


def _cat(xs, axis):
    return xs[0] if len(xs) == 1 else jnp.concatenate(xs, axis=axis)


def _x2(v):
    return jnp.concatenate([v, v], axis=0)


def _blk(b):
    return slice(b * LB, (b + 1) * LB)


def _rowsum8(a):
    return jnp.broadcast_to(jnp.sum(a, axis=0, keepdims=True), (8, a.shape[1]))


def _token(*deps):
    deps = [d for d in deps if d is not None]
    if not deps:
        return None
    if len(deps) == 1:
        return deps[0]
    bits = _as(deps[0], u32)
    for d in deps[1:]:
        bits = bits | _as(d, u32)
    return bits


def _lhs_ops(a11, a12, a21, a22):
    return [a11 + a22, a21 + a22, a11, a22, a11 + a12, a21 - a11, a12 - a22]


SIDX = {0: 0, 2: 1, 3: 2, 5: 3, 6: 4}
TOP = {0: ((0, 0), 1, (1, 1)), 1: ((0, 0),), 2: ((0, 1), -1, (1, 1)), 3: ((1, 0), -1, (0, 0)),
       4: ((1, 1),), 5: ((0, 0), 1, (0, 1)), 6: ((1, 0), 1, (1, 1))}


def _rhs_sums(b11, b12, b21, b22):
    return {0: b11 + b22, 2: b12 - b22, 3: b21 - b11, 5: b11 + b12, 6: b21 + b22}


def _rhs_op(p, blk):
    t = TOP[p]
    if len(t) == 1:
        return blk(*t[0])
    return blk(*t[0]) + blk(*t[2]) if t[1] > 0 else blk(*t[0]) - blk(*t[2])


def _combine(m, n=None):
    c12 = lambda: m[2] + m[4]
    c21 = lambda: m[1] + m[3]
    x = lambda: (m[2] - m[1]) + m[0]
    c = [lambda: (x() + m[6]) + (c21() - c12()), c12, c21, lambda: x() + m[5]]
    return [f() for f in c] if n is None else c[n]()


def _kernel(x_hbm, wqkv_hbm, wo_hbm, w1_hbm, b1_hbm, w2_hbm, b2_hbm, out_hbm,
            x_v, wqkv_v, wo_v, w1_v, w2_v, b1_v, b2_v, out_v,
            wt_s, lw_s, wo_s, wq_s, xnT_s, ra_s, lh_s, um_s, lc_s, qk_s, v_s, pr_s, op_s,
            b2f_s, rs_s, ll_s, rr_s, ola_s, olb_s, one_s, sems):
    sem_ctr = [1]

    class Group:
        def __init__(self, pairs):
            self.cps = [pltpu.make_async_copy(a, b, sems.at[sem_ctr[0]]) for (a, b) in pairs]
            sem_ctr[0] += 1

        def start(self):
            for c in self.cps:
                c.start()

        def wait(self):
            for c in self.cps:
                c.wait()

    def cp_x(p0, p1):
        return [(x_hbm.at[0, :, pl.ds(p * 2 * LB, 2 * LB)], x_v.at[p]) for p in range(p0, p1)]

    def cp_w2(p0, p1):
        return [(w2_hbm.at[:, pl.ds(p * 2 * LB, 2 * LB)], w2_v.at[p]) for p in range(p0, p1)]

    def cp_w1(b0, b1, i0=0, i1=NFP):
        sl = pl.ds(b0 * LB, (b1 - b0) * LB)
        cl = pl.ds(i0 * 2 * LB, (i1 - i0) * 2 * LB)
        return [(w1_hbm.at[sl, cl], w1_v.at[sl, cl])]

    tl = []
    mxu = [0, 0, 0, 0]
    nxt = [0]
    hist = []
    tasks = []
    dls = []
    ready = set()
    pos = []
    true = {}

    def tie(v, z):
        if z is None:
            return v
        def fit(a):
            a = _cat([a] * (v.shape[0] // 8), 0)
            return a if v.shape[1] == LB else a[:, 0:v.shape[1]]
        if v.shape not in true:
            true[v.shape] = fit(pos[0]) > 0
        return lax.select(true[v.shape], v, fit(_as(z, v.dtype)))

    def tie8(v, z):
        return v if z is None else jnp.concatenate([tie(v[0:8], z), v[8:16]], axis=0)

    def add_tasks(todo):
        tasks.extend(todo)
        tasks.sort(key=lambda x: x[0])

    def flush(t=None):
        while tasks and (t is None or tasks[0][0] < t):
            _, fn, args = tasks.pop(0)
            fn(*args)

    def reset():
        assert not tasks
        dls.clear()
        tl.clear()
        hist.clear()
        mxu[:] = [0, 0, 0, 0]
        nxt[0] = 0

    def now():
        return sum(mxu) // 4

    def wait(name, *cps):
        flush()
        if SCOPES:
            with jax.named_scope("wait_" + name):
                for c in cps:
                    c.wait()
        else:
            for c in cps:
                c.wait()
        reset()

    def mm1(lhs, rhs, pace=True):
        flush(now())
        start = mxu[nxt[0]]
        due = [v for (t, v) in dls if t <= start] if pace else []
        if due:
            dls[:] = [(t, v) for (t, v) in dls if t > start]
            tile = _up(tie(pltpu.bitcast(lhs[0:16, 0:LB], u32), _token(*due)))
            row = tile if lhs.shape[1] == LB else jnp.concatenate([tile, lhs[0:16, LB:]], axis=1)
            lhs = jnp.concatenate([row, lhs[16:]], axis=0)
        r = jnp.dot(lhs, rhs, preferred_element_type=f32)
        m, k = lhs.shape
        first_done = None
        for _ in range(-(-rhs.shape[1] // LB)):
            end = 0
            for _ in range(-(-k // LB)):
                mxu[nxt[0]] += m
                end = max(end, mxu[nxt[0]])
                nxt[0] = (nxt[0] + 1) % 4
            if first_done is None:
                first_done = end
        if pace:
            tl.append((first_done - m, first_done, r))
        return r

    def mm(lhs, rhs, init=None):
        k = lhs.shape[1]
        r, k0 = init, 0
        while k0 < k:
            k1 = min(k, k0 + (4 - nxt[0]) * LB)
            part = mm1(lhs[:, k0:k1], rhs[k0:k1], pace=k1 - k0 > LB)
            r = part if r is None else r + part
            k0 = k1
        return r

    def at(t, *more):
        best = None
        if t is not None and t >= 0:
            t = min(t, now() - 1)
            for (a, b, r) in tl:
                if a <= t and (best is None or min(b, t) > best[0]):
                    row = int(min((t - a) / (b - a), 0.999) * (r.shape[0] // 8)) * 8
                    best = (min(b, t), r, row)
        return _token(None if best is None else best[1][best[2]:best[2] + 8, 0:LB], *more)

    def strassen(lhs, rhs, order, split_last=False, init=None, m=None):
        m = [None] * 7 if m is None else m
        for p in order:
            flush(now())
            l, r = lhs(p), rhs(p)
            c0 = None if init is None else init[p]
            if split_last and p == order[-1]:
                kk = (-(-r.shape[0] // LB) - 2) * LB
                hm = l.shape[0] // 2
                hd = mm(l[:, :kk], r[:kk], c0) if kk else c0
                tail = jnp.concatenate([mm(l[:hm, kk:], r[kk:]), mm(l[hm:, kk:], r[kk:])], axis=0)
                m[p] = tail if hd is None else hd + tail
            else:
                m[p] = mm(l, r, c0)
        return m

    def wrows(hh, g, z=None):
        p, d = divmod(2 * g, DH)
        t = [jnp.concatenate([wt_s[c, pl.ds(p * D + hh * HD + d + e, HH, stride=DH), :]
                              for e in range(2)], axis=0) for c in range(2)]
        return _unword(jnp.concatenate([tie(t[0], z), tie(t[1][:, 0:HD - LB], z)], axis=1))

    wt_done = set()

    def prep_wqkv(part, ga, gb, paced):
        def need(hh, p, z):
            lo = p * D + hh * HD
            for ct in range(lo // LB, -(-(lo + HD) // LB)):
                if ct in wt_done:
                    continue
                wt_done.add(ct)
                cols = slice(ct * LB, min((ct + 1) * LB, 3 * D))
                wd = _word(wqkv_v[0:HD, cols], wqkv_v[HD:D, cols])
                wd = jnp.concatenate([tie(wd[r:r + 8], z if r % LB == 0 else None) for r in range(0, HD, 8)], axis=0)
                wT = wd.T
                wt_s[0, cols, :] = wT[:, 0:LB]
                wt_s[1, cols, 0:HD - LB] = wT[:, LB:HD]

        def put(p, g, v):
            lw_s[p * (HA // 2) + g * 8:p * (HA // 2) + g * 8 + 8, :] = _pk(v)

        def half(hh, g0, g1, t0=None, dur=None):
            pr, ps = ((2, 4), (3, 1))[hh]
            for g in range(g0, g1):
                t = None if t0 is None else t0 + (g - g0) * dur // (g1 - g0)
                need(hh, 2 * g // DH, at(None if t is None else t - P["W2X"]))
                a1, a2 = wrows(hh, g, at(t))
                put(pr, g, a2 if hh else a1)
                put(ps, g, a1 + a2)
            if g1 == gb:
                ready.update({("lw", part, pr), ("lw", part, ps)})

        def rest(g0, g1, t0, dur):
            assert ("lw", part, 1) in ready
            for g in range(g0, g1):
                z = at(t0 + (g - g0) * dur // (g1 - g0))
                ops = _lhs_ops(*wrows(0, g, z), *wrows(1, g, z))
                for p in (0, 5, 6):
                    put(p, g, ops[p])
            if g1 == gb:
                ready.update({("lw", part, 0), ("lw", part, 5), ("lw", part, 6)})
        t2, d2, t3, d3 = paced
        half(0, ga, gb)
        n = (gb - ga) // 14
        add_tasks([(now() + t2 + (k + 1) * d2 // n, half,
                    (1, ga + 14 * k, ga + 14 * k + 14, now() + t2 + k * d2 // n, d2 // n)) for k in range(n)])
        n = (gb - ga) // 7
        add_tasks([(now() + t3 + (k + 1) * d3 // n, rest,
                    (ga + 7 * k, ga + 7 * k + 7, now() + t3 + k * d3 // n, d3 // n)) for k in range(n)])

    def prep_wo_a(t0, dur):
        for g in range(HD // 16):
            w = _word(wo_v[g * 16:g * 16 + 16, :], wo_v[HD + g * 16:HD + g * 16 + 16, :])
            z = at(t0 + g * dur // (HD // 16))
            for c in range(4):
                cw = min(LB, D - c * LB)
                wo_s[c, g * 16:g * 16 + 16, 0:cw] = tie(w[:, c * LB:c * LB + cw], z)
        ready.add("wo")

    def prep_wo_b(h, t0, dur):
        assert "wo" in ready
        for c in range(4):
            cw = min(LB, D - c * LB)
            rows = [wo_s[c, pl.ds(d, HH, stride=DH), :][:, 0:cw] for d in range(h * DH // 2, (h + 1) * DH // 2)]
            rows.append(jnp.zeros((LB - QD, cw), i32))
            wq_s[c * LB:c * LB + cw, _blk(h)] = jnp.concatenate(rows, axis=0).T
        outs = []
        for g in range(HD // 16):
            z = at(t0 + g * dur // (HD // 16))
            a = [v for r in (g * 16, HD + g * 16) for v in _unword(tie(wq_s[r:r + 16, _blk(h)], z))]
            for p, v in enumerate(_lhs_ops(*a)):
                lc_s[p * QD + g * 8:p * QD + g * 8 + 8, _blk(NFP + h)] = _pk(v)
                outs.append(v[0:8])
        ready.update({("lc", NFP + h, g) for g in range(HD // 16)})
        dls.append((t0 + dur + 250, _token(*outs)))

    RG = 16
    NG = D // RG
    stat2 = {}

    def ln(b, t0=None, dur=None):
        def xg(g):
            return x_v[b // 2, g * RG:(g + 1) * RG, _blk(b % 2)].astype(f32)

        def step(v, g, fr, s, q):
            if t0 is None or g % 4:
                return v
            acc = [] if s is None else [s[0:8], s[8:16], q[0:8], q[8:16]]
            return tie(v, at(t0 + fr * dur, *acc))

        x0 = jnp.broadcast_to(xg(0)[0:1], (8, LB))
        s = q = None
        for g in range(NG):
            x0 = step(x0, g, P["LNA"] * g / NG, s, q)
            c = xg(g) - _x2(x0)
            s = c if s is None else s + c
            q = c * c if q is None else q + c * c
        dm = _rowsum8(s) * (1.0 / D)
        mu = x0 + dm
        r1 = lax.rsqrt(jnp.maximum(_rowsum8(q) * (1.0 / D) - dm * dm, 0.0) + EPS)
        s = q = None
        for g in range(NG):
            mu = step(mu, g, P["LNB"] + P["LNBD"] * g / NG, s, q)
            xn = (xg(g) - _x2(mu)) * _x2(r1)
            xnT_s[g * 8:g * 8 + 8, _blk(b)] = _pk(xn)
            s = xn if s is None else s + xn
            q = xn * xn if q is None else q + xn * xn
        mu2 = _rowsum8(s) * (1.0 / D)
        var2 = jnp.maximum(_rowsum8(q) * (1.0 / D) - mu2 * mu2, 0.0)
        stat2[b] = (mu2, 0.5 * lax.rsqrt(var2 + EPS))

    def hpair(b, t0=None, dur=None):
        ng = HD // RG
        st = [stat2.pop(b), stat2.pop(b + 1)]
        for g in range(ng):
            zz = [at(None if t0 is None else t0 + (4 * g + k * P["SH4"]) * dur // (4 * ng)) for k in (0, 1, 2, 3)]
            xq = [_upf(tie(xnT_s[r:r + 8, _blk(b + e)], zz[2 * (r >= QD) + e]))
                  for r in (g * 8, QD + g * 8) for e in range(2)]
            hq = [(v - _x2(st[n % 2][0])) * _x2(st[n % 2][1]) for n, v in enumerate(xq)]
            ro = (b // 2) * QD + g * 8
            for p, v in _rhs_sums(*xq).items():
                ra_s[ro:ro + 8, _blk(SIDX[p])] = _pk(v)
            for p, v in enumerate(_lhs_ops(*hq)):
                lh_s[p * QD + g * 8:p * QD + g * 8 + 8, _blk(b // 2)] = _pk(v)
        ready.add(("xn", b))
        if b >= 6:
            got = ra_s[(b // 2) * QD:(b // 2 + 1) * QD, :]
            dls.append((t0 + dur + P["HL"], _token(*[got[r:r + 8, _blk(c)] for r in range(0, QD, 8) for c in range(5)])))

    def ln_tasks(b, t, lnd, hsd):
        for fn, bb, dur, adv in ((ln, b, lnd, P["LNV"]), (ln, b + 1, lnd, P["LNW"]), (hpair, b, hsd, 1.0)):
            add_tasks([(t + int(dur * adv), fn, (bb, t, dur))])
            t += int(dur * adv)
        return t

    def tsum(kp, i, slot_, n, t0, dur):
        for g in range(LB // 16):
            z, z2 = at(t0 + g * dur // 8), at(t0 + g * dur // 8 + P["SGT"])
            t1, t2 = [w1_v[(2 * kp + e) * LB + g * 16:(2 * kp + e) * LB + g * 16 + 16,
                           2 * i * LB:(2 * i + 2) * LB].astype(f32) for e in range(2)]
            ro = slot_ * RSK + n * (LB // 2) + g * 8
            for p, v in _rhs_sums(tie8(t1[:, :LB], z), t1[:, LB:], t2[:, :LB], tie8(t2[:, LB:], z2)).items():
                rs_s[ro:ro + 8, _blk(SIDX[p])] = _pk(v)
        ready.add(("rs", kp, i))

    def u_rhs(p, i, kps, slot_, n0):
        if p in SIDX:
            assert all(("rs", kp, i) in ready for kp in kps)
            ro = slot_ * RSK + n0 * (LB // 2)
            return _up(rs_s[ro:ro + len(kps) * (LB // 2), _blk(SIDX[p])])
        e = 0 if p == 1 else 1
        return _cat([w1_v[_blk(2 * kp + e), _blk(2 * i + e)] for kp in kps], 0)

    LATE = (NFP - 1, 6)

    def ujob(kp, i, p, split):
        flush(now())
        assert ("xn", 2 * kp) in ready
        l, r = _up(lh_s[p * QD:(p + 1) * QD, _blk(kp)]), u_rhs(p, i, [kp], 3 + kp, i)
        v = jnp.concatenate([mm1(l[:QD], r), mm1(l[QD:], r)], axis=0) if split else mm1(l, r)
        if p in (2, 3):
            v = v + 0.5 * b1_v[2 * i + 3 - p:2 * i + 4 - p, :].astype(f32)
        rows = slice(p * HD, (p + 1) * HD)
        um_s[rows, _blk(i)] = v

    def u_early(kp, i0, i1, carry, n, t0, dt, nsplit=0):
        for k, i in enumerate(range(i0, i1)):
            add_tasks([(t0 + (k + 1) * dt, tsum, (kp, i, 3 + kp, i, t0 + k * dt, dt))])
        jobs = (carry + [(kp, i, p) for i in range(i0, i1) for p in (1, 4)]
                + [(kp, i, p) for i in range(i0, i1) for p in SIDX if (i, p) != LATE])
        for c, job in enumerate(jobs[:n]):
            ujob(*job, c >= n - nsplit)
        return jobs[n:]

    def gelu_half(hx, z):
        c = 0.7978845608028654
        return hx + hx * jnp.tanh(tie(hx * (2.0 * c + (8.0 * c * 0.044715) * (hx * hx)), z))

    def u_epilogue(i, m, gs, t0, dur):
        for n, g in enumerate(gs):
            t = None if t0 is None else t0 + n * dur // len(gs) - P["UG"]
            q = _combine([x[g * 16:g * 16 + 16] for x in m])
            gl = [gelu_half(v, at(None if t is None else t - k * P["UM"])) for v, k in zip(q, (0, 3, 2, 1))]
            for p, v in enumerate(_lhs_ops(*gl)):
                lc_s[p * QD + g * 8:p * QD + g * 8 + 8, _blk(i)] = _pk(v)
            ready.add(("lc", i, g))

    def u_last(i, order, edur):
        kps = list(range(UB0 // 2, NP))
        m = strassen(lambda p: _up(lh_s[p * QD:(p + 1) * QD, (0 if (i, p) == LATE else UB0 // 2 * LB):]),
                     lambda p: _cat([u_rhs(p, i, [0], 3, i)] * ((i, p) == LATE) + [u_rhs(p, i, kps, i % 3, 0)], 0),
                     order, init=[None if (i, p) == LATE else um_s[p * HD:(p + 1) * HD, _blk(i)] for p in range(7)])
        if edur is None:
            u_epilogue(i, m, list(range(HD // 16)), None, None)
        else:
            t = now() + P["UE0"]
            add_tasks([(t + (g + 1) * edur // 7, u_epilogue, (i, m, [g, g + 7], t + g * edur // 7, edur // 7))
                       for g in range(7)])

    def llsum(qd, g, t0, dur):
        i0 = 2 * qd if qd < NQ else NFP
        assert all(("lc", i0 + e, g + 7 * h) in ready for e in range(2) for h in range(2))
        for p in range(7):
            zz = [at(t0 + p * dur // 7), at(t0 + p * dur // 7 + P["SGT"])]
            a = [tie(lc_s[p * QD + h * ED + g * 8:p * QD + h * ED + g * 8 + 8, _blk(i0 + e)], zz[h] if h == e else None)
                 for h in range(2) for e in range(2)]
            ops = _lhs_ops(*[_upf(v) for v in a])
            for q in (0, 1, 4, 5, 6):
                r = (p * 7 + q) * ED + g * 8
                ll_s[r:r + 8, _blk(qd)] = _pk(ops[q])
        ready.add(("ll", qd, g))

    AORD = (4, 2, 1, 3, 0, 5, 6)

    def stage_a(b, parts="qkv", order=AORD, split_last=False, m=None):
        r0, r1 = {"q": (0, HD), "kv": (HD, HA), "qkv": (0, HA)}[parts]

        def lhs(p):
            assert all(("lw", pt, p) in ready for pt in ("q", "kv") if pt in parts)
            return _up(lw_s[(p * HA + r0) // 2:(p * HA + r1) // 2, :])

        def rhs(p):
            assert ("xn", b) in ready
            if p in SIDX:
                return _up(ra_s[(b // 2) * QD:(b // 2 + 1) * QD, _blk(SIDX[p])])
            return _up(xnT_s[0:QD, _blk(b)] if p == 1 else xnT_s[QD:HD, _blk(b + 1)])
        m = strassen(lhs, rhs, order, split_last, m=m)
        for n, ps in enumerate((range(7), (2, 4), (1, 3), (0, 1, 2, 5))):
            if all(m[p] is not None for p in ps) and any(p in order for p in ps):
                hh, e = divmod(n, 2)
                c = _combine(m, n)
                qk_s[b + e, hh * D + r0:hh * D + min(r1, D), :] = c[0:min(r1, D) - r0]
                if r1 > D:
                    v_s[b + e + 1, hh * HD:(hh + 1) * HD, :] = c[D - r0:]
        if all(v is not None for v in m):
            ready.update({(pt, b + e) for pt in ("q", "kv") if pt in parts for e in range(2)})
        return m

    lane0 = lax.broadcasted_iota(i32, (HH, LB), 1)
    zeros8 = jnp.zeros((HH, LB), f32)

    def mk_shift(z):
        lane = tie(lane0, z)
        masks = {}

        def pick(n, a, b):
            if n not in masks:
                masks[n] = lane < n
            return lax.select(masks[n], a, b)

        def fwd(cur, prev, sh):
            return cur if sh == 0 else pltpu.roll(pick(LB - sh, cur, prev), sh, 1)

        def bwd(cur, nxt_):
            return pltpu.roll(pick(SH, nxt_, cur), LB - SH, 1)
        return fwd, bwd

    def grp_shift(t, bd):
        lag = max(2, -(-P["LAG"] * DH // (G * bd)))
        return mk_shift(at(t, *(hist[-lag] if len(hist) >= lag else [])))

    raw, probs = {}, {}

    def attn_qk(j, hh, t, bd):
        jn = min(j + 1, NB - 1)
        assert ("q", jn) in ready and ("kv", j) in ready
        acc = [None] * WH
        accp = [None] * WH
        for d in range(DH):
            if d % G == 0:
                if d > 0:
                    hist.append(acc + accp)
                fwd, bwd = grp_shift(t + d * bd // DH, bd)
            r = hh * D + d * HH
            q = qk_s[j, r:r + HH, :]
            qp = bwd(q, qk_s[jn, r:r + HH, :])
            k = qk_s[j, HD + r:HD + r + HH, :]
            kp = qk_s[j - 1, HD + r:HD + r + HH, :] if j > 0 else zeros8
            for a in range(WH):
                ks = fwd(k, kp, DIL * a)
                t0, t1 = q * ks, qp * ks
                acc[a] = t0 if d == 0 else acc[a] + t0
                accp[a] = t1 if d == 0 else accp[a] + t1
        hist.append(acc + accp)
        raw[j, hh] = (acc, accp)

    def attn_sm(j, hh, t):
        fwd, _ = mk_shift(at(t))
        acc, accp = raw[j, hh]
        prev = raw.pop((j - 1, hh))[1] if j > 0 else [zeros8] * WH
        lg = acc + [fwd(accp[a], prev[a], SH) for a in range(WH)]
        lg = [a * SCALE for a in lg]
        if j == 0:
            lg = [lg[0]] + [jnp.where(lane0 >= DIL * w, lg[w], -1e9) for w in range(1, W)]
        m = lg[0]
        for w in range(1, W):
            m = jnp.maximum(m, lg[w])
        e = [jnp.exp(l - m) for l in lg]
        den = e[0]
        for w in range(1, W):
            den = den + e[w]
        inv = 1.0 / den
        p = [x * inv for x in e]
        for a in range(WH):
            pr_s[j, (hh * W + a) * HH:(hh * W + a + 1) * HH, :] = p[a]
        probs[j, hh] = p[WH:]

    def attn_pp(j, hh, t):
        _, bwd = mk_shift(at(t))
        p = probs.pop((j, hh))
        pn = probs[j + 1, hh] if j + 1 < NB else p
        for a in range(WH):
            pr_s[j, (hh * W + WH + a) * HH:(hh * W + WH + a + 1) * HH, :] = bwd(p[a], pn[a])
        ready.add(("pr", j, hh))

    def attn_pv(j, hh, dst, e, t, bd):
        assert not isinstance(j, int) or ("pr", j, hh) in ready
        assert e == 0 or ("o", dst, hh, e - 1) in ready
        pa = [pr_s[j, (hh * W + a) * HH:(hh * W + a + 1) * HH, :] for a in range(W)]
        p, pp = pa[:WH], pa[WH:]
        outs = []
        for d in range(DH):
            if d % G == 0:
                if d > 0:
                    hist.append([])
                fwd, _ = grp_shift(t + d * bd // DH, bd)
            r = hh * HD + d * HH
            v = v_s[j + 1, r:r + HH, :]
            vp = v_s[j, r:r + HH, :]
            o = op = None
            for a in range(WH):
                vs = fwd(v, vp, DIL * a)
                o = p[a] * vs if a == 0 else o + p[a] * vs
                op = pp[a] * vs if a == 0 else op + pp[a] * vs
            opp = zeros8 if (isinstance(j, int) and j == 0) else op_s[r:r + HH, :]
            op_s[r:r + HH, :] = op
            outs.append(o + fwd(op, opp, SH))
            ol[dst][r:r + HH, _blk(e)] = outs[-1]
        hist.append([])
        ready.add(("o", dst, hh, e))
        dls.append((t + bd + P["PVL"], _token(*outs)))

    ol = [ola_s, olb_s]
    mains = [("qk", j, hh) for j in range(NB) for hh in range(2)]
    mains = (mains[:P["PVPOS"]] + [("pv", j, hh) for j in range(4) for hh in range(2)]
             + mains[P["PVPOS"]:] + [None, None])
    slot_ctr = [0]

    def slot(t, bd):
        n = slot_ctr[0]
        slot_ctr[0] += 1
        it = mains[n]
        if it is None:
            pass
        elif it[0] == "qk":
            attn_qk(it[1], it[2], t, bd)
        else:
            attn_pv(it[1], it[2], 0, it[1], t, bd)
        if n >= 1 and mains[n - 1] is not None and mains[n - 1][0] == "qk":
            attn_sm(mains[n - 1][1], mains[n - 1][2], t + P["LS"])
        if n >= 2 and mains[n - 2] is not None and mains[n - 2][0] == "qk":
            _, j, hh = mains[n - 2]
            if j > 0:
                attn_pp(j - 1, hh, t + P["PP"])
            if j == NB - 1:
                attn_pp(j, hh, t + P["PP"])

    NRG = 8 * (NQ + 1) + 7
    PD = 8 * QD
    BORD = (1, 3, 2, 4, 0, 5, 6)
    LORD = (2, 4, 1, 3, 0, 5, 6)
    LAST_PARTS = [(0, QD, 1, 2), (QD, HD, 0, 2), (0, QD, 0, 1)]

    def rr_prep(p, pa, src, n0, n1, t0, dur):
        assert ("rr", p) not in ready
        for n in range(n0, n1):
            z = at(t0 + (n - n0) * dur // (n1 - n0))
            z2 = at(t0 + (n - n0) * dur // (n1 - n0) + P["SGR"])
            qd, g = divmod(n, 8)

            def wrow(i):
                return _rhs_op(p, lambda x, y: w2_v[pa + y, (2 * i + x) * LB + g * 16:(2 * i + x) * LB + g * 16 + 16, :]
                               .astype(f32))

            def orow(h):
                def blk(x, y):
                    assert ("o", src, x, 2 * y + 1) in ready
                    r = x * HD + h * QD + g * 16
                    return ol[src][r:r + 16, y * 2 * LB:(y + 1) * 2 * LB]
                return _rhs_op(p, blk)
            ro = p * RRK + g * 8
            if qd == NQ:
                if p in SIDX:
                    r = wrow(2 * NQ)
                    for e in range(2):
                        rr_s[ro:ro + 8, _blk(7 + e)] = _pk(tie8(r[:, _blk(e)], z))
                continue
            r1, r2 = (wrow(2 * qd), wrow(2 * qd + 1)) if qd < NQ else (orow(0), orow(1))
            ro += min(qd, NQ) * (LB // 2)
            c11, c22 = tie8(r1[:, :LB], z), tie8(r2[:, LB:], z2)
            sm = _rhs_sums(c11, r1[:, LB:], r2[:, :LB], c22)
            if p in SIDX or qd > NQ:
                sm.update({1: c11, 4: c22})
            for q, v in sm.items():
                rr_s[ro:ro + 8, _blk(q)] = _pk(v)
        if n1 == NRG:
            ready.add(("rr", p))

    def rr_tasks(p, pa, src, t0, t1):
        cuts = list(range(0, NRG, 8)) + [NRG]
        acc, tot = 0, sum(P["RW"])
        for a, b, w in zip(cuts[:-1], cuts[1:], P["RW"]):
            ta, tb = t0 + acc * (t1 - t0) // tot, t0 + (acc + w) * (t1 - t0) // tot
            add_tasks([(tb, rr_prep, (p, pa, src, a, b, ta, tb - ta))])
            acc += w

    def out_copy(pidx, e0, e1, r0, r1):
        off = pidx * (2 * LB) + e0 * LB
        if not isinstance(pidx, int):
            off = pl.multiple_of(off, LB)
        rs = pl.ds(r0, r1 - r0)
        return pltpu.make_async_copy(out_v.at[pidx, rs, pl.ds(e0 * LB, (e1 - e0) * LB)],
                                     out_hbm.at[0, rs, pl.ds(off, (e1 - e0) * LB)], sems.at[0])

    def b_out(pa, n, m, part, t0=None, dur=None):
        a, y = divmod(n, 2)
        r0, r1, e0, e1 = part
        cols = slice(e0 * LB, e1 * LB)
        for r in range(r0, r1, 16):
            c = _combine([None if v is None else v[r:r + 16, cols] for v in m], n)
            rows = slice(a * HD + r, a * HD + r + 16)
            o = c + x_v[pa + y, rows, cols].astype(f32)
            if t0 is not None:
                o = jnp.concatenate([tie(o[:, 0:LB], at(t0 + (r - r0) * dur // (r1 - r0))), o[:, LB:]], axis=1)
            out_v[pa + y, rows, cols] = o.astype(bf16)
        out_copy(pa + y, e0, e1, a * HD + r0, a * HD + r1).start()

    def big_piece(pa, pan, cur, last):
        t0 = now()
        for n in range(7):
            ta, tb = t0 + n * PD + P["RR0"], t0 + n * PD + P["RR1"]
            if n < 6:
                rr_tasks(BORD[n + 1], pa, cur, ta, tb)
            else:
                rr_tasks(BORD[0], pan, 1 - cur, ta, tb - (P["RRM"] if last else 0))
        ready.difference_update({("o", 1 - cur, hh, e) for hh in range(2) for e in range(4)})
        for n in range(8):
            e, hh = divmod(n, 2)
            t = t0 + P["BV0"] + n * P["BVS"]
            add_tasks([(t + P["BVD"], attn_pv, (pan * 2 + e, hh, 1 - cur, e, t, P["BVD"]))])
        m = [None] * 7
        for p in BORD:
            flush(now())
            assert ("rr", p) in ready
            x, y = TOP[p][0]

            def lhs(q):
                if q in (2, 3):
                    rows = slice(p * QD + (q - 2) * ED, p * QD + (q - 1) * ED)
                    return _up(jnp.concatenate([lc_s[rows, _blk(2 * qd + q - 2)] for qd in range(NQ)]
                                               + [lc_s[rows, (NFP + q - 2) * LB:(NFP + q - 2) * LB + QD]], axis=1))
                return _up(ll_s[(p * 7 + q) * ED:(p * 7 + q + 1) * ED, 0:KL])

            def rhs(q):
                if p in SIDX or q in SIDX:
                    return _up(rr_s[p * RRK:p * RRK + KL // 2, _blk(q)])
                h = 0 if q == 1 else 1
                return _cat([w2_v[pa + y, _blk(2 * (2 * qd + h) + x), _blk(h)] for qd in range(NQ)]
                            + [_up(rr_s[p * RRK + NQ * LB // 2:p * RRK + KL // 2, _blk(q)])], 0)
            rl = (_up(rr_s[p * RRK:p * RRK + LB // 2, 7 * LB:9 * LB]) if p in SIDX
                  else w2_v[pa + y, _blk(4 * NQ + x), :])
            ll = _up(lc_s[p * QD:(p + 1) * QD, _blk(2 * NQ)])
            ex = [mm1(ll[:QD], rl), mm1(ll[QD:], rl)]
            e12, e21 = ex[0][:, LB:], ex[1][:, :LB]
            e11 = (ex[0][:, :LB] + e12) - e21
            lf = strassen(lhs, rhs, LORD)
            ready.discard(("rr", p))
            if p in (2, 3):
                for q in (2, 3):
                    lf[q] = lf[q] + b2f_s[pa + 3 - p, 0:1, _blk(3 - q)]
            c12 = (lf[2] + e12) + lf[4]
            c21 = (lf[1] + e21) + lf[3]
            xx = (lf[2] - lf[1]) + lf[0]
            c22 = (xx + ex[1][:, LB:]) + lf[5]
            c11 = ((xx + e11) + (c21 - c12)) + lf[6]
            m[p] = jnp.concatenate([jnp.concatenate([c11, c12], axis=1),
                                    jnp.concatenate([c21, c22], axis=1)], axis=0)
            n = {3: 2, 4: 1, 5: 3, 6: 0}.get(p)
            if n is not None and not (last and n == 0):
                t, epd = now() + P["EP0"], P["EPL"] if (last and n == 3) else P["EPD"]
                add_tasks([(t + epd, b_out, (pa, n, list(m), (0, HD, 0, 2), t, epd))])
        if last:
            flush()
            for part in LAST_PARTS:
                b_out(pa, 0, m, part)

    def c_body(it, carry):
        reset()
        pos[:] = [one_s[...]]
        true.clear()
        ready.update({("rr", BORD[0])} | {("o", 0, hh, e) for hh in range(2) for e in range(4)})
        big_piece(4 * it, 4 * it + 2, 0, False)
        big_piece(4 * it + 2, lax.rem(4 * it + 4, NP), 1, True)
        assert ("rr", BORD[0]) in ready and all(("o", 0, hh, 3) in ready for hh in range(2))
        return carry

    E1 = P["E1"]
    x0 = Group(cp_x(0, 1))
    g1 = Group([(b1_hbm, b1_v)] + cp_w1(0, 2, 0, E1))
    g2 = Group(cp_w1(0, 2, E1, NFP) + cp_x(1, 2))
    wq, wkv = [[(wqkv_hbm.at[:, cl], wqkv_v.at[:, cl])] for cl in (pl.ds(0, 4 * LB), pl.ds(4 * LB, 3 * D - 4 * LB))]
    g3 = Group(wq)
    g4 = Group(wkv + cp_x(2, 3))
    g5 = Group(cp_x(3, NP))
    g6 = Group(cp_w1(UB0, NB) + [(wo_hbm, wo_v), (b2_hbm, b2_v)] + cp_w2(0, 1))
    g7 = Group(cp_w2(1, NP))
    for c in (x0, g1, g2, g3, g4, g5, g6, g7):
        c.start()

    v_s[0] = jnp.zeros((D, LB), f32)
    for buf in (xnT_s, ra_s, lh_s, rs_s, rr_s, ola_s, olb_s, ll_s, lc_s):
        buf[0:8, 0:64] = jnp.zeros((8, 64), buf.dtype)

    wait("x0", x0)
    one_s[...] = lax.shift_right_logical(pltpu.bitcast(x_v[0, 0:16, 0:LB], i32), 1) | 1
    pos[:] = [one_s[...]]
    ln(0)
    ln(1)
    hpair(0)
    wait("r1", g1)
    jobs = u_early(0, 0, E1, [], 7 * E1 // 4 * 4, P["T1"], 100)
    wait("r2", g2)
    t, dt = P["L2T"], P["L2D"]
    add_tasks([(t + int((k + 1) * dt * P["LNV"]), ln, (2 + k, t + int(k * dt * P["LNV"]), dt)) for k in range(2)])
    jobs = u_early(0, E1, NFP, jobs, P["N2"], P["T2"], 100)
    wait("wq", g3)
    add_tasks([(P["H2T"] + P["H2D"], hpair, (2, P["H2T"], P["H2D"]))])
    u_early(0, 0, 0, jobs, len(jobs), 0, 1, nsplit=P["S3"])
    prep_wqkv("q", 0, HD // 16, [P[k] for k in ("QA", "QB", "QC", "QE")])
    stage_a(0, "q", split_last=True)
    m = stage_a(2, "q", AORD[:P["NA3"]])
    wait("wkv", g4)
    stage_a(2, "q", AORD[P["NA3"]:], split_last=True, m=m)
    prep_wqkv("kv", HD // 16, HA // 16, [P[k] for k in ("KA", "KB", "KC", "KE")])
    t = ln_tasks(4, now() + P["L4T"], P["LND"], P["HSD"])
    n4 = min(4, (now() + 14 * HD - P["MARG"] - t) // P["BD"])
    add_tasks([(t + (n + 1) * P["BD"], slot, (t + n * P["BD"], P["BD"])) for n in range(n4)])
    stage_a(0, "kv")
    stage_a(2, "kv", order=(6,) + AORD[:6])

    wait("mid", g5)
    AD = 7 * HA // 2
    t = P["L5T"]
    for b in range(6, NB, 2):
        t = ln_tasks(b, t, P["LND"], P["HSD"])
    n5 = ((NP - 2) * AD - P["MARG"] - t) // P["BD"]
    add_tasks([(t + (n + 1) * P["BD"], slot, (t + n * P["BD"], P["BD"])) for n in range(n5)])
    n5 += n4
    for n, b in enumerate(range(4, NB, 2)):
        stage_a(b, order=(6,) + AORD[:6] if n % 2 else AORD)

    wait("fin", g6)
    UD = 7 * NUP * HD // 4
    for i in range(NFP):
        t0, dt = (-200, 130) if i == 0 else (800, 270) if i == 1 else ((i - 1) * UD + P["US0"], P["USD"])
        add_tasks([(t0 + (k + 1) * dt, tsum, (UB0 // 2 + k, i, i % 3, k, t0 + k * dt, dt)) for k in range(NUP)])
    left = len(mains) - n5 - 2
    bd = (NFP * UD - P["R6E"] - P["R6S"]) // left
    add_tasks([(P["R6S"] + (n + 1) * bd, slot, (P["R6S"] + n * bd, bd)) for n in range(left)])
    t = P["R6S"] + left * bd
    add_tasks([(t + (n + 1) * 300, slot, (t + n * 300, 300)) for n in range(2)])
    for qd, t0, t1 in ((NQ, UD + P["LL0"], 3 * UD), (0, 3 * UD + P["LL0"], 5 * UD), (1, 5 * UD + P["LL0"], 6 * UD + 200),
                       (2, 6 * UD + P["LL2"], 6 * UD + P["LL2"] + P["UEL"])):
        dt = (t1 - t0) // 7
        add_tasks([(t0 + (g + 1) * dt, llsum, (qd, g, t0 + g * dt, dt)) for g in range(7)])
    rr_tasks(BORD[0], 0, 0, P["RP0"], P["RP1"])
    add_tasks([(P["PW0"] + P["PWD"], prep_wo_a, (P["PW0"], P["PWD"]))])
    add_tasks([(P["PW1"] + (h + 1) * P["PWE"], prep_wo_b, (h, P["PW1"] + h * P["PWE"], P["PWE"])) for h in range(2)])
    for b in range(NB):
        b2f_s[b // 2, 0:1, _blk(b % 2)] = b2_v[b:b + 1, :].astype(f32)
    for i in range(NFP):
        u_last(i, (1, 4, 2, 3, 0, 5, 6) if i == 0 else (4, 2, 1, 3, 0, 5, 6),
               None if i == NFP - 1 else P["UEL"] if i == NFP - 2 else P["UED"])
    flush()
    assert slot_ctr[0] == len(mains) and all(("ll", qd, g) in ready for qd in range(NQ + 1) for g in range(7))
    assert all(("pr", j, hh) in ready for j in range(NB) for hh in range(2)) and ("rr", BORD[0]) in ready

    wait("w2", g7)
    lax.fori_loop(0, NP // 4, c_body, 0)
    outs = []
    for pa in range(0, NP, 2):
        outs += [out_copy(pa + n % 2, 0, 2, n // 2 * HD, (n // 2 + 1) * HD) for n in (1, 2, 3)]
        outs += [out_copy(pa, e0, e1, r0, r1) for (r0, r1, e0, e1) in (LAST_PARTS if pa % 4 else [(0, HD, 0, 2)])]
    wait("out", *outs)


@jax.jit
def pallas_parallel_sum__sliding_local_dilated__mixer_token_mlp__prompt_kernel(A_x, A_wqkv, A_wo, B_x, B_w1, B_b1, B_w2, B_b2):
    del B_x
    hbm = pl.BlockSpec(memory_space=pltpu.HBM)
    outT = pl.pallas_call(
        _kernel,
        out_shape=jax.ShapeDtypeStruct((1, D, S), bf16),
        in_specs=[hbm] * 7,
        out_specs=hbm,
        scratch_shapes=[
            pltpu.VMEM((NP, D, 2 * LB), bf16),
            pltpu.VMEM((D, 3 * D), bf16),
            pltpu.VMEM((D, D), bf16),
            pltpu.VMEM((S, F), bf16),
            pltpu.VMEM((NP, F, 2 * LB), bf16),
            pltpu.VMEM((NFB, LB), bf16),
            pltpu.VMEM((NB, LB), bf16),
            pltpu.VMEM((NP, D, 2 * LB), bf16),
            pltpu.VMEM((2, 3 * D + 64, LB), i32),
            pltpu.VMEM((7 * HA // 2, HD), u32),
            pltpu.VMEM((4, HD + 32, LB), i32),
            pltpu.VMEM((D, 2 * LB), i32),
            pltpu.VMEM((HD, S), u32),
            pltpu.VMEM((NP * QD, 5 * LB), u32),
            pltpu.VMEM((7 * QD, NP * LB), u32),
            pltpu.VMEM((7 * HD, NFP * LB), f32),
            pltpu.VMEM((7 * QD, (NFP + 2) * LB), u32),
            pltpu.VMEM((NB, 2 * D, LB), f32),
            pltpu.VMEM((NB + 1, D, LB), f32),
            pltpu.VMEM((NB, 2 * W * HH, LB), f32),
            pltpu.VMEM((D, LB), f32),
            pltpu.VMEM((NP, 32, 2 * LB), f32),
            pltpu.VMEM((4 * RSK, 5 * LB), u32),
            pltpu.VMEM((49 * ED, 4 * LB), u32),
            pltpu.VMEM((7 * RRK, 9 * LB), u32),
            pltpu.VMEM((D, 4 * LB), f32),
            pltpu.VMEM((D, 4 * LB), f32),
            pltpu.VMEM((8, LB), i32),
            pltpu.SemaphoreType.DMA((9,)),
        ],
        compiler_params=pltpu.CompilerParams(vmem_limit_bytes=100 * 1024 * 1024,
                                             disable_bounds_checks=True,
                                             disable_semaphore_checks=True),
    )(jnp.swapaxes(A_x, 1, 2), A_wqkv, A_wo, B_w1, B_b1.reshape(NFB, LB), B_w2, B_b2.reshape(NB, LB))
    return jnp.swapaxes(outT, 1, 2)
```

```python
import jax
import jax.numpy as jnp
from jax import lax
import jax.experimental.pallas as pl
import jax.experimental.pallas.tpu as pltpu

S, D, F = 2048, 448, 1792
H, DH, W, DIL = 16, 28, 8, 2
LB = 128
NB = S // LB
NP = NB // 2
NFB = F // LB
NFP = NFB // 2
HH = H // 2
WH = W // 2
SH = DIL * WH
HD = D // 2
QD = D // 4
ED = D // 8
HA = 3 * HD
UB0 = 2
NUP = (NB - UB0) // 2
RSK = NFP * LB // 2
NQ = NFP // 2
KL = NQ * LB + QD
RRK = 2 * LB
EPS = 1e-5
SCALE = DH ** -0.5
f32 = jnp.float32
bf16 = jnp.bfloat16
u32 = jnp.uint32
i32 = jnp.int32

SCOPES = False
P = dict(
    E1=3, N2=16, NA3=2, T1=-200, T2=-200, S3=0, L2T=230, L2D=380, H2T=900, H2D=360, L4T=1000, L5T=60, W2X=500,
    QA=-410, QB=200, QC=-200, QE=330, KA=50, KB=320, KC=450, KE=390,
    LND=400, HSD=360, HL=300, LNA=0.32, LNB=0.42, LNBD=0.33, LNV=0.8, LNW=0.86,
    BD=370, MARG=300, LAG=200, LS=150, PP=130, PVL=500, PVPOS=12,
    US0=100, USD=360, UE0=240, UED=2320, UEL=1700, UG=70, UM=0, R6S=1750, R6E=3150,
    LL0=300, LL2=550, RP0=16600, RP1=18700, PW0=560, PWD=300, PW1=1380, PWE=400,
    RR0=-48, RR1=800, RRM=-20, RW=(8, 8, 8, 2, 7), BV0=117, BVS=717, BVD=620, EP0=0, EPD=864, EPL=290, SGR=8, SGT=8, SH4=1,
)
G = 4


def _as(x, dtype):
    return x if x.dtype == dtype else pltpu.bitcast(x, dtype)


def _pk(x):
    return pltpu.bitcast(x.astype(bf16), u32)


def _up(x):
    return pltpu.bitcast(x, bf16)


def _upf(x):
    return pltpu.bitcast(x, bf16).astype(f32)


def _word(lo, hi):
    lo, hi = [pltpu.bitcast(v.astype(f32), i32) for v in (lo, hi)]
    return lax.shift_right_logical(lo, 16) | hi


def _unword(w):
    return [pltpu.bitcast(w << 16, f32), pltpu.bitcast(w & -65536, f32)]


def _cat(xs, axis):
    return xs[0] if len(xs) == 1 else jnp.concatenate(xs, axis=axis)


def _x2(v):
    return jnp.concatenate([v, v], axis=0)


def _blk(b):
    return slice(b * LB, (b + 1) * LB)


def _rowsum8(a):
    return jnp.broadcast_to(jnp.sum(a, axis=0, keepdims=True), (8, a.shape[1]))


def _token(*deps):
    deps = [d for d in deps if d is not None]
    if not deps:
        return None
    if len(deps) == 1:
        return deps[0]
    bits = _as(deps[0], u32)
    for d in deps[1:]:
        bits = bits | _as(d, u32)
    return bits


def _lhs_ops(a11, a12, a21, a22):
    return [a11 + a22, a21 + a22, a11, a22, a11 + a12, a21 - a11, a12 - a22]


SIDX = {0: 0, 2: 1, 3: 2, 5: 3, 6: 4}
TOP = {0: ((0, 0), 1, (1, 1)), 1: ((0, 0),), 2: ((0, 1), -1, (1, 1)), 3: ((1, 0), -1, (0, 0)),
       4: ((1, 1),), 5: ((0, 0), 1, (0, 1)), 6: ((1, 0), 1, (1, 1))}


def _rhs_sums(b11, b12, b21, b22):
    return {0: b11 + b22, 2: b12 - b22, 3: b21 - b11, 5: b11 + b12, 6: b21 + b22}


def _rhs_op(p, blk):
    t = TOP[p]
    if len(t) == 1:
        return blk(*t[0])
    return blk(*t[0]) + blk(*t[2]) if t[1] > 0 else blk(*t[0]) - blk(*t[2])


def _combine(m, n=None):
    c12 = lambda: m[2] + m[4]
    c21 = lambda: m[1] + m[3]
    x = lambda: (m[2] - m[1]) + m[0]
    c = [lambda: (x() + m[6]) + (c21() - c12()), c12, c21, lambda: x() + m[5]]
    return [f() for f in c] if n is None else c[n]()


def _kernel(x_hbm, wqkv_hbm, wo_hbm, w1_hbm, b1_hbm, w2_hbm, b2_hbm, out_hbm,
            x_v, wqkv_v, wo_v, w1_v, w2_v, b1_v, b2_v, out_v,
            wt_s, lw_s, wo_s, wq_s, xnT_s, ra_s, lh_s, um_s, lc_s, qk_s, v_s, pr_s, op_s,
            b2f_s, rs_s, ll_s, rr_s, ola_s, olb_s, one_s, sems):
    sem_ctr = [1]

    class Group:
        def __init__(self, pairs):
            self.cps = [pltpu.make_async_copy(a, b, sems.at[sem_ctr[0]]) for (a, b) in pairs]
            sem_ctr[0] += 1

        def start(self):
            for c in self.cps:
                c.start()

        def wait(self):
            for c in self.cps:
                c.wait()

    def cp_x(p0, p1):
        return [(x_hbm.at[0, :, pl.ds(p * 2 * LB, 2 * LB)], x_v.at[p]) for p in range(p0, p1)]

    def cp_w2(p0, p1):
        return [(w2_hbm.at[:, pl.ds(p * 2 * LB, 2 * LB)], w2_v.at[p]) for p in range(p0, p1)]

    def cp_w1(b0, b1, i0=0, i1=NFP):
        sl = pl.ds(b0 * LB, (b1 - b0) * LB)
        cl = pl.ds(i0 * 2 * LB, (i1 - i0) * 2 * LB)
        return [(w1_hbm.at[sl, cl], w1_v.at[sl, cl])]

    tl = []
    mxu = [0, 0, 0, 0]
    nxt = [0]
    hist = []
    tasks = []
    dls = []
    ready = set()
    pos = []
    true = {}

    def tie(v, z):
        if z is None:
            return v
        def fit(a):
            a = _cat([a] * (v.shape[0] // 8), 0)
            return a if v.shape[1] == LB else a[:, 0:v.shape[1]]
        if v.shape not in true:
            true[v.shape] = fit(pos[0]) > 0
        return lax.select(true[v.shape], v, fit(_as(z, v.dtype)))

    def tie8(v, z):
        return v if z is None else jnp.concatenate([tie(v[0:8], z), v[8:16]], axis=0)

    def add_tasks(todo):
        tasks.extend(todo)
        tasks.sort(key=lambda x: x[0])

    def flush(t=None):
        while tasks and (t is None or tasks[0][0] < t):
            _, fn, args = tasks.pop(0)
            fn(*args)

    def reset():
        assert not tasks
        dls.clear()
        tl.clear()
        hist.clear()
        mxu[:] = [0, 0, 0, 0]
        nxt[0] = 0

    def now():
        return sum(mxu) // 4

    def wait(name, *cps):
        flush()
        if SCOPES:
            with jax.named_scope("wait_" + name):
                for c in cps:
                    c.wait()
        else:
            for c in cps:
                c.wait()
        reset()

    def mm1(lhs, rhs, pace=True):
        flush(now())
        start = mxu[nxt[0]]
        due = [v for (t, v) in dls if t <= start] if pace else []
        if due:
            dls[:] = [(t, v) for (t, v) in dls if t > start]
            tile = _up(tie(pltpu.bitcast(lhs[0:16, 0:LB], u32), _token(*due)))
            row = tile if lhs.shape[1] == LB else jnp.concatenate([tile, lhs[0:16, LB:]], axis=1)
            lhs = jnp.concatenate([row, lhs[16:]], axis=0)
        r = jnp.dot(lhs, rhs, preferred_element_type=f32)
        m, k = lhs.shape
        first_done = None
        for _ in range(-(-rhs.shape[1] // LB)):
            end = 0
            for _ in range(-(-k // LB)):
                mxu[nxt[0]] += m
                end = max(end, mxu[nxt[0]])
                nxt[0] = (nxt[0] + 1) % 4
            if first_done is None:
                first_done = end
        if pace:
            tl.append((first_done - m, first_done, r))
        return r

    def mm(lhs, rhs, init=None):
        k = lhs.shape[1]
        r, k0 = init, 0
        while k0 < k:
            k1 = min(k, k0 + (4 - nxt[0]) * LB)
            part = mm1(lhs[:, k0:k1], rhs[k0:k1], pace=k1 - k0 > LB)
            r = part if r is None else r + part
            k0 = k1
        return r

    def at(t, *more):
        best = None
        if t is not None and t >= 0:
            t = min(t, now() - 1)
            for (a, b, r) in tl:
                if a <= t and (best is None or min(b, t) > best[0]):
                    row = int(min((t - a) / (b - a), 0.999) * (r.shape[0] // 8)) * 8
                    best = (min(b, t), r, row)
        return _token(None if best is None else best[1][best[2]:best[2] + 8, 0:LB], *more)

    def strassen(lhs, rhs, order, split_last=False, init=None, m=None):
        m = [None] * 7 if m is None else m
        for p in order:
            flush(now())
            l, r = lhs(p), rhs(p)
            c0 = None if init is None else init[p]
            if split_last and p == order[-1]:
                kk = (-(-r.shape[0] // LB) - 2) * LB
                hm = l.shape[0] // 2
                hd = mm(l[:, :kk], r[:kk], c0) if kk else c0
                tail = jnp.concatenate([mm(l[:hm, kk:], r[kk:]), mm(l[hm:, kk:], r[kk:])], axis=0)
                m[p] = tail if hd is None else hd + tail
            else:
                m[p] = mm(l, r, c0)
        return m

    def wcol(hh, p):
        return p * D + (1 - hh if p == 1 else hh) * HD

    def wrows(hh, g, z=None):
        p, d = divmod(2 * g, DH)
        t = [jnp.concatenate([wt_s[c, pl.ds(wcol(hh, p) + d + e, HH, stride=DH), :]
                              for e in range(2)], axis=0) for c in range(2)]
        return _unword(jnp.concatenate([tie(t[0], z), tie(t[1][:, 0:HD - LB], z)], axis=1))

    wt_done = set()

    def prep_wqkv(part, ga, gb, paced):
        def need(hh, p, z):
            lo = wcol(hh, p)
            for ct in range(lo // LB, -(-(lo + HD) // LB)):
                if ct in wt_done:
                    continue
                wt_done.add(ct)
                cols = slice(ct * LB, min((ct + 1) * LB, 3 * D))
                wd = _word(wqkv_v[0:HD, cols], wqkv_v[HD:D, cols])
                wd = jnp.concatenate([tie(wd[r:r + 8], z if r % LB == 0 else None) for r in range(0, HD, 8)], axis=0)
                wT = wd.T
                wt_s[0, cols, :] = wT[:, 0:LB]
                wt_s[1, cols, 0:HD - LB] = wT[:, LB:HD]

        def put(p, g, v):
            lw_s[p * (HA // 2) + g * 8:p * (HA // 2) + g * 8 + 8, :] = _pk(v)

        def half(hh, g0, g1, t0=None, dur=None):
            pr, ps = ((2, 4), (3, 1))[hh]
            for g in range(g0, g1):
                t = None if t0 is None else t0 + (g - g0) * dur // (g1 - g0)
                need(hh, 2 * g // DH, at(None if t is None else t - P["W2X"]))
                a1, a2 = wrows(hh, g, at(t))
                put(pr, g, a2 if hh else a1)
                put(ps, g, a1 + a2)
            if g1 == gb:
                ready.update({("lw", part, pr), ("lw", part, ps)})

        def rest(g0, g1, t0, dur):
            assert ("lw", part, 1) in ready
            for g in range(g0, g1):
                z = at(t0 + (g - g0) * dur // (g1 - g0))
                ops = _lhs_ops(*wrows(0, g, z), *wrows(1, g, z))
                for p in (0, 5, 6):
                    put(p, g, ops[p])
            if g1 == gb:
                ready.update({("lw", part, 0), ("lw", part, 5), ("lw", part, 6)})
        t2, d2, t3, d3 = paced
        half(0, ga, gb)
        n = (gb - ga) // 14
        add_tasks([(now() + t2 + (k + 1) * d2 // n, half,
                    (1, ga + 14 * k, ga + 14 * k + 14, now() + t2 + k * d2 // n, d2 // n)) for k in range(n)])
        n = (gb - ga) // 7
        add_tasks([(now() + t3 + (k + 1) * d3 // n, rest,
                    (ga + 7 * k, ga + 7 * k + 7, now() + t3 + k * d3 // n, d3 // n)) for k in range(n)])

    def prep_wo_a(t0, dur):
        for g in range(HD // 16):
            w = _word(wo_v[g * 16:g * 16 + 16, :], wo_v[HD + g * 16:HD + g * 16 + 16, :])
            z = at(t0 + g * dur // (HD // 16))
            for c in range(4):
                cw = min(LB, D - c * LB)
                wo_s[c, g * 16:g * 16 + 16, 0:cw] = tie(w[:, c * LB:c * LB + cw], z)
        ready.add("wo")

    def prep_wo_b(h, t0, dur):
        assert "wo" in ready
        for c in range(4):
            cw = min(LB, D - c * LB)
            rows = [wo_s[c, pl.ds(d, HH, stride=DH), :][:, 0:cw] for d in range(h * DH // 2, (h + 1) * DH // 2)]
            rows.append(jnp.zeros((LB - QD, cw), i32))
            wq_s[c * LB:c * LB + cw, _blk(h)] = jnp.concatenate(rows, axis=0).T
        outs = []
        for g in range(HD // 16):
            z = at(t0 + g * dur // (HD // 16))
            a = [v for r in (g * 16, HD + g * 16) for v in _unword(tie(wq_s[r:r + 16, _blk(h)], z))]
            for p, v in enumerate(_lhs_ops(*a)):
                lc_s[p * QD + g * 8:p * QD + g * 8 + 8, _blk(NFP + h)] = _pk(v)
                outs.append(v[0:8])
        ready.update({("lc", NFP + h, g) for g in range(HD // 16)})
        dls.append((t0 + dur + 250, _token(*outs)))

    RG = 16
    NG = D // RG
    stat2 = {}

    def ln(b, t0=None, dur=None):
        def xg(g):
            return x_v[b // 2, g * RG:(g + 1) * RG, _blk(b % 2)].astype(f32)

        def step(v, g, fr, s, q):
            if t0 is None or g % 4:
                return v
            acc = [] if s is None else [s[0:8], s[8:16], q[0:8], q[8:16]]
            return tie(v, at(t0 + fr * dur, *acc))

        x0 = jnp.broadcast_to(xg(0)[0:1], (8, LB))
        s = q = None
        for g in range(NG):
            x0 = step(x0, g, P["LNA"] * g / NG, s, q)
            c = xg(g) - _x2(x0)
            s = c if s is None else s + c
            q = c * c if q is None else q + c * c
        dm = _rowsum8(s) * (1.0 / D)
        mu = x0 + dm
        r1 = lax.rsqrt(jnp.maximum(_rowsum8(q) * (1.0 / D) - dm * dm, 0.0) + EPS)
        s = q = None
        for g in range(NG):
            mu = step(mu, g, P["LNB"] + P["LNBD"] * g / NG, s, q)
            xn = (xg(g) - _x2(mu)) * _x2(r1)
            xnT_s[g * 8:g * 8 + 8, _blk(b)] = _pk(xn)
            s = xn if s is None else s + xn
            q = xn * xn if q is None else q + xn * xn
        mu2 = _rowsum8(s) * (1.0 / D)
        var2 = jnp.maximum(_rowsum8(q) * (1.0 / D) - mu2 * mu2, 0.0)
        stat2[b] = (mu2, 0.5 * lax.rsqrt(var2 + EPS))

    def hpair(b, t0=None, dur=None):
        ng = HD // RG
        st = [stat2.pop(b), stat2.pop(b + 1)]
        for g in range(ng):
            zz = [at(None if t0 is None else t0 + (4 * g + k * P["SH4"]) * dur // (4 * ng)) for k in (0, 1, 2, 3)]
            xq = [_upf(tie(xnT_s[r:r + 8, _blk(b + e)], zz[2 * (r >= QD) + e]))
                  for r in (g * 8, QD + g * 8) for e in range(2)]
            hq = [(v - _x2(st[n % 2][0])) * _x2(st[n % 2][1]) for n, v in enumerate(xq)]
            ro = (b // 2) * QD + g * 8
            for p, v in _rhs_sums(*xq).items():
                ra_s[ro:ro + 8, _blk(SIDX[p])] = _pk(v)
            for p, v in enumerate(_lhs_ops(*hq)):
                lh_s[p * QD + g * 8:p * QD + g * 8 + 8, _blk(b // 2)] = _pk(v)
        ready.add(("xn", b))
        if b >= 6:
            got = ra_s[(b // 2) * QD:(b // 2 + 1) * QD, :]
            dls.append((t0 + dur + P["HL"], _token(*[got[r:r + 8, _blk(c)] for r in range(0, QD, 8) for c in range(5)])))

    def ln_tasks(b, t, lnd, hsd):
        for fn, bb, dur, adv in ((ln, b, lnd, P["LNV"]), (ln, b + 1, lnd, P["LNW"]), (hpair, b, hsd, 1.0)):
            add_tasks([(t + int(dur * adv), fn, (bb, t, dur))])
            t += int(dur * adv)
        return t

    def tsum(kp, i, slot_, n, t0, dur):
        for g in range(LB // 16):
            z, z2 = at(t0 + g * dur // 8), at(t0 + g * dur // 8 + P["SGT"])
            t1, t2 = [w1_v[(2 * kp + e) * LB + g * 16:(2 * kp + e) * LB + g * 16 + 16,
                           2 * i * LB:(2 * i + 2) * LB].astype(f32) for e in range(2)]
            ro = slot_ * RSK + n * (LB // 2) + g * 8
            for p, v in _rhs_sums(tie8(t1[:, :LB], z), t1[:, LB:], t2[:, :LB], tie8(t2[:, LB:], z2)).items():
                rs_s[ro:ro + 8, _blk(SIDX[p])] = _pk(v)
        ready.add(("rs", kp, i))

    def u_rhs(p, i, kps, slot_, n0):
        if p in SIDX:
            assert all(("rs", kp, i) in ready for kp in kps)
            ro = slot_ * RSK + n0 * (LB // 2)
            return _up(rs_s[ro:ro + len(kps) * (LB // 2), _blk(SIDX[p])])
        e = 0 if p == 1 else 1
        return _cat([w1_v[_blk(2 * kp + e), _blk(2 * i + e)] for kp in kps], 0)

    LATE = (NFP - 1, 6)

    def ujob(kp, i, p, split):
        flush(now())
        assert ("xn", 2 * kp) in ready
        l, r = _up(lh_s[p * QD:(p + 1) * QD, _blk(kp)]), u_rhs(p, i, [kp], 3 + kp, i)
        v = jnp.concatenate([mm1(l[:QD], r), mm1(l[QD:], r)], axis=0) if split else mm1(l, r)
        if p in (2, 3):
            v = v + 0.5 * b1_v[2 * i + 3 - p:2 * i + 4 - p, :].astype(f32)
        rows = slice(p * HD, (p + 1) * HD)
        um_s[rows, _blk(i)] = v

    def u_early(kp, i0, i1, carry, n, t0, dt, nsplit=0):
        for k, i in enumerate(range(i0, i1)):
            add_tasks([(t0 + (k + 1) * dt, tsum, (kp, i, 3 + kp, i, t0 + k * dt, dt))])
        jobs = (carry + [(kp, i, p) for i in range(i0, i1) for p in (1, 4)]
                + [(kp, i, p) for i in range(i0, i1) for p in SIDX if (i, p) != LATE])
        for c, job in enumerate(jobs[:n]):
            ujob(*job, c >= n - nsplit)
        return jobs[n:]

    def gelu_half(hx, z):
        c = 0.7978845608028654
        return hx + hx * jnp.tanh(tie(hx * (2.0 * c + (8.0 * c * 0.044715) * (hx * hx)), z))

    def u_epilogue(i, m, gs, t0, dur):
        for n, g in enumerate(gs):
            t = None if t0 is None else t0 + n * dur // len(gs) - P["UG"]
            q = _combine([x[g * 16:g * 16 + 16] for x in m])
            gl = [gelu_half(v, at(None if t is None else t - k * P["UM"])) for v, k in zip(q, (0, 3, 2, 1))]
            for p, v in enumerate(_lhs_ops(*gl)):
                lc_s[p * QD + g * 8:p * QD + g * 8 + 8, _blk(i)] = _pk(v)
            ready.add(("lc", i, g))

    def u_last(i, order, edur):
        kps = list(range(UB0 // 2, NP))
        m = strassen(lambda p: _up(lh_s[p * QD:(p + 1) * QD, (0 if (i, p) == LATE else UB0 // 2 * LB):]),
                     lambda p: _cat([u_rhs(p, i, [0], 3, i)] * ((i, p) == LATE) + [u_rhs(p, i, kps, i % 3, 0)], 0),
                     order, init=[None if (i, p) == LATE else um_s[p * HD:(p + 1) * HD, _blk(i)] for p in range(7)])
        if edur is None:
            u_epilogue(i, m, list(range(HD // 16)), None, None)
        else:
            t = now() + P["UE0"]
            add_tasks([(t + (g + 1) * edur // 7, u_epilogue, (i, m, [g, g + 7], t + g * edur // 7, edur // 7))
                       for g in range(7)])

    def llsum(qd, g, t0, dur):
        i0 = 2 * qd if qd < NQ else NFP
        assert all(("lc", i0 + e, g + 7 * h) in ready for e in range(2) for h in range(2))
        for p in range(7):
            zz = [at(t0 + p * dur // 7), at(t0 + p * dur // 7 + P["SGT"])]
            a = [tie(lc_s[p * QD + h * ED + g * 8:p * QD + h * ED + g * 8 + 8, _blk(i0 + e)], zz[h] if h == e else None)
                 for h in range(2) for e in range(2)]
            ops = _lhs_ops(*[_upf(v) for v in a])
            for q in (0, 1, 4, 5, 6):
                r = (p * 7 + q) * ED + g * 8
                ll_s[r:r + 8, _blk(qd)] = _pk(ops[q])
        ready.add(("ll", qd, g))

    AORD = (4, 2, 1, 3, 0, 5, 6)

    def stage_a(b, parts="qkv", order=AORD, split_last=False, m=None):
        r0, r1 = {"q": (0, HD), "kv": (HD, HA), "qkv": (0, HA)}[parts]

        def lhs(p):
            assert all(("lw", pt, p) in ready for pt in ("q", "kv") if pt in parts)
            return _up(lw_s[(p * HA + r0) // 2:(p * HA + r1) // 2, :])

        def rhs(p):
            assert ("xn", b) in ready
            if p in SIDX:
                return _up(ra_s[(b // 2) * QD:(b // 2 + 1) * QD, _blk(SIDX[p])])
            return _up(xnT_s[0:QD, _blk(b)] if p == 1 else xnT_s[QD:HD, _blk(b + 1)])
        m = strassen(lhs, rhs, order, split_last, m=m)
        for n, ps in enumerate((range(7), (2, 4), (1, 3), (0, 1, 2, 5))):
            if all(m[p] is not None for p in ps) and any(p in order for p in ps):
                hh, e = divmod(n, 2)
                c = _combine(m, n)
                qk_s[b + e, hh * D + r0:hh * D + min(r1, D), :] = c[0:min(r1, D) - r0]
                if r1 > D:
                    v_s[b + e + 1, hh * HD:(hh + 1) * HD, :] = c[D - r0:]
        if all(v is not None for v in m):
            ready.update({(pt, b + e) for pt in ("q", "kv") if pt in parts for e in range(2)})
        return m

    lane0 = lax.broadcasted_iota(i32, (HH, LB), 1)
    zeros8 = jnp.zeros((HH, LB), f32)

    def mk_shift(z):
        lane = tie(lane0, z)
        masks = {}

        def pick(n, a, b):
            if n not in masks:
                masks[n] = lane < n
            return lax.select(masks[n], a, b)

        def fwd(cur, prev, sh):
            return cur if sh == 0 else pltpu.roll(pick(LB - sh, cur, prev), sh, 1)

        def bwd(cur, nxt_):
            return pltpu.roll(pick(SH, nxt_, cur), LB - SH, 1)
        return fwd, bwd

    def grp_shift(t, bd):
        lag = max(2, -(-P["LAG"] * DH // (G * bd)))
        return mk_shift(at(t, *(hist[-lag] if len(hist) >= lag else [])))

    raw, probs = {}, {}

    def attn_qk(j, hh, t, bd):
        jn = min(j + 1, NB - 1)
        assert ("q", jn) in ready and ("kv", j) in ready
        acc = [None] * WH
        accp = [None] * WH
        for d in range(DH):
            if d % G == 0:
                if d > 0:
                    hist.append(acc + accp)
                fwd, bwd = grp_shift(t + d * bd // DH, bd)
            r = hh * D + d * HH
            q = qk_s[j, r:r + HH, :]
            qp = bwd(q, qk_s[jn, r:r + HH, :])
            rk = (1 - hh) * D + HD + d * HH
            k = qk_s[j, rk:rk + HH, :]
            kp = qk_s[j - 1, rk:rk + HH, :] if j > 0 else zeros8
            for a in range(WH):
                ks = fwd(k, kp, DIL * a)
                t0, t1 = q * ks, qp * ks
                acc[a] = t0 if d == 0 else acc[a] + t0
                accp[a] = t1 if d == 0 else accp[a] + t1
        hist.append(acc + accp)
        raw[j, hh] = (acc, accp)

    def attn_sm(j, hh, t):
        fwd, _ = mk_shift(at(t))
        acc, accp = raw[j, hh]
        prev = raw.pop((j - 1, hh))[1] if j > 0 else [zeros8] * WH
        lg = acc + [fwd(accp[a], prev[a], SH) for a in range(WH)]
        lg = [a * SCALE for a in lg]
        if j == 0:
            lg = [lg[0]] + [jnp.where(lane0 >= DIL * w, lg[w], -1e9) for w in range(1, W)]
        m = lg[0]
        for w in range(1, W):
            m = jnp.maximum(m, lg[w])
        e = [jnp.exp(l - m) for l in lg]
        den = e[0]
        for w in range(1, W):
            den = den + e[w]
        inv = 1.0 / den
        p = [x * inv for x in e]
        for a in range(WH):
            pr_s[j, (hh * W + a) * HH:(hh * W + a + 1) * HH, :] = p[a]
        probs[j, hh] = p[WH:]

    def attn_pp(j, hh, t):
        _, bwd = mk_shift(at(t))
        p = probs.pop((j, hh))
        pn = probs[j + 1, hh] if j + 1 < NB else p
        for a in range(WH):
            pr_s[j, (hh * W + WH + a) * HH:(hh * W + WH + a + 1) * HH, :] = bwd(p[a], pn[a])
        ready.add(("pr", j, hh))

    def attn_pv(j, hh, dst, e, t, bd):
        assert not isinstance(j, int) or ("pr", j, hh) in ready
        assert e == 0 or ("o", dst, hh, e - 1) in ready
        pa = [pr_s[j, (hh * W + a) * HH:(hh * W + a + 1) * HH, :] for a in range(W)]
        p, pp = pa[:WH], pa[WH:]
        outs = []
        for d in range(DH):
            if d % G == 0:
                if d > 0:
                    hist.append([])
                fwd, _ = grp_shift(t + d * bd // DH, bd)
            r = hh * HD + d * HH
            v = v_s[j + 1, r:r + HH, :]
            vp = v_s[j, r:r + HH, :]
            o = op = None
            for a in range(WH):
                vs = fwd(v, vp, DIL * a)
                o = p[a] * vs if a == 0 else o + p[a] * vs
                op = pp[a] * vs if a == 0 else op + pp[a] * vs
            opp = zeros8 if (isinstance(j, int) and j == 0) else op_s[r:r + HH, :]
            op_s[r:r + HH, :] = op
            outs.append(o + fwd(op, opp, SH))
            ol[dst][r:r + HH, _blk(e)] = outs[-1]
        hist.append([])
        ready.add(("o", dst, hh, e))
        dls.append((t + bd + P["PVL"], _token(*outs)))

    ol = [ola_s, olb_s]
    mains = [("qk", j, hh) for j in range(NB) for hh in range(2)]
    mains = (mains[:P["PVPOS"]] + [("pv", j, hh) for j in range(4) for hh in range(2)]
             + mains[P["PVPOS"]:] + [None, None])
    slot_ctr = [0]

    def slot(t, bd):
        n = slot_ctr[0]
        slot_ctr[0] += 1
        it = mains[n]
        if it is None:
            pass
        elif it[0] == "qk":
            attn_qk(it[1], it[2], t, bd)
        else:
            attn_pv(it[1], it[2], 0, it[1], t, bd)
        if n >= 1 and mains[n - 1] is not None and mains[n - 1][0] == "qk":
            attn_sm(mains[n - 1][1], mains[n - 1][2], t + P["LS"])
        if n >= 2 and mains[n - 2] is not None and mains[n - 2][0] == "qk":
            _, j, hh = mains[n - 2]
            if j > 0:
                attn_pp(j - 1, hh, t + P["PP"])
            if j == NB - 1:
                attn_pp(j, hh, t + P["PP"])

    NRG = 8 * (NQ + 1) + 7
    PD = 8 * QD
    BORD = (1, 3, 2, 4, 0, 5, 6)
    LORD = (2, 4, 1, 3, 0, 5, 6)
    LAST_PARTS = [(0, QD, 1, 2), (QD, HD, 0, 2), (0, QD, 0, 1)]

    def rr_prep(p, pa, src, n0, n1, t0, dur):
        assert ("rr", p) not in ready
        for n in range(n0, n1):
            z = at(t0 + (n - n0) * dur // (n1 - n0))
            z2 = at(t0 + (n - n0) * dur // (n1 - n0) + P["SGR"])
            qd, g = divmod(n, 8)

            def wrow(i):
                return _rhs_op(p, lambda x, y: w2_v[pa + y, (2 * i + x) * LB + g * 16:(2 * i + x) * LB + g * 16 + 16, :]
                               .astype(f32))

            def orow(h):
                def blk(x, y):
                    assert ("o", src, x, 2 * y + 1) in ready
                    r = x * HD + h * QD + g * 16
                    return ol[src][r:r + 16, y * 2 * LB:(y + 1) * 2 * LB]
                return _rhs_op(p, blk)
            ro = p * RRK + g * 8
            if qd == NQ:
                if p in SIDX:
                    r = wrow(2 * NQ)
                    for e in range(2):
                        rr_s[ro:ro + 8, _blk(7 + e)] = _pk(tie8(r[:, _blk(e)], z))
                continue
            r1, r2 = (wrow(2 * qd), wrow(2 * qd + 1)) if qd < NQ else (orow(0), orow(1))
            ro += min(qd, NQ) * (LB // 2)
            c11, c22 = tie8(r1[:, :LB], z), tie8(r2[:, LB:], z2)
            sm = _rhs_sums(c11, r1[:, LB:], r2[:, :LB], c22)
            if p in SIDX or qd > NQ:
                sm.update({1: c11, 4: c22})
            for q, v in sm.items():
                rr_s[ro:ro + 8, _blk(q)] = _pk(v)
        if n1 == NRG:
            ready.add(("rr", p))

    def rr_tasks(p, pa, src, t0, t1):
        cuts = list(range(0, NRG, 8)) + [NRG]
        acc, tot = 0, sum(P["RW"])
        for a, b, w in zip(cuts[:-1], cuts[1:], P["RW"]):
            ta, tb = t0 + acc * (t1 - t0) // tot, t0 + (acc + w) * (t1 - t0) // tot
            add_tasks([(tb, rr_prep, (p, pa, src, a, b, ta, tb - ta))])
            acc += w

    def out_copy(pidx, e0, e1, r0, r1):
        off = pidx * (2 * LB) + e0 * LB
        if not isinstance(pidx, int):
            off = pl.multiple_of(off, LB)
        rs = pl.ds(r0, r1 - r0)
        return pltpu.make_async_copy(out_v.at[pidx, rs, pl.ds(e0 * LB, (e1 - e0) * LB)],
                                     out_hbm.at[0, rs, pl.ds(off, (e1 - e0) * LB)], sems.at[0])

    def b_out(pa, n, m, part, t0=None, dur=None):
        a, y = divmod(n, 2)
        r0, r1, e0, e1 = part
        cols = slice(e0 * LB, e1 * LB)
        for r in range(r0, r1, 16):
            c = _combine([None if v is None else v[r:r + 16, cols] for v in m], n)
            rows = slice(a * HD + r, a * HD + r + 16)
            o = c + x_v[pa + y, rows, cols].astype(f32)
            if t0 is not None:
                o = jnp.concatenate([tie(o[:, 0:LB], at(t0 + (r - r0) * dur // (r1 - r0))), o[:, LB:]], axis=1)
            out_v[pa + y, rows, cols] = o.astype(bf16)
        out_copy(pa + y, e0, e1, a * HD + r0, a * HD + r1).start()

    def big_piece(pa, pan, cur, last):
        t0 = now()
        for n in range(7):
            ta, tb = t0 + n * PD + P["RR0"], t0 + n * PD + P["RR1"]
            if n < 6:
                rr_tasks(BORD[n + 1], pa, cur, ta, tb)
            else:
                rr_tasks(BORD[0], pan, 1 - cur, ta, tb - (P["RRM"] if last else 0))
        ready.difference_update({("o", 1 - cur, hh, e) for hh in range(2) for e in range(4)})
        for n in range(8):
            e, hh = divmod(n, 2)
            t = t0 + P["BV0"] + n * P["BVS"]
            add_tasks([(t + P["BVD"], attn_pv, (pan * 2 + e, hh, 1 - cur, e, t, P["BVD"]))])
        m = [None] * 7
        for p in BORD:
            flush(now())
            assert ("rr", p) in ready
            x, y = TOP[p][0]

            def lhs(q):
                if q in (2, 3):
                    rows = slice(p * QD + (q - 2) * ED, p * QD + (q - 1) * ED)
                    return _up(jnp.concatenate([lc_s[rows, _blk(2 * qd + q - 2)] for qd in range(NQ)]
                                               + [lc_s[rows, (NFP + q - 2) * LB:(NFP + q - 2) * LB + QD]], axis=1))
                return _up(ll_s[(p * 7 + q) * ED:(p * 7 + q + 1) * ED, 0:KL])

            def rhs(q):
                if p in SIDX or q in SIDX:
                    return _up(rr_s[p * RRK:p * RRK + KL // 2, _blk(q)])
                h = 0 if q == 1 else 1
                return _cat([w2_v[pa + y, _blk(2 * (2 * qd + h) + x), _blk(h)] for qd in range(NQ)]
                            + [_up(rr_s[p * RRK + NQ * LB // 2:p * RRK + KL // 2, _blk(q)])], 0)
            rl = (_up(rr_s[p * RRK:p * RRK + LB // 2, 7 * LB:9 * LB]) if p in SIDX
                  else w2_v[pa + y, _blk(4 * NQ + x), :])
            ll = _up(lc_s[p * QD:(p + 1) * QD, _blk(2 * NQ)])
            ex = [mm1(ll[:QD], rl), mm1(ll[QD:], rl)]
            e12, e21 = ex[0][:, LB:], ex[1][:, :LB]
            e11 = (ex[0][:, :LB] + e12) - e21
            lf = strassen(lhs, rhs, LORD)
            ready.discard(("rr", p))
            if p in (2, 3):
                for q in (2, 3):
                    lf[q] = lf[q] + b2f_s[pa + 3 - p, 0:1, _blk(3 - q)]
            c12 = (lf[2] + e12) + lf[4]
            c21 = (lf[1] + e21) + lf[3]
            xx = (lf[2] - lf[1]) + lf[0]
            c22 = (xx + ex[1][:, LB:]) + lf[5]
            c11 = ((xx + e11) + (c21 - c12)) + lf[6]
            m[p] = jnp.concatenate([jnp.concatenate([c11, c12], axis=1),
                                    jnp.concatenate([c21, c22], axis=1)], axis=0)
            n = {3: 2, 4: 1, 5: 3, 6: 0}.get(p)
            if n is not None and not (last and n == 0):
                t, epd = now() + P["EP0"], P["EPL"] if (last and n == 3) else P["EPD"]
                add_tasks([(t + epd, b_out, (pa, n, list(m), (0, HD, 0, 2), t, epd))])
        if last:
            flush()
            for part in LAST_PARTS:
                b_out(pa, 0, m, part)

    def c_body(it, carry):
        reset()
        pos[:] = [one_s[...]]
        true.clear()
        ready.update({("rr", BORD[0])} | {("o", 0, hh, e) for hh in range(2) for e in range(4)})
        big_piece(4 * it, 4 * it + 2, 0, False)
        big_piece(4 * it + 2, lax.rem(4 * it + 4, NP), 1, True)
        assert ("rr", BORD[0]) in ready and all(("o", 0, hh, 3) in ready for hh in range(2))
        return carry

    E1 = P["E1"]
    x0 = Group(cp_x(0, 1))
    g1 = Group([(b1_hbm, b1_v)] + cp_w1(0, 2, 0, E1))
    g2 = Group(cp_w1(0, 2, E1, NFP) + cp_x(1, 2))
    wq, wkv = [[(wqkv_hbm.at[:, cl], wqkv_v.at[:, cl])] for cl in (pl.ds(0, 4 * LB), pl.ds(4 * LB, 3 * D - 4 * LB))]
    g3 = Group(wq)
    g4 = Group(wkv + cp_x(2, 3))
    g5 = Group(cp_x(3, NP))
    g6 = Group(cp_w1(UB0, NB) + [(wo_hbm, wo_v), (b2_hbm, b2_v)] + cp_w2(0, 1))
    g7 = Group(cp_w2(1, NP))
    for c in (x0, g1, g2, g3, g4, g5, g6, g7):
        c.start()

    v_s[0] = jnp.zeros((D, LB), f32)
    for buf in (xnT_s, ra_s, lh_s, rs_s, rr_s, ola_s, olb_s, ll_s, lc_s):
        buf[0:8, 0:64] = jnp.zeros((8, 64), buf.dtype)

    wait("x0", x0)
    one_s[...] = lax.shift_right_logical(pltpu.bitcast(x_v[0, 0:16, 0:LB], i32), 1) | 1
    pos[:] = [one_s[...]]
    ln(0)
    ln(1)
    hpair(0)
    wait("r1", g1)
    jobs = u_early(0, 0, E1, [], 7 * E1 // 4 * 4, P["T1"], 100)
    wait("r2", g2)
    t, dt = P["L2T"], P["L2D"]
    add_tasks([(t + int((k + 1) * dt * P["LNV"]), ln, (2 + k, t + int(k * dt * P["LNV"]), dt)) for k in range(2)])
    jobs = u_early(0, E1, NFP, jobs, P["N2"], P["T2"], 100)
    wait("wq", g3)
    add_tasks([(P["H2T"] + P["H2D"], hpair, (2, P["H2T"], P["H2D"]))])
    u_early(0, 0, 0, jobs, len(jobs), 0, 1, nsplit=P["S3"])
    prep_wqkv("q", 0, HD // 16, [P[k] for k in ("QA", "QB", "QC", "QE")])
    stage_a(0, "q", split_last=True)
    m = stage_a(2, "q", AORD[:P["NA3"]])
    wait("wkv", g4)
    stage_a(2, "q", AORD[P["NA3"]:], split_last=True, m=m)
    prep_wqkv("kv", HD // 16, HA // 16, [P[k] for k in ("KA", "KB", "KC", "KE")])
    t = ln_tasks(4, now() + P["L4T"], P["LND"], P["HSD"])
    n4 = min(4, (now() + 14 * HD - P["MARG"] - t) // P["BD"])
    add_tasks([(t + (n + 1) * P["BD"], slot, (t + n * P["BD"], P["BD"])) for n in range(n4)])
    stage_a(0, "kv")
    stage_a(2, "kv", order=(6,) + AORD[:6])

    wait("mid", g5)
    AD = 7 * HA // 2
    t = P["L5T"]
    for b in range(6, NB, 2):
        t = ln_tasks(b, t, P["LND"], P["HSD"])
    n5 = ((NP - 2) * AD - P["MARG"] - t) // P["BD"]
    add_tasks([(t + (n + 1) * P["BD"], slot, (t + n * P["BD"], P["BD"])) for n in range(n5)])
    n5 += n4
    for n, b in enumerate(range(4, NB, 2)):
        stage_a(b, order=(6,) + AORD[:6] if n % 2 else AORD)

    wait("fin", g6)
    UD = 7 * NUP * HD // 4
    for i in range(NFP):
        t0, dt = (-200, 130) if i == 0 else (800, 270) if i == 1 else ((i - 1) * UD + P["US0"], P["USD"])
        add_tasks([(t0 + (k + 1) * dt, tsum, (UB0 // 2 + k, i, i % 3, k, t0 + k * dt, dt)) for k in range(NUP)])
    left = len(mains) - n5 - 2
    bd = (NFP * UD - P["R6E"] - P["R6S"]) // left
    add_tasks([(P["R6S"] + (n + 1) * bd, slot, (P["R6S"] + n * bd, bd)) for n in range(left)])
    t = P["R6S"] + left * bd
    add_tasks([(t + (n + 1) * 300, slot, (t + n * 300, 300)) for n in range(2)])
    for qd, t0, t1 in ((NQ, UD + P["LL0"], 3 * UD), (0, 3 * UD + P["LL0"], 5 * UD), (1, 5 * UD + P["LL0"], 6 * UD + 200),
                       (2, 6 * UD + P["LL2"], 6 * UD + P["LL2"] + P["UEL"])):
        dt = (t1 - t0) // 7
        add_tasks([(t0 + (g + 1) * dt, llsum, (qd, g, t0 + g * dt, dt)) for g in range(7)])
    rr_tasks(BORD[0], 0, 0, P["RP0"], P["RP1"])
    add_tasks([(P["PW0"] + P["PWD"], prep_wo_a, (P["PW0"], P["PWD"]))])
    add_tasks([(P["PW1"] + (h + 1) * P["PWE"], prep_wo_b, (h, P["PW1"] + h * P["PWE"], P["PWE"])) for h in range(2)])
    for b in range(NB):
        b2f_s[b // 2, 0:1, _blk(b % 2)] = b2_v[b:b + 1, :].astype(f32)
    for i in range(NFP):
        u_last(i, (1, 4, 2, 3, 0, 5, 6) if i == 0 else (4, 2, 1, 3, 0, 5, 6),
               None if i == NFP - 1 else P["UEL"] if i == NFP - 2 else P["UED"])
    flush()
    assert slot_ctr[0] == len(mains) and all(("ll", qd, g) in ready for qd in range(NQ + 1) for g in range(7))
    assert all(("pr", j, hh) in ready for j in range(NB) for hh in range(2)) and ("rr", BORD[0]) in ready

    wait("w2", g7)
    lax.fori_loop(0, NP // 4, c_body, 0)
    outs = []
    for pa in range(0, NP, 2):
        outs += [out_copy(pa + n % 2, 0, 2, n // 2 * HD, (n // 2 + 1) * HD) for n in (1, 2, 3)]
        outs += [out_copy(pa, e0, e1, r0, r1) for (r0, r1, e0, e1) in (LAST_PARTS if pa % 4 else [(0, HD, 0, 2)])]
    wait("out", *outs)


@jax.jit
def pallas_parallel_sum__sliding_local_dilated__mixer_token_mlp__prompt_kernel(A_x, A_wqkv, A_wo, B_x, B_w1, B_b1, B_w2, B_b2):
    del B_x
    hbm = pl.BlockSpec(memory_space=pltpu.HBM)
    outT = pl.pallas_call(
        _kernel,
        out_shape=jax.ShapeDtypeStruct((1, D, S), bf16),
        in_specs=[hbm] * 7,
        out_specs=hbm,
        scratch_shapes=[
            pltpu.VMEM((NP, D, 2 * LB), bf16),
            pltpu.VMEM((D, 3 * D), bf16),
            pltpu.VMEM((D, D), bf16),
            pltpu.VMEM((S, F), bf16),
            pltpu.VMEM((NP, F, 2 * LB), bf16),
            pltpu.VMEM((NFB, LB), bf16),
            pltpu.VMEM((NB, LB), bf16),
            pltpu.VMEM((NP, D, 2 * LB), bf16),
            pltpu.VMEM((2, 3 * D + 64, LB), i32),
            pltpu.VMEM((7 * HA // 2, HD), u32),
            pltpu.VMEM((4, HD + 32, LB), i32),
            pltpu.VMEM((D, 2 * LB), i32),
            pltpu.VMEM((HD, S), u32),
            pltpu.VMEM((NP * QD, 5 * LB), u32),
            pltpu.VMEM((7 * QD, NP * LB), u32),
            pltpu.VMEM((7 * HD, NFP * LB), f32),
            pltpu.VMEM((7 * QD, (NFP + 2) * LB), u32),
            pltpu.VMEM((NB, 2 * D, LB), f32),
            pltpu.VMEM((NB + 1, D, LB), f32),
            pltpu.VMEM((NB, 2 * W * HH, LB), f32),
            pltpu.VMEM((D, LB), f32),
            pltpu.VMEM((NP, 32, 2 * LB), f32),
            pltpu.VMEM((4 * RSK, 5 * LB), u32),
            pltpu.VMEM((49 * ED, 4 * LB), u32),
            pltpu.VMEM((7 * RRK, 9 * LB), u32),
            pltpu.VMEM((D, 4 * LB), f32),
            pltpu.VMEM((D, 4 * LB), f32),
            pltpu.VMEM((8, LB), i32),
            pltpu.SemaphoreType.DMA((9,)),
        ],
        compiler_params=pltpu.CompilerParams(vmem_limit_bytes=100 * 1024 * 1024,
                                             disable_bounds_checks=True,
                                             disable_semaphore_checks=True),
    )(jnp.swapaxes(A_x, 1, 2), A_wqkv, A_wo, B_w1, B_b1.reshape(NFB, LB), B_w2, B_b2.reshape(NB, LB))
    return jnp.swapaxes(outT, 1, 2)
```

```python
import jax
import jax.numpy as jnp
from jax import lax
import jax.experimental.pallas as pl
import jax.experimental.pallas.tpu as pltpu

S, D, F = 2048, 448, 1792
H, DH, W, DIL = 16, 28, 8, 2
LB = 128
NB = S // LB
NP = NB // 2
NFB = F // LB
NFP = NFB // 2
HH = H // 2
WH = W // 2
SH = DIL * WH
HD = D // 2
QD = D // 4
ED = D // 8
HA = 3 * HD
UB0 = 2
NUP = (NB - UB0) // 2
RSK = NFP * LB // 2
NQ = NFP // 2
KL = NQ * LB + QD
RRK = 2 * LB
EPS = 1e-5
EPS_BF16 = 1.0013580322265625e-05
SCALE = DH ** -0.5
f32 = jnp.float32
bf16 = jnp.bfloat16
u32 = jnp.uint32
i32 = jnp.int32

SCOPES = False
P = dict(
    E1=3, N2=16, NA3=2, T1=-200, T2=-200, S3=0, L2T=100, L2D=440, H2T=900, H2D=360, L4T=1000, L5T=60, W2X=500,
    QA=-410, QB=200, QC=-200, QE=330, KA=50, KB=320, KC=450, KE=390,
    LND=420, HSD=360, HL=300, LNA=0.28, LNB=0.46, LNBD=0.38, LNV=0.86, LNW=0.93,
    BD=370, MARG=300, LAG=200, LS=150, PP=130, PVL=500, PVPOS=12,
    US0=100, USD=360, UE0=240, UED=2320, UEL=1700, UG=70, UM=0, R6S=1750, R6E=3150,
    LL0=300, LL2=550, RP0=16600, RP1=18700, PW0=560, PWD=300, PW1=1380, PWE=400,
    RR0=-48, RR1=800, RRM=-20, RW=(8, 8, 8, 2, 7), BV0=117, BVS=717, BVD=620, EP0=0, EPD=864, EPL=290, SGR=8, SGT=8, SH4=1,
)
G = 4


def _as(x, dtype):
    return x if x.dtype == dtype else pltpu.bitcast(x, dtype)


def _pk(x):
    return pltpu.bitcast(x.astype(bf16), u32)


def _up(x):
    return pltpu.bitcast(x, bf16)


def _upf(x):
    return pltpu.bitcast(x, bf16).astype(f32)


def _rb(x):
    return x.astype(bf16).astype(f32)


def _word(lo, hi):
    lo, hi = [pltpu.bitcast(v.astype(f32), i32) for v in (lo, hi)]
    return lax.shift_right_logical(lo, 16) | hi


def _unword(w):
    return [pltpu.bitcast(w << 16, f32), pltpu.bitcast(w & -65536, f32)]


def _cat(xs, axis):
    return xs[0] if len(xs) == 1 else jnp.concatenate(xs, axis=axis)


def _x2(v):
    return jnp.concatenate([v, v], axis=0)


def _blk(b):
    return slice(b * LB, (b + 1) * LB)


def _rowsum8(a):
    return jnp.broadcast_to(jnp.sum(a, axis=0, keepdims=True), (8, a.shape[1]))


def _token(*deps):
    deps = [d for d in deps if d is not None]
    if not deps:
        return None
    if len(deps) == 1:
        return deps[0]
    bits = _as(deps[0], u32)
    for d in deps[1:]:
        bits = bits | _as(d, u32)
    return bits


def _lhs_ops(a11, a12, a21, a22):
    return [a11 + a22, a21 + a22, a11, a22, a11 + a12, a21 - a11, a12 - a22]


SIDX = {0: 0, 2: 1, 3: 2, 5: 3, 6: 4}
TOP = {0: ((0, 0), 1, (1, 1)), 1: ((0, 0),), 2: ((0, 1), -1, (1, 1)), 3: ((1, 0), -1, (0, 0)),
       4: ((1, 1),), 5: ((0, 0), 1, (0, 1)), 6: ((1, 0), 1, (1, 1))}


def _rhs_sums(b11, b12, b21, b22):
    return {0: b11 + b22, 2: b12 - b22, 3: b21 - b11, 5: b11 + b12, 6: b21 + b22}


def _rhs_op(p, blk):
    t = TOP[p]
    if len(t) == 1:
        return blk(*t[0])
    return blk(*t[0]) + blk(*t[2]) if t[1] > 0 else blk(*t[0]) - blk(*t[2])


def _combine(m, n=None):
    c12 = lambda: m[2] + m[4]
    c21 = lambda: m[1] + m[3]
    x = lambda: (m[2] - m[1]) + m[0]
    c = [lambda: (x() + m[6]) + (c21() - c12()), c12, c21, lambda: x() + m[5]]
    return [f() for f in c] if n is None else c[n]()


def _kernel(x_hbm, wqkv_hbm, wo_hbm, w1_hbm, b1_hbm, w2_hbm, b2_hbm, out_hbm,
            x_v, wqkv_v, wo_v, w1_v, w2_v, b1_v, b2_v, out_v,
            wt_s, lw_s, wo_s, wq_s, xnT_s, ra_s, lh_s, um_s, lc_s, qk_s, v_s, pr_s, op_s,
            b2f_s, rs_s, ll_s, rr_s, ola_s, olb_s, one_s, sems):
    sem_ctr = [1]

    class Group:
        def __init__(self, pairs):
            self.cps = [pltpu.make_async_copy(a, b, sems.at[sem_ctr[0]]) for (a, b) in pairs]
            sem_ctr[0] += 1

        def start(self):
            for c in self.cps:
                c.start()

        def wait(self):
            for c in self.cps:
                c.wait()

    def cp_x(p0, p1):
        return [(x_hbm.at[0, :, pl.ds(p * 2 * LB, 2 * LB)], x_v.at[p]) for p in range(p0, p1)]

    def cp_w2(p0, p1):
        return [(w2_hbm.at[:, pl.ds(p * 2 * LB, 2 * LB)], w2_v.at[p]) for p in range(p0, p1)]

    def cp_w1(b0, b1, i0=0, i1=NFP):
        sl = pl.ds(b0 * LB, (b1 - b0) * LB)
        cl = pl.ds(i0 * 2 * LB, (i1 - i0) * 2 * LB)
        return [(w1_hbm.at[sl, cl], w1_v.at[sl, cl])]

    tl = []
    mxu = [0, 0, 0, 0]
    nxt = [0]
    hist = []
    tasks = []
    dls = []
    ready = set()
    pos = []
    true = {}

    def tie(v, z):
        if z is None:
            return v
        def fit(a):
            a = _cat([a] * (v.shape[0] // 8), 0)
            return a if v.shape[1] == LB else a[:, 0:v.shape[1]]
        if v.shape not in true:
            true[v.shape] = fit(pos[0]) > 0
        return lax.select(true[v.shape], v, fit(_as(z, v.dtype)))

    def tie8(v, z):
        return v if z is None else jnp.concatenate([tie(v[0:8], z), v[8:16]], axis=0)

    def add_tasks(todo):
        tasks.extend(todo)
        tasks.sort(key=lambda x: x[0])

    def flush(t=None):
        while tasks and (t is None or tasks[0][0] < t):
            _, fn, args = tasks.pop(0)
            fn(*args)

    def reset():
        assert not tasks
        dls.clear()
        tl.clear()
        hist.clear()
        mxu[:] = [0, 0, 0, 0]
        nxt[0] = 0

    def now():
        return sum(mxu) // 4

    def wait(name, *cps):
        flush()
        if SCOPES:
            with jax.named_scope("wait_" + name):
                for c in cps:
                    c.wait()
        else:
            for c in cps:
                c.wait()
        reset()

    def mm1(lhs, rhs, pace=True):
        flush(now())
        start = mxu[nxt[0]]
        due = [v for (t, v) in dls if t <= start] if pace else []
        if due:
            dls[:] = [(t, v) for (t, v) in dls if t > start]
            tile = _up(tie(pltpu.bitcast(lhs[0:16, 0:LB], u32), _token(*due)))
            row = tile if lhs.shape[1] == LB else jnp.concatenate([tile, lhs[0:16, LB:]], axis=1)
            lhs = jnp.concatenate([row, lhs[16:]], axis=0)
        r = jnp.dot(lhs, rhs, preferred_element_type=f32)
        m, k = lhs.shape
        first_done = None
        for _ in range(-(-rhs.shape[1] // LB)):
            end = 0
            for _ in range(-(-k // LB)):
                mxu[nxt[0]] += m
                end = max(end, mxu[nxt[0]])
                nxt[0] = (nxt[0] + 1) % 4
            if first_done is None:
                first_done = end
        if pace:
            tl.append((first_done - m, first_done, r))
        return r

    def mm(lhs, rhs, init=None):
        k = lhs.shape[1]
        r, k0 = init, 0
        while k0 < k:
            k1 = min(k, k0 + (4 - nxt[0]) * LB)
            part = mm1(lhs[:, k0:k1], rhs[k0:k1], pace=k1 - k0 > LB)
            r = part if r is None else r + part
            k0 = k1
        return r

    def at(t, *more):
        best = None
        if t is not None and t >= 0:
            t = min(t, now() - 1)
            for (a, b, r) in tl:
                if a <= t and (best is None or min(b, t) > best[0]):
                    row = int(min((t - a) / (b - a), 0.999) * (r.shape[0] // 8)) * 8
                    best = (min(b, t), r, row)
        return _token(None if best is None else best[1][best[2]:best[2] + 8, 0:LB], *more)

    def strassen(lhs, rhs, order, split_last=False, init=None, m=None):
        m = [None] * 7 if m is None else m
        for p in order:
            flush(now())
            l, r = lhs(p), rhs(p)
            c0 = None if init is None else init[p]
            if split_last and p == order[-1]:
                kk = (-(-r.shape[0] // LB) - 2) * LB
                hm = l.shape[0] // 2
                hd = mm(l[:, :kk], r[:kk], c0) if kk else c0
                tail = jnp.concatenate([mm(l[:hm, kk:], r[kk:]), mm(l[hm:, kk:], r[kk:])], axis=0)
                m[p] = tail if hd is None else hd + tail
            else:
                m[p] = mm(l, r, c0)
        return m

    def wcol(hh, p):
        return p * D + (1 - hh if p == 1 else hh) * HD

    def wrows(hh, g, z=None):
        p, d = divmod(2 * g, DH)
        t = [jnp.concatenate([wt_s[c, pl.ds(wcol(hh, p) + d + e, HH, stride=DH), :]
                              for e in range(2)], axis=0) for c in range(2)]
        return _unword(jnp.concatenate([tie(t[0], z), tie(t[1][:, 0:HD - LB], z)], axis=1))

    wt_done = set()

    def prep_wqkv(part, ga, gb, paced):
        def need(hh, p, z):
            lo = wcol(hh, p)
            for ct in range(lo // LB, -(-(lo + HD) // LB)):
                if ct in wt_done:
                    continue
                wt_done.add(ct)
                cols = slice(ct * LB, min((ct + 1) * LB, 3 * D))
                wd = _word(wqkv_v[0:HD, cols], wqkv_v[HD:D, cols])
                wd = jnp.concatenate([tie(wd[r:r + 8], z if r % LB == 0 else None) for r in range(0, HD, 8)], axis=0)
                wT = wd.T
                wt_s[0, cols, :] = wT[:, 0:LB]
                wt_s[1, cols, 0:HD - LB] = wT[:, LB:HD]

        def put(p, g, v):
            lw_s[p * (HA // 2) + g * 8:p * (HA // 2) + g * 8 + 8, :] = _pk(v)

        def half(hh, g0, g1, t0=None, dur=None):
            pr, ps = ((2, 4), (3, 1))[hh]
            for g in range(g0, g1):
                t = None if t0 is None else t0 + (g - g0) * dur // (g1 - g0)
                need(hh, 2 * g // DH, at(None if t is None else t - P["W2X"]))
                a1, a2 = wrows(hh, g, at(t))
                put(pr, g, a2 if hh else a1)
                put(ps, g, a1 + a2)
            if g1 == gb:
                ready.update({("lw", part, pr), ("lw", part, ps)})

        def rest(g0, g1, t0, dur):
            assert ("lw", part, 1) in ready
            for g in range(g0, g1):
                z = at(t0 + (g - g0) * dur // (g1 - g0))
                ops = _lhs_ops(*wrows(0, g, z), *wrows(1, g, z))
                for p in (0, 5, 6):
                    put(p, g, ops[p])
            if g1 == gb:
                ready.update({("lw", part, 0), ("lw", part, 5), ("lw", part, 6)})
        t2, d2, t3, d3 = paced
        half(0, ga, gb)
        n = (gb - ga) // 14
        add_tasks([(now() + t2 + (k + 1) * d2 // n, half,
                    (1, ga + 14 * k, ga + 14 * k + 14, now() + t2 + k * d2 // n, d2 // n)) for k in range(n)])
        n = (gb - ga) // 7
        add_tasks([(now() + t3 + (k + 1) * d3 // n, rest,
                    (ga + 7 * k, ga + 7 * k + 7, now() + t3 + k * d3 // n, d3 // n)) for k in range(n)])

    def prep_wo_a(t0, dur):
        for g in range(HD // 16):
            w = _word(wo_v[g * 16:g * 16 + 16, :], wo_v[HD + g * 16:HD + g * 16 + 16, :])
            z = at(t0 + g * dur // (HD // 16))
            for c in range(4):
                cw = min(LB, D - c * LB)
                wo_s[c, g * 16:g * 16 + 16, 0:cw] = tie(w[:, c * LB:c * LB + cw], z)
        ready.add("wo")

    def prep_wo_b(h, t0, dur):
        assert "wo" in ready
        for c in range(4):
            cw = min(LB, D - c * LB)
            rows = [wo_s[c, pl.ds(d, HH, stride=DH), :][:, 0:cw] for d in range(h * DH // 2, (h + 1) * DH // 2)]
            rows.append(jnp.zeros((LB - QD, cw), i32))
            wq_s[c * LB:c * LB + cw, _blk(h)] = jnp.concatenate(rows, axis=0).T
        outs = []
        for g in range(HD // 16):
            z = at(t0 + g * dur // (HD // 16))
            a = [v for r in (g * 16, HD + g * 16) for v in _unword(tie(wq_s[r:r + 16, _blk(h)], z))]
            for p, v in enumerate(_lhs_ops(*a)):
                lc_s[p * QD + g * 8:p * QD + g * 8 + 8, _blk(NFP + h)] = _pk(v)
                outs.append(v[0:8])
        ready.update({("lc", NFP + h, g) for g in range(HD // 16)})
        dls.append((t0 + dur + 250, _token(*outs)))

    RG = 16
    NG = D // RG
    stat2 = {}

    def ln(b, t0=None, dur=None):
        def xg(g):
            return x_v[b // 2, g * RG:(g + 1) * RG, _blk(b % 2)].astype(f32)

        def step(v, g, fr, s, q):
            if t0 is None or g % 4:
                return v
            acc = [] if s is None else [s[0:8], s[8:16], q[0:8], q[8:16]]
            return tie(v, at(t0 + fr * dur, *acc))

        x0 = jnp.broadcast_to(xg(0)[0:1], (8, LB))
        s = q = None
        for g in range(NG):
            x0 = step(x0, g, P["LNA"] * g / NG, s, q)
            c = xg(g) - _x2(x0)
            s = c if s is None else s + c
            q = c * c if q is None else q + c * c
        dm = _rowsum8(s) * (1.0 / D)
        mu = _rb(x0 + dm)
        var = _rb(jnp.maximum(_rowsum8(q) * (1.0 / D) - dm * dm, 0.0))
        r1 = 1.0 / _rb(jnp.sqrt(_rb(var + EPS_BF16)))
        s = q = None
        for g in range(NG):
            mu = step(mu, g, P["LNB"] + P["LNBD"] * g / NG, s, q)
            xn = _rb(xg(g) - _x2(mu)) * _x2(r1)
            xnT_s[g * 8:g * 8 + 8, _blk(b)] = _pk(xn)
            s = xn if s is None else s + xn
            q = xn * xn if q is None else q + xn * xn
        mu2 = _rowsum8(s) * (1.0 / D)
        var2 = jnp.maximum(_rowsum8(q) * (1.0 / D) - mu2 * mu2, 0.0)
        stat2[b] = (mu2, 0.5 * lax.rsqrt(var2 + EPS))

    def hpair(b, t0=None, dur=None):
        ng = HD // RG
        st = [stat2.pop(b), stat2.pop(b + 1)]
        for g in range(ng):
            zz = [at(None if t0 is None else t0 + (4 * g + k * P["SH4"]) * dur // (4 * ng)) for k in (0, 1, 2, 3)]
            xq = [_upf(tie(xnT_s[r:r + 8, _blk(b + e)], zz[2 * (r >= QD) + e]))
                  for r in (g * 8, QD + g * 8) for e in range(2)]
            hq = [(v - _x2(st[n % 2][0])) * _x2(st[n % 2][1]) for n, v in enumerate(xq)]
            ro = (b // 2) * QD + g * 8
            for p, v in _rhs_sums(*xq).items():
                ra_s[ro:ro + 8, _blk(SIDX[p])] = _pk(v)
            for p, v in enumerate(_lhs_ops(*hq)):
                lh_s[p * QD + g * 8:p * QD + g * 8 + 8, _blk(b // 2)] = _pk(v)
        ready.add(("xn", b))
        if b >= 6:
            got = ra_s[(b // 2) * QD:(b // 2 + 1) * QD, :]
            dls.append((t0 + dur + P["HL"], _token(*[got[r:r + 8, _blk(c)] for r in range(0, QD, 8) for c in range(5)])))

    def ln_tasks(b, t, lnd, hsd):
        for fn, bb, dur, adv in ((ln, b, lnd, P["LNV"]), (ln, b + 1, lnd, P["LNW"]), (hpair, b, hsd, 1.0)):
            add_tasks([(t + int(dur * adv), fn, (bb, t, dur))])
            t += int(dur * adv)
        return t

    def tsum(kp, i, slot_, n, t0, dur):
        for g in range(LB // 16):
            z, z2 = at(t0 + g * dur // 8), at(t0 + g * dur // 8 + P["SGT"])
            t1, t2 = [w1_v[(2 * kp + e) * LB + g * 16:(2 * kp + e) * LB + g * 16 + 16,
                           2 * i * LB:(2 * i + 2) * LB].astype(f32) for e in range(2)]
            ro = slot_ * RSK + n * (LB // 2) + g * 8
            for p, v in _rhs_sums(tie8(t1[:, :LB], z), t1[:, LB:], t2[:, :LB], tie8(t2[:, LB:], z2)).items():
                rs_s[ro:ro + 8, _blk(SIDX[p])] = _pk(v)
        ready.add(("rs", kp, i))

    def u_rhs(p, i, kps, slot_, n0):
        if p in SIDX:
            assert all(("rs", kp, i) in ready for kp in kps)
            ro = slot_ * RSK + n0 * (LB // 2)
            return _up(rs_s[ro:ro + len(kps) * (LB // 2), _blk(SIDX[p])])
        e = 0 if p == 1 else 1
        return _cat([w1_v[_blk(2 * kp + e), _blk(2 * i + e)] for kp in kps], 0)

    LATE = (NFP - 1, 6)

    def ujob(kp, i, p, split):
        flush(now())
        assert ("xn", 2 * kp) in ready
        l, r = _up(lh_s[p * QD:(p + 1) * QD, _blk(kp)]), u_rhs(p, i, [kp], 3 + kp, i)
        v = jnp.concatenate([mm1(l[:QD], r), mm1(l[QD:], r)], axis=0) if split else mm1(l, r)
        if p in (2, 3):
            v = v + 0.5 * b1_v[2 * i + 3 - p:2 * i + 4 - p, :].astype(f32)
        rows = slice(p * HD, (p + 1) * HD)
        um_s[rows, _blk(i)] = v

    def u_early(kp, i0, i1, carry, n, t0, dt, nsplit=0):
        for k, i in enumerate(range(i0, i1)):
            add_tasks([(t0 + (k + 1) * dt, tsum, (kp, i, 3 + kp, i, t0 + k * dt, dt))])
        jobs = (carry + [(kp, i, p) for i in range(i0, i1) for p in (1, 4)]
                + [(kp, i, p) for i in range(i0, i1) for p in SIDX if (i, p) != LATE])
        for c, job in enumerate(jobs[:n]):
            ujob(*job, c >= n - nsplit)
        return jobs[n:]

    def gelu_half(hx, z):
        c = 0.7978845608028654
        return hx + hx * jnp.tanh(tie(hx * (2.0 * c + (8.0 * c * 0.044715) * (hx * hx)), z))

    def u_epilogue(i, m, gs, t0, dur):
        for n, g in enumerate(gs):
            t = None if t0 is None else t0 + n * dur // len(gs) - P["UG"]
            q = _combine([x[g * 16:g * 16 + 16] for x in m])
            gl = [gelu_half(v, at(None if t is None else t - k * P["UM"])) for v, k in zip(q, (0, 3, 2, 1))]
            for p, v in enumerate(_lhs_ops(*gl)):
                lc_s[p * QD + g * 8:p * QD + g * 8 + 8, _blk(i)] = _pk(v)
            ready.add(("lc", i, g))

    def u_last(i, order, edur):
        kps = list(range(UB0 // 2, NP))
        m = strassen(lambda p: _up(lh_s[p * QD:(p + 1) * QD, (0 if (i, p) == LATE else UB0 // 2 * LB):]),
                     lambda p: _cat([u_rhs(p, i, [0], 3, i)] * ((i, p) == LATE) + [u_rhs(p, i, kps, i % 3, 0)], 0),
                     order, init=[None if (i, p) == LATE else um_s[p * HD:(p + 1) * HD, _blk(i)] for p in range(7)])
        if edur is None:
            u_epilogue(i, m, list(range(HD // 16)), None, None)
        else:
            t = now() + P["UE0"]
            add_tasks([(t + (g + 1) * edur // 7, u_epilogue, (i, m, [g, g + 7], t + g * edur // 7, edur // 7))
                       for g in range(7)])

    def llsum(qd, g, t0, dur):
        i0 = 2 * qd if qd < NQ else NFP
        assert all(("lc", i0 + e, g + 7 * h) in ready for e in range(2) for h in range(2))
        for p in range(7):
            zz = [at(t0 + p * dur // 7), at(t0 + p * dur // 7 + P["SGT"])]
            a = [tie(lc_s[p * QD + h * ED + g * 8:p * QD + h * ED + g * 8 + 8, _blk(i0 + e)], zz[h] if h == e else None)
                 for h in range(2) for e in range(2)]
            ops = _lhs_ops(*[_upf(v) for v in a])
            for q in (0, 1, 4, 5, 6):
                r = (p * 7 + q) * ED + g * 8
                ll_s[r:r + 8, _blk(qd)] = _pk(ops[q])
        ready.add(("ll", qd, g))

    AORD = (4, 2, 1, 3, 0, 5, 6)

    def stage_a(b, parts="qkv", order=AORD, split_last=False, m=None):
        r0, r1 = {"q": (0, HD), "kv": (HD, HA), "qkv": (0, HA)}[parts]

        def lhs(p):
            assert all(("lw", pt, p) in ready for pt in ("q", "kv") if pt in parts)
            return _up(lw_s[(p * HA + r0) // 2:(p * HA + r1) // 2, :])

        def rhs(p):
            assert ("xn", b) in ready
            if p in SIDX:
                return _up(ra_s[(b // 2) * QD:(b // 2 + 1) * QD, _blk(SIDX[p])])
            return _up(xnT_s[0:QD, _blk(b)] if p == 1 else xnT_s[QD:HD, _blk(b + 1)])
        m = strassen(lhs, rhs, order, split_last, m=m)
        for n, ps in enumerate((range(7), (2, 4), (1, 3), (0, 1, 2, 5))):
            if all(m[p] is not None for p in ps) and any(p in order for p in ps):
                hh, e = divmod(n, 2)
                c = _combine(m, n)
                qk_s[b + e, hh * D + r0:hh * D + min(r1, D), :] = c[0:min(r1, D) - r0]
                if r1 > D:
                    v_s[b + e + 1, hh * HD:(hh + 1) * HD, :] = c[D - r0:]
        if all(v is not None for v in m):
            ready.update({(pt, b + e) for pt in ("q", "kv") if pt in parts for e in range(2)})
        return m

    lane0 = lax.broadcasted_iota(i32, (HH, LB), 1)
    zeros8 = jnp.zeros((HH, LB), f32)

    def mk_shift(z):
        lane = tie(lane0, z)
        masks = {}

        def pick(n, a, b):
            if n not in masks:
                masks[n] = lane < n
            return lax.select(masks[n], a, b)

        def fwd(cur, prev, sh):
            return cur if sh == 0 else pltpu.roll(pick(LB - sh, cur, prev), sh, 1)

        def bwd(cur, nxt_):
            return pltpu.roll(pick(SH, nxt_, cur), LB - SH, 1)
        return fwd, bwd

    def grp_shift(t, bd):
        lag = max(2, -(-P["LAG"] * DH // (G * bd)))
        return mk_shift(at(t, *(hist[-lag] if len(hist) >= lag else [])))

    raw, probs = {}, {}

    def attn_qk(j, hh, t, bd):
        jn = min(j + 1, NB - 1)
        assert ("q", jn) in ready and ("kv", j) in ready
        acc = [None] * WH
        accp = [None] * WH
        for d in range(DH):
            if d % G == 0:
                if d > 0:
                    hist.append(acc + accp)
                fwd, bwd = grp_shift(t + d * bd // DH, bd)
            r = hh * D + d * HH
            q = qk_s[j, r:r + HH, :]
            qp = bwd(q, qk_s[jn, r:r + HH, :])
            rk = (1 - hh) * D + HD + d * HH
            k = qk_s[j, rk:rk + HH, :]
            kp = qk_s[j - 1, rk:rk + HH, :] if j > 0 else zeros8
            for a in range(WH):
                ks = fwd(k, kp, DIL * a)
                t0, t1 = q * ks, qp * ks
                acc[a] = t0 if d == 0 else acc[a] + t0
                accp[a] = t1 if d == 0 else accp[a] + t1
        hist.append(acc + accp)
        raw[j, hh] = (acc, accp)

    def attn_sm(j, hh, t):
        fwd, _ = mk_shift(at(t))
        acc, accp = raw[j, hh]
        prev = raw.pop((j - 1, hh))[1] if j > 0 else [zeros8] * WH
        lg = acc + [fwd(accp[a], prev[a], SH) for a in range(WH)]
        lg = [a * SCALE for a in lg]
        if j == 0:
            lg = [lg[0]] + [jnp.where(lane0 >= DIL * w, lg[w], -1e9) for w in range(1, W)]
        m = lg[0]
        for w in range(1, W):
            m = jnp.maximum(m, lg[w])
        e = [jnp.exp(l - m) for l in lg]
        den = e[0]
        for w in range(1, W):
            den = den + e[w]
        inv = 1.0 / den
        p = [x * inv for x in e]
        for a in range(WH):
            pr_s[j, (hh * W + a) * HH:(hh * W + a + 1) * HH, :] = p[a]
        probs[j, hh] = p[WH:]

    def attn_pp(j, hh, t):
        _, bwd = mk_shift(at(t))
        p = probs.pop((j, hh))
        pn = probs[j + 1, hh] if j + 1 < NB else p
        for a in range(WH):
            pr_s[j, (hh * W + WH + a) * HH:(hh * W + WH + a + 1) * HH, :] = bwd(p[a], pn[a])
        ready.add(("pr", j, hh))

    def attn_pv(j, hh, dst, e, t, bd):
        assert not isinstance(j, int) or ("pr", j, hh) in ready
        assert e == 0 or ("o", dst, hh, e - 1) in ready
        pa = [pr_s[j, (hh * W + a) * HH:(hh * W + a + 1) * HH, :] for a in range(W)]
        p, pp = pa[:WH], pa[WH:]
        outs = []
        for d in range(DH):
            if d % G == 0:
                if d > 0:
                    hist.append([])
                fwd, _ = grp_shift(t + d * bd // DH, bd)
            r = hh * HD + d * HH
            v = v_s[j + 1, r:r + HH, :]
            vp = v_s[j, r:r + HH, :]
            o = op = None
            for a in range(WH):
                vs = fwd(v, vp, DIL * a)
                o = p[a] * vs if a == 0 else o + p[a] * vs
                op = pp[a] * vs if a == 0 else op + pp[a] * vs
            opp = zeros8 if (isinstance(j, int) and j == 0) else op_s[r:r + HH, :]
            op_s[r:r + HH, :] = op
            outs.append(o + fwd(op, opp, SH))
            ol[dst][r:r + HH, _blk(e)] = outs[-1]
        hist.append([])
        ready.add(("o", dst, hh, e))
        dls.append((t + bd + P["PVL"], _token(*outs)))

    ol = [ola_s, olb_s]
    mains = [("qk", j, hh) for j in range(NB) for hh in range(2)]
    mains = (mains[:P["PVPOS"]] + [("pv", j, hh) for j in range(4) for hh in range(2)]
             + mains[P["PVPOS"]:] + [None, None])
    slot_ctr = [0]

    def slot(t, bd):
        n = slot_ctr[0]
        slot_ctr[0] += 1
        it = mains[n]
        if it is None:
            pass
        elif it[0] == "qk":
            attn_qk(it[1], it[2], t, bd)
        else:
            attn_pv(it[1], it[2], 0, it[1], t, bd)
        if n >= 1 and mains[n - 1] is not None and mains[n - 1][0] == "qk":
            attn_sm(mains[n - 1][1], mains[n - 1][2], t + P["LS"])
        if n >= 2 and mains[n - 2] is not None and mains[n - 2][0] == "qk":
            _, j, hh = mains[n - 2]
            if j > 0:
                attn_pp(j - 1, hh, t + P["PP"])
            if j == NB - 1:
                attn_pp(j, hh, t + P["PP"])

    NRG = 8 * (NQ + 1) + 7
    PD = 8 * QD
    BORD = (1, 3, 2, 4, 0, 5, 6)
    LORD = (2, 4, 1, 3, 0, 5, 6)
    LAST_PARTS = [(0, QD, 1, 2), (QD, HD, 0, 2), (0, QD, 0, 1)]

    def rr_prep(p, pa, src, n0, n1, t0, dur):
        assert ("rr", p) not in ready
        for n in range(n0, n1):
            z = at(t0 + (n - n0) * dur // (n1 - n0))
            z2 = at(t0 + (n - n0) * dur // (n1 - n0) + P["SGR"])
            qd, g = divmod(n, 8)

            def wrow(i):
                return _rhs_op(p, lambda x, y: w2_v[pa + y, (2 * i + x) * LB + g * 16:(2 * i + x) * LB + g * 16 + 16, :]
                               .astype(f32))

            def orow(h):
                def blk(x, y):
                    assert ("o", src, x, 2 * y + 1) in ready
                    r = x * HD + h * QD + g * 16
                    return ol[src][r:r + 16, y * 2 * LB:(y + 1) * 2 * LB]
                return _rhs_op(p, blk)
            ro = p * RRK + g * 8
            if qd == NQ:
                if p in SIDX:
                    r = wrow(2 * NQ)
                    for e in range(2):
                        rr_s[ro:ro + 8, _blk(7 + e)] = _pk(tie8(r[:, _blk(e)], z))
                continue
            r1, r2 = (wrow(2 * qd), wrow(2 * qd + 1)) if qd < NQ else (orow(0), orow(1))
            ro += min(qd, NQ) * (LB // 2)
            c11, c22 = tie8(r1[:, :LB], z), tie8(r2[:, LB:], z2)
            sm = _rhs_sums(c11, r1[:, LB:], r2[:, :LB], c22)
            if p in SIDX or qd > NQ:
                sm.update({1: c11, 4: c22})
            for q, v in sm.items():
                rr_s[ro:ro + 8, _blk(q)] = _pk(v)
        if n1 == NRG:
            ready.add(("rr", p))

    def rr_tasks(p, pa, src, t0, t1):
        cuts = list(range(0, NRG, 8)) + [NRG]
        acc, tot = 0, sum(P["RW"])
        for a, b, w in zip(cuts[:-1], cuts[1:], P["RW"]):
            ta, tb = t0 + acc * (t1 - t0) // tot, t0 + (acc + w) * (t1 - t0) // tot
            add_tasks([(tb, rr_prep, (p, pa, src, a, b, ta, tb - ta))])
            acc += w

    def out_copy(pidx, e0, e1, r0, r1):
        off = pidx * (2 * LB) + e0 * LB
        if not isinstance(pidx, int):
            off = pl.multiple_of(off, LB)
        rs = pl.ds(r0, r1 - r0)
        return pltpu.make_async_copy(out_v.at[pidx, rs, pl.ds(e0 * LB, (e1 - e0) * LB)],
                                     out_hbm.at[0, rs, pl.ds(off, (e1 - e0) * LB)], sems.at[0])

    def b_out(pa, n, m, part, t0=None, dur=None):
        a, y = divmod(n, 2)
        r0, r1, e0, e1 = part
        cols = slice(e0 * LB, e1 * LB)
        for r in range(r0, r1, 16):
            c = _combine([None if v is None else v[r:r + 16, cols] for v in m], n)
            rows = slice(a * HD + r, a * HD + r + 16)
            o = c + x_v[pa + y, rows, cols].astype(f32)
            if t0 is not None:
                o = jnp.concatenate([tie(o[:, 0:LB], at(t0 + (r - r0) * dur // (r1 - r0))), o[:, LB:]], axis=1)
            out_v[pa + y, rows, cols] = o.astype(bf16)
        out_copy(pa + y, e0, e1, a * HD + r0, a * HD + r1).start()

    def big_piece(pa, pan, cur, last):
        t0 = now()
        for n in range(7):
            ta, tb = t0 + n * PD + P["RR0"], t0 + n * PD + P["RR1"]
            if n < 6:
                rr_tasks(BORD[n + 1], pa, cur, ta, tb)
            else:
                rr_tasks(BORD[0], pan, 1 - cur, ta, tb - (P["RRM"] if last else 0))
        ready.difference_update({("o", 1 - cur, hh, e) for hh in range(2) for e in range(4)})
        for n in range(8):
            e, hh = divmod(n, 2)
            t = t0 + P["BV0"] + n * P["BVS"]
            add_tasks([(t + P["BVD"], attn_pv, (pan * 2 + e, hh, 1 - cur, e, t, P["BVD"]))])
        m = [None] * 7
        for p in BORD:
            flush(now())
            assert ("rr", p) in ready
            x, y = TOP[p][0]

            def lhs(q):
                if q in (2, 3):
                    rows = slice(p * QD + (q - 2) * ED, p * QD + (q - 1) * ED)
                    return _up(jnp.concatenate([lc_s[rows, _blk(2 * qd + q - 2)] for qd in range(NQ)]
                                               + [lc_s[rows, (NFP + q - 2) * LB:(NFP + q - 2) * LB + QD]], axis=1))
                return _up(ll_s[(p * 7 + q) * ED:(p * 7 + q + 1) * ED, 0:KL])

            def rhs(q):
                if p in SIDX or q in SIDX:
                    return _up(rr_s[p * RRK:p * RRK + KL // 2, _blk(q)])
                h = 0 if q == 1 else 1
                return _cat([w2_v[pa + y, _blk(2 * (2 * qd + h) + x), _blk(h)] for qd in range(NQ)]
                            + [_up(rr_s[p * RRK + NQ * LB // 2:p * RRK + KL // 2, _blk(q)])], 0)
            rl = (_up(rr_s[p * RRK:p * RRK + LB // 2, 7 * LB:9 * LB]) if p in SIDX
                  else w2_v[pa + y, _blk(4 * NQ + x), :])
            ll = _up(lc_s[p * QD:(p + 1) * QD, _blk(2 * NQ)])
            ex = [mm1(ll[:QD], rl), mm1(ll[QD:], rl)]
            e12, e21 = ex[0][:, LB:], ex[1][:, :LB]
            e11 = (ex[0][:, :LB] + e12) - e21
            lf = strassen(lhs, rhs, LORD)
            ready.discard(("rr", p))
            if p in (2, 3):
                for q in (2, 3):
                    lf[q] = lf[q] + b2f_s[pa + 3 - p, 0:1, _blk(3 - q)]
            c12 = (lf[2] + e12) + lf[4]
            c21 = (lf[1] + e21) + lf[3]
            xx = (lf[2] - lf[1]) + lf[0]
            c22 = (xx + ex[1][:, LB:]) + lf[5]
            c11 = ((xx + e11) + (c21 - c12)) + lf[6]
            m[p] = jnp.concatenate([jnp.concatenate([c11, c12], axis=1),
                                    jnp.concatenate([c21, c22], axis=1)], axis=0)
            n = {3: 2, 4: 1, 5: 3, 6: 0}.get(p)
            if n is not None and not (last and n == 0):
                t, epd = now() + P["EP0"], P["EPL"] if (last and n == 3) else P["EPD"]
                add_tasks([(t + epd, b_out, (pa, n, list(m), (0, HD, 0, 2), t, epd))])
        if last:
            flush()
            for part in LAST_PARTS:
                b_out(pa, 0, m, part)

    def c_body(it, carry):
        reset()
        pos[:] = [one_s[...]]
        true.clear()
        ready.update({("rr", BORD[0])} | {("o", 0, hh, e) for hh in range(2) for e in range(4)})
        big_piece(4 * it, 4 * it + 2, 0, False)
        big_piece(4 * it + 2, lax.rem(4 * it + 4, NP), 1, True)
        assert ("rr", BORD[0]) in ready and all(("o", 0, hh, 3) in ready for hh in range(2))
        return carry

    E1 = P["E1"]
    x0 = Group(cp_x(0, 1))
    g1 = Group([(b1_hbm, b1_v)] + cp_w1(0, 2, 0, E1))
    g2 = Group(cp_w1(0, 2, E1, NFP) + cp_x(1, 2))
    wq, wkv = [[(wqkv_hbm.at[:, cl], wqkv_v.at[:, cl])] for cl in (pl.ds(0, 4 * LB), pl.ds(4 * LB, 3 * D - 4 * LB))]
    g3 = Group(wq)
    g4 = Group(wkv + cp_x(2, 3))
    g5 = Group(cp_x(3, NP))
    g6 = Group(cp_w1(UB0, NB) + [(wo_hbm, wo_v), (b2_hbm, b2_v)] + cp_w2(0, 1))
    g7 = Group(cp_w2(1, NP))
    for c in (x0, g1, g2, g3, g4, g5, g6, g7):
        c.start()

    v_s[0] = jnp.zeros((D, LB), f32)
    for buf in (xnT_s, ra_s, lh_s, rs_s, rr_s, ola_s, olb_s, ll_s, lc_s):
        buf[0:8, 0:64] = jnp.zeros((8, 64), buf.dtype)

    wait("x0", x0)
    one_s[...] = lax.shift_right_logical(pltpu.bitcast(x_v[0, 0:16, 0:LB], i32), 1) | 1
    pos[:] = [one_s[...]]
    ln(0)
    ln(1)
    hpair(0)
    wait("r1", g1)
    jobs = u_early(0, 0, E1, [], 7 * E1 // 4 * 4, P["T1"], 100)
    wait("r2", g2)
    t, dt = P["L2T"], P["L2D"]
    add_tasks([(t + int((k + 1) * dt * P["LNV"]), ln, (2 + k, t + int(k * dt * P["LNV"]), dt)) for k in range(2)])
    jobs = u_early(0, E1, NFP, jobs, P["N2"], P["T2"], 100)
    wait("wq", g3)
    add_tasks([(P["H2T"] + P["H2D"], hpair, (2, P["H2T"], P["H2D"]))])
    u_early(0, 0, 0, jobs, len(jobs), 0, 1, nsplit=P["S3"])
    prep_wqkv("q", 0, HD // 16, [P[k] for k in ("QA", "QB", "QC", "QE")])
    stage_a(0, "q", split_last=True)
    m = stage_a(2, "q", AORD[:P["NA3"]])
    wait("wkv", g4)
    stage_a(2, "q", AORD[P["NA3"]:], split_last=True, m=m)
    prep_wqkv("kv", HD // 16, HA // 16, [P[k] for k in ("KA", "KB", "KC", "KE")])
    t = ln_tasks(4, now() + P["L4T"], P["LND"], P["HSD"])
    n4 = min(4, (now() + 14 * HD - P["MARG"] - t) // P["BD"])
    add_tasks([(t + (n + 1) * P["BD"], slot, (t + n * P["BD"], P["BD"])) for n in range(n4)])
    stage_a(0, "kv")
    stage_a(2, "kv", order=(6,) + AORD[:6])

    wait("mid", g5)
    AD = 7 * HA // 2
    t = P["L5T"]
    for b in range(6, NB, 2):
        t = ln_tasks(b, t, P["LND"], P["HSD"])
    n5 = ((NP - 2) * AD - P["MARG"] - t) // P["BD"]
    add_tasks([(t + (n + 1) * P["BD"], slot, (t + n * P["BD"], P["BD"])) for n in range(n5)])
    n5 += n4
    for n, b in enumerate(range(4, NB, 2)):
        stage_a(b, order=(6,) + AORD[:6] if n % 2 else AORD)

    wait("fin", g6)
    UD = 7 * NUP * HD // 4
    for i in range(NFP):
        t0, dt = (-200, 130) if i == 0 else (800, 270) if i == 1 else ((i - 1) * UD + P["US0"], P["USD"])
        add_tasks([(t0 + (k + 1) * dt, tsum, (UB0 // 2 + k, i, i % 3, k, t0 + k * dt, dt)) for k in range(NUP)])
    left = len(mains) - n5 - 2
    bd = (NFP * UD - P["R6E"] - P["R6S"]) // left
    add_tasks([(P["R6S"] + (n + 1) * bd, slot, (P["R6S"] + n * bd, bd)) for n in range(left)])
    t = P["R6S"] + left * bd
    add_tasks([(t + (n + 1) * 300, slot, (t + n * 300, 300)) for n in range(2)])
    for qd, t0, t1 in ((NQ, UD + P["LL0"], 3 * UD), (0, 3 * UD + P["LL0"], 5 * UD), (1, 5 * UD + P["LL0"], 6 * UD + 200),
                       (2, 6 * UD + P["LL2"], 6 * UD + P["LL2"] + P["UEL"])):
        dt = (t1 - t0) // 7
        add_tasks([(t0 + (g + 1) * dt, llsum, (qd, g, t0 + g * dt, dt)) for g in range(7)])
    rr_tasks(BORD[0], 0, 0, P["RP0"], P["RP1"])
    add_tasks([(P["PW0"] + P["PWD"], prep_wo_a, (P["PW0"], P["PWD"]))])
    add_tasks([(P["PW1"] + (h + 1) * P["PWE"], prep_wo_b, (h, P["PW1"] + h * P["PWE"], P["PWE"])) for h in range(2)])
    for b in range(NB):
        b2f_s[b // 2, 0:1, _blk(b % 2)] = b2_v[b:b + 1, :].astype(f32)
    for i in range(NFP):
        u_last(i, (1, 4, 2, 3, 0, 5, 6) if i == 0 else (4, 2, 1, 3, 0, 5, 6),
               None if i == NFP - 1 else P["UEL"] if i == NFP - 2 else P["UED"])
    flush()
    assert slot_ctr[0] == len(mains) and all(("ll", qd, g) in ready for qd in range(NQ + 1) for g in range(7))
    assert all(("pr", j, hh) in ready for j in range(NB) for hh in range(2)) and ("rr", BORD[0]) in ready

    wait("w2", g7)
    lax.fori_loop(0, NP // 4, c_body, 0)
    outs = []
    for pa in range(0, NP, 2):
        outs += [out_copy(pa + n % 2, 0, 2, n // 2 * HD, (n // 2 + 1) * HD) for n in (1, 2, 3)]
        outs += [out_copy(pa, e0, e1, r0, r1) for (r0, r1, e0, e1) in (LAST_PARTS if pa % 4 else [(0, HD, 0, 2)])]
    wait("out", *outs)


@jax.jit
def pallas_parallel_sum__sliding_local_dilated__mixer_token_mlp__prompt_kernel(A_x, A_wqkv, A_wo, B_x, B_w1, B_b1, B_w2, B_b2):
    del B_x
    hbm = pl.BlockSpec(memory_space=pltpu.HBM)
    outT = pl.pallas_call(
        _kernel,
        out_shape=jax.ShapeDtypeStruct((1, D, S), bf16),
        in_specs=[hbm] * 7,
        out_specs=hbm,
        scratch_shapes=[
            pltpu.VMEM((NP, D, 2 * LB), bf16),
            pltpu.VMEM((D, 3 * D), bf16),
            pltpu.VMEM((D, D), bf16),
            pltpu.VMEM((S, F), bf16),
            pltpu.VMEM((NP, F, 2 * LB), bf16),
            pltpu.VMEM((NFB, LB), bf16),
            pltpu.VMEM((NB, LB), bf16),
            pltpu.VMEM((NP, D, 2 * LB), bf16),
            pltpu.VMEM((2, 3 * D + 64, LB), i32),
            pltpu.VMEM((7 * HA // 2, HD), u32),
            pltpu.VMEM((4, HD + 32, LB), i32),
            pltpu.VMEM((D, 2 * LB), i32),
            pltpu.VMEM((HD, S), u32),
            pltpu.VMEM((NP * QD, 5 * LB), u32),
            pltpu.VMEM((7 * QD, NP * LB), u32),
            pltpu.VMEM((7 * HD, NFP * LB), f32),
            pltpu.VMEM((7 * QD, (NFP + 2) * LB), u32),
            pltpu.VMEM((NB, 2 * D, LB), f32),
            pltpu.VMEM((NB + 1, D, LB), f32),
            pltpu.VMEM((NB, 2 * W * HH, LB), f32),
            pltpu.VMEM((D, LB), f32),
            pltpu.VMEM((NP, 32, 2 * LB), f32),
            pltpu.VMEM((4 * RSK, 5 * LB), u32),
            pltpu.VMEM((49 * ED, 4 * LB), u32),
            pltpu.VMEM((7 * RRK, 9 * LB), u32),
            pltpu.VMEM((D, 4 * LB), f32),
            pltpu.VMEM((D, 4 * LB), f32),
            pltpu.VMEM((8, LB), i32),
            pltpu.SemaphoreType.DMA((9,)),
        ],
        compiler_params=pltpu.CompilerParams(vmem_limit_bytes=100 * 1024 * 1024,
                                             disable_bounds_checks=True,
                                             disable_semaphore_checks=True),
    )(jnp.swapaxes(A_x, 1, 2), A_wqkv, A_wo, B_w1, B_b1.reshape(NFB, LB), B_w2, B_b2.reshape(NB, LB))
    return jnp.swapaxes(outT, 1, 2)
```

```python
import jax
import jax.numpy as jnp
from jax import lax
import jax.experimental.pallas as pl
import jax.experimental.pallas.tpu as pltpu

S, D, F = 2048, 448, 1792
H, DH, W, DIL = 16, 28, 8, 2
LB = 128
NB = S // LB
NP = NB // 2
NFB = F // LB
NFP = NFB // 2
HH = H // 2
WH = W // 2
SH = DIL * WH
HD = D // 2
QD = D // 4
ED = D // 8
HA = 3 * HD
UB0 = 2
NUP = (NB - UB0) // 2
RSK = NFP * LB // 2
NQ = NFP // 2
KL = NQ * LB + QD
RRK = 2 * LB
EPS = 1e-5
EPS_BF16 = 1.0013580322265625e-05
SCALE = DH ** -0.5
f32 = jnp.float32
bf16 = jnp.bfloat16
u32 = jnp.uint32
i32 = jnp.int32

SCOPES = False
P = dict(
    E1=3, N2=16, NA3=2, T1=-200, T2=-200, S3=0, L2T=100, L2D=440, H2T=900, H2D=360, L4T=1000, L5T=60, W2X=500,
    QA=-410, QB=200, QC=-200, QE=330, KA=50, KB=320, KC=450, KE=390,
    LND=420, HSD=350, HL=180, LNA=0.28, LNB=0.46, LNBD=0.38, LNV=0.86, LNW=0.93,
    BD=370, MARG=300, LAG=200, LS=150, PP=130, PVL=500, PVPOS=12,
    US0=100, USD=360, UE0=240, UED=2320, UEL=1700, UG=70, UM=0, R6S=1750, R6E=3150,
    LL0=300, LL2=550, RP0=16600, RP1=18700, PW0=560, PWD=300, PW1=1380, PWE=400,
    RR0=-48, RR1=800, RRM=-20, RW=(8, 8, 8, 2, 7), BV0=117, BVS=717, BVD=620, EP0=0, EPD=864, EPL=290, SGR=8, SGT=8, SH4=1,
)
G = 4


def _as(x, dtype):
    return x if x.dtype == dtype else pltpu.bitcast(x, dtype)


def _pk(x):
    return pltpu.bitcast(x.astype(bf16), u32)


def _up(x):
    return pltpu.bitcast(x, bf16)


def _upf(x):
    return pltpu.bitcast(x, bf16).astype(f32)


def _rb(x):
    return x.astype(bf16).astype(f32)


def _word(lo, hi):
    lo, hi = [pltpu.bitcast(v.astype(f32), i32) for v in (lo, hi)]
    return lax.shift_right_logical(lo, 16) | hi


def _unword(w):
    return [pltpu.bitcast(w << 16, f32), pltpu.bitcast(w & -65536, f32)]


def _cat(xs, axis):
    return xs[0] if len(xs) == 1 else jnp.concatenate(xs, axis=axis)


def _x2(v):
    return jnp.concatenate([v, v], axis=0)


def _blk(b):
    return slice(b * LB, (b + 1) * LB)


def _rowsum8(a):
    return jnp.broadcast_to(jnp.sum(a, axis=0, keepdims=True), (8, a.shape[1]))


def _token(*deps):
    deps = [d for d in deps if d is not None]
    if not deps:
        return None
    if len(deps) == 1:
        return deps[0]
    bits = _as(deps[0], u32)
    for d in deps[1:]:
        bits = bits | _as(d, u32)
    return bits


def _lhs_ops(a11, a12, a21, a22):
    return [a11 + a22, a21 + a22, a11, a22, a11 + a12, a21 - a11, a12 - a22]


SIDX = {0: 0, 2: 1, 3: 2, 5: 3, 6: 4}
TOP = {0: ((0, 0), 1, (1, 1)), 1: ((0, 0),), 2: ((0, 1), -1, (1, 1)), 3: ((1, 0), -1, (0, 0)),
       4: ((1, 1),), 5: ((0, 0), 1, (0, 1)), 6: ((1, 0), 1, (1, 1))}


def _rhs_sums(b11, b12, b21, b22):
    return {0: b11 + b22, 2: b12 - b22, 3: b21 - b11, 5: b11 + b12, 6: b21 + b22}


def _rhs_op(p, blk):
    t = TOP[p]
    if len(t) == 1:
        return blk(*t[0])
    return blk(*t[0]) + blk(*t[2]) if t[1] > 0 else blk(*t[0]) - blk(*t[2])


def _combine(m, n=None):
    c12 = lambda: m[2] + m[4]
    c21 = lambda: m[1] + m[3]
    x = lambda: (m[2] - m[1]) + m[0]
    c = [lambda: (x() + m[6]) + (c21() - c12()), c12, c21, lambda: x() + m[5]]
    return [f() for f in c] if n is None else c[n]()


def _kernel(x_hbm, wqkv_hbm, wo_hbm, w1_hbm, b1_hbm, w2_hbm, b2_hbm, out_hbm,
            x_v, wqkv_v, wo_v, w1_v, w2_v, b1_v, b2_v, out_v,
            wt_s, lw_s, wo_s, wq_s, xnT_s, ra_s, lh_s, um_s, lc_s, qk_s, v_s, pr_s, op_s,
            b2f_s, rs_s, ll_s, rr_s, ola_s, olb_s, one_s, sems):
    sem_ctr = [1]

    class Group:
        def __init__(self, pairs):
            self.cps = [pltpu.make_async_copy(a, b, sems.at[sem_ctr[0]]) for (a, b) in pairs]
            sem_ctr[0] += 1

        def start(self):
            for c in self.cps:
                c.start()

        def wait(self):
            for c in self.cps:
                c.wait()

    def cp_x(p0, p1):
        return [(x_hbm.at[0, :, pl.ds(p * 2 * LB, 2 * LB)], x_v.at[p]) for p in range(p0, p1)]

    def cp_w2(p0, p1):
        return [(w2_hbm.at[:, pl.ds(p * 2 * LB, 2 * LB)], w2_v.at[p]) for p in range(p0, p1)]

    def cp_w1(b0, b1, i0=0, i1=NFP):
        sl = pl.ds(b0 * LB, (b1 - b0) * LB)
        cl = pl.ds(i0 * 2 * LB, (i1 - i0) * 2 * LB)
        return [(w1_hbm.at[sl, cl], w1_v.at[sl, cl])]

    tl = []
    mxu = [0, 0, 0, 0]
    nxt = [0]
    hist = []
    tasks = []
    dls = []
    ready = set()
    pos = []
    true = {}

    def tie(v, z):
        if z is None:
            return v
        def fit(a):
            a = _cat([a] * (v.shape[0] // 8), 0)
            return a if v.shape[1] == LB else a[:, 0:v.shape[1]]
        if v.shape not in true:
            true[v.shape] = fit(pos[0]) > 0
        return lax.select(true[v.shape], v, fit(_as(z, v.dtype)))

    def tie8(v, z):
        return v if z is None else jnp.concatenate([tie(v[0:8], z), v[8:16]], axis=0)

    def add_tasks(todo):
        tasks.extend(todo)
        tasks.sort(key=lambda x: x[0])

    def flush(t=None):
        while tasks and (t is None or tasks[0][0] < t):
            _, fn, args = tasks.pop(0)
            fn(*args)

    def reset():
        assert not tasks
        dls.clear()
        tl.clear()
        hist.clear()
        mxu[:] = [0, 0, 0, 0]
        nxt[0] = 0

    def now():
        return sum(mxu) // 4

    def wait(name, *cps):
        flush()
        if SCOPES:
            with jax.named_scope("wait_" + name):
                for c in cps:
                    c.wait()
        else:
            for c in cps:
                c.wait()
        reset()

    def mm1(lhs, rhs, pace=True):
        flush(now())
        start = mxu[nxt[0]]
        due = [v for (t, v) in dls if t <= start] if pace else []
        if due:
            dls[:] = [(t, v) for (t, v) in dls if t > start]
            tile = _up(tie(pltpu.bitcast(lhs[0:16, 0:LB], u32), _token(*due)))
            row = tile if lhs.shape[1] == LB else jnp.concatenate([tile, lhs[0:16, LB:]], axis=1)
            lhs = jnp.concatenate([row, lhs[16:]], axis=0)
        r = jnp.dot(lhs, rhs, preferred_element_type=f32)
        m, k = lhs.shape
        first_done = None
        for _ in range(-(-rhs.shape[1] // LB)):
            end = 0
            for _ in range(-(-k // LB)):
                mxu[nxt[0]] += m
                end = max(end, mxu[nxt[0]])
                nxt[0] = (nxt[0] + 1) % 4
            if first_done is None:
                first_done = end
        if pace:
            tl.append((first_done - m, first_done, r))
        return r

    def mm(lhs, rhs, init=None):
        k = lhs.shape[1]
        r, k0 = init, 0
        while k0 < k:
            k1 = min(k, k0 + (4 - nxt[0]) * LB)
            part = mm1(lhs[:, k0:k1], rhs[k0:k1], pace=k1 - k0 > LB)
            r = part if r is None else r + part
            k0 = k1
        return r

    def at(t, *more):
        best = None
        if t is not None and t >= 0:
            t = min(t, now() - 1)
            for (a, b, r) in tl:
                if a <= t and (best is None or min(b, t) > best[0]):
                    row = int(min((t - a) / (b - a), 0.999) * (r.shape[0] // 8)) * 8
                    best = (min(b, t), r, row)
        return _token(None if best is None else best[1][best[2]:best[2] + 8, 0:LB], *more)

    def strassen(lhs, rhs, order, split_last=False, init=None, m=None):
        m = [None] * 7 if m is None else m
        for p in order:
            flush(now())
            l, r = lhs(p), rhs(p)
            c0 = None if init is None else init[p]
            if split_last and p == order[-1]:
                kk = (-(-r.shape[0] // LB) - 2) * LB
                hm = l.shape[0] // 2
                hd = mm(l[:, :kk], r[:kk], c0) if kk else c0
                tail = jnp.concatenate([mm(l[:hm, kk:], r[kk:]), mm(l[hm:, kk:], r[kk:])], axis=0)
                m[p] = tail if hd is None else hd + tail
            else:
                m[p] = mm(l, r, c0)
        return m

    def wcol(hh, p):
        return p * D + (1 - hh if p == 1 else hh) * HD

    def wrows(hh, g, z=None):
        p, d = divmod(2 * g, DH)
        t = [jnp.concatenate([wt_s[c, pl.ds(wcol(hh, p) + d + e, HH, stride=DH), :]
                              for e in range(2)], axis=0) for c in range(2)]
        return _unword(jnp.concatenate([tie(t[0], z), tie(t[1][:, 0:HD - LB], z)], axis=1))

    wt_done = set()

    def prep_wqkv(part, ga, gb, paced):
        def need(hh, p, z):
            lo = wcol(hh, p)
            for ct in range(lo // LB, -(-(lo + HD) // LB)):
                if ct in wt_done:
                    continue
                wt_done.add(ct)
                cols = slice(ct * LB, min((ct + 1) * LB, 3 * D))
                wd = _word(wqkv_v[0:HD, cols], wqkv_v[HD:D, cols])
                wd = jnp.concatenate([tie(wd[r:r + 8], z if r % LB == 0 else None) for r in range(0, HD, 8)], axis=0)
                wT = wd.T
                wt_s[0, cols, :] = wT[:, 0:LB]
                wt_s[1, cols, 0:HD - LB] = wT[:, LB:HD]

        def put(p, g, v):
            lw_s[p * (HA // 2) + g * 8:p * (HA // 2) + g * 8 + 8, :] = _pk(v)

        def half(hh, g0, g1, t0=None, dur=None):
            pr, ps = ((2, 4), (3, 1))[hh]
            for g in range(g0, g1):
                t = None if t0 is None else t0 + (g - g0) * dur // (g1 - g0)
                need(hh, 2 * g // DH, at(None if t is None else t - P["W2X"]))
                a1, a2 = wrows(hh, g, at(t))
                put(pr, g, a2 if hh else a1)
                put(ps, g, a1 + a2)
            if g1 == gb:
                ready.update({("lw", part, pr), ("lw", part, ps)})

        def rest(g0, g1, t0, dur):
            assert ("lw", part, 1) in ready
            for g in range(g0, g1):
                z = at(t0 + (g - g0) * dur // (g1 - g0))
                ops = _lhs_ops(*wrows(0, g, z), *wrows(1, g, z))
                for p in (0, 5, 6):
                    put(p, g, ops[p])
            if g1 == gb:
                ready.update({("lw", part, 0), ("lw", part, 5), ("lw", part, 6)})
        t2, d2, t3, d3 = paced
        half(0, ga, gb)
        n = (gb - ga) // 14
        add_tasks([(now() + t2 + (k + 1) * d2 // n, half,
                    (1, ga + 14 * k, ga + 14 * k + 14, now() + t2 + k * d2 // n, d2 // n)) for k in range(n)])
        n = (gb - ga) // 7
        add_tasks([(now() + t3 + (k + 1) * d3 // n, rest,
                    (ga + 7 * k, ga + 7 * k + 7, now() + t3 + k * d3 // n, d3 // n)) for k in range(n)])

    def prep_wo_a(t0, dur):
        for g in range(HD // 16):
            w = _word(wo_v[g * 16:g * 16 + 16, :], wo_v[HD + g * 16:HD + g * 16 + 16, :])
            z = at(t0 + g * dur // (HD // 16))
            for c in range(4):
                cw = min(LB, D - c * LB)
                wo_s[c, g * 16:g * 16 + 16, 0:cw] = tie(w[:, c * LB:c * LB + cw], z)
        ready.add("wo")

    def prep_wo_b(h, t0, dur):
        assert "wo" in ready
        for c in range(4):
            cw = min(LB, D - c * LB)
            rows = [wo_s[c, pl.ds(d, HH, stride=DH), :][:, 0:cw] for d in range(h * DH // 2, (h + 1) * DH // 2)]
            rows.append(jnp.zeros((LB - QD, cw), i32))
            wq_s[c * LB:c * LB + cw, _blk(h)] = jnp.concatenate(rows, axis=0).T
        outs = []
        for g in range(HD // 16):
            z = at(t0 + g * dur // (HD // 16))
            a = [v for r in (g * 16, HD + g * 16) for v in _unword(tie(wq_s[r:r + 16, _blk(h)], z))]
            for p, v in enumerate(_lhs_ops(*a)):
                lc_s[p * QD + g * 8:p * QD + g * 8 + 8, _blk(NFP + h)] = _pk(v)
                outs.append(v[0:8])
        ready.update({("lc", NFP + h, g) for g in range(HD // 16)})
        dls.append((t0 + dur + 250, _token(*outs)))

    RG = 16
    NG = D // RG
    stat2 = {}

    def ln(b, t0=None, dur=None):
        def xg(g):
            return x_v[b // 2, g * RG:(g + 1) * RG, _blk(b % 2)].astype(f32)

        def step(v, g, fr, s, q):
            if t0 is None or g % 4:
                return v
            acc = [] if s is None else [s[0:8], s[8:16], q[0:8], q[8:16]]
            return tie(v, at(t0 + fr * dur, *acc))

        x0 = jnp.broadcast_to(xg(0)[0:1], (8, LB))
        s = q = None
        for g in range(NG):
            x0 = step(x0, g, P["LNA"] * g / NG, s, q)
            c = xg(g) - _x2(x0)
            s = c if s is None else s + c
            q = c * c if q is None else q + c * c
        dm = _rowsum8(s) * (1.0 / D)
        mu = _rb(x0 + dm)
        var = _rb(jnp.maximum(_rowsum8(q) * (1.0 / D) - dm * dm, 0.0))
        r1 = 1.0 / _rb(jnp.sqrt(_rb(var + EPS_BF16)))
        s = q = None
        for g in range(NG):
            mu = step(mu, g, P["LNB"] + P["LNBD"] * g / NG, s, q)
            xn = _rb(xg(g) - _x2(mu)) * _x2(r1)
            xnT_s[g * 8:g * 8 + 8, _blk(b)] = _pk(xn)
            s = xn if s is None else s + xn
            q = xn * xn if q is None else q + xn * xn
        mu2 = _rowsum8(s) * (1.0 / D)
        var2 = jnp.maximum(_rowsum8(q) * (1.0 / D) - mu2 * mu2, 0.0)
        stat2[b] = (mu2, 0.5 * lax.rsqrt(var2 + EPS))

    def hpair(b, t0=None, dur=None):
        ng = HD // RG
        st = [stat2.pop(b), stat2.pop(b + 1)]
        for g in range(ng):
            zz = [at(None if t0 is None else t0 + (4 * g + k * P["SH4"]) * dur // (4 * ng)) for k in (0, 1, 2, 3)]
            xq = [_upf(tie(xnT_s[r:r + 8, _blk(b + e)], zz[2 * (r >= QD) + e]))
                  for r in (g * 8, QD + g * 8) for e in range(2)]
            hq = [(v - _x2(st[n % 2][0])) * _x2(st[n % 2][1]) for n, v in enumerate(xq)]
            ro = (b // 2) * QD + g * 8
            for p, v in _rhs_sums(*xq).items():
                ra_s[ro:ro + 8, _blk(SIDX[p])] = _pk(v)
            for p, v in enumerate(_lhs_ops(*hq)):
                lh_s[p * QD + g * 8:p * QD + g * 8 + 8, _blk(b // 2)] = _pk(v)
        ready.add(("xn", b))
        if b >= 6:
            got = ra_s[(b // 2) * QD:(b // 2 + 1) * QD, :]
            dls.append((t0 + dur + P["HL"], _token(*[got[r:r + 8, _blk(c)] for r in range(0, QD, 8) for c in range(5)])))

    def ln_tasks(b, t, lnd, hsd):
        for fn, bb, dur, adv in ((ln, b, lnd, P["LNV"]), (ln, b + 1, lnd, P["LNW"]), (hpair, b, hsd, 1.0)):
            add_tasks([(t + int(dur * adv), fn, (bb, t, dur))])
            t += int(dur * adv)
        return t

    def tsum(kp, i, slot_, n, t0, dur):
        for g in range(LB // 16):
            z, z2 = at(t0 + g * dur // 8), at(t0 + g * dur // 8 + P["SGT"])
            t1, t2 = [w1_v[(2 * kp + e) * LB + g * 16:(2 * kp + e) * LB + g * 16 + 16,
                           2 * i * LB:(2 * i + 2) * LB].astype(f32) for e in range(2)]
            ro = slot_ * RSK + n * (LB // 2) + g * 8
            for p, v in _rhs_sums(tie8(t1[:, :LB], z), t1[:, LB:], t2[:, :LB], tie8(t2[:, LB:], z2)).items():
                rs_s[ro:ro + 8, _blk(SIDX[p])] = _pk(v)
        ready.add(("rs", kp, i))

    def u_rhs(p, i, kps, slot_, n0):
        if p in SIDX:
            assert all(("rs", kp, i) in ready for kp in kps)
            ro = slot_ * RSK + n0 * (LB // 2)
            return _up(rs_s[ro:ro + len(kps) * (LB // 2), _blk(SIDX[p])])
        e = 0 if p == 1 else 1
        return _cat([w1_v[_blk(2 * kp + e), _blk(2 * i + e)] for kp in kps], 0)

    LATE = (NFP - 1, 6)

    def ujob(kp, i, p, split):
        flush(now())
        assert ("xn", 2 * kp) in ready
        l, r = _up(lh_s[p * QD:(p + 1) * QD, _blk(kp)]), u_rhs(p, i, [kp], 3 + kp, i)
        v = jnp.concatenate([mm1(l[:QD], r), mm1(l[QD:], r)], axis=0) if split else mm1(l, r)
        rows = slice(p * HD, (p + 1) * HD)
        um_s[rows, _blk(i)] = v

    def u_early(kp, i0, i1, carry, n, t0, dt, nsplit=0):
        for k, i in enumerate(range(i0, i1)):
            add_tasks([(t0 + (k + 1) * dt, tsum, (kp, i, 3 + kp, i, t0 + k * dt, dt))])
        jobs = (carry + [(kp, i, p) for i in range(i0, i1) for p in (1, 4)]
                + [(kp, i, p) for i in range(i0, i1) for p in SIDX if (i, p) != LATE])
        for c, job in enumerate(jobs[:n]):
            ujob(*job, c >= n - nsplit)
        return jobs[n:]

    def gelu_half(hx, z):
        c = 0.7978845608028654
        return hx + hx * jnp.tanh(tie(hx * (2.0 * c + (8.0 * c * 0.044715) * (hx * hx)), z))

    def u_epilogue(i, m, gs, t0, dur):
        for n, g in enumerate(gs):
            t = None if t0 is None else t0 + n * dur // len(gs) - P["UG"]
            q = _combine([x[g * 16:g * 16 + 16] for x in m])
            gl = [gelu_half(v, at(None if t is None else t - k * P["UM"])) for v, k in zip(q, (0, 3, 2, 1))]
            for p, v in enumerate(_lhs_ops(*gl)):
                lc_s[p * QD + g * 8:p * QD + g * 8 + 8, _blk(i)] = _pk(v)
            ready.add(("lc", i, g))

    def u_last(i, order, edur):
        kps = list(range(UB0 // 2, NP))
        init = [None if (i, p) == LATE else um_s[p * HD:(p + 1) * HD, _blk(i)] for p in range(7)]
        for p in (2, 3):
            init[p] = init[p] + 0.5 * b1_v[2 * i + 3 - p:2 * i + 4 - p, :].astype(f32)
        m = strassen(lambda p: _up(lh_s[p * QD:(p + 1) * QD, (0 if (i, p) == LATE else UB0 // 2 * LB):]),
                     lambda p: _cat([u_rhs(p, i, [0], 3, i)] * ((i, p) == LATE) + [u_rhs(p, i, kps, i % 3, 0)], 0),
                     order, init=init)
        if edur is None:
            u_epilogue(i, m, list(range(HD // 16)), None, None)
        else:
            t = now() + P["UE0"]
            add_tasks([(t + (g + 1) * edur // 7, u_epilogue, (i, m, [g, g + 7], t + g * edur // 7, edur // 7))
                       for g in range(7)])

    def llsum(qd, g, t0, dur):
        i0 = 2 * qd if qd < NQ else NFP
        assert all(("lc", i0 + e, g + 7 * h) in ready for e in range(2) for h in range(2))
        for p in range(7):
            zz = [at(t0 + p * dur // 7), at(t0 + p * dur // 7 + P["SGT"])]
            a = [tie(lc_s[p * QD + h * ED + g * 8:p * QD + h * ED + g * 8 + 8, _blk(i0 + e)], zz[h] if h == e else None)
                 for h in range(2) for e in range(2)]
            ops = _lhs_ops(*[_upf(v) for v in a])
            for q in (0, 1, 4, 5, 6):
                r = (p * 7 + q) * ED + g * 8
                ll_s[r:r + 8, _blk(qd)] = _pk(ops[q])
        ready.add(("ll", qd, g))

    AORD = (4, 2, 1, 3, 0, 5, 6)

    def stage_a(b, parts="qkv", order=AORD, split_last=False, m=None):
        r0, r1 = {"q": (0, HD), "kv": (HD, HA), "qkv": (0, HA)}[parts]

        def lhs(p):
            assert all(("lw", pt, p) in ready for pt in ("q", "kv") if pt in parts)
            return _up(lw_s[(p * HA + r0) // 2:(p * HA + r1) // 2, :])

        def rhs(p):
            assert ("xn", b) in ready
            if p in SIDX:
                return _up(ra_s[(b // 2) * QD:(b // 2 + 1) * QD, _blk(SIDX[p])])
            return _up(xnT_s[0:QD, _blk(b)] if p == 1 else xnT_s[QD:HD, _blk(b + 1)])
        m = strassen(lhs, rhs, order, split_last, m=m)
        for n, ps in enumerate((range(7), (2, 4), (1, 3), (0, 1, 2, 5))):
            if all(m[p] is not None for p in ps) and any(p in order for p in ps):
                hh, e = divmod(n, 2)
                c = _combine(m, n)
                qk_s[b + e, hh * D + r0:hh * D + min(r1, D), :] = c[0:min(r1, D) - r0]
                if r1 > D:
                    v_s[b + e + 1, hh * HD:(hh + 1) * HD, :] = c[D - r0:]
        if all(v is not None for v in m):
            ready.update({(pt, b + e) for pt in ("q", "kv") if pt in parts for e in range(2)})
        return m

    lane0 = lax.broadcasted_iota(i32, (HH, LB), 1)
    zeros8 = jnp.zeros((HH, LB), f32)

    def mk_shift(z):
        lane = tie(lane0, z)
        masks = {}

        def pick(n, a, b):
            if n not in masks:
                masks[n] = lane < n
            return lax.select(masks[n], a, b)

        def fwd(cur, prev, sh):
            return cur if sh == 0 else pltpu.roll(pick(LB - sh, cur, prev), sh, 1)

        def bwd(cur, nxt_):
            return pltpu.roll(pick(SH, nxt_, cur), LB - SH, 1)
        return fwd, bwd

    def grp_shift(t, bd):
        lag = max(2, -(-P["LAG"] * DH // (G * bd)))
        return mk_shift(at(t, *(hist[-lag] if len(hist) >= lag else [])))

    raw, probs = {}, {}

    def attn_qk(j, hh, t, bd):
        jn = min(j + 1, NB - 1)
        assert ("q", jn) in ready and ("kv", j) in ready
        acc = [None] * WH
        accp = [None] * WH
        for d in range(DH):
            if d % G == 0:
                if d > 0:
                    hist.append(acc + accp)
                fwd, bwd = grp_shift(t + d * bd // DH, bd)
            r = hh * D + d * HH
            q = qk_s[j, r:r + HH, :]
            qp = bwd(q, qk_s[jn, r:r + HH, :])
            rk = (1 - hh) * D + HD + d * HH
            k = qk_s[j, rk:rk + HH, :]
            kp = qk_s[j - 1, rk:rk + HH, :] if j > 0 else zeros8
            for a in range(WH):
                ks = fwd(k, kp, DIL * a)
                t0, t1 = q * ks, qp * ks
                acc[a] = t0 if d == 0 else acc[a] + t0
                accp[a] = t1 if d == 0 else accp[a] + t1
        hist.append(acc + accp)
        raw[j, hh] = (acc, accp)

    def attn_sm(j, hh, t):
        fwd, _ = mk_shift(at(t))
        acc, accp = raw[j, hh]
        prev = raw.pop((j - 1, hh))[1] if j > 0 else [zeros8] * WH
        lg = acc + [fwd(accp[a], prev[a], SH) for a in range(WH)]
        lg = [a * SCALE for a in lg]
        if j == 0:
            lg = [lg[0]] + [jnp.where(lane0 >= DIL * w, lg[w], -1e9) for w in range(1, W)]
        m = lg[0]
        for w in range(1, W):
            m = jnp.maximum(m, lg[w])
        e = [jnp.exp(l - m) for l in lg]
        den = e[0]
        for w in range(1, W):
            den = den + e[w]
        inv = 1.0 / den
        p = [x * inv for x in e]
        for a in range(WH):
            pr_s[j, (hh * W + a) * HH:(hh * W + a + 1) * HH, :] = p[a]
        probs[j, hh] = p[WH:]

    def attn_pp(j, hh, t):
        _, bwd = mk_shift(at(t))
        p = probs.pop((j, hh))
        pn = probs[j + 1, hh] if j + 1 < NB else p
        for a in range(WH):
            pr_s[j, (hh * W + WH + a) * HH:(hh * W + WH + a + 1) * HH, :] = bwd(p[a], pn[a])
        ready.add(("pr", j, hh))

    def attn_pv(j, hh, dst, e, t, bd):
        assert not isinstance(j, int) or ("pr", j, hh) in ready
        assert e == 0 or ("o", dst, hh, e - 1) in ready
        pa = [pr_s[j, (hh * W + a) * HH:(hh * W + a + 1) * HH, :] for a in range(W)]
        p, pp = pa[:WH], pa[WH:]
        outs = []
        for d in range(DH):
            if d % G == 0:
                if d > 0:
                    hist.append([])
                fwd, _ = grp_shift(t + d * bd // DH, bd)
            r = hh * HD + d * HH
            v = v_s[j + 1, r:r + HH, :]
            vp = v_s[j, r:r + HH, :]
            o = op = None
            for a in range(WH):
                vs = fwd(v, vp, DIL * a)
                o = p[a] * vs if a == 0 else o + p[a] * vs
                op = pp[a] * vs if a == 0 else op + pp[a] * vs
            opp = zeros8 if (isinstance(j, int) and j == 0) else op_s[r:r + HH, :]
            op_s[r:r + HH, :] = op
            outs.append(o + fwd(op, opp, SH))
            ol[dst][r:r + HH, _blk(e)] = outs[-1]
        hist.append([])
        ready.add(("o", dst, hh, e))
        dls.append((t + bd + P["PVL"], _token(*outs)))

    ol = [ola_s, olb_s]
    mains = [("qk", j, hh) for j in range(NB) for hh in range(2)]
    mains = (mains[:P["PVPOS"]] + [("pv", j, hh) for j in range(4) for hh in range(2)]
             + mains[P["PVPOS"]:] + [None, None])
    slot_ctr = [0]

    def slot(t, bd):
        n = slot_ctr[0]
        slot_ctr[0] += 1
        it = mains[n]
        if it is None:
            pass
        elif it[0] == "qk":
            attn_qk(it[1], it[2], t, bd)
        else:
            attn_pv(it[1], it[2], 0, it[1], t, bd)
        if n >= 1 and mains[n - 1] is not None and mains[n - 1][0] == "qk":
            attn_sm(mains[n - 1][1], mains[n - 1][2], t + P["LS"])
        if n >= 2 and mains[n - 2] is not None and mains[n - 2][0] == "qk":
            _, j, hh = mains[n - 2]
            if j > 0:
                attn_pp(j - 1, hh, t + P["PP"])
            if j == NB - 1:
                attn_pp(j, hh, t + P["PP"])

    NRG = 8 * (NQ + 1) + 7
    PD = 8 * QD
    BORD = (1, 3, 2, 4, 0, 5, 6)
    LORD = (2, 4, 1, 3, 0, 5, 6)
    LAST_PARTS = [(0, QD, 1, 2), (QD, HD, 0, 2), (0, QD, 0, 1)]

    def rr_prep(p, pa, src, n0, n1, t0, dur):
        assert ("rr", p) not in ready
        for n in range(n0, n1):
            z = at(t0 + (n - n0) * dur // (n1 - n0))
            z2 = at(t0 + (n - n0) * dur // (n1 - n0) + P["SGR"])
            qd, g = divmod(n, 8)

            def wrow(i):
                return _rhs_op(p, lambda x, y: w2_v[pa + y, (2 * i + x) * LB + g * 16:(2 * i + x) * LB + g * 16 + 16, :]
                               .astype(f32))

            def orow(h):
                def blk(x, y):
                    assert ("o", src, x, 2 * y + 1) in ready
                    r = x * HD + h * QD + g * 16
                    return ol[src][r:r + 16, y * 2 * LB:(y + 1) * 2 * LB]
                return _rhs_op(p, blk)
            ro = p * RRK + g * 8
            if qd == NQ:
                if p in SIDX:
                    r = wrow(2 * NQ)
                    for e in range(2):
                        rr_s[ro:ro + 8, _blk(7 + e)] = _pk(tie8(r[:, _blk(e)], z))
                continue
            r1, r2 = (wrow(2 * qd), wrow(2 * qd + 1)) if qd < NQ else (orow(0), orow(1))
            ro += min(qd, NQ) * (LB // 2)
            c11, c22 = tie8(r1[:, :LB], z), tie8(r2[:, LB:], z2)
            sm = _rhs_sums(c11, r1[:, LB:], r2[:, :LB], c22)
            if p in SIDX or qd > NQ:
                sm.update({1: c11, 4: c22})
            for q, v in sm.items():
                rr_s[ro:ro + 8, _blk(q)] = _pk(v)
        if n1 == NRG:
            ready.add(("rr", p))

    def rr_tasks(p, pa, src, t0, t1):
        cuts = list(range(0, NRG, 8)) + [NRG]
        acc, tot = 0, sum(P["RW"])
        for a, b, w in zip(cuts[:-1], cuts[1:], P["RW"]):
            ta, tb = t0 + acc * (t1 - t0) // tot, t0 + (acc + w) * (t1 - t0) // tot
            add_tasks([(tb, rr_prep, (p, pa, src, a, b, ta, tb - ta))])
            acc += w

    def out_copy(pidx, e0, e1, r0, r1):
        off = pidx * (2 * LB) + e0 * LB
        if not isinstance(pidx, int):
            off = pl.multiple_of(off, LB)
        rs = pl.ds(r0, r1 - r0)
        return pltpu.make_async_copy(out_v.at[pidx, rs, pl.ds(e0 * LB, (e1 - e0) * LB)],
                                     out_hbm.at[0, rs, pl.ds(off, (e1 - e0) * LB)], sems.at[0])

    def b_out(pa, n, m, part, t0=None, dur=None):
        a, y = divmod(n, 2)
        r0, r1, e0, e1 = part
        cols = slice(e0 * LB, e1 * LB)
        for r in range(r0, r1, 16):
            c = _combine([None if v is None else v[r:r + 16, cols] for v in m], n)
            rows = slice(a * HD + r, a * HD + r + 16)
            o = c + x_v[pa + y, rows, cols].astype(f32)
            if t0 is not None:
                o = jnp.concatenate([tie(o[:, 0:LB], at(t0 + (r - r0) * dur // (r1 - r0))), o[:, LB:]], axis=1)
            out_v[pa + y, rows, cols] = o.astype(bf16)
        out_copy(pa + y, e0, e1, a * HD + r0, a * HD + r1).start()

    def big_piece(pa, pan, cur, last):
        t0 = now()
        for n in range(7):
            ta, tb = t0 + n * PD + P["RR0"], t0 + n * PD + P["RR1"]
            if n < 6:
                rr_tasks(BORD[n + 1], pa, cur, ta, tb)
            else:
                rr_tasks(BORD[0], pan, 1 - cur, ta, tb - (P["RRM"] if last else 0))
        ready.difference_update({("o", 1 - cur, hh, e) for hh in range(2) for e in range(4)})
        for n in range(8):
            e, hh = divmod(n, 2)
            t = t0 + P["BV0"] + n * P["BVS"]
            add_tasks([(t + P["BVD"], attn_pv, (pan * 2 + e, hh, 1 - cur, e, t, P["BVD"]))])
        m = [None] * 7
        for p in BORD:
            flush(now())
            assert ("rr", p) in ready
            x, y = TOP[p][0]

            def lhs(q):
                if q in (2, 3):
                    rows = slice(p * QD + (q - 2) * ED, p * QD + (q - 1) * ED)
                    return _up(jnp.concatenate([lc_s[rows, _blk(2 * qd + q - 2)] for qd in range(NQ)]
                                               + [lc_s[rows, (NFP + q - 2) * LB:(NFP + q - 2) * LB + QD]], axis=1))
                return _up(ll_s[(p * 7 + q) * ED:(p * 7 + q + 1) * ED, 0:KL])

            def rhs(q):
                if p in SIDX or q in SIDX:
                    return _up(rr_s[p * RRK:p * RRK + KL // 2, _blk(q)])
                h = 0 if q == 1 else 1
                return _cat([w2_v[pa + y, _blk(2 * (2 * qd + h) + x), _blk(h)] for qd in range(NQ)]
                            + [_up(rr_s[p * RRK + NQ * LB // 2:p * RRK + KL // 2, _blk(q)])], 0)
            rl = (_up(rr_s[p * RRK:p * RRK + LB // 2, 7 * LB:9 * LB]) if p in SIDX
                  else w2_v[pa + y, _blk(4 * NQ + x), :])
            ll = _up(lc_s[p * QD:(p + 1) * QD, _blk(2 * NQ)])
            ex = [mm1(ll[:QD], rl), mm1(ll[QD:], rl)]
            e12, e21 = ex[0][:, LB:], ex[1][:, :LB]
            e11 = (ex[0][:, :LB] + e12) - e21
            lf = strassen(lhs, rhs, LORD)
            ready.discard(("rr", p))
            if p in (2, 3):
                for q in (2, 3):
                    lf[q] = lf[q] + b2f_s[pa + 3 - p, 0:1, _blk(3 - q)]
            c12 = (lf[2] + e12) + lf[4]
            c21 = (lf[1] + e21) + lf[3]
            xx = (lf[2] - lf[1]) + lf[0]
            c22 = (xx + ex[1][:, LB:]) + lf[5]
            c11 = ((xx + e11) + (c21 - c12)) + lf[6]
            m[p] = jnp.concatenate([jnp.concatenate([c11, c12], axis=1),
                                    jnp.concatenate([c21, c22], axis=1)], axis=0)
            n = {3: 2, 4: 1, 5: 3, 6: 0}.get(p)
            if n is not None and not (last and n == 0):
                t, epd = now() + P["EP0"], P["EPL"] if (last and n == 3) else P["EPD"]
                add_tasks([(t + epd, b_out, (pa, n, list(m), (0, HD, 0, 2), t, epd))])
        if last:
            flush()
            for part in LAST_PARTS:
                b_out(pa, 0, m, part)

    def c_body(it, carry):
        reset()
        pos[:] = [one_s[...]]
        true.clear()
        ready.update({("rr", BORD[0])} | {("o", 0, hh, e) for hh in range(2) for e in range(4)})
        big_piece(4 * it, 4 * it + 2, 0, False)
        big_piece(4 * it + 2, lax.rem(4 * it + 4, NP), 1, True)
        assert ("rr", BORD[0]) in ready and all(("o", 0, hh, 3) in ready for hh in range(2))
        return carry

    E1 = P["E1"]
    x0 = Group(cp_x(0, 1))
    g1 = Group(cp_w1(0, 2, 0, E1))
    g2 = Group(cp_w1(0, 2, E1, NFP) + cp_x(1, 2))
    wq, wkv = [[(wqkv_hbm.at[:, cl], wqkv_v.at[:, cl])] for cl in (pl.ds(0, 4 * LB), pl.ds(4 * LB, 3 * D - 4 * LB))]
    g3 = Group(wq)
    g4 = Group(wkv + cp_x(2, 3))
    g5 = Group(cp_x(3, NP))
    g6 = Group(cp_w1(UB0, NB) + [(wo_hbm, wo_v), (b1_hbm, b1_v), (b2_hbm, b2_v)] + cp_w2(0, 1))
    g7 = Group(cp_w2(1, NP))
    for c in (x0, g1, g2, g3, g4, g5, g6, g7):
        c.start()

    v_s[0] = jnp.zeros((D, LB), f32)
    for buf in (xnT_s, ra_s, lh_s, rs_s, rr_s, ola_s, olb_s, ll_s, lc_s):
        buf[0:8, 0:64] = jnp.zeros((8, 64), buf.dtype)

    wait("x0", x0)
    one_s[...] = lax.shift_right_logical(pltpu.bitcast(x_v[0, 0:16, 0:LB], i32), 1) | 1
    pos[:] = [one_s[...]]
    ln(0)
    ln(1)
    hpair(0)
    wait("r1", g1)
    jobs = u_early(0, 0, E1, [], 7 * E1 // 4 * 4, P["T1"], 100)
    wait("r2", g2)
    t, dt = P["L2T"], P["L2D"]
    add_tasks([(t + int((k + 1) * dt * P["LNV"]), ln, (2 + k, t + int(k * dt * P["LNV"]), dt)) for k in range(2)])
    jobs = u_early(0, E1, NFP, jobs, P["N2"], P["T2"], 100)
    wait("wq", g3)
    add_tasks([(P["H2T"] + P["H2D"], hpair, (2, P["H2T"], P["H2D"]))])
    u_early(0, 0, 0, jobs, len(jobs), 0, 1, nsplit=P["S3"])
    prep_wqkv("q", 0, HD // 16, [P[k] for k in ("QA", "QB", "QC", "QE")])
    stage_a(0, "q", split_last=True)
    m = stage_a(2, "q", AORD[:P["NA3"]])
    wait("wkv", g4)
    stage_a(2, "q", AORD[P["NA3"]:], split_last=True, m=m)
    prep_wqkv("kv", HD // 16, HA // 16, [P[k] for k in ("KA", "KB", "KC", "KE")])
    t = ln_tasks(4, now() + P["L4T"], P["LND"], P["HSD"])
    n4 = min(4, (now() + 14 * HD - P["MARG"] - t) // P["BD"])
    add_tasks([(t + (n + 1) * P["BD"], slot, (t + n * P["BD"], P["BD"])) for n in range(n4)])
    stage_a(0, "kv")
    stage_a(2, "kv", order=(6,) + AORD[:6])

    wait("mid", g5)
    AD = 7 * HA // 2
    t = P["L5T"]
    for b in range(6, NB, 2):
        t = ln_tasks(b, t, P["LND"], P["HSD"])
    n5 = ((NP - 2) * AD - P["MARG"] - t) // P["BD"]
    add_tasks([(t + (n + 1) * P["BD"], slot, (t + n * P["BD"], P["BD"])) for n in range(n5)])
    n5 += n4
    for n, b in enumerate(range(4, NB, 2)):
        stage_a(b, order=(6,) + AORD[:6] if n % 2 else AORD)

    wait("fin", g6)
    UD = 7 * NUP * HD // 4
    for i in range(NFP):
        t0, dt = (-200, 130) if i == 0 else (800, 270) if i == 1 else ((i - 1) * UD + P["US0"], P["USD"])
        add_tasks([(t0 + (k + 1) * dt, tsum, (UB0 // 2 + k, i, i % 3, k, t0 + k * dt, dt)) for k in range(NUP)])
    left = len(mains) - n5 - 2
    bd = (NFP * UD - P["R6E"] - P["R6S"]) // left
    add_tasks([(P["R6S"] + (n + 1) * bd, slot, (P["R6S"] + n * bd, bd)) for n in range(left)])
    t = P["R6S"] + left * bd
    add_tasks([(t + (n + 1) * 300, slot, (t + n * 300, 300)) for n in range(2)])
    for qd, t0, t1 in ((NQ, UD + P["LL0"], 3 * UD), (0, 3 * UD + P["LL0"], 5 * UD), (1, 5 * UD + P["LL0"], 6 * UD + 200),
                       (2, 6 * UD + P["LL2"], 6 * UD + P["LL2"] + P["UEL"])):
        dt = (t1 - t0) // 7
        add_tasks([(t0 + (g + 1) * dt, llsum, (qd, g, t0 + g * dt, dt)) for g in range(7)])
    rr_tasks(BORD[0], 0, 0, P["RP0"], P["RP1"])
    add_tasks([(P["PW0"] + P["PWD"], prep_wo_a, (P["PW0"], P["PWD"]))])
    add_tasks([(P["PW1"] + (h + 1) * P["PWE"], prep_wo_b, (h, P["PW1"] + h * P["PWE"], P["PWE"])) for h in range(2)])
    for b in range(NB):
        b2f_s[b // 2, 0:1, _blk(b % 2)] = b2_v[b:b + 1, :].astype(f32)
    for i in range(NFP):
        u_last(i, (1, 4, 2, 3, 0, 5, 6) if i == 0 else (4, 2, 1, 3, 0, 5, 6),
               None if i == NFP - 1 else P["UEL"] if i == NFP - 2 else P["UED"])
    flush()
    assert slot_ctr[0] == len(mains) and all(("ll", qd, g) in ready for qd in range(NQ + 1) for g in range(7))
    assert all(("pr", j, hh) in ready for j in range(NB) for hh in range(2)) and ("rr", BORD[0]) in ready

    wait("w2", g7)
    lax.fori_loop(0, NP // 4, c_body, 0)
    outs = []
    for pa in range(0, NP, 2):
        outs += [out_copy(pa + n % 2, 0, 2, n // 2 * HD, (n // 2 + 1) * HD) for n in (1, 2, 3)]
        outs += [out_copy(pa, e0, e1, r0, r1) for (r0, r1, e0, e1) in (LAST_PARTS if pa % 4 else [(0, HD, 0, 2)])]
    wait("out", *outs)


@jax.jit
def pallas_parallel_sum__sliding_local_dilated__mixer_token_mlp__prompt_kernel(A_x, A_wqkv, A_wo, B_x, B_w1, B_b1, B_w2, B_b2):
    del B_x
    hbm = pl.BlockSpec(memory_space=pltpu.HBM)
    outT = pl.pallas_call(
        _kernel,
        out_shape=jax.ShapeDtypeStruct((1, D, S), bf16),
        in_specs=[hbm] * 7,
        out_specs=hbm,
        scratch_shapes=[
            pltpu.VMEM((NP, D, 2 * LB), bf16),
            pltpu.VMEM((D, 3 * D), bf16),
            pltpu.VMEM((D, D), bf16),
            pltpu.VMEM((S, F), bf16),
            pltpu.VMEM((NP, F, 2 * LB), bf16),
            pltpu.VMEM((NFB, LB), bf16),
            pltpu.VMEM((NB, LB), bf16),
            pltpu.VMEM((NP, D, 2 * LB), bf16),
            pltpu.VMEM((2, 3 * D + 64, LB), i32),
            pltpu.VMEM((7 * HA // 2, HD), u32),
            pltpu.VMEM((4, HD + 32, LB), i32),
            pltpu.VMEM((D, 2 * LB), i32),
            pltpu.VMEM((HD, S), u32),
            pltpu.VMEM((NP * QD, 5 * LB), u32),
            pltpu.VMEM((7 * QD, NP * LB), u32),
            pltpu.VMEM((7 * HD, NFP * LB), f32),
            pltpu.VMEM((7 * QD, (NFP + 2) * LB), u32),
            pltpu.VMEM((NB, 2 * D, LB), f32),
            pltpu.VMEM((NB + 1, D, LB), f32),
            pltpu.VMEM((NB, 2 * W * HH, LB), f32),
            pltpu.VMEM((D, LB), f32),
            pltpu.VMEM((NP, 32, 2 * LB), f32),
            pltpu.VMEM((4 * RSK, 5 * LB), u32),
            pltpu.VMEM((49 * ED, 4 * LB), u32),
            pltpu.VMEM((7 * RRK, 9 * LB), u32),
            pltpu.VMEM((D, 4 * LB), f32),
            pltpu.VMEM((D, 4 * LB), f32),
            pltpu.VMEM((8, LB), i32),
            pltpu.SemaphoreType.DMA((9,)),
        ],
        compiler_params=pltpu.CompilerParams(vmem_limit_bytes=100 * 1024 * 1024,
                                             disable_bounds_checks=True,
                                             disable_semaphore_checks=True),
    )(jnp.swapaxes(A_x, 1, 2), A_wqkv, A_wo, B_w1, B_b1.reshape(NFB, LB), B_w2, B_b2.reshape(NB, LB))
    return jnp.swapaxes(outT, 1, 2)
```

```python
import jax
import jax.numpy as jnp
from jax import lax
import jax.experimental.pallas as pl
import jax.experimental.pallas.tpu as pltpu

S, D, F = 2048, 448, 1792
H, DH, W, DIL = 16, 28, 8, 2
LB = 128
NB = S // LB
NP = NB // 2
NFB = F // LB
NFP = NFB // 2
HH = H // 2
WH = W // 2
SH = DIL * WH
HD = D // 2
QD = D // 4
ED = D // 8
HA = 3 * HD
UB0 = 2
NUP = (NB - UB0) // 2
RSK = NFP * LB // 2
NQ = NFP // 2
KL = NQ * LB + QD
RRK = 2 * LB
EPS = 1e-5
EPS_BF16 = 1.0013580322265625e-05
SCALE = DH ** -0.5
f32 = jnp.float32
bf16 = jnp.bfloat16
u32 = jnp.uint32
i32 = jnp.int32

SCOPES = False
P = dict(
    E1=3, E2=6, T3=-100, N2=16, NA3=2, T1=-200, T2=-200, L2T=100, L2D=440, H2T=900, H2D=360, L4T=1000, L5T=60, W2X=500,
    QA=-410, QB=200, QC=-200, QE=330, KA=50, KB=320, KC=450, KE=390,
    LND=420, HSD=350, HL=180, LNA=0.28, LNB=0.46, LNBD=0.38, LNV=0.86, LNW=0.93,
    BD=355, MARG=300, LAG=200, LS=150, PP=130, PVL=500, PVPOS=20,
    US0=100, USD=360, UE0=240, UED=2320, UEL=1700, UG=70, UM=0, R6S=1750, R6E=3150,
    LL0=300, LL2=550, RP0=16600, RP1=18700, PW0=560, PWD=300, PW1=1380, PWE=400,
    RR0=-48, RR1=800, RRM=-20, RW=(8, 8, 8, 2, 7), BV0=117, BVS=717, BVD=620, EP0=0, EPD=864, EPL=290, SGR=8, SGT=8, SH4=1,
)
G = 4


def _as(x, dtype):
    return x if x.dtype == dtype else pltpu.bitcast(x, dtype)


def _pk(x):
    return pltpu.bitcast(x.astype(bf16), u32)


def _up(x):
    return pltpu.bitcast(x, bf16)


def _upf(x):
    return pltpu.bitcast(x, bf16).astype(f32)


def _rb(x):
    return x.astype(bf16).astype(f32)


def _word(lo, hi):
    lo, hi = [pltpu.bitcast(v.astype(f32), i32) for v in (lo, hi)]
    return lax.shift_right_logical(lo, 16) | hi


def _unword(w):
    return [pltpu.bitcast(w << 16, f32), pltpu.bitcast(w & -65536, f32)]


def _cat(xs, axis):
    return xs[0] if len(xs) == 1 else jnp.concatenate(xs, axis=axis)


def _x2(v):
    return jnp.concatenate([v, v], axis=0)


def _blk(b):
    return slice(b * LB, (b + 1) * LB)


def _rowsum8(a):
    return jnp.broadcast_to(jnp.sum(a, axis=0, keepdims=True), (8, a.shape[1]))


def _token(*deps):
    deps = [d for d in deps if d is not None]
    if not deps:
        return None
    if len(deps) == 1:
        return deps[0]
    bits = _as(deps[0], u32)
    for d in deps[1:]:
        bits = bits | _as(d, u32)
    return bits


def _lhs_ops(a11, a12, a21, a22):
    return [a11 + a22, a21 + a22, a11, a22, a11 + a12, a21 - a11, a12 - a22]


SIDX = {0: 0, 2: 1, 3: 2, 5: 3, 6: 4}
TOP = {0: ((0, 0), 1, (1, 1)), 1: ((0, 0),), 2: ((0, 1), -1, (1, 1)), 3: ((1, 0), -1, (0, 0)),
       4: ((1, 1),), 5: ((0, 0), 1, (0, 1)), 6: ((1, 0), 1, (1, 1))}


def _rhs_sums(b11, b12, b21, b22):
    return {0: b11 + b22, 2: b12 - b22, 3: b21 - b11, 5: b11 + b12, 6: b21 + b22}


def _rhs_op(p, blk):
    t = TOP[p]
    if len(t) == 1:
        return blk(*t[0])
    return blk(*t[0]) + blk(*t[2]) if t[1] > 0 else blk(*t[0]) - blk(*t[2])


def _combine(m, n=None):
    c12 = lambda: m[2] + m[4]
    c21 = lambda: m[1] + m[3]
    x = lambda: (m[2] - m[1]) + m[0]
    c = [lambda: (x() + m[6]) + (c21() - c12()), c12, c21, lambda: x() + m[5]]
    return [f() for f in c] if n is None else c[n]()


def _kernel(x_hbm, wqkv_hbm, wo_hbm, w1_hbm, b1_hbm, w2_hbm, b2_hbm, out_hbm,
            x_v, w2_v, out_v, v_s, pr_s, b2f_s, wqkv_v, wo_v, w1_v, b1_v, b2_v, wt_s, lw_s, wo_s,
            wq_s, xnT_s, ra_s, lh_s, um_s, lc_s, qk_s, op_s, rs_s, ll_s, rr_s, ola_s, olb_s, one_s, sems):
    sem_ctr = [1]

    class Group:
        def __init__(self, pairs):
            self.cps = [pltpu.make_async_copy(a, b, sems.at[sem_ctr[0]]) for (a, b) in pairs]
            sem_ctr[0] += 1

        def start(self):
            for c in self.cps:
                c.start()

        def wait(self):
            for c in self.cps:
                c.wait()

    def cp_x(p0, p1):
        return [(x_hbm.at[0, :, pl.ds(p * 2 * LB, 2 * LB)], x_v.at[p]) for p in range(p0, p1)]

    def cp_w2(p0, p1):
        return [(w2_hbm.at[:, pl.ds(p * 2 * LB, 2 * LB)], w2_v.at[p]) for p in range(p0, p1)]

    def cp_w1(b0, b1, i0=0, i1=NFP):
        sl = pl.ds(b0 * LB, (b1 - b0) * LB)
        cl = pl.ds(i0 * 2 * LB, (i1 - i0) * 2 * LB)
        return [(w1_hbm.at[sl, cl], w1_v.at[sl, cl])]

    tl = []
    mxu = [0, 0, 0, 0]
    nxt = [0]
    hist = []
    tasks = []
    dls = []
    ready = set()
    pos = []
    true = {}

    def tie(v, z):
        if z is None:
            return v
        def fit(a):
            a = _cat([a] * (v.shape[0] // 8), 0)
            return a if v.shape[1] == LB else a[:, 0:v.shape[1]]
        if v.shape not in true:
            true[v.shape] = fit(pos[0]) > 0
        return lax.select(true[v.shape], v, fit(_as(z, v.dtype)))

    def tie8(v, z):
        return v if z is None else jnp.concatenate([tie(v[0:8], z), v[8:16]], axis=0)

    def add_tasks(todo):
        tasks.extend(todo)
        tasks.sort(key=lambda x: x[0])

    def flush(t=None):
        while tasks and (t is None or tasks[0][0] < t):
            _, fn, args = tasks.pop(0)
            fn(*args)

    def reset():
        assert not tasks
        dls.clear()
        tl.clear()
        hist.clear()
        mxu[:] = [0, 0, 0, 0]
        nxt[0] = 0

    def now():
        return sum(mxu) // 4

    def wait(name, *cps):
        flush()
        if SCOPES:
            with jax.named_scope("wait_" + name):
                for c in cps:
                    c.wait()
        else:
            for c in cps:
                c.wait()
        reset()

    def mm1(lhs, rhs, pace=True):
        flush(now())
        start = mxu[nxt[0]]
        due = [v for (t, v) in dls if t <= start] if pace else []
        if due:
            dls[:] = [(t, v) for (t, v) in dls if t > start]
            tile = _up(tie(pltpu.bitcast(lhs[0:16, 0:LB], u32), _token(*due)))
            row = tile if lhs.shape[1] == LB else jnp.concatenate([tile, lhs[0:16, LB:]], axis=1)
            lhs = jnp.concatenate([row, lhs[16:]], axis=0)
        r = jnp.dot(lhs, rhs, preferred_element_type=f32)
        m, k = lhs.shape
        first_done = None
        for _ in range(-(-rhs.shape[1] // LB)):
            end = 0
            for _ in range(-(-k // LB)):
                mxu[nxt[0]] += m
                end = max(end, mxu[nxt[0]])
                nxt[0] = (nxt[0] + 1) % 4
            if first_done is None:
                first_done = end
        if pace:
            tl.append((first_done - m, first_done, r))
        return r

    def mm(lhs, rhs, init=None):
        k = lhs.shape[1]
        r, k0 = init, 0
        while k0 < k:
            k1 = min(k, k0 + (4 - nxt[0]) * LB)
            part = mm1(lhs[:, k0:k1], rhs[k0:k1], pace=k1 - k0 > LB)
            r = part if r is None else r + part
            k0 = k1
        return r

    def at(t, *more):
        best = None
        if t is not None and t >= 0:
            t = min(t, now() - 1)
            for (a, b, r) in tl:
                if a <= t and (best is None or min(b, t) > best[0]):
                    row = int(min((t - a) / (b - a), 0.999) * (r.shape[0] // 8)) * 8
                    best = (min(b, t), r, row)
        return _token(None if best is None else best[1][best[2]:best[2] + 8, 0:LB], *more)

    def strassen(lhs, rhs, order, split_last=False, init=None, m=None):
        m = [None] * 7 if m is None else m
        for p in order:
            flush(now())
            l, r = lhs(p), rhs(p)
            c0 = None if init is None else init[p]
            if split_last and p == order[-1]:
                kk = (-(-r.shape[0] // LB) - 2) * LB
                hm = l.shape[0] // 2
                hd = mm(l[:, :kk], r[:kk], c0) if kk else c0
                tail = jnp.concatenate([mm(l[:hm, kk:], r[kk:]), mm(l[hm:, kk:], r[kk:])], axis=0)
                m[p] = tail if hd is None else hd + tail
            else:
                m[p] = mm(l, r, c0)
        return m

    def wcol(hh, p):
        return p * D + (1 - hh if p == 1 else hh) * HD

    def wrows(hh, g, z=None):
        p, d = divmod(2 * g, DH)
        t = [jnp.concatenate([wt_s[c, pl.ds(wcol(hh, p) + d + e, HH, stride=DH), :]
                              for e in range(2)], axis=0) for c in range(2)]
        return _unword(jnp.concatenate([tie(t[0], z), tie(t[1][:, 0:HD - LB], z)], axis=1))

    wt_done = set()

    def prep_wqkv(part, ga, gb, paced):
        def need(hh, p, z):
            lo = wcol(hh, p)
            for ct in range(lo // LB, -(-(lo + HD) // LB)):
                if ct in wt_done:
                    continue
                wt_done.add(ct)
                cols = slice(ct * LB, min((ct + 1) * LB, 3 * D))
                wd = _word(wqkv_v[0:HD, cols], wqkv_v[HD:D, cols])
                wd = jnp.concatenate([tie(wd[r:r + 8], z if r % LB == 0 else None) for r in range(0, HD, 8)], axis=0)
                wT = wd.T
                wt_s[0, cols, :] = wT[:, 0:LB]
                wt_s[1, cols, 0:HD - LB] = wT[:, LB:HD]

        def put(p, g, v):
            lw_s[p * (HA // 2) + g * 8:p * (HA // 2) + g * 8 + 8, :] = _pk(v)

        def half(hh, g0, g1, t0=None, dur=None):
            pr, ps = ((2, 4), (3, 1))[hh]
            for g in range(g0, g1):
                t = None if t0 is None else t0 + (g - g0) * dur // (g1 - g0)
                need(hh, 2 * g // DH, at(None if t is None else t - P["W2X"]))
                a1, a2 = wrows(hh, g, at(t))
                put(pr, g, a2 if hh else a1)
                put(ps, g, a1 + a2)
            if g1 == gb:
                ready.update({("lw", part, pr), ("lw", part, ps)})

        def rest(g0, g1, t0, dur):
            assert ("lw", part, 1) in ready
            for g in range(g0, g1):
                z = at(t0 + (g - g0) * dur // (g1 - g0))
                ops = _lhs_ops(*wrows(0, g, z), *wrows(1, g, z))
                for p in (0, 5, 6):
                    put(p, g, ops[p])
            if g1 == gb:
                ready.update({("lw", part, 0), ("lw", part, 5), ("lw", part, 6)})
        t2, d2, t3, d3 = paced
        half(0, ga, gb)
        n = (gb - ga) // 14
        add_tasks([(now() + t2 + (k + 1) * d2 // n, half,
                    (1, ga + 14 * k, ga + 14 * k + 14, now() + t2 + k * d2 // n, d2 // n)) for k in range(n)])
        n = (gb - ga) // 7
        add_tasks([(now() + t3 + (k + 1) * d3 // n, rest,
                    (ga + 7 * k, ga + 7 * k + 7, now() + t3 + k * d3 // n, d3 // n)) for k in range(n)])

    def prep_wo_a(t0, dur):
        for g in range(HD // 16):
            w = _word(wo_v[g * 16:g * 16 + 16, :], wo_v[HD + g * 16:HD + g * 16 + 16, :])
            z = at(t0 + g * dur // (HD // 16))
            for c in range(4):
                cw = min(LB, D - c * LB)
                wo_s[c, g * 16:g * 16 + 16, 0:cw] = tie(w[:, c * LB:c * LB + cw], z)
        ready.add("wo")

    def prep_wo_b(h, t0, dur):
        assert "wo" in ready
        for c in range(4):
            cw = min(LB, D - c * LB)
            rows = [wo_s[c, pl.ds(d, HH, stride=DH), :][:, 0:cw] for d in range(h * DH // 2, (h + 1) * DH // 2)]
            rows.append(jnp.zeros((LB - QD, cw), i32))
            wq_s[c * LB:c * LB + cw, _blk(h)] = jnp.concatenate(rows, axis=0).T
        outs = []
        for g in range(HD // 16):
            z = at(t0 + g * dur // (HD // 16))
            a = [v for r in (g * 16, HD + g * 16) for v in _unword(tie(wq_s[r:r + 16, _blk(h)], z))]
            for p, v in enumerate(_lhs_ops(*a)):
                lc_s[p * QD + g * 8:p * QD + g * 8 + 8, _blk(NFP + h)] = _pk(v)
                outs.append(v[0:8])
        ready.update({("lc", NFP + h, g) for g in range(HD // 16)})
        dls.append((t0 + dur + 250, _token(*outs)))

    RG = 16
    NG = D // RG
    stat2 = {}

    def ln(b, t0=None, dur=None):
        def xg(g):
            return x_v[b // 2, g * RG:(g + 1) * RG, _blk(b % 2)].astype(f32)

        def step(v, g, fr, s, q):
            if t0 is None or g % 4:
                return v
            acc = [] if s is None else [s[0:8], s[8:16], q[0:8], q[8:16]]
            return tie(v, at(t0 + fr * dur, *acc))

        x0 = jnp.broadcast_to(xg(0)[0:1], (8, LB))
        s = q = None
        for g in range(NG):
            x0 = step(x0, g, P["LNA"] * g / NG, s, q)
            c = xg(g) - _x2(x0)
            s = c if s is None else s + c
            q = c * c if q is None else q + c * c
        dm = _rowsum8(s) * (1.0 / D)
        mu = _rb(x0 + dm)
        var = _rb(jnp.maximum(_rowsum8(q) * (1.0 / D) - dm * dm, 0.0))
        r1 = 1.0 / _rb(jnp.sqrt(_rb(var + EPS_BF16)))
        s = q = None
        for g in range(NG):
            mu = step(mu, g, P["LNB"] + P["LNBD"] * g / NG, s, q)
            xn = _rb(xg(g) - _x2(mu)) * _x2(r1)
            xnT_s[g * 8:g * 8 + 8, _blk(b)] = _pk(xn)
            s = xn if s is None else s + xn
            q = xn * xn if q is None else q + xn * xn
        mu2 = _rowsum8(s) * (1.0 / D)
        var2 = jnp.maximum(_rowsum8(q) * (1.0 / D) - mu2 * mu2, 0.0)
        stat2[b] = (mu2, 0.5 * lax.rsqrt(var2 + EPS))

    def hpair(b, t0=None, dur=None):
        ng = HD // RG
        st = [stat2.pop(b), stat2.pop(b + 1)]
        for g in range(ng):
            zz = [at(None if t0 is None else t0 + (4 * g + k * P["SH4"]) * dur // (4 * ng)) for k in (0, 1, 2, 3)]
            xq = [_upf(tie(xnT_s[r:r + 8, _blk(b + e)], zz[2 * (r >= QD) + e]))
                  for r in (g * 8, QD + g * 8) for e in range(2)]
            hq = [(v - _x2(st[n % 2][0])) * _x2(st[n % 2][1]) for n, v in enumerate(xq)]
            ro = (b // 2) * QD + g * 8
            for p, v in _rhs_sums(*xq).items():
                ra_s[ro:ro + 8, _blk(SIDX[p])] = _pk(v)
            for p, v in enumerate(_lhs_ops(*hq)):
                lh_s[p * QD + g * 8:p * QD + g * 8 + 8, _blk(b // 2)] = _pk(v)
        ready.add(("xn", b))
        if b >= 6:
            got = ra_s[(b // 2) * QD:(b // 2 + 1) * QD, :]
            dls.append((t0 + dur + P["HL"], _token(*[got[r:r + 8, _blk(c)] for r in range(0, QD, 8) for c in range(5)])))

    def ln_tasks(b, t, lnd, hsd):
        for fn, bb, dur, adv in ((ln, b, lnd, P["LNV"]), (ln, b + 1, lnd, P["LNW"]), (hpair, b, hsd, 1.0)):
            add_tasks([(t + int(dur * adv), fn, (bb, t, dur))])
            t += int(dur * adv)
        return t

    def tsum(kp, i, slot_, n, t0, dur):
        for g in range(LB // 16):
            z, z2 = at(t0 + g * dur // 8), at(t0 + g * dur // 8 + P["SGT"])
            t1, t2 = [w1_v[(2 * kp + e) * LB + g * 16:(2 * kp + e) * LB + g * 16 + 16,
                           2 * i * LB:(2 * i + 2) * LB].astype(f32) for e in range(2)]
            ro = slot_ * RSK + n * (LB // 2) + g * 8
            for p, v in _rhs_sums(tie8(t1[:, :LB], z), t1[:, LB:], t2[:, :LB], tie8(t2[:, LB:], z2)).items():
                rs_s[ro:ro + 8, _blk(SIDX[p])] = _pk(v)
        ready.add(("rs", kp, i))

    def u_rhs(p, i, kps, slot_, n0):
        if p in SIDX:
            assert all(("rs", kp, i) in ready for kp in kps)
            ro = slot_ * RSK + n0 * (LB // 2)
            return _up(rs_s[ro:ro + len(kps) * (LB // 2), _blk(SIDX[p])])
        e = 0 if p == 1 else 1
        return _cat([w1_v[_blk(2 * kp + e), _blk(2 * i + e)] for kp in kps], 0)

    LATE = (NFP - 1, 6)

    def ujob(kp, i, p, split):
        flush(now())
        assert ("xn", 2 * kp) in ready
        l, r = _up(lh_s[p * QD:(p + 1) * QD, _blk(kp)]), u_rhs(p, i, [kp], 3 + kp, i)
        v = jnp.concatenate([mm1(l[:QD], r), mm1(l[QD:], r)], axis=0) if split else mm1(l, r)
        rows = slice(p * HD, (p + 1) * HD)
        um_s[rows, _blk(i)] = v

    def u_early(kp, i0, i1, carry, n, t0, dt, nsplit=0):
        for k, i in enumerate(range(i0, i1)):
            add_tasks([(t0 + (k + 1) * dt, tsum, (kp, i, 3 + kp, i, t0 + k * dt, dt))])
        jobs = (carry + [(kp, i, p) for i in range(i0, i1) for p in (1, 4)]
                + [(kp, i, p) for i in range(i0, i1) for p in SIDX if (i, p) != LATE])
        for c, job in enumerate(jobs[:n]):
            ujob(*job, c >= n - nsplit)
        return jobs[n:]

    def gelu_half(hx, z):
        c = 0.7978845608028654
        return hx + hx * jnp.tanh(tie(hx * (2.0 * c + (8.0 * c * 0.044715) * (hx * hx)), z))

    def u_epilogue(i, m, gs, t0, dur):
        for n, g in enumerate(gs):
            t = None if t0 is None else t0 + n * dur // len(gs) - P["UG"]
            q = _combine([x[g * 16:g * 16 + 16] for x in m])
            gl = [gelu_half(v, at(None if t is None else t - k * P["UM"])) for v, k in zip(q, (0, 3, 2, 1))]
            for p, v in enumerate(_lhs_ops(*gl)):
                lc_s[p * QD + g * 8:p * QD + g * 8 + 8, _blk(i)] = _pk(v)
            ready.add(("lc", i, g))

    def u_last(i, order, edur):
        kps = list(range(UB0 // 2, NP))
        init = [None if (i, p) == LATE else um_s[p * HD:(p + 1) * HD, _blk(i)] for p in range(7)]
        for p in (2, 3):
            init[p] = init[p] + 0.5 * b1_v[2 * i + 3 - p:2 * i + 4 - p, :].astype(f32)
        m = strassen(lambda p: _up(lh_s[p * QD:(p + 1) * QD, (0 if (i, p) == LATE else UB0 // 2 * LB):]),
                     lambda p: _cat([u_rhs(p, i, [0], 3, i)] * ((i, p) == LATE) + [u_rhs(p, i, kps, i % 3, 0)], 0),
                     order, init=init)
        if edur is None:
            u_epilogue(i, m, list(range(HD // 16)), None, None)
        else:
            t = now() + P["UE0"]
            add_tasks([(t + (g + 1) * edur // 7, u_epilogue, (i, m, [g, g + 7], t + g * edur // 7, edur // 7))
                       for g in range(7)])

    def llsum(qd, g, t0, dur):
        i0 = 2 * qd if qd < NQ else NFP
        assert all(("lc", i0 + e, g + 7 * h) in ready for e in range(2) for h in range(2))
        for p in range(7):
            zz = [at(t0 + p * dur // 7), at(t0 + p * dur // 7 + P["SGT"])]
            a = [tie(lc_s[p * QD + h * ED + g * 8:p * QD + h * ED + g * 8 + 8, _blk(i0 + e)], zz[h] if h == e else None)
                 for h in range(2) for e in range(2)]
            ops = _lhs_ops(*[_upf(v) for v in a])
            for q in (0, 1, 4, 5, 6):
                r = (p * 7 + q) * ED + g * 8
                ll_s[r:r + 8, _blk(qd)] = _pk(ops[q])
        ready.add(("ll", qd, g))

    AORD = (4, 2, 1, 3, 0, 5, 6)

    def stage_a(b, parts="qkv", order=AORD, split_last=False, m=None):
        r0, r1 = {"q": (0, HD), "kv": (HD, HA), "qkv": (0, HA)}[parts]

        def lhs(p):
            assert all(("lw", pt, p) in ready for pt in ("q", "kv") if pt in parts)
            return _up(lw_s[(p * HA + r0) // 2:(p * HA + r1) // 2, :])

        def rhs(p):
            assert ("xn", b) in ready
            if p in SIDX:
                return _up(ra_s[(b // 2) * QD:(b // 2 + 1) * QD, _blk(SIDX[p])])
            return _up(xnT_s[0:QD, _blk(b)] if p == 1 else xnT_s[QD:HD, _blk(b + 1)])
        m = strassen(lhs, rhs, order, split_last, m=m)
        for n, ps in enumerate((range(7), (2, 4), (1, 3), (0, 1, 2, 5))):
            if all(m[p] is not None for p in ps) and any(p in order for p in ps):
                hh, e = divmod(n, 2)
                c = _combine(m, n)
                qk_s[b + e, hh * D + r0:hh * D + min(r1, D), :] = c[0:min(r1, D) - r0]
                if r1 > D:
                    v_s[b + e + 1, hh * HD:(hh + 1) * HD, :] = c[D - r0:]
        if all(v is not None for v in m):
            ready.update({(pt, b + e) for pt in ("q", "kv") if pt in parts for e in range(2)})
        return m

    lane0 = lax.broadcasted_iota(i32, (HH, LB), 1)
    zeros8 = jnp.zeros((HH, LB), f32)

    def mk_shift(z):
        lane = tie(lane0, z)
        masks = {}

        def pick(n, a, b):
            if n not in masks:
                masks[n] = lane < n
            return lax.select(masks[n], a, b)

        def fwd(cur, prev, sh):
            return cur if sh == 0 else pltpu.roll(pick(LB - sh, cur, prev), sh, 1)

        def bwd(cur, nxt_):
            return pltpu.roll(pick(SH, nxt_, cur), LB - SH, 1)
        return fwd, bwd

    def grp_shift(t, bd):
        lag = max(2, -(-P["LAG"] * DH // (G * bd)))
        return mk_shift(at(t, *(hist[-lag] if len(hist) >= lag else [])))

    raw, probs = {}, {}

    def attn_qk(j, hh, t, bd):
        jn = min(j + 1, NB - 1)
        assert ("q", jn) in ready and ("kv", j) in ready
        acc = [None] * WH
        accp = [None] * WH
        for d in range(DH):
            if d % G == 0:
                if d > 0:
                    hist.append(acc + accp)
                fwd, bwd = grp_shift(t + d * bd // DH, bd)
            r = hh * D + d * HH
            q = qk_s[j, r:r + HH, :]
            qp = bwd(q, qk_s[jn, r:r + HH, :])
            rk = (1 - hh) * D + HD + d * HH
            k = qk_s[j, rk:rk + HH, :]
            kp = qk_s[j - 1, rk:rk + HH, :] if j > 0 else zeros8
            for a in range(WH):
                ks = fwd(k, kp, DIL * a)
                t0, t1 = q * ks, qp * ks
                acc[a] = t0 if d == 0 else acc[a] + t0
                accp[a] = t1 if d == 0 else accp[a] + t1
        hist.append(acc + accp)
        raw[j, hh] = (acc, accp)

    def attn_sm(j, hh, t):
        fwd, _ = mk_shift(at(t))
        acc, accp = raw[j, hh]
        prev = raw.pop((j - 1, hh))[1] if j > 0 else [zeros8] * WH
        lg = acc + [fwd(accp[a], prev[a], SH) for a in range(WH)]
        lg = [a * SCALE for a in lg]
        if j == 0:
            lg = [lg[0]] + [jnp.where(lane0 >= DIL * w, lg[w], -1e9) for w in range(1, W)]
        m = lg[0]
        for w in range(1, W):
            m = jnp.maximum(m, lg[w])
        e = [jnp.exp(l - m) for l in lg]
        den = e[0]
        for w in range(1, W):
            den = den + e[w]
        inv = 1.0 / den
        p = [x * inv for x in e]
        for a in range(WH):
            pr_s[j, (hh * W + a) * HH:(hh * W + a + 1) * HH, :] = p[a]
        probs[j, hh] = p[WH:]

    def attn_pp(j, hh, t):
        _, bwd = mk_shift(at(t))
        p = probs.pop((j, hh))
        pn = probs[j + 1, hh] if j + 1 < NB else p
        for a in range(WH):
            pr_s[j, (hh * W + WH + a) * HH:(hh * W + WH + a + 1) * HH, :] = bwd(p[a], pn[a])
        ready.add(("pr", j, hh))

    def attn_pv(j, hh, dst, e, t, bd):
        assert not isinstance(j, int) or ("pr", j, hh) in ready
        assert e == 0 or ("o", dst, hh, e - 1) in ready
        pa = [pr_s[j, (hh * W + a) * HH:(hh * W + a + 1) * HH, :] for a in range(W)]
        p, pp = pa[:WH], pa[WH:]
        outs = []
        for d in range(DH):
            if d % G == 0:
                if d > 0:
                    hist.append([])
                fwd, _ = grp_shift(t + d * bd // DH, bd)
            r = hh * HD + d * HH
            v = v_s[j + 1, r:r + HH, :]
            vp = v_s[j, r:r + HH, :]
            o = op = None
            for a in range(WH):
                vs = fwd(v, vp, DIL * a)
                o = p[a] * vs if a == 0 else o + p[a] * vs
                op = pp[a] * vs if a == 0 else op + pp[a] * vs
            opp = zeros8 if (isinstance(j, int) and j == 0) else op_s[r:r + HH, :]
            op_s[r:r + HH, :] = op
            outs.append(o + fwd(op, opp, SH))
            ol[dst][r:r + HH, _blk(e)] = outs[-1]
        hist.append([])
        ready.add(("o", dst, hh, e))
        dls.append((t + bd + P["PVL"], _token(*outs)))

    ol = [ola_s, olb_s]
    mains = [("qk", j, hh) for j in range(NB) for hh in range(2)]
    mains = (mains[:P["PVPOS"]] + [("pv", j, hh) for j in range(4) for hh in range(2)]
             + mains[P["PVPOS"]:] + [None, None])
    slot_ctr = [0]

    def slot(t, bd):
        n = slot_ctr[0]
        slot_ctr[0] += 1
        it = mains[n]
        if it is None:
            pass
        elif it[0] == "qk":
            attn_qk(it[1], it[2], t, bd)
        else:
            attn_pv(it[1], it[2], 0, it[1], t, bd)
        if n >= 1 and mains[n - 1] is not None and mains[n - 1][0] == "qk":
            attn_sm(mains[n - 1][1], mains[n - 1][2], t + P["LS"])
        if n >= 2 and mains[n - 2] is not None and mains[n - 2][0] == "qk":
            _, j, hh = mains[n - 2]
            if j > 0:
                attn_pp(j - 1, hh, t + P["PP"])
            if j == NB - 1:
                attn_pp(j, hh, t + P["PP"])

    NRG = 8 * (NQ + 1) + 7
    PD = 8 * QD
    BORD = (1, 3, 2, 4, 0, 5, 6)
    LORD = (2, 4, 1, 3, 0, 5, 6)
    LAST_PARTS = [(0, QD, 1, 2), (QD, HD, 0, 2), (0, QD, 0, 1)]

    def rr_prep(p, pa, src, n0, n1, t0, dur):
        assert ("rr", p) not in ready
        for n in range(n0, n1):
            z = at(t0 + (n - n0) * dur // (n1 - n0))
            z2 = at(t0 + (n - n0) * dur // (n1 - n0) + P["SGR"])
            qd, g = divmod(n, 8)

            def wrow(i):
                return _rhs_op(p, lambda x, y: w2_v[pa + y, (2 * i + x) * LB + g * 16:(2 * i + x) * LB + g * 16 + 16, :]
                               .astype(f32))

            def orow(h):
                def blk(x, y):
                    assert ("o", src, x, 2 * y + 1) in ready
                    r = x * HD + h * QD + g * 16
                    return ol[src][r:r + 16, y * 2 * LB:(y + 1) * 2 * LB]
                return _rhs_op(p, blk)
            ro = p * RRK + g * 8
            if qd == NQ:
                if p in SIDX:
                    r = wrow(2 * NQ)
                    for e in range(2):
                        rr_s[ro:ro + 8, _blk(7 + e)] = _pk(tie8(r[:, _blk(e)], z))
                continue
            r1, r2 = (wrow(2 * qd), wrow(2 * qd + 1)) if qd < NQ else (orow(0), orow(1))
            ro += min(qd, NQ) * (LB // 2)
            c11, c22 = tie8(r1[:, :LB], z), tie8(r2[:, LB:], z2)
            sm = _rhs_sums(c11, r1[:, LB:], r2[:, :LB], c22)
            if p in SIDX or qd > NQ:
                sm.update({1: c11, 4: c22})
            for q, v in sm.items():
                rr_s[ro:ro + 8, _blk(q)] = _pk(v)
        if n1 == NRG:
            ready.add(("rr", p))

    def rr_tasks(p, pa, src, t0, t1):
        cuts = list(range(0, NRG, 8)) + [NRG]
        acc, tot = 0, sum(P["RW"])
        for a, b, w in zip(cuts[:-1], cuts[1:], P["RW"]):
            ta, tb = t0 + acc * (t1 - t0) // tot, t0 + (acc + w) * (t1 - t0) // tot
            add_tasks([(tb, rr_prep, (p, pa, src, a, b, ta, tb - ta))])
            acc += w

    def out_copy(pidx, e0, e1, r0, r1):
        off = pidx * (2 * LB) + e0 * LB
        if not isinstance(pidx, int):
            off = pl.multiple_of(off, LB)
        rs = pl.ds(r0, r1 - r0)
        return pltpu.make_async_copy(out_v.at[pidx, rs, pl.ds(e0 * LB, (e1 - e0) * LB)],
                                     out_hbm.at[0, rs, pl.ds(off, (e1 - e0) * LB)], sems.at[0])

    def b_out(pa, n, m, part, t0=None, dur=None):
        a, y = divmod(n, 2)
        r0, r1, e0, e1 = part
        cols = slice(e0 * LB, e1 * LB)
        for r in range(r0, r1, 16):
            c = _combine([None if v is None else v[r:r + 16, cols] for v in m], n)
            rows = slice(a * HD + r, a * HD + r + 16)
            o = c + x_v[pa + y, rows, cols].astype(f32)
            if t0 is not None:
                o = jnp.concatenate([tie(o[:, 0:LB], at(t0 + (r - r0) * dur // (r1 - r0))), o[:, LB:]], axis=1)
            out_v[pa + y, rows, cols] = o.astype(bf16)
        out_copy(pa + y, e0, e1, a * HD + r0, a * HD + r1).start()

    def big_piece(pa, pan, cur, last):
        t0 = now()
        for n in range(7):
            ta, tb = t0 + n * PD + P["RR0"], t0 + n * PD + P["RR1"]
            if n < 6:
                rr_tasks(BORD[n + 1], pa, cur, ta, tb)
            else:
                rr_tasks(BORD[0], pan, 1 - cur, ta, tb - (P["RRM"] if last else 0))
        ready.difference_update({("o", 1 - cur, hh, e) for hh in range(2) for e in range(4)})
        for n in range(8):
            e, hh = divmod(n, 2)
            t = t0 + P["BV0"] + n * P["BVS"]
            add_tasks([(t + P["BVD"], attn_pv, (pan * 2 + e, hh, 1 - cur, e, t, P["BVD"]))])
        m = [None] * 7
        for p in BORD:
            flush(now())
            assert ("rr", p) in ready
            x, y = TOP[p][0]

            def lhs(q):
                if q in (2, 3):
                    rows = slice(p * QD + (q - 2) * ED, p * QD + (q - 1) * ED)
                    return _up(jnp.concatenate([lc_s[rows, _blk(2 * qd + q - 2)] for qd in range(NQ)]
                                               + [lc_s[rows, (NFP + q - 2) * LB:(NFP + q - 2) * LB + QD]], axis=1))
                return _up(ll_s[(p * 7 + q) * ED:(p * 7 + q + 1) * ED, 0:KL])

            def rhs(q):
                if p in SIDX or q in SIDX:
                    return _up(rr_s[p * RRK:p * RRK + KL // 2, _blk(q)])
                h = 0 if q == 1 else 1
                return _cat([w2_v[pa + y, _blk(2 * (2 * qd + h) + x), _blk(h)] for qd in range(NQ)]
                            + [_up(rr_s[p * RRK + NQ * LB // 2:p * RRK + KL // 2, _blk(q)])], 0)
            rl = (_up(rr_s[p * RRK:p * RRK + LB // 2, 7 * LB:9 * LB]) if p in SIDX
                  else w2_v[pa + y, _blk(4 * NQ + x), :])
            ll = _up(lc_s[p * QD:(p + 1) * QD, _blk(2 * NQ)])
            ex = [mm1(ll[:QD], rl), mm1(ll[QD:], rl)]
            e12, e21 = ex[0][:, LB:], ex[1][:, :LB]
            e11 = (ex[0][:, :LB] + e12) - e21
            lf = strassen(lhs, rhs, LORD)
            ready.discard(("rr", p))
            if p in (2, 3):
                for q in (2, 3):
                    lf[q] = lf[q] + b2f_s[pa + 3 - p, 0:1, _blk(3 - q)]
            c12 = (lf[2] + e12) + lf[4]
            c21 = (lf[1] + e21) + lf[3]
            xx = (lf[2] - lf[1]) + lf[0]
            c22 = (xx + ex[1][:, LB:]) + lf[5]
            c11 = ((xx + e11) + (c21 - c12)) + lf[6]
            m[p] = jnp.concatenate([jnp.concatenate([c11, c12], axis=1),
                                    jnp.concatenate([c21, c22], axis=1)], axis=0)
            n = {3: 2, 4: 1, 5: 3, 6: 0}.get(p)
            if n is not None and not (last and n == 0):
                t, epd = now() + P["EP0"], P["EPL"] if (last and n == 3) else P["EPD"]
                add_tasks([(t + epd, b_out, (pa, n, list(m), (0, HD, 0, 2), t, epd))])
        if last:
            flush()
            for part in LAST_PARTS:
                b_out(pa, 0, m, part)

    def c_body(it, carry):
        reset()
        pos[:] = [one_s[...]]
        true.clear()
        ready.update({("rr", BORD[0])} | {("o", 0, hh, e) for hh in range(2) for e in range(4)})
        big_piece(4 * it, 4 * it + 2, 0, False)
        big_piece(4 * it + 2, lax.rem(4 * it + 4, NP), 1, True)
        assert ("rr", BORD[0]) in ready and all(("o", 0, hh, 3) in ready for hh in range(2))
        return carry

    E1, E2 = P["E1"], P["E2"]
    x0 = Group(cp_x(0, 1))
    g1 = Group(cp_w1(0, 2, 0, E1))
    g2 = Group(cp_w1(0, 2, E1, E2) + cp_x(1, 2))
    wq, wkv = [[(wqkv_hbm.at[:, cl], wqkv_v.at[:, cl])] for cl in (pl.ds(0, 4 * LB), pl.ds(4 * LB, 3 * D - 4 * LB))]
    g3 = Group((cp_w1(0, 2, E2, NFP) if E2 < NFP else []) + wq)
    g4 = Group(wkv + cp_x(2, 3))
    g5 = Group(cp_x(3, NP))
    g6 = Group(cp_w1(UB0, NB) + [(wo_hbm, wo_v), (b1_hbm, b1_v), (b2_hbm, b2_v)] + cp_w2(0, 1))
    g7 = Group(cp_w2(1, NP))
    for c in (x0, g1, g2, g3, g4, g5, g6, g7):
        c.start()

    v_s[0] = jnp.zeros((D, LB), f32)
    for buf in (xnT_s, ra_s, lh_s, rs_s, rr_s, ola_s, olb_s, ll_s, lc_s):
        buf[0:8, 0:64] = jnp.zeros((8, 64), buf.dtype)

    wait("x0", x0)
    one_s[...] = lax.shift_right_logical(pltpu.bitcast(x_v[0, 0:16, 0:LB], i32), 1) | 1
    pos[:] = [one_s[...]]
    ln(0)
    ln(1)
    hpair(0)
    wait("r1", g1)
    jobs = u_early(0, 0, E1, [], 7 * E1 // 4 * 4, P["T1"], 100)
    wait("r2", g2)
    t, dt = P["L2T"], P["L2D"]
    add_tasks([(t + int((k + 1) * dt * P["LNV"]), ln, (2 + k, t + int(k * dt * P["LNV"]), dt)) for k in range(2)])
    jobs = u_early(0, E1, E2, jobs, P["N2"], P["T2"], 100)
    wait("wq", g3)
    add_tasks([(P["H2T"] + P["H2D"], hpair, (2, P["H2T"], P["H2D"]))])
    u_early(0, E2, NFP, jobs, 7 * NFP, P["T3"], 100)
    prep_wqkv("q", 0, HD // 16, [P[k] for k in ("QA", "QB", "QC", "QE")])
    stage_a(0, "q", split_last=True)
    m = stage_a(2, "q", AORD[:P["NA3"]])
    wait("wkv", g4)
    stage_a(2, "q", AORD[P["NA3"]:], split_last=True, m=m)
    prep_wqkv("kv", HD // 16, HA // 16, [P[k] for k in ("KA", "KB", "KC", "KE")])
    t = ln_tasks(4, now() + P["L4T"], P["LND"], P["HSD"])
    n4 = min(4, (now() + 14 * HD - P["MARG"] - t) // P["BD"])
    add_tasks([(t + (n + 1) * P["BD"], slot, (t + n * P["BD"], P["BD"])) for n in range(n4)])
    stage_a(0, "kv")
    stage_a(2, "kv", order=(6,) + AORD[:6])

    wait("mid", g5)
    AD = 7 * HA // 2
    t = P["L5T"]
    for b in range(6, NB, 2):
        t = ln_tasks(b, t, P["LND"], P["HSD"])
    n5 = ((NP - 2) * AD - P["MARG"] - t) // P["BD"]
    add_tasks([(t + (n + 1) * P["BD"], slot, (t + n * P["BD"], P["BD"])) for n in range(n5)])
    n5 += n4
    for n, b in enumerate(range(4, NB, 2)):
        stage_a(b, order=(6,) + AORD[:6] if n % 2 else AORD)

    wait("fin", g6)
    UD = 7 * NUP * HD // 4
    for i in range(NFP):
        t0, dt = (-200, 130) if i == 0 else (800, 270) if i == 1 else ((i - 1) * UD + P["US0"], P["USD"])
        add_tasks([(t0 + (k + 1) * dt, tsum, (UB0 // 2 + k, i, i % 3, k, t0 + k * dt, dt)) for k in range(NUP)])
    left = len(mains) - n5 - 2
    bd = (NFP * UD - P["R6E"] - P["R6S"]) // left
    add_tasks([(P["R6S"] + (n + 1) * bd, slot, (P["R6S"] + n * bd, bd)) for n in range(left)])
    t = P["R6S"] + left * bd
    add_tasks([(t + (n + 1) * 300, slot, (t + n * 300, 300)) for n in range(2)])
    for qd, t0, t1 in ((NQ, UD + P["LL0"], 3 * UD), (0, 3 * UD + P["LL0"], 5 * UD), (1, 5 * UD + P["LL0"], 6 * UD + 200),
                       (2, 6 * UD + P["LL2"], 6 * UD + P["LL2"] + P["UEL"])):
        dt = (t1 - t0) // 7
        add_tasks([(t0 + (g + 1) * dt, llsum, (qd, g, t0 + g * dt, dt)) for g in range(7)])
    rr_tasks(BORD[0], 0, 0, P["RP0"], P["RP1"])
    add_tasks([(P["PW0"] + P["PWD"], prep_wo_a, (P["PW0"], P["PWD"]))])
    add_tasks([(P["PW1"] + (h + 1) * P["PWE"], prep_wo_b, (h, P["PW1"] + h * P["PWE"], P["PWE"])) for h in range(2)])
    for b in range(NB):
        b2f_s[b // 2, 0:1, _blk(b % 2)] = b2_v[b:b + 1, :].astype(f32)
    for i in range(NFP):
        u_last(i, (1, 4, 2, 3, 0, 5, 6) if i == 0 else (4, 2, 1, 3, 0, 5, 6),
               None if i == NFP - 1 else P["UEL"] if i == NFP - 2 else P["UED"])
    flush()
    assert slot_ctr[0] == len(mains) and all(("ll", qd, g) in ready for qd in range(NQ + 1) for g in range(7))
    assert all(("pr", j, hh) in ready for j in range(NB) for hh in range(2)) and ("rr", BORD[0]) in ready

    wait("w2", g7)
    lax.fori_loop(0, NP // 4, c_body, 0)
    outs = []
    for pa in range(0, NP, 2):
        outs += [out_copy(pa + n % 2, 0, 2, n // 2 * HD, (n // 2 + 1) * HD) for n in (1, 2, 3)]
        outs += [out_copy(pa, e0, e1, r0, r1) for (r0, r1, e0, e1) in (LAST_PARTS if pa % 4 else [(0, HD, 0, 2)])]
    wait("out", *outs)


@jax.jit
def pallas_parallel_sum__sliding_local_dilated__mixer_token_mlp__prompt_kernel(A_x, A_wqkv, A_wo, B_x, B_w1, B_b1, B_w2, B_b2):
    del B_x
    hbm = pl.BlockSpec(memory_space=pltpu.HBM)
    outT = pl.pallas_call(
        _kernel,
        out_shape=jax.ShapeDtypeStruct((1, D, S), bf16),
        in_specs=[hbm] * 7,
        out_specs=hbm,
        scratch_shapes=[
            pltpu.VMEM((NP, D, 2 * LB), bf16),
            pltpu.VMEM((NP, F, 2 * LB), bf16),
            pltpu.VMEM((NP, D, 2 * LB), bf16),
            pltpu.VMEM((NB + 1, D, LB), f32),
            pltpu.VMEM((NB, 2 * W * HH, LB), f32),
            pltpu.VMEM((NP, 32, 2 * LB), f32),
            pltpu.VMEM((D, 3 * D), bf16),
            pltpu.VMEM((D, D), bf16),
            pltpu.VMEM((S, F), bf16),
            pltpu.VMEM((NFB, LB), bf16),
            pltpu.VMEM((NB, LB), bf16),
            pltpu.VMEM((2, 3 * D + 64, LB), i32),
            pltpu.VMEM((7 * HA // 2, HD), u32),
            pltpu.VMEM((4, HD + 32, LB), i32),
            pltpu.VMEM((D, 2 * LB), i32),
            pltpu.VMEM((HD, S), u32),
            pltpu.VMEM((NP * QD, 5 * LB), u32),
            pltpu.VMEM((7 * QD, NP * LB), u32),
            pltpu.VMEM((7 * HD, NFP * LB), f32),
            pltpu.VMEM((7 * QD, (NFP + 2) * LB), u32),
            pltpu.VMEM((NB, 2 * D, LB), f32),
            pltpu.VMEM((D, LB), f32),
            pltpu.VMEM((4 * RSK, 5 * LB), u32),
            pltpu.VMEM((49 * ED, 4 * LB), u32),
            pltpu.VMEM((7 * RRK, 9 * LB), u32),
            pltpu.VMEM((D, 4 * LB), f32),
            pltpu.VMEM((D, 4 * LB), f32),
            pltpu.VMEM((8, LB), i32),
            pltpu.SemaphoreType.DMA((9,)),
        ],
        compiler_params=pltpu.CompilerParams(vmem_limit_bytes=100 * 1024 * 1024,
                                             disable_bounds_checks=True,
                                             disable_semaphore_checks=True),
    )(jnp.swapaxes(A_x, 1, 2), A_wqkv, A_wo, B_w1, B_b1.reshape(NFB, LB), B_w2, B_b2.reshape(NB, LB))
    return jnp.swapaxes(outT, 1, 2)
```

```python
import jax
import jax.numpy as jnp
from jax import lax
import jax.experimental.pallas as pl
import jax.experimental.pallas.tpu as pltpu

S, D, F = 2048, 448, 1792
H, DH, W, DIL = 16, 28, 8, 2
LB = 128
NB = S // LB
NP = NB // 2
NFB = F // LB
NFP = NFB // 2
HH = H // 2
WH = W // 2
SH = DIL * WH
HD = D // 2
QD = D // 4
ED = D // 8
HA = 3 * HD
HB0 = 4
NKT = (NB - HB0) // 3
NNT = -(-NFB // 3)
RSK = NFP * LB // 2
RHK = NKT * LB // 2
NQ = NFP // 2
KL = NQ * LB + QD
RRK = 2 * LB
EPS = 1e-5
EPS_BF16 = 1.0013580322265625e-05
SCALE = DH ** -0.5
f32 = jnp.float32
bf16 = jnp.bfloat16
u32 = jnp.uint32
i32 = jnp.int32

SCOPES = False
P = dict(
    E1=3, E2=6, T3=-100, N2=16, NA3=2, T1=-200, T2=-200, L2T=100, L2D=440, H2T=900, H2D=360, L4T=1000, L5T=60, W2X=500,
    QA=-410, QB=200, QC=-200, QE=330, KA=50, KB=320, KC=450, KE=390,
    LND=420, HSD=200, HTD=480, NH5=4, N4=2, N5=20, TM0=0, TMD=330, HT6=500, SGH=8, HL=180, LNA=0.28, LNB=0.46, LNBD=0.38, LNV=0.86,
    BD=355, MARG=300, LAG=200, LS=150, PP=130, PVL=500, PVPOS=20,
    US0=600, UE0=100, UED=3000, UEL=1600, UG=70, R6S=3300, R6E=2400,
    LL0=600, LL2=600, RP0=13000, RP1=16000, PW0=300, PWD=300, PW1=1000, PWE=600,
    RR0=-48, RR1=800, RRM=-20, RW=(8, 8, 8, 2, 7), BV0=117, BVS=717, BVD=620, EP0=0, EPD=864, EPL=290, SGR=8, SGT=8,
)
G = 4


def _as(x, dtype):
    return x if x.dtype == dtype else pltpu.bitcast(x, dtype)


def _pk(x):
    return pltpu.bitcast(x.astype(bf16), u32)


def _up(x):
    return pltpu.bitcast(x, bf16)


def _upf(x):
    return pltpu.bitcast(x, bf16).astype(f32)


def _rb(x):
    return x.astype(bf16).astype(f32)


def _word(lo, hi):
    lo, hi = [pltpu.bitcast(v.astype(f32), i32) for v in (lo, hi)]
    return lax.shift_right_logical(lo, 16) | hi


def _unword(w):
    return [pltpu.bitcast(w << 16, f32), pltpu.bitcast(w & -65536, f32)]


def _cat(xs, axis):
    return xs[0] if len(xs) == 1 else jnp.concatenate(xs, axis=axis)


def _x2(v):
    return jnp.concatenate([v, v], axis=0)


def _blk(b):
    return slice(b * LB, (b + 1) * LB)


def _rowsum8(a):
    return jnp.broadcast_to(jnp.sum(a, axis=0, keepdims=True), (8, a.shape[1]))


def _token(*deps):
    deps = [d for d in deps if d is not None]
    if not deps:
        return None
    if len(deps) == 1:
        return deps[0]
    bits = _as(deps[0], u32)
    for d in deps[1:]:
        bits = bits | _as(d, u32)
    return bits


def _lhs_ops(a11, a12, a21, a22):
    return [a11 + a22, a21 + a22, a11, a22, a11 + a12, a21 - a11, a12 - a22]


SIDX = {0: 0, 2: 1, 3: 2, 5: 3, 6: 4}
TOP = {0: ((0, 0), 1, (1, 1)), 1: ((0, 0),), 2: ((0, 1), -1, (1, 1)), 3: ((1, 0), -1, (0, 0)),
       4: ((1, 1),), 5: ((0, 0), 1, (0, 1)), 6: ((1, 0), 1, (1, 1))}


def _rhs_sums(b11, b12, b21, b22):
    return {0: b11 + b22, 2: b12 - b22, 3: b21 - b11, 5: b11 + b12, 6: b21 + b22}


def _rhs_op(p, blk):
    t = TOP[p]
    if len(t) == 1:
        return blk(*t[0])
    return blk(*t[0]) + blk(*t[2]) if t[1] > 0 else blk(*t[0]) - blk(*t[2])


def _combine(m, n=None):
    c12 = lambda: m[2] + m[4]
    c21 = lambda: m[1] + m[3]
    x = lambda: (m[2] - m[1]) + m[0]
    c = [lambda: (x() + m[6]) + (c21() - c12()), c12, c21, lambda: x() + m[5]]
    return [f() for f in c] if n is None else c[n]()


def _hk_lhs(a):
    s = [a[0][k] + a[1][k] for k in range(3)]
    return [a[0][0], s[0], s[1], a[1][1], a[0][0] + a[1][1], a[0][1] - a[0][0], a[1][0] - a[1][1], a[0][2],
            a[1][2], s[0] - a[1][2], s[2] - s[0], a[1][2] - a[1][0], s[1] - a[0][2], s[2] - s[1], a[0][2] - a[0][1]]


HKB = [((0, 0, 1), (1, 0, 1), (0, 2, -1)), ((0, 0, 1), (2, 0, 1), (0, 1, -1)), ((1, 1, 1), (2, 1, 1), (1, 0, -1)),
       ((1, 1, 1), (0, 1, 1), (1, 2, -1)), ((0, 1, 1), (1, 0, 1)), ((1, 0, 1),), ((0, 1, 1),),
       ((2, 2, 1), (1, 2, 1), (2, 0, -1)), ((2, 2, 1), (0, 2, 1), (2, 1, -1)), ((2, 0, 1), (0, 2, 1)), ((2, 0, 1),),
       ((0, 2, 1),), ((2, 1, 1), (1, 2, 1)), ((2, 1, 1),), ((1, 2, 1),)]


def _hk_terms(nj):
    out = {}
    for p, t in enumerate(HKB):
        t = [x for x in t if x[1] < nj]
        if t and (nj == 3 or p not in (7, 8)):
            out[p] = t
    return out


def _hk_combine(m, nj):
    x, y = (m[9] + m[11], m[12] + m[14]) if nj == 3 else (m[9], m[12])
    x0, y3 = x + m[0], y + m[3]
    c = [[(m[5] + m[10]) + x0, ((m[4] + m[5]) - y3) + m[2]], [((m[4] + m[6]) - x0) + m[1], (m[6] + m[13]) + y3]]
    if nj == 3:
        c[0].append(((m[10] - m[14]) + x) + m[7])
        c[1].append(((m[13] - m[11]) + y) + m[8])
    return c


def _kernel(x_hbm, wqkv_hbm, wo_hbm, w1_hbm, b1_hbm, w2_hbm, b2_hbm, out_hbm,
            x_v, w2_v, out_v, v_s, pr_s, b2f_s, wqkv_v, wo_v, w1_v, b1_v, b2_v, wt_s, lw_s, wo_s,
            wq_s, xnT_s, ra_s, lh_s, lk_s, rh_s, u0_s, um_s, lc_s, qk_s, op_s, rs_s, ll_s, rr_s, ola_s, olb_s, one_s, sems):
    sem_ctr = [1]

    class Group:
        def __init__(self, pairs):
            self.cps = [pltpu.make_async_copy(a, b, sems.at[sem_ctr[0]]) for (a, b) in pairs]
            sem_ctr[0] += 1

        def start(self):
            for c in self.cps:
                c.start()

        def wait(self):
            for c in self.cps:
                c.wait()

    def cp_x(p0, p1):
        return [(x_hbm.at[0, :, pl.ds(p * 2 * LB, 2 * LB)], x_v.at[p]) for p in range(p0, p1)]

    def cp_w2(p0, p1):
        return [(w2_hbm.at[:, pl.ds(p * 2 * LB, 2 * LB)], w2_v.at[p]) for p in range(p0, p1)]

    def cp_w1(b0, b1, i0=0, i1=NFP):
        sl = pl.ds(b0 * LB, (b1 - b0) * LB)
        cl = pl.ds(i0 * 2 * LB, (i1 - i0) * 2 * LB)
        return [(w1_hbm.at[sl, cl], w1_v.at[sl, cl])]

    tl = []
    mxu = [0, 0, 0, 0]
    nxt = [0]
    hist = []
    tasks = []
    dls = []
    ready = set()
    pos = []
    true = {}

    def tie(v, z):
        if z is None:
            return v
        def fit(a):
            a = _cat([a] * (v.shape[0] // 8), 0)
            return a if v.shape[1] == LB else a[:, 0:v.shape[1]]
        if v.shape not in true:
            true[v.shape] = fit(pos[0]) > 0
        return lax.select(true[v.shape], v, fit(_as(z, v.dtype)))

    def tie8(v, z):
        return v if z is None else jnp.concatenate([tie(v[0:8], z), v[8:16]], axis=0)

    def add_tasks(todo):
        tasks.extend(todo)
        tasks.sort(key=lambda x: x[0])

    def flush(t=None):
        while tasks and (t is None or tasks[0][0] < t):
            _, fn, args = tasks.pop(0)
            fn(*args)

    def reset():
        assert not tasks
        dls.clear()
        tl.clear()
        hist.clear()
        mxu[:] = [0, 0, 0, 0]
        nxt[0] = 0

    def now():
        return sum(mxu) // 4

    def wait(name, *cps):
        flush()
        if SCOPES:
            with jax.named_scope("wait_" + name):
                for c in cps:
                    c.wait()
        else:
            for c in cps:
                c.wait()
        reset()

    def mm1(lhs, rhs, pace=True):
        flush(now())
        start = mxu[nxt[0]]
        due = [v for (t, v) in dls if t <= start] if pace else []
        if due:
            dls[:] = [(t, v) for (t, v) in dls if t > start]
            tile = _up(tie(pltpu.bitcast(lhs[0:16, 0:LB], u32), _token(*due)))
            row = tile if lhs.shape[1] == LB else jnp.concatenate([tile, lhs[0:16, LB:]], axis=1)
            lhs = jnp.concatenate([row, lhs[16:]], axis=0)
        r = jnp.dot(lhs, rhs, preferred_element_type=f32)
        m, k = lhs.shape
        first_done = None
        for _ in range(-(-rhs.shape[1] // LB)):
            end = 0
            for _ in range(-(-k // LB)):
                mxu[nxt[0]] += m
                end = max(end, mxu[nxt[0]])
                nxt[0] = (nxt[0] + 1) % 4
            if first_done is None:
                first_done = end
        if pace:
            tl.append((first_done - m, first_done, r))
        return r

    def mm(lhs, rhs, init=None):
        k = lhs.shape[1]
        r, k0 = init, 0
        while k0 < k:
            k1 = min(k, k0 + (4 - nxt[0]) * LB)
            part = mm1(lhs[:, k0:k1], rhs[k0:k1], pace=k1 - k0 > LB)
            r = part if r is None else r + part
            k0 = k1
        return r

    def at(t, *more):
        best = None
        if t is not None and t >= 0:
            t = min(t, now() - 1)
            for (a, b, r) in tl:
                if a <= t and (best is None or min(b, t) > best[0]):
                    row = int(min((t - a) / (b - a), 0.999) * (r.shape[0] // 8)) * 8
                    best = (min(b, t), r, row)
        return _token(None if best is None else best[1][best[2]:best[2] + 8, 0:LB], *more)

    def strassen(lhs, rhs, order, split_last=False, init=None, m=None):
        m = [None] * 7 if m is None else m
        for p in order:
            flush(now())
            l, r = lhs(p), rhs(p)
            c0 = None if init is None else init[p]
            if split_last and p == order[-1]:
                kk = (-(-r.shape[0] // LB) - 2) * LB
                hm = l.shape[0] // 2
                hd = mm(l[:, :kk], r[:kk], c0) if kk else c0
                tail = jnp.concatenate([mm(l[:hm, kk:], r[kk:]), mm(l[hm:, kk:], r[kk:])], axis=0)
                m[p] = tail if hd is None else hd + tail
            else:
                m[p] = mm(l, r, c0)
        return m

    def wcol(hh, p):
        return p * D + (1 - hh if p == 1 else hh) * HD

    def wrows(hh, g, z=None):
        p, d = divmod(2 * g, DH)
        t = [jnp.concatenate([wt_s[c, pl.ds(wcol(hh, p) + d + e, HH, stride=DH), :]
                              for e in range(2)], axis=0) for c in range(2)]
        return _unword(jnp.concatenate([tie(t[0], z), tie(t[1][:, 0:HD - LB], z)], axis=1))

    wt_done = set()

    def prep_wqkv(part, ga, gb, paced):
        def need(hh, p, z):
            lo = wcol(hh, p)
            for ct in range(lo // LB, -(-(lo + HD) // LB)):
                if ct in wt_done:
                    continue
                wt_done.add(ct)
                cols = slice(ct * LB, min((ct + 1) * LB, 3 * D))
                wd = _word(wqkv_v[0:HD, cols], wqkv_v[HD:D, cols])
                wd = jnp.concatenate([tie(wd[r:r + 8], z if r % LB == 0 else None) for r in range(0, HD, 8)], axis=0)
                wT = wd.T
                wt_s[0, cols, :] = wT[:, 0:LB]
                wt_s[1, cols, 0:HD - LB] = wT[:, LB:HD]

        def put(p, g, v):
            lw_s[p * (HA // 2) + g * 8:p * (HA // 2) + g * 8 + 8, :] = _pk(v)

        def half(hh, g0, g1, t0=None, dur=None):
            pr, ps = ((2, 4), (3, 1))[hh]
            for g in range(g0, g1):
                t = None if t0 is None else t0 + (g - g0) * dur // (g1 - g0)
                need(hh, 2 * g // DH, at(None if t is None else t - P["W2X"]))
                a1, a2 = wrows(hh, g, at(t))
                put(pr, g, a2 if hh else a1)
                put(ps, g, a1 + a2)
            if g1 == gb:
                ready.update({("lw", part, pr), ("lw", part, ps)})

        def rest(g0, g1, t0, dur):
            assert ("lw", part, 1) in ready
            for g in range(g0, g1):
                z = at(t0 + (g - g0) * dur // (g1 - g0))
                ops = _lhs_ops(*wrows(0, g, z), *wrows(1, g, z))
                for p in (0, 5, 6):
                    put(p, g, ops[p])
            if g1 == gb:
                ready.update({("lw", part, 0), ("lw", part, 5), ("lw", part, 6)})
        t2, d2, t3, d3 = paced
        half(0, ga, gb)
        n = (gb - ga) // 14
        add_tasks([(now() + t2 + (k + 1) * d2 // n, half,
                    (1, ga + 14 * k, ga + 14 * k + 14, now() + t2 + k * d2 // n, d2 // n)) for k in range(n)])
        n = (gb - ga) // 7
        add_tasks([(now() + t3 + (k + 1) * d3 // n, rest,
                    (ga + 7 * k, ga + 7 * k + 7, now() + t3 + k * d3 // n, d3 // n)) for k in range(n)])

    def prep_wo_a(t0, dur):
        for g in range(HD // 16):
            w = _word(wo_v[g * 16:g * 16 + 16, :], wo_v[HD + g * 16:HD + g * 16 + 16, :])
            z = at(t0 + g * dur // (HD // 16))
            for c in range(4):
                cw = min(LB, D - c * LB)
                wo_s[c, g * 16:g * 16 + 16, 0:cw] = tie(w[:, c * LB:c * LB + cw], z)
        ready.add("wo")

    def prep_wo_b(h, t0, dur):
        assert "wo" in ready
        for c in range(4):
            cw = min(LB, D - c * LB)
            rows = [wo_s[c, pl.ds(d, HH, stride=DH), :][:, 0:cw] for d in range(h * DH // 2, (h + 1) * DH // 2)]
            rows.append(jnp.zeros((LB - QD, cw), i32))
            wq_s[c * LB:c * LB + cw, _blk(h)] = jnp.concatenate(rows, axis=0).T
        outs = []
        for g in range(HD // 16):
            z = at(t0 + g * dur // (HD // 16))
            a = [v for r in (g * 16, HD + g * 16) for v in _unword(tie(wq_s[r:r + 16, _blk(h)], z))]
            for p, v in enumerate(_lhs_ops(*a)):
                lc_s[p * QD + g * 8:p * QD + g * 8 + 8, _blk(NFP + h)] = _pk(v)
                outs.append(v[0:8])
        ready.update({("lc", NFP + h, g) for g in range(HD // 16)})
        dls.append((t0 + dur + 250, _token(*outs)))

    RG = 16
    NG = D // RG
    stat2 = {}

    def ln(b, t0=None, dur=None):
        def xg(g):
            return x_v[b // 2, g * RG:(g + 1) * RG, _blk(b % 2)].astype(f32)

        def step(v, g, fr, s, q):
            if t0 is None or g % 4:
                return v
            acc = [] if s is None else [s[0:8], s[8:16], q[0:8], q[8:16]]
            return tie(v, at(t0 + fr * dur, *acc))

        x0 = jnp.broadcast_to(xg(0)[0:1], (8, LB))
        s = q = None
        for g in range(NG):
            x0 = step(x0, g, P["LNA"] * g / NG, s, q)
            c = xg(g) - _x2(x0)
            s = c if s is None else s + c
            q = c * c if q is None else q + c * c
        dm = _rowsum8(s) * (1.0 / D)
        mu = _rb(x0 + dm)
        var = _rb(jnp.maximum(_rowsum8(q) * (1.0 / D) - dm * dm, 0.0))
        r1 = 1.0 / _rb(jnp.sqrt(_rb(var + EPS_BF16)))
        s = q = None
        for g in range(NG):
            mu = step(mu, g, P["LNB"] + P["LNBD"] * g / NG, s, q)
            xn = _rb(xg(g) - _x2(mu)) * _x2(r1)
            xnT_s[g * 8:g * 8 + 8, _blk(b)] = _pk(xn)
            s = xn if s is None else s + xn
            q = xn * xn if q is None else q + xn * xn
        mu2 = _rowsum8(s) * (1.0 / D)
        var2 = jnp.maximum(_rowsum8(q) * (1.0 / D) - mu2 * mu2, 0.0)
        stat2[b] = (mu2, 0.5 * lax.rsqrt(var2 + EPS))

    def hpair(b, t0=None, dur=None):
        ng = HD // RG
        st = [stat2[b], stat2[b + 1]]
        for g in range(ng):
            if b < HB0:
                zz = [at(None if t0 is None else t0 + (4 * g + k) * dur // (4 * ng)) for k in range(4)]
            else:
                zz = [at(t0 + g * dur // ng), None, None, at(t0 + g * dur // ng + P["SGT"])]
            xq = [_upf(tie(xnT_s[r:r + 8, _blk(b + e)], zz[2 * (r >= QD) + e]))
                  for r in (g * 8, QD + g * 8) for e in range(2)]
            ro = (b // 2) * QD + g * 8
            for p, v in _rhs_sums(*xq).items():
                ra_s[ro:ro + 8, _blk(SIDX[p])] = _pk(v)
            if b < HB0:
                hq = [(v - _x2(st[n % 2][0])) * _x2(st[n % 2][1]) for n, v in enumerate(xq)]
                for p, v in enumerate(_lhs_ops(*hq)):
                    lh_s[p * QD + g * 8:p * QD + g * 8 + 8, _blk(b // 2)] = _pk(v)
        ready.add(("xn", b))
        if b >= 6:
            got = ra_s[(b // 2) * QD:(b // 2 + 1) * QD, :]
            dls.append((t0 + dur + P["HL"], _token(*[got[r:r + 8, _blk(c)] for r in range(0, QD, 8) for c in range(5)])))

    def htile(b, r, z=None):
        return (_upf(tie(xnT_s[r:r + 8, _blk(b)], z)) - _x2(stat2[b][0])) * _x2(stat2[b][1])

    def htriple(t, t0, dur):
        ng = HD // RG
        for g in range(ng):
            zz = [at(t0 + (3 * g + k) * dur // (3 * ng)) for k in range(3)]
            a = [[htile(HB0 + 3 * t + k, h * QD + g * 8, zz[k]) for k in range(3)] for h in range(2)]
            for p, v in enumerate(_hk_lhs(a)):
                lk_s[p * QD + g * 8:p * QD + g * 8 + 8, _blk(t)] = _pk(v)
        ready.add(("lh", t))

    def ln_tasks(b, t, lnd, hsd):
        for fn, bb, dur, adv in ((ln, b, lnd, P["LNV"]), (ln, b + 1, lnd, P["LNV"]), (hpair, b, hsd, 1.0)):
            add_tasks([(t + int(dur * adv), fn, (bb, t, dur))])
            t += int(dur * adv)
        return t

    def tsum(kp, i, slot_, n, t0, dur):
        for g in range(LB // 16):
            z, z2 = at(t0 + g * dur // 8), at(t0 + g * dur // 8 + P["SGT"])
            t1, t2 = [w1_v[(2 * kp + e) * LB + g * 16:(2 * kp + e) * LB + g * 16 + 16,
                           2 * i * LB:(2 * i + 2) * LB].astype(f32) for e in range(2)]
            ro = slot_ * RSK + n * (LB // 2) + g * 8
            for p, v in _rhs_sums(tie8(t1[:, :LB], z), t1[:, LB:], t2[:, :LB], tie8(t2[:, LB:], z2)).items():
                rs_s[ro:ro + 8, _blk(SIDX[p])] = _pk(v)
        ready.add(("rs", kp, i))

    def u_rhs(p, i, kps, slot_, n0):
        if p in SIDX:
            assert all(("rs", kp, i) in ready for kp in kps)
            ro = slot_ * RSK + n0 * (LB // 2)
            return _up(rs_s[ro:ro + len(kps) * (LB // 2), _blk(SIDX[p])])
        e = 0 if p == 1 else 1
        return _cat([w1_v[_blk(2 * kp + e), _blk(2 * i + e)] for kp in kps], 0)

    LATE = (NFP - 1, 6)

    def ujob(kp, i, p, split):
        flush(now())
        assert ("xn", 2 * kp) in ready
        l, r = _up(lh_s[p * QD:(p + 1) * QD, _blk(kp)]), u_rhs(p, i, [kp], kp, i)
        v = jnp.concatenate([mm1(l[:QD], r), mm1(l[QD:], r)], axis=0) if split else mm1(l, r)
        rows = slice(p * HD, (p + 1) * HD)
        um_s[rows, _blk(i)] = v

    def u_early(kp, i0, i1, carry, n, t0, dt, nsplit=0):
        for k, i in enumerate(range(i0, i1)):
            add_tasks([(t0 + (k + 1) * dt, tsum, (kp, i, kp, i, t0 + k * dt, dt))])
        jobs = (carry + [(kp, i, p) for i in range(i0, i1) for p in (1, 4)]
                + [(kp, i, p) for i in range(i0, i1) for p in SIDX if (i, p) != LATE])
        for c, job in enumerate(jobs[:n]):
            ujob(*job, c >= n - nsplit)
        return jobs[n:]

    def u_mid():
        jobs = [(i, p) for i in range(2) for p in (4, 1)]
        for i in range(NFP):
            jobs += [(i, p) for p in (2, 3, 0, 5, 6)] + [(i + 2, p) for p in (4, 1) if i + 2 < NFP]
        m = [[None] * 7 for _ in range(NFP)]
        for i, p in jobs:
            flush(now())
            late = (i, p) == LATE
            l = _up(lh_s[p * QD:(p + 1) * QD, (0 if late else LB):])
            r = _cat([u_rhs(p, i, [0], 0, i)] * late + [u_rhs(p, i, [1], 1, i)], 0)
            v = jnp.concatenate([mm1(l[:QD], r), mm1(l[QD:], r)], axis=0) if late else mm1(l, r)
            if not late:
                v = v + um_s[p * HD:(p + 1) * HD, _blk(i)]
            if p in (2, 3):
                v = v + 0.5 * b1_v[2 * i + 3 - p:2 * i + 4 - p, :].astype(f32)
            m[i][p] = v
            if p == 6:
                for n, c in enumerate(_combine(m[i])):
                    u0_s[n // 2 * HD:(n // 2 + 1) * HD, _blk(2 * i + n % 2)] = c

    def nj_of(i):
        return min(3, NFB - 3 * i)

    def hsum(t, i, t0, dur):
        nj = nj_of(i)
        sums = [(p, tm) for p, tm in _hk_terms(nj).items() if len(tm) > 1]
        tied = {(1, 0): 0, (2, 0): 1, (1, 2): 2, (2, 2): 3} if nj == 3 else {(1, 0): 0, (0, 1): 2}
        for g in range(LB // 16):
            b = {}
            for k in range(3):
                r = (HB0 + 3 * t + k) * LB + g * 16
                w = w1_v[r:r + 16, 3 * i * LB:(3 * i + nj) * LB].astype(f32)
                for j in range(nj):
                    z = at(t0 + g * dur // 8 + tied[k, j] * P["SGH"]) if (k, j) in tied else None
                    b[k, j] = tie8(w[:, _blk(j)], z)
            ro = (i % 2) * RHK + t * (LB // 2) + g * 8
            for n, (p, tm) in enumerate(sums):
                v = b[tm[0][:2]]
                for (k, j, sg) in tm[1:]:
                    v = v + b[k, j] if sg > 0 else v - b[k, j]
                rh_s[ro:ro + 8, _blk(n)] = _pk(v)
        ready.add(("rh", t, i))

    def gelu_half(hx, z):
        c = 0.7978845608028654
        return hx + hx * jnp.tanh(tie(hx * (2.0 * c + (8.0 * c * 0.044715) * (hx * hx)), z))

    gl = {}

    def u_epilogue(i, m, gs, t0, dur):
        nj = nj_of(i)
        for n, g in enumerate(gs):
            c = _hk_combine({p: v[g * 16:g * 16 + 16] for p, v in m.items()}, nj)
            for j in range(nj):
                f = 3 * i + j
                t = None if t0 is None else t0 + (n * nj + j) * dur // (len(gs) * nj) - P["UG"]
                gl[f, g] = [gelu_half(c[h][j] + u0_s[h * HD + g * 16:h * HD + g * 16 + 16, _blk(f)], at(t))
                            for h in range(2)]
                if f % 2 == 1:
                    g0, g1 = gl.pop((f - 1, g)), gl.pop((f, g))
                    for p, v in enumerate(_lhs_ops(g0[0], g1[0], g0[1], g1[1])):
                        lc_s[p * QD + g * 8:p * QD + g * 8 + 8, _blk(f // 2)] = _pk(v)
                    ready.add(("lc", f // 2, g))

    def u_last(i, edur):
        terms = _hk_terms(nj_of(i))
        sums = [p for p, tm in terms.items() if len(tm) > 1]
        m = {}
        order = ((10, 11, 14, 5, 13, 6, 9, 7, 0, 12, 8, 3, 4, 1, 2) if i == 0
                 else (10, 11, 9, 14, 7, 5, 0, 13, 12, 8, 6, 3, 4, 1, 2))
        for p in [p for p in order if p in terms]:
            flush(now())
            assert all(("lh", t) in ready for t in range(NKT))
            if p in sums:
                assert all(("rh", t, i) in ready for t in range(NKT))
                r = _up(rh_s[(i % 2) * RHK:(i % 2 + 1) * RHK, _blk(sums.index(p))])
            else:
                k, j, _ = terms[p][0]
                r = _cat([w1_v[_blk(HB0 + 3 * t + k), _blk(3 * i + j)] for t in range(NKT)], 0)
            m[p] = mm(_up(lk_s[p * QD:(p + 1) * QD, :]), r)
        if edur is None:
            u_epilogue(i, m, list(range(HD // 16)), None, None)
        else:
            t = now() + P["UE0"]
            add_tasks([(t + (g + 1) * edur // 7, u_epilogue, (i, m, [g, g + 7], t + g * edur // 7, edur // 7))
                       for g in range(7)])

    def llsum(qd, g, t0, dur):
        i0 = 2 * qd if qd < NQ else NFP
        assert all(("lc", i0 + e, g + 7 * h) in ready for e in range(2) for h in range(2))
        for p in range(7):
            zz = [at(t0 + p * dur // 7), at(t0 + p * dur // 7 + P["SGT"])]
            a = [tie(lc_s[p * QD + h * ED + g * 8:p * QD + h * ED + g * 8 + 8, _blk(i0 + e)], zz[h] if h == e else None)
                 for h in range(2) for e in range(2)]
            ops = _lhs_ops(*[_upf(v) for v in a])
            for q in (0, 1, 4, 5, 6):
                r = (p * 7 + q) * ED + g * 8
                ll_s[r:r + 8, _blk(qd)] = _pk(ops[q])
        ready.add(("ll", qd, g))

    AORD = (4, 2, 1, 3, 0, 5, 6)

    def stage_a(b, parts="qkv", order=AORD, split_last=False, m=None):
        r0, r1 = {"q": (0, HD), "kv": (HD, HA), "qkv": (0, HA)}[parts]

        def lhs(p):
            assert all(("lw", pt, p) in ready for pt in ("q", "kv") if pt in parts)
            return _up(lw_s[(p * HA + r0) // 2:(p * HA + r1) // 2, :])

        def rhs(p):
            assert ("xn", b) in ready
            if p in SIDX:
                return _up(ra_s[(b // 2) * QD:(b // 2 + 1) * QD, _blk(SIDX[p])])
            return _up(xnT_s[0:QD, _blk(b)] if p == 1 else xnT_s[QD:HD, _blk(b + 1)])
        m = strassen(lhs, rhs, order, split_last, m=m)
        for n, ps in enumerate((range(7), (2, 4), (1, 3), (0, 1, 2, 5))):
            if all(m[p] is not None for p in ps) and any(p in order for p in ps):
                hh, e = divmod(n, 2)
                c = _combine(m, n)
                qk_s[b + e, hh * D + r0:hh * D + min(r1, D), :] = c[0:min(r1, D) - r0]
                if r1 > D:
                    v_s[b + e + 1, hh * HD:(hh + 1) * HD, :] = c[D - r0:]
        if all(v is not None for v in m):
            ready.update({(pt, b + e) for pt in ("q", "kv") if pt in parts for e in range(2)})
        return m

    lane0 = lax.broadcasted_iota(i32, (HH, LB), 1)
    zeros8 = jnp.zeros((HH, LB), f32)

    def mk_shift(z):
        lane = tie(lane0, z)
        masks = {}

        def pick(n, a, b):
            if n not in masks:
                masks[n] = lane < n
            return lax.select(masks[n], a, b)

        def fwd(cur, prev, sh):
            return cur if sh == 0 else pltpu.roll(pick(LB - sh, cur, prev), sh, 1)

        def bwd(cur, nxt_):
            return pltpu.roll(pick(SH, nxt_, cur), LB - SH, 1)
        return fwd, bwd

    def grp_shift(t, bd):
        lag = max(2, -(-P["LAG"] * DH // (G * bd)))
        return mk_shift(at(t, *(hist[-lag] if len(hist) >= lag else [])))

    raw, probs = {}, {}

    def attn_qk(j, hh, t, bd):
        jn = min(j + 1, NB - 1)
        assert ("q", jn) in ready and ("kv", j) in ready
        acc = [None] * WH
        accp = [None] * WH
        for d in range(DH):
            if d % G == 0:
                if d > 0:
                    hist.append(acc + accp)
                fwd, bwd = grp_shift(t + d * bd // DH, bd)
            r = hh * D + d * HH
            q = qk_s[j, r:r + HH, :]
            qp = bwd(q, qk_s[jn, r:r + HH, :])
            rk = (1 - hh) * D + HD + d * HH
            k = qk_s[j, rk:rk + HH, :]
            kp = qk_s[j - 1, rk:rk + HH, :] if j > 0 else zeros8
            for a in range(WH):
                ks = fwd(k, kp, DIL * a)
                t0, t1 = q * ks, qp * ks
                acc[a] = t0 if d == 0 else acc[a] + t0
                accp[a] = t1 if d == 0 else accp[a] + t1
        hist.append(acc + accp)
        raw[j, hh] = (acc, accp)

    def attn_sm(j, hh, t):
        fwd, _ = mk_shift(at(t))
        acc, accp = raw[j, hh]
        prev = raw.pop((j - 1, hh))[1] if j > 0 else [zeros8] * WH
        lg = acc + [fwd(accp[a], prev[a], SH) for a in range(WH)]
        lg = [a * SCALE for a in lg]
        if j == 0:
            lg = [lg[0]] + [jnp.where(lane0 >= DIL * w, lg[w], -1e9) for w in range(1, W)]
        m = lg[0]
        for w in range(1, W):
            m = jnp.maximum(m, lg[w])
        e = [jnp.exp(l - m) for l in lg]
        den = e[0]
        for w in range(1, W):
            den = den + e[w]
        inv = 1.0 / den
        p = [x * inv for x in e]
        for a in range(WH):
            pr_s[j, (hh * W + a) * HH:(hh * W + a + 1) * HH, :] = p[a]
        probs[j, hh] = p[WH:]

    def attn_pp(j, hh, t):
        _, bwd = mk_shift(at(t))
        p = probs.pop((j, hh))
        pn = probs[j + 1, hh] if j + 1 < NB else p
        for a in range(WH):
            pr_s[j, (hh * W + WH + a) * HH:(hh * W + WH + a + 1) * HH, :] = bwd(p[a], pn[a])
        ready.add(("pr", j, hh))

    def attn_pv(j, hh, dst, e, t, bd):
        assert not isinstance(j, int) or ("pr", j, hh) in ready
        assert e == 0 or ("o", dst, hh, e - 1) in ready
        pa = [pr_s[j, (hh * W + a) * HH:(hh * W + a + 1) * HH, :] for a in range(W)]
        p, pp = pa[:WH], pa[WH:]
        outs = []
        for d in range(DH):
            if d % G == 0:
                if d > 0:
                    hist.append([])
                fwd, _ = grp_shift(t + d * bd // DH, bd)
            r = hh * HD + d * HH
            v = v_s[j + 1, r:r + HH, :]
            vp = v_s[j, r:r + HH, :]
            o = op = None
            for a in range(WH):
                vs = fwd(v, vp, DIL * a)
                o = p[a] * vs if a == 0 else o + p[a] * vs
                op = pp[a] * vs if a == 0 else op + pp[a] * vs
            opp = zeros8 if (isinstance(j, int) and j == 0) else op_s[r:r + HH, :]
            op_s[r:r + HH, :] = op
            outs.append(o + fwd(op, opp, SH))
            ol[dst][r:r + HH, _blk(e)] = outs[-1]
        hist.append([])
        ready.add(("o", dst, hh, e))
        dls.append((t + bd + P["PVL"], _token(*outs)))

    ol = [ola_s, olb_s]
    mains = [("qk", j, hh) for j in range(NB) for hh in range(2)]
    mains = (mains[:P["PVPOS"]] + [("pv", j, hh) for j in range(4) for hh in range(2)]
             + mains[P["PVPOS"]:] + [None, None])
    slot_ctr = [0]

    def slot(t, bd):
        n = slot_ctr[0]
        slot_ctr[0] += 1
        it = mains[n]
        if it is None:
            pass
        elif it[0] == "qk":
            attn_qk(it[1], it[2], t, bd)
        else:
            attn_pv(it[1], it[2], 0, it[1], t, bd)
        if n >= 1 and mains[n - 1] is not None and mains[n - 1][0] == "qk":
            attn_sm(mains[n - 1][1], mains[n - 1][2], t + P["LS"])
        if n >= 2 and mains[n - 2] is not None and mains[n - 2][0] == "qk":
            _, j, hh = mains[n - 2]
            if j > 0:
                attn_pp(j - 1, hh, t + P["PP"])
            if j == NB - 1:
                attn_pp(j, hh, t + P["PP"])

    NRG = 8 * (NQ + 1) + 7
    PD = 8 * QD
    BORD = (1, 3, 2, 4, 0, 5, 6)
    LORD = (2, 4, 1, 3, 0, 5, 6)
    LAST_PARTS = [(0, QD, 1, 2), (QD, HD, 0, 2), (0, QD, 0, 1)]

    def rr_prep(p, pa, src, n0, n1, t0, dur):
        assert ("rr", p) not in ready
        for n in range(n0, n1):
            z = at(t0 + (n - n0) * dur // (n1 - n0))
            z2 = at(t0 + (n - n0) * dur // (n1 - n0) + P["SGR"])
            qd, g = divmod(n, 8)

            def wrow(i):
                return _rhs_op(p, lambda x, y: w2_v[pa + y, (2 * i + x) * LB + g * 16:(2 * i + x) * LB + g * 16 + 16, :]
                               .astype(f32))

            def orow(h):
                def blk(x, y):
                    assert ("o", src, x, 2 * y + 1) in ready
                    r = x * HD + h * QD + g * 16
                    return ol[src][r:r + 16, y * 2 * LB:(y + 1) * 2 * LB]
                return _rhs_op(p, blk)
            ro = p * RRK + g * 8
            if qd == NQ:
                if p in SIDX:
                    r = wrow(2 * NQ)
                    for e in range(2):
                        rr_s[ro:ro + 8, _blk(7 + e)] = _pk(tie8(r[:, _blk(e)], z))
                continue
            r1, r2 = (wrow(2 * qd), wrow(2 * qd + 1)) if qd < NQ else (orow(0), orow(1))
            ro += min(qd, NQ) * (LB // 2)
            c11, c22 = tie8(r1[:, :LB], z), tie8(r2[:, LB:], z2)
            sm = _rhs_sums(c11, r1[:, LB:], r2[:, :LB], c22)
            if p in SIDX or qd > NQ:
                sm.update({1: c11, 4: c22})
            for q, v in sm.items():
                rr_s[ro:ro + 8, _blk(q)] = _pk(v)
        if n1 == NRG:
            ready.add(("rr", p))

    def rr_tasks(p, pa, src, t0, t1):
        cuts = list(range(0, NRG, 8)) + [NRG]
        acc, tot = 0, sum(P["RW"])
        for a, b, w in zip(cuts[:-1], cuts[1:], P["RW"]):
            ta, tb = t0 + acc * (t1 - t0) // tot, t0 + (acc + w) * (t1 - t0) // tot
            add_tasks([(tb, rr_prep, (p, pa, src, a, b, ta, tb - ta))])
            acc += w

    def out_copy(pidx, e0, e1, r0, r1):
        off = pidx * (2 * LB) + e0 * LB
        if not isinstance(pidx, int):
            off = pl.multiple_of(off, LB)
        rs = pl.ds(r0, r1 - r0)
        return pltpu.make_async_copy(out_v.at[pidx, rs, pl.ds(e0 * LB, (e1 - e0) * LB)],
                                     out_hbm.at[0, rs, pl.ds(off, (e1 - e0) * LB)], sems.at[0])

    def b_out(pa, n, m, part, t0=None, dur=None):
        a, y = divmod(n, 2)
        r0, r1, e0, e1 = part
        cols = slice(e0 * LB, e1 * LB)
        for r in range(r0, r1, 16):
            c = _combine([None if v is None else v[r:r + 16, cols] for v in m], n)
            rows = slice(a * HD + r, a * HD + r + 16)
            o = c + x_v[pa + y, rows, cols].astype(f32)
            if t0 is not None:
                o = jnp.concatenate([tie(o[:, 0:LB], at(t0 + (r - r0) * dur // (r1 - r0))), o[:, LB:]], axis=1)
            out_v[pa + y, rows, cols] = o.astype(bf16)
        out_copy(pa + y, e0, e1, a * HD + r0, a * HD + r1).start()

    def big_piece(pa, pan, cur, last):
        t0 = now()
        for n in range(7):
            ta, tb = t0 + n * PD + P["RR0"], t0 + n * PD + P["RR1"]
            if n < 6:
                rr_tasks(BORD[n + 1], pa, cur, ta, tb)
            else:
                rr_tasks(BORD[0], pan, 1 - cur, ta, tb - (P["RRM"] if last else 0))
        ready.difference_update({("o", 1 - cur, hh, e) for hh in range(2) for e in range(4)})
        for n in range(8):
            e, hh = divmod(n, 2)
            t = t0 + P["BV0"] + n * P["BVS"]
            add_tasks([(t + P["BVD"], attn_pv, (pan * 2 + e, hh, 1 - cur, e, t, P["BVD"]))])
        m = [None] * 7
        for p in BORD:
            flush(now())
            assert ("rr", p) in ready
            x, y = TOP[p][0]

            def lhs(q):
                if q in (2, 3):
                    rows = slice(p * QD + (q - 2) * ED, p * QD + (q - 1) * ED)
                    return _up(jnp.concatenate([lc_s[rows, _blk(2 * qd + q - 2)] for qd in range(NQ)]
                                               + [lc_s[rows, (NFP + q - 2) * LB:(NFP + q - 2) * LB + QD]], axis=1))
                return _up(ll_s[(p * 7 + q) * ED:(p * 7 + q + 1) * ED, 0:KL])

            def rhs(q):
                if p in SIDX or q in SIDX:
                    return _up(rr_s[p * RRK:p * RRK + KL // 2, _blk(q)])
                h = 0 if q == 1 else 1
                return _cat([w2_v[pa + y, _blk(2 * (2 * qd + h) + x), _blk(h)] for qd in range(NQ)]
                            + [_up(rr_s[p * RRK + NQ * LB // 2:p * RRK + KL // 2, _blk(q)])], 0)
            rl = (_up(rr_s[p * RRK:p * RRK + LB // 2, 7 * LB:9 * LB]) if p in SIDX
                  else w2_v[pa + y, _blk(4 * NQ + x), :])
            ll = _up(lc_s[p * QD:(p + 1) * QD, _blk(2 * NQ)])
            ex = [mm1(ll[:QD], rl), mm1(ll[QD:], rl)]
            e12, e21 = ex[0][:, LB:], ex[1][:, :LB]
            e11 = (ex[0][:, :LB] + e12) - e21
            lf = strassen(lhs, rhs, LORD)
            ready.discard(("rr", p))
            if p in (2, 3):
                for q in (2, 3):
                    lf[q] = lf[q] + b2f_s[pa + 3 - p, 0:1, _blk(3 - q)]
            c12 = (lf[2] + e12) + lf[4]
            c21 = (lf[1] + e21) + lf[3]
            xx = (lf[2] - lf[1]) + lf[0]
            c22 = (xx + ex[1][:, LB:]) + lf[5]
            c11 = ((xx + e11) + (c21 - c12)) + lf[6]
            m[p] = jnp.concatenate([jnp.concatenate([c11, c12], axis=1),
                                    jnp.concatenate([c21, c22], axis=1)], axis=0)
            n = {3: 2, 4: 1, 5: 3, 6: 0}.get(p)
            if n is not None and not (last and n == 0):
                t, epd = now() + P["EP0"], P["EPL"] if (last and n == 3) else P["EPD"]
                add_tasks([(t + epd, b_out, (pa, n, list(m), (0, HD, 0, 2), t, epd))])
        if last:
            flush()
            for part in LAST_PARTS:
                b_out(pa, 0, m, part)

    def c_body(it, carry):
        reset()
        pos[:] = [one_s[...]]
        true.clear()
        ready.update({("rr", BORD[0])} | {("o", 0, hh, e) for hh in range(2) for e in range(4)})
        big_piece(4 * it, 4 * it + 2, 0, False)
        big_piece(4 * it + 2, lax.rem(4 * it + 4, NP), 1, True)
        assert ("rr", BORD[0]) in ready and all(("o", 0, hh, 3) in ready for hh in range(2))
        return carry

    E1, E2 = P["E1"], P["E2"]
    x0 = Group(cp_x(0, 1))
    g1 = Group(cp_w1(0, 2, 0, E1))
    g2 = Group(cp_w1(0, 2, E1, E2) + cp_x(1, 2))
    wq, wkv = [[(wqkv_hbm.at[:, cl], wqkv_v.at[:, cl])] for cl in (pl.ds(0, 4 * LB), pl.ds(4 * LB, 3 * D - 4 * LB))]
    g3 = Group((cp_w1(0, 2, E2, NFP) if E2 < NFP else []) + wq)
    g4 = Group(wkv + cp_x(2, 3))
    g5 = Group(cp_x(3, NP))
    g6 = Group(cp_w1(2, NB) + [(wo_hbm, wo_v), (b1_hbm, b1_v), (b2_hbm, b2_v)] + cp_w2(0, 1))
    g7 = Group(cp_w2(1, NP))
    for c in (x0, g1, g2, g3, g4, g5, g6, g7):
        c.start()

    v_s[0] = jnp.zeros((D, LB), f32)
    for buf in (xnT_s, ra_s, lh_s, lk_s, rh_s, rs_s, rr_s, ola_s, olb_s, ll_s, lc_s):
        buf[0:8, 0:64] = jnp.zeros((8, 64), buf.dtype)

    wait("x0", x0)
    one_s[...] = lax.shift_right_logical(pltpu.bitcast(x_v[0, 0:16, 0:LB], i32), 1) | 1
    pos[:] = [one_s[...]]
    ln(0)
    ln(1)
    hpair(0)
    wait("r1", g1)
    jobs = u_early(0, 0, E1, [], 7 * E1 // 4 * 4, P["T1"], 100)
    wait("r2", g2)
    t, dt = P["L2T"], P["L2D"]
    add_tasks([(t + int((k + 1) * dt * P["LNV"]), ln, (2 + k, t + int(k * dt * P["LNV"]), dt)) for k in range(2)])
    jobs = u_early(0, E1, E2, jobs, P["N2"], P["T2"], 100)
    wait("wq", g3)
    add_tasks([(P["H2T"] + P["H2D"], hpair, (2, P["H2T"], P["H2D"]))])
    u_early(0, E2, NFP, jobs, 7 * NFP, P["T3"], 100)
    prep_wqkv("q", 0, HD // 16, [P[k] for k in ("QA", "QB", "QC", "QE")])
    stage_a(0, "q", split_last=True)
    m = stage_a(2, "q", AORD[:P["NA3"]])
    wait("wkv", g4)
    stage_a(2, "q", AORD[P["NA3"]:], split_last=True, m=m)
    prep_wqkv("kv", HD // 16, HA // 16, [P[k] for k in ("KA", "KB", "KC", "KE")])
    t = ln_tasks(4, now() + P["L4T"], P["LND"], P["HSD"])
    n4 = P["N4"]
    add_tasks([(t + (n + 1) * P["BD"], slot, (t + n * P["BD"], P["BD"])) for n in range(n4)])
    stage_a(0, "kv")
    stage_a(2, "kv", order=(6,) + AORD[:6])

    wait("mid", g5)
    AD = 7 * HA // 2
    t = P["L5T"]
    for b in range(6, NB, 2):
        t = ln_tasks(b, t, P["LND"], P["HSD"])
    for k in range(P["NH5"]):
        add_tasks([(t + P["HTD"], htriple, (k, t, P["HTD"]))])
        t += P["HTD"]
    n5 = P["N5"]
    bd = ((NP - 2) * AD - P["MARG"] - t) // n5
    add_tasks([(t + (n + 1) * bd, slot, (t + n * bd, bd)) for n in range(n5)])
    n5 += n4
    for n, b in enumerate(range(4, NB, 2)):
        stage_a(b, order=(6,) + AORD[:6] if n % 2 else AORD)

    wait("fin", g6)
    UM = (7 * NFP + 1) * HD // 4
    UD = 15 * NKT * HD // 4
    r6 = UM + (NNT - 1) * UD + 11 * NKT * HD // 4
    add_tasks([(i * P["TMD"] + P["TM0"], tsum, (1, i, 1, i, (i - 1) * P["TMD"] + P["TM0"], P["TMD"])) for i in range(NFP)])
    t, dt = P["HT6"], (UM - 100 - P["HT6"]) // max(NKT - P["NH5"], 1)
    add_tasks([(t + (k + 1) * dt, htriple, (P["NH5"] + k, t + k * dt, dt)) for k in range(NKT - P["NH5"])])
    for i in range(NNT):
        t0, t1 = (UM - P["US0"], UM + 1200) if i == 0 else (UM + (i - 1) * UD + (1300 if i == 1 else 400), UM + i * UD + 350)
        dt = (t1 - t0) // NKT
        add_tasks([(t0 + (k + 1) * dt, hsum, (k, i, t0 + k * dt, dt)) for k in range(NKT)])
    left = len(mains) - n5 - 2
    bd = (r6 - P["R6E"] - P["R6S"]) // left
    add_tasks([(P["R6S"] + (n + 1) * bd, slot, (P["R6S"] + n * bd, bd)) for n in range(left)])
    t = P["R6S"] + left * bd
    add_tasks([(t + (n + 1) * 300, slot, (t + n * 300, 300)) for n in range(2)])
    for qd, t0, t1 in ((NQ, UD, 2 * UD), (0, 2 * UD + P["LL0"], 3 * UD + P["LL0"]), (1, 3 * UD + P["LL0"], 4 * UD + P["LL0"]),
                       (2, 4 * UD + P["LL2"], 4 * UD + P["LL2"] + P["UEL"])):
        dt = (t1 - t0) // 7
        add_tasks([(UM + t0 + (g + 1) * dt, llsum, (qd, g, UM + t0 + g * dt, dt)) for g in range(7)])
    rr_tasks(BORD[0], 0, 0, P["RP0"], P["RP1"])
    add_tasks([(P["PW0"] + P["PWD"], prep_wo_a, (P["PW0"], P["PWD"]))])
    add_tasks([(P["PW1"] + (h + 1) * P["PWE"], prep_wo_b, (h, P["PW1"] + h * P["PWE"], P["PWE"])) for h in range(2)])
    for b in range(NB):
        b2f_s[b // 2, 0:1, _blk(b % 2)] = b2_v[b:b + 1, :].astype(f32)
    u_mid()
    for i in range(NNT):
        u_last(i, None if i == NNT - 1 else P["UEL"] if i == NNT - 2 else P["UED"])
    flush()
    assert slot_ctr[0] == len(mains) and all(("ll", qd, g) in ready for qd in range(NQ + 1) for g in range(7))
    assert all(("pr", j, hh) in ready for j in range(NB) for hh in range(2)) and ("rr", BORD[0]) in ready

    wait("w2", g7)
    lax.fori_loop(0, NP // 4, c_body, 0)
    outs = []
    for pa in range(0, NP, 2):
        outs += [out_copy(pa + n % 2, 0, 2, n // 2 * HD, (n // 2 + 1) * HD) for n in (1, 2, 3)]
        outs += [out_copy(pa, e0, e1, r0, r1) for (r0, r1, e0, e1) in (LAST_PARTS if pa % 4 else [(0, HD, 0, 2)])]
    wait("out", *outs)


@jax.jit
def pallas_parallel_sum__sliding_local_dilated__mixer_token_mlp__prompt_kernel(A_x, A_wqkv, A_wo, B_x, B_w1, B_b1, B_w2, B_b2):
    del B_x
    hbm = pl.BlockSpec(memory_space=pltpu.HBM)
    outT = pl.pallas_call(
        _kernel,
        out_shape=jax.ShapeDtypeStruct((1, D, S), bf16),
        in_specs=[hbm] * 7,
        out_specs=hbm,
        scratch_shapes=[
            pltpu.VMEM((NP, D, 2 * LB), bf16),
            pltpu.VMEM((NP, F, 2 * LB), bf16),
            pltpu.VMEM((NP, D, 2 * LB), bf16),
            pltpu.VMEM((NB + 1, D, LB), f32),
            pltpu.VMEM((NB, 2 * W * HH, LB), f32),
            pltpu.VMEM((NP, 32, 2 * LB), f32),
            pltpu.VMEM((D, 3 * D), bf16),
            pltpu.VMEM((D, D), bf16),
            pltpu.VMEM((S, F), bf16),
            pltpu.VMEM((NFB, LB), bf16),
            pltpu.VMEM((NB, LB), bf16),
            pltpu.VMEM((2, 3 * D + 64, LB), i32),
            pltpu.VMEM((7 * HA // 2, HD), u32),
            pltpu.VMEM((4, HD + 32, LB), i32),
            pltpu.VMEM((D, 2 * LB), i32),
            pltpu.VMEM((HD, S), u32),
            pltpu.VMEM((NP * QD, 5 * LB), u32),
            pltpu.VMEM((7 * QD, 2 * LB), u32),
            pltpu.VMEM((15 * QD, NKT * LB), u32),
            pltpu.VMEM((2 * RHK, 9 * LB), u32),
            pltpu.VMEM((D, F), f32),
            pltpu.VMEM((7 * HD, NFP * LB), f32),
            pltpu.VMEM((7 * QD, (NFP + 2) * LB), u32),
            pltpu.VMEM((NB, 2 * D, LB), f32),
            pltpu.VMEM((D, LB), f32),
            pltpu.VMEM((2 * RSK, 5 * LB), u32),
            pltpu.VMEM((49 * ED, 4 * LB), u32),
            pltpu.VMEM((7 * RRK, 9 * LB), u32),
            pltpu.VMEM((D, 4 * LB), f32),
            pltpu.VMEM((D, 4 * LB), f32),
            pltpu.VMEM((8, LB), i32),
            pltpu.SemaphoreType.DMA((9,)),
        ],
        compiler_params=pltpu.CompilerParams(vmem_limit_bytes=100 * 1024 * 1024,
                                             disable_bounds_checks=True,
                                             disable_semaphore_checks=True),
    )(jnp.swapaxes(A_x, 1, 2), A_wqkv, A_wo, B_w1, B_b1.reshape(NFB, LB), B_w2, B_b2.reshape(NB, LB))
    return jnp.swapaxes(outT, 1, 2)
```

```python
import jax
import jax.numpy as jnp
from jax import lax
import jax.experimental.pallas as pl
import jax.experimental.pallas.tpu as pltpu

S, D, F = 2048, 448, 1792
H, DH, W, DIL = 16, 28, 8, 2
LB = 128
NB = S // LB
NP = NB // 2
NFB = F // LB
NFP = NFB // 2
HH = H // 2
WH = W // 2
SH = DIL * WH
HD = D // 2
QD = D // 4
ED = D // 8
HA = 3 * HD
HB0 = 4
NKT = (NB - HB0) // 3
NNT = -(-NFB // 3)
RSK = NFP * LB // 2
RHK = NKT * LB // 2
NQ = NFP // 2
KL = NQ * LB + QD
RRK = 2 * LB
EPS = 1e-5
EPS_BF16 = 1.0013580322265625e-05
SCALE = DH ** -0.5
f32 = jnp.float32
bf16 = jnp.bfloat16
u32 = jnp.uint32
i32 = jnp.int32

SCOPES = False
P = dict(
    E1=3, E2=6, T3=-20, N2=16, NA3=2, T1=-200, T2=-200, L2T=100, L2D=440, H2T=900, H2D=340, L4T=920, L5T=0, W2X=500,
    QA=-330, QB=260, QC=-240, QE=420, KA=50, KB=230, KC=390, KE=450,
    LND=420, HSD=200, HTD=540, NH5=4, N4=2, N5=20, TM0=0, TMD=330, HT6=500, SGH=8, HL=140, LNA=0.28, LNB=0.46, LNBD=0.38, LNV=0.86,
    BD=375, MARG=300, LAG=200, LS=150, PP=130, PVL=500, PVPOS=18,
    US0=0, UE0=100, UED=3000, UEL=1600, UG=70, R6S=2850, R6E=1950,
    LL0=600, LL2=800, RP0=13000, RP1=15100, PW0=180, PWD=300, PW1=1000, PWE=600,
    RR0=-48, RR1=800, RRM=-20, RW=(8, 8, 8, 2, 7), BV0=117, BVS=717, BVD=620, EP0=0, EPD=864, EPL=290, SGR=8, SGT=8,
)
G = 4


def _as(x, dtype):
    return x if x.dtype == dtype else pltpu.bitcast(x, dtype)


def _pk(x):
    return pltpu.bitcast(x.astype(bf16), u32)


def _up(x):
    return pltpu.bitcast(x, bf16)


def _upf(x):
    return pltpu.bitcast(x, bf16).astype(f32)


def _rb(x):
    return x.astype(bf16).astype(f32)


def _word(lo, hi):
    lo, hi = [pltpu.bitcast(v.astype(f32), i32) for v in (lo, hi)]
    return lax.shift_right_logical(lo, 16) | hi


def _unword(w):
    return [pltpu.bitcast(w << 16, f32), pltpu.bitcast(w & -65536, f32)]


def _cat(xs, axis):
    return xs[0] if len(xs) == 1 else jnp.concatenate(xs, axis=axis)


def _x2(v):
    return jnp.concatenate([v, v], axis=0)


def _blk(b):
    return slice(b * LB, (b + 1) * LB)


def _rowsum8(a):
    return jnp.broadcast_to(jnp.sum(a, axis=0, keepdims=True), (8, a.shape[1]))


def _token(*deps):
    deps = [d for d in deps if d is not None]
    if not deps:
        return None
    if len(deps) == 1:
        return deps[0]
    bits = _as(deps[0], u32)
    for d in deps[1:]:
        bits = bits | _as(d, u32)
    return bits


def _lhs_ops(a11, a12, a21, a22):
    return [a11 + a22, a21 + a22, a11, a22, a11 + a12, a21 - a11, a12 - a22]


SIDX = {0: 0, 2: 1, 3: 2, 5: 3, 6: 4}
TOP = {0: ((0, 0), 1, (1, 1)), 1: ((0, 0),), 2: ((0, 1), -1, (1, 1)), 3: ((1, 0), -1, (0, 0)),
       4: ((1, 1),), 5: ((0, 0), 1, (0, 1)), 6: ((1, 0), 1, (1, 1))}


def _rhs_sums(b11, b12, b21, b22):
    return {0: b11 + b22, 2: b12 - b22, 3: b21 - b11, 5: b11 + b12, 6: b21 + b22}


def _rhs_op(p, blk):
    t = TOP[p]
    if len(t) == 1:
        return blk(*t[0])
    return blk(*t[0]) + blk(*t[2]) if t[1] > 0 else blk(*t[0]) - blk(*t[2])


def _combine(m, n=None):
    c12 = lambda: m[2] + m[4]
    c21 = lambda: m[1] + m[3]
    x = lambda: (m[2] - m[1]) + m[0]
    c = [lambda: (x() + m[6]) + (c21() - c12()), c12, c21, lambda: x() + m[5]]
    return [f() for f in c] if n is None else c[n]()


def _hk_lhs(a):
    s = [a[0][k] + a[1][k] for k in range(3)]
    return [a[0][0], s[0], s[1], a[1][1], a[0][0] + a[1][1], a[0][1] - a[0][0], a[1][0] - a[1][1], a[0][2],
            a[1][2], s[0] - a[1][2], s[2] - s[0], a[1][2] - a[1][0], s[1] - a[0][2], s[2] - s[1], a[0][2] - a[0][1]]


HKB = [((0, 0, 1), (1, 0, 1), (0, 2, -1)), ((0, 0, 1), (2, 0, 1), (0, 1, -1)), ((1, 1, 1), (2, 1, 1), (1, 0, -1)),
       ((1, 1, 1), (0, 1, 1), (1, 2, -1)), ((0, 1, 1), (1, 0, 1)), ((1, 0, 1),), ((0, 1, 1),),
       ((2, 2, 1), (1, 2, 1), (2, 0, -1)), ((2, 2, 1), (0, 2, 1), (2, 1, -1)), ((2, 0, 1), (0, 2, 1)), ((2, 0, 1),),
       ((0, 2, 1),), ((2, 1, 1), (1, 2, 1)), ((2, 1, 1),), ((1, 2, 1),)]


def _hk_terms(nj):
    out = {}
    for p, t in enumerate(HKB):
        t = [x for x in t if x[1] < nj]
        if t and (nj == 3 or p not in (7, 8)):
            out[p] = t
    return out


def _hk_combine(m, nj):
    x, y = (m[9] + m[11], m[12] + m[14]) if nj == 3 else (m[9], m[12])
    x0, y3 = x + m[0], y + m[3]
    c = [[(m[5] + m[10]) + x0, ((m[4] + m[5]) - y3) + m[2]], [((m[4] + m[6]) - x0) + m[1], (m[6] + m[13]) + y3]]
    if nj == 3:
        c[0].append(((m[10] - m[14]) + x) + m[7])
        c[1].append(((m[13] - m[11]) + y) + m[8])
    return c


def _kernel(x_hbm, wqkv_hbm, wo_hbm, w1_hbm, b1_hbm, w2_hbm, b2_hbm, out_hbm,
            x_v, w2_v, out_v, v_s, pr_s, b2f_s, wqkv_v, wo_v, w1_v, b1_v, b2_v, wt_s, lw_s, wo_s,
            wq_s, xnT_s, ra_s, lh_s, lk_s, rh_s, u0_s, um_s, lc_s, qk_s, op_s, rs_s, ll_s, rr_s, ola_s, olb_s, one_s, sems):
    sem_ctr = [1]

    class Group:
        def __init__(self, pairs):
            self.cps = [pltpu.make_async_copy(a, b, sems.at[sem_ctr[0]]) for (a, b) in pairs]
            sem_ctr[0] += 1

        def start(self):
            for c in self.cps:
                c.start()

        def wait(self):
            for c in self.cps:
                c.wait()

    def cp_x(p0, p1):
        return [(x_hbm.at[0, :, pl.ds(p * 2 * LB, 2 * LB)], x_v.at[p]) for p in range(p0, p1)]

    def cp_w2(p0, p1):
        return [(w2_hbm.at[:, pl.ds(p * 2 * LB, 2 * LB)], w2_v.at[p]) for p in range(p0, p1)]

    def cp_w1(b0, b1, i0=0, i1=NFP):
        sl = pl.ds(b0 * LB, (b1 - b0) * LB)
        cl = pl.ds(i0 * 2 * LB, (i1 - i0) * 2 * LB)
        return [(w1_hbm.at[sl, cl], w1_v.at[sl, cl])]

    tl = []
    mxu = [0, 0, 0, 0]
    nxt = [0]
    hist = []
    tasks = []
    dls = []
    ready = set()
    pos = []
    true = {}

    def tie(v, z):
        if z is None:
            return v
        def fit(a):
            a = _cat([a] * (v.shape[0] // 8), 0)
            return a if v.shape[1] == LB else a[:, 0:v.shape[1]]
        if v.shape not in true:
            true[v.shape] = fit(pos[0]) > 0
        return lax.select(true[v.shape], v, fit(_as(z, v.dtype)))

    def tie8(v, z):
        return v if z is None else jnp.concatenate([tie(v[0:8], z), v[8:16]], axis=0)

    def add_tasks(todo):
        tasks.extend(todo)
        tasks.sort(key=lambda x: x[0])

    def flush(t=None):
        while tasks and (t is None or tasks[0][0] < t):
            _, fn, args = tasks.pop(0)
            fn(*args)

    def reset():
        assert not tasks
        dls.clear()
        tl.clear()
        hist.clear()
        mxu[:] = [0, 0, 0, 0]
        nxt[0] = 0

    def now():
        return sum(mxu) // 4

    def wait(name, *cps):
        flush()
        if SCOPES:
            with jax.named_scope("wait_" + name):
                for c in cps:
                    c.wait()
        else:
            for c in cps:
                c.wait()
        reset()

    def mm1(lhs, rhs, pace=True):
        flush(now())
        start = mxu[nxt[0]]
        due = [v for (t, v) in dls if t <= start] if pace else []
        if due:
            dls[:] = [(t, v) for (t, v) in dls if t > start]
            tile = _up(tie(pltpu.bitcast(lhs[0:16, 0:LB], u32), _token(*due)))
            row = tile if lhs.shape[1] == LB else jnp.concatenate([tile, lhs[0:16, LB:]], axis=1)
            lhs = jnp.concatenate([row, lhs[16:]], axis=0)
        r = jnp.dot(lhs, rhs, preferred_element_type=f32)
        m, k = lhs.shape
        first_done = None
        for _ in range(-(-rhs.shape[1] // LB)):
            end = 0
            for _ in range(-(-k // LB)):
                mxu[nxt[0]] += m
                end = max(end, mxu[nxt[0]])
                nxt[0] = (nxt[0] + 1) % 4
            if first_done is None:
                first_done = end
        if pace:
            tl.append((first_done - m, first_done, r))
        return r

    def mm(lhs, rhs, init=None):
        k = lhs.shape[1]
        r, k0 = init, 0
        while k0 < k:
            k1 = min(k, k0 + (4 - nxt[0]) * LB)
            part = mm1(lhs[:, k0:k1], rhs[k0:k1], pace=k1 - k0 > LB)
            r = part if r is None else r + part
            k0 = k1
        return r

    def at(t, *more):
        best = None
        if t is not None and t >= 0:
            t = min(t, now() - 1)
            for (a, b, r) in tl:
                if a <= t and (best is None or min(b, t) > best[0]):
                    row = int(min((t - a) / (b - a), 0.999) * (r.shape[0] // 8)) * 8
                    best = (min(b, t), r, row)
        return _token(None if best is None else best[1][best[2]:best[2] + 8, 0:LB], *more)

    def strassen(lhs, rhs, order, split_last=False, init=None, m=None):
        m = [None] * 7 if m is None else m
        for p in order:
            flush(now())
            l, r = lhs(p), rhs(p)
            c0 = None if init is None else init[p]
            if split_last and p == order[-1]:
                kk = (-(-r.shape[0] // LB) - 2) * LB
                hm = l.shape[0] // 2
                hd = mm(l[:, :kk], r[:kk], c0) if kk else c0
                tail = jnp.concatenate([mm(l[:hm, kk:], r[kk:]), mm(l[hm:, kk:], r[kk:])], axis=0)
                m[p] = tail if hd is None else hd + tail
            else:
                m[p] = mm(l, r, c0)
        return m

    def wcol(hh, p):
        return p * D + (1 - hh if p == 1 else hh) * HD

    def wrows(hh, g, z=None):
        p, d = divmod(2 * g, DH)
        t = [jnp.concatenate([wt_s[c, pl.ds(wcol(hh, p) + d + e, HH, stride=DH), :]
                              for e in range(2)], axis=0) for c in range(2)]
        return _unword(jnp.concatenate([tie(t[0], z), tie(t[1][:, 0:HD - LB], z)], axis=1))

    wt_done = set()

    def prep_wqkv(part, ga, gb, paced):
        def need(hh, p, z):
            lo = wcol(hh, p)
            for ct in range(lo // LB, -(-(lo + HD) // LB)):
                if ct in wt_done:
                    continue
                wt_done.add(ct)
                cols = slice(ct * LB, min((ct + 1) * LB, 3 * D))
                wd = _word(wqkv_v[0:HD, cols], wqkv_v[HD:D, cols])
                wd = jnp.concatenate([tie(wd[r:r + 8], z if r % LB == 0 else None) for r in range(0, HD, 8)], axis=0)
                wT = wd.T
                wt_s[0, cols, :] = wT[:, 0:LB]
                wt_s[1, cols, 0:HD - LB] = wT[:, LB:HD]

        def put(p, g, v):
            lw_s[p * (HA // 2) + g * 8:p * (HA // 2) + g * 8 + 8, :] = _pk(v)

        def half(hh, g0, g1, t0=None, dur=None):
            pr, ps = ((2, 4), (3, 1))[hh]
            for g in range(g0, g1):
                t = None if t0 is None else t0 + (g - g0) * dur // (g1 - g0)
                need(hh, 2 * g // DH, at(None if t is None else t - P["W2X"]))
                a1, a2 = wrows(hh, g, at(t))
                put(pr, g, a2 if hh else a1)
                put(ps, g, a1 + a2)
            if g1 == gb:
                ready.update({("lw", part, pr), ("lw", part, ps)})

        def rest(g0, g1, t0, dur):
            assert ("lw", part, 1) in ready
            for g in range(g0, g1):
                z = at(t0 + (g - g0) * dur // (g1 - g0))
                ops = _lhs_ops(*wrows(0, g, z), *wrows(1, g, z))
                for p in (0, 5, 6):
                    put(p, g, ops[p])
            if g1 == gb:
                ready.update({("lw", part, 0), ("lw", part, 5), ("lw", part, 6)})
        t2, d2, t3, d3 = paced
        half(0, ga, gb)
        n = (gb - ga) // 14
        add_tasks([(now() + t2 + (k + 1) * d2 // n, half,
                    (1, ga + 14 * k, ga + 14 * k + 14, now() + t2 + k * d2 // n, d2 // n)) for k in range(n)])
        n = (gb - ga) // 7
        add_tasks([(now() + t3 + (k + 1) * d3 // n, rest,
                    (ga + 7 * k, ga + 7 * k + 7, now() + t3 + k * d3 // n, d3 // n)) for k in range(n)])

    def prep_wo_a(t0, dur):
        for g in range(HD // 16):
            w = _word(wo_v[g * 16:g * 16 + 16, :], wo_v[HD + g * 16:HD + g * 16 + 16, :])
            z = at(t0 + g * dur // (HD // 16))
            for c in range(4):
                cw = min(LB, D - c * LB)
                wo_s[c, g * 16:g * 16 + 16, 0:cw] = tie(w[:, c * LB:c * LB + cw], z)
        ready.add("wo")

    def prep_wo_b(h, t0, dur):
        assert "wo" in ready
        for c in range(4):
            cw = min(LB, D - c * LB)
            rows = [wo_s[c, pl.ds(d, HH, stride=DH), :][:, 0:cw] for d in range(h * DH // 2, (h + 1) * DH // 2)]
            rows.append(jnp.zeros((LB - QD, cw), i32))
            wq_s[c * LB:c * LB + cw, _blk(h)] = jnp.concatenate(rows, axis=0).T
        outs = []
        for g in range(HD // 16):
            z = at(t0 + g * dur // (HD // 16))
            a = [v for r in (g * 16, HD + g * 16) for v in _unword(tie(wq_s[r:r + 16, _blk(h)], z))]
            for p, v in enumerate(_lhs_ops(*a)):
                lc_s[p * QD + g * 8:p * QD + g * 8 + 8, _blk(NFP + h)] = _pk(v)
                outs.append(v[0:8])
        ready.update({("lc", NFP + h, g) for g in range(HD // 16)})
        dls.append((t0 + dur + 250, _token(*outs)))

    RG = 16
    NG = D // RG
    stat2 = {}

    def ln(b, t0=None, dur=None):
        def xg(g):
            return x_v[b // 2, g * RG:(g + 1) * RG, _blk(b % 2)].astype(f32)

        def step(v, g, fr, s, q):
            if t0 is None or g % 4:
                return v
            acc = [] if s is None else [s[0:8], s[8:16], q[0:8], q[8:16]]
            return tie(v, at(t0 + fr * dur, *acc))

        x0 = jnp.broadcast_to(xg(0)[0:1], (8, LB))
        s = q = None
        for g in range(NG):
            x0 = step(x0, g, P["LNA"] * g / NG, s, q)
            c = xg(g) - _x2(x0)
            s = c if s is None else s + c
            q = c * c if q is None else q + c * c
        dm = _rowsum8(s) * (1.0 / D)
        mu = _rb(x0 + dm)
        var = _rb(jnp.maximum(_rowsum8(q) * (1.0 / D) - dm * dm, 0.0))
        r1 = 1.0 / _rb(jnp.sqrt(_rb(var + EPS_BF16)))
        s = q = None
        for g in range(NG):
            mu = step(mu, g, P["LNB"] + P["LNBD"] * g / NG, s, q)
            xn = _rb(xg(g) - _x2(mu)) * _x2(r1)
            xnT_s[g * 8:g * 8 + 8, _blk(b)] = _pk(xn)
            s = xn if s is None else s + xn
            q = xn * xn if q is None else q + xn * xn
        mu2 = _rowsum8(s) * (1.0 / D)
        var2 = jnp.maximum(_rowsum8(q) * (1.0 / D) - mu2 * mu2, 0.0)
        stat2[b] = (mu2, 0.5 * lax.rsqrt(var2 + EPS))

    def hpair(b, t0=None, dur=None):
        ng = HD // RG
        st = [stat2[b], stat2[b + 1]]
        for g in range(ng):
            if b < HB0:
                zz = [at(None if t0 is None else t0 + (4 * g + k) * dur // (4 * ng)) for k in range(4)]
            else:
                zz = [at(t0 + g * dur // ng), None, None, at(t0 + g * dur // ng + P["SGT"])]
            xq = [_upf(tie(xnT_s[r:r + 8, _blk(b + e)], zz[2 * (r >= QD) + e]))
                  for r in (g * 8, QD + g * 8) for e in range(2)]
            ro = (b // 2) * QD + g * 8
            for p, v in _rhs_sums(*xq).items():
                ra_s[ro:ro + 8, _blk(SIDX[p])] = _pk(v)
            if b < HB0:
                hq = [(v - _x2(st[n % 2][0])) * _x2(st[n % 2][1]) for n, v in enumerate(xq)]
                for p, v in enumerate(_lhs_ops(*hq)):
                    lh_s[p * QD + g * 8:p * QD + g * 8 + 8, _blk(b // 2)] = _pk(v)
        ready.add(("xn", b))
        if b >= 6:
            got = ra_s[(b // 2) * QD:(b // 2 + 1) * QD, :]
            dls.append((t0 + dur + P["HL"], _token(*[got[r:r + 8, _blk(c)] for r in range(0, QD, 8) for c in range(5)])))

    def htile(b, r, z=None):
        return (_upf(tie(xnT_s[r:r + 8, _blk(b)], z)) - _x2(stat2[b][0])) * _x2(stat2[b][1])

    def htriple(t, t0, dur):
        ng = HD // RG
        for g in range(ng):
            zz = [at(t0 + (3 * g + k) * dur // (3 * ng)) for k in range(3)]
            a = [[htile(HB0 + 3 * t + k, h * QD + g * 8, zz[k]) for k in range(3)] for h in range(2)]
            for p, v in enumerate(_hk_lhs(a)):
                lk_s[p * QD + g * 8:p * QD + g * 8 + 8, _blk(t)] = _pk(v)
        ready.add(("lh", t))

    def ln_tasks(b, t, lnd, hsd):
        for fn, bb, dur, adv in ((ln, b, lnd, P["LNV"]), (ln, b + 1, lnd, P["LNV"]), (hpair, b, hsd, 1.0)):
            add_tasks([(t + int(dur * adv), fn, (bb, t, dur))])
            t += int(dur * adv)
        return t

    def tsum(kp, i, slot_, n, t0, dur):
        for g in range(LB // 16):
            z, z2 = at(t0 + g * dur // 8), at(t0 + g * dur // 8 + P["SGT"])
            t1, t2 = [w1_v[(2 * kp + e) * LB + g * 16:(2 * kp + e) * LB + g * 16 + 16,
                           2 * i * LB:(2 * i + 2) * LB].astype(f32) for e in range(2)]
            ro = slot_ * RSK + n * (LB // 2) + g * 8
            for p, v in _rhs_sums(tie8(t1[:, :LB], z), t1[:, LB:], t2[:, :LB], tie8(t2[:, LB:], z2)).items():
                rs_s[ro:ro + 8, _blk(SIDX[p])] = _pk(v)
        ready.add(("rs", kp, i))

    def u_rhs(p, i, kps, slot_, n0):
        if p in SIDX:
            assert all(("rs", kp, i) in ready for kp in kps)
            ro = slot_ * RSK + n0 * (LB // 2)
            return _up(rs_s[ro:ro + len(kps) * (LB // 2), _blk(SIDX[p])])
        e = 0 if p == 1 else 1
        return _cat([w1_v[_blk(2 * kp + e), _blk(2 * i + e)] for kp in kps], 0)

    LATE = (NFP - 1, 6)

    def ujob(kp, i, p, split):
        flush(now())
        assert ("xn", 2 * kp) in ready
        l, r = _up(lh_s[p * QD:(p + 1) * QD, _blk(kp)]), u_rhs(p, i, [kp], kp, i)
        v = jnp.concatenate([mm1(l[:QD], r), mm1(l[QD:], r)], axis=0) if split else mm1(l, r)
        rows = slice(p * HD, (p + 1) * HD)
        um_s[rows, _blk(i)] = v

    def u_early(kp, i0, i1, carry, n, t0, dt, nsplit=0):
        for k, i in enumerate(range(i0, i1)):
            add_tasks([(t0 + (k + 1) * dt, tsum, (kp, i, kp, i, t0 + k * dt, dt))])
        jobs = (carry + [(kp, i, p) for i in range(i0, i1) for p in (1, 4)]
                + [(kp, i, p) for i in range(i0, i1) for p in SIDX if (i, p) != LATE])
        for c, job in enumerate(jobs[:n]):
            ujob(*job, c >= n - nsplit)
        return jobs[n:]

    def u_mid():
        jobs = [(i, p) for i in range(2) for p in (4, 1)]
        for i in range(NFP):
            jobs += [(i, p) for p in (2, 3, 0, 5, 6)] + [(i + 2, p) for p in (4, 1) if i + 2 < NFP]
        m = [[None] * 7 for _ in range(NFP)]
        for i, p in jobs:
            flush(now())
            late = (i, p) == LATE
            l = _up(lh_s[p * QD:(p + 1) * QD, (0 if late else LB):])
            r = _cat([u_rhs(p, i, [0], 0, i)] * late + [u_rhs(p, i, [1], 1, i)], 0)
            v = jnp.concatenate([mm1(l[:QD], r), mm1(l[QD:], r)], axis=0) if late else mm1(l, r)
            if not late:
                v = v + um_s[p * HD:(p + 1) * HD, _blk(i)]
            if p in (2, 3):
                v = v + 0.5 * b1_v[2 * i + 3 - p:2 * i + 4 - p, :].astype(f32)
            m[i][p] = v
            if p == 6:
                for n, c in enumerate(_combine(m[i])):
                    u0_s[n // 2 * HD:(n // 2 + 1) * HD, _blk(2 * i + n % 2)] = c

    def nj_of(i):
        return min(3, NFB - 3 * i)

    def hsum(t, i, t0, dur):
        nj = nj_of(i)
        sums = [(p, tm) for p, tm in _hk_terms(nj).items() if len(tm) > 1]
        tied = {(1, 0): 0, (2, 0): 1, (1, 2): 2, (2, 2): 3} if nj == 3 else {(1, 0): 0, (0, 1): 2}
        for g in range(LB // 16):
            b = {}
            for k in range(3):
                r = (HB0 + 3 * t + k) * LB + g * 16
                w = w1_v[r:r + 16, 3 * i * LB:(3 * i + nj) * LB].astype(f32)
                for j in range(nj):
                    z = at(t0 + g * dur // 8 + tied[k, j] * P["SGH"]) if (k, j) in tied else None
                    b[k, j] = tie8(w[:, _blk(j)], z)
            ro = (i % 2) * RHK + t * (LB // 2) + g * 8
            for n, (p, tm) in enumerate(sums):
                v = b[tm[0][:2]]
                for (k, j, sg) in tm[1:]:
                    v = v + b[k, j] if sg > 0 else v - b[k, j]
                rh_s[ro:ro + 8, _blk(n)] = _pk(v)
        ready.add(("rh", t, i))

    def gelu_half(hx, z):
        c = 0.7978845608028654
        return hx + hx * jnp.tanh(tie(hx * (2.0 * c + (8.0 * c * 0.044715) * (hx * hx)), z))

    gl = {}

    def u_epilogue(i, m, gs, t0, dur):
        nj = nj_of(i)
        for n, g in enumerate(gs):
            c = _hk_combine({p: v[g * 16:g * 16 + 16] for p, v in m.items()}, nj)
            for j in range(nj):
                f = 3 * i + j
                t = None if t0 is None else t0 + (n * nj + j) * dur // (len(gs) * nj) - P["UG"]
                gl[f, g] = [gelu_half(c[h][j] + u0_s[h * HD + g * 16:h * HD + g * 16 + 16, _blk(f)], at(t))
                            for h in range(2)]
                if f % 2 == 1:
                    g0, g1 = gl.pop((f - 1, g)), gl.pop((f, g))
                    for p, v in enumerate(_lhs_ops(g0[0], g1[0], g0[1], g1[1])):
                        lc_s[p * QD + g * 8:p * QD + g * 8 + 8, _blk(f // 2)] = _pk(v)
                    ready.add(("lc", f // 2, g))

    def u_last(i, edur):
        terms = _hk_terms(nj_of(i))
        sums = [p for p, tm in terms.items() if len(tm) > 1]
        m = {}
        order = ((10, 11, 14, 5, 13, 6, 9, 7, 0, 12, 8, 3, 4, 1, 2) if i == 0
                 else (10, 11, 9, 14, 7, 5, 0, 13, 12, 8, 6, 3, 4, 1, 2))
        for p in [p for p in order if p in terms]:
            flush(now())
            assert all(("lh", t) in ready for t in range(NKT))
            if p in sums:
                assert all(("rh", t, i) in ready for t in range(NKT))
                r = _up(rh_s[(i % 2) * RHK:(i % 2 + 1) * RHK, _blk(sums.index(p))])
            else:
                k, j, _ = terms[p][0]
                r = _cat([w1_v[_blk(HB0 + 3 * t + k), _blk(3 * i + j)] for t in range(NKT)], 0)
            m[p] = mm(_up(lk_s[p * QD:(p + 1) * QD, :]), r)
        if edur is None:
            u_epilogue(i, m, list(range(HD // 16)), None, None)
        else:
            t = now() + P["UE0"]
            add_tasks([(t + (g + 1) * edur // 7, u_epilogue, (i, m, [g, g + 7], t + g * edur // 7, edur // 7))
                       for g in range(7)])

    def llsum(qd, g, t0, dur):
        i0 = 2 * qd if qd < NQ else NFP
        assert all(("lc", i0 + e, g + 7 * h) in ready for e in range(2) for h in range(2))
        for p in range(7):
            zz = [at(t0 + p * dur // 7), at(t0 + p * dur // 7 + P["SGT"])]
            a = [tie(lc_s[p * QD + h * ED + g * 8:p * QD + h * ED + g * 8 + 8, _blk(i0 + e)], zz[h] if h == e else None)
                 for h in range(2) for e in range(2)]
            ops = _lhs_ops(*[_upf(v) for v in a])
            for q in (0, 1, 4, 5, 6):
                r = (p * 7 + q) * ED + g * 8
                ll_s[r:r + 8, _blk(qd)] = _pk(ops[q])
        ready.add(("ll", qd, g))

    AORD = (4, 2, 1, 3, 0, 5, 6)

    def stage_a(b, parts="qkv", order=AORD, split_last=False, m=None):
        r0, r1 = {"q": (0, HD), "kv": (HD, HA), "qkv": (0, HA)}[parts]

        def lhs(p):
            assert all(("lw", pt, p) in ready for pt in ("q", "kv") if pt in parts)
            return _up(lw_s[(p * HA + r0) // 2:(p * HA + r1) // 2, :])

        def rhs(p):
            assert ("xn", b) in ready
            if p in SIDX:
                return _up(ra_s[(b // 2) * QD:(b // 2 + 1) * QD, _blk(SIDX[p])])
            return _up(xnT_s[0:QD, _blk(b)] if p == 1 else xnT_s[QD:HD, _blk(b + 1)])
        m = strassen(lhs, rhs, order, split_last, m=m)
        for n, ps in enumerate((range(7), (2, 4), (1, 3), (0, 1, 2, 5))):
            if all(m[p] is not None for p in ps) and any(p in order for p in ps):
                hh, e = divmod(n, 2)
                c = _combine(m, n)
                qk_s[b + e, hh * D + r0:hh * D + min(r1, D), :] = c[0:min(r1, D) - r0]
                if r1 > D:
                    v_s[b + e + 1, hh * HD:(hh + 1) * HD, :] = c[D - r0:]
        if all(v is not None for v in m):
            ready.update({(pt, b + e) for pt in ("q", "kv") if pt in parts for e in range(2)})
        return m

    lane0 = lax.broadcasted_iota(i32, (HH, LB), 1)
    zeros8 = jnp.zeros((HH, LB), f32)

    def mk_shift(z):
        lane = tie(lane0, z)
        masks = {}

        def pick(n, a, b):
            if n not in masks:
                masks[n] = lane < n
            return lax.select(masks[n], a, b)

        def fwd(cur, prev, sh):
            return cur if sh == 0 else pltpu.roll(pick(LB - sh, cur, prev), sh, 1)

        def bwd(cur, nxt_):
            return pltpu.roll(pick(SH, nxt_, cur), LB - SH, 1)
        return fwd, bwd

    def grp_shift(t, bd):
        lag = max(2, -(-P["LAG"] * DH // (G * bd)))
        return mk_shift(at(t, *(hist[-lag] if len(hist) >= lag else [])))

    raw, probs = {}, {}

    def attn_qk(j, hh, t, bd):
        jn = min(j + 1, NB - 1)
        assert ("q", jn) in ready and ("kv", j) in ready
        acc = [None] * WH
        accp = [None] * WH
        for d in range(DH):
            if d % G == 0:
                if d > 0:
                    hist.append(acc + accp)
                fwd, bwd = grp_shift(t + d * bd // DH, bd)
            r = hh * D + d * HH
            q = qk_s[j, r:r + HH, :]
            qp = bwd(q, qk_s[jn, r:r + HH, :])
            rk = (1 - hh) * D + HD + d * HH
            k = qk_s[j, rk:rk + HH, :]
            kp = qk_s[j - 1, rk:rk + HH, :] if j > 0 else zeros8
            for a in range(WH):
                ks = fwd(k, kp, DIL * a)
                t0, t1 = q * ks, qp * ks
                acc[a] = t0 if d == 0 else acc[a] + t0
                accp[a] = t1 if d == 0 else accp[a] + t1
        hist.append(acc + accp)
        raw[j, hh] = (acc, accp)

    def attn_sm(j, hh, t):
        fwd, _ = mk_shift(at(t))
        acc, accp = raw[j, hh]
        prev = raw.pop((j - 1, hh))[1] if j > 0 else [zeros8] * WH
        lg = acc + [fwd(accp[a], prev[a], SH) for a in range(WH)]
        lg = [a * SCALE for a in lg]
        if j == 0:
            lg = [lg[0]] + [jnp.where(lane0 >= DIL * w, lg[w], -1e9) for w in range(1, W)]
        m = lg[0]
        for w in range(1, W):
            m = jnp.maximum(m, lg[w])
        e = [jnp.exp(l - m) for l in lg]
        den = e[0]
        for w in range(1, W):
            den = den + e[w]
        inv = 1.0 / den
        p = [x * inv for x in e]
        for a in range(WH):
            pr_s[j, (hh * W + a) * HH:(hh * W + a + 1) * HH, :] = p[a]
        probs[j, hh] = p[WH:]

    def attn_pp(j, hh, t):
        _, bwd = mk_shift(at(t))
        p = probs.pop((j, hh))
        pn = probs[j + 1, hh] if j + 1 < NB else p
        for a in range(WH):
            pr_s[j, (hh * W + WH + a) * HH:(hh * W + WH + a + 1) * HH, :] = bwd(p[a], pn[a])
        ready.add(("pr", j, hh))

    def attn_pv(j, hh, dst, e, t, bd):
        assert not isinstance(j, int) or ("pr", j, hh) in ready
        assert e == 0 or ("o", dst, hh, e - 1) in ready
        pa = [pr_s[j, (hh * W + a) * HH:(hh * W + a + 1) * HH, :] for a in range(W)]
        p, pp = pa[:WH], pa[WH:]
        outs = []
        for d in range(DH):
            if d % G == 0:
                if d > 0:
                    hist.append([])
                fwd, _ = grp_shift(t + d * bd // DH, bd)
            r = hh * HD + d * HH
            v = v_s[j + 1, r:r + HH, :]
            vp = v_s[j, r:r + HH, :]
            o = op = None
            for a in range(WH):
                vs = fwd(v, vp, DIL * a)
                o = p[a] * vs if a == 0 else o + p[a] * vs
                op = pp[a] * vs if a == 0 else op + pp[a] * vs
            opp = zeros8 if (isinstance(j, int) and j == 0) else op_s[r:r + HH, :]
            op_s[r:r + HH, :] = op
            outs.append(o + fwd(op, opp, SH))
            ol[dst][r:r + HH, _blk(e)] = outs[-1]
        hist.append([])
        ready.add(("o", dst, hh, e))
        dls.append((t + bd + P["PVL"], _token(*outs)))

    ol = [ola_s, olb_s]
    mains = [("qk", j, hh) for j in range(NB) for hh in range(2)]
    mains = (mains[:P["PVPOS"]] + [("pv", j, hh) for j in range(4) for hh in range(2)]
             + mains[P["PVPOS"]:] + [None, None])
    slot_ctr = [0]

    def slot(t, bd):
        n = slot_ctr[0]
        slot_ctr[0] += 1
        it = mains[n]
        if it is None:
            pass
        elif it[0] == "qk":
            attn_qk(it[1], it[2], t, bd)
        else:
            attn_pv(it[1], it[2], 0, it[1], t, bd)
        if n >= 1 and mains[n - 1] is not None and mains[n - 1][0] == "qk":
            attn_sm(mains[n - 1][1], mains[n - 1][2], t + P["LS"])
        if n >= 2 and mains[n - 2] is not None and mains[n - 2][0] == "qk":
            _, j, hh = mains[n - 2]
            if j > 0:
                attn_pp(j - 1, hh, t + P["PP"])
            if j == NB - 1:
                attn_pp(j, hh, t + P["PP"])

    NRG = 8 * (NQ + 1) + 7
    PD = 8 * QD
    BORD = (1, 3, 2, 4, 0, 5, 6)
    LORD = (2, 4, 1, 3, 0, 5, 6)
    LAST_PARTS = [(0, QD, 1, 2), (QD, HD, 0, 2), (0, QD, 0, 1)]

    def rr_prep(p, pa, src, n0, n1, t0, dur):
        assert ("rr", p) not in ready
        for n in range(n0, n1):
            z = at(t0 + (n - n0) * dur // (n1 - n0))
            z2 = at(t0 + (n - n0) * dur // (n1 - n0) + P["SGR"])
            qd, g = divmod(n, 8)

            def wrow(i):
                return _rhs_op(p, lambda x, y: w2_v[pa + y, (2 * i + x) * LB + g * 16:(2 * i + x) * LB + g * 16 + 16, :]
                               .astype(f32))

            def orow(h):
                def blk(x, y):
                    assert ("o", src, x, 2 * y + 1) in ready
                    r = x * HD + h * QD + g * 16
                    return ol[src][r:r + 16, y * 2 * LB:(y + 1) * 2 * LB]
                return _rhs_op(p, blk)
            ro = p * RRK + g * 8
            if qd == NQ:
                if p in SIDX:
                    r = wrow(2 * NQ)
                    for e in range(2):
                        rr_s[ro:ro + 8, _blk(7 + e)] = _pk(tie8(r[:, _blk(e)], z))
                continue
            r1, r2 = (wrow(2 * qd), wrow(2 * qd + 1)) if qd < NQ else (orow(0), orow(1))
            ro += min(qd, NQ) * (LB // 2)
            c11, c22 = tie8(r1[:, :LB], z), tie8(r2[:, LB:], z2)
            sm = _rhs_sums(c11, r1[:, LB:], r2[:, :LB], c22)
            if p in SIDX or qd > NQ:
                sm.update({1: c11, 4: c22})
            for q, v in sm.items():
                rr_s[ro:ro + 8, _blk(q)] = _pk(v)
        if n1 == NRG:
            ready.add(("rr", p))

    def rr_tasks(p, pa, src, t0, t1):
        cuts = list(range(0, NRG, 8)) + [NRG]
        acc, tot = 0, sum(P["RW"])
        for a, b, w in zip(cuts[:-1], cuts[1:], P["RW"]):
            ta, tb = t0 + acc * (t1 - t0) // tot, t0 + (acc + w) * (t1 - t0) // tot
            add_tasks([(tb, rr_prep, (p, pa, src, a, b, ta, tb - ta))])
            acc += w

    def out_copy(pidx, e0, e1, r0, r1):
        off = pidx * (2 * LB) + e0 * LB
        if not isinstance(pidx, int):
            off = pl.multiple_of(off, LB)
        rs = pl.ds(r0, r1 - r0)
        return pltpu.make_async_copy(out_v.at[pidx, rs, pl.ds(e0 * LB, (e1 - e0) * LB)],
                                     out_hbm.at[0, rs, pl.ds(off, (e1 - e0) * LB)], sems.at[0])

    def b_out(pa, n, m, part, t0=None, dur=None):
        a, y = divmod(n, 2)
        r0, r1, e0, e1 = part
        cols = slice(e0 * LB, e1 * LB)
        for r in range(r0, r1, 16):
            c = _combine([None if v is None else v[r:r + 16, cols] for v in m], n)
            rows = slice(a * HD + r, a * HD + r + 16)
            o = c + x_v[pa + y, rows, cols].astype(f32)
            if t0 is not None:
                o = jnp.concatenate([tie(o[:, 0:LB], at(t0 + (r - r0) * dur // (r1 - r0))), o[:, LB:]], axis=1)
            out_v[pa + y, rows, cols] = o.astype(bf16)
        out_copy(pa + y, e0, e1, a * HD + r0, a * HD + r1).start()

    def big_piece(pa, pan, cur, last):
        t0 = now()
        for n in range(7):
            ta, tb = t0 + n * PD + P["RR0"], t0 + n * PD + P["RR1"]
            if n < 6:
                rr_tasks(BORD[n + 1], pa, cur, ta, tb)
            else:
                rr_tasks(BORD[0], pan, 1 - cur, ta, tb - (P["RRM"] if last else 0))
        ready.difference_update({("o", 1 - cur, hh, e) for hh in range(2) for e in range(4)})
        for n in range(8):
            e, hh = divmod(n, 2)
            t = t0 + P["BV0"] + n * P["BVS"]
            add_tasks([(t + P["BVD"], attn_pv, (pan * 2 + e, hh, 1 - cur, e, t, P["BVD"]))])
        m = [None] * 7
        for p in BORD:
            flush(now())
            assert ("rr", p) in ready
            x, y = TOP[p][0]

            def lhs(q):
                if q in (2, 3):
                    rows = slice(p * QD + (q - 2) * ED, p * QD + (q - 1) * ED)
                    return _up(jnp.concatenate([lc_s[rows, _blk(2 * qd + q - 2)] for qd in range(NQ)]
                                               + [lc_s[rows, (NFP + q - 2) * LB:(NFP + q - 2) * LB + QD]], axis=1))
                return _up(ll_s[(p * 7 + q) * ED:(p * 7 + q + 1) * ED, 0:KL])

            def rhs(q):
                if p in SIDX or q in SIDX:
                    return _up(rr_s[p * RRK:p * RRK + KL // 2, _blk(q)])
                h = 0 if q == 1 else 1
                return _cat([w2_v[pa + y, _blk(2 * (2 * qd + h) + x), _blk(h)] for qd in range(NQ)]
                            + [_up(rr_s[p * RRK + NQ * LB // 2:p * RRK + KL // 2, _blk(q)])], 0)
            rl = (_up(rr_s[p * RRK:p * RRK + LB // 2, 7 * LB:9 * LB]) if p in SIDX
                  else w2_v[pa + y, _blk(4 * NQ + x), :])
            ll = _up(lc_s[p * QD:(p + 1) * QD, _blk(2 * NQ)])
            ex = [mm1(ll[:QD], rl), mm1(ll[QD:], rl)]
            e12, e21 = ex[0][:, LB:], ex[1][:, :LB]
            e11 = (ex[0][:, :LB] + e12) - e21
            lf = strassen(lhs, rhs, LORD)
            ready.discard(("rr", p))
            if p in (2, 3):
                for q in (2, 3):
                    lf[q] = lf[q] + b2f_s[pa + 3 - p, 0:1, _blk(3 - q)]
            c12 = (lf[2] + e12) + lf[4]
            c21 = (lf[1] + e21) + lf[3]
            xx = (lf[2] - lf[1]) + lf[0]
            c22 = (xx + ex[1][:, LB:]) + lf[5]
            c11 = ((xx + e11) + (c21 - c12)) + lf[6]
            m[p] = jnp.concatenate([jnp.concatenate([c11, c12], axis=1),
                                    jnp.concatenate([c21, c22], axis=1)], axis=0)
            n = {3: 2, 4: 1, 5: 3, 6: 0}.get(p)
            if n is not None and not (last and n == 0):
                t, epd = now() + P["EP0"], P["EPL"] if (last and n == 3) else P["EPD"]
                add_tasks([(t + epd, b_out, (pa, n, list(m), (0, HD, 0, 2), t, epd))])
        if last:
            flush()
            for part in LAST_PARTS:
                b_out(pa, 0, m, part)

    def c_body(it, carry):
        reset()
        pos[:] = [one_s[...]]
        true.clear()
        ready.update({("rr", BORD[0])} | {("o", 0, hh, e) for hh in range(2) for e in range(4)})
        big_piece(4 * it, 4 * it + 2, 0, False)
        big_piece(4 * it + 2, lax.rem(4 * it + 4, NP), 1, True)
        assert ("rr", BORD[0]) in ready and all(("o", 0, hh, 3) in ready for hh in range(2))
        return carry

    E1, E2 = P["E1"], P["E2"]
    x0 = Group(cp_x(0, 1))
    g1 = Group(cp_w1(0, 2, 0, E1))
    g2 = Group(cp_w1(0, 2, E1, E2) + cp_x(1, 2))
    wq, wkv = [[(wqkv_hbm.at[:, cl], wqkv_v.at[:, cl])] for cl in (pl.ds(0, 4 * LB), pl.ds(4 * LB, 3 * D - 4 * LB))]
    g3 = Group((cp_w1(0, 2, E2, NFP) if E2 < NFP else []) + wq)
    g4 = Group(wkv + cp_x(2, 3))
    g5 = Group(cp_x(3, NP))
    g6 = Group(cp_w1(2, NB) + [(wo_hbm, wo_v), (b1_hbm, b1_v), (b2_hbm, b2_v)] + cp_w2(0, 1))
    g7 = Group(cp_w2(1, NP))
    for c in (x0, g1, g2, g3, g4, g5, g6, g7):
        c.start()

    v_s[0] = jnp.zeros((D, LB), f32)
    for buf in (xnT_s, ra_s, lh_s, lk_s, rh_s, rs_s, rr_s, ola_s, olb_s, ll_s, lc_s):
        buf[0:8, 0:64] = jnp.zeros((8, 64), buf.dtype)

    wait("x0", x0)
    one_s[...] = lax.shift_right_logical(pltpu.bitcast(x_v[0, 0:16, 0:LB], i32), 1) | 1
    pos[:] = [one_s[...]]
    ln(0)
    ln(1)
    hpair(0)
    wait("r1", g1)
    jobs = u_early(0, 0, E1, [], 7 * E1 // 4 * 4, P["T1"], 100)
    wait("r2", g2)
    t, dt = P["L2T"], P["L2D"]
    add_tasks([(t + int((k + 1) * dt * P["LNV"]), ln, (2 + k, t + int(k * dt * P["LNV"]), dt)) for k in range(2)])
    jobs = u_early(0, E1, E2, jobs, P["N2"], P["T2"], 100)
    wait("wq", g3)
    add_tasks([(P["H2T"] + P["H2D"], hpair, (2, P["H2T"], P["H2D"]))])
    u_early(0, E2, NFP, jobs, 7 * NFP, P["T3"], 100)
    prep_wqkv("q", 0, HD // 16, [P[k] for k in ("QA", "QB", "QC", "QE")])
    stage_a(0, "q", split_last=True)
    m = stage_a(2, "q", AORD[:P["NA3"]])
    wait("wkv", g4)
    stage_a(2, "q", AORD[P["NA3"]:], split_last=True, m=m)
    prep_wqkv("kv", HD // 16, HA // 16, [P[k] for k in ("KA", "KB", "KC", "KE")])
    t = ln_tasks(4, now() + P["L4T"], P["LND"], P["HSD"])
    n4 = P["N4"]
    add_tasks([(t + (n + 1) * P["BD"], slot, (t + n * P["BD"], P["BD"])) for n in range(n4)])
    stage_a(0, "kv")
    stage_a(2, "kv", order=(6,) + AORD[:6])

    wait("mid", g5)
    AD = 7 * HA // 2
    t = P["L5T"]
    for b in range(6, NB, 2):
        t = ln_tasks(b, t, P["LND"], P["HSD"])
    for k in range(P["NH5"]):
        add_tasks([(t + P["HTD"], htriple, (k, t, P["HTD"]))])
        t += P["HTD"]
    n5 = P["N5"]
    bd = ((NP - 2) * AD - P["MARG"] - t) // n5
    add_tasks([(t + (n + 1) * bd, slot, (t + n * bd, bd)) for n in range(n5)])
    n5 += n4
    for n, b in enumerate(range(4, NB, 2)):
        stage_a(b, order=(6,) + AORD[:6] if n % 2 else AORD)

    wait("fin", g6)
    UM = (7 * NFP + 1) * HD // 4
    UD = 15 * NKT * HD // 4
    r6 = UM + (NNT - 1) * UD + 11 * NKT * HD // 4
    add_tasks([(i * P["TMD"] + P["TM0"], tsum, (1, i, 1, i, (i - 1) * P["TMD"] + P["TM0"], P["TMD"])) for i in range(NFP)])
    t, dt = P["HT6"], (UM - 100 - P["HT6"]) // max(NKT - P["NH5"], 1)
    add_tasks([(t + (k + 1) * dt, htriple, (P["NH5"] + k, t + k * dt, dt)) for k in range(NKT - P["NH5"])])
    for i in range(NNT):
        t0, t1 = (UM - P["US0"], UM + 1200) if i == 0 else (UM + (i - 1) * UD + (1300 if i == 1 else 400), UM + i * UD + 350)
        dt = (t1 - t0) // NKT
        add_tasks([(t0 + (k + 1) * dt, hsum, (k, i, t0 + k * dt, dt)) for k in range(NKT)])
    left = len(mains) - n5 - 2
    bd = (r6 - P["R6E"] - P["R6S"]) // left
    add_tasks([(P["R6S"] + (n + 1) * bd, slot, (P["R6S"] + n * bd, bd)) for n in range(left)])
    t = P["R6S"] + left * bd
    add_tasks([(t + (n + 1) * 300, slot, (t + n * 300, 300)) for n in range(2)])
    for qd, t0, t1 in ((NQ, UD, 2 * UD), (0, 2 * UD + P["LL0"], 3 * UD + P["LL0"]), (1, 3 * UD + P["LL0"], 4 * UD + P["LL0"]),
                       (2, 4 * UD + P["LL2"], 4 * UD + P["LL2"] + P["UEL"])):
        dt = (t1 - t0) // 7
        add_tasks([(UM + t0 + (g + 1) * dt, llsum, (qd, g, UM + t0 + g * dt, dt)) for g in range(7)])
    rr_tasks(BORD[0], 0, 0, P["RP0"], P["RP1"])
    add_tasks([(P["PW0"] + P["PWD"], prep_wo_a, (P["PW0"], P["PWD"]))])
    add_tasks([(P["PW1"] + (h + 1) * P["PWE"], prep_wo_b, (h, P["PW1"] + h * P["PWE"], P["PWE"])) for h in range(2)])
    for b in range(NB):
        b2f_s[b // 2, 0:1, _blk(b % 2)] = b2_v[b:b + 1, :].astype(f32)
    u_mid()
    for i in range(NNT):
        u_last(i, None if i == NNT - 1 else P["UEL"] if i == NNT - 2 else P["UED"])
    flush()
    assert slot_ctr[0] == len(mains) and all(("ll", qd, g) in ready for qd in range(NQ + 1) for g in range(7))
    assert all(("pr", j, hh) in ready for j in range(NB) for hh in range(2)) and ("rr", BORD[0]) in ready

    wait("w2", g7)
    lax.fori_loop(0, NP // 4, c_body, 0)
    outs = []
    for pa in range(0, NP, 2):
        outs += [out_copy(pa + n % 2, 0, 2, n // 2 * HD, (n // 2 + 1) * HD) for n in (1, 2, 3)]
        outs += [out_copy(pa, e0, e1, r0, r1) for (r0, r1, e0, e1) in (LAST_PARTS if pa % 4 else [(0, HD, 0, 2)])]
    wait("out", *outs)


@jax.jit
def pallas_parallel_sum__sliding_local_dilated__mixer_token_mlp__prompt_kernel(A_x, A_wqkv, A_wo, B_x, B_w1, B_b1, B_w2, B_b2):
    del B_x
    hbm = pl.BlockSpec(memory_space=pltpu.HBM)
    outT = pl.pallas_call(
        _kernel,
        out_shape=jax.ShapeDtypeStruct((1, D, S), bf16),
        in_specs=[hbm] * 7,
        out_specs=hbm,
        scratch_shapes=[
            pltpu.VMEM((NP, D, 2 * LB), bf16),
            pltpu.VMEM((NP, F, 2 * LB), bf16),
            pltpu.VMEM((NP, D, 2 * LB), bf16),
            pltpu.VMEM((NB + 1, D, LB), f32),
            pltpu.VMEM((NB, 2 * W * HH, LB), f32),
            pltpu.VMEM((NP, 32, 2 * LB), f32),
            pltpu.VMEM((D, 3 * D), bf16),
            pltpu.VMEM((D, D), bf16),
            pltpu.VMEM((S, F), bf16),
            pltpu.VMEM((NFB, LB), bf16),
            pltpu.VMEM((NB, LB), bf16),
            pltpu.VMEM((2, 3 * D + 64, LB), i32),
            pltpu.VMEM((7 * HA // 2, HD), u32),
            pltpu.VMEM((4, HD + 32, LB), i32),
            pltpu.VMEM((D, 2 * LB), i32),
            pltpu.VMEM((HD, S), u32),
            pltpu.VMEM((NP * QD, 5 * LB), u32),
            pltpu.VMEM((7 * QD, 2 * LB), u32),
            pltpu.VMEM((15 * QD, NKT * LB), u32),
            pltpu.VMEM((2 * RHK, 9 * LB), u32),
            pltpu.VMEM((D, F), f32),
            pltpu.VMEM((7 * HD, NFP * LB), f32),
            pltpu.VMEM((7 * QD, (NFP + 2) * LB), u32),
            pltpu.VMEM((NB, 2 * D, LB), f32),
            pltpu.VMEM((D, LB), f32),
            pltpu.VMEM((2 * RSK, 5 * LB), u32),
            pltpu.VMEM((49 * ED, 4 * LB), u32),
            pltpu.VMEM((7 * RRK, 9 * LB), u32),
            pltpu.VMEM((D, 4 * LB), f32),
            pltpu.VMEM((D, 4 * LB), f32),
            pltpu.VMEM((8, LB), i32),
            pltpu.SemaphoreType.DMA((9,)),
        ],
        compiler_params=pltpu.CompilerParams(vmem_limit_bytes=100 * 1024 * 1024,
                                             disable_bounds_checks=True,
                                             disable_semaphore_checks=True),
    )(jnp.swapaxes(A_x, 1, 2), A_wqkv, A_wo, B_w1, B_b1.reshape(NFB, LB), B_w2, B_b2.reshape(NB, LB))
    return jnp.swapaxes(outT, 1, 2)
```

```python
import jax
import jax.numpy as jnp
from jax import lax
import jax.experimental.pallas as pl
import jax.experimental.pallas.tpu as pltpu

S, D, F = 2048, 448, 1792
H, DH, W, DIL = 16, 28, 8, 2
LB = 128
NB = S // LB
NP = NB // 2
NFB = F // LB
NFP = NFB // 2
HH = H // 2
WH = W // 2
SH = DIL * WH
HD = D // 2
QD = D // 4
ED = D // 8
HA = 3 * HD
HB0 = 4
NKT = (NB - HB0) // 3
NNT = -(-NFB // 3)
RSK = NFP * LB // 2
RHK = NKT * LB // 2
NQ = NFP // 2
KL = NQ * LB + QD
RRK = 2 * LB
EPS = 1e-5
EPS_BF16 = 1.0013580322265625e-05
SCALE = DH ** -0.5
f32 = jnp.float32
bf16 = jnp.bfloat16
u32 = jnp.uint32
i32 = jnp.int32

SCOPES = False
P = dict(
    E1=3, E2=6, T3=-20, N2=16, NA3=2, T1=-200, T2=-200, L2T=100, L2D=440, H2T=900, H2D=340, L4T=920, L5T=0, W2X=500,
    QA=-330, QB=260, QC=-240, QE=420, KA=50, KB=230, KC=390, KE=450,
    LND=420, HSD=200, HTD=525, NH5=4, N4=2, N5=20, TM0=0, TMD=330, HT6=500, SGH=8, HL=260, LNA=0.28, LNB=0.46, LNBD=0.38, LNV=0.86,
    BD=375, MARG=300, LAG=200, LS=150, PP=130, PVL=500, PVPOS=18,
    US0=0, UE0=100, UED=3000, UEL=1600, UG=70, R6S=3150, R6E=1950,
    LL0=600, LLO=1300, LLD=4000, LL2=800, RP0=13000, RP1=15100, PW0=300, PWD=300, PW1=1300, PWE=300,
    RR0=-48, RR1=800, RRM=-20, RW=(8, 8, 8, 2, 7), BV0=117, BVS=717, BVD=620, EP0=0, EPD=864, EPL=290, SGR=8, SGT=8,
)
G = 4


def _as(x, dtype):
    return x if x.dtype == dtype else pltpu.bitcast(x, dtype)


def _pk(x):
    return pltpu.bitcast(x.astype(bf16), u32)


def _up(x):
    return pltpu.bitcast(x, bf16)


def _upf(x):
    return pltpu.bitcast(x, bf16).astype(f32)


def _rb(x):
    return x.astype(bf16).astype(f32)


def _word(lo, hi):
    lo, hi = [pltpu.bitcast(v.astype(f32), i32) for v in (lo, hi)]
    return lax.shift_right_logical(lo, 16) | hi


def _unword(w):
    return [pltpu.bitcast(w << 16, f32), pltpu.bitcast(w & -65536, f32)]


def _cat(xs, axis):
    return xs[0] if len(xs) == 1 else jnp.concatenate(xs, axis=axis)


def _x2(v):
    return jnp.concatenate([v, v], axis=0)


def _blk(b):
    return slice(b * LB, (b + 1) * LB)


def _rowsum8(a):
    return jnp.broadcast_to(jnp.sum(a, axis=0, keepdims=True), (8, a.shape[1]))


def _token(*deps):
    deps = [d for d in deps if d is not None]
    if not deps:
        return None
    if len(deps) == 1:
        return deps[0]
    bits = _as(deps[0], u32)
    for d in deps[1:]:
        bits = bits | _as(d, u32)
    return bits


def _lhs_ops(a11, a12, a21, a22):
    return [a11 + a22, a21 + a22, a11, a22, a11 + a12, a21 - a11, a12 - a22]


SIDX = {0: 0, 2: 1, 3: 2, 5: 3, 6: 4}
TOP = {0: ((0, 0), 1, (1, 1)), 1: ((0, 0),), 2: ((0, 1), -1, (1, 1)), 3: ((1, 0), -1, (0, 0)),
       4: ((1, 1),), 5: ((0, 0), 1, (0, 1)), 6: ((1, 0), 1, (1, 1))}


def _rhs_sums(b11, b12, b21, b22):
    return {0: b11 + b22, 2: b12 - b22, 3: b21 - b11, 5: b11 + b12, 6: b21 + b22}


def _rhs_op(p, blk):
    t = TOP[p]
    if len(t) == 1:
        return blk(*t[0])
    return blk(*t[0]) + blk(*t[2]) if t[1] > 0 else blk(*t[0]) - blk(*t[2])


def _combine(m, n=None):
    c12 = lambda: m[2] + m[4]
    c21 = lambda: m[1] + m[3]
    x = lambda: (m[2] - m[1]) + m[0]
    c = [lambda: (x() + m[6]) + (c21() - c12()), c12, c21, lambda: x() + m[5]]
    return [f() for f in c] if n is None else c[n]()


def _hk_lhs(a):
    s = [a[0][k] + a[1][k] for k in range(3)]
    return [a[0][0], s[0], s[1], a[1][1], a[0][0] + a[1][1], a[0][1] - a[0][0], a[1][0] - a[1][1], a[0][2],
            a[1][2], s[0] - a[1][2], s[2] - s[0], a[1][2] - a[1][0], s[1] - a[0][2], s[2] - s[1], a[0][2] - a[0][1]]


HKB = [((0, 0, 1), (1, 0, 1), (0, 2, -1)), ((0, 0, 1), (2, 0, 1), (0, 1, -1)), ((1, 1, 1), (2, 1, 1), (1, 0, -1)),
       ((1, 1, 1), (0, 1, 1), (1, 2, -1)), ((0, 1, 1), (1, 0, 1)), ((1, 0, 1),), ((0, 1, 1),),
       ((2, 2, 1), (1, 2, 1), (2, 0, -1)), ((2, 2, 1), (0, 2, 1), (2, 1, -1)), ((2, 0, 1), (0, 2, 1)), ((2, 0, 1),),
       ((0, 2, 1),), ((2, 1, 1), (1, 2, 1)), ((2, 1, 1),), ((1, 2, 1),)]


def _hk_terms(nj):
    out = {}
    for p, t in enumerate(HKB):
        t = [x for x in t if x[1] < nj]
        if t and (nj == 3 or p not in (7, 8)):
            out[p] = t
    return out


def _hk_combine(m, nj):
    x, y = (m[9] + m[11], m[12] + m[14]) if nj == 3 else (m[9], m[12])
    x0, y3 = x + m[0], y + m[3]
    c = [[(m[5] + m[10]) + x0, ((m[4] + m[5]) - y3) + m[2]], [((m[4] + m[6]) - x0) + m[1], (m[6] + m[13]) + y3]]
    if nj == 3:
        c[0].append(((m[10] - m[14]) + x) + m[7])
        c[1].append(((m[13] - m[11]) + y) + m[8])
    return c


def _kernel(x_hbm, wqkv_hbm, wo_hbm, w1_hbm, b1_hbm, w2_hbm, b2_hbm, out_hbm,
            x_v, w2_v, out_v, v_s, pr_s, b2f_s, wqkv_v, wo_v, w1_v, b1_v, b2_v, wt_s, lw_s, wo_s,
            wq_s, xnT_s, ra_s, lh_s, lk_s, rh_s, u0_s, um_s, lc_s, g_s, qk_s, op_s, rs_s, ll_s, rr_s, ola_s, olb_s, one_s, sems):
    sem_ctr = [1]

    class Group:
        def __init__(self, pairs):
            self.cps = [pltpu.make_async_copy(a, b, sems.at[sem_ctr[0]]) for (a, b) in pairs]
            sem_ctr[0] += 1

        def start(self):
            for c in self.cps:
                c.start()

        def wait(self):
            for c in self.cps:
                c.wait()

    def cp_x(p0, p1):
        return [(x_hbm.at[0, :, pl.ds(p * 2 * LB, 2 * LB)], x_v.at[p]) for p in range(p0, p1)]

    def cp_w2(p0, p1):
        return [(w2_hbm.at[:, pl.ds(p * 2 * LB, 2 * LB)], w2_v.at[p]) for p in range(p0, p1)]

    def cp_w1(b0, b1, i0=0, i1=NFP):
        sl = pl.ds(b0 * LB, (b1 - b0) * LB)
        cl = pl.ds(i0 * 2 * LB, (i1 - i0) * 2 * LB)
        return [(w1_hbm.at[sl, cl], w1_v.at[sl, cl])]

    tl = []
    mxu = [0, 0, 0, 0]
    nxt = [0]
    hist = []
    tasks = []
    dls = []
    ready = set()
    pos = []
    true = {}

    def tie(v, z):
        if z is None:
            return v
        def fit(a):
            a = _cat([a] * (v.shape[0] // 8), 0)
            return a if v.shape[1] == LB else a[:, 0:v.shape[1]]
        if v.shape not in true:
            true[v.shape] = fit(pos[0]) > 0
        return lax.select(true[v.shape], v, fit(_as(z, v.dtype)))

    def tie8(v, z):
        return v if z is None else jnp.concatenate([tie(v[0:8], z), v[8:16]], axis=0)

    def add_tasks(todo):
        tasks.extend(todo)
        tasks.sort(key=lambda x: x[0])

    def flush(t=None):
        while tasks and (t is None or tasks[0][0] < t):
            _, fn, args = tasks.pop(0)
            fn(*args)

    def reset():
        assert not tasks
        dls.clear()
        tl.clear()
        hist.clear()
        mxu[:] = [0, 0, 0, 0]
        nxt[0] = 0

    def now():
        return sum(mxu) // 4

    def wait(name, *cps):
        flush()
        if SCOPES:
            with jax.named_scope("wait_" + name):
                for c in cps:
                    c.wait()
        else:
            for c in cps:
                c.wait()
        reset()

    def mm1(lhs, rhs, pace=True):
        flush(now())
        start = mxu[nxt[0]]
        due = [v for (t, v) in dls if t <= start] if pace else []
        if due:
            dls[:] = [(t, v) for (t, v) in dls if t > start]
            tile = _up(tie(pltpu.bitcast(lhs[0:16, 0:LB], u32), _token(*due)))
            row = tile if lhs.shape[1] == LB else jnp.concatenate([tile, lhs[0:16, LB:]], axis=1)
            lhs = jnp.concatenate([row, lhs[16:]], axis=0)
        r = jnp.dot(lhs, rhs, preferred_element_type=f32)
        m, k = lhs.shape
        first_done = None
        for _ in range(-(-rhs.shape[1] // LB)):
            end = 0
            for _ in range(-(-k // LB)):
                mxu[nxt[0]] += m
                end = max(end, mxu[nxt[0]])
                nxt[0] = (nxt[0] + 1) % 4
            if first_done is None:
                first_done = end
        if pace:
            tl.append((first_done - m, first_done, r))
        return r

    def mm(lhs, rhs, init=None):
        k = lhs.shape[1]
        r, k0 = init, 0
        while k0 < k:
            k1 = min(k, k0 + (4 - nxt[0]) * LB)
            part = mm1(lhs[:, k0:k1], rhs[k0:k1], pace=k1 - k0 > LB)
            r = part if r is None else r + part
            k0 = k1
        return r

    def at(t, *more):
        best = None
        if t is not None and t >= 0:
            t = min(t, now() - 1)
            for (a, b, r) in tl:
                if a <= t and (best is None or min(b, t) > best[0]):
                    row = int(min((t - a) / (b - a), 0.999) * (r.shape[0] // 8)) * 8
                    best = (min(b, t), r, row)
        return _token(None if best is None else best[1][best[2]:best[2] + 8, 0:LB], *more)

    def strassen(lhs, rhs, order, split_last=False, init=None, m=None):
        m = [None] * 7 if m is None else m
        for p in order:
            flush(now())
            l, r = lhs(p), rhs(p)
            c0 = None if init is None else init[p]
            if split_last and p == order[-1]:
                kk = (-(-r.shape[0] // LB) - 2) * LB
                hm = l.shape[0] // 2
                hd = mm(l[:, :kk], r[:kk], c0) if kk else c0
                tail = jnp.concatenate([mm(l[:hm, kk:], r[kk:]), mm(l[hm:, kk:], r[kk:])], axis=0)
                m[p] = tail if hd is None else hd + tail
            else:
                m[p] = mm(l, r, c0)
        return m

    def wcol(hh, p):
        return p * D + (1 - hh if p == 1 else hh) * HD

    def wrows(hh, g, z=None):
        p, d = divmod(2 * g, DH)
        t = [jnp.concatenate([wt_s[c, pl.ds(wcol(hh, p) + d + e, HH, stride=DH), :]
                              for e in range(2)], axis=0) for c in range(2)]
        return _unword(jnp.concatenate([tie(t[0], z), tie(t[1][:, 0:HD - LB], z)], axis=1))

    wt_done = set()

    def prep_wqkv(part, ga, gb, paced):
        def need(hh, p, z):
            lo = wcol(hh, p)
            for ct in range(lo // LB, -(-(lo + HD) // LB)):
                if ct in wt_done:
                    continue
                wt_done.add(ct)
                cols = slice(ct * LB, min((ct + 1) * LB, 3 * D))
                wd = _word(wqkv_v[0:HD, cols], wqkv_v[HD:D, cols])
                wd = jnp.concatenate([tie(wd[r:r + 8], z if r % LB == 0 else None) for r in range(0, HD, 8)], axis=0)
                wT = wd.T
                wt_s[0, cols, :] = wT[:, 0:LB]
                wt_s[1, cols, 0:HD - LB] = wT[:, LB:HD]

        def put(p, g, v):
            lw_s[p * (HA // 2) + g * 8:p * (HA // 2) + g * 8 + 8, :] = _pk(v)

        def half(hh, g0, g1, t0=None, dur=None):
            pr, ps = ((2, 4), (3, 1))[hh]
            for g in range(g0, g1):
                t = None if t0 is None else t0 + (g - g0) * dur // (g1 - g0)
                need(hh, 2 * g // DH, at(None if t is None else t - P["W2X"]))
                a1, a2 = wrows(hh, g, at(t))
                put(pr, g, a2 if hh else a1)
                put(ps, g, a1 + a2)
            if g1 == gb:
                ready.update({("lw", part, pr), ("lw", part, ps)})

        def rest(g0, g1, t0, dur):
            assert ("lw", part, 1) in ready
            for g in range(g0, g1):
                z = at(t0 + (g - g0) * dur // (g1 - g0))
                ops = _lhs_ops(*wrows(0, g, z), *wrows(1, g, z))
                for p in (0, 5, 6):
                    put(p, g, ops[p])
            if g1 == gb:
                ready.update({("lw", part, 0), ("lw", part, 5), ("lw", part, 6)})
        t2, d2, t3, d3 = paced
        half(0, ga, gb)
        n = (gb - ga) // 14
        add_tasks([(now() + t2 + (k + 1) * d2 // n, half,
                    (1, ga + 14 * k, ga + 14 * k + 14, now() + t2 + k * d2 // n, d2 // n)) for k in range(n)])
        n = (gb - ga) // 7
        add_tasks([(now() + t3 + (k + 1) * d3 // n, rest,
                    (ga + 7 * k, ga + 7 * k + 7, now() + t3 + k * d3 // n, d3 // n)) for k in range(n)])

    def prep_wo_a(t0, dur):
        for g in range(HD // 16):
            w = _word(wo_v[g * 16:g * 16 + 16, :], wo_v[HD + g * 16:HD + g * 16 + 16, :])
            z = at(t0 + g * dur // (HD // 16))
            for c in range(4):
                cw = min(LB, D - c * LB)
                wo_s[c, g * 16:g * 16 + 16, 0:cw] = tie(w[:, c * LB:c * LB + cw], z)
        ready.add("wo")

    def prep_wo_b(h, t_dl):
        assert "wo" in ready
        outs = []
        for c in range(4):
            cw = min(LB, D - c * LB)
            rows = [wo_s[c, pl.ds(d, HH, stride=DH), :][:, 0:cw] for d in range(h * DH // 2, (h + 1) * DH // 2)]
            rows.append(jnp.zeros((LB - QD, cw), i32))
            wT = jnp.concatenate(rows, axis=0).T
            wq_s[c * LB:c * LB + cw, _blk(h)] = wT
            outs += [wT[r:r + 8] for r in range(0, cw, 8)]
        ready.add(("wq", h))
        dls.append((t_dl, _token(*outs)))

    RG = 16
    NG = D // RG
    stat2 = {}

    def ln(b, t0=None, dur=None):
        def xg(g):
            return x_v[b // 2, g * RG:(g + 1) * RG, _blk(b % 2)].astype(f32)

        def step(v, g, fr, s, q):
            if t0 is None or g % 4:
                return v
            acc = [] if s is None else [s[0:8], s[8:16], q[0:8], q[8:16]]
            return tie(v, at(t0 + fr * dur, *acc))

        x0 = jnp.broadcast_to(xg(0)[0:1], (8, LB))
        s = q = None
        for g in range(NG):
            x0 = step(x0, g, P["LNA"] * g / NG, s, q)
            c = xg(g) - _x2(x0)
            s = c if s is None else s + c
            q = c * c if q is None else q + c * c
        dm = _rowsum8(s) * (1.0 / D)
        mu = _rb(x0 + dm)
        var = _rb(jnp.maximum(_rowsum8(q) * (1.0 / D) - dm * dm, 0.0))
        r1 = 1.0 / _rb(jnp.sqrt(_rb(var + EPS_BF16)))
        s = q = None
        for g in range(NG):
            mu = step(mu, g, P["LNB"] + P["LNBD"] * g / NG, s, q)
            xn = _rb(xg(g) - _x2(mu)) * _x2(r1)
            xnT_s[g * 8:g * 8 + 8, _blk(b)] = _pk(xn)
            s = xn if s is None else s + xn
            q = xn * xn if q is None else q + xn * xn
        mu2 = _rowsum8(s) * (1.0 / D)
        var2 = jnp.maximum(_rowsum8(q) * (1.0 / D) - mu2 * mu2, 0.0)
        stat2[b] = (mu2, 0.5 * lax.rsqrt(var2 + EPS))

    def hpair(b, t0=None, dur=None):
        ng = HD // RG
        st = [stat2[b], stat2[b + 1]]
        for g in range(ng):
            if b < HB0:
                zz = [at(None if t0 is None else t0 + (4 * g + k) * dur // (4 * ng)) for k in range(4)]
            else:
                zz = [at(t0 + g * dur // ng), None, None, at(t0 + g * dur // ng + P["SGT"])]
            xq = [_upf(tie(xnT_s[r:r + 8, _blk(b + e)], zz[2 * (r >= QD) + e]))
                  for r in (g * 8, QD + g * 8) for e in range(2)]
            ro = (b // 2) * QD + g * 8
            for p, v in _rhs_sums(*xq).items():
                ra_s[ro:ro + 8, _blk(SIDX[p])] = _pk(v)
            if b < HB0:
                hq = [(v - _x2(st[n % 2][0])) * _x2(st[n % 2][1]) for n, v in enumerate(xq)]
                for p, v in enumerate(_lhs_ops(*hq)):
                    lh_s[p * QD + g * 8:p * QD + g * 8 + 8, _blk(b // 2)] = _pk(v)
        ready.add(("xn", b))
        if b >= 6:
            got = ra_s[(b // 2) * QD:(b // 2 + 1) * QD, :]
            dls.append((t0 + dur + P["HL"], _token(*[got[r:r + 8, _blk(c)] for r in range(0, QD, 8) for c in range(5)])))

    def htile(b, r, z=None):
        return (_upf(tie(xnT_s[r:r + 8, _blk(b)], z)) - _x2(stat2[b][0])) * _x2(stat2[b][1])

    def htriple(t, t0, dur):
        ng = HD // RG
        for g in range(ng):
            zz = [at(t0 + (3 * g + k) * dur // (3 * ng)) for k in range(3)]
            a = [[htile(HB0 + 3 * t + k, h * QD + g * 8, zz[k]) for k in range(3)] for h in range(2)]
            for p, v in enumerate(_hk_lhs(a)):
                lk_s[p * QD + g * 8:p * QD + g * 8 + 8, _blk(t)] = _pk(v)
        ready.add(("lh", t))

    def ln_tasks(b, t, lnd, hsd):
        for fn, bb, dur, adv in ((ln, b, lnd, P["LNV"]), (ln, b + 1, lnd, P["LNV"]), (hpair, b, hsd, 1.0)):
            add_tasks([(t + int(dur * adv), fn, (bb, t, dur))])
            t += int(dur * adv)
        return t

    def tsum(kp, i, slot_, n, t0, dur):
        for g in range(LB // 16):
            z, z2 = at(t0 + g * dur // 8), at(t0 + g * dur // 8 + P["SGT"])
            t1, t2 = [w1_v[(2 * kp + e) * LB + g * 16:(2 * kp + e) * LB + g * 16 + 16,
                           2 * i * LB:(2 * i + 2) * LB].astype(f32) for e in range(2)]
            ro = slot_ * RSK + n * (LB // 2) + g * 8
            for p, v in _rhs_sums(tie8(t1[:, :LB], z), t1[:, LB:], t2[:, :LB], tie8(t2[:, LB:], z2)).items():
                rs_s[ro:ro + 8, _blk(SIDX[p])] = _pk(v)
        ready.add(("rs", kp, i))

    def u_rhs(p, i, kps, slot_, n0):
        if p in SIDX:
            assert all(("rs", kp, i) in ready for kp in kps)
            ro = slot_ * RSK + n0 * (LB // 2)
            return _up(rs_s[ro:ro + len(kps) * (LB // 2), _blk(SIDX[p])])
        e = 0 if p == 1 else 1
        return _cat([w1_v[_blk(2 * kp + e), _blk(2 * i + e)] for kp in kps], 0)

    LATE = (NFP - 1, 6)

    def ujob(kp, i, p, split):
        flush(now())
        assert ("xn", 2 * kp) in ready
        l, r = _up(lh_s[p * QD:(p + 1) * QD, _blk(kp)]), u_rhs(p, i, [kp], kp, i)
        v = jnp.concatenate([mm1(l[:QD], r), mm1(l[QD:], r)], axis=0) if split else mm1(l, r)
        rows = slice(p * HD, (p + 1) * HD)
        um_s[rows, _blk(i)] = v

    def u_early(kp, i0, i1, carry, n, t0, dt, nsplit=0):
        for k, i in enumerate(range(i0, i1)):
            add_tasks([(t0 + (k + 1) * dt, tsum, (kp, i, kp, i, t0 + k * dt, dt))])
        jobs = (carry + [(kp, i, p) for i in range(i0, i1) for p in (1, 4)]
                + [(kp, i, p) for i in range(i0, i1) for p in SIDX if (i, p) != LATE])
        for c, job in enumerate(jobs[:n]):
            ujob(*job, c >= n - nsplit)
        return jobs[n:]

    def u_mid():
        jobs = [(i, p) for i in range(2) for p in (4, 1)]
        for i in range(NFP):
            jobs += [(i, p) for p in (2, 3, 0, 5, 6)] + [(i + 2, p) for p in (4, 1) if i + 2 < NFP]
        m = [[None] * 7 for _ in range(NFP)]
        for i, p in jobs:
            flush(now())
            late = (i, p) == LATE
            l = _up(lh_s[p * QD:(p + 1) * QD, (0 if late else LB):])
            r = _cat([u_rhs(p, i, [0], 0, i)] * late + [u_rhs(p, i, [1], 1, i)], 0)
            v = jnp.concatenate([mm1(l[:QD], r), mm1(l[QD:], r)], axis=0) if late else mm1(l, r)
            if not late:
                v = v + um_s[p * HD:(p + 1) * HD, _blk(i)]
            if p in (2, 3):
                v = v + 0.5 * b1_v[2 * i + 3 - p:2 * i + 4 - p, :].astype(f32)
            m[i][p] = v
            if p == 6:
                for n, c in enumerate(_combine(m[i])):
                    u0_s[n // 2 * HD:(n // 2 + 1) * HD, _blk(2 * i + n % 2)] = c

    def nj_of(i):
        return min(3, NFB - 3 * i)

    def hsum(t, i, t0, dur):
        nj = nj_of(i)
        sums = [(p, tm) for p, tm in _hk_terms(nj).items() if len(tm) > 1]
        tied = {(1, 0): 0, (2, 0): 1, (1, 2): 2, (2, 2): 3} if nj == 3 else {(1, 0): 0, (0, 1): 2}
        for g in range(LB // 16):
            b = {}
            for k in range(3):
                r = (HB0 + 3 * t + k) * LB + g * 16
                w = w1_v[r:r + 16, 3 * i * LB:(3 * i + nj) * LB].astype(f32)
                for j in range(nj):
                    z = at(t0 + g * dur // 8 + tied[k, j] * P["SGH"]) if (k, j) in tied else None
                    b[k, j] = tie8(w[:, _blk(j)], z)
            ro = (i % 2) * RHK + t * (LB // 2) + g * 8
            for n, (p, tm) in enumerate(sums):
                v = b[tm[0][:2]]
                for (k, j, sg) in tm[1:]:
                    v = v + b[k, j] if sg > 0 else v - b[k, j]
                rh_s[ro:ro + 8, _blk(n)] = _pk(v)
        ready.add(("rh", t, i))

    def gelu_half(hx, z):
        c = 0.7978845608028654
        return hx + hx * jnp.tanh(tie(hx * (2.0 * c + (8.0 * c * 0.044715) * (hx * hx)), z))

    def u_epilogue(i, m, gs, t0, dur):
        nj = nj_of(i)
        for n, g in enumerate(gs):
            c = _hk_combine({p: v[g * 16:g * 16 + 16] for p, v in m.items()}, nj)
            for j in range(nj):
                f = 3 * i + j
                t = None if t0 is None else t0 + (n * nj + j) * dur // (len(gs) * nj) - P["UG"]
                gl = [gelu_half(c[h][j] + u0_s[h * HD + g * 16:h * HD + g * 16 + 16, _blk(f)], at(t))
                      for h in range(2)]
                if f < 4 * NQ:
                    for h in range(2):
                        g_s[h * HD + g * 16:h * HD + g * 16 + 16, _blk(f)] = gl[h]
                    ready.add(("g", f, g))
                elif j == 0:
                    g0 = gl
                else:
                    for p, v in enumerate(_lhs_ops(g0[0], gl[0], g0[1], gl[1])):
                        lc_s[p * QD + g * 8:p * QD + g * 8 + 8, :] = _pk(v)

    def u_last(i, edur):
        terms = _hk_terms(nj_of(i))
        sums = [p for p, tm in terms.items() if len(tm) > 1]
        m = {}
        order = ((10, 11, 14, 5, 13, 6, 9, 7, 0, 12, 8, 3, 4, 1, 2) if i == 0
                 else (10, 11, 9, 14, 7, 5, 0, 13, 12, 8, 6, 3, 4, 1, 2))
        for p in [p for p in order if p in terms]:
            flush(now())
            assert all(("lh", t) in ready for t in range(NKT))
            if p in sums:
                assert all(("rh", t, i) in ready for t in range(NKT))
                r = _up(rh_s[(i % 2) * RHK:(i % 2 + 1) * RHK, _blk(sums.index(p))])
            else:
                k, j, _ = terms[p][0]
                r = _cat([w1_v[_blk(HB0 + 3 * t + k), _blk(3 * i + j)] for t in range(NKT)], 0)
            m[p] = mm(_up(lk_s[p * QD:(p + 1) * QD, :]), r)
        if edur is None:
            u_epilogue(i, m, list(range(HD // 16)), None, None)
        else:
            t = now() + P["UE0"]
            add_tasks([(t + (g + 1) * edur // 7, u_epilogue, (i, m, [g, g + 7], t + g * edur // 7, edur // 7))
                       for g in range(7)])

    LTOP = [((0, 0), 1, (1, 1)), ((1, 0), 1, (1, 1)), ((0, 0),), ((1, 1),), ((0, 0), 1, (0, 1)),
            ((1, 0), -1, (0, 0)), ((0, 1), -1, (1, 1))]

    def llsum(qd, g, t0, dur):
        def tile(a, x, h, e):
            r = a * HD + h * QD + g * 16
            if qd < NQ:
                assert ("g", 4 * qd + 2 * e + x, g + 7 * h) in ready
                return g_s[r:r + 16, _blk(4 * qd + 2 * e + x)]
            assert ("wq", e) in ready
            return _unword(wq_s[r:r + 16, _blk(e)])[x]
        for p, t in enumerate(LTOP):
            zz = [at(t0 + p * dur // 7), at(t0 + p * dur // 7 + P["SGT"])]
            a = []
            for h in range(2):
                for e in range(2):
                    v = tile(*t[0], h, e)
                    if len(t) > 1:
                        v = v + tile(*t[2], h, e) if t[1] > 0 else v - tile(*t[2], h, e)
                    a.append(tie8(v, zz[h] if h == e else None))
            for q, v in enumerate(_lhs_ops(*a)):
                r = (p * 7 + q) * ED + g * 8
                ll_s[r:r + 8, _blk(qd)] = _pk(v)
        ready.add(("ll", qd, g))

    AORD = (4, 2, 1, 3, 0, 5, 6)

    def stage_a(b, parts="qkv", order=AORD, split_last=False, m=None):
        r0, r1 = {"q": (0, HD), "kv": (HD, HA), "qkv": (0, HA)}[parts]

        def lhs(p):
            assert all(("lw", pt, p) in ready for pt in ("q", "kv") if pt in parts)
            return _up(lw_s[(p * HA + r0) // 2:(p * HA + r1) // 2, :])

        def rhs(p):
            assert ("xn", b) in ready
            if p in SIDX:
                return _up(ra_s[(b // 2) * QD:(b // 2 + 1) * QD, _blk(SIDX[p])])
            return _up(xnT_s[0:QD, _blk(b)] if p == 1 else xnT_s[QD:HD, _blk(b + 1)])
        m = strassen(lhs, rhs, order, split_last, m=m)
        for n, ps in enumerate((range(7), (2, 4), (1, 3), (0, 1, 2, 5))):
            if all(m[p] is not None for p in ps) and any(p in order for p in ps):
                hh, e = divmod(n, 2)
                c = _combine(m, n)
                qk_s[b + e, hh * D + r0:hh * D + min(r1, D), :] = c[0:min(r1, D) - r0]
                if r1 > D:
                    v_s[b + e + 1, hh * HD:(hh + 1) * HD, :] = c[D - r0:]
        if all(v is not None for v in m):
            ready.update({(pt, b + e) for pt in ("q", "kv") if pt in parts for e in range(2)})
        return m

    lane0 = lax.broadcasted_iota(i32, (HH, LB), 1)
    zeros8 = jnp.zeros((HH, LB), f32)

    def mk_shift(z):
        lane = tie(lane0, z)
        masks = {}

        def pick(n, a, b):
            if n not in masks:
                masks[n] = lane < n
            return lax.select(masks[n], a, b)

        def fwd(cur, prev, sh):
            return cur if sh == 0 else pltpu.roll(pick(LB - sh, cur, prev), sh, 1)

        def bwd(cur, nxt_):
            return pltpu.roll(pick(SH, nxt_, cur), LB - SH, 1)
        return fwd, bwd

    def grp_shift(t, bd):
        lag = max(2, -(-P["LAG"] * DH // (G * bd)))
        return mk_shift(at(t, *(hist[-lag] if len(hist) >= lag else [])))

    raw, probs = {}, {}

    def attn_qk(j, hh, t, bd):
        jn = min(j + 1, NB - 1)
        assert ("q", jn) in ready and ("kv", j) in ready
        acc = [None] * WH
        accp = [None] * WH
        for d in range(DH):
            if d % G == 0:
                if d > 0:
                    hist.append(acc + accp)
                fwd, bwd = grp_shift(t + d * bd // DH, bd)
            r = hh * D + d * HH
            q = qk_s[j, r:r + HH, :]
            qp = bwd(q, qk_s[jn, r:r + HH, :])
            rk = (1 - hh) * D + HD + d * HH
            k = qk_s[j, rk:rk + HH, :]
            kp = qk_s[j - 1, rk:rk + HH, :] if j > 0 else zeros8
            for a in range(WH):
                ks = fwd(k, kp, DIL * a)
                t0, t1 = q * ks, qp * ks
                acc[a] = t0 if d == 0 else acc[a] + t0
                accp[a] = t1 if d == 0 else accp[a] + t1
        hist.append(acc + accp)
        raw[j, hh] = (acc, accp)

    def attn_sm(j, hh, t):
        fwd, _ = mk_shift(at(t))
        acc, accp = raw[j, hh]
        prev = raw.pop((j - 1, hh))[1] if j > 0 else [zeros8] * WH
        lg = acc + [fwd(accp[a], prev[a], SH) for a in range(WH)]
        lg = [a * SCALE for a in lg]
        if j == 0:
            lg = [lg[0]] + [jnp.where(lane0 >= DIL * w, lg[w], -1e9) for w in range(1, W)]
        m = lg[0]
        for w in range(1, W):
            m = jnp.maximum(m, lg[w])
        e = [jnp.exp(l - m) for l in lg]
        den = e[0]
        for w in range(1, W):
            den = den + e[w]
        inv = 1.0 / den
        p = [x * inv for x in e]
        for a in range(WH):
            pr_s[j, (hh * W + a) * HH:(hh * W + a + 1) * HH, :] = p[a]
        probs[j, hh] = p[WH:]

    def attn_pp(j, hh, t):
        _, bwd = mk_shift(at(t))
        p = probs.pop((j, hh))
        pn = probs[j + 1, hh] if j + 1 < NB else p
        for a in range(WH):
            pr_s[j, (hh * W + WH + a) * HH:(hh * W + WH + a + 1) * HH, :] = bwd(p[a], pn[a])
        ready.add(("pr", j, hh))

    def attn_pv(j, hh, dst, e, t, bd):
        assert not isinstance(j, int) or ("pr", j, hh) in ready
        assert e == 0 or ("o", dst, hh, e - 1) in ready
        pa = [pr_s[j, (hh * W + a) * HH:(hh * W + a + 1) * HH, :] for a in range(W)]
        p, pp = pa[:WH], pa[WH:]
        outs = []
        for d in range(DH):
            if d % G == 0:
                if d > 0:
                    hist.append([])
                fwd, _ = grp_shift(t + d * bd // DH, bd)
            r = hh * HD + d * HH
            v = v_s[j + 1, r:r + HH, :]
            vp = v_s[j, r:r + HH, :]
            o = op = None
            for a in range(WH):
                vs = fwd(v, vp, DIL * a)
                o = p[a] * vs if a == 0 else o + p[a] * vs
                op = pp[a] * vs if a == 0 else op + pp[a] * vs
            opp = zeros8 if (isinstance(j, int) and j == 0) else op_s[r:r + HH, :]
            op_s[r:r + HH, :] = op
            outs.append(o + fwd(op, opp, SH))
            ol[dst][r:r + HH, _blk(e)] = outs[-1]
        hist.append([])
        ready.add(("o", dst, hh, e))
        dls.append((t + bd + P["PVL"], _token(*outs)))

    ol = [ola_s, olb_s]
    mains = [("qk", j, hh) for j in range(NB) for hh in range(2)]
    mains = (mains[:P["PVPOS"]] + [("pv", j, hh) for j in range(4) for hh in range(2)]
             + mains[P["PVPOS"]:] + [None, None])
    slot_ctr = [0]

    def slot(t, bd):
        n = slot_ctr[0]
        slot_ctr[0] += 1
        it = mains[n]
        if it is None:
            pass
        elif it[0] == "qk":
            attn_qk(it[1], it[2], t, bd)
        else:
            attn_pv(it[1], it[2], 0, it[1], t, bd)
        if n >= 1 and mains[n - 1] is not None and mains[n - 1][0] == "qk":
            attn_sm(mains[n - 1][1], mains[n - 1][2], t + P["LS"])
        if n >= 2 and mains[n - 2] is not None and mains[n - 2][0] == "qk":
            _, j, hh = mains[n - 2]
            if j > 0:
                attn_pp(j - 1, hh, t + P["PP"])
            if j == NB - 1:
                attn_pp(j, hh, t + P["PP"])

    NRG = 8 * (NQ + 1) + 7
    PD = 8 * QD
    BORD = (1, 3, 2, 4, 0, 5, 6)
    LORD = (2, 4, 1, 3, 0, 5, 6)
    LAST_PARTS = [(0, QD, 1, 2), (QD, HD, 0, 2), (0, QD, 0, 1)]

    def rr_prep(p, pa, src, n0, n1, t0, dur):
        assert ("rr", p) not in ready
        for n in range(n0, n1):
            z = at(t0 + (n - n0) * dur // (n1 - n0))
            z2 = at(t0 + (n - n0) * dur // (n1 - n0) + P["SGR"])
            qd, g = divmod(n, 8)

            def wrow(i):
                return _rhs_op(p, lambda x, y: w2_v[pa + y, (2 * i + x) * LB + g * 16:(2 * i + x) * LB + g * 16 + 16, :]
                               .astype(f32))

            def orow(h):
                def blk(x, y):
                    assert ("o", src, x, 2 * y + 1) in ready
                    r = x * HD + h * QD + g * 16
                    return ol[src][r:r + 16, y * 2 * LB:(y + 1) * 2 * LB]
                return _rhs_op(p, blk)
            ro = p * RRK + g * 8
            if qd == NQ:
                if p in SIDX:
                    r = wrow(2 * NQ)
                    for e in range(2):
                        rr_s[ro:ro + 8, _blk(7 + e)] = _pk(tie8(r[:, _blk(e)], z))
                continue
            r1, r2 = (wrow(2 * qd), wrow(2 * qd + 1)) if qd < NQ else (orow(0), orow(1))
            ro += min(qd, NQ) * (LB // 2)
            c11, c22 = tie8(r1[:, :LB], z), tie8(r2[:, LB:], z2)
            sm = _rhs_sums(c11, r1[:, LB:], r2[:, :LB], c22)
            if p in SIDX or qd > NQ:
                sm.update({1: c11, 4: c22})
            for q, v in sm.items():
                rr_s[ro:ro + 8, _blk(q)] = _pk(v)
        if n1 == NRG:
            ready.add(("rr", p))

    def rr_tasks(p, pa, src, t0, t1):
        cuts = list(range(0, NRG, 8)) + [NRG]
        acc, tot = 0, sum(P["RW"])
        for a, b, w in zip(cuts[:-1], cuts[1:], P["RW"]):
            ta, tb = t0 + acc * (t1 - t0) // tot, t0 + (acc + w) * (t1 - t0) // tot
            add_tasks([(tb, rr_prep, (p, pa, src, a, b, ta, tb - ta))])
            acc += w

    def out_copy(pidx, e0, e1, r0, r1):
        off = pidx * (2 * LB) + e0 * LB
        if not isinstance(pidx, int):
            off = pl.multiple_of(off, LB)
        rs = pl.ds(r0, r1 - r0)
        return pltpu.make_async_copy(out_v.at[pidx, rs, pl.ds(e0 * LB, (e1 - e0) * LB)],
                                     out_hbm.at[0, rs, pl.ds(off, (e1 - e0) * LB)], sems.at[0])

    def b_out(pa, n, m, part, t0=None, dur=None):
        a, y = divmod(n, 2)
        r0, r1, e0, e1 = part
        cols = slice(e0 * LB, e1 * LB)
        for r in range(r0, r1, 16):
            c = _combine([None if v is None else v[r:r + 16, cols] for v in m], n)
            rows = slice(a * HD + r, a * HD + r + 16)
            o = c + x_v[pa + y, rows, cols].astype(f32)
            if t0 is not None:
                o = jnp.concatenate([tie(o[:, 0:LB], at(t0 + (r - r0) * dur // (r1 - r0))), o[:, LB:]], axis=1)
            out_v[pa + y, rows, cols] = o.astype(bf16)
        out_copy(pa + y, e0, e1, a * HD + r0, a * HD + r1).start()

    def big_piece(pa, pan, cur, last):
        t0 = now()
        for n in range(7):
            ta, tb = t0 + n * PD + P["RR0"], t0 + n * PD + P["RR1"]
            if n < 6:
                rr_tasks(BORD[n + 1], pa, cur, ta, tb)
            else:
                rr_tasks(BORD[0], pan, 1 - cur, ta, tb - (P["RRM"] if last else 0))
        ready.difference_update({("o", 1 - cur, hh, e) for hh in range(2) for e in range(4)})
        for n in range(8):
            e, hh = divmod(n, 2)
            t = t0 + P["BV0"] + n * P["BVS"]
            add_tasks([(t + P["BVD"], attn_pv, (pan * 2 + e, hh, 1 - cur, e, t, P["BVD"]))])
        m = [None] * 7
        for p in BORD:
            flush(now())
            assert ("rr", p) in ready
            x, y = TOP[p][0]

            def lhs(q):
                return _up(ll_s[(p * 7 + q) * ED:(p * 7 + q + 1) * ED, 0:KL])

            def rhs(q):
                if p in SIDX or q in SIDX:
                    return _up(rr_s[p * RRK:p * RRK + KL // 2, _blk(q)])
                h = 0 if q == 1 else 1
                return _cat([w2_v[pa + y, _blk(2 * (2 * qd + h) + x), _blk(h)] for qd in range(NQ)]
                            + [_up(rr_s[p * RRK + NQ * LB // 2:p * RRK + KL // 2, _blk(q)])], 0)
            rl = (_up(rr_s[p * RRK:p * RRK + LB // 2, 7 * LB:9 * LB]) if p in SIDX
                  else w2_v[pa + y, _blk(4 * NQ + x), :])
            ll = _up(lc_s[p * QD:(p + 1) * QD, :])
            ex = [mm1(ll[:QD], rl), mm1(ll[QD:], rl)]
            e12, e21 = ex[0][:, LB:], ex[1][:, :LB]
            e11 = (ex[0][:, :LB] + e12) - e21
            lf = strassen(lhs, rhs, LORD)
            ready.discard(("rr", p))
            if p in (2, 3):
                for q in (2, 3):
                    lf[q] = lf[q] + b2f_s[pa + 3 - p, 0:1, _blk(3 - q)]
            c12 = (lf[2] + e12) + lf[4]
            c21 = (lf[1] + e21) + lf[3]
            xx = (lf[2] - lf[1]) + lf[0]
            c22 = (xx + ex[1][:, LB:]) + lf[5]
            c11 = ((xx + e11) + (c21 - c12)) + lf[6]
            m[p] = jnp.concatenate([jnp.concatenate([c11, c12], axis=1),
                                    jnp.concatenate([c21, c22], axis=1)], axis=0)
            n = {3: 2, 4: 1, 5: 3, 6: 0}.get(p)
            if n is not None and not (last and n == 0):
                t, epd = now() + P["EP0"], P["EPL"] if (last and n == 3) else P["EPD"]
                add_tasks([(t + epd, b_out, (pa, n, list(m), (0, HD, 0, 2), t, epd))])
        if last:
            flush()
            for part in LAST_PARTS:
                b_out(pa, 0, m, part)

    def c_body(it, carry):
        reset()
        pos[:] = [one_s[...]]
        true.clear()
        ready.update({("rr", BORD[0])} | {("o", 0, hh, e) for hh in range(2) for e in range(4)})
        big_piece(4 * it, 4 * it + 2, 0, False)
        big_piece(4 * it + 2, lax.rem(4 * it + 4, NP), 1, True)
        assert ("rr", BORD[0]) in ready and all(("o", 0, hh, 3) in ready for hh in range(2))
        return carry

    E1, E2 = P["E1"], P["E2"]
    x0 = Group(cp_x(0, 1))
    g1 = Group(cp_w1(0, 2, 0, E1))
    g2 = Group(cp_w1(0, 2, E1, E2) + cp_x(1, 2))
    wq, wkv = [[(wqkv_hbm.at[:, cl], wqkv_v.at[:, cl])] for cl in (pl.ds(0, 4 * LB), pl.ds(4 * LB, 3 * D - 4 * LB))]
    g3 = Group((cp_w1(0, 2, E2, NFP) if E2 < NFP else []) + wq)
    g4 = Group(wkv + cp_x(2, 3))
    g5 = Group(cp_x(3, NP))
    g6 = Group(cp_w1(2, NB) + [(wo_hbm, wo_v), (b1_hbm, b1_v), (b2_hbm, b2_v)] + cp_w2(0, 1))
    g7 = Group(cp_w2(1, NP))
    for c in (x0, g1, g2, g3, g4, g5, g6, g7):
        c.start()

    v_s[0] = jnp.zeros((D, LB), f32)
    for buf in (xnT_s, ra_s, lh_s, lk_s, rh_s, rs_s, rr_s, ola_s, olb_s, ll_s, lc_s, g_s, wq_s):
        buf[0:8, 0:64] = jnp.zeros((8, 64), buf.dtype)

    wait("x0", x0)
    one_s[...] = lax.shift_right_logical(pltpu.bitcast(x_v[0, 0:16, 0:LB], i32), 1) | 1
    pos[:] = [one_s[...]]
    ln(0)
    ln(1)
    hpair(0)
    wait("r1", g1)
    jobs = u_early(0, 0, E1, [], 7 * E1 // 4 * 4, P["T1"], 100)
    wait("r2", g2)
    t, dt = P["L2T"], P["L2D"]
    add_tasks([(t + int((k + 1) * dt * P["LNV"]), ln, (2 + k, t + int(k * dt * P["LNV"]), dt)) for k in range(2)])
    jobs = u_early(0, E1, E2, jobs, P["N2"], P["T2"], 100)
    wait("wq", g3)
    add_tasks([(P["H2T"] + P["H2D"], hpair, (2, P["H2T"], P["H2D"]))])
    u_early(0, E2, NFP, jobs, 7 * NFP, P["T3"], 100)
    prep_wqkv("q", 0, HD // 16, [P[k] for k in ("QA", "QB", "QC", "QE")])
    stage_a(0, "q", split_last=True)
    m = stage_a(2, "q", AORD[:P["NA3"]])
    wait("wkv", g4)
    stage_a(2, "q", AORD[P["NA3"]:], split_last=True, m=m)
    prep_wqkv("kv", HD // 16, HA // 16, [P[k] for k in ("KA", "KB", "KC", "KE")])
    t = ln_tasks(4, now() + P["L4T"], P["LND"], P["HSD"])
    n4 = P["N4"]
    add_tasks([(t + (n + 1) * P["BD"], slot, (t + n * P["BD"], P["BD"])) for n in range(n4)])
    stage_a(0, "kv")
    stage_a(2, "kv", order=(6,) + AORD[:6])

    wait("mid", g5)
    AD = 7 * HA // 2
    t = P["L5T"]
    for b in range(6, NB, 2):
        t = ln_tasks(b, t, P["LND"], P["HSD"])
    for k in range(P["NH5"]):
        add_tasks([(t + P["HTD"], htriple, (k, t, P["HTD"]))])
        t += P["HTD"]
    n5 = P["N5"]
    bd = ((NP - 2) * AD - P["MARG"] - t) // n5
    add_tasks([(t + (n + 1) * bd, slot, (t + n * bd, bd)) for n in range(n5)])
    n5 += n4
    for n, b in enumerate(range(4, NB, 2)):
        stage_a(b, order=(6,) + AORD[:6] if n % 2 else AORD)

    wait("fin", g6)
    UM = (7 * NFP + 1) * HD // 4
    UD = 15 * NKT * HD // 4
    r6 = UM + (NNT - 1) * UD + 11 * NKT * HD // 4
    add_tasks([(i * P["TMD"] + P["TM0"], tsum, (1, i, 1, i, (i - 1) * P["TMD"] + P["TM0"], P["TMD"])) for i in range(NFP)])
    t, dt = P["HT6"], (UM - 100 - P["HT6"]) // max(NKT - P["NH5"], 1)
    add_tasks([(t + (k + 1) * dt, htriple, (P["NH5"] + k, t + k * dt, dt)) for k in range(NKT - P["NH5"])])
    for i in range(NNT):
        t0, t1 = (UM - P["US0"], UM + 1200) if i == 0 else (UM + (i - 1) * UD + (1300 if i == 1 else 400), UM + i * UD + 350)
        dt = (t1 - t0) // NKT
        add_tasks([(t0 + (k + 1) * dt, hsum, (k, i, t0 + k * dt, dt)) for k in range(NKT)])
    left = len(mains) - n5 - 2
    bd = (r6 - P["R6E"] - P["R6S"]) // left
    add_tasks([(P["R6S"] + (n + 1) * bd, slot, (P["R6S"] + n * bd, bd)) for n in range(left)])
    t = P["R6S"] + left * bd
    add_tasks([(t + (n + 1) * 300, slot, (t + n * 300, 300)) for n in range(2)])
    for qd, t0, t1 in ((NQ, P["LLO"], P["LLO"] + P["LLD"]), (0, 2 * UD + P["LL0"], 3 * UD + P["LL0"]), (1, 3 * UD + P["LL0"], 4 * UD + P["LL0"]),
                       (2, 4 * UD + P["LL2"], 4 * UD + P["LL2"] + P["UEL"])):
        dt = (t1 - t0) // 7
        add_tasks([(UM + t0 + (g + 1) * dt, llsum, (qd, g, UM + t0 + g * dt, dt)) for g in range(7)])
    rr_tasks(BORD[0], 0, 0, P["RP0"], P["RP1"])
    add_tasks([(P["PW0"] + P["PWD"], prep_wo_a, (P["PW0"], P["PWD"]))])
    add_tasks([(P["PW0"] + P["PWD"] + 1, prep_wo_b, (h, P["PW1"] + h * P["PWE"])) for h in range(2)])
    for b in range(NB):
        b2f_s[b // 2, 0:1, _blk(b % 2)] = b2_v[b:b + 1, :].astype(f32)
    u_mid()
    for i in range(NNT):
        u_last(i, None if i == NNT - 1 else P["UEL"] if i == NNT - 2 else P["UED"])
    flush()
    assert slot_ctr[0] == len(mains) and all(("ll", qd, g) in ready for qd in range(NQ + 1) for g in range(7))
    assert all(("pr", j, hh) in ready for j in range(NB) for hh in range(2)) and ("rr", BORD[0]) in ready

    wait("w2", g7)
    lax.fori_loop(0, NP // 4, c_body, 0)
    outs = []
    for pa in range(0, NP, 2):
        outs += [out_copy(pa + n % 2, 0, 2, n // 2 * HD, (n // 2 + 1) * HD) for n in (1, 2, 3)]
        outs += [out_copy(pa, e0, e1, r0, r1) for (r0, r1, e0, e1) in (LAST_PARTS if pa % 4 else [(0, HD, 0, 2)])]
    wait("out", *outs)


@jax.jit
def pallas_parallel_sum__sliding_local_dilated__mixer_token_mlp__prompt_kernel(A_x, A_wqkv, A_wo, B_x, B_w1, B_b1, B_w2, B_b2):
    del B_x
    hbm = pl.BlockSpec(memory_space=pltpu.HBM)
    outT = pl.pallas_call(
        _kernel,
        out_shape=jax.ShapeDtypeStruct((1, D, S), bf16),
        in_specs=[hbm] * 7,
        out_specs=hbm,
        scratch_shapes=[
            pltpu.VMEM((NP, D, 2 * LB), bf16),
            pltpu.VMEM((NP, F, 2 * LB), bf16),
            pltpu.VMEM((NP, D, 2 * LB), bf16),
            pltpu.VMEM((NB + 1, D, LB), f32),
            pltpu.VMEM((NB, 2 * W * HH, LB), f32),
            pltpu.VMEM((NP, 32, 2 * LB), f32),
            pltpu.VMEM((D, 3 * D), bf16),
            pltpu.VMEM((D, D), bf16),
            pltpu.VMEM((S, F), bf16),
            pltpu.VMEM((NFB, LB), bf16),
            pltpu.VMEM((NB, LB), bf16),
            pltpu.VMEM((2, 3 * D + 64, LB), i32),
            pltpu.VMEM((7 * HA // 2, HD), u32),
            pltpu.VMEM((4, HD + 32, LB), i32),
            pltpu.VMEM((D, 2 * LB), i32),
            pltpu.VMEM((HD, S), u32),
            pltpu.VMEM((NP * QD, 5 * LB), u32),
            pltpu.VMEM((7 * QD, 2 * LB), u32),
            pltpu.VMEM((15 * QD, NKT * LB), u32),
            pltpu.VMEM((2 * RHK, 9 * LB), u32),
            pltpu.VMEM((D, F), f32),
            pltpu.VMEM((7 * HD, NFP * LB), f32),
            pltpu.VMEM((7 * QD, LB), u32),
            pltpu.VMEM((D, 4 * NQ * LB), f32),
            pltpu.VMEM((NB, 2 * D, LB), f32),
            pltpu.VMEM((D, LB), f32),
            pltpu.VMEM((2 * RSK, 5 * LB), u32),
            pltpu.VMEM((49 * ED, 4 * LB), u32),
            pltpu.VMEM((7 * RRK, 9 * LB), u32),
            pltpu.VMEM((D, 4 * LB), f32),
            pltpu.VMEM((D, 4 * LB), f32),
            pltpu.VMEM((8, LB), i32),
            pltpu.SemaphoreType.DMA((9,)),
        ],
        compiler_params=pltpu.CompilerParams(vmem_limit_bytes=100 * 1024 * 1024,
                                             disable_bounds_checks=True,
                                             disable_semaphore_checks=True),
    )(jnp.swapaxes(A_x, 1, 2), A_wqkv, A_wo, B_w1, B_b1.reshape(NFB, LB), B_w2, B_b2.reshape(NB, LB))
    return jnp.swapaxes(outT, 1, 2)
```

```python
import jax
import jax.numpy as jnp
from jax import lax
import jax.experimental.pallas as pl
import jax.experimental.pallas.tpu as pltpu

S, D, F = 2048, 448, 1792
H, DH, W, DIL = 16, 28, 8, 2
LB = 128
NB = S // LB
NP = NB // 2
NFB = F // LB
NFP = NFB // 2
HH = H // 2
WH = W // 2
SH = DIL * WH
HD = D // 2
QD = D // 4
ED = D // 8
HA = 3 * HD
HB0 = 4
NKT = (NB - HB0) // 3
NNT = -(-NFB // 3)
RSK = NFP * LB // 2
RHK = NKT * LB // 2
NQ = NFP // 2
KL = NQ * LB + QD
RRK = 2 * LB
EPS = 1e-5
EPS_BF16 = 1.0013580322265625e-05
SCALE = DH ** -0.5
f32 = jnp.float32
bf16 = jnp.bfloat16
u32 = jnp.uint32
i32 = jnp.int32

SCOPES = False
P = dict(
    E1=3, E2=6, T3=-20, N2=16, NA3=2, T1=-200, T2=-200, L2T=100, L2D=440, H2T=900, H2D=340, L4T=920, L5T=0, W2X=500,
    QA=-330, QB=260, QC=-240, QE=420, KA=50, KB=230, KC=390, KE=450,
    LND=420, HSD=200, HTD=525, NH5=4, N4=2, N5=20, TM0=0, TMD=330, HT6=500, SGH=8, HL=260, LNA=0.28, LNB=0.46, LNBD=0.38, LNV=0.86,
    BD=375, MARG=300, LAG=200, LS=150, PP=130, PVL=500, PVPOS=18,
    US0=0, UE0=100, UED=3000, UEL=1600, UG=70, R6S=3150, R6E=1950,
    LL0=600, LLO=1300, LLD=4000, LL2=800, RP0=13000, RP1=15100, PW0=300, PWD=300, PW1=1300, PWE=300,
    RR0=-48, RR1=800, RRM=-20, RW=(8, 8, 8, 2, 7), BV0=117, BVS=717, BVD=620, EP0=0, EPD=864, EPL=290, SGR=8, SGT=8,
)
G = 4


def _as(x, dtype):
    return x if x.dtype == dtype else pltpu.bitcast(x, dtype)


def _pk(x):
    return pltpu.bitcast(x.astype(bf16), u32)


def _up(x):
    return pltpu.bitcast(x, bf16)


def _upf(x):
    return pltpu.bitcast(x, bf16).astype(f32)


def _rb(x):
    return x.astype(bf16).astype(f32)


def _word(lo, hi):
    lo, hi = [pltpu.bitcast(v.astype(f32), i32) for v in (lo, hi)]
    return lax.shift_right_logical(lo, 16) | hi


def _unword(w):
    return [pltpu.bitcast(w << 16, f32), pltpu.bitcast(w & -65536, f32)]


def _cat(xs, axis):
    return xs[0] if len(xs) == 1 else jnp.concatenate(xs, axis=axis)


def _x2(v):
    return jnp.concatenate([v, v], axis=0)


def _blk(b):
    return slice(b * LB, (b + 1) * LB)


def _rowsum8(a):
    return jnp.broadcast_to(jnp.sum(a, axis=0, keepdims=True), (8, a.shape[1]))


def _token(*deps):
    deps = [d for d in deps if d is not None]
    if not deps:
        return None
    if len(deps) == 1:
        return deps[0]
    bits = _as(deps[0], u32)
    for d in deps[1:]:
        bits = bits | _as(d, u32)
    return bits


def _lhs_ops(a11, a12, a21, a22):
    return [a11 + a22, a21 + a22, a11, a22, a11 + a12, a21 - a11, a12 - a22]


SIDX = {0: 0, 2: 1, 3: 2, 5: 3, 6: 4}
TOP = {0: ((0, 0), 1, (1, 1)), 1: ((0, 0),), 2: ((0, 1), -1, (1, 1)), 3: ((1, 0), -1, (0, 0)),
       4: ((1, 1),), 5: ((0, 0), 1, (0, 1)), 6: ((1, 0), 1, (1, 1))}


def _rhs_sums(b11, b12, b21, b22):
    return {0: b11 + b22, 2: b12 - b22, 3: b21 - b11, 5: b11 + b12, 6: b21 + b22}


def _rhs_op(p, blk):
    t = TOP[p]
    if len(t) == 1:
        return blk(*t[0])
    return blk(*t[0]) + blk(*t[2]) if t[1] > 0 else blk(*t[0]) - blk(*t[2])


def _combine(m, n=None):
    c12 = lambda: m[2] + m[4]
    c21 = lambda: m[1] + m[3]
    x = lambda: (m[2] - m[1]) + m[0]
    c = [lambda: (x() + m[6]) + (c21() - c12()), c12, c21, lambda: x() + m[5]]
    return [f() for f in c] if n is None else c[n]()


def _hk_lhs(a):
    s = [a[0][k] + a[1][k] for k in range(3)]
    return [a[0][0], s[0], s[1], a[1][1], a[0][0] + a[1][1], a[0][1] - a[0][0], a[1][0] - a[1][1], a[0][2],
            a[1][2], s[0] - a[1][2], s[2] - s[0], a[1][2] - a[1][0], s[1] - a[0][2], s[2] - s[1], a[0][2] - a[0][1]]


HKB = [((0, 0, 1), (1, 0, 1), (0, 2, -1)), ((0, 0, 1), (2, 0, 1), (0, 1, -1)), ((1, 1, 1), (2, 1, 1), (1, 0, -1)),
       ((1, 1, 1), (0, 1, 1), (1, 2, -1)), ((0, 1, 1), (1, 0, 1)), ((1, 0, 1),), ((0, 1, 1),),
       ((2, 2, 1), (1, 2, 1), (2, 0, -1)), ((2, 2, 1), (0, 2, 1), (2, 1, -1)), ((2, 0, 1), (0, 2, 1)), ((2, 0, 1),),
       ((0, 2, 1),), ((2, 1, 1), (1, 2, 1)), ((2, 1, 1),), ((1, 2, 1),)]


def _hk_terms(nj):
    out = {}
    for p, t in enumerate(HKB):
        t = [x for x in t if x[1] < nj]
        if t and (nj == 3 or p not in (7, 8)):
            out[p] = t
    return out


def _hk_combine(m, nj):
    x, y = (m[9] + m[11], m[12] + m[14]) if nj == 3 else (m[9], m[12])
    x0, y3 = x + m[0], y + m[3]
    c = [[(m[5] + m[10]) + x0, ((m[4] + m[5]) - y3) + m[2]], [((m[4] + m[6]) - x0) + m[1], (m[6] + m[13]) + y3]]
    if nj == 3:
        c[0].append(((m[10] - m[14]) + x) + m[7])
        c[1].append(((m[13] - m[11]) + y) + m[8])
    return c


def _kernel(x_hbm, wqkv_hbm, wo_hbm, w1_hbm, b1_hbm, w2_hbm, b2_hbm, out_hbm,
            x_v, w2_v, out_v, v_s, pr_s, b2f_s, wqkv_v, wo_v, w1_v, b1_v, b2_v, wt_s, lw_s, wo_s,
            wq_s, xnT_s, ra_s, lh_s, lk_s, rh_s, u0_s, um_s, lc_s, g_s, qk_s, op_s, rs_s, ll_s, rr_s, ola_s, olb_s, one_s, sems):
    sem_ctr = [1]

    class Group:
        def __init__(self, pairs):
            self.cps = [pltpu.make_async_copy(a, b, sems.at[sem_ctr[0]]) for (a, b) in pairs]
            sem_ctr[0] += 1

        def start(self):
            for c in self.cps:
                c.start()

        def wait(self):
            for c in self.cps:
                c.wait()

    def cp_x(p0, p1):
        return [(x_hbm.at[0, :, pl.ds(p * 2 * LB, 2 * LB)], x_v.at[p]) for p in range(p0, p1)]

    def cp_w2(p0, p1):
        return [(w2_hbm.at[:, pl.ds(p * 2 * LB, 2 * LB)], w2_v.at[p]) for p in range(p0, p1)]

    def cp_w1(b0, b1, i0=0, i1=NFP):
        sl = pl.ds(b0 * LB, (b1 - b0) * LB)
        cl = pl.ds(i0 * 2 * LB, (i1 - i0) * 2 * LB)
        return [(w1_hbm.at[sl, cl], w1_v.at[sl, cl])]

    tl = []
    mxu = [0, 0, 0, 0]
    nxt = [0]
    hist = []
    tasks = []
    dls = []
    ready = set()
    pos = []
    true = {}

    def tie(v, z):
        if z is None:
            return v
        def fit(a):
            a = _cat([a] * (v.shape[0] // 8), 0)
            return a if v.shape[1] == LB else a[:, 0:v.shape[1]]
        if v.shape not in true:
            true[v.shape] = fit(pos[0]) > 0
        return lax.select(true[v.shape], v, fit(_as(z, v.dtype)))

    def tie8(v, z):
        return v if z is None else jnp.concatenate([tie(v[0:8], z), v[8:16]], axis=0)

    def add_tasks(todo):
        tasks.extend(todo)
        tasks.sort(key=lambda x: x[0])

    def flush(t=None):
        while tasks and (t is None or tasks[0][0] < t):
            _, fn, args = tasks.pop(0)
            fn(*args)

    def reset():
        assert not tasks
        dls.clear()
        tl.clear()
        hist.clear()
        mxu[:] = [0, 0, 0, 0]
        nxt[0] = 0

    def now():
        return sum(mxu) // 4

    def wait(name, *cps):
        flush()
        if SCOPES:
            with jax.named_scope("wait_" + name):
                for c in cps:
                    c.wait()
        else:
            for c in cps:
                c.wait()
        reset()

    def mm1(lhs, rhs, pace=True):
        flush(now())
        start = mxu[nxt[0]]
        due = [v for (t, v) in dls if t <= start] if pace else []
        if due:
            dls[:] = [(t, v) for (t, v) in dls if t > start]
            tile = _up(tie(pltpu.bitcast(lhs[0:16, 0:LB], u32), _token(*due)))
            row = tile if lhs.shape[1] == LB else jnp.concatenate([tile, lhs[0:16, LB:]], axis=1)
            lhs = jnp.concatenate([row, lhs[16:]], axis=0)
        r = jnp.dot(lhs, rhs, preferred_element_type=f32)
        m, k = lhs.shape
        first_done = None
        for _ in range(-(-rhs.shape[1] // LB)):
            end = 0
            for _ in range(-(-k // LB)):
                mxu[nxt[0]] += m
                end = max(end, mxu[nxt[0]])
                nxt[0] = (nxt[0] + 1) % 4
            if first_done is None:
                first_done = end
        if pace:
            tl.append((first_done - m, first_done, r))
        return r

    def mm(lhs, rhs, init=None):
        k = lhs.shape[1]
        r, k0 = init, 0
        while k0 < k:
            k1 = min(k, k0 + (4 - nxt[0]) * LB)
            part = mm1(lhs[:, k0:k1], rhs[k0:k1], pace=k1 - k0 > LB)
            r = part if r is None else r + part
            k0 = k1
        return r

    def at(t, *more):
        best = None
        if t is not None and t >= 0:
            t = min(t, now() - 1)
            for (a, b, r) in tl:
                if a <= t and (best is None or min(b, t) > best[0]):
                    row = int(min((t - a) / (b - a), 0.999) * (r.shape[0] // 8)) * 8
                    best = (min(b, t), r, row)
        return _token(None if best is None else best[1][best[2]:best[2] + 8, 0:LB], *more)

    def strassen(lhs, rhs, order, split_last=False, init=None, m=None):
        m = [None] * 7 if m is None else m
        for p in order:
            flush(now())
            l, r = lhs(p), rhs(p)
            c0 = None if init is None else init[p]
            if split_last and p == order[-1]:
                kk = (-(-r.shape[0] // LB) - 2) * LB
                hm = l.shape[0] // 2
                hd = mm(l[:, :kk], r[:kk], c0) if kk else c0
                tail = jnp.concatenate([mm(l[:hm, kk:], r[kk:]), mm(l[hm:, kk:], r[kk:])], axis=0)
                m[p] = tail if hd is None else hd + tail
            else:
                m[p] = mm(l, r, c0)
        return m

    def wcol(hh, p):
        return p * D + (1 - hh if p == 1 else hh) * HD

    def wrows(hh, g, z=None):
        p, d = divmod(2 * g, DH)
        t = [jnp.concatenate([wt_s[c, pl.ds(wcol(hh, p) + d + e, HH, stride=DH), :]
                              for e in range(2)], axis=0) for c in range(2)]
        return _unword(jnp.concatenate([tie(t[0], z), tie(t[1][:, 0:HD - LB], z)], axis=1))

    wt_done = set()

    def prep_wqkv(part, ga, gb, paced):
        def need(hh, p, z):
            lo = wcol(hh, p)
            for ct in range(lo // LB, -(-(lo + HD) // LB)):
                if ct in wt_done:
                    continue
                wt_done.add(ct)
                cols = slice(ct * LB, min((ct + 1) * LB, 3 * D))
                wd = _word(wqkv_v[0:HD, cols], wqkv_v[HD:D, cols])
                wd = jnp.concatenate([tie(wd[r:r + 8], z if r % LB == 0 else None) for r in range(0, HD, 8)], axis=0)
                wT = wd.T
                wt_s[0, cols, :] = wT[:, 0:LB]
                wt_s[1, cols, 0:HD - LB] = wT[:, LB:HD]

        def put(p, g, v):
            lw_s[p * (HA // 2) + g * 8:p * (HA // 2) + g * 8 + 8, :] = _pk(v)

        def half(hh, g0, g1, t0=None, dur=None):
            pr, ps = ((2, 4), (3, 1))[hh]
            for g in range(g0, g1):
                t = None if t0 is None else t0 + (g - g0) * dur // (g1 - g0)
                need(hh, 2 * g // DH, at(None if t is None else t - P["W2X"]))
                a1, a2 = wrows(hh, g, at(t))
                put(pr, g, a2 if hh else a1)
                put(ps, g, a1 + a2)
            if g1 == gb:
                ready.update({("lw", part, pr), ("lw", part, ps)})

        def rest(g0, g1, t0, dur):
            assert ("lw", part, 1) in ready
            for g in range(g0, g1):
                z = at(t0 + (g - g0) * dur // (g1 - g0))
                ops = _lhs_ops(*wrows(0, g, z), *wrows(1, g, z))
                for p in (0, 5, 6):
                    put(p, g, ops[p])
            if g1 == gb:
                ready.update({("lw", part, 0), ("lw", part, 5), ("lw", part, 6)})
        t2, d2, t3, d3 = paced
        half(0, ga, gb)
        n = (gb - ga) // 14
        add_tasks([(now() + t2 + (k + 1) * d2 // n, half,
                    (1, ga + 14 * k, ga + 14 * k + 14, now() + t2 + k * d2 // n, d2 // n)) for k in range(n)])
        n = (gb - ga) // 7
        add_tasks([(now() + t3 + (k + 1) * d3 // n, rest,
                    (ga + 7 * k, ga + 7 * k + 7, now() + t3 + k * d3 // n, d3 // n)) for k in range(n)])

    def prep_wo_a(t0, dur):
        for g in range(HD // 16):
            w = _word(wo_v[g * 16:g * 16 + 16, :], wo_v[HD + g * 16:HD + g * 16 + 16, :])
            z = at(t0 + g * dur // (HD // 16))
            for c in range(4):
                cw = min(LB, D - c * LB)
                wo_s[c, g * 16:g * 16 + 16, 0:cw] = tie(w[:, c * LB:c * LB + cw], z)
        ready.add("wo")

    def prep_wo_b(h, t_dl):
        assert "wo" in ready
        outs = []
        for c in range(4):
            cw = min(LB, D - c * LB)
            rows = [wo_s[c, pl.ds(d, HH, stride=DH), :][:, 0:cw] for d in range(h * DH // 2, (h + 1) * DH // 2)]
            rows.append(jnp.zeros((LB - QD, cw), i32))
            wT = jnp.concatenate(rows, axis=0).T
            wq_s[c * LB:c * LB + cw, _blk(h)] = wT
            outs += [wT[r:r + 8] for r in range(0, cw, 8)]
        ready.add(("wq", h))
        dls.append((t_dl, _token(*outs)))

    RG = 16
    NG = D // RG
    stat2 = {}

    def ln(b, t0=None, dur=None):
        def xg(g):
            return x_v[b // 2, g * RG:(g + 1) * RG, _blk(b % 2)].astype(f32)

        def step(v, g, fr, s, q):
            if t0 is None or g % 4:
                return v
            acc = [] if s is None else [s[0:8], s[8:16], q[0:8], q[8:16]]
            return tie(v, at(t0 + fr * dur, *acc))

        x0 = jnp.broadcast_to(xg(0)[0:1], (8, LB))
        s = q = None
        for g in range(NG):
            x0 = step(x0, g, P["LNA"] * g / NG, s, q)
            c = xg(g) - _x2(x0)
            s = c if s is None else s + c
            q = c * c if q is None else q + c * c
        dm = _rowsum8(s) * (1.0 / D)
        mu = _rb(x0 + dm)
        var = _rb(jnp.maximum(_rowsum8(q) * (1.0 / D) - dm * dm, 0.0))
        r1 = 1.0 / _rb(jnp.sqrt(_rb(var + EPS_BF16)))
        s = q = None
        for g in range(NG):
            mu = step(mu, g, P["LNB"] + P["LNBD"] * g / NG, s, q)
            xn = _rb(xg(g) - _x2(mu)) * _x2(r1)
            xnT_s[g * 8:g * 8 + 8, _blk(b)] = _pk(xn)
            s = xn if s is None else s + xn
            q = xn * xn if q is None else q + xn * xn
        mu2 = _rowsum8(s) * (1.0 / D)
        var2 = jnp.maximum(_rowsum8(q) * (1.0 / D) - mu2 * mu2, 0.0)
        stat2[b] = (mu2, 0.5 * lax.rsqrt(var2 + EPS))

    def hpair(b, t0=None, dur=None):
        ng = HD // RG
        st = [stat2[b], stat2[b + 1]]
        for g in range(ng):
            if b < HB0:
                zz = [at(None if t0 is None else t0 + (4 * g + k) * dur // (4 * ng)) for k in range(4)]
            else:
                zz = [at(t0 + g * dur // ng), None, None, at(t0 + g * dur // ng + P["SGT"])]
            xq = [_upf(tie(xnT_s[r:r + 8, _blk(b + e)], zz[2 * (r >= QD) + e]))
                  for r in (g * 8, QD + g * 8) for e in range(2)]
            ro = (b // 2) * QD + g * 8
            for p, v in _rhs_sums(*xq).items():
                ra_s[ro:ro + 8, _blk(SIDX[p])] = _pk(v)
            if b < HB0:
                hq = [(v - _x2(st[n % 2][0])) * _x2(st[n % 2][1]) for n, v in enumerate(xq)]
                for p, v in enumerate(_lhs_ops(*hq)):
                    lh_s[p * QD + g * 8:p * QD + g * 8 + 8, _blk(b // 2)] = _pk(v)
        ready.add(("xn", b))
        if b >= 6:
            got = ra_s[(b // 2) * QD:(b // 2 + 1) * QD, :]
            dls.append((t0 + dur + P["HL"], _token(*[got[r:r + 8, _blk(c)] for r in range(0, QD, 8) for c in range(5)])))

    def htile(b, r, z=None):
        return (_upf(tie(xnT_s[r:r + 8, _blk(b)], z)) - _x2(stat2[b][0])) * _x2(stat2[b][1])

    def htriple(t, t0, dur):
        ng = HD // RG
        for g in range(ng):
            zz = [at(t0 + (3 * g + k) * dur // (3 * ng)) for k in range(3)]
            a = [[htile(HB0 + 3 * t + k, h * QD + g * 8, zz[k]) for k in range(3)] for h in range(2)]
            for p, v in enumerate(_hk_lhs(a)):
                lk_s[p * QD + g * 8:p * QD + g * 8 + 8, _blk(t)] = _pk(v)
        ready.add(("lh", t))

    def ln_tasks(b, t, lnd, hsd):
        for fn, bb, dur, adv in ((ln, b, lnd, P["LNV"]), (ln, b + 1, lnd, P["LNV"]), (hpair, b, hsd, 1.0)):
            add_tasks([(t + int(dur * adv), fn, (bb, t, dur))])
            t += int(dur * adv)
        return t

    def tsum(kp, i, slot_, n, t0, dur):
        for g in range(LB // 16):
            z, z2 = at(t0 + g * dur // 8), at(t0 + g * dur // 8 + P["SGT"])
            t1, t2 = [w1_v[(2 * kp + e) * LB + g * 16:(2 * kp + e) * LB + g * 16 + 16,
                           2 * i * LB:(2 * i + 2) * LB].astype(f32) for e in range(2)]
            ro = slot_ * RSK + n * (LB // 2) + g * 8
            for p, v in _rhs_sums(tie8(t1[:, :LB], z), t1[:, LB:], t2[:, :LB], tie8(t2[:, LB:], z2)).items():
                rs_s[ro:ro + 8, _blk(SIDX[p])] = _pk(v)
        ready.add(("rs", kp, i))

    def u_rhs(p, i, kps, slot_, n0):
        if p in SIDX:
            assert all(("rs", kp, i) in ready for kp in kps)
            ro = slot_ * RSK + n0 * (LB // 2)
            return _up(rs_s[ro:ro + len(kps) * (LB // 2), _blk(SIDX[p])])
        e = 0 if p == 1 else 1
        return _cat([w1_v[_blk(2 * kp + e), _blk(2 * i + e)] for kp in kps], 0)

    LATE = (NFP - 1, 6)

    def ujob(kp, i, p):
        flush(now())
        assert ("xn", 2 * kp) in ready
        l, r = _up(lh_s[p * QD:(p + 1) * QD, _blk(kp)]), u_rhs(p, i, [kp], kp, i)
        um_s[p * HD:(p + 1) * HD, _blk(i)] = mm1(l, r)

    def u_early(kp, i0, i1, carry, n, t0, dt):
        for k, i in enumerate(range(i0, i1)):
            add_tasks([(t0 + (k + 1) * dt, tsum, (kp, i, kp, i, t0 + k * dt, dt))])
        jobs = (carry + [(kp, i, p) for i in range(i0, i1) for p in (1, 4)]
                + [(kp, i, p) for i in range(i0, i1) for p in SIDX if (i, p) != LATE])
        for job in jobs[:n]:
            ujob(*job)
        return jobs[n:]

    def u_mid():
        jobs = [(i, p) for i in range(2) for p in (4, 1)]
        for i in range(NFP):
            jobs += [(i, p) for p in (2, 3, 0, 5, 6)] + [(i + 2, p) for p in (4, 1) if i + 2 < NFP]
        m = [[None] * 7 for _ in range(NFP)]
        for i, p in jobs:
            flush(now())
            late = (i, p) == LATE
            l = _up(lh_s[p * QD:(p + 1) * QD, (0 if late else LB):])
            r = _cat([u_rhs(p, i, [0], 0, i)] * late + [u_rhs(p, i, [1], 1, i)], 0)
            v = jnp.concatenate([mm1(l[:QD], r), mm1(l[QD:], r)], axis=0) if late else mm1(l, r)
            if not late:
                v = v + um_s[p * HD:(p + 1) * HD, _blk(i)]
            if p in (2, 3):
                v = v + 0.5 * b1_v[2 * i + 3 - p:2 * i + 4 - p, :].astype(f32)
            m[i][p] = v
            if p == 6:
                for n, c in enumerate(_combine(m[i])):
                    u0_s[n // 2 * HD:(n // 2 + 1) * HD, _blk(2 * i + n % 2)] = c

    def nj_of(i):
        return min(3, NFB - 3 * i)

    def hsum(t, i, t0, dur):
        nj = nj_of(i)
        sums = [(p, tm) for p, tm in _hk_terms(nj).items() if len(tm) > 1]
        tied = {(1, 0): 0, (2, 0): 1, (1, 2): 2, (2, 2): 3} if nj == 3 else {(1, 0): 0, (0, 1): 2}
        for g in range(LB // 16):
            b = {}
            for k in range(3):
                r = (HB0 + 3 * t + k) * LB + g * 16
                w = w1_v[r:r + 16, 3 * i * LB:(3 * i + nj) * LB].astype(f32)
                for j in range(nj):
                    z = at(t0 + g * dur // 8 + tied[k, j] * P["SGH"]) if (k, j) in tied else None
                    b[k, j] = tie8(w[:, _blk(j)], z)
            ro = (i % 2) * RHK + t * (LB // 2) + g * 8
            for n, (p, tm) in enumerate(sums):
                v = b[tm[0][:2]]
                for (k, j, sg) in tm[1:]:
                    v = v + b[k, j] if sg > 0 else v - b[k, j]
                rh_s[ro:ro + 8, _blk(n)] = _pk(v)
        ready.add(("rh", t, i))

    def gelu_half(hx, z):
        c = 0.7978845608028654
        return hx + hx * jnp.tanh(tie(hx * (2.0 * c + (8.0 * c * 0.044715) * (hx * hx)), z))

    def u_epilogue(i, m, gs, t0, dur):
        nj = nj_of(i)
        for n, g in enumerate(gs):
            c = _hk_combine({p: v[g * 16:g * 16 + 16] for p, v in m.items()}, nj)
            for j in range(nj):
                f = 3 * i + j
                t = None if t0 is None else t0 + (n * nj + j) * dur // (len(gs) * nj) - P["UG"]
                gl = [gelu_half(c[h][j] + u0_s[h * HD + g * 16:h * HD + g * 16 + 16, _blk(f)], at(t))
                      for h in range(2)]
                if f < 4 * NQ:
                    for h in range(2):
                        g_s[h * HD + g * 16:h * HD + g * 16 + 16, _blk(f)] = gl[h]
                    ready.add(("g", f, g))
                elif j == 0:
                    g0 = gl
                else:
                    for p, v in enumerate(_lhs_ops(g0[0], gl[0], g0[1], gl[1])):
                        lc_s[p * QD + g * 8:p * QD + g * 8 + 8, :] = _pk(v)

    def u_last(i, edur):
        terms = _hk_terms(nj_of(i))
        sums = [p for p, tm in terms.items() if len(tm) > 1]
        m = {}
        order = ((10, 11, 14, 5, 13, 6, 9, 7, 0, 12, 8, 3, 4, 1, 2) if i == 0
                 else (10, 11, 9, 14, 7, 5, 0, 13, 12, 8, 6, 3, 4, 1, 2))
        for p in [p for p in order if p in terms]:
            flush(now())
            assert all(("lh", t) in ready for t in range(NKT))
            if p in sums:
                assert all(("rh", t, i) in ready for t in range(NKT))
                r = _up(rh_s[(i % 2) * RHK:(i % 2 + 1) * RHK, _blk(sums.index(p))])
            else:
                k, j, _ = terms[p][0]
                r = _cat([w1_v[_blk(HB0 + 3 * t + k), _blk(3 * i + j)] for t in range(NKT)], 0)
            m[p] = mm(_up(lk_s[p * QD:(p + 1) * QD, :]), r)
        if edur is None:
            u_epilogue(i, m, list(range(HD // 16)), None, None)
        else:
            t = now() + P["UE0"]
            add_tasks([(t + (g + 1) * edur // 7, u_epilogue, (i, m, [g, g + 7], t + g * edur // 7, edur // 7))
                       for g in range(7)])

    LTOP = [((0, 0), 1, (1, 1)), ((1, 0), 1, (1, 1)), ((0, 0),), ((1, 1),), ((0, 0), 1, (0, 1)),
            ((1, 0), -1, (0, 0)), ((0, 1), -1, (1, 1))]

    def llsum(qd, g, t0, dur):
        def tile(a, x, h, e):
            r = a * HD + h * QD + g * 16
            if qd < NQ:
                assert ("g", 4 * qd + 2 * e + x, g + 7 * h) in ready
                return g_s[r:r + 16, _blk(4 * qd + 2 * e + x)]
            assert ("wq", e) in ready
            return _unword(wq_s[r:r + 16, _blk(e)])[x]
        for p, t in enumerate(LTOP):
            zz = [at(t0 + p * dur // 7), at(t0 + p * dur // 7 + P["SGT"])]
            a = []
            for h in range(2):
                for e in range(2):
                    v = tile(*t[0], h, e)
                    if len(t) > 1:
                        v = v + tile(*t[2], h, e) if t[1] > 0 else v - tile(*t[2], h, e)
                    a.append(tie8(v, zz[h] if h == e else None))
            for q, v in enumerate(_lhs_ops(*a)):
                r = (p * 7 + q) * ED + g * 8
                ll_s[r:r + 8, _blk(qd)] = _pk(v)
        ready.add(("ll", qd, g))

    AORD = (4, 2, 1, 3, 0, 5, 6)

    def stage_a(b, parts="qkv", order=AORD, split_last=False, m=None):
        r0, r1 = {"q": (0, HD), "kv": (HD, HA), "qkv": (0, HA)}[parts]

        def lhs(p):
            assert all(("lw", pt, p) in ready for pt in ("q", "kv") if pt in parts)
            return _up(lw_s[(p * HA + r0) // 2:(p * HA + r1) // 2, :])

        def rhs(p):
            assert ("xn", b) in ready
            if p in SIDX:
                return _up(ra_s[(b // 2) * QD:(b // 2 + 1) * QD, _blk(SIDX[p])])
            return _up(xnT_s[0:QD, _blk(b)] if p == 1 else xnT_s[QD:HD, _blk(b + 1)])
        m = strassen(lhs, rhs, order, split_last, m=m)
        for n, ps in enumerate((range(7), (2, 4), (1, 3), (0, 1, 2, 5))):
            if all(m[p] is not None for p in ps) and any(p in order for p in ps):
                hh, e = divmod(n, 2)
                c = _combine(m, n)
                qk_s[b + e, hh * D + r0:hh * D + min(r1, D), :] = c[0:min(r1, D) - r0]
                if r1 > D:
                    v_s[b + e + 1, hh * HD:(hh + 1) * HD, :] = c[D - r0:]
        if all(v is not None for v in m):
            ready.update({(pt, b + e) for pt in ("q", "kv") if pt in parts for e in range(2)})
        return m

    lane0 = lax.broadcasted_iota(i32, (HH, LB), 1)
    zeros8 = jnp.zeros((HH, LB), f32)

    def mk_shift(z):
        lane = tie(lane0, z)
        masks = {}

        def pick(n, a, b):
            if n not in masks:
                masks[n] = lane < n
            return lax.select(masks[n], a, b)

        def fwd(cur, prev, sh):
            return cur if sh == 0 else pltpu.roll(pick(LB - sh, cur, prev), sh, 1)

        def bwd(cur, nxt_):
            return pltpu.roll(pick(SH, nxt_, cur), LB - SH, 1)
        return fwd, bwd

    def grp_shift(t, bd):
        lag = max(2, -(-P["LAG"] * DH // (G * bd)))
        return mk_shift(at(t, *(hist[-lag] if len(hist) >= lag else [])))

    raw, probs = {}, {}

    def attn_qk(j, hh, t, bd):
        jn = min(j + 1, NB - 1)
        assert ("q", jn) in ready and ("kv", j) in ready
        acc = [None] * WH
        accp = [None] * WH
        for d in range(DH):
            if d % G == 0:
                if d > 0:
                    hist.append(acc + accp)
                fwd, bwd = grp_shift(t + d * bd // DH, bd)
            r = hh * D + d * HH
            q = qk_s[j, r:r + HH, :]
            qp = bwd(q, qk_s[jn, r:r + HH, :])
            rk = (1 - hh) * D + HD + d * HH
            k = qk_s[j, rk:rk + HH, :]
            kp = qk_s[j - 1, rk:rk + HH, :] if j > 0 else zeros8
            for a in range(WH):
                ks = fwd(k, kp, DIL * a)
                t0, t1 = q * ks, qp * ks
                acc[a] = t0 if d == 0 else acc[a] + t0
                accp[a] = t1 if d == 0 else accp[a] + t1
        hist.append(acc + accp)
        raw[j, hh] = (acc, accp)

    def attn_sm(j, hh, t):
        fwd, _ = mk_shift(at(t))
        acc, accp = raw[j, hh]
        prev = raw.pop((j - 1, hh))[1] if j > 0 else [zeros8] * WH
        lg = acc + [fwd(accp[a], prev[a], SH) for a in range(WH)]
        lg = [a * SCALE for a in lg]
        if j == 0:
            lg = [lg[0]] + [jnp.where(lane0 >= DIL * w, lg[w], -1e9) for w in range(1, W)]
        m = lg[0]
        for w in range(1, W):
            m = jnp.maximum(m, lg[w])
        e = [jnp.exp(l - m) for l in lg]
        den = e[0]
        for w in range(1, W):
            den = den + e[w]
        inv = 1.0 / den
        p = [x * inv for x in e]
        for a in range(WH):
            pr_s[j, (hh * W + a) * HH:(hh * W + a + 1) * HH, :] = p[a]
        probs[j, hh] = p[WH:]

    def attn_pp(j, hh, t):
        _, bwd = mk_shift(at(t))
        p = probs.pop((j, hh))
        pn = probs[j + 1, hh] if j + 1 < NB else p
        for a in range(WH):
            pr_s[j, (hh * W + WH + a) * HH:(hh * W + WH + a + 1) * HH, :] = bwd(p[a], pn[a])
        ready.add(("pr", j, hh))

    def attn_pv(j, hh, dst, e, t, bd):
        assert not isinstance(j, int) or ("pr", j, hh) in ready
        assert e == 0 or ("o", dst, hh, e - 1) in ready
        pa = [pr_s[j, (hh * W + a) * HH:(hh * W + a + 1) * HH, :] for a in range(W)]
        p, pp = pa[:WH], pa[WH:]
        outs = []
        for d in range(DH):
            if d % G == 0:
                if d > 0:
                    hist.append([])
                fwd, _ = grp_shift(t + d * bd // DH, bd)
            r = hh * HD + d * HH
            v = v_s[j + 1, r:r + HH, :]
            vp = v_s[j, r:r + HH, :]
            o = op = None
            for a in range(WH):
                vs = fwd(v, vp, DIL * a)
                o = p[a] * vs if a == 0 else o + p[a] * vs
                op = pp[a] * vs if a == 0 else op + pp[a] * vs
            opp = zeros8 if (isinstance(j, int) and j == 0) else op_s[r:r + HH, :]
            op_s[r:r + HH, :] = op
            outs.append(o + fwd(op, opp, SH))
            ol[dst][r:r + HH, _blk(e)] = outs[-1]
        hist.append([])
        ready.add(("o", dst, hh, e))
        dls.append((t + bd + P["PVL"], _token(*outs)))

    ol = [ola_s, olb_s]
    mains = [("qk", j, hh) for j in range(NB) for hh in range(2)]
    mains = (mains[:P["PVPOS"]] + [("pv", j, hh) for j in range(4) for hh in range(2)]
             + mains[P["PVPOS"]:] + [None, None])
    slot_ctr = [0]

    def slot(t, bd):
        n = slot_ctr[0]
        slot_ctr[0] += 1
        it = mains[n]
        if it is None:
            pass
        elif it[0] == "qk":
            attn_qk(it[1], it[2], t, bd)
        else:
            attn_pv(it[1], it[2], 0, it[1], t, bd)
        if n >= 1 and mains[n - 1] is not None and mains[n - 1][0] == "qk":
            attn_sm(mains[n - 1][1], mains[n - 1][2], t + P["LS"])
        if n >= 2 and mains[n - 2] is not None and mains[n - 2][0] == "qk":
            _, j, hh = mains[n - 2]
            if j > 0:
                attn_pp(j - 1, hh, t + P["PP"])
            if j == NB - 1:
                attn_pp(j, hh, t + P["PP"])

    NRG = 8 * (NQ + 1) + 7
    PD = 8 * QD
    BORD = (1, 3, 2, 4, 0, 5, 6)
    LORD = (2, 4, 1, 3, 0, 5, 6)
    LAST_PARTS = [(0, QD, 1, 2), (QD, HD, 0, 2), (0, QD, 0, 1)]

    def rr_prep(p, pa, src, n0, n1, t0, dur):
        assert ("rr", p) not in ready
        for n in range(n0, n1):
            z = at(t0 + (n - n0) * dur // (n1 - n0))
            z2 = at(t0 + (n - n0) * dur // (n1 - n0) + P["SGR"])
            qd, g = divmod(n, 8)

            def wrow(i):
                return _rhs_op(p, lambda x, y: w2_v[pa + y, (2 * i + x) * LB + g * 16:(2 * i + x) * LB + g * 16 + 16, :]
                               .astype(f32))

            def orow(h):
                def blk(x, y):
                    assert ("o", src, x, 2 * y + 1) in ready
                    r = x * HD + h * QD + g * 16
                    return ol[src][r:r + 16, y * 2 * LB:(y + 1) * 2 * LB]
                return _rhs_op(p, blk)
            ro = p * RRK + g * 8
            if qd == NQ:
                if p in SIDX:
                    r = wrow(2 * NQ)
                    for e in range(2):
                        rr_s[ro:ro + 8, _blk(7 + e)] = _pk(tie8(r[:, _blk(e)], z))
                continue
            r1, r2 = (wrow(2 * qd), wrow(2 * qd + 1)) if qd < NQ else (orow(0), orow(1))
            ro += min(qd, NQ) * (LB // 2)
            c11, c22 = tie8(r1[:, :LB], z), tie8(r2[:, LB:], z2)
            sm = _rhs_sums(c11, r1[:, LB:], r2[:, :LB], c22)
            if p in SIDX or qd > NQ:
                sm.update({1: c11, 4: c22})
            for q, v in sm.items():
                rr_s[ro:ro + 8, _blk(q)] = _pk(v)
        if n1 == NRG:
            ready.add(("rr", p))

    def rr_tasks(p, pa, src, t0, t1):
        cuts = list(range(0, NRG, 8)) + [NRG]
        acc, tot = 0, sum(P["RW"])
        for a, b, w in zip(cuts[:-1], cuts[1:], P["RW"]):
            ta, tb = t0 + acc * (t1 - t0) // tot, t0 + (acc + w) * (t1 - t0) // tot
            add_tasks([(tb, rr_prep, (p, pa, src, a, b, ta, tb - ta))])
            acc += w

    def out_copy(pidx, e0, e1, r0, r1):
        off = pidx * (2 * LB) + e0 * LB
        if not isinstance(pidx, int):
            off = pl.multiple_of(off, LB)
        rs = pl.ds(r0, r1 - r0)
        return pltpu.make_async_copy(out_v.at[pidx, rs, pl.ds(e0 * LB, (e1 - e0) * LB)],
                                     out_hbm.at[0, rs, pl.ds(off, (e1 - e0) * LB)], sems.at[0])

    def b_out(pa, n, m, part, t0=None, dur=None):
        a, y = divmod(n, 2)
        r0, r1, e0, e1 = part
        cols = slice(e0 * LB, e1 * LB)
        for r in range(r0, r1, 16):
            c = _combine([None if v is None else v[r:r + 16, cols] for v in m], n)
            rows = slice(a * HD + r, a * HD + r + 16)
            o = c + x_v[pa + y, rows, cols].astype(f32)
            if t0 is not None:
                o = jnp.concatenate([tie(o[:, 0:LB], at(t0 + (r - r0) * dur // (r1 - r0))), o[:, LB:]], axis=1)
            out_v[pa + y, rows, cols] = o.astype(bf16)
        out_copy(pa + y, e0, e1, a * HD + r0, a * HD + r1).start()

    def big_piece(pa, pan, cur, last):
        t0 = now()
        for n in range(7):
            ta, tb = t0 + n * PD + P["RR0"], t0 + n * PD + P["RR1"]
            if n < 6:
                rr_tasks(BORD[n + 1], pa, cur, ta, tb)
            else:
                rr_tasks(BORD[0], pan, 1 - cur, ta, tb - (P["RRM"] if last else 0))
        ready.difference_update({("o", 1 - cur, hh, e) for hh in range(2) for e in range(4)})
        for n in range(8):
            e, hh = divmod(n, 2)
            t = t0 + P["BV0"] + n * P["BVS"]
            add_tasks([(t + P["BVD"], attn_pv, (pan * 2 + e, hh, 1 - cur, e, t, P["BVD"]))])
        m = [None] * 7
        for p in BORD:
            flush(now())
            assert ("rr", p) in ready
            x, y = TOP[p][0]

            def lhs(q):
                return _up(ll_s[(p * 7 + q) * ED:(p * 7 + q + 1) * ED, 0:KL])

            def rhs(q):
                if p in SIDX or q in SIDX:
                    return _up(rr_s[p * RRK:p * RRK + KL // 2, _blk(q)])
                h = 0 if q == 1 else 1
                return _cat([w2_v[pa + y, _blk(2 * (2 * qd + h) + x), _blk(h)] for qd in range(NQ)]
                            + [_up(rr_s[p * RRK + NQ * LB // 2:p * RRK + KL // 2, _blk(q)])], 0)
            rl = (_up(rr_s[p * RRK:p * RRK + LB // 2, 7 * LB:9 * LB]) if p in SIDX
                  else w2_v[pa + y, _blk(4 * NQ + x), :])
            ll = _up(lc_s[p * QD:(p + 1) * QD, :])
            ex = [mm1(ll[:QD], rl), mm1(ll[QD:], rl)]
            e12, e21 = ex[0][:, LB:], ex[1][:, :LB]
            e11 = (ex[0][:, :LB] + e12) - e21
            lf = strassen(lhs, rhs, LORD)
            ready.discard(("rr", p))
            if p in (2, 3):
                for q in (2, 3):
                    lf[q] = lf[q] + b2f_s[pa + 3 - p, 0:1, _blk(3 - q)]
            c12 = (lf[2] + e12) + lf[4]
            c21 = (lf[1] + e21) + lf[3]
            xx = (lf[2] - lf[1]) + lf[0]
            c22 = (xx + ex[1][:, LB:]) + lf[5]
            c11 = ((xx + e11) + (c21 - c12)) + lf[6]
            m[p] = jnp.concatenate([jnp.concatenate([c11, c12], axis=1),
                                    jnp.concatenate([c21, c22], axis=1)], axis=0)
            n = {3: 2, 4: 1, 5: 3, 6: 0}.get(p)
            if n is not None and not (last and n == 0):
                t, epd = now() + P["EP0"], P["EPL"] if (last and n == 3) else P["EPD"]
                add_tasks([(t + epd, b_out, (pa, n, list(m), (0, HD, 0, 2), t, epd))])
        if last:
            flush()
            for part in LAST_PARTS:
                b_out(pa, 0, m, part)

    def c_body(it, carry):
        reset()
        pos[:] = [one_s[...]]
        true.clear()
        ready.update({("rr", BORD[0])} | {("o", 0, hh, e) for hh in range(2) for e in range(4)})
        big_piece(4 * it, 4 * it + 2, 0, False)
        big_piece(4 * it + 2, lax.rem(4 * it + 4, NP), 1, True)
        assert ("rr", BORD[0]) in ready and all(("o", 0, hh, 3) in ready for hh in range(2))
        return carry

    E1, E2 = P["E1"], P["E2"]
    x0 = Group(cp_x(0, 1))
    g1 = Group(cp_w1(0, 2, 0, E1))
    g2 = Group(cp_w1(0, 2, E1, E2) + cp_x(1, 2))
    wq, wkv = [[(wqkv_hbm.at[:, cl], wqkv_v.at[:, cl])] for cl in (pl.ds(0, 4 * LB), pl.ds(4 * LB, 3 * D - 4 * LB))]
    g3 = Group((cp_w1(0, 2, E2, NFP) if E2 < NFP else []) + wq)
    g4 = Group(wkv + cp_x(2, 3))
    g5 = Group(cp_x(3, NP))
    g6 = Group(cp_w1(2, NB) + [(wo_hbm, wo_v), (b1_hbm, b1_v), (b2_hbm, b2_v)] + cp_w2(0, 1))
    g7 = Group(cp_w2(1, NP))
    for c in (x0, g1, g2, g3, g4, g5, g6, g7):
        c.start()

    v_s[0] = jnp.zeros((D, LB), f32)
    for buf in (xnT_s, ra_s, lh_s, lk_s, rh_s, rs_s, rr_s, ola_s, olb_s, ll_s, lc_s, g_s, wq_s):
        buf[0:8, 0:64] = jnp.zeros((8, 64), buf.dtype)

    wait("x0", x0)
    one_s[...] = lax.shift_right_logical(pltpu.bitcast(x_v[0, 0:16, 0:LB], i32), 1) | 1
    pos[:] = [one_s[...]]
    ln(0)
    ln(1)
    hpair(0)
    wait("r1", g1)
    jobs = u_early(0, 0, E1, [], 7 * E1 // 4 * 4, P["T1"], 100)
    wait("r2", g2)
    t, dt = P["L2T"], P["L2D"]
    add_tasks([(t + int((k + 1) * dt * P["LNV"]), ln, (2 + k, t + int(k * dt * P["LNV"]), dt)) for k in range(2)])
    jobs = u_early(0, E1, E2, jobs, P["N2"], P["T2"], 100)
    wait("wq", g3)
    add_tasks([(P["H2T"] + P["H2D"], hpair, (2, P["H2T"], P["H2D"]))])
    u_early(0, E2, NFP, jobs, 7 * NFP, P["T3"], 100)
    prep_wqkv("q", 0, HD // 16, [P[k] for k in ("QA", "QB", "QC", "QE")])
    stage_a(0, "q", split_last=True)
    m = stage_a(2, "q", AORD[:P["NA3"]])
    wait("wkv", g4)
    stage_a(2, "q", AORD[P["NA3"]:], split_last=True, m=m)
    prep_wqkv("kv", HD // 16, HA // 16, [P[k] for k in ("KA", "KB", "KC", "KE")])
    t = ln_tasks(4, now() + P["L4T"], P["LND"], P["HSD"])
    n4 = P["N4"]
    add_tasks([(t + (n + 1) * P["BD"], slot, (t + n * P["BD"], P["BD"])) for n in range(n4)])
    stage_a(0, "kv")
    stage_a(2, "kv", order=(6,) + AORD[:6])

    wait("mid", g5)
    AD = 7 * HA // 2
    t = P["L5T"]
    for b in range(6, NB, 2):
        t = ln_tasks(b, t, P["LND"], P["HSD"])
    for k in range(P["NH5"]):
        add_tasks([(t + P["HTD"], htriple, (k, t, P["HTD"]))])
        t += P["HTD"]
    n5 = P["N5"]
    bd = ((NP - 2) * AD - P["MARG"] - t) // n5
    add_tasks([(t + (n + 1) * bd, slot, (t + n * bd, bd)) for n in range(n5)])
    n5 += n4
    for n, b in enumerate(range(4, NB, 2)):
        stage_a(b, order=(6,) + AORD[:6] if n % 2 else AORD)

    wait("fin", g6)
    UM = (7 * NFP + 1) * HD // 4
    UD = 15 * NKT * HD // 4
    r6 = UM + (NNT - 1) * UD + 11 * NKT * HD // 4
    add_tasks([(i * P["TMD"] + P["TM0"], tsum, (1, i, 1, i, (i - 1) * P["TMD"] + P["TM0"], P["TMD"])) for i in range(NFP)])
    t, dt = P["HT6"], (UM - 100 - P["HT6"]) // max(NKT - P["NH5"], 1)
    add_tasks([(t + (k + 1) * dt, htriple, (P["NH5"] + k, t + k * dt, dt)) for k in range(NKT - P["NH5"])])
    for i in range(NNT):
        t0, t1 = (UM - P["US0"], UM + 1200) if i == 0 else (UM + (i - 1) * UD + (1300 if i == 1 else 400), UM + i * UD + 350)
        dt = (t1 - t0) // NKT
        add_tasks([(t0 + (k + 1) * dt, hsum, (k, i, t0 + k * dt, dt)) for k in range(NKT)])
    left = len(mains) - n5 - 2
    bd = (r6 - P["R6E"] - P["R6S"]) // left
    add_tasks([(P["R6S"] + (n + 1) * bd, slot, (P["R6S"] + n * bd, bd)) for n in range(left)])
    t = P["R6S"] + left * bd
    add_tasks([(t + (n + 1) * 300, slot, (t + n * 300, 300)) for n in range(2)])
    for qd, t0, t1 in ((NQ, P["LLO"], P["LLO"] + P["LLD"]), (0, 2 * UD + P["LL0"], 3 * UD + P["LL0"]), (1, 3 * UD + P["LL0"], 4 * UD + P["LL0"]),
                       (2, 4 * UD + P["LL2"], 4 * UD + P["LL2"] + P["UEL"])):
        dt = (t1 - t0) // 7
        add_tasks([(UM + t0 + (g + 1) * dt, llsum, (qd, g, UM + t0 + g * dt, dt)) for g in range(7)])
    rr_tasks(BORD[0], 0, 0, P["RP0"], P["RP1"])
    add_tasks([(P["PW0"] + P["PWD"], prep_wo_a, (P["PW0"], P["PWD"]))])
    add_tasks([(P["PW0"] + P["PWD"] + 1, prep_wo_b, (h, P["PW1"] + h * P["PWE"])) for h in range(2)])
    for b in range(NB):
        b2f_s[b // 2, 0:1, _blk(b % 2)] = b2_v[b:b + 1, :].astype(f32)
    u_mid()
    for i in range(NNT):
        u_last(i, None if i == NNT - 1 else P["UEL"] if i == NNT - 2 else P["UED"])
    flush()
    assert slot_ctr[0] == len(mains) and all(("ll", qd, g) in ready for qd in range(NQ + 1) for g in range(7))
    assert all(("pr", j, hh) in ready for j in range(NB) for hh in range(2)) and ("rr", BORD[0]) in ready

    wait("w2", g7)
    lax.fori_loop(0, NP // 4, c_body, 0)
    outs = []
    for pa in range(0, NP, 2):
        outs += [out_copy(pa + n % 2, 0, 2, n // 2 * HD, (n // 2 + 1) * HD) for n in (1, 2, 3)]
        outs += [out_copy(pa, e0, e1, r0, r1) for (r0, r1, e0, e1) in (LAST_PARTS if pa % 4 else [(0, HD, 0, 2)])]
    wait("out", *outs)


@jax.jit
def pallas_parallel_sum__sliding_local_dilated__mixer_token_mlp__prompt_kernel(
    A_x: jax.Array,
    A_wqkv: jax.Array,
    A_wo: jax.Array,
    B_x: jax.Array,
    B_w1: jax.Array,
    B_b1: jax.Array,
    B_w2: jax.Array,
    B_b2: jax.Array,
):
    del B_x
    hbm = pl.BlockSpec(memory_space=pltpu.HBM)
    outT = pl.pallas_call(
        _kernel,
        out_shape=jax.ShapeDtypeStruct((1, D, S), bf16),
        in_specs=[hbm] * 7,
        out_specs=hbm,
        scratch_shapes=[
            pltpu.VMEM((NP, D, 2 * LB), bf16),
            pltpu.VMEM((NP, F, 2 * LB), bf16),
            pltpu.VMEM((NP, D, 2 * LB), bf16),
            pltpu.VMEM((NB + 1, D, LB), f32),
            pltpu.VMEM((NB, 2 * W * HH, LB), f32),
            pltpu.VMEM((NP, 32, 2 * LB), f32),
            pltpu.VMEM((D, 3 * D), bf16),
            pltpu.VMEM((D, D), bf16),
            pltpu.VMEM((S, F), bf16),
            pltpu.VMEM((NFB, LB), bf16),
            pltpu.VMEM((NB, LB), bf16),
            pltpu.VMEM((2, 3 * D + 64, LB), i32),
            pltpu.VMEM((7 * HA // 2, HD), u32),
            pltpu.VMEM((4, HD + 32, LB), i32),
            pltpu.VMEM((D, 2 * LB), i32),
            pltpu.VMEM((HD, S), u32),
            pltpu.VMEM((NP * QD, 5 * LB), u32),
            pltpu.VMEM((7 * QD, 2 * LB), u32),
            pltpu.VMEM((15 * QD, NKT * LB), u32),
            pltpu.VMEM((2 * RHK, 9 * LB), u32),
            pltpu.VMEM((D, F), f32),
            pltpu.VMEM((7 * HD, NFP * LB), f32),
            pltpu.VMEM((7 * QD, LB), u32),
            pltpu.VMEM((D, 4 * NQ * LB), f32),
            pltpu.VMEM((NB, 2 * D, LB), f32),
            pltpu.VMEM((D, LB), f32),
            pltpu.VMEM((2 * RSK, 5 * LB), u32),
            pltpu.VMEM((49 * ED, 4 * LB), u32),
            pltpu.VMEM((7 * RRK, 9 * LB), u32),
            pltpu.VMEM((D, 4 * LB), f32),
            pltpu.VMEM((D, 4 * LB), f32),
            pltpu.VMEM((8, LB), i32),
            pltpu.SemaphoreType.DMA((9,)),
        ],
        compiler_params=pltpu.CompilerParams(vmem_limit_bytes=100 * 1024 * 1024,
                                             disable_bounds_checks=True,
                                             disable_semaphore_checks=True),
    )(jnp.swapaxes(A_x, 1, 2), A_wqkv, A_wo, B_w1, B_b1.reshape(NFB, LB), B_w2, B_b2.reshape(NB, LB))
    return jnp.swapaxes(outT, 1, 2)
```

```python
import jax
import jax.numpy as jnp
from jax import lax
import jax.experimental.pallas as pl
import jax.experimental.pallas.tpu as pltpu

S, D, F = 2048, 448, 1792
H, DH, W, DIL = 16, 28, 8, 2
LB = 128
NB = S // LB
NP = NB // 2
NFB = F // LB
NFP = NFB // 2
HH = H // 2
WH = W // 2
SH = DIL * WH
HD = D // 2
QD = D // 4
ED = D // 8
HA = 3 * HD
HB0 = 4
NKT = (NB - HB0) // 3
NNT = -(-NFB // 3)
RSK = NFP * LB // 2
RHK = NKT * LB // 2
NQ = NFP // 2
KL = NQ * LB + QD
RRK = 2 * LB
EPS = 1e-5
EPS_BF16 = 1.0013580322265625e-05
SCALE = DH ** -0.5
f32 = jnp.float32
bf16 = jnp.bfloat16
u32 = jnp.uint32
i32 = jnp.int32

SCOPES = False
P = dict(
    E1=3, E2=6, T3=-20, N2=16, NA3=2, T1=-200, T2=-200, L2T=100, L2D=440, H2T=900, H2D=340, L4T=920, L5T=0, W2X=500,
    QA=-330, QB=260, QC=-240, QE=420, KA=50, KB=230, KC=390, KE=450,
    LND=420, HSD=200, HTD=525, NH5=4, N4=2, N5=20, TM0=0, TMD=330, HT6=500, SGH=8, HL=260, LNA=0.28, LNB=0.46, LNBD=0.38, LNV=0.86,
    BD=375, MARG=300, LAG=200, LS=150, PP=130, PVL=500, PVPOS=18,
    US0=0, UE0=100, UED=3000, UEL=1600, UG=70, R6S=3150, R6E=1950,
    LL0=600, LLO=1300, LLD=4000, LL2=800, RP0=13000, RP1=15100, PW0=300, PWD=300, PW1=1300, PWE=300,
    RR0=-48, RR1=800, RRM=10, RW=(8, 8, 8, 2, 7), RO=(4, 3, 0, 1, 2), BV0=117, BVS=717, BVD=620, EP0=0, EPD=864, EPL=410, SGR=8, SGT=8,
)
G = 4


def _as(x, dtype):
    return x if x.dtype == dtype else pltpu.bitcast(x, dtype)


def _pk(x):
    return pltpu.bitcast(x.astype(bf16), u32)


def _up(x):
    return pltpu.bitcast(x, bf16)


def _upf(x):
    return pltpu.bitcast(x, bf16).astype(f32)


def _rb(x):
    return x.astype(bf16).astype(f32)


def _word(lo, hi):
    lo, hi = [pltpu.bitcast(v.astype(f32), i32) for v in (lo, hi)]
    return lax.shift_right_logical(lo, 16) | hi


def _unword(w):
    return [pltpu.bitcast(w << 16, f32), pltpu.bitcast(w & -65536, f32)]


def _cat(xs, axis):
    return xs[0] if len(xs) == 1 else jnp.concatenate(xs, axis=axis)


def _x2(v):
    return jnp.concatenate([v, v], axis=0)


def _blk(b):
    return slice(b * LB, (b + 1) * LB)


def _rowsum8(a):
    return jnp.broadcast_to(jnp.sum(a, axis=0, keepdims=True), (8, a.shape[1]))


def _token(*deps):
    deps = [d for d in deps if d is not None]
    if not deps:
        return None
    if len(deps) == 1:
        return deps[0]
    bits = _as(deps[0], u32)
    for d in deps[1:]:
        bits = bits | _as(d, u32)
    return bits


def _lhs_ops(a11, a12, a21, a22):
    return [a11 + a22, a21 + a22, a11, a22, a11 + a12, a21 - a11, a12 - a22]


SIDX = {0: 0, 2: 1, 3: 2, 5: 3, 6: 4}
TOP = {0: ((0, 0), 1, (1, 1)), 1: ((0, 0),), 2: ((0, 1), -1, (1, 1)), 3: ((1, 0), -1, (0, 0)),
       4: ((1, 1),), 5: ((0, 0), 1, (0, 1)), 6: ((1, 0), 1, (1, 1))}


def _rhs_sums(b11, b12, b21, b22):
    return {0: b11 + b22, 2: b12 - b22, 3: b21 - b11, 5: b11 + b12, 6: b21 + b22}


def _rhs_op(p, blk):
    t = TOP[p]
    if len(t) == 1:
        return blk(*t[0])
    return blk(*t[0]) + blk(*t[2]) if t[1] > 0 else blk(*t[0]) - blk(*t[2])


def _combine(m, n=None):
    c12 = lambda: m[2] + m[4]
    c21 = lambda: m[1] + m[3]
    x = lambda: (m[2] - m[1]) + m[0]
    c = [lambda: (x() + m[6]) + (c21() - c12()), c12, c21, lambda: x() + m[5]]
    return [f() for f in c] if n is None else c[n]()


def _hk_lhs(a):
    s = [a[0][k] + a[1][k] for k in range(3)]
    return [a[0][0], s[0], s[1], a[1][1], a[0][0] + a[1][1], a[0][1] - a[0][0], a[1][0] - a[1][1], a[0][2],
            a[1][2], s[0] - a[1][2], s[2] - s[0], a[1][2] - a[1][0], s[1] - a[0][2], s[2] - s[1], a[0][2] - a[0][1]]


HKB = [((0, 0, 1), (1, 0, 1), (0, 2, -1)), ((0, 0, 1), (2, 0, 1), (0, 1, -1)), ((1, 1, 1), (2, 1, 1), (1, 0, -1)),
       ((1, 1, 1), (0, 1, 1), (1, 2, -1)), ((0, 1, 1), (1, 0, 1)), ((1, 0, 1),), ((0, 1, 1),),
       ((2, 2, 1), (1, 2, 1), (2, 0, -1)), ((2, 2, 1), (0, 2, 1), (2, 1, -1)), ((2, 0, 1), (0, 2, 1)), ((2, 0, 1),),
       ((0, 2, 1),), ((2, 1, 1), (1, 2, 1)), ((2, 1, 1),), ((1, 2, 1),)]


def _hk_terms(nj):
    out = {}
    for p, t in enumerate(HKB):
        t = [x for x in t if x[1] < nj]
        if t and (nj == 3 or p not in (7, 8)):
            out[p] = t
    return out


def _hk_combine(m, nj):
    x, y = (m[9] + m[11], m[12] + m[14]) if nj == 3 else (m[9], m[12])
    x0, y3 = x + m[0], y + m[3]
    c = [[(m[5] + m[10]) + x0, ((m[4] + m[5]) - y3) + m[2]], [((m[4] + m[6]) - x0) + m[1], (m[6] + m[13]) + y3]]
    if nj == 3:
        c[0].append(((m[10] - m[14]) + x) + m[7])
        c[1].append(((m[13] - m[11]) + y) + m[8])
    return c


def _kernel(x_hbm, wqkv_hbm, wo_hbm, w1_hbm, b1_hbm, w2_hbm, b2_hbm, out_hbm,
            x_v, w2_v, out_v, v_s, pr_s, b2f_s, wqkv_v, wo_v, w1_v, b1_v, b2_v, wt_s, lw_s, wo_s,
            wq_s, xnT_s, ra_s, lh_s, lk_s, rh_s, u0_s, um_s, lc_s, g_s, qk_s, op_s, rs_s, ll_s, rr_s, ola_s, olb_s, one_s, sems):
    sem_ctr = [1]

    class Group:
        def __init__(self, pairs):
            self.cps = [pltpu.make_async_copy(a, b, sems.at[sem_ctr[0]]) for (a, b) in pairs]
            sem_ctr[0] += 1

        def start(self):
            for c in self.cps:
                c.start()

        def wait(self):
            for c in self.cps:
                c.wait()

    def cp_x(p0, p1):
        return [(x_hbm.at[0, :, pl.ds(p * 2 * LB, 2 * LB)], x_v.at[p]) for p in range(p0, p1)]

    def cp_w2(p0, p1):
        return [(w2_hbm.at[:, pl.ds(p * 2 * LB, 2 * LB)], w2_v.at[p]) for p in range(p0, p1)]

    def cp_w1(b0, b1, i0=0, i1=NFP):
        sl = pl.ds(b0 * LB, (b1 - b0) * LB)
        cl = pl.ds(i0 * 2 * LB, (i1 - i0) * 2 * LB)
        return [(w1_hbm.at[sl, cl], w1_v.at[sl, cl])]

    tl = []
    mxu = [0, 0, 0, 0]
    nxt = [0]
    hist = []
    tasks = []
    dls = []
    ready = set()
    pos = []
    true = {}

    def tie(v, z):
        if z is None:
            return v
        def fit(a):
            a = _cat([a] * (v.shape[0] // 8), 0)
            return a if v.shape[1] == LB else a[:, 0:v.shape[1]]
        if v.shape not in true:
            true[v.shape] = fit(pos[0]) > 0
        return lax.select(true[v.shape], v, fit(_as(z, v.dtype)))

    def tie8(v, z):
        return v if z is None else jnp.concatenate([tie(v[0:8], z), v[8:16]], axis=0)

    def add_tasks(todo):
        tasks.extend(todo)
        tasks.sort(key=lambda x: x[0])

    def flush(t=None):
        while tasks and (t is None or tasks[0][0] < t):
            _, fn, args = tasks.pop(0)
            fn(*args)

    def reset():
        assert not tasks
        dls.clear()
        tl.clear()
        hist.clear()
        mxu[:] = [0, 0, 0, 0]
        nxt[0] = 0

    def now():
        return sum(mxu) // 4

    def wait(name, *cps):
        flush()
        if SCOPES:
            with jax.named_scope("wait_" + name):
                for c in cps:
                    c.wait()
        else:
            for c in cps:
                c.wait()
        reset()

    def mm1(lhs, rhs, pace=True):
        flush(now())
        start = mxu[nxt[0]]
        due = [v for (t, v) in dls if t <= start] if pace else []
        if due:
            dls[:] = [(t, v) for (t, v) in dls if t > start]
            tile = _up(tie(pltpu.bitcast(lhs[0:16, 0:LB], u32), _token(*due)))
            row = tile if lhs.shape[1] == LB else jnp.concatenate([tile, lhs[0:16, LB:]], axis=1)
            lhs = jnp.concatenate([row, lhs[16:]], axis=0)
        r = jnp.dot(lhs, rhs, preferred_element_type=f32)
        m, k = lhs.shape
        first_done = None
        for _ in range(-(-rhs.shape[1] // LB)):
            end = 0
            for _ in range(-(-k // LB)):
                mxu[nxt[0]] += m
                end = max(end, mxu[nxt[0]])
                nxt[0] = (nxt[0] + 1) % 4
            if first_done is None:
                first_done = end
        if pace:
            tl.append((first_done - m, first_done, r))
        return r

    def mm(lhs, rhs, init=None):
        k = lhs.shape[1]
        r, k0 = init, 0
        while k0 < k:
            k1 = min(k, k0 + (4 - nxt[0]) * LB)
            part = mm1(lhs[:, k0:k1], rhs[k0:k1], pace=k1 - k0 > LB)
            r = part if r is None else r + part
            k0 = k1
        return r

    def at(t, *more):
        best = None
        if t is not None and t >= 0:
            t = min(t, now() - 1)
            for (a, b, r) in tl:
                if a <= t and (best is None or min(b, t) > best[0]):
                    row = int(min((t - a) / (b - a), 0.999) * (r.shape[0] // 8)) * 8
                    best = (min(b, t), r, row)
        return _token(None if best is None else best[1][best[2]:best[2] + 8, 0:LB], *more)

    def strassen(lhs, rhs, order, split_last=False, init=None, m=None):
        m = [None] * 7 if m is None else m
        for p in order:
            flush(now())
            l, r = lhs(p), rhs(p)
            c0 = None if init is None else init[p]
            if split_last and p == order[-1]:
                kk = (-(-r.shape[0] // LB) - 2) * LB
                hm = l.shape[0] // 2
                hd = mm(l[:, :kk], r[:kk], c0) if kk else c0
                tail = jnp.concatenate([mm(l[:hm, kk:], r[kk:]), mm(l[hm:, kk:], r[kk:])], axis=0)
                m[p] = tail if hd is None else hd + tail
            else:
                m[p] = mm(l, r, c0)
        return m

    def wcol(hh, p):
        return p * D + (1 - hh if p == 1 else hh) * HD

    def wrows(hh, g, z=None):
        p, d = divmod(2 * g, DH)
        t = [jnp.concatenate([wt_s[c, pl.ds(wcol(hh, p) + d + e, HH, stride=DH), :]
                              for e in range(2)], axis=0) for c in range(2)]
        return _unword(jnp.concatenate([tie(t[0], z), tie(t[1][:, 0:HD - LB], z)], axis=1))

    wt_done = set()

    def prep_wqkv(part, ga, gb, paced):
        def need(hh, p, z):
            lo = wcol(hh, p)
            for ct in range(lo // LB, -(-(lo + HD) // LB)):
                if ct in wt_done:
                    continue
                wt_done.add(ct)
                cols = slice(ct * LB, min((ct + 1) * LB, 3 * D))
                wd = _word(wqkv_v[0:HD, cols], wqkv_v[HD:D, cols])
                wd = jnp.concatenate([tie(wd[r:r + 8], z if r % LB == 0 else None) for r in range(0, HD, 8)], axis=0)
                wT = wd.T
                wt_s[0, cols, :] = wT[:, 0:LB]
                wt_s[1, cols, 0:HD - LB] = wT[:, LB:HD]

        def put(p, g, v):
            lw_s[p * (HA // 2) + g * 8:p * (HA // 2) + g * 8 + 8, :] = _pk(v)

        def half(hh, g0, g1, t0=None, dur=None):
            pr, ps = ((2, 4), (3, 1))[hh]
            for g in range(g0, g1):
                t = None if t0 is None else t0 + (g - g0) * dur // (g1 - g0)
                need(hh, 2 * g // DH, at(None if t is None else t - P["W2X"]))
                a1, a2 = wrows(hh, g, at(t))
                put(pr, g, a2 if hh else a1)
                put(ps, g, a1 + a2)
            if g1 == gb:
                ready.update({("lw", part, pr), ("lw", part, ps)})

        def rest(g0, g1, t0, dur):
            assert ("lw", part, 1) in ready
            for g in range(g0, g1):
                z = at(t0 + (g - g0) * dur // (g1 - g0))
                ops = _lhs_ops(*wrows(0, g, z), *wrows(1, g, z))
                for p in (0, 5, 6):
                    put(p, g, ops[p])
            if g1 == gb:
                ready.update({("lw", part, 0), ("lw", part, 5), ("lw", part, 6)})
        t2, d2, t3, d3 = paced
        half(0, ga, gb)
        n = (gb - ga) // 14
        add_tasks([(now() + t2 + (k + 1) * d2 // n, half,
                    (1, ga + 14 * k, ga + 14 * k + 14, now() + t2 + k * d2 // n, d2 // n)) for k in range(n)])
        n = (gb - ga) // 7
        add_tasks([(now() + t3 + (k + 1) * d3 // n, rest,
                    (ga + 7 * k, ga + 7 * k + 7, now() + t3 + k * d3 // n, d3 // n)) for k in range(n)])

    def prep_wo_a(t0, dur):
        for g in range(HD // 16):
            w = _word(wo_v[g * 16:g * 16 + 16, :], wo_v[HD + g * 16:HD + g * 16 + 16, :])
            z = at(t0 + g * dur // (HD // 16))
            for c in range(4):
                cw = min(LB, D - c * LB)
                wo_s[c, g * 16:g * 16 + 16, 0:cw] = tie(w[:, c * LB:c * LB + cw], z)
        ready.add("wo")

    def prep_wo_b(h, t_dl):
        assert "wo" in ready
        outs = []
        for c in range(4):
            cw = min(LB, D - c * LB)
            rows = [wo_s[c, pl.ds(d, HH, stride=DH), :][:, 0:cw] for d in range(h * DH // 2, (h + 1) * DH // 2)]
            rows.append(jnp.zeros((LB - QD, cw), i32))
            wT = jnp.concatenate(rows, axis=0).T
            wq_s[c * LB:c * LB + cw, _blk(h)] = wT
            outs += [wT[r:r + 8] for r in range(0, cw, 8)]
        ready.add(("wq", h))
        dls.append((t_dl, _token(*outs)))

    RG = 16
    NG = D // RG
    stat2 = {}

    def ln(b, t0=None, dur=None):
        def xg(g):
            return x_v[b // 2, g * RG:(g + 1) * RG, _blk(b % 2)].astype(f32)

        def step(v, g, fr, s, q):
            if t0 is None or g % 4:
                return v
            acc = [] if s is None else [s[0:8], s[8:16], q[0:8], q[8:16]]
            return tie(v, at(t0 + fr * dur, *acc))

        x0 = jnp.broadcast_to(xg(0)[0:1], (8, LB))
        s = q = None
        for g in range(NG):
            x0 = step(x0, g, P["LNA"] * g / NG, s, q)
            c = xg(g) - _x2(x0)
            s = c if s is None else s + c
            q = c * c if q is None else q + c * c
        dm = _rowsum8(s) * (1.0 / D)
        mu = _rb(x0 + dm)
        var = _rb(jnp.maximum(_rowsum8(q) * (1.0 / D) - dm * dm, 0.0))
        r1 = 1.0 / _rb(jnp.sqrt(_rb(var + EPS_BF16)))
        s = q = None
        for g in range(NG):
            mu = step(mu, g, P["LNB"] + P["LNBD"] * g / NG, s, q)
            xn = _rb(xg(g) - _x2(mu)) * _x2(r1)
            xnT_s[g * 8:g * 8 + 8, _blk(b)] = _pk(xn)
            s = xn if s is None else s + xn
            q = xn * xn if q is None else q + xn * xn
        mu2 = _rowsum8(s) * (1.0 / D)
        var2 = jnp.maximum(_rowsum8(q) * (1.0 / D) - mu2 * mu2, 0.0)
        stat2[b] = (mu2, 0.5 * lax.rsqrt(var2 + EPS))

    def hpair(b, t0=None, dur=None):
        ng = HD // RG
        st = [stat2[b], stat2[b + 1]]
        for g in range(ng):
            if b < HB0:
                zz = [at(None if t0 is None else t0 + (4 * g + k) * dur // (4 * ng)) for k in range(4)]
            else:
                zz = [at(t0 + g * dur // ng), None, None, at(t0 + g * dur // ng + P["SGT"])]
            xq = [_upf(tie(xnT_s[r:r + 8, _blk(b + e)], zz[2 * (r >= QD) + e]))
                  for r in (g * 8, QD + g * 8) for e in range(2)]
            ro = (b // 2) * QD + g * 8
            for p, v in _rhs_sums(*xq).items():
                ra_s[ro:ro + 8, _blk(SIDX[p])] = _pk(v)
            if b < HB0:
                hq = [(v - _x2(st[n % 2][0])) * _x2(st[n % 2][1]) for n, v in enumerate(xq)]
                for p, v in enumerate(_lhs_ops(*hq)):
                    lh_s[p * QD + g * 8:p * QD + g * 8 + 8, _blk(b // 2)] = _pk(v)
        ready.add(("xn", b))
        if b >= 6:
            got = ra_s[(b // 2) * QD:(b // 2 + 1) * QD, :]
            dls.append((t0 + dur + P["HL"], _token(*[got[r:r + 8, _blk(c)] for r in range(0, QD, 8) for c in range(5)])))

    def htile(b, r, z=None):
        return (_upf(tie(xnT_s[r:r + 8, _blk(b)], z)) - _x2(stat2[b][0])) * _x2(stat2[b][1])

    def htriple(t, t0, dur):
        ng = HD // RG
        for g in range(ng):
            zz = [at(t0 + (3 * g + k) * dur // (3 * ng)) for k in range(3)]
            a = [[htile(HB0 + 3 * t + k, h * QD + g * 8, zz[k]) for k in range(3)] for h in range(2)]
            for p, v in enumerate(_hk_lhs(a)):
                lk_s[p * QD + g * 8:p * QD + g * 8 + 8, _blk(t)] = _pk(v)
        ready.add(("lh", t))

    def ln_tasks(b, t, lnd, hsd):
        for fn, bb, dur, adv in ((ln, b, lnd, P["LNV"]), (ln, b + 1, lnd, P["LNV"]), (hpair, b, hsd, 1.0)):
            add_tasks([(t + int(dur * adv), fn, (bb, t, dur))])
            t += int(dur * adv)
        return t

    def tsum(kp, i, slot_, n, t0, dur):
        for g in range(LB // 16):
            z, z2 = at(t0 + g * dur // 8), at(t0 + g * dur // 8 + P["SGT"])
            t1, t2 = [w1_v[(2 * kp + e) * LB + g * 16:(2 * kp + e) * LB + g * 16 + 16,
                           2 * i * LB:(2 * i + 2) * LB].astype(f32) for e in range(2)]
            ro = slot_ * RSK + n * (LB // 2) + g * 8
            for p, v in _rhs_sums(tie8(t1[:, :LB], z), t1[:, LB:], t2[:, :LB], tie8(t2[:, LB:], z2)).items():
                rs_s[ro:ro + 8, _blk(SIDX[p])] = _pk(v)
        ready.add(("rs", kp, i))

    def u_rhs(p, i, kps, slot_, n0):
        if p in SIDX:
            assert all(("rs", kp, i) in ready for kp in kps)
            ro = slot_ * RSK + n0 * (LB // 2)
            return _up(rs_s[ro:ro + len(kps) * (LB // 2), _blk(SIDX[p])])
        e = 0 if p == 1 else 1
        return _cat([w1_v[_blk(2 * kp + e), _blk(2 * i + e)] for kp in kps], 0)

    LATE = (NFP - 1, 6)

    def ujob(kp, i, p):
        flush(now())
        assert ("xn", 2 * kp) in ready
        l, r = _up(lh_s[p * QD:(p + 1) * QD, _blk(kp)]), u_rhs(p, i, [kp], kp, i)
        um_s[p * HD:(p + 1) * HD, _blk(i)] = mm1(l, r)

    def u_early(kp, i0, i1, carry, n, t0, dt):
        for k, i in enumerate(range(i0, i1)):
            add_tasks([(t0 + (k + 1) * dt, tsum, (kp, i, kp, i, t0 + k * dt, dt))])
        jobs = (carry + [(kp, i, p) for i in range(i0, i1) for p in (1, 4)]
                + [(kp, i, p) for i in range(i0, i1) for p in SIDX if (i, p) != LATE])
        for job in jobs[:n]:
            ujob(*job)
        return jobs[n:]

    def u_mid():
        jobs = [(i, p) for i in range(2) for p in (4, 1)]
        for i in range(NFP):
            jobs += [(i, p) for p in (2, 3, 0, 5, 6)] + [(i + 2, p) for p in (4, 1) if i + 2 < NFP]
        m = [[None] * 7 for _ in range(NFP)]
        for i, p in jobs:
            flush(now())
            late = (i, p) == LATE
            l = _up(lh_s[p * QD:(p + 1) * QD, (0 if late else LB):])
            r = _cat([u_rhs(p, i, [0], 0, i)] * late + [u_rhs(p, i, [1], 1, i)], 0)
            v = jnp.concatenate([mm1(l[:QD], r), mm1(l[QD:], r)], axis=0) if late else mm1(l, r)
            if not late:
                v = v + um_s[p * HD:(p + 1) * HD, _blk(i)]
            if p in (2, 3):
                v = v + 0.5 * b1_v[2 * i + 3 - p:2 * i + 4 - p, :].astype(f32)
            m[i][p] = v
            if p == 6:
                for n, c in enumerate(_combine(m[i])):
                    u0_s[n // 2 * HD:(n // 2 + 1) * HD, _blk(2 * i + n % 2)] = c

    def nj_of(i):
        return min(3, NFB - 3 * i)

    def hsum(t, i, t0, dur):
        nj = nj_of(i)
        sums = [(p, tm) for p, tm in _hk_terms(nj).items() if len(tm) > 1]
        tied = {(1, 0): 0, (2, 0): 1, (1, 2): 2, (2, 2): 3} if nj == 3 else {(1, 0): 0, (0, 1): 2}
        for g in range(LB // 16):
            b = {}
            for k in range(3):
                r = (HB0 + 3 * t + k) * LB + g * 16
                w = w1_v[r:r + 16, 3 * i * LB:(3 * i + nj) * LB].astype(f32)
                for j in range(nj):
                    z = at(t0 + g * dur // 8 + tied[k, j] * P["SGH"]) if (k, j) in tied else None
                    b[k, j] = tie8(w[:, _blk(j)], z)
            ro = (i % 2) * RHK + t * (LB // 2) + g * 8
            for n, (p, tm) in enumerate(sums):
                v = b[tm[0][:2]]
                for (k, j, sg) in tm[1:]:
                    v = v + b[k, j] if sg > 0 else v - b[k, j]
                rh_s[ro:ro + 8, _blk(n)] = _pk(v)
        ready.add(("rh", t, i))

    def gelu_half(hx, z):
        c = 0.7978845608028654
        return hx + hx * jnp.tanh(tie(hx * (2.0 * c + (8.0 * c * 0.044715) * (hx * hx)), z))

    def u_epilogue(i, m, gs, t0, dur):
        nj = nj_of(i)
        for n, g in enumerate(gs):
            c = _hk_combine({p: v[g * 16:g * 16 + 16] for p, v in m.items()}, nj)
            for j in range(nj):
                f = 3 * i + j
                t = None if t0 is None else t0 + (n * nj + j) * dur // (len(gs) * nj) - P["UG"]
                gl = [gelu_half(c[h][j] + u0_s[h * HD + g * 16:h * HD + g * 16 + 16, _blk(f)], at(t))
                      for h in range(2)]
                if f < 4 * NQ:
                    for h in range(2):
                        g_s[h * HD + g * 16:h * HD + g * 16 + 16, _blk(f)] = gl[h]
                    ready.add(("g", f, g))
                elif j == 0:
                    g0 = gl
                else:
                    for p, v in enumerate(_lhs_ops(g0[0], gl[0], g0[1], gl[1])):
                        lc_s[p * QD + g * 8:p * QD + g * 8 + 8, :] = _pk(v)

    def u_last(i, edur):
        terms = _hk_terms(nj_of(i))
        sums = [p for p, tm in terms.items() if len(tm) > 1]
        m = {}
        order = ((10, 11, 14, 5, 13, 6, 9, 7, 0, 12, 8, 3, 4, 1, 2) if i == 0
                 else (10, 11, 9, 14, 7, 5, 0, 13, 12, 8, 6, 3, 4, 1, 2))
        for p in [p for p in order if p in terms]:
            flush(now())
            assert all(("lh", t) in ready for t in range(NKT))
            if p in sums:
                assert all(("rh", t, i) in ready for t in range(NKT))
                r = _up(rh_s[(i % 2) * RHK:(i % 2 + 1) * RHK, _blk(sums.index(p))])
            else:
                k, j, _ = terms[p][0]
                r = _cat([w1_v[_blk(HB0 + 3 * t + k), _blk(3 * i + j)] for t in range(NKT)], 0)
            m[p] = mm(_up(lk_s[p * QD:(p + 1) * QD, :]), r)
        if edur is None:
            u_epilogue(i, m, list(range(HD // 16)), None, None)
        else:
            t = now() + P["UE0"]
            add_tasks([(t + (g + 1) * edur // 7, u_epilogue, (i, m, [g, g + 7], t + g * edur // 7, edur // 7))
                       for g in range(7)])

    LTOP = [((0, 0), 1, (1, 1)), ((1, 0), 1, (1, 1)), ((0, 0),), ((1, 1),), ((0, 0), 1, (0, 1)),
            ((1, 0), -1, (0, 0)), ((0, 1), -1, (1, 1))]

    def llsum(qd, g, t0, dur):
        def tile(a, x, h, e):
            r = a * HD + h * QD + g * 16
            if qd < NQ:
                assert ("g", 4 * qd + 2 * e + x, g + 7 * h) in ready
                return g_s[r:r + 16, _blk(4 * qd + 2 * e + x)]
            assert ("wq", e) in ready
            return _unword(wq_s[r:r + 16, _blk(e)])[x]
        for p, t in enumerate(LTOP):
            zz = [at(t0 + p * dur // 7), at(t0 + p * dur // 7 + P["SGT"])]
            a = []
            for h in range(2):
                for e in range(2):
                    v = tile(*t[0], h, e)
                    if len(t) > 1:
                        v = v + tile(*t[2], h, e) if t[1] > 0 else v - tile(*t[2], h, e)
                    a.append(tie8(v, zz[h] if h == e else None))
            for q, v in enumerate(_lhs_ops(*a)):
                r = (p * 7 + q) * ED + g * 8
                ll_s[r:r + 8, _blk(qd)] = _pk(v)
        ready.add(("ll", qd, g))

    AORD = (4, 2, 1, 3, 0, 5, 6)

    def stage_a(b, parts="qkv", order=AORD, split_last=False, m=None):
        r0, r1 = {"q": (0, HD), "kv": (HD, HA), "qkv": (0, HA)}[parts]

        def lhs(p):
            assert all(("lw", pt, p) in ready for pt in ("q", "kv") if pt in parts)
            return _up(lw_s[(p * HA + r0) // 2:(p * HA + r1) // 2, :])

        def rhs(p):
            assert ("xn", b) in ready
            if p in SIDX:
                return _up(ra_s[(b // 2) * QD:(b // 2 + 1) * QD, _blk(SIDX[p])])
            return _up(xnT_s[0:QD, _blk(b)] if p == 1 else xnT_s[QD:HD, _blk(b + 1)])
        m = strassen(lhs, rhs, order, split_last, m=m)
        for n, ps in enumerate((range(7), (2, 4), (1, 3), (0, 1, 2, 5))):
            if all(m[p] is not None for p in ps) and any(p in order for p in ps):
                hh, e = divmod(n, 2)
                c = _combine(m, n)
                qk_s[b + e, hh * D + r0:hh * D + min(r1, D), :] = c[0:min(r1, D) - r0]
                if r1 > D:
                    v_s[b + e + 1, hh * HD:(hh + 1) * HD, :] = c[D - r0:]
        if all(v is not None for v in m):
            ready.update({(pt, b + e) for pt in ("q", "kv") if pt in parts for e in range(2)})
        return m

    lane0 = lax.broadcasted_iota(i32, (HH, LB), 1)
    zeros8 = jnp.zeros((HH, LB), f32)

    def mk_shift(z):
        lane = tie(lane0, z)
        masks = {}

        def pick(n, a, b):
            if n not in masks:
                masks[n] = lane < n
            return lax.select(masks[n], a, b)

        def fwd(cur, prev, sh):
            return cur if sh == 0 else pltpu.roll(pick(LB - sh, cur, prev), sh, 1)

        def bwd(cur, nxt_):
            return pltpu.roll(pick(SH, nxt_, cur), LB - SH, 1)
        return fwd, bwd

    def grp_shift(t, bd):
        lag = max(2, -(-P["LAG"] * DH // (G * bd)))
        return mk_shift(at(t, *(hist[-lag] if len(hist) >= lag else [])))

    raw, probs = {}, {}

    def attn_qk(j, hh, t, bd):
        jn = min(j + 1, NB - 1)
        assert ("q", jn) in ready and ("kv", j) in ready
        acc = [None] * WH
        accp = [None] * WH
        for d in range(DH):
            if d % G == 0:
                if d > 0:
                    hist.append(acc + accp)
                fwd, bwd = grp_shift(t + d * bd // DH, bd)
            r = hh * D + d * HH
            q = qk_s[j, r:r + HH, :]
            qp = bwd(q, qk_s[jn, r:r + HH, :])
            rk = (1 - hh) * D + HD + d * HH
            k = qk_s[j, rk:rk + HH, :]
            kp = qk_s[j - 1, rk:rk + HH, :] if j > 0 else zeros8
            for a in range(WH):
                ks = fwd(k, kp, DIL * a)
                t0, t1 = q * ks, qp * ks
                acc[a] = t0 if d == 0 else acc[a] + t0
                accp[a] = t1 if d == 0 else accp[a] + t1
        hist.append(acc + accp)
        raw[j, hh] = (acc, accp)

    def attn_sm(j, hh, t):
        fwd, _ = mk_shift(at(t))
        acc, accp = raw[j, hh]
        prev = raw.pop((j - 1, hh))[1] if j > 0 else [zeros8] * WH
        lg = acc + [fwd(accp[a], prev[a], SH) for a in range(WH)]
        lg = [a * SCALE for a in lg]
        if j == 0:
            lg = [lg[0]] + [jnp.where(lane0 >= DIL * w, lg[w], -1e9) for w in range(1, W)]
        m = lg[0]
        for w in range(1, W):
            m = jnp.maximum(m, lg[w])
        e = [jnp.exp(l - m) for l in lg]
        den = e[0]
        for w in range(1, W):
            den = den + e[w]
        inv = 1.0 / den
        p = [x * inv for x in e]
        for a in range(WH):
            pr_s[j, (hh * W + a) * HH:(hh * W + a + 1) * HH, :] = p[a]
        probs[j, hh] = p[WH:]

    def attn_pp(j, hh, t):
        _, bwd = mk_shift(at(t))
        p = probs.pop((j, hh))
        pn = probs[j + 1, hh] if j + 1 < NB else p
        for a in range(WH):
            pr_s[j, (hh * W + WH + a) * HH:(hh * W + WH + a + 1) * HH, :] = bwd(p[a], pn[a])
        ready.add(("pr", j, hh))

    def attn_pv(j, hh, dst, e, t, bd):
        assert not isinstance(j, int) or ("pr", j, hh) in ready
        assert e == 0 or ("o", dst, hh, e - 1) in ready
        pa = [pr_s[j, (hh * W + a) * HH:(hh * W + a + 1) * HH, :] for a in range(W)]
        p, pp = pa[:WH], pa[WH:]
        outs = []
        for d in range(DH):
            if d % G == 0:
                if d > 0:
                    hist.append([])
                fwd, _ = grp_shift(t + d * bd // DH, bd)
            r = hh * HD + d * HH
            v = v_s[j + 1, r:r + HH, :]
            vp = v_s[j, r:r + HH, :]
            o = op = None
            for a in range(WH):
                vs = fwd(v, vp, DIL * a)
                o = p[a] * vs if a == 0 else o + p[a] * vs
                op = pp[a] * vs if a == 0 else op + pp[a] * vs
            opp = zeros8 if (isinstance(j, int) and j == 0) else op_s[r:r + HH, :]
            op_s[r:r + HH, :] = op
            outs.append(o + fwd(op, opp, SH))
            ol[dst][r:r + HH, _blk(e)] = outs[-1]
        hist.append([])
        ready.add(("o", dst, hh, e))
        dls.append((t + bd + P["PVL"], _token(*outs)))

    ol = [ola_s, olb_s]
    mains = [("qk", j, hh) for j in range(NB) for hh in range(2)]
    mains = (mains[:P["PVPOS"]] + [("pv", j, hh) for j in range(4) for hh in range(2)]
             + mains[P["PVPOS"]:] + [None, None])
    slot_ctr = [0]

    def slot(t, bd):
        n = slot_ctr[0]
        slot_ctr[0] += 1
        it = mains[n]
        if it is None:
            pass
        elif it[0] == "qk":
            attn_qk(it[1], it[2], t, bd)
        else:
            attn_pv(it[1], it[2], 0, it[1], t, bd)
        if n >= 1 and mains[n - 1] is not None and mains[n - 1][0] == "qk":
            attn_sm(mains[n - 1][1], mains[n - 1][2], t + P["LS"])
        if n >= 2 and mains[n - 2] is not None and mains[n - 2][0] == "qk":
            _, j, hh = mains[n - 2]
            if j > 0:
                attn_pp(j - 1, hh, t + P["PP"])
            if j == NB - 1:
                attn_pp(j, hh, t + P["PP"])

    NRG = 8 * (NQ + 1) + 7
    PD = 8 * QD
    BORD = (1, 3, 2, 4, 0, 5, 6)
    LORD = (2, 4, 1, 3, 0, 5, 6)
    LAST_PARTS = [(0, QD, 1, 2), (QD, HD, 0, 2), (0, QD, 0, 1)]

    def rr_prep(p, pa, src, n0, n1, t0, dur, done):
        assert ("rr", p) not in ready
        for n in range(n0, n1):
            z = at(t0 + (n - n0) * dur // (n1 - n0))
            z2 = at(t0 + (n - n0) * dur // (n1 - n0) + P["SGR"])
            qd, g = divmod(n, 8)

            def wrow(i):
                return _rhs_op(p, lambda x, y: w2_v[pa + y, (2 * i + x) * LB + g * 16:(2 * i + x) * LB + g * 16 + 16, :]
                               .astype(f32))

            def orow(h):
                def blk(x, y):
                    assert ("o", src, x, 2 * y + 1) in ready
                    r = x * HD + h * QD + g * 16
                    return ol[src][r:r + 16, y * 2 * LB:(y + 1) * 2 * LB]
                return _rhs_op(p, blk)
            ro = p * RRK + g * 8
            if qd == NQ:
                if p in SIDX:
                    r = wrow(2 * NQ)
                    for e in range(2):
                        rr_s[ro:ro + 8, _blk(7 + e)] = _pk(tie8(r[:, _blk(e)], z))
                continue
            r1, r2 = (wrow(2 * qd), wrow(2 * qd + 1)) if qd < NQ else (orow(0), orow(1))
            ro += min(qd, NQ) * (LB // 2)
            c11, c22 = tie8(r1[:, :LB], z), tie8(r2[:, LB:], z2)
            sm = _rhs_sums(c11, r1[:, LB:], r2[:, :LB], c22)
            if p in SIDX or qd > NQ:
                sm.update({1: c11, 4: c22})
            for q, v in sm.items():
                rr_s[ro:ro + 8, _blk(q)] = _pk(v)
        if done:
            ready.add(("rr", p))

    def rr_tasks(p, pa, src, t0, t1):
        cuts = list(range(0, NRG, 8)) + [NRG]
        acc, tot = 0, sum(P["RW"])
        for k, n in enumerate(P["RO"]):
            ta, tb = t0 + acc * (t1 - t0) // tot, t0 + (acc + P["RW"][n]) * (t1 - t0) // tot
            add_tasks([(tb, rr_prep, (p, pa, src, cuts[n], cuts[n + 1], ta, tb - ta, k == NQ + 1))])
            acc += P["RW"][n]

    def out_copy(pidx, e0, e1, r0, r1):
        off = pidx * (2 * LB) + e0 * LB
        if not isinstance(pidx, int):
            off = pl.multiple_of(off, LB)
        rs = pl.ds(r0, r1 - r0)
        return pltpu.make_async_copy(out_v.at[pidx, rs, pl.ds(e0 * LB, (e1 - e0) * LB)],
                                     out_hbm.at[0, rs, pl.ds(off, (e1 - e0) * LB)], sems.at[0])

    def b_out(pa, n, m, part, t0=None, dur=None):
        a, y = divmod(n, 2)
        r0, r1, e0, e1 = part
        cols = slice(e0 * LB, e1 * LB)
        for r in range(r0, r1, 16):
            c = _combine([None if v is None else v[r:r + 16, cols] for v in m], n)
            rows = slice(a * HD + r, a * HD + r + 16)
            o = c + x_v[pa + y, rows, cols].astype(f32)
            if t0 is not None:
                o = jnp.concatenate([tie(o[:, 0:LB], at(t0 + (r - r0) * dur // (r1 - r0))), o[:, LB:]], axis=1)
            out_v[pa + y, rows, cols] = o.astype(bf16)
        out_copy(pa + y, e0, e1, a * HD + r0, a * HD + r1).start()

    def big_piece(pa, pan, cur, last):
        t0 = now()
        for n in range(7):
            ta, tb = t0 + n * PD + P["RR0"], t0 + n * PD + P["RR1"]
            if n < 6:
                rr_tasks(BORD[n + 1], pa, cur, ta, tb)
            else:
                rr_tasks(BORD[0], pan, 1 - cur, ta, tb - (P["RRM"] if last else 0))
        ready.difference_update({("o", 1 - cur, hh, e) for hh in range(2) for e in range(4)})
        for n in range(8):
            e, hh = divmod(n, 2)
            t = t0 + P["BV0"] + n * P["BVS"]
            add_tasks([(t + P["BVD"], attn_pv, (pan * 2 + e, hh, 1 - cur, e, t, P["BVD"]))])
        m = [None] * 7
        for p in BORD:
            flush(now())
            assert ("rr", p) in ready
            x, y = TOP[p][0]

            def lhs(q):
                return _up(ll_s[(p * 7 + q) * ED:(p * 7 + q + 1) * ED, 0:KL])

            def rhs(q):
                if p in SIDX or q in SIDX:
                    return _up(rr_s[p * RRK:p * RRK + KL // 2, _blk(q)])
                h = 0 if q == 1 else 1
                return _cat([w2_v[pa + y, _blk(2 * (2 * qd + h) + x), _blk(h)] for qd in range(NQ)]
                            + [_up(rr_s[p * RRK + NQ * LB // 2:p * RRK + KL // 2, _blk(q)])], 0)
            rl = (_up(rr_s[p * RRK:p * RRK + LB // 2, 7 * LB:9 * LB]) if p in SIDX
                  else w2_v[pa + y, _blk(4 * NQ + x), :])
            ll = _up(lc_s[p * QD:(p + 1) * QD, :])
            ex = [mm1(ll[:QD], rl), mm1(ll[QD:], rl)]
            e12, e21 = ex[0][:, LB:], ex[1][:, :LB]
            e11 = (ex[0][:, :LB] + e12) - e21
            lf = strassen(lhs, rhs, LORD)
            ready.discard(("rr", p))
            if p in (2, 3):
                for q in (2, 3):
                    lf[q] = lf[q] + b2f_s[pa + 3 - p, 0:1, _blk(3 - q)]
            c12 = (lf[2] + e12) + lf[4]
            c21 = (lf[1] + e21) + lf[3]
            xx = (lf[2] - lf[1]) + lf[0]
            c22 = (xx + ex[1][:, LB:]) + lf[5]
            c11 = ((xx + e11) + (c21 - c12)) + lf[6]
            m[p] = jnp.concatenate([jnp.concatenate([c11, c12], axis=1),
                                    jnp.concatenate([c21, c22], axis=1)], axis=0)
            n = {3: 2, 4: 1, 5: 3, 6: 0}.get(p)
            if n is not None and not (last and n == 0):
                t, epd = now() + P["EP0"], P["EPL"] if (last and n == 3) else P["EPD"]
                add_tasks([(t + epd, b_out, (pa, n, list(m), (0, HD, 0, 2), t, epd))])
        if last:
            flush()
            for part in LAST_PARTS:
                b_out(pa, 0, m, part)

    def c_body(it, carry):
        reset()
        pos[:] = [one_s[...]]
        true.clear()
        ready.update({("rr", BORD[0])} | {("o", 0, hh, e) for hh in range(2) for e in range(4)})
        big_piece(4 * it, 4 * it + 2, 0, False)
        big_piece(4 * it + 2, lax.rem(4 * it + 4, NP), 1, True)
        assert ("rr", BORD[0]) in ready and all(("o", 0, hh, 3) in ready for hh in range(2))
        return carry

    E1, E2 = P["E1"], P["E2"]
    x0 = Group(cp_x(0, 1))
    g1 = Group(cp_w1(0, 2, 0, E1))
    g2 = Group(cp_w1(0, 2, E1, E2) + cp_x(1, 2))
    wq, wkv = [[(wqkv_hbm.at[:, cl], wqkv_v.at[:, cl])] for cl in (pl.ds(0, 4 * LB), pl.ds(4 * LB, 3 * D - 4 * LB))]
    g3 = Group((cp_w1(0, 2, E2, NFP) if E2 < NFP else []) + wq)
    g4 = Group(wkv + cp_x(2, 3))
    g5 = Group(cp_x(3, NP))
    g6 = Group(cp_w1(2, NB) + [(wo_hbm, wo_v), (b1_hbm, b1_v), (b2_hbm, b2_v)] + cp_w2(0, 1))
    g7 = Group(cp_w2(1, NP))
    for c in (x0, g1, g2, g3, g4, g5, g6, g7):
        c.start()

    v_s[0] = jnp.zeros((D, LB), f32)
    for buf in (xnT_s, ra_s, lh_s, lk_s, rh_s, rs_s, rr_s, ola_s, olb_s, ll_s, lc_s, g_s, wq_s):
        buf[0:8, 0:64] = jnp.zeros((8, 64), buf.dtype)

    wait("x0", x0)
    one_s[...] = lax.shift_right_logical(pltpu.bitcast(x_v[0, 0:16, 0:LB], i32), 1) | 1
    pos[:] = [one_s[...]]
    ln(0)
    ln(1)
    hpair(0)
    wait("r1", g1)
    jobs = u_early(0, 0, E1, [], 7 * E1 // 4 * 4, P["T1"], 100)
    wait("r2", g2)
    t, dt = P["L2T"], P["L2D"]
    add_tasks([(t + int((k + 1) * dt * P["LNV"]), ln, (2 + k, t + int(k * dt * P["LNV"]), dt)) for k in range(2)])
    jobs = u_early(0, E1, E2, jobs, P["N2"], P["T2"], 100)
    wait("wq", g3)
    add_tasks([(P["H2T"] + P["H2D"], hpair, (2, P["H2T"], P["H2D"]))])
    u_early(0, E2, NFP, jobs, 7 * NFP, P["T3"], 100)
    prep_wqkv("q", 0, HD // 16, [P[k] for k in ("QA", "QB", "QC", "QE")])
    stage_a(0, "q", split_last=True)
    m = stage_a(2, "q", AORD[:P["NA3"]])
    wait("wkv", g4)
    stage_a(2, "q", AORD[P["NA3"]:], split_last=True, m=m)
    prep_wqkv("kv", HD // 16, HA // 16, [P[k] for k in ("KA", "KB", "KC", "KE")])
    t = ln_tasks(4, now() + P["L4T"], P["LND"], P["HSD"])
    n4 = P["N4"]
    add_tasks([(t + (n + 1) * P["BD"], slot, (t + n * P["BD"], P["BD"])) for n in range(n4)])
    stage_a(0, "kv")
    stage_a(2, "kv", order=(6,) + AORD[:6])

    wait("mid", g5)
    AD = 7 * HA // 2
    t = P["L5T"]
    for b in range(6, NB, 2):
        t = ln_tasks(b, t, P["LND"], P["HSD"])
    for k in range(P["NH5"]):
        add_tasks([(t + P["HTD"], htriple, (k, t, P["HTD"]))])
        t += P["HTD"]
    n5 = P["N5"]
    bd = ((NP - 2) * AD - P["MARG"] - t) // n5
    add_tasks([(t + (n + 1) * bd, slot, (t + n * bd, bd)) for n in range(n5)])
    n5 += n4
    for n, b in enumerate(range(4, NB, 2)):
        stage_a(b, order=(6,) + AORD[:6] if n % 2 else AORD)

    wait("fin", g6)
    UM = (7 * NFP + 1) * HD // 4
    UD = 15 * NKT * HD // 4
    r6 = UM + (NNT - 1) * UD + 11 * NKT * HD // 4
    add_tasks([(i * P["TMD"] + P["TM0"], tsum, (1, i, 1, i, (i - 1) * P["TMD"] + P["TM0"], P["TMD"])) for i in range(NFP)])
    t, dt = P["HT6"], (UM - 100 - P["HT6"]) // max(NKT - P["NH5"], 1)
    add_tasks([(t + (k + 1) * dt, htriple, (P["NH5"] + k, t + k * dt, dt)) for k in range(NKT - P["NH5"])])
    for i in range(NNT):
        t0, t1 = (UM - P["US0"], UM + 1200) if i == 0 else (UM + (i - 1) * UD + (1300 if i == 1 else 400), UM + i * UD + 350)
        dt = (t1 - t0) // NKT
        add_tasks([(t0 + (k + 1) * dt, hsum, (k, i, t0 + k * dt, dt)) for k in range(NKT)])
    left = len(mains) - n5 - 2
    bd = (r6 - P["R6E"] - P["R6S"]) // left
    add_tasks([(P["R6S"] + (n + 1) * bd, slot, (P["R6S"] + n * bd, bd)) for n in range(left)])
    t = P["R6S"] + left * bd
    add_tasks([(t + (n + 1) * 300, slot, (t + n * 300, 300)) for n in range(2)])
    for qd, t0, t1 in ((NQ, P["LLO"], P["LLO"] + P["LLD"]), (0, 2 * UD + P["LL0"], 3 * UD + P["LL0"]), (1, 3 * UD + P["LL0"], 4 * UD + P["LL0"]),
                       (2, 4 * UD + P["LL2"], 4 * UD + P["LL2"] + P["UEL"])):
        dt = (t1 - t0) // 7
        add_tasks([(UM + t0 + (g + 1) * dt, llsum, (qd, g, UM + t0 + g * dt, dt)) for g in range(7)])
    rr_tasks(BORD[0], 0, 0, P["RP0"], P["RP1"])
    add_tasks([(P["PW0"] + P["PWD"], prep_wo_a, (P["PW0"], P["PWD"]))])
    add_tasks([(P["PW0"] + P["PWD"] + 1, prep_wo_b, (h, P["PW1"] + h * P["PWE"])) for h in range(2)])
    for b in range(NB):
        b2f_s[b // 2, 0:1, _blk(b % 2)] = b2_v[b:b + 1, :].astype(f32)
    u_mid()
    for i in range(NNT):
        u_last(i, None if i == NNT - 1 else P["UEL"] if i == NNT - 2 else P["UED"])
    flush()
    assert slot_ctr[0] == len(mains) and all(("ll", qd, g) in ready for qd in range(NQ + 1) for g in range(7))
    assert all(("pr", j, hh) in ready for j in range(NB) for hh in range(2)) and ("rr", BORD[0]) in ready

    wait("w2", g7)
    lax.fori_loop(0, NP // 4, c_body, 0)
    outs = []
    for pa in range(0, NP, 2):
        outs += [out_copy(pa + n % 2, 0, 2, n // 2 * HD, (n // 2 + 1) * HD) for n in (1, 2, 3)]
        outs += [out_copy(pa, e0, e1, r0, r1) for (r0, r1, e0, e1) in (LAST_PARTS if pa % 4 else [(0, HD, 0, 2)])]
    wait("out", *outs)


@jax.jit
def pallas_parallel_sum__sliding_local_dilated__mixer_token_mlp__prompt_kernel(
    A_x: jax.Array,
    A_wqkv: jax.Array,
    A_wo: jax.Array,
    B_x: jax.Array,
    B_w1: jax.Array,
    B_b1: jax.Array,
    B_w2: jax.Array,
    B_b2: jax.Array,
):
    del B_x
    hbm = pl.BlockSpec(memory_space=pltpu.HBM)
    outT = pl.pallas_call(
        _kernel,
        out_shape=jax.ShapeDtypeStruct((1, D, S), bf16),
        in_specs=[hbm] * 7,
        out_specs=hbm,
        scratch_shapes=[
            pltpu.VMEM((NP, D, 2 * LB), bf16),
            pltpu.VMEM((NP, F, 2 * LB), bf16),
            pltpu.VMEM((NP, D, 2 * LB), bf16),
            pltpu.VMEM((NB + 1, D, LB), f32),
            pltpu.VMEM((NB, 2 * W * HH, LB), f32),
            pltpu.VMEM((NP, 32, 2 * LB), f32),
            pltpu.VMEM((D, 3 * D), bf16),
            pltpu.VMEM((D, D), bf16),
            pltpu.VMEM((S, F), bf16),
            pltpu.VMEM((NFB, LB), bf16),
            pltpu.VMEM((NB, LB), bf16),
            pltpu.VMEM((2, 3 * D + 64, LB), i32),
            pltpu.VMEM((7 * HA // 2, HD), u32),
            pltpu.VMEM((4, HD + 32, LB), i32),
            pltpu.VMEM((D, 2 * LB), i32),
            pltpu.VMEM((HD, S), u32),
            pltpu.VMEM((NP * QD, 5 * LB), u32),
            pltpu.VMEM((7 * QD, 2 * LB), u32),
            pltpu.VMEM((15 * QD, NKT * LB), u32),
            pltpu.VMEM((2 * RHK, 9 * LB), u32),
            pltpu.VMEM((D, F), f32),
            pltpu.VMEM((7 * HD, NFP * LB), f32),
            pltpu.VMEM((7 * QD, LB), u32),
            pltpu.VMEM((D, 4 * NQ * LB), f32),
            pltpu.VMEM((NB, 2 * D, LB), f32),
            pltpu.VMEM((D, LB), f32),
            pltpu.VMEM((2 * RSK, 5 * LB), u32),
            pltpu.VMEM((49 * ED, 4 * LB), u32),
            pltpu.VMEM((7 * RRK, 9 * LB), u32),
            pltpu.VMEM((D, 4 * LB), f32),
            pltpu.VMEM((D, 4 * LB), f32),
            pltpu.VMEM((8, LB), i32),
            pltpu.SemaphoreType.DMA((9,)),
        ],
        compiler_params=pltpu.CompilerParams(vmem_limit_bytes=100 * 1024 * 1024,
                                             disable_bounds_checks=True,
                                             disable_semaphore_checks=True),
    )(jnp.swapaxes(A_x, 1, 2), A_wqkv, A_wo, B_w1, B_b1.reshape(NFB, LB), B_w2, B_b2.reshape(NB, LB))
    return jnp.swapaxes(outT, 1, 2)
```
